```python
import jax
import jax.numpy as jnp

def _softmax(x, axis=-1):
    return jax.nn.softmax(x, axis=axis)
def _gelu(x):
    return jax.nn.gelu(x, approximate=True)
def _silu(x):
    return jax.nn.silu(x)
def _sigmoid(x):
    return jax.nn.sigmoid(x)
def _layernorm(x, axis=-1, eps=1e-5):
    m = jnp.mean(x, axis=axis, keepdims=True)
    v = jnp.var(x, axis=axis, keepdims=True)
    return (x - m) / jnp.sqrt(v + eps)
def _scatter_add(tgt, idx, src, axis=0):
    return tgt.at[idx].add(src)
def _segment_sum(src, seg, n):
    return jax.ops.segment_sum(src, seg, n)
class _Rng:
    def __init__(self, key):
        self._k = key
    def _next(self):
        self._k, sub = jax.random.split(self._k)
        return sub
    def normal(self, shape):
        return jax.random.normal(self._next(), shape, dtype=jnp.bfloat16)
    def randint(self, lo, hi, shape):
        return jax.random.randint(self._next(), shape, lo, hi, dtype=jnp.int32)
    def uniform(self, shape, lo=0.0, hi=1.0):
        return jax.random.uniform(self._next(), shape, jnp.bfloat16, lo, hi)
    def permutation(self, n):
        return jax.random.permutation(self._next(), n)


kernel_name = 'sequential_preLN__linear_attn_block__moe_arch_mod__prompt'

def setup_inputs():
    _rng = _Rng(jax.random.key(int.from_bytes(__import__("os").urandom(4), "little")))
    _w = (lambda a: (lambda t: t.astype(jnp.bfloat16) if jnp.issubdtype(t.dtype, jnp.floating) else t)(jnp.asarray(a)))
    def _A_setup():
        B, S, D = 1, 2048, 1024
        return {
            "x": _w((lambda *s: _rng.normal(s) * 0.05)(B, S, D)),
            "wqkv": _w((lambda *s: _rng.normal(s) * 0.05)(D, 3 * D)),
            "wo": _w((lambda *s: _rng.normal(s) * 0.05)(D, D)),
        }
    _A_in = _A_setup()

    def _B_setup():
        B, S, D, F, C = 1, 2048, 1024, 3584, 2
        return {
            "x": _w((lambda *s: _rng.normal(s) * 0.05)(B, S, D)),
            "w_r": _w((lambda *s: _rng.normal(s) * 0.05)(D)),
            "w_gate": _w((lambda *s: _rng.normal(s) * 0.05)(D, F)),
            "w_up": _w((lambda *s: _rng.normal(s) * 0.05)(D, F)),
            "w_down": _w((lambda *s: _rng.normal(s) * 0.05)(F, D)),
        }
    _B_in = _B_setup()

    return {
        "A_x": _A_in["x"],
        "A_wqkv": _A_in["wqkv"],
        "A_wo": _A_in["wo"],
        "B_x": _B_in["x"],
        "B_w_r": _B_in["w_r"],
        "B_w_gate": _B_in["w_gate"],
        "B_w_up": _B_in["w_up"],
        "B_w_down": _B_in["w_down"],
    }

def reference(A_x, A_wqkv, A_wo, B_x, B_w_r, B_w_gate, B_w_up, B_w_down):
    def _A_ref(x, wqkv, wo):
        B, S, D = x.shape
        H = 32; Dh = D // H
        qkv = (lambda x, *d: x.transpose(*d))((x @ wqkv).reshape(B, S, 3, H, Dh), 2, 0, 3, 1, 4)
        q, k, v = qkv[0], qkv[1], qkv[2]
        phi = lambda t: jnp.where(t > 0, t + 1, jnp.exp(t)) + 1e-6
        pq, pk = phi(q), phi(k)
        kv = jnp.einsum("bhsd,bhse->bhde", pk, v)
        z = jnp.einsum("bhsd->bhd", pk)
        num = jnp.einsum("bhqd,bhde->bhqe", pq, kv)
        den = jnp.einsum("bhqd,bhd->bhq", pq, z)[..., None] + 1e-6
        o = num / den
        return (lambda x, *d: x.transpose(*d))(o, 0, 2, 1, 3).reshape(B, S, D) @ wo

    def _B_ref(x, w_r, w_gate, w_up, w_down):
        B, S, D = x.shape
        C = 2
        r = x @ w_r
        idx = jnp.argsort(-r, axis=-1)[:, :C]
        idx_e = jnp.repeat(idx.reshape(B, C, 1), D, axis=2)
        x_sel = jnp.take_along_axis(x, idx_e, axis=1)
        g = _silu(x_sel @ w_gate)
        u = x_sel @ w_up
        y = (g * u) @ w_down
        r_sel = _sigmoid(jnp.take_along_axis(r, idx, axis=1))
        y = y * r_sel.reshape(B, C, 1)
        b_off = (jnp.arange(B) * S).reshape(B, 1)
        flat_idx = (idx + b_off).reshape(B * C)
        zero = (x * 0.0).reshape(B * S, D)
        upd = _scatter_add(zero, flat_idx, y.reshape(B * C, D), axis=0)
        return x + upd.reshape(B, S, D)

    x = A_x
    h = x + _A_ref(_layernorm(x, axis=-1), A_wqkv, A_wo)
    h2 = h + _B_ref(_layernorm(h, axis=-1), B_w_r, B_w_gate, B_w_up, B_w_down)
    return h2
```

```python
import jax
import jax.numpy as jnp
from jax import lax
import jax.experimental.pallas as pl
import jax.experimental.pallas.tpu as pltpu

S = 2048
D = 1024
F = 3584
H = 32
DH = D // H
LANES = 128
NC = D // LANES

T1 = 256
R1 = 256
T2 = 256

F32 = jnp.float32
BF16 = jnp.bfloat16
U32 = jnp.uint32
I32 = jnp.int32

NX = S // T1
SEM_X = 0
SEM_WK = SEM_X + NX
SEM_WQ = SEM_WK + 1
SEM_WV = SEM_WQ + 1
SEM_WO = SEM_WV + 1
SEM_WR = SEM_WO + 1
SEM_WG = SEM_WR + 1
SEM_WU = SEM_WG + 1
SEM_WD = SEM_WU + 1
SEM_OUT = SEM_WD + 1
NOUT = S // T2
SEM_FIX = SEM_OUT + NOUT
NSEM = SEM_FIX + 2

INT_MIN = -(2 ** 31)


def _layernorm(x):
    mu = jnp.sum(x, axis=-1, keepdims=True) * (1.0 / D)
    xc = x - mu
    var = jnp.sum(xc * xc, axis=-1, keepdims=True) * (1.0 / D)
    return xc * lax.rsqrt(var + 1e-5)


def _phi(t):
    return jnp.where(t > 0, t + 1.0, jnp.exp(t)) + 1e-6


def _pack_rows(a, b):
    return (pltpu.bitcast(a, U32) >> 16) | pltpu.bitcast(b, U32)


def _load_packed(ref):
    return jnp.concatenate([pltpu.bitcast(ref[c], BF16) for c in range(NC)], axis=1)


def _kernel(x_hbm, wqkv_hbm, wo_hbm, wr_hbm, wg_hbm, wu_hbm, wd_hbm, out_hbm,
            x_v, wk_v, wq_v, wv_v, wo_v, wr_v, wg_v, wu_v, wd_v,
            ln1_v, pkt_v, zacc_v, wqp_v, mp_v, ln2_v, out_v, sems):

    def x_copy(i):
        rows = pl.ds(i * T1, T1)
        return pltpu.make_async_copy(x_hbm.at[rows, :], x_v.at[rows, :], sems.at[SEM_X + i])

    def out_copy(i):
        rows = pl.ds(i * T2, T2)
        return pltpu.make_async_copy(out_v.at[rows, :], out_hbm.at[rows, :], sems.at[SEM_OUT + i])

    wk_copy = pltpu.make_async_copy(wqkv_hbm.at[:, pl.ds(D, D)], wk_v, sems.at[SEM_WK])
    wq_copy = pltpu.make_async_copy(wqkv_hbm.at[:, pl.ds(0, D)], wq_v, sems.at[SEM_WQ])
    wv_copy = pltpu.make_async_copy(wqkv_hbm.at[:, pl.ds(2 * D, D)], wv_v, sems.at[SEM_WV])
    wo_copy = pltpu.make_async_copy(wo_hbm, wo_v, sems.at[SEM_WO])
    wr_copy = pltpu.make_async_copy(wr_hbm, wr_v, sems.at[SEM_WR])
    wg_copy = pltpu.make_async_copy(wg_hbm, wg_v, sems.at[SEM_WG])
    wu_copy = pltpu.make_async_copy(wu_hbm, wu_v, sems.at[SEM_WU])
    wd_copy = pltpu.make_async_copy(wd_hbm, wd_v.at[:, pl.ds(0, D)], sems.at[SEM_WD])

    x_copy(0).start()
    wk_copy.start()
    for i in range(1, NX):
        x_copy(i).start()
    wq_copy.start()
    wv_copy.start()
    wo_copy.start()
    wr_copy.start()
    wg_copy.start()
    wu_copy.start()
    wd_copy.start()

    zacc_v[...] = jnp.zeros_like(zacc_v)
    wk_copy.wait()

    def p1a(i, carry):
        x_copy(i).wait()
        r0 = pl.multiple_of(i * T1, T1)
        ln = _layernorm(x_v[pl.ds(r0, T1), :].astype(F32)).astype(BF16)
        ln1_v[pl.ds(r0, T1), :] = ln
        k = jnp.dot(ln, wk_v[...], preferred_element_type=F32)
        pkt = _phi(k).T
        pkt_v[:, pl.ds(r0, T1)] = pkt.astype(BF16)
        zs = pkt[:, 0:LANES]
        for j in range(1, T1 // LANES):
            zs = zs + pkt[:, j * LANES:(j + 1) * LANES]
        zacc_v[...] += zs
        return carry

    lax.fori_loop(0, NX, p1a, 0)

    wq_copy.wait()
    wv_copy.wait()
    wo_copy.wait()
    row_h = lax.broadcasted_iota(I32, (LANES, LANES), 0) // DH
    col_h = lax.broadcasted_iota(I32, (LANES, LANES), 1) // DH
    diag = row_h == col_h
    GPB = R1 // LANES

    def p1b(j, carry):
        r0 = pl.multiple_of(j * R1, R1)
        g = jnp.dot(pkt_v[pl.ds(r0, R1), :], ln1_v[...], preferred_element_type=F32).astype(BF16)
        wqt = wq_v[:, pl.ds(r0, R1)].astype(F32).T
        for hp in range(R1 // (2 * DH)):
            w = _pack_rows(wqt[hp * 2 * DH:hp * 2 * DH + DH, :], wqt[hp * 2 * DH + DH:(hp + 1) * 2 * DH, :])
            base = j * (R1 // (2 * DH)) + hp
            for c in range(NC):
                wqp_v[c, pl.ds(base, DH, stride=H // 2), :] = w[:, c * LANES:(c + 1) * LANES]
        for gi in range(GPB):
            c0 = pl.multiple_of(r0 + gi * LANES, LANES)
            kv = jnp.dot(g[gi * LANES:(gi + 1) * LANES, :], wv_v[:, pl.ds(c0, LANES)],
                         preferred_element_type=F32)
            kv = jnp.where(diag, kv, 0.0).astype(BF16)
            m = jnp.dot(kv, wo_v[pl.ds(c0, LANES), :], preferred_element_type=F32)
            m = m.astype(BF16).astype(F32)
            for hp in range(LANES // (2 * DH)):
                w = _pack_rows(m[hp * 2 * DH:hp * 2 * DH + DH, :], m[hp * 2 * DH + DH:(hp + 1) * 2 * DH, :])
                base = (j * GPB + gi) * (LANES // (2 * DH)) + hp
                for c in range(NC):
                    mp_v[c, pl.ds(base, DH, stride=H // 2), :] = w[:, c * LANES:(c + 1) * LANES]
        return carry

    lax.fori_loop(0, D // R1, p1b, 0)

    zp = jnp.concatenate([zacc_v[pl.ds(d, H, stride=DH), :] for d in range(DH)], axis=0)
    zrow = jnp.sum(zp.T, axis=0, keepdims=True)

    wr_copy.wait()
    wr8 = wr_v[...].astype(F32)
    wr_row = jnp.concatenate([wr8[c:c + 1, :] for c in range(NC)], axis=1)

    def p2(i, carry):
        top1, top2 = carry
        r0 = pl.multiple_of(i * T2, T2)
        q = lax.dot_general(ln1_v[pl.ds(r0, T2), :], _load_packed(wqp_v),
                            (((1,), (1,)), ((), ())), preferred_element_type=F32)
        pq = _phi(q)
        t = pq * zrow
        den = t[:, 0:LANES]
        for c in range(1, NC):
            den = den + t[:, c * LANES:(c + 1) * LANES]
        den = den + pltpu.roll(den, DH, 1)
        den = den + pltpu.roll(den, 2 * DH, 1)
        inv = 1.0 / (den + 1e-6)
        pqn = (pq * jnp.concatenate([inv] * NC, axis=1)).astype(BF16)
        attn = jnp.dot(pqn, _load_packed(mp_v), preferred_element_type=F32)
        h = x_v[pl.ds(r0, T2), :].astype(F32) + attn
        ln2 = _layernorm(h)
        ln2_v[pl.ds(r0, T2), :] = ln2.astype(BF16)
        out_v[pl.ds(r0, T2), :] = (h + ln2).astype(BF16)
        out_copy(i).start()
        r = jnp.sum(ln2 * wr_row, axis=-1, keepdims=True)
        r = r.astype(BF16).astype(F32) + 0.0
        b = pltpu.bitcast(r, I32)
        srt = b ^ ((b >> 31) & 0x7FFFFFFF)
        row = r0 + lax.broadcasted_iota(I32, (T2, 1), 0)
        key = (srt & jnp.int32(-65536)) | (0xFFFF - row)
        for gidx in range(T2 // 8):
            kx = key[gidx * 8:(gidx + 1) * 8, :]
            top2 = jnp.maximum(top2, jnp.minimum(top1, kx))
            top1 = jnp.maximum(top1, kx)
        return top1, top2

    init = jnp.full((8, 1), INT_MIN, I32)
    top1, top2 = lax.fori_loop(0, NOUT, p2, (init, init))

    k1 = jnp.max(top1)
    k2 = jnp.max(jnp.where(top1 == k1, top2, top1))
    keys = (k1, k2)
    idx = [0xFFFF - (kk & 0xFFFF) for kk in keys]
    grp = [pl.multiple_of((ii >> 4) << 4, 16) for ii in idx]

    sub16 = lax.broadcasted_iota(I32, (16, 1), 0)
    sub8 = lax.broadcasted_iota(I32, (8, 1), 0)
    xsel = jnp.zeros((8, D), F32)
    rsel = jnp.zeros((8, 1), F32)
    for c in range(2):
        blk = ln2_v[pl.ds(grp[c], 16), :].astype(F32)
        rowv = jnp.sum(jnp.where(sub16 == (idx[c] & 15), blk, 0.0), axis=0, keepdims=True)
        xsel = jnp.where(sub8 == c, rowv, xsel)
        kv_ = jnp.full((8, 1), keys[c], I32) & jnp.int32(-65536)
        bits = kv_ ^ ((kv_ >> 31) & 0x7FFF0000)
        rsel = jnp.where(sub8 == c, pltpu.bitcast(bits, F32), rsel)
    xsel = xsel.astype(BF16)

    wg_copy.wait()
    wu_copy.wait()
    wd_copy.wait()
    gate = jnp.dot(xsel, wg_v[...], preferred_element_type=F32)
    up = jnp.dot(xsel, wu_v[...], preferred_element_type=F32)
    act = (gate * jax.nn.sigmoid(gate) * up).astype(BF16)
    y = jnp.dot(act, wd_v[:, 0:D], preferred_element_type=F32)
    y = y * jax.nn.sigmoid(rsel)

    for i in range(NOUT):
        out_copy(i).wait()

    for c in range(2):
        cur = out_v[pl.ds(grp[c], 16), :].astype(F32)
        upd = jnp.where(sub16 == (idx[c] & 15), y[c:c + 1, :], 0.0)
        out_v[pl.ds(grp[c], 16), :] = (cur + upd).astype(BF16)

    def fix_copy(c):
        rows = pl.ds(grp[c], 16)
        return pltpu.make_async_copy(out_v.at[rows, :], out_hbm.at[rows, :], sems.at[SEM_FIX + c])

    fix_copy(0).start()

    @pl.when(grp[0] != grp[1])
    def _():
        fix_copy(1).start()
        fix_copy(1).wait()

    fix_copy(0).wait()


@jax.jit
def pallas_sequential_preLN__linear_attn_block__moe_arch_mod__prompt_kernel(
    A_x: jax.Array,
    A_wqkv: jax.Array,
    A_wo: jax.Array,
    B_x: jax.Array,
    B_w_r: jax.Array,
    B_w_gate: jax.Array,
    B_w_up: jax.Array,
    B_w_down: jax.Array,
):
    del B_x
    x = A_x.reshape(S, D)
    wr = B_w_r.reshape(NC, LANES)
    any_spec = pl.BlockSpec(memory_space=pl.ANY)
    out = pl.pallas_call(
        _kernel,
        out_shape=jax.ShapeDtypeStruct((S, D), BF16),
        in_specs=[any_spec] * 7,
        out_specs=any_spec,
        scratch_shapes=[
            pltpu.VMEM((S, D), BF16),
            pltpu.VMEM((D, D), BF16),
            pltpu.VMEM((D, D), BF16),
            pltpu.VMEM((D, D), BF16),
            pltpu.VMEM((D, D), BF16),
            pltpu.VMEM((NC, LANES), BF16),
            pltpu.VMEM((D, F), BF16),
            pltpu.VMEM((D, F), BF16),
            pltpu.VMEM((F, D + LANES), BF16),
            pltpu.VMEM((S, D), BF16),
            pltpu.VMEM((D, S), BF16),
            pltpu.VMEM((D, LANES), F32),
            pltpu.VMEM((NC, D // 2, LANES), U32),
            pltpu.VMEM((NC, D // 2, LANES), U32),
            pltpu.VMEM((S, D), BF16),
            pltpu.VMEM((S, D), BF16),
            pltpu.SemaphoreType.DMA((NSEM,)),
        ],
        compiler_params=pltpu.CompilerParams(vmem_limit_bytes=100 * 1024 * 1024),
    )(x, A_wqkv, A_wo, wr, B_w_gate, B_w_up, B_w_down)
    return out.reshape(1, S, D)
```

```python
import jax
import jax.numpy as jnp
from jax import lax
import jax.experimental.pallas as pl
import jax.experimental.pallas.tpu as pltpu

S = 2048
D = 1024
F = 3584
H = 32
DH = D // H
LANES = 128
NC = D // LANES

T = 256
NB = S // T
WKQ = 4
LNR_E = 16
CHAIN_R = True
LAG = 2
LAG_E = 3
TAIL = ((128, 16), (64, 16), (32, 16), (32, 32))
LNR = 8
PSTR = 20

F32 = jnp.float32
BF16 = jnp.bfloat16
U32 = jnp.uint32
I32 = jnp.int32

SEM_X = 0
SEM_WK = SEM_X + NB
SEM_WQ = SEM_WK + WKQ
SEM_WV = SEM_WQ + 1
SEM_WO = SEM_WV + 1
SEM_WR = SEM_WO + 1
SEM_WG = SEM_WR + 1
SEM_WU = SEM_WG + 1
SEM_WD = SEM_WU + 1
SEM_OUT = SEM_WD + 1
SEM_FIX = SEM_OUT + 3
NSEM = SEM_FIX + 2

INT_MIN = -(2 ** 31)


def _layernorm(x):
    mu = jnp.sum(x, axis=-1, keepdims=True) * (1.0 / D)
    xc = x - mu
    var = jnp.sum(xc * xc, axis=-1, keepdims=True) * (1.0 / D)
    return xc * lax.rsqrt(var + 1e-5)


def _phi(t):
    return jnp.where(t > 0, t + 1.0, jnp.exp(t)) + 1e-6


def _pack_rows(a, b):
    return (pltpu.bitcast(a, U32) >> 16) | pltpu.bitcast(b, U32)


def _load_packed(ref):
    cols = []
    for c in range(NC):
        w = jnp.concatenate([ref[c, d * PSTR:d * PSTR + H // 2, :] for d in range(DH)], axis=0)
        cols.append(pltpu.bitcast(w, BF16))
    return jnp.concatenate(cols, axis=1)


def _store_interleaved(ref, val, head0):
    for hp in range(val.shape[0] // (2 * DH)):
        w = _pack_rows(val[hp * 2 * DH:hp * 2 * DH + DH, :], val[hp * 2 * DH + DH:(hp + 1) * 2 * DH, :])
        for c in range(NC):
            ref[c, pl.ds(head0 // 2 + hp, DH, stride=PSTR), :] = w[:, c * LANES:(c + 1) * LANES]


def _rows(r0, n, half=False):
    if half:
        r0, n = r0 // 2, n // 2
    if not isinstance(r0, int):
        r0 = pl.multiple_of(r0, n)
    return pl.ds(r0, n)


def _kernel(x_hbm, wqkv_hbm, wo_hbm, wr_hbm, wg_hbm, wu_hbm, wd_hbm, out_hbm,
            x_v, wk_v, wq_v, wv_v, wo_v, wr_v, wg_v, wu_v, wd_v,
            ln1_v, pkt_v, zacc_v, g_v, wqp_v, mp_v, pqn_v, attn_v, ln2_v, out_v, zero_v, sems):

    def x_copy(i):
        rows = pl.ds(i * T, T)
        return pltpu.make_async_copy(x_hbm.at[rows, :], x_v.at[rows, :], sems.at[SEM_X + i])

    def out_copy(i):
        b0, nb = ((0, NB - 2), (NB - 2, 1), (NB - 1, 1))[i]
        return pltpu.make_async_copy(out_v.at[pl.ds((b0 + 1) * T, nb * T), :], out_hbm.at[pl.ds(b0 * T, nb * T), :],
                                     sems.at[SEM_OUT + i])

    WQ = D // WKQ

    def wk_copy(j):
        return pltpu.make_async_copy(wqkv_hbm.at[:, pl.ds(D + j * WQ, WQ)], wk_v.at[:, pl.ds(j * WQ, WQ)],
                                     sems.at[SEM_WK + j])

    wq_copy = pltpu.make_async_copy(wqkv_hbm.at[:, pl.ds(0, D)], wq_v, sems.at[SEM_WQ])
    wv_copy = pltpu.make_async_copy(wqkv_hbm.at[:, pl.ds(2 * D, D)], wv_v, sems.at[SEM_WV])
    wo_copy = pltpu.make_async_copy(wo_hbm, wo_v, sems.at[SEM_WO])
    wr_copy = pltpu.make_async_copy(wr_hbm, wr_v, sems.at[SEM_WR])
    wg_copy = pltpu.make_async_copy(wg_hbm, wg_v, sems.at[SEM_WG])
    wu_copy = pltpu.make_async_copy(wu_hbm, wu_v, sems.at[SEM_WU])
    wd_copy = pltpu.make_async_copy(wd_hbm, wd_v.at[:, pl.ds(0, D)], sems.at[SEM_WD])

    x_copy(0).start()
    for j in range(WKQ):
        wk_copy(j).start()
    for i in range(1, NB):
        x_copy(i).start()
    wq_copy.start()
    wv_copy.start()
    wo_copy.start()
    wr_copy.start()
    wg_copy.start()
    wu_copy.start()
    wd_copy.start()

    TH = T // 2

    def ln1_block(xr0, lnr, b):
        ln = _layernorm(x_v[_rows(xr0, T), :].astype(F32)).astype(BF16)
        lnr[b * TH:(b + 1) * TH, :] = pltpu.bitcast(ln, U32)

    def ln1_load(lnr, b):
        return pltpu.bitcast(lnr[b * TH:(b + 1) * TH, :], BF16)

    def k_mm(lnr, b, c0, nc):
        return jnp.dot(ln1_load(lnr, b), wk_v[:, c0:c0 + nc], preferred_element_type=F32)

    def k_part(lnr, pkr, b, c0, nc, first=False, k=None):
        if k is None:
            k = k_mm(lnr, b, c0, nc)
        pkt = _phi(k).T
        pkr[c0 // 2:(c0 + nc) // 2, b * T:(b + 1) * T] = pltpu.bitcast(pkt.astype(BF16), U32)
        zs = pkt[:, 0:LANES]
        for j in range(1, T // LANES):
            zs = zs + pkt[:, j * LANES:(j + 1) * LANES]
        if first:
            zacc_v[c0:c0 + nc, :] = zs
        else:
            zacc_v[c0:c0 + nc, :] += zs

    def g_part(lnr, pkr, b, c0=0, nc=D):
        return jnp.dot(pltpu.bitcast(pkr[c0 // 2:(c0 + nc) // 2, b * T:(b + 1) * T], BF16), ln1_load(lnr, b),
                       preferred_element_type=F32)

    attn_v[0:T, :] = jnp.zeros((T, D), F32)
    zero_v[...] = jnp.zeros_like(zero_v)

    def k0(j, k=None):
        k_part(ln1_v, pkt_v, 0, j * WQ, WQ, first=True, k=k)

    def g0(j):
        g_v[j * WQ:(j + 1) * WQ, :] = g_part(ln1_v, pkt_v, 0, j * WQ, WQ)

    x_copy(0).wait()
    ln1_block(0, ln1_v, 0)
    wk_copy(0).wait()
    k00 = k_mm(ln1_v, 0, 0, WQ)
    wk_copy(1).wait()
    k0(0, k00)
    k0(1)
    g0(0)
    wk_copy(2).wait()
    wk_copy(3).wait()
    k0(2)
    k0(3)
    g0(1)
    x_copy(1).wait()
    x_copy(2).wait()
    ln1_block(T, ln1_v, 1)
    g0(2)
    k_part(ln1_v, pkt_v, 1, 0, D)
    ln1_block(2 * T, ln1_v, 2)
    g0(3)

    def p1(i, carry):
        r0 = pl.multiple_of(i * T, T)
        lnr = ln1_v.at[pl.ds(pl.multiple_of(i * TH, TH), 3 * TH), :]
        pkr = pkt_v.at[:, pl.ds(r0, 2 * T)]
        k_part(lnr, pkr, 1, 0, D)
        ln1_block(jnp.minimum(r0 + 2 * T, S - T), lnr, 2)
        g_v[...] += g_part(lnr, pkr, 0)
        return carry

    for i in range(3, NB):
        x_copy(i).wait()
    lax.fori_loop(1, NB - 1, p1, 0)

    wq_copy.wait()
    wv_copy.wait()
    wo_copy.wait()
    wr_copy.wait()
    for c in range(NC):
        _store_interleaved(wqp_v, wq_v[:, c * LANES:(c + 1) * LANES].astype(F32).T, c * (LANES // DH))
    g = (g_v[...] + g_part(ln1_v, pkt_v, NB - 1)).astype(BF16)
    zp = jnp.concatenate([zacc_v[pl.ds(d, H, stride=DH), :] for d in range(DH)], axis=0)
    zrow = jnp.sum(zp.T, axis=0, keepdims=True)
    wr8 = wr_v[...].astype(F32)
    wr_row = jnp.concatenate([wr8[c:c + 1, :] for c in range(NC)], axis=1)

    def q_part(lnr, pqr, b):
        q = lax.dot_general(ln1_load(lnr, b), _load_packed(wqp_v),
                            (((1,), (1,)), ((), ())), preferred_element_type=F32)
        pq = _phi(q)
        t = pq * zrow
        den = t[:, 0:LANES]
        for c in range(1, NC):
            den = den + t[:, c * LANES:(c + 1) * LANES]
        den = den + pltpu.roll(den, DH, 1)
        den = den + pltpu.roll(den, 2 * DH, 1)
        inv = 1.0 / (den + 1e-6)
        pqn = (pq * jnp.concatenate([inv] * NC, axis=1)).astype(BF16)
        pqr[b * TH:(b + 1) * TH, :] = pltpu.bitcast(pqn, U32)

    def o_part(pqr, r0, n=T):
        return jnp.dot(pltpu.bitcast(pqr[r0 // 2:(r0 + n) // 2, :], BF16), _load_packed(mp_v),
                       preferred_element_type=F32)

    zero_u = zero_v[...]

    def ln2_unit(attn, xr0, r0, n, valid, top1, top2, tok):
        h = x_v[_rows(xr0, n), :].astype(F32) + attn
        s0 = h[:, 0:LANES]
        if tok is not None:
            s0 = s0 + jnp.concatenate([tok] * (n // 8), axis=0)
        for c in range(1, NC):
            s0 = s0 + h[:, c * LANES:(c + 1) * LANES]
        mu = jnp.sum(s0, axis=-1, keepdims=True) * (1.0 / D)
        xc = h - mu
        var = jnp.sum(xc * xc, axis=-1, keepdims=True) * (1.0 / D)
        ln2 = xc * lax.rsqrt(var + 1e-5)
        ln2_v[_rows(r0, n), :] = ln2.astype(BF16)
        out_v[_rows(r0, n), :] = (h + ln2).astype(BF16)
        r = jnp.sum(ln2 * wr_row, axis=-1, keepdims=True)
        r = r.astype(BF16).astype(F32) + 0.0
        b = pltpu.bitcast(r, I32)
        srt = b ^ ((b >> 31) & 0x7FFFFFFF)
        row = xr0 + lax.broadcasted_iota(I32, (n, 1), 0)
        key = (srt & jnp.int32(-65536)) | (0xFFFF - row)
        if valid is not None:
            key = jnp.where(valid, key, INT_MIN)
        for gidx in range(n // 8):
            kx = key[gidx * 8:(gidx + 1) * 8, :]
            top2 = jnp.maximum(top2, jnp.minimum(top1, kx))
            top1 = jnp.maximum(top1, kx)
        ntok = pltpu.bitcast(pltpu.bitcast(jnp.broadcast_to((r if CHAIN_R else mu)[n - 8:n, :], (8, LANES)), U32) & zero_u, F32)
        return top1, top2, ntok

    def ln2_part(attn_ref, a0, xr0, r0, valid, top1, top2, n=T, u=LNR, toks=None, lag=LAG):
        toks = [] if toks is None else toks
        for j in range(n // u):
            tok = toks[-lag] if len(toks) >= lag else None
            top1, top2, tok = ln2_unit(attn_ref[a0 + j * u:a0 + (j + 1) * u, :], xr0 + j * u, r0 + j * u,
                                       u, valid, top1, top2, tok)
            toks.append(tok)
        return top1, top2

    q_part(ln1_v, pqn_v, 0)
    row_h = lax.broadcasted_iota(I32, (LANES, LANES), 0) // DH
    col_h = lax.broadcasted_iota(I32, (LANES, LANES), 1) // DH
    diag = row_h == col_h
    for c in range(NC):
        cs = slice(c * LANES, (c + 1) * LANES)
        kv = jnp.dot(g[cs, :], wv_v[:, cs], preferred_element_type=F32)
        kv = jnp.where(diag, kv, 0.0).astype(BF16)
        m = jnp.dot(kv, wo_v[cs, :], preferred_element_type=F32)
        _store_interleaved(mp_v, m.astype(BF16).astype(F32), c * (LANES // DH))


    def p2(i, carry):
        top1, top2 = carry
        r0 = pl.multiple_of(i * T, T)
        hb = pl.multiple_of(i * TH, TH)
        lnr = ln1_v.at[pl.ds(hb, 2 * TH), :]
        pqr = pqn_v.at[pl.ds(hb, 2 * TH), :]
        atr = attn_v.at[pl.ds(r0, 2 * T), :]
        top1, top2 = ln2_part(atr, 0, jnp.maximum(r0 - T, 0), r0, i > 0, top1, top2)
        q_part(lnr, pqr, 1)
        atr[T:2 * T, :] = o_part(pqr, 0)
        return top1, top2

    init = jnp.full((8, 1), INT_MIN, I32)
    top1, top2 = lax.fori_loop(0, NB - 1, p2, (init, init))

    out_copy(0).start()
    toks = []
    top1, top2 = ln2_part(attn_v, S - T, S - 2 * T, S - T, None, top1, top2, u=LNR_E, toks=toks, lag=LAG_E)
    out_copy(1).start()
    r0 = S - T
    for n, u in TAIL:
        top1, top2 = ln2_part(o_part(pqn_v, r0, n), 0, r0, r0 + T, None, top1, top2, n=n, u=u, toks=toks, lag=LAG_E)
        r0 += n
    out_copy(2).start()

    k1 = jnp.max(top1)
    k2 = jnp.max(jnp.where(top1 == k1, top2, top1))
    keys = (k1, k2)
    idx = [0xFFFF - (kk & 0xFFFF) for kk in keys]
    grp = [pl.multiple_of((ii >> 4) << 4, 16) for ii in idx]
    vgrp = [pl.multiple_of(gg + T, 16) for gg in grp]

    sub16 = lax.broadcasted_iota(I32, (16, 1), 0)
    sub8 = lax.broadcasted_iota(I32, (8, 1), 0)
    xsel = jnp.zeros((8, D), F32)
    rsel = jnp.zeros((8, 1), F32)
    for c in range(2):
        blk = ln2_v[pl.ds(vgrp[c], 16), :].astype(F32)
        rowv = jnp.sum(jnp.where(sub16 == (idx[c] & 15), blk, 0.0), axis=0, keepdims=True)
        xsel = jnp.where(sub8 == c, rowv, xsel)
        kv_ = jnp.full((8, 1), keys[c], I32) & jnp.int32(-65536)
        bits = kv_ ^ ((kv_ >> 31) & 0x7FFF0000)
        rsel = jnp.where(sub8 == c, pltpu.bitcast(bits, F32), rsel)
    xsel = xsel.astype(BF16)

    wg_copy.wait()
    wu_copy.wait()
    wd_copy.wait()
    gate = jnp.dot(xsel, wg_v[...], preferred_element_type=F32)
    up = jnp.dot(xsel, wu_v[...], preferred_element_type=F32)
    act = (gate * jax.nn.sigmoid(gate) * up).astype(BF16)
    y = jnp.dot(act, wd_v[:, 0:D], preferred_element_type=F32)
    y = y * jax.nn.sigmoid(rsel)

    for i in range(3):
        out_copy(i).wait()

    for c in range(2):
        cur = out_v[pl.ds(vgrp[c], 16), :].astype(F32)
        upd = jnp.where(sub16 == (idx[c] & 15), y[c:c + 1, :], 0.0)
        out_v[pl.ds(vgrp[c], 16), :] = (cur + upd).astype(BF16)

    def fix_copy(c):
        return pltpu.make_async_copy(out_v.at[pl.ds(vgrp[c], 16), :], out_hbm.at[pl.ds(grp[c], 16), :],
                                     sems.at[SEM_FIX + c])

    fix_copy(0).start()

    @pl.when(grp[0] != grp[1])
    def _():
        fix_copy(1).start()
        fix_copy(1).wait()

    fix_copy(0).wait()


@jax.jit
def pallas_sequential_preLN__linear_attn_block__moe_arch_mod__prompt_kernel(
    A_x: jax.Array,
    A_wqkv: jax.Array,
    A_wo: jax.Array,
    B_x: jax.Array,
    B_w_r: jax.Array,
    B_w_gate: jax.Array,
    B_w_up: jax.Array,
    B_w_down: jax.Array,
):
    del B_x
    x = A_x.reshape(S, D)
    wr = B_w_r.reshape(NC, LANES)
    any_spec = pl.BlockSpec(memory_space=pl.ANY)
    out = pl.pallas_call(
        _kernel,
        out_shape=jax.ShapeDtypeStruct((S, D), BF16),
        in_specs=[any_spec] * 7,
        out_specs=any_spec,
        scratch_shapes=[
            pltpu.VMEM((S, D), BF16),
            pltpu.VMEM((D, D + LANES), BF16),
            pltpu.VMEM((D, D), BF16),
            pltpu.VMEM((D, D), BF16),
            pltpu.VMEM((D, D), BF16),
            pltpu.VMEM((NC, LANES), BF16),
            pltpu.VMEM((D, F), BF16),
            pltpu.VMEM((D, F), BF16),
            pltpu.VMEM((F, D + LANES), BF16),
            pltpu.VMEM(((S + T) // 2, D), U32),
            pltpu.VMEM((D // 2, S), U32),
            pltpu.VMEM((D, LANES), F32),
            pltpu.VMEM((D, D), F32),
            pltpu.VMEM((NC, DH * PSTR, LANES), U32),
            pltpu.VMEM((NC, DH * PSTR, LANES), U32),
            pltpu.VMEM((S // 2, D), U32),
            pltpu.VMEM((S, D), F32),
            pltpu.VMEM((S + T, D), BF16),
            pltpu.VMEM((S + T, D), BF16),
            pltpu.VMEM((8, LANES), U32),
            pltpu.SemaphoreType.DMA((NSEM,)),
        ],
        compiler_params=pltpu.CompilerParams(vmem_limit_bytes=110 * 1024 * 1024),
    )(x, A_wqkv, A_wo, wr, B_w_gate, B_w_up, B_w_down)
    return out.reshape(1, S, D)
```

```python
import jax
import jax.numpy as jnp
from jax import lax
import jax.experimental.pallas as pl
import jax.experimental.pallas.tpu as pltpu

S = 2048
D = 1024
F = 3584
H = 32
DH = D // H
LANES = 128
NC = D // LANES

TB = 512
NBLK = S // TB
TX = 256
NX = S // TX
WKQ = 4
WQ = D // WKQ
OCH = (64, 64, 64, 64, 64, 64, 64, 64)
DEF = OCH[-1]
LNU = 8
LAG = 5
L1U = 8
L1LAG = 2
L1LAG0 = 4
ZP = 36
PSTR = 20

F32 = jnp.float32
BF16 = jnp.bfloat16
U32 = jnp.uint32
I32 = jnp.int32

SEM_X = 0
SEM_WK = SEM_X + NX
SEM_WQ = SEM_WK + WKQ
SEM_WV = SEM_WQ + 1
SEM_WO = SEM_WV + 1
SEM_WR = SEM_WO + 1
SEM_WG = SEM_WR + 1
SEM_WU = SEM_WG + 1
SEM_WD = SEM_WU + 1
SEM_OUT = SEM_WD + 1
SEM_FIX = SEM_OUT + NBLK + 1
NSEM = SEM_FIX + 2

INT_MIN = -(2 ** 31)


def _layernorm(x, tok=None):
    s0 = x[:, 0:LANES]
    if tok is not None:
        s0 = s0 + jnp.concatenate([tok] * (x.shape[0] // 8), axis=0)
    for c in range(1, NC):
        s0 = s0 + x[:, c * LANES:(c + 1) * LANES]
    mu = jnp.sum(s0, axis=-1, keepdims=True) * (1.0 / D)
    xc = x - mu
    var = jnp.sum(xc * xc, axis=-1, keepdims=True) * (1.0 / D)
    return xc * lax.rsqrt(var + 1e-5)


def _phi(t):
    return jnp.where(t > 0, t + 1.0, jnp.exp(t)) + 1e-6


def _pack_rows(a, b):
    return (pltpu.bitcast(a, U32) >> 16) | pltpu.bitcast(b, U32)


def _load_packed(ref):
    cols = []
    for c in range(NC):
        w = jnp.concatenate([ref[c, d * PSTR:d * PSTR + H // 2, :] for d in range(DH)], axis=0)
        cols.append(pltpu.bitcast(w, BF16))
    return jnp.concatenate(cols, axis=1)


def _store_interleaved(ref, val, head0):
    acc = None
    for hp in range(val.shape[0] // (2 * DH)):
        w = _pack_rows(val[hp * 2 * DH:hp * 2 * DH + DH, :], val[hp * 2 * DH + DH:(hp + 1) * 2 * DH, :])
        for c in range(NC):
            ref[c, pl.ds(head0 // 2 + hp, DH, stride=PSTR), :] = w[:, c * LANES:(c + 1) * LANES]
            for g in range(DH // 8):
                piece = w[g * 8:(g + 1) * 8, c * LANES:(c + 1) * LANES]
                acc = piece if acc is None else acc | piece
    return acc


def _kernel(x_hbm, wqkv_hbm, wo_hbm, wr_hbm, wg_hbm, wu_hbm, wd_hbm, out_hbm,
            x_v, wk_v, wq_v, wv_v, wo_v, wr_v, wg_v, wu_v, wd_v,
            ln1_v, pkt_v, zacc_v, g_v, wqp_v, mp_v, pqn_v, attn_v, ln2_v, out_v, zero_v, sems):

    def x_copy(i):
        rows = pl.ds(i * TX, TX)
        return pltpu.make_async_copy(x_hbm.at[rows, :], x_v.at[pl.ds(DEF + i * TX, TX), :], sems.at[SEM_X + i])

    def out_copy(i):
        if isinstance(i, int) and i >= NBLK - 1:
            r0, n = ((S - TB, TB - DEF), (S - DEF, DEF))[i - (NBLK - 1)]
        else:
            r0, n = pl.multiple_of(i * TB, TB), TB
        return pltpu.make_async_copy(out_v.at[pl.ds(DEF + r0, n), :], out_hbm.at[pl.ds(r0, n), :],
                                     sems.at[SEM_OUT + i])

    def wk_copy(j):
        return pltpu.make_async_copy(wqkv_hbm.at[:, pl.ds(D + j * WQ, WQ)], wk_v.at[:, pl.ds(j * WQ, WQ)],
                                     sems.at[SEM_WK + j])

    wq_copy = pltpu.make_async_copy(wqkv_hbm.at[:, pl.ds(0, D)], wq_v, sems.at[SEM_WQ])
    wv_copy = pltpu.make_async_copy(wqkv_hbm.at[:, pl.ds(2 * D, D)], wv_v, sems.at[SEM_WV])
    wo_copy = pltpu.make_async_copy(wo_hbm, wo_v, sems.at[SEM_WO])
    wr_copy = pltpu.make_async_copy(wr_hbm, wr_v, sems.at[SEM_WR])
    wg_copy = pltpu.make_async_copy(wg_hbm, wg_v, sems.at[SEM_WG])
    wu_copy = pltpu.make_async_copy(wu_hbm, wu_v, sems.at[SEM_WU])
    wd_copy = pltpu.make_async_copy(wd_hbm, wd_v.at[:, pl.ds(0, D)], sems.at[SEM_WD])

    x_copy(0).start()
    for j in range(WKQ):
        wk_copy(j).start()
    for i in range(1, NX):
        x_copy(i).start()
    wq_copy.start()
    wv_copy.start()
    wo_copy.start()
    wr_copy.start()
    wg_copy.start()
    wu_copy.start()
    wd_copy.start()

    def ln1_rows(xr, xr0, lnr, r0, n):
        ln = _layernorm(xr[xr0:xr0 + n, :].astype(F32)).astype(BF16)
        lnr[r0 // 2:(r0 + n) // 2, :] = pltpu.bitcast(ln, U32)

    def ln1_rows_paced(xr, xr0, lnr, r0, n, L1LAG=L1LAG):
        zero_u = zero_v[...]
        toks = []
        lns = []
        for j in range(n // L1U):
            x = xr[xr0 + j * L1U:xr0 + (j + 1) * L1U, :].astype(F32)
            tok = toks[-L1LAG] if len(toks) >= L1LAG else None
            ln = _layernorm(x, tok)
            toks.append(pltpu.bitcast(pltpu.bitcast(ln[L1U - 8:L1U, 0:LANES], U32) & zero_u, F32))
            lns.append(ln)
            if (j + 1) * L1U % 16 == 0:
                grp = jnp.concatenate(lns, axis=0).astype(BF16)
                e = r0 + (j + 1) * L1U
                lnr[(e - grp.shape[0]) // 2:e // 2, :] = pltpu.bitcast(grp, U32)
                lns = []

    def ln1_load(lnr, r0, n):
        return pltpu.bitcast(lnr[r0 // 2:(r0 + n) // 2, :], BF16)

    def k_mm(lnr, r0, n, c0, nc):
        return jnp.dot(ln1_load(lnr, r0, n), wk_v[:, c0:c0 + nc], preferred_element_type=F32)

    def k_post(k, p0, c0, first=False):
        n, nc = k.shape
        pkt = _phi(k).T
        pkt_v[c0 // 2:(c0 + nc) // 2, p0:p0 + n] = pltpu.bitcast(pkt.astype(BF16), U32)
        zs = pkt[:, 0:LANES]
        for j in range(1, n // LANES):
            zs = zs + pkt[:, j * LANES:(j + 1) * LANES]
        for hh in range(nc // DH):
            z0 = (c0 // DH + hh) * ZP
            if first:
                zacc_v[z0:z0 + DH, :] = zs[hh * DH:(hh + 1) * DH, :]
            else:
                zacc_v[z0:z0 + DH, :] += zs[hh * DH:(hh + 1) * DH, :]

    def g_acc(lnr, r0, n, c0, nc, first=False):
        g = jnp.dot(pltpu.bitcast(pkt_v[c0 // 2:(c0 + nc) // 2, r0:r0 + n], BF16), ln1_load(lnr, r0, n),
                    preferred_element_type=F32)
        if first:
            g_v[c0:c0 + nc, :] = g
        else:
            g_v[c0:c0 + nc, :] += g

    attn_v[...] = jnp.zeros_like(attn_v)
    x_v[0:DEF, :] = jnp.zeros((DEF, D), BF16)
    zero_v[...] = jnp.zeros_like(zero_v)

    def k0(j):
        k_post(k_mm(ln1_v, 0, TX, j * WQ, WQ), 0, j * WQ, first=True)

    def g0(j):
        g_acc(ln1_v, 0, TX, j * WQ, WQ, first=True)

    x_copy(0).wait()
    ln1_rows(x_v, DEF, ln1_v, 0, TX)
    wk_copy(0).wait()
    k00 = k_mm(ln1_v, 0, TX, 0, WQ)
    wk_copy(1).wait()
    k_post(k00, 0, 0, first=True)
    k0(1)
    g0(0)
    wk_copy(2).wait()
    wk_copy(3).wait()
    k0(2)
    k0(3)
    g0(1)
    for i in range(1, 4):
        x_copy(i).wait()
    ln1_rows(x_v, DEF + TX, ln1_v, TX, TX)
    g0(2)
    HD = D // 2
    k_post(k_mm(ln1_v, TX, TX, 0, HD), TX, 0)
    k_post(k_mm(ln1_v, TX, TX, HD, HD), TX, HD)
    ln1_rows_paced(x_v, DEF + TB, ln1_v, TB, TB, L1LAG0)
    g0(3)
    g_acc(ln1_v, TX, TX, 0, HD)
    g_acc(ln1_v, TX, TX, HD, HD)

    def p1(i, carry):
        lnr = ln1_v.at[pl.ds(pl.multiple_of(i * (TB // 2), TB // 2), TB), :]
        xr = x_v.at[pl.ds(pl.multiple_of(jnp.minimum(i + 1, NBLK - 1) * TB, TB), TB + DEF), :]
        k_post(k_mm(lnr, 0, TB, 0, HD), 0, 0)
        k_post(k_mm(lnr, 0, TB, HD, HD), 0, HD)
        ln1_rows_paced(xr, DEF, lnr, TB, TB)
        g_acc(lnr, 0, TB, 0, HD)
        g_acc(lnr, 0, TB, HD, HD)
        return carry

    for i in range(4, NX):
        x_copy(i).wait()
    lax.fori_loop(1, NBLK, p1, 0)

    wq_copy.wait()
    wv_copy.wait()
    wo_copy.wait()
    wr_copy.wait()
    zero_u = zero_v[...]
    wtok = []
    for c in range(NC):
        wtok.append(zero_u & _store_interleaved(wqp_v, wq_v[:, c * LANES:(c + 1) * LANES].astype(F32).T,
                                                c * (LANES // DH)))
    zp = jnp.concatenate([zacc_v[pl.ds(d, H, stride=ZP), :] for d in range(DH)], axis=0)
    zrow = jnp.sum(zp.T, axis=0, keepdims=True)
    wr8 = wr_v[...].astype(F32)
    wr_row = jnp.concatenate([wr8[c:c + 1, :] for c in range(NC)], axis=1)

    row_h = lax.broadcasted_iota(I32, (LANES, LANES), 0) // DH
    col_h = lax.broadcasted_iota(I32, (LANES, LANES), 1) // DH
    diag = row_h == col_h
    for c in range(NC):
        cs = slice(c * LANES, (c + 1) * LANES)
        gb = g_v[cs, :]
        if c >= 1:
            tk = wtok[c - 1] if c < NC - 1 else wtok[c - 1] | wtok[c]
            gb = jnp.concatenate([jnp.concatenate([gb[0:8, 0:LANES] + pltpu.bitcast(tk, F32), gb[0:8, LANES:]], axis=1),
                                  gb[8:, :]], axis=0)
        kv = jnp.dot(gb.astype(BF16), wv_v[:, cs], preferred_element_type=F32)
        kv = jnp.where(diag, kv, 0.0).astype(BF16)
        m = jnp.dot(kv, wo_v[cs, :], preferred_element_type=F32)
        _store_interleaved(mp_v, m.astype(BF16).astype(F32), c * (LANES // DH))

    def q_part(lnr, r0, n):
        q = lax.dot_general(ln1_load(lnr, r0, n), _load_packed(wqp_v),
                            (((1,), (1,)), ((), ())), preferred_element_type=F32)
        pq = _phi(q)
        t = pq * zrow
        den = t[:, 0:LANES]
        for c in range(1, NC):
            den = den + t[:, c * LANES:(c + 1) * LANES]
        den = den + pltpu.roll(den, DH, 1)
        den = den + pltpu.roll(den, 2 * DH, 1)
        inv = 1.0 / (den + 1e-6)
        pqn = (pq * jnp.concatenate([inv] * NC, axis=1)).astype(BF16)
        pqn_v[r0 // 2:(r0 + n) // 2, :] = pltpu.bitcast(pqn, U32)

    def o_part(r0, n):
        return jnp.dot(pltpu.bitcast(pqn_v[r0 // 2:(r0 + n) // 2, :], BF16), _load_packed(mp_v),
                       preferred_element_type=F32)

    def ln2_unit(attn, xr, l2r, outr, r0, row0, valid, top1, top2, tok):
        n = attn.shape[0]
        h = xr[r0:r0 + n, :].astype(F32) + attn
        ln2 = _layernorm(h, tok)
        l2r[r0:r0 + n, :] = ln2.astype(BF16)
        outr[r0:r0 + n, :] = (h + ln2).astype(BF16)
        r = jnp.sum(ln2 * wr_row, axis=-1, keepdims=True)
        r = r.astype(BF16).astype(F32) + 0.0
        b = pltpu.bitcast(r, I32)
        srt = b ^ ((b >> 31) & 0x7FFFFFFF)
        row = (row0 + r0) + lax.broadcasted_iota(I32, (n, 1), 0)
        key = (srt & jnp.int32(-65536)) | (0xFFFF - row)
        if valid is not None:
            key = jnp.where(valid, key, INT_MIN)
        for gidx in range(n // 8):
            kx = key[gidx * 8:(gidx + 1) * 8, :]
            top2 = jnp.maximum(top2, jnp.minimum(top1, kx))
            top1 = jnp.maximum(top1, kx)
        ntok = pltpu.bitcast(pltpu.bitcast(jnp.broadcast_to(r[n - 8:n, :], (8, LANES)), U32) & zero_u, F32)
        return top1, top2, ntok

    def ln2_part(attn, xr, l2r, outr, r0, row0, valid, top1, top2, toks):
        n = attn.shape[0]
        u = min(LNU, n)
        for j in range(n // u):
            tok = toks[-LAG] if len(toks) >= LAG else None
            top1, top2, tok = ln2_unit(attn[j * u:(j + 1) * u, :], xr, l2r, outr, r0 + j * u, row0, valid,
                                       top1, top2, tok)
            toks.append(tok)
        return top1, top2

    def p2(i, carry):
        top1, top2 = carry
        b0 = pl.multiple_of(i * TB, TB)
        lnr = ln1_v.at[pl.ds(pl.multiple_of(i * (TB // 2), TB // 2), TB // 2), :]
        xr = x_v.at[pl.ds(b0, TB + DEF), :]
        l2r = ln2_v.at[pl.ds(b0, TB + DEF), :]
        outr = out_v.at[pl.ds(b0, TB + DEF), :]
        row0 = b0 - DEF
        toks = []
        top1, top2 = ln2_part(attn_v[...], xr, l2r, outr, 0, row0, i > 0, top1, top2, toks)

        @pl.when(i > 0)
        def _():
            out_copy(i - 1).start()

        q_part(lnr, 0, TX)
        q_part(lnr, TX, TX)
        r0 = 0
        for n in OCH[:-1]:
            top1, top2 = ln2_part(o_part(r0, n), xr, l2r, outr, DEF + r0, row0, None, top1, top2, toks)
            r0 += n
        attn_v[...] = o_part(r0, DEF)
        return top1, top2

    init = jnp.full((8, 1), INT_MIN, I32)
    top1, top2 = lax.fori_loop(0, NBLK, p2, (init, init))

    out_copy(NBLK - 1).start()
    top1, top2, _ = ln2_unit(attn_v[...], x_v, ln2_v, out_v, S, -DEF, None, top1, top2, None)
    out_copy(NBLK).start()

    k1 = jnp.max(top1)
    k2 = jnp.max(jnp.where(top1 == k1, top2, top1))
    keys = (k1, k2)
    idx = [0xFFFF - (kk & 0xFFFF) for kk in keys]
    grp = [pl.multiple_of((ii >> 4) << 4, 16) for ii in idx]
    vgrp = [pl.multiple_of(gg + DEF, 16) for gg in grp]

    sub16 = lax.broadcasted_iota(I32, (16, 1), 0)
    sub8 = lax.broadcasted_iota(I32, (8, 1), 0)
    xsel = jnp.zeros((8, D), F32)
    rsel = jnp.zeros((8, 1), F32)
    for c in range(2):
        blk = ln2_v[pl.ds(vgrp[c], 16), :].astype(F32)
        rowv = jnp.sum(jnp.where(sub16 == (idx[c] & 15), blk, 0.0), axis=0, keepdims=True)
        xsel = jnp.where(sub8 == c, rowv, xsel)
        kv_ = jnp.full((8, 1), keys[c], I32) & jnp.int32(-65536)
        bits = kv_ ^ ((kv_ >> 31) & 0x7FFF0000)
        rsel = jnp.where(sub8 == c, pltpu.bitcast(bits, F32), rsel)
    xsel = xsel.astype(BF16)

    wg_copy.wait()
    wu_copy.wait()
    wd_copy.wait()
    gate = jnp.dot(xsel, wg_v[...], preferred_element_type=F32)
    up = jnp.dot(xsel, wu_v[...], preferred_element_type=F32)
    act = (gate * jax.nn.sigmoid(gate) * up).astype(BF16)
    y = jnp.dot(act, wd_v[:, 0:D], preferred_element_type=F32)
    y = y * jax.nn.sigmoid(rsel)

    for i in range(NBLK + 1):
        out_copy(i).wait()

    for c in range(2):
        cur = out_v[pl.ds(vgrp[c], 16), :].astype(F32)
        upd = jnp.where(sub16 == (idx[c] & 15), y[c:c + 1, :], 0.0)
        out_v[pl.ds(vgrp[c], 16), :] = (cur + upd).astype(BF16)

    def fix_copy(c):
        return pltpu.make_async_copy(out_v.at[pl.ds(vgrp[c], 16), :], out_hbm.at[pl.ds(grp[c], 16), :],
                                     sems.at[SEM_FIX + c])

    fix_copy(0).start()

    @pl.when(grp[0] != grp[1])
    def _():
        fix_copy(1).start()
        fix_copy(1).wait()

    fix_copy(0).wait()


@jax.jit
def pallas_sequential_preLN__linear_attn_block__moe_arch_mod__prompt_kernel(
    A_x: jax.Array,
    A_wqkv: jax.Array,
    A_wo: jax.Array,
    B_x: jax.Array,
    B_w_r: jax.Array,
    B_w_gate: jax.Array,
    B_w_up: jax.Array,
    B_w_down: jax.Array,
):
    del B_x
    x = A_x.reshape(S, D)
    wr = B_w_r.reshape(NC, LANES)
    any_spec = pl.BlockSpec(memory_space=pl.ANY)
    out = pl.pallas_call(
        _kernel,
        out_shape=jax.ShapeDtypeStruct((S, D), BF16),
        in_specs=[any_spec] * 7,
        out_specs=any_spec,
        scratch_shapes=[
            pltpu.VMEM((S + DEF, D), BF16),
            pltpu.VMEM((D, D + LANES), BF16),
            pltpu.VMEM((D, D), BF16),
            pltpu.VMEM((D, D), BF16),
            pltpu.VMEM((D, D), BF16),
            pltpu.VMEM((NC, LANES), BF16),
            pltpu.VMEM((D, F), BF16),
            pltpu.VMEM((D, F), BF16),
            pltpu.VMEM((F, D + LANES), BF16),
            pltpu.VMEM(((S + TB) // 2, D), U32),
            pltpu.VMEM((D // 2, TB), U32),
            pltpu.VMEM((H * ZP, LANES), F32),
            pltpu.VMEM((D, D), F32),
            pltpu.VMEM((NC, DH * PSTR, LANES), U32),
            pltpu.VMEM((NC, DH * PSTR, LANES), U32),
            pltpu.VMEM((TB // 2, D), U32),
            pltpu.VMEM((DEF, D), F32),
            pltpu.VMEM((S + DEF, D), BF16),
            pltpu.VMEM((S + DEF, D), BF16),
            pltpu.VMEM((8, LANES), U32),
            pltpu.SemaphoreType.DMA((NSEM,)),
        ],
        compiler_params=pltpu.CompilerParams(vmem_limit_bytes=110 * 1024 * 1024),
    )(x, A_wqkv, A_wo, wr, B_w_gate, B_w_up, B_w_down)
    return out.reshape(1, S, D)
```

```python
import jax
import jax.numpy as jnp
from jax import lax
import jax.experimental.pallas as pl
import jax.experimental.pallas.tpu as pltpu

S = 2048
D = 1024
F = 3584
H = 32
DH = D // H
LANES = 128
NC = D // LANES

TB = 512
NBLK = S // TB
TX = 256
OCH = (64, 64, 64, 64, 64, 64, 64, 64)
DEF = OCH[-1]
LNU = 8
LAG = 5
L1U = 8
L1LAG = 2
L1LAG0 = 4
ZP = 36
KVLAG = 1
KVGATE = ((), (), (0,), (1,), (2,), (3,), (4,), (5,))
MGATE = ((), (), (), (), (), (), (6,), (7,))
PSTR = 20

F32 = jnp.float32
BF16 = jnp.bfloat16
U32 = jnp.uint32
I32 = jnp.int32

XP = ((0, 128), (128, 128), (256, 768), (1024, 1024))
WKP = ((0, 128), (128, 128), (256, 256), (512, 512))

SEM_X = 0
SEM_WK = SEM_X + len(XP)
SEM_W3 = SEM_WK + len(WKP)
SEM_WR = SEM_W3 + 1
SEM_WGU = SEM_WR + 1
SEM_WD = SEM_WGU + 1
SEM_OUT = SEM_WD + 1
SEM_FIX = SEM_OUT + 2
NSEM = SEM_FIX + 2

INT_MIN = -(2 ** 31)
CPX = dict(disable_bounds_checks=True, disable_semaphore_checks=True)


def _layernorm(x, tok=None, w=None):
    s0 = x[:, 0:LANES]
    if tok is not None:
        s0 = s0 + jnp.concatenate([tok] * (x.shape[0] // 8), axis=0)
    for c in range(1, NC):
        s0 = s0 + x[:, c * LANES:(c + 1) * LANES]
    mu = jnp.sum(s0, axis=-1, keepdims=True) * (1.0 / D)
    xc = x - mu
    var = jnp.sum(xc * xc, axis=-1, keepdims=True) * (1.0 / D)
    rstd = lax.rsqrt(var + 1e-5)
    if w is None:
        return xc * rstd
    return xc * rstd, jnp.sum(xc * w, axis=-1, keepdims=True) * rstd


def _phi(t):
    return jnp.where(t > 0, t + 1.0, jnp.exp(t)) + 1e-6


def _pack_rows(a, b):
    return (pltpu.bitcast(a, U32) >> 16) | pltpu.bitcast(b, U32)


def _load_packed(ref):
    cols = []
    for c in range(NC):
        w = jnp.concatenate([ref[c, d * PSTR:d * PSTR + H // 2, :] for d in range(DH)], axis=0)
        cols.append(pltpu.bitcast(w, BF16))
    return jnp.concatenate(cols, axis=1)


def _store_interleaved(ref, val, head0):
    acc = None
    for hp in range(val.shape[0] // (2 * DH)):
        w = _pack_rows(val[hp * 2 * DH:hp * 2 * DH + DH, :], val[hp * 2 * DH + DH:(hp + 1) * 2 * DH, :])
        for c in range(NC):
            ref[c, pl.ds(head0 // 2 + hp, DH, stride=PSTR), :] = w[:, c * LANES:(c + 1) * LANES]
            for g in range(DH // 8):
                piece = w[g * 8:(g + 1) * 8, c * LANES:(c + 1) * LANES]
                acc = piece if acc is None else acc | piece
    return acc


def _kernel(x_hbm, wqkv_hbm, wo_hbm, wr_hbm, wg_hbm, wu_hbm, wd_hbm, out_hbm,
            x_v, wk_v, w3_v, wr_v, wgu_v, wd_v,
            ln1_v, pkt_v, zacc_v, g_v, wqp_v, mp_v, pqn_v, attn_v, lo_v, fix_v, zero_v, sems):

    ln2_v, out_v = lo_v.at[0], lo_v.at[1]

    wq_v, wv_v, wo_v = w3_v.at[0], w3_v.at[1], w3_v.at[2]
    wg_v, wu_v = wgu_v.at[0], wgu_v.at[1]

    def x_copy(i):
        r0, n = XP[i]
        return pltpu.make_async_copy(x_hbm.at[pl.ds(r0, n), :], x_v.at[pl.ds(DEF + r0, n), :], sems.at[SEM_X + i])

    def out_copy(r0, n, s):
        return pltpu.make_async_copy(out_v.at[pl.ds(DEF + r0, n), :], out_hbm.at[pl.ds(r0, n), :],
                                     sems.at[SEM_OUT + s])

    def wk_copy(j):
        c0, n = WKP[j]
        return pltpu.make_async_copy(wqkv_hbm.at[:, pl.ds(D + c0, n)], wk_v.at[:, pl.ds(c0, n)],
                                     sems.at[SEM_WK + j])

    wr_copy = pltpu.make_async_copy(wr_hbm, wr_v, sems.at[SEM_WR])
    wd_copy = pltpu.make_async_copy(wd_hbm, wd_v.at[:, pl.ds(0, D)], sems.at[SEM_WD])

    x_copy(0).start()
    x_copy(1).start()
    wr_copy.start()
    for j in range(len(WKP)):
        wk_copy(j).start()
    x_copy(2).start()
    x_copy(3).start()
    pltpu.make_async_copy(wqkv_hbm.at[:, pl.ds(0, D)], wq_v, sems.at[SEM_W3]).start()
    pltpu.make_async_copy(wqkv_hbm.at[:, pl.ds(2 * D, D)], wv_v, sems.at[SEM_W3]).start()
    pltpu.make_async_copy(wo_hbm, wo_v, sems.at[SEM_W3]).start()
    pltpu.make_async_copy(wg_hbm, wg_v, sems.at[SEM_WGU]).start()
    pltpu.make_async_copy(wu_hbm, wu_v, sems.at[SEM_WGU]).start()
    wd_copy.start()

    def ln1_rows(xr, xr0, lnr, r0, n):
        ln = _layernorm(xr[xr0:xr0 + n, :].astype(F32)).astype(BF16)
        lnr[r0 // 2:(r0 + n) // 2, :] = pltpu.bitcast(ln, U32)

    def ln1_rows_paced(xr, xr0, lnr, r0, n, L1LAG=L1LAG):
        zero_u = zero_v[...]
        toks = []
        lns = []
        for j in range(n // L1U):
            x = xr[xr0 + j * L1U:xr0 + (j + 1) * L1U, :].astype(F32)
            tok = toks[-L1LAG] if len(toks) >= L1LAG else None
            ln = _layernorm(x, tok)
            toks.append(pltpu.bitcast(pltpu.bitcast(ln[L1U - 8:L1U, 0:LANES], U32) & zero_u, F32))
            lns.append(ln)
            if (j + 1) * L1U % 16 == 0:
                grp = jnp.concatenate(lns, axis=0).astype(BF16)
                e = r0 + (j + 1) * L1U
                lnr[(e - grp.shape[0]) // 2:e // 2, :] = pltpu.bitcast(grp, U32)
                lns = []

    def ln1_load(lnr, r0, n):
        return pltpu.bitcast(lnr[r0 // 2:(r0 + n) // 2, :], BF16)

    def k_mm(lnr, r0, n, c0, nc):
        return jnp.dot(ln1_load(lnr, r0, n), wk_v[:, c0:c0 + nc], preferred_element_type=F32)

    def k_post(k, p0, c0, first=False):
        n, nc = k.shape
        pkt = _phi(k).T
        pkt_v[c0 // 2:(c0 + nc) // 2, p0:p0 + n] = pltpu.bitcast(pkt.astype(BF16), U32)
        zs = pkt[:, 0:LANES]
        for j in range(1, n // LANES):
            zs = zs + pkt[:, j * LANES:(j + 1) * LANES]
        for hh in range(nc // DH):
            z0 = (c0 // DH + hh) * ZP
            if first:
                zacc_v[z0:z0 + DH, :] = zs[hh * DH:(hh + 1) * DH, :]
            else:
                zacc_v[z0:z0 + DH, :] += zs[hh * DH:(hh + 1) * DH, :]

    def g_acc(lnr, r0, n, c0, nc, first=False):
        g = jnp.dot(pltpu.bitcast(pkt_v[c0 // 2:(c0 + nc) // 2, r0:r0 + n], BF16), ln1_load(lnr, r0, n),
                    preferred_element_type=F32)
        if first:
            g_v[c0:c0 + nc, :] = g
        else:
            g_v[c0:c0 + nc, :] += g

    attn_v[...] = jnp.zeros_like(attn_v)
    x_v[0:DEF, :] = jnp.zeros((DEF, D), BF16)
    zero_v[...] = jnp.zeros_like(zero_v)

    def k0(c0, nc):
        k_post(k_mm(ln1_v, 0, TX, c0, nc), 0, c0, first=True)

    def g0(c0, nc):
        g_acc(ln1_v, 0, TX, c0, nc, first=True)

    x_copy(0).wait()
    ln1_rows(x_v, DEF, ln1_v, 0, 128)
    x_copy(1).wait()
    ln1_rows(x_v, DEF + 128, ln1_v, 128, 128)
    wr_copy.wait()
    wk_copy(0).wait()
    k00 = k_mm(ln1_v, 0, TX, 0, 128)
    wk_copy(1).wait()
    k_post(k00, 0, 0, first=True)
    k0(128, 128)
    g0(0, 128)
    wk_copy(2).wait()
    k0(256, 256)
    g0(128, 128)
    wk_copy(3).wait()
    k0(512, 512)
    g0(256, 256)
    x_copy(2).wait()
    ln1_rows(x_v, DEF + TX, ln1_v, TX, TX)
    g0(512, 256)
    HD = D // 2
    k_post(k_mm(ln1_v, TX, TX, 0, HD), TX, 0)
    k_post(k_mm(ln1_v, TX, TX, HD, HD), TX, HD)
    ln1_rows_paced(x_v, DEF + TB, ln1_v, TB, TB, L1LAG0)
    g0(768, 256)
    g_acc(ln1_v, TX, TX, 0, HD)
    g_acc(ln1_v, TX, TX, HD, HD)

    def p1(i, carry):
        lnr = ln1_v.at[pl.ds(pl.multiple_of(i * (TB // 2), TB // 2), TB), :]
        xr = x_v.at[pl.ds(pl.multiple_of(jnp.minimum(i + 1, NBLK - 1) * TB, TB), TB + DEF), :]
        k_post(k_mm(lnr, 0, TB, 0, HD), 0, 0)
        k_post(k_mm(lnr, 0, TB, HD, HD), 0, HD)
        ln1_rows_paced(xr, DEF, lnr, TB, TB)
        g_acc(lnr, 0, TB, 0, HD)
        g_acc(lnr, 0, TB, HD, HD)
        return carry

    x_copy(3).wait()
    lax.fori_loop(1, NBLK, p1, 0)

    pltpu.make_async_copy(w3_v, w3_v, sems.at[SEM_W3]).wait()
    zero_u = zero_v[...]
    wtok = []
    for c in range(NC):
        wtok.append(zero_u & _store_interleaved(wqp_v, wq_v[:, c * LANES:(c + 1) * LANES].astype(F32).T,
                                                c * (LANES // DH)))
    zp = jnp.concatenate([zacc_v[pl.ds(d, H, stride=ZP), :] for d in range(DH)], axis=0)
    zrow = jnp.sum(zp.T, axis=0, keepdims=True)
    wr8 = wr_v[...].astype(F32)
    wr_row = jnp.concatenate([wr8[c:c + 1, :] for c in range(NC)], axis=1)

    row_h = lax.broadcasted_iota(I32, (LANES, LANES), 0) // DH
    col_h = lax.broadcasted_iota(I32, (LANES, LANES), 1) // DH
    diag = row_h == col_h
    def kv_part(c):
        cs = slice(c * LANES, (c + 1) * LANES)
        gb = g_v[cs, :]
        tk = None
        for cc in KVGATE[c]:
            tk = wtok[cc] if tk is None else tk | wtok[cc]
        if tk is not None:
            gb = jnp.concatenate([jnp.concatenate([gb[0:8, 0:LANES] + pltpu.bitcast(tk, F32), gb[0:8, LANES:]], axis=1),
                                  gb[8:, :]], axis=0)
        kv = jnp.dot(gb.astype(BF16), wv_v[:, cs], preferred_element_type=F32)
        return jnp.where(diag, kv, 0.0)

    def m_part(c, kv):
        cs = slice(c * LANES, (c + 1) * LANES)
        tk = None
        for cc in MGATE[c]:
            tk = wtok[cc] if tk is None else tk | wtok[cc]
        if tk is not None:
            kv = jnp.concatenate([kv[0:8, :] + pltpu.bitcast(tk, F32), kv[8:, :]], axis=0)
        m = jnp.dot(kv.astype(BF16), wo_v[cs, :], preferred_element_type=F32)
        _store_interleaved(mp_v, m.astype(BF16).astype(F32), c * (LANES // DH))

    kvs = {}
    for c in range(NC + KVLAG):
        if c < NC:
            kvs[c] = kv_part(c)
        if c >= KVLAG:
            m_part(c - KVLAG, kvs[c - KVLAG])

    def q_part(lnr, r0, n):
        q = lax.dot_general(ln1_load(lnr, r0, n), _load_packed(wqp_v),
                            (((1,), (1,)), ((), ())), preferred_element_type=F32)
        pq = _phi(q)
        t = pq * zrow
        den = t[:, 0:LANES]
        for c in range(1, NC):
            den = den + t[:, c * LANES:(c + 1) * LANES]
        den = den + pltpu.roll(den, DH, 1)
        den = den + pltpu.roll(den, 2 * DH, 1)
        inv = 1.0 / (den + 1e-6)
        pqn = (pq * jnp.concatenate([inv] * NC, axis=1)).astype(BF16)
        pqn_v[r0 // 2:(r0 + n) // 2, :] = pltpu.bitcast(pqn, U32)

    def o_part(r0, n):
        return jnp.dot(pltpu.bitcast(pqn_v[r0 // 2:(r0 + n) // 2, :], BF16), _load_packed(mp_v),
                       preferred_element_type=F32)

    def ln2_unit(attn, xr, l2r, outr, r0, row0, valid, top1, top2, tok, fast=False):
        n = attn.shape[0]
        h = xr[r0:r0 + n, :].astype(F32) + attn
        if fast:
            ln2, r = _layernorm(h, tok, wr_row)
        else:
            ln2 = _layernorm(h, tok)
            r = jnp.sum(ln2 * wr_row, axis=-1, keepdims=True)
        l2r[r0:r0 + n, :] = ln2.astype(BF16)
        res = h + ln2
        outr[r0:r0 + n, :] = res.astype(BF16)
        r = r.astype(BF16).astype(F32) + 0.0
        b = pltpu.bitcast(r, I32)
        srt = b ^ ((b >> 31) & 0x7FFFFFFF)
        row = (row0 + r0) + lax.broadcasted_iota(I32, (n, 1), 0)
        key = (srt & jnp.int32(-65536)) | (0xFFFF - row)
        if valid is not None:
            key = jnp.where(valid, key, INT_MIN)
        for gidx in range(n // 8):
            kx = key[gidx * 8:(gidx + 1) * 8, :]
            top2 = jnp.maximum(top2, jnp.minimum(top1, kx))
            top1 = jnp.maximum(top1, kx)
        ntok = pltpu.bitcast(pltpu.bitcast(jnp.broadcast_to(r[n - 8:n, :], (8, LANES)), U32) & zero_u, F32)
        return top1, top2, ntok

    def ln2_part(attn, xr, l2r, outr, r0, row0, valid, top1, top2, toks):
        n = attn.shape[0]
        u = min(LNU, n)
        for j in range(n // u):
            tok = toks[-LAG] if len(toks) >= LAG else None
            top1, top2, tok = ln2_unit(attn[j * u:(j + 1) * u, :], xr, l2r, outr, r0 + j * u, row0, valid,
                                       top1, top2, tok)
            toks.append(tok)
        return top1, top2

    def p2(i, carry):
        top1, top2 = carry
        b0 = pl.multiple_of(i * TB, TB)
        lnr = ln1_v.at[pl.ds(pl.multiple_of(i * (TB // 2), TB // 2), TB // 2), :]
        xr = x_v.at[pl.ds(b0, TB + DEF), :]
        l2r = ln2_v.at[pl.ds(b0, TB + DEF), :]
        outr = out_v.at[pl.ds(b0, TB + DEF), :]
        row0 = b0 - DEF
        toks = []
        top1, top2 = ln2_part(attn_v[...], xr, l2r, outr, 0, row0, i > 0, top1, top2, toks)

        @pl.when(i > 0)
        def _():
            out_copy(pl.multiple_of((i - 1) * TB, TB), TB, 0).start()

        q_part(lnr, 0, TX)
        q_part(lnr, TX, TX)
        r0 = 0
        for n in OCH[:-1]:
            top1, top2 = ln2_part(o_part(r0, n), xr, l2r, outr, DEF + r0, row0, None, top1, top2, toks)
            r0 += n
        attn_v[...] = o_part(r0, DEF)
        return top1, top2

    init = jnp.full((8, 1), INT_MIN, I32)
    top1, top2 = lax.fori_loop(0, NBLK, p2, (init, init))

    pltpu.make_async_copy(wgu_v, wgu_v, sems.at[SEM_WGU]).wait()
    wd_copy.wait()
    out_copy(0, S - TB, 0).wait()
    out_copy(S - TB, TB - DEF, 1).start()
    top1, top2, _ = ln2_unit(attn_v[...], x_v, ln2_v, out_v, S, -DEF, None, top1, top2, None, fast=True)
    out_copy(S - DEF, DEF, 1).start()

    def submax(v):
        for sh in (4, 2, 1):
            v = jnp.maximum(v, pltpu.roll(v, sh, 0))
        return v

    top1 = jnp.broadcast_to(top1, (8, LANES))
    top2 = jnp.broadcast_to(top2, (8, LANES))
    k1v = submax(top1)
    k2v = submax(jnp.where(top1 == k1v, top2, top1))
    keyv = (k1v, k2v)
    idx = [0xFFFF - (kk[0, 0] & 0xFFFF) for kk in keyv]
    grp = [pl.multiple_of((ii >> 3) << 3, 8) for ii in idx]
    vgrp = [pl.multiple_of(gg + DEF, 8) for gg in grp]

    xsel = jnp.concatenate([ln2_v[pl.ds(vgrp[c], 8), :] for c in range(2)], axis=0)
    gate = jnp.dot(xsel, wg_v[...], preferred_element_type=F32)
    up = jnp.dot(xsel, wu_v[...], preferred_element_type=F32)
    act = (gate * jax.nn.sigmoid(gate) * up).astype(BF16)
    y = jnp.dot(act, wd_v[:, 0:D], preferred_element_type=F32)

    sub8 = lax.broadcasted_iota(I32, (8, LANES), 0)
    scale = []
    for c in range(2):
        hi = keyv[c] & jnp.int32(-65536)
        score = pltpu.bitcast(hi ^ ((hi >> 31) & 0x7FFF0000), F32)
        scale.append((((0xFFFF - (keyv[c] & 0xFFFF)) & 7) == sub8, jax.nn.sigmoid(score)))
    same = ((0xFFFF - (k1v & 0xFFFF)) >> 3) == ((0xFFFF - (k2v & 0xFFFF)) >> 3)
    upd = []
    for c in range(2):
        sel, sg = scale[c]
        upd.append(jnp.concatenate(
            [jnp.where(sel, y[c * 8:(c + 1) * 8, j * LANES:(j + 1) * LANES] * sg, 0.0) for j in range(NC)], axis=1))
    same_w = jnp.concatenate([same] * NC, axis=1)
    fix_v[0] = (out_v[pl.ds(vgrp[0], 8), :].astype(F32) + upd[0] + jnp.where(same_w, upd[1], 0.0)).astype(BF16)
    fix_v[1] = (out_v[pl.ds(vgrp[1], 8), :].astype(F32) + upd[1]).astype(BF16)

    def fix_copy(c):
        return pltpu.make_async_copy(fix_v.at[c], out_hbm.at[pl.ds(grp[c], 8), :], sems.at[SEM_FIX + c])

    out_copy(S - TB, TB, 1).wait()
    fix_copy(0).start()

    @pl.when(grp[0] != grp[1])
    def _():
        fix_copy(1).start()
        fix_copy(1).wait()

    fix_copy(0).wait()


@jax.jit
def pallas_sequential_preLN__linear_attn_block__moe_arch_mod__prompt_kernel(
    A_x: jax.Array,
    A_wqkv: jax.Array,
    A_wo: jax.Array,
    B_x: jax.Array,
    B_w_r: jax.Array,
    B_w_gate: jax.Array,
    B_w_up: jax.Array,
    B_w_down: jax.Array,
):
    del B_x
    x = A_x.reshape(S, D)
    wr = B_w_r.reshape(NC, LANES)
    any_spec = pl.BlockSpec(memory_space=pl.ANY)
    out = pl.pallas_call(
        _kernel,
        out_shape=jax.ShapeDtypeStruct((S, D), BF16),
        in_specs=[any_spec] * 7,
        out_specs=any_spec,
        scratch_shapes=[
            pltpu.VMEM((S + DEF, D), BF16),
            pltpu.VMEM((D, D + LANES), BF16),
            pltpu.VMEM((3, D, D), BF16),
            pltpu.VMEM((NC, LANES), BF16),
            pltpu.VMEM((2, D, F), BF16),
            pltpu.VMEM((F, D + LANES), BF16),
            pltpu.VMEM(((S + TB) // 2, D), U32),
            pltpu.VMEM((D // 2, TB), U32),
            pltpu.VMEM((H * ZP, LANES), F32),
            pltpu.VMEM((D, D), F32),
            pltpu.VMEM((NC, DH * PSTR, LANES), U32),
            pltpu.VMEM((NC, DH * PSTR, LANES), U32),
            pltpu.VMEM((TB // 2, D), U32),
            pltpu.VMEM((DEF, D), F32),
            pltpu.VMEM((2, S + DEF, D), BF16),
            pltpu.VMEM((2, 8, D), BF16),
            pltpu.VMEM((8, LANES), U32),
            pltpu.SemaphoreType.DMA((NSEM,)),
        ],
        compiler_params=pltpu.CompilerParams(vmem_limit_bytes=110 * 1024 * 1024, **CPX),
    )(x, A_wqkv, A_wo, wr, B_w_gate, B_w_up, B_w_down)
    return out.reshape(1, S, D)
```

```python
import jax
import jax.numpy as jnp
from jax import lax
import jax.experimental.pallas as pl
import jax.experimental.pallas.tpu as pltpu

S = 2048
D = 1024
F = 3584
H = 32
DH = D // H
LANES = 128
NC = D // LANES

TB = 512
NBLK = S // TB
TX = 256
OCH = (64, 64, 64, 64, 64, 64, 64, 64)
DEF = OCH[-1]
LNU = 8
LAG = 5
L1U = 8
L1LAG = 2
L1LAG0 = 4
ZP = 36
KVLAG = 1
KVGATE = ((), (), (0,), (1,), (2,), (3,), (4,), (5,))
MGATE = ((), (), (), (), (), (), (6,), (7,))
PSTR = 20

F32 = jnp.float32
BF16 = jnp.bfloat16
U32 = jnp.uint32
I32 = jnp.int32

XP = ((0, 128), (128, 128), (256, 768), (1024, 1024))
WKP = ((0, 128), (128, 128), (256, 256), (512, 512))

SEM_X = 0
SEM_WK = SEM_X + len(XP)
SEM_W3 = SEM_WK + len(WKP)
SEM_WR = SEM_W3 + 1
SEM_WGU = SEM_WR + 1
SEM_WD = SEM_WGU + 1
SEM_OUT = SEM_WD + 1
SEM_FIX = SEM_OUT + 2
NSEM = SEM_FIX + 2

INT_MIN = -(2 ** 31)
CPX = dict(disable_bounds_checks=True, disable_semaphore_checks=True)


def _layernorm(x, tok=None, w=None):
    s0 = x[:, 0:LANES]
    if tok is not None:
        s0 = s0 + jnp.concatenate([tok] * (x.shape[0] // 8), axis=0)
    for c in range(1, NC):
        s0 = s0 + x[:, c * LANES:(c + 1) * LANES]
    mu = jnp.sum(s0, axis=-1, keepdims=True) * (1.0 / D)
    xc = x - mu
    var = jnp.sum(xc * xc, axis=-1, keepdims=True) * (1.0 / D)
    rstd = lax.rsqrt(var + 1e-5)
    if w is None:
        return xc * rstd
    return xc * rstd, jnp.sum(xc * w, axis=-1, keepdims=True) * rstd


def _phi(t):
    return jnp.where(t > 0, t + 1.0, jnp.exp(t)) + 1e-6


def _pack_rows(a, b):
    return (pltpu.bitcast(a, U32) >> 16) | pltpu.bitcast(b, U32)


def _load_packed(ref):
    cols = []
    for c in range(NC):
        w = jnp.concatenate([ref[c, d * PSTR:d * PSTR + H // 2, :] for d in range(DH)], axis=0)
        cols.append(pltpu.bitcast(w, BF16))
    return jnp.concatenate(cols, axis=1)


def _store_interleaved(ref, val, head0):
    acc = None
    for hp in range(val.shape[0] // (2 * DH)):
        w = _pack_rows(val[hp * 2 * DH:hp * 2 * DH + DH, :], val[hp * 2 * DH + DH:(hp + 1) * 2 * DH, :])
        for c in range(NC):
            ref[c, pl.ds(head0 // 2 + hp, DH, stride=PSTR), :] = w[:, c * LANES:(c + 1) * LANES]
            for g in range(DH // 8):
                piece = w[g * 8:(g + 1) * 8, c * LANES:(c + 1) * LANES]
                acc = piece if acc is None else acc | piece
    return acc


def _kernel(x_hbm, wqkv_hbm, wo_hbm, wr_hbm, wg_hbm, wu_hbm, wd_hbm, out_hbm,
            x_v, wk_v, w3_v, wr_v, wgu_v, wd_v,
            ln1_v, pkt_v, zacc_v, g_v, wqp_v, mp_v, pqn_v, attn_v, lo_v, fix_v, zero_v, sems):

    ln2_v, out_v = lo_v.at[0], lo_v.at[1]

    wq_v, wv_v, wo_v = w3_v.at[0], w3_v.at[1], w3_v.at[2]
    wg_v, wu_v = wgu_v.at[0], wgu_v.at[1]

    def x_copy(i):
        r0, n = XP[i]
        return pltpu.make_async_copy(x_hbm.at[pl.ds(r0, n), :], x_v.at[pl.ds(DEF + r0, n), :], sems.at[SEM_X + i])

    def out_copy(r0, n, s):
        return pltpu.make_async_copy(out_v.at[pl.ds(DEF + r0, n), :], out_hbm.at[pl.ds(r0, n), :],
                                     sems.at[SEM_OUT + s])

    def wk_copy(j):
        c0, n = WKP[j]
        return pltpu.make_async_copy(wqkv_hbm.at[:, pl.ds(D + c0, n)], wk_v.at[:, pl.ds(c0, n)],
                                     sems.at[SEM_WK + j])

    wr_copy = pltpu.make_async_copy(wr_hbm, wr_v, sems.at[SEM_WR])
    wd_copy = pltpu.make_async_copy(wd_hbm, wd_v.at[:, pl.ds(0, D)], sems.at[SEM_WD])

    x_copy(0).start()
    wk_copy(0).start()
    x_copy(1).start()
    wr_copy.start()
    for j in range(1, len(WKP)):
        wk_copy(j).start()
    x_copy(2).start()
    x_copy(3).start()
    pltpu.make_async_copy(wqkv_hbm.at[:, pl.ds(0, D)], wq_v, sems.at[SEM_W3]).start()
    pltpu.make_async_copy(wqkv_hbm.at[:, pl.ds(2 * D, D)], wv_v, sems.at[SEM_W3]).start()
    pltpu.make_async_copy(wo_hbm, wo_v, sems.at[SEM_W3]).start()
    pltpu.make_async_copy(wg_hbm, wg_v, sems.at[SEM_WGU]).start()
    pltpu.make_async_copy(wu_hbm, wu_v, sems.at[SEM_WGU]).start()
    wd_copy.start()

    def ln1_rows(xr, xr0, lnr, r0, n):
        ln = _layernorm(xr[xr0:xr0 + n, :].astype(F32)).astype(BF16)
        lnr[r0 // 2:(r0 + n) // 2, :] = pltpu.bitcast(ln, U32)

    def ln1_rows_paced(xr, xr0, lnr, r0, n, L1LAG=L1LAG):
        zero_u = zero_v[...]
        toks = []
        lns = []
        for j in range(n // L1U):
            x = xr[xr0 + j * L1U:xr0 + (j + 1) * L1U, :].astype(F32)
            tok = toks[-L1LAG] if len(toks) >= L1LAG else None
            ln = _layernorm(x, tok)
            toks.append(pltpu.bitcast(pltpu.bitcast(ln[L1U - 8:L1U, 0:LANES], U32) & zero_u, F32))
            lns.append(ln)
            if (j + 1) * L1U % 16 == 0:
                grp = jnp.concatenate(lns, axis=0).astype(BF16)
                e = r0 + (j + 1) * L1U
                lnr[(e - grp.shape[0]) // 2:e // 2, :] = pltpu.bitcast(grp, U32)
                lns = []

    def ln1_load(lnr, r0, n):
        return pltpu.bitcast(lnr[r0 // 2:(r0 + n) // 2, :], BF16)

    def k_mm(lnr, r0, n, c0, nc):
        return jnp.dot(ln1_load(lnr, r0, n), wk_v[:, c0:c0 + nc], preferred_element_type=F32)

    def k_post(k, p0, c0, first=False):
        n, nc = k.shape
        pkt = _phi(k).T
        pkt_v[c0 // 2:(c0 + nc) // 2, p0:p0 + n] = pltpu.bitcast(pkt.astype(BF16), U32)
        zs = pkt[:, 0:LANES]
        for j in range(1, n // LANES):
            zs = zs + pkt[:, j * LANES:(j + 1) * LANES]
        for hh in range(nc // DH):
            z0 = (c0 // DH + hh) * ZP
            if first:
                zacc_v[z0:z0 + DH, :] = zs[hh * DH:(hh + 1) * DH, :]
            else:
                zacc_v[z0:z0 + DH, :] += zs[hh * DH:(hh + 1) * DH, :]

    def g_acc(lnr, r0, n, c0, nc, first=False):
        g = jnp.dot(pltpu.bitcast(pkt_v[c0 // 2:(c0 + nc) // 2, r0:r0 + n], BF16), ln1_load(lnr, r0, n),
                    preferred_element_type=F32)
        if first:
            g_v[c0:c0 + nc, :] = g
        else:
            g_v[c0:c0 + nc, :] += g

    attn_v[...] = jnp.zeros_like(attn_v)
    x_v[0:DEF, :] = jnp.zeros((DEF, D), BF16)
    zero_v[...] = jnp.zeros_like(zero_v)

    def k0(c0, nc):
        k_post(k_mm(ln1_v, 0, TX, c0, nc), 0, c0, first=True)

    def g0(c0, nc):
        g_acc(ln1_v, 0, TX, c0, nc, first=True)

    x_copy(0).wait()
    ln1_rows(x_v, DEF, ln1_v, 0, 128)
    wk_copy(0).wait()
    ka = k_mm(ln1_v, 0, 128, 0, 128)
    x_copy(1).wait()
    wr_copy.wait()
    ln1_rows(x_v, DEF + 128, ln1_v, 128, 128)
    k_post(ka, 0, 0, first=True)
    g_acc(ln1_v, 0, 128, 0, 128, first=True)
    wk_copy(1).wait()
    k_post(k_mm(ln1_v, 128, 128, 0, 128), 128, 0)
    k0(128, 128)
    g_acc(ln1_v, 128, 128, 0, 128)
    wk_copy(2).wait()
    k0(256, 256)
    g0(128, 128)
    g0(256, 256)
    wk_copy(3).wait()
    k0(512, 256)
    k0(768, 256)
    g0(512, 256)
    x_copy(2).wait()
    ln1_rows(x_v, DEF + TX, ln1_v, TX, TX)
    g0(768, 256)
    HD = D // 2
    k_post(k_mm(ln1_v, TX, TX, 0, HD), TX, 0)
    k_post(k_mm(ln1_v, TX, TX, HD, HD), TX, HD)
    ln1_rows_paced(x_v, DEF + TB, ln1_v, TB, TB, L1LAG0)
    g_acc(ln1_v, TX, TX, 0, HD)
    g_acc(ln1_v, TX, TX, HD, HD)

    def p1(i, carry):
        lnr = ln1_v.at[pl.ds(pl.multiple_of(i * (TB // 2), TB // 2), TB), :]
        xr = x_v.at[pl.ds(pl.multiple_of(jnp.minimum(i + 1, NBLK - 1) * TB, TB), TB + DEF), :]
        k_post(k_mm(lnr, 0, TB, 0, HD), 0, 0)
        k_post(k_mm(lnr, 0, TB, HD, HD), 0, HD)
        ln1_rows_paced(xr, DEF, lnr, TB, TB)
        g_acc(lnr, 0, TB, 0, HD)
        g_acc(lnr, 0, TB, HD, HD)
        return carry

    x_copy(3).wait()
    lax.fori_loop(1, NBLK, p1, 0)

    pltpu.make_async_copy(w3_v, w3_v, sems.at[SEM_W3]).wait()
    zero_u = zero_v[...]
    wtok = []
    for c in range(NC):
        wtok.append(zero_u & _store_interleaved(wqp_v, wq_v[:, c * LANES:(c + 1) * LANES].astype(F32).T,
                                                c * (LANES // DH)))
    zp = jnp.concatenate([zacc_v[pl.ds(d, H, stride=ZP), :] for d in range(DH)], axis=0)
    zrow = jnp.sum(zp.T, axis=0, keepdims=True)
    wr8 = wr_v[...].astype(F32)
    wr_row = jnp.concatenate([wr8[c:c + 1, :] for c in range(NC)], axis=1)

    row_h = lax.broadcasted_iota(I32, (LANES, LANES), 0) // DH
    col_h = lax.broadcasted_iota(I32, (LANES, LANES), 1) // DH
    diag = row_h == col_h
    def kv_part(c):
        cs = slice(c * LANES, (c + 1) * LANES)
        gb = g_v[cs, :]
        tk = None
        for cc in KVGATE[c]:
            tk = wtok[cc] if tk is None else tk | wtok[cc]
        if tk is not None:
            gb = jnp.concatenate([jnp.concatenate([gb[0:8, 0:LANES] + pltpu.bitcast(tk, F32), gb[0:8, LANES:]], axis=1),
                                  gb[8:, :]], axis=0)
        kv = jnp.dot(gb.astype(BF16), wv_v[:, cs], preferred_element_type=F32)
        return jnp.where(diag, kv, 0.0)

    def m_part(c, kv):
        cs = slice(c * LANES, (c + 1) * LANES)
        tk = None
        for cc in MGATE[c]:
            tk = wtok[cc] if tk is None else tk | wtok[cc]
        if tk is not None:
            kv = jnp.concatenate([kv[0:8, :] + pltpu.bitcast(tk, F32), kv[8:, :]], axis=0)
        m = jnp.dot(kv.astype(BF16), wo_v[cs, :], preferred_element_type=F32)
        _store_interleaved(mp_v, m.astype(BF16).astype(F32), c * (LANES // DH))

    kvs = {}
    for c in range(NC + KVLAG):
        if c < NC:
            kvs[c] = kv_part(c)
        if c >= KVLAG:
            m_part(c - KVLAG, kvs[c - KVLAG])

    def q_part(lnr, r0, n):
        q = lax.dot_general(ln1_load(lnr, r0, n), _load_packed(wqp_v),
                            (((1,), (1,)), ((), ())), preferred_element_type=F32)
        pq = _phi(q)
        t = pq * zrow
        den = t[:, 0:LANES]
        for c in range(1, NC):
            den = den + t[:, c * LANES:(c + 1) * LANES]
        den = den + pltpu.roll(den, DH, 1)
        den = den + pltpu.roll(den, 2 * DH, 1)
        inv = 1.0 / (den + 1e-6)
        pqn = (pq * jnp.concatenate([inv] * NC, axis=1)).astype(BF16)
        pqn_v[r0 // 2:(r0 + n) // 2, :] = pltpu.bitcast(pqn, U32)

    def o_part(r0, n):
        return jnp.dot(pltpu.bitcast(pqn_v[r0 // 2:(r0 + n) // 2, :], BF16), _load_packed(mp_v),
                       preferred_element_type=F32)

    def ln2_unit(attn, xr, l2r, outr, r0, row0, valid, top1, top2, tok, fast=False):
        n = attn.shape[0]
        h = xr[r0:r0 + n, :].astype(F32) + attn
        if fast:
            ln2, r = _layernorm(h, tok, wr_row)
        else:
            ln2 = _layernorm(h, tok)
            r = jnp.sum(ln2 * wr_row, axis=-1, keepdims=True)
        l2r[r0:r0 + n, :] = ln2.astype(BF16)
        res = h + ln2
        outr[r0:r0 + n, :] = res.astype(BF16)
        r = r.astype(BF16).astype(F32) + 0.0
        b = pltpu.bitcast(r, I32)
        srt = b ^ ((b >> 31) & 0x7FFFFFFF)
        row = (row0 + r0) + lax.broadcasted_iota(I32, (n, 1), 0)
        key = (srt & jnp.int32(-65536)) | (0xFFFF - row)
        if valid is not None:
            key = jnp.where(valid, key, INT_MIN)
        for gidx in range(n // 8):
            kx = key[gidx * 8:(gidx + 1) * 8, :]
            top2 = jnp.maximum(top2, jnp.minimum(top1, kx))
            top1 = jnp.maximum(top1, kx)
        ntok = pltpu.bitcast(pltpu.bitcast(jnp.broadcast_to(r[n - 8:n, :], (8, LANES)), U32) & zero_u, F32)
        return top1, top2, ntok

    def ln2_part(attn, xr, l2r, outr, r0, row0, valid, top1, top2, toks):
        n = attn.shape[0]
        u = min(LNU, n)
        for j in range(n // u):
            tok = toks[-LAG] if len(toks) >= LAG else None
            top1, top2, tok = ln2_unit(attn[j * u:(j + 1) * u, :], xr, l2r, outr, r0 + j * u, row0, valid,
                                       top1, top2, tok)
            toks.append(tok)
        return top1, top2

    def p2(i, carry):
        top1, top2 = carry
        b0 = pl.multiple_of(i * TB, TB)
        lnr = ln1_v.at[pl.ds(pl.multiple_of(i * (TB // 2), TB // 2), TB // 2), :]
        xr = x_v.at[pl.ds(b0, TB + DEF), :]
        l2r = ln2_v.at[pl.ds(b0, TB + DEF), :]
        outr = out_v.at[pl.ds(b0, TB + DEF), :]
        row0 = b0 - DEF
        toks = []
        top1, top2 = ln2_part(attn_v[...], xr, l2r, outr, 0, row0, i > 0, top1, top2, toks)

        @pl.when(i > 0)
        def _():
            out_copy(pl.multiple_of((i - 1) * TB, TB), TB, 0).start()

        q_part(lnr, 0, TX)
        q_part(lnr, TX, TX)
        r0 = 0
        for n in OCH[:-1]:
            top1, top2 = ln2_part(o_part(r0, n), xr, l2r, outr, DEF + r0, row0, None, top1, top2, toks)
            r0 += n
        attn_v[...] = o_part(r0, DEF)
        return top1, top2

    init = jnp.full((8, 1), INT_MIN, I32)
    top1, top2 = lax.fori_loop(0, NBLK, p2, (init, init))

    pltpu.make_async_copy(wgu_v, wgu_v, sems.at[SEM_WGU]).wait()
    wd_copy.wait()
    out_copy(0, S - TB, 0).wait()
    out_copy(S - TB, TB - DEF, 1).start()
    top1, top2, _ = ln2_unit(attn_v[...], x_v, ln2_v, out_v, S, -DEF, None, top1, top2, None, fast=True)
    out_copy(S - DEF, DEF, 1).start()

    def submax(v):
        for sh in (4, 2, 1):
            v = jnp.maximum(v, pltpu.roll(v, sh, 0))
        return v

    top1 = jnp.broadcast_to(top1, (8, LANES))
    top2 = jnp.broadcast_to(top2, (8, LANES))
    k1v = submax(top1)
    k2v = submax(jnp.where(top1 == k1v, top2, top1))
    keyv = (k1v, k2v)
    idx = [0xFFFF - (kk[0, 0] & 0xFFFF) for kk in keyv]
    grp = [pl.multiple_of((ii >> 3) << 3, 8) for ii in idx]
    vgrp = [pl.multiple_of(gg + DEF, 8) for gg in grp]

    xsel = jnp.concatenate([ln2_v[pl.ds(vgrp[c], 8), :] for c in range(2)], axis=0)
    gate = jnp.dot(xsel, wg_v[...], preferred_element_type=F32)
    up = jnp.dot(xsel, wu_v[...], preferred_element_type=F32)
    act = (gate * jax.nn.sigmoid(gate) * up).astype(BF16)
    y = jnp.dot(act, wd_v[:, 0:D], preferred_element_type=F32)

    sub8 = lax.broadcasted_iota(I32, (8, LANES), 0)
    scale = []
    for c in range(2):
        hi = keyv[c] & jnp.int32(-65536)
        score = pltpu.bitcast(hi ^ ((hi >> 31) & 0x7FFF0000), F32)
        scale.append((((0xFFFF - (keyv[c] & 0xFFFF)) & 7) == sub8, jax.nn.sigmoid(score)))
    same = ((0xFFFF - (k1v & 0xFFFF)) >> 3) == ((0xFFFF - (k2v & 0xFFFF)) >> 3)
    upd = []
    for c in range(2):
        sel, sg = scale[c]
        upd.append(jnp.concatenate(
            [jnp.where(sel, y[c * 8:(c + 1) * 8, j * LANES:(j + 1) * LANES] * sg, 0.0) for j in range(NC)], axis=1))
    same_w = jnp.concatenate([same] * NC, axis=1)
    fix_v[0] = (out_v[pl.ds(vgrp[0], 8), :].astype(F32) + upd[0] + jnp.where(same_w, upd[1], 0.0)).astype(BF16)
    fix_v[1] = (out_v[pl.ds(vgrp[1], 8), :].astype(F32) + upd[1]).astype(BF16)

    def fix_copy(c):
        return pltpu.make_async_copy(fix_v.at[c], out_hbm.at[pl.ds(grp[c], 8), :], sems.at[SEM_FIX + c])

    out_copy(S - TB, TB, 1).wait()
    fix_copy(0).start()

    @pl.when(grp[0] != grp[1])
    def _():
        fix_copy(1).start()
        fix_copy(1).wait()

    fix_copy(0).wait()


@jax.jit
def pallas_sequential_preLN__linear_attn_block__moe_arch_mod__prompt_kernel(
    A_x: jax.Array,
    A_wqkv: jax.Array,
    A_wo: jax.Array,
    B_x: jax.Array,
    B_w_r: jax.Array,
    B_w_gate: jax.Array,
    B_w_up: jax.Array,
    B_w_down: jax.Array,
):
    del B_x
    x = A_x.reshape(S, D)
    wr = B_w_r.reshape(NC, LANES)
    any_spec = pl.BlockSpec(memory_space=pl.ANY)
    out = pl.pallas_call(
        _kernel,
        out_shape=jax.ShapeDtypeStruct((S, D), BF16),
        in_specs=[any_spec] * 7,
        out_specs=any_spec,
        scratch_shapes=[
            pltpu.VMEM((S + DEF, D), BF16),
            pltpu.VMEM((D, D + LANES), BF16),
            pltpu.VMEM((3, D, D), BF16),
            pltpu.VMEM((NC, LANES), BF16),
            pltpu.VMEM((2, D, F), BF16),
            pltpu.VMEM((F, D + LANES), BF16),
            pltpu.VMEM(((S + TB) // 2, D), U32),
            pltpu.VMEM((D // 2, TB), U32),
            pltpu.VMEM((H * ZP, LANES), F32),
            pltpu.VMEM((D, D), F32),
            pltpu.VMEM((NC, DH * PSTR, LANES), U32),
            pltpu.VMEM((NC, DH * PSTR, LANES), U32),
            pltpu.VMEM((TB // 2, D), U32),
            pltpu.VMEM((DEF, D), F32),
            pltpu.VMEM((2, S + DEF, D), BF16),
            pltpu.VMEM((2, 8, D), BF16),
            pltpu.VMEM((8, LANES), U32),
            pltpu.SemaphoreType.DMA((NSEM,)),
        ],
        compiler_params=pltpu.CompilerParams(vmem_limit_bytes=110 * 1024 * 1024, **CPX),
    )(x, A_wqkv, A_wo, wr, B_w_gate, B_w_up, B_w_down)
    return out.reshape(1, S, D)
```

```python
import jax
import jax.numpy as jnp
from jax import lax
import jax.experimental.pallas as pl
import jax.experimental.pallas.tpu as pltpu

S = 2048
D = 1024
F = 3584
H = 32
DH = D // H
LANES = 128
NC = D // LANES

P0 = 512
TB = 384
NB1 = (S - P0) // TB
TX = 256
TB2 = 544
NB2 = 3
L0 = NB2 * TB2
RL = S - L0
OCL = (32, 64, 64, 64, 64, 64, 64)
QS = (288, 128)
NPRE = 24
NGAP = 9
GLAG = (None, None, None, None, None, 22, 11)
LAG_L = 4
OUT_AT = (160, 288, 352)
OCH = (32, 64, 64, 64, 64, 64, 64, 64, 64)
DEF = OCH[-1]
LNU = 8
LAG = 5
L1U = 8
L1LAG = 2
L1LAG0 = 4
ZP = 36
KVLAG = 1
KVGATE = ((), (), (0,), (1,), (2,), (3,), (4,), (5,))
MGATE = ((), (), (), (), (), (), (6,), (7,))
PSTR = 20

F32 = jnp.float32
BF16 = jnp.bfloat16
U32 = jnp.uint32
I32 = jnp.int32

XP = ((0, 128), (128, 128), (256, 768), (1024, 1024))
WKP = ((0, 128), (128, 128), (256, 256), (512, 512))

SEM_X = 0
SEM_WK = SEM_X + len(XP)
SEM_W3 = SEM_WK + len(WKP)
SEM_WR = SEM_W3 + 1
SEM_WGU = SEM_WR + 1
SEM_WD = SEM_WGU + 1
SEM_OUT = SEM_WD + 1
SEM_FIX = SEM_OUT + 2
NSEM = SEM_FIX + 2

INT_MIN = -(2 ** 31)
CPX = dict(disable_bounds_checks=True, disable_semaphore_checks=True)


def _layernorm(x, tok=None, w=None):
    s0 = x[:, 0:LANES]
    if tok is not None:
        s0 = s0 + jnp.concatenate([tok] * (x.shape[0] // 8), axis=0)
    for c in range(1, NC):
        s0 = s0 + x[:, c * LANES:(c + 1) * LANES]
    mu = jnp.sum(s0, axis=-1, keepdims=True) * (1.0 / D)
    xc = x - mu
    var = jnp.sum(xc * xc, axis=-1, keepdims=True) * (1.0 / D)
    rstd = lax.rsqrt(var + 1e-5)
    if w is None:
        return xc * rstd
    return xc * rstd, jnp.sum(xc * w, axis=-1, keepdims=True) * rstd


def _phi(t):
    return jnp.where(t > 0, t + 1.0, jnp.exp(t)) + 1e-6


def _pack_rows(a, b):
    return (pltpu.bitcast(a, U32) >> 16) | pltpu.bitcast(b, U32)


def _load_packed(ref):
    cols = []
    for c in range(NC):
        w = jnp.concatenate([ref[c, d * PSTR:d * PSTR + H // 2, :] for d in range(DH)], axis=0)
        cols.append(pltpu.bitcast(w, BF16))
    return jnp.concatenate(cols, axis=1)


def _store_interleaved(ref, val, head0):
    acc = None
    for hp in range(val.shape[0] // (2 * DH)):
        w = _pack_rows(val[hp * 2 * DH:hp * 2 * DH + DH, :], val[hp * 2 * DH + DH:(hp + 1) * 2 * DH, :])
        for c in range(NC):
            ref[c, pl.ds(head0 // 2 + hp, DH, stride=PSTR), :] = w[:, c * LANES:(c + 1) * LANES]
            for g in range(DH // 8):
                piece = w[g * 8:(g + 1) * 8, c * LANES:(c + 1) * LANES]
                acc = piece if acc is None else acc | piece
    return acc


def _kernel(x_hbm, wqkv_hbm, wo_hbm, wr_hbm, wg_hbm, wu_hbm, wd_hbm, out_hbm,
            x_v, wk_v, w3_v, wr_v, wgu_v, wd_v,
            ln1_v, pkt_v, zacc_v, g_v, wqp_v, mp_v, pqn_v, attn_v, lo_v, fix_v, pf_v, ysel_v, zero_v, sems):

    ln2_v, out_v = lo_v.at[0], lo_v.at[1]

    wqkv_hbm, wo_hbm, wg_hbm, wu_hbm, wd_hbm = (r.bitcast(U32) for r in (wqkv_hbm, wo_hbm, wg_hbm, wu_hbm, wd_hbm))

    def wload(ref, r0, nr, cols):
        rows = pl.ds(r0 // 2, nr // 2) if isinstance(r0, int) else pl.ds(pl.multiple_of(r0 // 2, nr // 2), nr // 2)
        return pltpu.bitcast(ref[rows, cols], BF16)

    wq_v, wv_v, wo_v = w3_v.at[0], w3_v.at[1], w3_v.at[2]
    wg_v, wu_v = wgu_v.at[0], wgu_v.at[1]

    def x_copy(i):
        r0, n = XP[i]
        return pltpu.make_async_copy(x_hbm.at[pl.ds(r0, n), :], x_v.at[pl.ds(DEF + r0, n), :], sems.at[SEM_X + i])

    def out_copy(r0, n, s):
        return pltpu.make_async_copy(out_v.at[pl.ds(DEF + r0, n), :], out_hbm.at[pl.ds(r0, n), :],
                                     sems.at[SEM_OUT + s])

    def wk_copy(j):
        c0, n = WKP[j]
        return pltpu.make_async_copy(wqkv_hbm.at[:, pl.ds(D + c0, n)], wk_v.at[:, pl.ds(c0, n)],
                                     sems.at[SEM_WK + j])

    wr_copy = pltpu.make_async_copy(wr_hbm, wr_v, sems.at[SEM_WR])
    wd_copy = pltpu.make_async_copy(wd_hbm, wd_v, sems.at[SEM_WD])

    x_copy(0).start()
    wk_copy(0).start()
    x_copy(1).start()
    wr_copy.start()
    for j in range(1, len(WKP)):
        wk_copy(j).start()
    x_copy(2).start()
    x_copy(3).start()
    pltpu.make_async_copy(wqkv_hbm.at[:, pl.ds(0, D)], wq_v, sems.at[SEM_W3]).start()
    pltpu.make_async_copy(wqkv_hbm.at[:, pl.ds(2 * D, D)], wv_v, sems.at[SEM_W3]).start()
    pltpu.make_async_copy(wo_hbm, wo_v, sems.at[SEM_W3]).start()
    pltpu.make_async_copy(wg_hbm, wg_v, sems.at[SEM_WGU]).start()
    pltpu.make_async_copy(wu_hbm, wu_v, sems.at[SEM_WGU]).start()
    wd_copy.start()

    def ln1_rows(xr, xr0, lnr, r0, n):
        ln = _layernorm(xr[xr0:xr0 + n, :].astype(F32)).astype(BF16)
        lnr[r0 // 2:(r0 + n) // 2, :] = pltpu.bitcast(ln, U32)

    def ln1_rows_paced(xr, xr0, lnr, r0, n, L1LAG=L1LAG):
        zero_u = zero_v[...]
        toks = []
        lns = []
        for j in range(n // L1U):
            x = xr[xr0 + j * L1U:xr0 + (j + 1) * L1U, :].astype(F32)
            tok = toks[-L1LAG] if len(toks) >= L1LAG else None
            ln = _layernorm(x, tok)
            toks.append(pltpu.bitcast(pltpu.bitcast(ln[L1U - 8:L1U, 0:LANES], U32) & zero_u, F32))
            lns.append(ln)
            if (j + 1) * L1U % 16 == 0:
                grp = jnp.concatenate(lns, axis=0).astype(BF16)
                e = r0 + (j + 1) * L1U
                lnr[(e - grp.shape[0]) // 2:e // 2, :] = pltpu.bitcast(grp, U32)
                lns = []

    def ln1_load(lnr, r0, n):
        return pltpu.bitcast(lnr[r0 // 2:(r0 + n) // 2, :], BF16)

    def k_mm(lnr, r0, n, c0, nc):
        return jnp.dot(ln1_load(lnr, r0, n), wload(wk_v, 0, D, slice(c0, c0 + nc)), preferred_element_type=F32)

    def k_post(k, p0, c0, first=False):
        n, nc = k.shape
        pkt = _phi(k).T
        pkt_v[c0 // 2:(c0 + nc) // 2, p0:p0 + n] = pltpu.bitcast(pkt.astype(BF16), U32)
        zs = pkt[:, 0:LANES]
        for j in range(1, n // LANES):
            zs = zs + pkt[:, j * LANES:(j + 1) * LANES]
        for hh in range(nc // DH):
            z0 = (c0 // DH + hh) * ZP
            if first:
                zacc_v[z0:z0 + DH, :] = zs[hh * DH:(hh + 1) * DH, :]
            else:
                zacc_v[z0:z0 + DH, :] += zs[hh * DH:(hh + 1) * DH, :]

    def g_acc(lnr, r0, n, c0, nc, first=False):
        g = jnp.dot(pltpu.bitcast(pkt_v[c0 // 2:(c0 + nc) // 2, r0:r0 + n], BF16), ln1_load(lnr, r0, n),
                    preferred_element_type=F32)
        if first:
            g_v[c0:c0 + nc, :] = g
        else:
            g_v[c0:c0 + nc, :] += g

    attn_v[...] = jnp.zeros_like(attn_v)
    x_v[0:DEF, :] = jnp.zeros((DEF, D), BF16)
    zero_v[...] = jnp.zeros_like(zero_v)

    def k0(c0, nc):
        k_post(k_mm(ln1_v, 0, TX, c0, nc), 0, c0, first=True)

    def g0(c0, nc):
        g_acc(ln1_v, 0, TX, c0, nc, first=True)

    x_copy(0).wait()
    ln1_rows(x_v, DEF, ln1_v, 0, 128)
    wk_copy(0).wait()
    ka = k_mm(ln1_v, 0, 128, 0, 128)
    x_copy(1).wait()
    wr_copy.wait()
    ln1_rows(x_v, DEF + 128, ln1_v, 128, 128)
    k_post(ka, 0, 0, first=True)
    g_acc(ln1_v, 0, 128, 0, 128, first=True)
    wk_copy(1).wait()
    k_post(k_mm(ln1_v, 128, 128, 0, 128), 128, 0)
    k0(128, 128)
    g_acc(ln1_v, 128, 128, 0, 128)
    wk_copy(2).wait()
    k0(256, 256)
    g0(128, 128)
    g0(256, 256)
    wk_copy(3).wait()
    k0(512, 256)
    k0(768, 256)
    g0(512, 256)
    x_copy(2).wait()
    ln1_rows(x_v, DEF + TX, ln1_v, TX, TX)
    g0(768, 256)
    HD = D // 2
    k_post(k_mm(ln1_v, TX, TX, 0, HD), TX, 0)
    k_post(k_mm(ln1_v, TX, TX, HD, HD), TX, HD)
    ln1_rows_paced(x_v, DEF + P0, ln1_v, P0, TB, L1LAG0)
    g_acc(ln1_v, TX, TX, 0, HD)
    g_acc(ln1_v, TX, TX, HD, HD)

    def p1(i, carry):
        lnr = ln1_v.at[pl.ds(pl.multiple_of(P0 // 2 + i * (TB // 2), 64), TB), :]
        xr = x_v.at[pl.ds(pl.multiple_of(P0 + jnp.minimum(i + 1, NB1 - 1) * TB, 128), TB + DEF), :]
        k_post(k_mm(lnr, 0, TB, 0, HD), 0, 0)
        k_post(k_mm(lnr, 0, TB, HD, HD), 0, HD)
        ln1_rows_paced(xr, DEF, lnr, TB, TB)
        g_acc(lnr, 0, TB, 0, HD)
        g_acc(lnr, 0, TB, HD, HD)
        return carry

    x_copy(3).wait()
    lax.fori_loop(0, NB1, p1, 0)

    pltpu.make_async_copy(w3_v, w3_v, sems.at[SEM_W3]).wait()
    zero_u = zero_v[...]
    wtok = []
    for c in range(NC):
        wtok.append(zero_u & _store_interleaved(wqp_v, wload(wq_v, 0, D, slice(c * LANES, (c + 1) * LANES)).astype(F32).T,
                                                c * (LANES // DH)))
    zp = jnp.concatenate([zacc_v[pl.ds(d, H, stride=ZP), :] for d in range(DH)], axis=0)
    zrow = jnp.sum(zp.T, axis=0, keepdims=True)
    wr8 = wr_v[...].astype(F32)
    wr_row = jnp.concatenate([wr8[c:c + 1, :] for c in range(NC)], axis=1)

    row_h = lax.broadcasted_iota(I32, (LANES, LANES), 0) // DH
    col_h = lax.broadcasted_iota(I32, (LANES, LANES), 1) // DH
    diag = row_h == col_h
    def kv_part(c):
        cs = slice(c * LANES, (c + 1) * LANES)
        gb = g_v[cs, :]
        tk = None
        for cc in KVGATE[c]:
            tk = wtok[cc] if tk is None else tk | wtok[cc]
        if tk is not None:
            gb = jnp.concatenate([jnp.concatenate([gb[0:8, 0:LANES] + pltpu.bitcast(tk, F32), gb[0:8, LANES:]], axis=1),
                                  gb[8:, :]], axis=0)
        kv = jnp.dot(gb.astype(BF16), wload(wv_v, 0, D, cs), preferred_element_type=F32)
        return jnp.where(diag, kv, 0.0)

    def m_part(c, kv):
        cs = slice(c * LANES, (c + 1) * LANES)
        tk = None
        for cc in MGATE[c]:
            tk = wtok[cc] if tk is None else tk | wtok[cc]
        if tk is not None:
            kv = jnp.concatenate([kv[0:8, :] + pltpu.bitcast(tk, F32), kv[8:, :]], axis=0)
        m = jnp.dot(kv.astype(BF16), wload(wo_v, c * LANES, LANES, slice(None)), preferred_element_type=F32)
        _store_interleaved(mp_v, m.astype(BF16).astype(F32), c * (LANES // DH))

    kvs = {}
    for c in range(NC + KVLAG):
        if c < NC:
            kvs[c] = kv_part(c)
        if c >= KVLAG:
            m_part(c - KVLAG, kvs[c - KVLAG])

    def make_key(score, row):
        b = pltpu.bitcast(score, I32)
        srt = b ^ ((b >> 31) & 0x7FFFFFFF)
        return (srt & jnp.int32(-65536)) | (0xFFFF - row)

    def push_keys(key, top1, top2):
        for gidx in range(key.shape[0] // 8):
            kx = key[gidx * 8:(gidx + 1) * 8, :]
            top2 = jnp.maximum(top2, jnp.minimum(top1, kx))
            top1 = jnp.maximum(top1, kx)
        return top1, top2

    def colsum(t):
        acc = t[:, 0:LANES]
        for c in range(1, NC):
            acc = acc + t[:, c * LANES:(c + 1) * LANES]
        return acc

    def q_part(lnr, l0, r0, n, hint=None):
        q = lax.dot_general(ln1_load(lnr, l0 + r0, n), _load_packed(wqp_v),
                            (((1,), (1,)), ((), ())), preferred_element_type=F32)
        pq = _phi(q)
        den = colsum(pq * zrow)
        den = den + pltpu.roll(den, DH, 1)
        den = den + pltpu.roll(den, 2 * DH, 1)
        inv = 1.0 / (den + 1e-6)
        pqn = pq * jnp.concatenate([inv] * NC, axis=1)
        pqn_v[r0 // 2:(r0 + n) // 2, :] = pltpu.bitcast(pqn.astype(BF16), U32)
        if hint is None:
            return None
        urow, wrc, p1, p2 = hint
        pf_v[r0:r0 + n, :] = pqn
        xb = x_v[DEF + l0 + r0:DEF + l0 + r0 + n, :].astype(F32)
        num = jnp.sum(colsum(xb * wrc) + colsum(pq * urow) * inv, axis=-1, keepdims=True)
        return push_keys(make_key(num, (l0 + r0) + lax.broadcasted_iota(I32, (n, 1), 0)), p1, p2)

    def o_part(r0, n):
        return jnp.dot(pltpu.bitcast(pqn_v[r0 // 2:(r0 + n) // 2, :], BF16), _load_packed(mp_v),
                       preferred_element_type=F32)

    def ln2_unit(attn, xr, l2r, outr, r0, row0, valid, top1, top2, tok, fast=False, is_h=False):
        n = attn.shape[0]
        h = attn if is_h else xr[r0:r0 + n, :].astype(F32) + attn
        if fast:
            ln2, r = _layernorm(h, tok, wr_row)
        else:
            ln2 = _layernorm(h, tok)
            r = jnp.sum(ln2 * wr_row, axis=-1, keepdims=True)
        l2r[r0:r0 + n, :] = ln2.astype(BF16)
        res = h + ln2
        outr[r0:r0 + n, :] = res.astype(BF16)
        r = r.astype(BF16).astype(F32) + 0.0
        key = make_key(r, (row0 + r0) + lax.broadcasted_iota(I32, (n, 1), 0))
        if valid is not None:
            key = jnp.where(valid, key, INT_MIN)
        top1, top2 = push_keys(key, top1, top2)
        ntok = pltpu.bitcast(pltpu.bitcast(jnp.broadcast_to(r[n - 8:n, :], (8, LANES)), U32) & zero_u, F32)
        return top1, top2, ntok

    def ln2_part(attn, xr, l2r, outr, r0, row0, valid, top1, top2, toks, lag=LAG, **kw):
        n = attn.shape[0]
        u = min(LNU, n)
        for j in range(n // u):
            tok = toks[-lag] if len(toks) >= lag else None
            top1, top2, tok = ln2_unit(attn[j * u:(j + 1) * u, :], xr, l2r, outr, r0 + j * u, row0, valid,
                                       top1, top2, tok, **kw)
            toks.append(tok)
        return top1, top2

    def p2(i, carry):
        top1, top2 = carry
        b0 = pl.multiple_of(i * TB2, 16)
        lnr = ln1_v.at[pl.ds(pl.multiple_of(i * (TB2 // 2), 8), TB2 // 2), :]
        xr = x_v.at[pl.ds(b0, TB2 + DEF), :]
        l2r = ln2_v.at[pl.ds(b0, TB2 + DEF), :]
        outr = out_v.at[pl.ds(b0, TB2 + DEF), :]
        row0 = b0 - DEF
        toks = []
        top1, top2 = ln2_part(attn_v[...], xr, l2r, outr, 0, row0, i > 0, top1, top2, toks)

        @pl.when(i > 0)
        def _():
            out_copy(pl.multiple_of((i - 1) * TB2, 16), TB2, 0).start()

        qa = (TB2 // 32) * 16
        q_part(lnr, 0, 0, qa)
        q_part(lnr, 0, qa, TB2 - qa)
        r0 = 0
        for n in OCH[:-1]:
            top1, top2 = ln2_part(o_part(r0, n), xr, l2r, outr, DEF + r0, row0, None, top1, top2, toks)
            r0 += n
        attn_v[...] = o_part(r0, DEF)
        return top1, top2

    init = jnp.full((8, 1), INT_MIN, I32)
    top1, top2 = lax.fori_loop(0, NB2, p2, (init, init))

    pltpu.make_async_copy(wgu_v, wgu_v, sems.at[SEM_WGU]).wait()
    wd_copy.wait()
    sub8 = lax.broadcasted_iota(I32, (8, LANES), 0)

    def submax(v):
        for sh in (4, 2, 1):
            v = jnp.maximum(v, pltpu.roll(v, sh, 0))
        return v

    def subsum(v):
        for sh in (4, 2, 1):
            v = v + pltpu.roll(v, sh, 0)
        return v

    def best2(t1, t2):
        t1 = jnp.broadcast_to(t1, (8, LANES))
        t2 = jnp.broadcast_to(t2, (8, LANES))
        k1v = submax(t1)
        return k1v, submax(jnp.where(t1 == k1v, t2, t1))

    def key_row(k):
        return 0xFFFF - (k & 0xFFFF)

    def wide(m):
        return jnp.concatenate([m] * NC, axis=1)

    def m_tile(c, k0, nk):
        w = jnp.concatenate([mp_v[c, d * PSTR:d * PSTR + H // 2, :] for d in range(k0 // H, (k0 + nk) // H)], axis=0)
        return pltpu.bitcast(w, BF16)

    toks = []
    top1, top2 = ln2_part(attn_v[...], x_v, ln2_v, out_v, L0, -DEF, None, top1, top2, toks, lag=LAG_L)
    out_copy(L0 - TB2, TB2, 0).start()
    oldk = best2(top1, top2)
    oldx = []
    for kk in oldk:
        g8 = pl.multiple_of(((key_row(kk[0, 0]) >> 3) << 3) + DEF, 8)
        rows = ln2_v[pl.ds(g8, 8), :].astype(F32)
        oldx.append(subsum(jnp.where(wide((key_row(kk) & 7) == sub8), rows, 0.0)))

    wrc = wr_row - jnp.sum(wr_row, axis=-1, keepdims=True) * (1.0 / D)
    uparts = []
    for k0 in range(0, D, LANES):
        mrows = jnp.concatenate([m_tile(c, k0, LANES) for c in range(NC)], axis=1).astype(F32)
        part = colsum(mrows * wrc)
        if uparts:
            tok = pltpu.bitcast(pltpu.bitcast(jnp.broadcast_to(uparts[-1], (8, LANES)), U32) & zero_u, F32)
            mrows = jnp.concatenate([mrows[:, 0:LANES] + jnp.concatenate([tok] * (LANES // 8), axis=0),
                                     mrows[:, LANES:]], axis=1)
            part = colsum(mrows * wrc)
        uparts.append(jnp.sum(part.T, axis=0, keepdims=True))
    urow = jnp.concatenate(uparts, axis=1)
    p1, p2_, r0 = init, init, 0
    for n in QS:
        p1, p2_ = q_part(ln1_v, L0, r0, n, (urow, wrc, p1, p2_))
        r0 += n

    cand_p, cand_x = [], []
    for pk_ in (p1, p2_):
        cp = jnp.zeros((8, D), F32)
        cx = jnp.zeros((8, D), F32)
        for s in range(8):
            g8 = pl.multiple_of((key_row(pk_[s, 0]) >> 3) << 3, 8)
            m = wide(sub8 == s)
            cp = jnp.where(m, pf_v[pl.ds(g8 - L0, 8), :], cp)
            cx = jnp.where(m, x_v[pl.ds(g8 + DEF, 8), :].astype(F32), cx)
        cand_p.append(cp)
        cand_x.append(cx)
    cand_p = jnp.concatenate(cand_p, axis=0).astype(BF16)
    cand_x = jnp.concatenate(cand_x, axis=0)
    ids_lo = key_row(jnp.broadcast_to(p1, (8, LANES)))
    ids_hi = jnp.where(sub8 < 6, key_row(jnp.broadcast_to(p2_, (8, LANES))),
                       jnp.where(sub8 == 6, key_row(oldk[0]), key_row(oldk[1])))

    st = dict(top1=top1, top2=top2, pend=[], step=0, sent=0)

    def gated(v):
        tok = None
        while st["pend"] and st["pend"][0][0] <= st["step"]:
            t = st["pend"].pop(0)[1]
            tok = t if tok is None else tok | t
        if tok is None:
            return v
        u = pltpu.bitcast(v, U32)
        return pltpu.bitcast(jnp.concatenate([u[:, 0:LANES] | tok, u[:, LANES:]], axis=1), BF16)

    def o_units():
        HW = D // 2
        r0 = -OCL[0]
        for ci, n in enumerate(OCL):
            r0 += OCL[ci - 1] if ci else OCL[0]
            lhs = pltpu.bitcast(pqn_v[r0 // 2:(r0 + n) // 2, :], BF16)
            halves = []
            for c0 in range(0, NC, NC // 2):
                acc = x_v[DEF + L0 + r0:DEF + L0 + r0 + n, c0 * LANES:c0 * LANES + HW].astype(F32)
                for k0 in range(0, D, LANES):
                    w = jnp.concatenate([m_tile(c, k0, LANES) for c in range(c0, c0 + NC // 2)], axis=1)
                    acc = acc + jnp.dot(lhs[:, k0:k0 + LANES], w, preferred_element_type=F32)
                    if k0 + LANES == D:
                        halves.append(acc)
                        if len(halves) == 2:
                            last = r0 + n == RL
                            tk = [] if last else toks
                            st["top1"], st["top2"] = ln2_part(
                                jnp.concatenate(halves, axis=1), x_v, ln2_v, out_v, DEF + L0 + r0, -DEF, None,
                                st["top1"], st["top2"], tk, lag=n if last else LAG_L, is_h=True, fast=last)
                            if GLAG[ci] is not None:
                                st["pend"].append((st["step"] + GLAG[ci],
                                                   pltpu.bitcast(jnp.broadcast_to(st["top1"], (8, LANES)), U32) & zero_u))
                            if r0 + n in OUT_AT or last:
                                out_copy(L0 + st["sent"], r0 + n - st["sent"], 1).start()
                                st["sent"] = r0 + n
                    yield

    res = {}

    def c_units():
        parts = []
        for c in range(NC):
            parts.append(jnp.dot(cand_p, m_tile(c, 0, D), preferred_element_type=F32))
            yield
        xs = _layernorm(cand_x + jnp.concatenate(parts, axis=1))
        hi = jnp.where(wide(sub8 < 6), xs[8:16, :], jnp.where(wide(sub8 == 6), oldx[0], oldx[1]))
        res["xs"] = jnp.concatenate([xs[0:8, :], hi], axis=0).astype(BF16)

    def f_units():
        xs = res["xs"]
        acts = []
        for j in range(F // LANES):
            cs = slice(j * LANES, (j + 1) * LANES)
            g = jnp.dot(gated(xs), wload(wg_v, 0, D, cs), preferred_element_type=F32)
            yield
            u = jnp.dot(xs, wload(wu_v, 0, D, cs), preferred_element_type=F32)
            acts.append((g * jax.nn.sigmoid(g) * u).astype(BF16))
            yield
        ys = [None] * NC
        for c in range(NC):
            for k0 in range(0, F, D):
                nk = min(D, F - k0)
                a = jnp.concatenate(acts[k0 // LANES:(k0 + nk) // LANES], axis=1)
                p = jnp.dot(gated(a), wload(wd_v, k0, nk, slice(c * LANES, (c + 1) * LANES)),
                            preferred_element_type=F32)
                ys[c] = p if ys[c] is None else ys[c] + p
                yield
        res["y"] = jnp.concatenate(ys, axis=1)

    ou = o_units()

    def o_step():
        next(ou, None)
        st["step"] += 1

    for _ in range(NPRE):
        o_step()
    for _ in c_units():
        o_step()
    for _ in range(NGAP):
        o_step()
    for _ in f_units():
        o_step()
    for _ in ou:
        pass

    keyv = best2(st["top1"], st["top2"])
    idx = [key_row(kk[0, 0]) for kk in keyv]
    grp = [pl.multiple_of((ii >> 3) << 3, 8) for ii in idx]
    vgrp = [pl.multiple_of(gg + DEF, 8) for gg in grp]
    y = res["y"]
    hits = None
    for c in range(2):
        m_lo = ids_lo == key_row(keyv[c])
        m_hi = ids_hi == key_row(keyv[c])
        yrow = subsum(jnp.where(wide(m_lo), y[0:8, :], 0.0) + jnp.where(wide(m_hi), y[8:16, :], 0.0))
        ysel_v[c * 8:(c + 1) * 8, :] = yrow
        hit = submax(jnp.where(m_lo | m_hi, 1, 0))
        hits = hit if hits is None else hits + hit

    @pl.when(hits[0, 0] < 2)
    def _():
        xsel = jnp.concatenate([ln2_v[pl.ds(vgrp[c], 8), :] for c in range(2)], axis=0)

        def ffn_tile(j, acc):
            cs = pl.ds(pl.multiple_of(j * LANES, LANES), LANES)
            g = jnp.dot(xsel, wload(wg_v, 0, D, cs), preferred_element_type=F32)
            u = jnp.dot(xsel, wload(wu_v, 0, D, cs), preferred_element_type=F32)
            a = (g * jax.nn.sigmoid(g) * u).astype(BF16)
            wd_t = pltpu.bitcast(wd_v[pl.ds(pl.multiple_of(j * (LANES // 2), LANES // 2), LANES // 2), :], BF16)
            return acc + jnp.dot(a, wd_t, preferred_element_type=F32)

        ysel_v[...] = lax.fori_loop(0, F // LANES, ffn_tile, jnp.zeros((16, D), F32))

    upd = []
    for c in range(2):
        hi = keyv[c] & jnp.int32(-65536)
        score = pltpu.bitcast(hi ^ ((hi >> 31) & 0x7FFF0000), F32)
        sel = (key_row(keyv[c]) & 7) == sub8
        upd.append(jnp.where(wide(sel), ysel_v[c * 8:(c + 1) * 8, :] * wide(jax.nn.sigmoid(score)), 0.0))
    same = (key_row(keyv[0]) >> 3) == (key_row(keyv[1]) >> 3)
    fix_v[0] = (out_v[pl.ds(vgrp[0], 8), :].astype(F32) + upd[0] + jnp.where(wide(same), upd[1], 0.0)).astype(BF16)
    fix_v[1] = (out_v[pl.ds(vgrp[1], 8), :].astype(F32) + upd[1]).astype(BF16)

    def fix_copy(c):
        return pltpu.make_async_copy(fix_v.at[c], out_hbm.at[pl.ds(grp[c], 8), :], sems.at[SEM_FIX + c])

    out_copy(0, L0, 0).wait()
    out_copy(L0, RL, 1).wait()
    fix_copy(0).start()

    @pl.when(grp[0] != grp[1])
    def _():
        fix_copy(1).start()
        fix_copy(1).wait()

    fix_copy(0).wait()


@jax.jit
def pallas_sequential_preLN__linear_attn_block__moe_arch_mod__prompt_kernel(
    A_x: jax.Array,
    A_wqkv: jax.Array,
    A_wo: jax.Array,
    B_x: jax.Array,
    B_w_r: jax.Array,
    B_w_gate: jax.Array,
    B_w_up: jax.Array,
    B_w_down: jax.Array,
):
    del B_x
    x = A_x.reshape(S, D)
    wr = B_w_r.reshape(NC, LANES)
    any_spec = pl.BlockSpec(memory_space=pl.ANY)
    out = pl.pallas_call(
        _kernel,
        out_shape=jax.ShapeDtypeStruct((S, D), BF16),
        in_specs=[any_spec] * 7,
        out_specs=any_spec,
        scratch_shapes=[
            pltpu.VMEM((S + DEF, D), BF16),
            pltpu.VMEM((D // 2, D), U32),
            pltpu.VMEM((3, D // 2, D), U32),
            pltpu.VMEM((NC, LANES), BF16),
            pltpu.VMEM((2, D // 2, F), U32),
            pltpu.VMEM((F // 2, D), U32),
            pltpu.VMEM(((S + TB) // 2, D), U32),
            pltpu.VMEM((D // 2, max(TB, P0)), U32),
            pltpu.VMEM((H * ZP, LANES), F32),
            pltpu.VMEM((D, D), F32),
            pltpu.VMEM((NC, DH * PSTR, LANES), U32),
            pltpu.VMEM((NC, DH * PSTR, LANES), U32),
            pltpu.VMEM((TB2 // 2, D), U32),
            pltpu.VMEM((DEF, D), F32),
            pltpu.VMEM((2, S + DEF, D), BF16),
            pltpu.VMEM((2, 8, D), BF16),
            pltpu.VMEM((RL, D), F32),
            pltpu.VMEM((16, D), F32),
            pltpu.VMEM((8, LANES), U32),
            pltpu.SemaphoreType.DMA((NSEM,)),
        ],
        compiler_params=pltpu.CompilerParams(vmem_limit_bytes=110 * 1024 * 1024, **CPX),
    )(x, A_wqkv, A_wo, wr, B_w_gate, B_w_up, B_w_down)
    return out.reshape(1, S, D)
```

```python
import jax
import jax.numpy as jnp
from jax import lax
import jax.experimental.pallas as pl
import jax.experimental.pallas.tpu as pltpu

S = 2048
D = 1024
F = 3584
H = 32
DH = D // H
LANES = 128
NC = D // LANES

P0 = 512
TB = 384
NB1 = (S - P0) // TB
TX = 256
TB2 = 544
NB2 = 3
L0 = NB2 * TB2
RL = S - L0
OCL = (32, 64, 64, 64, 64, 64, 64)
QS = (224, 128, 64)
ONT = 2
NPRE = 24
NGAP = 9
GLAG = (None, None, None, None, None, 20, 8)
LAG_L = 3
OUT_AT = (160, 288, 352, 416)
OCH = (64, 64, 64, 64, 64, 64, 64, 32, 64)
DEF = OCH[-1]
LNU = 8
LAG = 5
L1U = 8
L1LAG = 2
L1LAG0 = 4
ZP = 36
KVLAG = 1
KVGATE = ((), (), (0,), (1,), (2,), (3,), (4,), (5,))
MGATE = ((), (), (), (), (), (), (6,), (7,))
PSTR = 20

F32 = jnp.float32
BF16 = jnp.bfloat16
U32 = jnp.uint32
I32 = jnp.int32

XP = ((0, 128), (128, 128), (256, 768), (1024, 1024))
WKP = ((0, 128), (128, 128), (256, 256), (512, 512))

SEM_X = 0
SEM_WK = SEM_X + len(XP)
SEM_W3 = SEM_WK + len(WKP)
SEM_WR = SEM_W3 + 1
SEM_WGU = SEM_WR + 1
SEM_WD = SEM_WGU + 1
SEM_OUT = SEM_WD + 1
NSEM = SEM_OUT + 5

INT_MIN = -(2 ** 31)
CPX = dict(disable_bounds_checks=True, disable_semaphore_checks=True)


def _layernorm(x, tok=None, w=None):
    s0 = x[:, 0:LANES]
    if tok is not None:
        s0 = s0 + jnp.concatenate([tok] * (x.shape[0] // 8), axis=0)
    for c in range(1, NC):
        s0 = s0 + x[:, c * LANES:(c + 1) * LANES]
    mu = jnp.sum(s0, axis=-1, keepdims=True) * (1.0 / D)
    xc = x - mu
    var = jnp.sum(xc * xc, axis=-1, keepdims=True) * (1.0 / D)
    rstd = lax.rsqrt(var + 1e-5)
    if w is None:
        return xc * rstd
    return xc * rstd, jnp.sum(xc * w, axis=-1, keepdims=True) * rstd


def _phi(t):
    return jnp.where(t > 0, t + 1.0, jnp.exp(t)) + 1e-6


def _pack_rows(a, b):
    return (pltpu.bitcast(a, U32) >> 16) | pltpu.bitcast(b, U32)


def _load_packed(ref):
    cols = []
    for c in range(NC):
        w = jnp.concatenate([ref[c, d * PSTR:d * PSTR + H // 2, :] for d in range(DH)], axis=0)
        cols.append(pltpu.bitcast(w, BF16))
    return jnp.concatenate(cols, axis=1)


def _store_interleaved(ref, val, head0):
    acc = None
    for hp in range(val.shape[0] // (2 * DH)):
        w = _pack_rows(val[hp * 2 * DH:hp * 2 * DH + DH, :], val[hp * 2 * DH + DH:(hp + 1) * 2 * DH, :])
        for c in range(NC):
            ref[c, pl.ds(head0 // 2 + hp, DH, stride=PSTR), :] = w[:, c * LANES:(c + 1) * LANES]
            for g in range(DH // 8):
                piece = w[g * 8:(g + 1) * 8, c * LANES:(c + 1) * LANES]
                acc = piece if acc is None else acc | piece
    return acc


def _kernel(x_hbm, wqkv_hbm, wo_hbm, wr_hbm, wg_hbm, wu_hbm, wd_hbm, out_hbm,
            x_v, wk_v, w3_v, wr_v, wgu_v, wd_v,
            ln1_v, pkt_v, zacc_v, g_v, wqp_v, mp_v, pqn_v, attn_v, lo_v, zero_v, sems):

    ln2_v, out_v = lo_v.at[0], lo_v.at[1]

    wqkv_hbm, wo_hbm, wg_hbm, wu_hbm, wd_hbm = (r.bitcast(U32) for r in (wqkv_hbm, wo_hbm, wg_hbm, wu_hbm, wd_hbm))

    def wload(ref, r0, nr, cols):
        rows = pl.ds(r0 // 2, nr // 2) if isinstance(r0, int) else pl.ds(pl.multiple_of(r0 // 2, nr // 2), nr // 2)
        return pltpu.bitcast(ref[rows, cols], BF16)

    wq_v, wv_v, wo_v = w3_v.at[0], w3_v.at[1], w3_v.at[2]
    wg_v, wu_v = wgu_v.at[0], wgu_v.at[1]

    def x_copy(i):
        r0, n = XP[i]
        return pltpu.make_async_copy(x_hbm.at[pl.ds(r0, n), :], x_v.at[pl.ds(DEF + r0, n), :], sems.at[SEM_X + i])

    def out_copy(r0, n, s):
        return pltpu.make_async_copy(out_v.at[pl.ds(DEF + r0, n), :], out_hbm.at[pl.ds(r0, n), :],
                                     sems.at[SEM_OUT + s])

    def wk_copy(j):
        c0, n = WKP[j]
        return pltpu.make_async_copy(wqkv_hbm.at[:, pl.ds(D + c0, n)], wk_v.at[:, pl.ds(c0, n)],
                                     sems.at[SEM_WK + j])

    wr_copy = pltpu.make_async_copy(wr_hbm, wr_v, sems.at[SEM_WR])
    wd_copy = pltpu.make_async_copy(wd_hbm, wd_v, sems.at[SEM_WD])

    x_copy(0).start()
    wk_copy(0).start()
    x_copy(1).start()
    wr_copy.start()
    for j in range(1, len(WKP)):
        wk_copy(j).start()
    x_copy(2).start()
    x_copy(3).start()
    pltpu.make_async_copy(wqkv_hbm.at[:, pl.ds(0, D)], wq_v, sems.at[SEM_W3]).start()
    pltpu.make_async_copy(wqkv_hbm.at[:, pl.ds(2 * D, D)], wv_v, sems.at[SEM_W3]).start()
    pltpu.make_async_copy(wo_hbm, wo_v, sems.at[SEM_W3]).start()
    pltpu.make_async_copy(wg_hbm, wg_v, sems.at[SEM_WGU]).start()
    pltpu.make_async_copy(wu_hbm, wu_v, sems.at[SEM_WGU]).start()
    wd_copy.start()

    def ln1_rows(xr, xr0, lnr, r0, n):
        ln = _layernorm(xr[xr0:xr0 + n, :].astype(F32)).astype(BF16)
        lnr[r0 // 2:(r0 + n) // 2, :] = pltpu.bitcast(ln, U32)

    def ln1_rows_paced(xr, xr0, lnr, r0, n, L1LAG=L1LAG):
        zero_u = zero_v[...]
        toks = []
        lns = []
        for j in range(n // L1U):
            x = xr[xr0 + j * L1U:xr0 + (j + 1) * L1U, :].astype(F32)
            tok = toks[-L1LAG] if len(toks) >= L1LAG else None
            ln = _layernorm(x, tok)
            toks.append(pltpu.bitcast(pltpu.bitcast(ln[L1U - 8:L1U, 0:LANES], U32) & zero_u, F32))
            lns.append(ln)
            if (j + 1) * L1U % 16 == 0:
                grp = jnp.concatenate(lns, axis=0).astype(BF16)
                e = r0 + (j + 1) * L1U
                lnr[(e - grp.shape[0]) // 2:e // 2, :] = pltpu.bitcast(grp, U32)
                lns = []

    def ln1_load(lnr, r0, n):
        return pltpu.bitcast(lnr[r0 // 2:(r0 + n) // 2, :], BF16)

    def k_mm(lnr, r0, n, c0, nc):
        return jnp.dot(ln1_load(lnr, r0, n), wload(wk_v, 0, D, slice(c0, c0 + nc)), preferred_element_type=F32)

    def k_post(k, p0, c0, first=False):
        n, nc = k.shape
        pkt = _phi(k).T
        pkt_v[c0 // 2:(c0 + nc) // 2, p0:p0 + n] = pltpu.bitcast(pkt.astype(BF16), U32)
        zs = pkt[:, 0:LANES]
        for j in range(1, n // LANES):
            zs = zs + pkt[:, j * LANES:(j + 1) * LANES]
        for hh in range(nc // DH):
            z0 = (c0 // DH + hh) * ZP
            if first:
                zacc_v[z0:z0 + DH, :] = zs[hh * DH:(hh + 1) * DH, :]
            else:
                zacc_v[z0:z0 + DH, :] += zs[hh * DH:(hh + 1) * DH, :]

    def g_acc(lnr, r0, n, c0, nc, first=False):
        g = jnp.dot(pltpu.bitcast(pkt_v[c0 // 2:(c0 + nc) // 2, r0:r0 + n], BF16), ln1_load(lnr, r0, n),
                    preferred_element_type=F32)
        if first:
            g_v[c0:c0 + nc, :] = g
        else:
            g_v[c0:c0 + nc, :] += g

    attn_v[...] = jnp.zeros_like(attn_v)
    x_v[0:DEF, :] = jnp.zeros((DEF, D), BF16)
    zero_v[...] = jnp.zeros_like(zero_v)

    def k0(c0, nc):
        k_post(k_mm(ln1_v, 0, TX, c0, nc), 0, c0, first=True)

    def g0(c0, nc):
        g_acc(ln1_v, 0, TX, c0, nc, first=True)

    x_copy(0).wait()
    ln1_rows(x_v, DEF, ln1_v, 0, 128)
    wk_copy(0).wait()
    ka = k_mm(ln1_v, 0, 128, 0, 128)
    x_copy(1).wait()
    wr_copy.wait()
    ln1_rows(x_v, DEF + 128, ln1_v, 128, 128)
    k_post(ka, 0, 0, first=True)
    g_acc(ln1_v, 0, 128, 0, 128, first=True)
    wk_copy(1).wait()
    k_post(k_mm(ln1_v, 128, 128, 0, 128), 128, 0)
    k0(128, 128)
    g_acc(ln1_v, 128, 128, 0, 128)
    wk_copy(2).wait()
    k0(256, 256)
    g0(128, 128)
    g0(256, 256)
    wk_copy(3).wait()
    k0(512, 256)
    k0(768, 256)
    g0(512, 256)
    x_copy(2).wait()
    ln1_rows(x_v, DEF + TX, ln1_v, TX, TX)
    g0(768, 256)
    HD = D // 2
    k_post(k_mm(ln1_v, TX, TX, 0, HD), TX, 0)
    k_post(k_mm(ln1_v, TX, TX, HD, HD), TX, HD)
    ln1_rows_paced(x_v, DEF + P0, ln1_v, P0, TB, L1LAG0)
    g_acc(ln1_v, TX, TX, 0, HD)
    g_acc(ln1_v, TX, TX, HD, HD)

    def p1(i, carry):
        lnr = ln1_v.at[pl.ds(pl.multiple_of(P0 // 2 + i * (TB // 2), 64), TB), :]
        xr = x_v.at[pl.ds(pl.multiple_of(P0 + jnp.minimum(i + 1, NB1 - 1) * TB, 128), TB + DEF), :]
        k_post(k_mm(lnr, 0, TB, 0, HD), 0, 0)
        k_post(k_mm(lnr, 0, TB, HD, HD), 0, HD)
        ln1_rows_paced(xr, DEF, lnr, TB, TB)
        g_acc(lnr, 0, TB, 0, HD)
        g_acc(lnr, 0, TB, HD, HD)
        return carry

    x_copy(3).wait()
    lax.fori_loop(0, NB1, p1, 0)

    pltpu.make_async_copy(w3_v, w3_v, sems.at[SEM_W3]).wait()
    zero_u = zero_v[...]
    wtok = []
    for c in range(NC):
        wtok.append(zero_u & _store_interleaved(wqp_v, wload(wq_v, 0, D, slice(c * LANES, (c + 1) * LANES)).astype(F32).T,
                                                c * (LANES // DH)))
    zp = jnp.concatenate([zacc_v[pl.ds(d, H, stride=ZP), :] for d in range(DH)], axis=0)
    zrow = jnp.sum(zp.T, axis=0, keepdims=True)
    wr8 = wr_v[...].astype(F32)
    wr_row = jnp.concatenate([wr8[c:c + 1, :] for c in range(NC)], axis=1)

    row_h = lax.broadcasted_iota(I32, (LANES, LANES), 0) // DH
    col_h = lax.broadcasted_iota(I32, (LANES, LANES), 1) // DH
    diag = row_h == col_h
    def kv_part(c):
        cs = slice(c * LANES, (c + 1) * LANES)
        gb = g_v[cs, :]
        tk = None
        for cc in KVGATE[c]:
            tk = wtok[cc] if tk is None else tk | wtok[cc]
        if tk is not None:
            gb = jnp.concatenate([jnp.concatenate([gb[0:8, 0:LANES] + pltpu.bitcast(tk, F32), gb[0:8, LANES:]], axis=1),
                                  gb[8:, :]], axis=0)
        kv = jnp.dot(gb.astype(BF16), wload(wv_v, 0, D, cs), preferred_element_type=F32)
        return jnp.where(diag, kv, 0.0)

    def m_part(c, kv):
        cs = slice(c * LANES, (c + 1) * LANES)
        tk = None
        for cc in MGATE[c]:
            tk = wtok[cc] if tk is None else tk | wtok[cc]
        if tk is not None:
            kv = jnp.concatenate([kv[0:8, :] + pltpu.bitcast(tk, F32), kv[8:, :]], axis=0)
        m = jnp.dot(kv.astype(BF16), wload(wo_v, c * LANES, LANES, slice(None)), preferred_element_type=F32)
        _store_interleaved(mp_v, m.astype(BF16).astype(F32), c * (LANES // DH))

    kvs = {}
    for c in range(NC + KVLAG):
        if c < NC:
            kvs[c] = kv_part(c)
        if c >= KVLAG:
            m_part(c - KVLAG, kvs[c - KVLAG])

    def make_key(score, row):
        b = pltpu.bitcast(score, I32)
        srt = b ^ ((b >> 31) & 0x7FFFFFFF)
        return (srt & jnp.int32(-65536)) | (0xFFFF - row)

    def push_keys(key, top1, top2):
        for gidx in range(key.shape[0] // 8):
            kx = key[gidx * 8:(gidx + 1) * 8, :]
            top2 = jnp.maximum(top2, jnp.minimum(top1, kx))
            top1 = jnp.maximum(top1, kx)
        return top1, top2

    def colsum(t):
        acc = t[:, 0:LANES]
        for c in range(1, NC):
            acc = acc + t[:, c * LANES:(c + 1) * LANES]
        return acc

    def q_part(lnr, l0, r0, n, hint=None):
        q = lax.dot_general(ln1_load(lnr, l0 + r0, n), _load_packed(wqp_v),
                            (((1,), (1,)), ((), ())), preferred_element_type=F32)
        pq = _phi(q)
        den = colsum(pq * zrow)
        den = den + pltpu.roll(den, DH, 1)
        den = den + pltpu.roll(den, 2 * DH, 1)
        inv = 1.0 / (den + 1e-6)
        pqn = pq * jnp.concatenate([inv] * NC, axis=1)
        pqn_v[r0 // 2:(r0 + n) // 2, :] = pltpu.bitcast(pqn.astype(BF16), U32)
        if hint is None:
            return None
        urow, wrc, p1, p2 = hint
        xb = x_v[DEF + l0 + r0:DEF + l0 + r0 + n, :].astype(F32)
        num = jnp.sum(colsum(xb * wrc) + colsum(pq * urow) * inv, axis=-1, keepdims=True)
        return push_keys(make_key(num, (l0 + r0) + lax.broadcasted_iota(I32, (n, 1), 0)), p1, p2)

    def o_part(r0, n):
        return jnp.dot(pltpu.bitcast(pqn_v[r0 // 2:(r0 + n) // 2, :], BF16), _load_packed(mp_v),
                       preferred_element_type=F32)

    def ln2_unit(attn, xr, l2r, outr, r0, row0, valid, top1, top2, tok, fast=False, is_h=False):
        n = attn.shape[0]
        h = attn if is_h else xr[r0:r0 + n, :].astype(F32) + attn
        if fast:
            ln2, r = _layernorm(h, tok, wr_row)
        else:
            ln2 = _layernorm(h, tok)
            r = jnp.sum(ln2 * wr_row, axis=-1, keepdims=True)
        l2r[r0:r0 + n, :] = ln2.astype(BF16)
        res = h + ln2
        outr[r0:r0 + n, :] = res.astype(BF16)
        r = r.astype(BF16).astype(F32) + 0.0
        key = make_key(r, (row0 + r0) + lax.broadcasted_iota(I32, (n, 1), 0))
        if valid is not None:
            key = jnp.where(valid, key, INT_MIN)
        top1, top2 = push_keys(key, top1, top2)
        ntok = pltpu.bitcast(pltpu.bitcast(jnp.broadcast_to(r[n - 8:n, :], (8, LANES)), U32) & zero_u, F32)
        return top1, top2, ntok

    def ln2_part(attn, xr, l2r, outr, r0, row0, valid, top1, top2, toks, lag=LAG, **kw):
        n = attn.shape[0]
        u = min(LNU, n)
        for j in range(n // u):
            tok = toks[-lag] if len(toks) >= lag else None
            top1, top2, tok = ln2_unit(attn[j * u:(j + 1) * u, :], xr, l2r, outr, r0 + j * u, row0, valid,
                                       top1, top2, tok, **kw)
            toks.append(tok)
        return top1, top2

    def p2(i, carry):
        top1, top2 = carry
        b0 = pl.multiple_of(i * TB2, 16)
        lnr = ln1_v.at[pl.ds(pl.multiple_of(i * (TB2 // 2), 8), TB2 // 2), :]
        xr = x_v.at[pl.ds(b0, TB2 + DEF), :]
        l2r = ln2_v.at[pl.ds(b0, TB2 + DEF), :]
        outr = out_v.at[pl.ds(b0, TB2 + DEF), :]
        row0 = b0 - DEF
        toks = []
        top1, top2 = ln2_part(attn_v[...], xr, l2r, outr, 0, row0, i > 0, top1, top2, toks)

        @pl.when(i > 0)
        def _():
            out_copy(pl.multiple_of((i - 1) * TB2, 16), TB2, 0).start()

        qa = (TB2 // 32) * 16
        q_part(lnr, 0, 0, qa)
        q_part(lnr, 0, qa, TB2 - qa)
        r0 = 0
        for n in OCH[:-1]:
            top1, top2 = ln2_part(o_part(r0, n), xr, l2r, outr, DEF + r0, row0, None, top1, top2, toks)
            r0 += n
        attn_v[...] = o_part(r0, DEF)
        return top1, top2

    init = jnp.full((8, 1), INT_MIN, I32)
    top1, top2 = lax.fori_loop(0, NB2, p2, (init, init))

    pltpu.make_async_copy(wgu_v, wgu_v, sems.at[SEM_WGU]).wait()
    wd_copy.wait()
    sub8 = lax.broadcasted_iota(I32, (8, LANES), 0)

    def submax(v):
        for sh in (4, 2, 1):
            v = jnp.maximum(v, pltpu.roll(v, sh, 0))
        return v

    def subsum(v):
        for sh in (4, 2, 1):
            v = v + pltpu.roll(v, sh, 0)
        return v

    def best2(t1, t2):
        t1 = jnp.broadcast_to(t1, (8, LANES))
        t2 = jnp.broadcast_to(t2, (8, LANES))
        k1v = submax(t1)
        return k1v, submax(jnp.where(t1 == k1v, t2, t1))

    def key_row(k):
        return 0xFFFF - (k & 0xFFFF)

    def wide(m):
        return jnp.concatenate([m] * NC, axis=1)

    def m_tile(c, k0, nk):
        w = jnp.concatenate([mp_v[c, d * PSTR:d * PSTR + H // 2, :] for d in range(k0 // H, (k0 + nk) // H)], axis=0)
        return pltpu.bitcast(w, BF16)

    toks = []
    top1, top2 = ln2_part(attn_v[...], x_v, ln2_v, out_v, L0, -DEF, None, top1, top2, toks, lag=LAG_L)
    out_copy(L0 - TB2, TB2, 0).start()
    oldk = best2(top1, top2)
    oldx = []
    for kk in oldk:
        g8 = pl.multiple_of(((key_row(kk[0, 0]) >> 3) << 3) + DEF, 8)
        rows = ln2_v[pl.ds(g8, 8), :].astype(F32)
        oldx.append(subsum(jnp.where(wide((key_row(kk) & 7) == sub8), rows, 0.0)))

    wrc = wr_row - jnp.sum(wr_row, axis=-1, keepdims=True) * (1.0 / D)
    uparts = []
    for k0 in range(0, D, LANES):
        mrows = jnp.concatenate([m_tile(c, k0, LANES) for c in range(NC)], axis=1).astype(F32)
        part = colsum(mrows * wrc)
        if uparts:
            tok = pltpu.bitcast(pltpu.bitcast(jnp.broadcast_to(uparts[-1], (8, LANES)), U32) & zero_u, F32)
            mrows = jnp.concatenate([mrows[:, 0:LANES] + jnp.concatenate([tok] * (LANES // 8), axis=0),
                                     mrows[:, LANES:]], axis=1)
            part = colsum(mrows * wrc)
        uparts.append(jnp.sum(part.T, axis=0, keepdims=True))
    urow = jnp.concatenate(uparts, axis=1)
    p1, p2_, r0 = init, init, 0
    for n in QS:
        p1, p2_ = q_part(ln1_v, L0, r0, n, (urow, wrc, p1, p2_))
        r0 += n

    cand_p, cand_x = [], []
    for pk_ in (p1, p2_):
        cp = jnp.zeros((8, D), F32)
        cx = jnp.zeros((8, D), F32)
        for s in range(8):
            row = key_row(pk_[s, 0])
            g8 = pl.multiple_of((row >> 3) << 3, 8)
            m = wide(sub8 == s)
            pair = jnp.broadcast_to(pqn_v[pl.ds((row - L0) >> 1, 1), :], (8, D))
            half = pair & jnp.uint32(0xFFFF0000) if s % 2 else pair << 16
            cp = jnp.where(m, pltpu.bitcast(half, F32), cp)
            cx = jnp.where(m, x_v[pl.ds(g8 + DEF, 8), :].astype(F32), cx)
        cand_p.append(cp)
        cand_x.append(cx)
    cand_p = jnp.concatenate(cand_p, axis=0).astype(BF16)
    cand_x = jnp.concatenate(cand_x, axis=0)
    ids_lo = key_row(jnp.broadcast_to(p1, (8, LANES)))
    ids_hi = jnp.where(sub8 < 6, key_row(jnp.broadcast_to(p2_, (8, LANES))),
                       jnp.where(sub8 == 6, key_row(oldk[0]), key_row(oldk[1])))

    st = dict(top1=top1, top2=top2, pend=[], step=0, sent=0)

    def gated(v):
        tok = None
        while st["pend"] and st["pend"][0][0] <= st["step"]:
            t = st["pend"].pop(0)[1]
            tok = t if tok is None else tok | t
        if tok is None:
            return v
        u = pltpu.bitcast(v, U32)
        return pltpu.bitcast(jnp.concatenate([u[:, 0:LANES] | tok, u[:, LANES:]], axis=1), BF16)

    def o_units():
        r0 = -OCL[0]
        for ci, n in enumerate(OCL):
            r0 += OCL[ci - 1] if ci else OCL[0]
            lhs = pltpu.bitcast(pqn_v[r0 // 2:(r0 + n) // 2, :], BF16)
            halves = []
            for c0 in range(0, NC, ONT):
                acc = x_v[DEF + L0 + r0:DEF + L0 + r0 + n, c0 * LANES:(c0 + ONT) * LANES].astype(F32)
                ks = (4 // ONT) * LANES
                for k0 in range(0, D, ks):
                    w = jnp.concatenate([m_tile(c, k0, ks) for c in range(c0, c0 + ONT)], axis=1)
                    acc = acc + jnp.dot(lhs[:, k0:k0 + ks], w, preferred_element_type=F32)
                    if k0 + ks == D:
                        halves.append(acc)
                        if len(halves) == NC // ONT:
                            last = r0 + n == RL
                            tk = [] if last else toks
                            st["top1"], st["top2"] = ln2_part(
                                jnp.concatenate(halves, axis=1), x_v, ln2_v, out_v, DEF + L0 + r0, -DEF, None,
                                st["top1"], st["top2"], tk, lag=n if last else LAG_L, is_h=True, fast=last)
                            if GLAG[ci] is not None:
                                st["pend"].append((st["step"] + GLAG[ci],
                                                   pltpu.bitcast(jnp.broadcast_to(st["top1"], (8, LANES)), U32) & zero_u))
                            if r0 + n in OUT_AT:
                                out_copy(L0 + st["sent"], r0 + n - st["sent"], 1).start()
                                st["sent"] = r0 + n
                    yield

    res = {}

    def c_units():
        parts = []
        for c in range(NC):
            parts.append(jnp.dot(cand_p, m_tile(c, 0, D), preferred_element_type=F32))
            yield
        xs = _layernorm(cand_x + jnp.concatenate(parts, axis=1))
        hi = jnp.where(wide(sub8 < 6), xs[8:16, :], jnp.where(wide(sub8 == 6), oldx[0], oldx[1]))
        res["xs"] = jnp.concatenate([xs[0:8, :], hi], axis=0).astype(BF16)

    def f_units():
        xs = res["xs"]
        acts = []
        for j in range(F // LANES):
            cs = slice(j * LANES, (j + 1) * LANES)
            g = jnp.dot(gated(xs), wload(wg_v, 0, D, cs), preferred_element_type=F32)
            yield
            u = jnp.dot(xs, wload(wu_v, 0, D, cs), preferred_element_type=F32)
            acts.append((g * jax.nn.sigmoid(g) * u).astype(BF16))
            yield
        ys = [None] * NC
        for c in range(NC):
            for k0 in range(0, F, D):
                nk = min(D, F - k0)
                a = jnp.concatenate(acts[k0 // LANES:(k0 + nk) // LANES], axis=1)
                p = jnp.dot(gated(a), wload(wd_v, k0, nk, slice(c * LANES, (c + 1) * LANES)),
                            preferred_element_type=F32)
                ys[c] = p if ys[c] is None else ys[c] + p
                yield
        res["y"] = jnp.concatenate(ys, axis=1)

    ou = o_units()

    def o_step():
        next(ou, None)
        st["step"] += 1

    for _ in range(NPRE):
        o_step()
    for _ in c_units():
        o_step()
    for _ in range(NGAP):
        o_step()
    for _ in f_units():
        o_step()
    for _ in ou:
        pass

    keyv = best2(st["top1"], st["top2"])
    idx = [key_row(kk[0, 0]) for kk in keyv]
    grp = [pl.multiple_of((ii >> 3) << 3, 8) for ii in idx]
    vgrp = [pl.multiple_of(gg + DEF, 8) for gg in grp]
    y = res["y"]
    hits = None
    yrows = []
    for c in range(2):
        m_lo = ids_lo == key_row(keyv[c])
        m_hi = ids_hi == key_row(keyv[c])
        yrows.append(subsum(jnp.where(wide(m_lo), y[0:8, :], 0.0) + jnp.where(wide(m_hi), y[8:16, :], 0.0)))
        hit = submax(jnp.where(m_lo | m_hi, 1, 0))
        hits = hit if hits is None else hits + hit
    hit_all = hits[0, 0] == 2

    tail0 = L0 + st["sent"]
    tail_copy = out_copy(tail0, S - tail0, 2) if tail0 < S else None
    fix_needed = (grp[0] < tail0, jnp.logical_and(grp[1] < tail0, grp[1] != grp[0]))

    def fix_copy(c):
        return out_copy(grp[c], 8, 3 + c)

    def finish(ysel):
        for c in range(2):
            hi = keyv[c] & jnp.int32(-65536)
            score = pltpu.bitcast(hi ^ ((hi >> 31) & 0x7FFF0000), F32)
            sel = (key_row(keyv[c]) & 7) == sub8
            upd = jnp.where(wide(sel), ysel[c] * wide(jax.nn.sigmoid(score)), 0.0)
            out_v[pl.ds(vgrp[c], 8), :] = (out_v[pl.ds(vgrp[c], 8), :].astype(F32) + upd).astype(BF16)
        if tail_copy is not None:
            tail_copy.start()
        for c in range(2):
            @pl.when(fix_needed[c])
            def _():
                fix_copy(c).start()

    out_copy(0, L0, 0).wait()
    out_copy(L0, tail0 - L0, 1).wait()

    @pl.when(hit_all)
    def _():
        finish(yrows)

    @pl.when(jnp.logical_not(hit_all))
    def _():
        xsel = jnp.concatenate([ln2_v[pl.ds(vgrp[c], 8), :] for c in range(2)], axis=0)

        def ffn_tile(j, acc):
            cs = pl.ds(pl.multiple_of(j * LANES, LANES), LANES)
            g = jnp.dot(xsel, wload(wg_v, 0, D, cs), preferred_element_type=F32)
            u = jnp.dot(xsel, wload(wu_v, 0, D, cs), preferred_element_type=F32)
            a = (g * jax.nn.sigmoid(g) * u).astype(BF16)
            wd_t = pltpu.bitcast(wd_v[pl.ds(pl.multiple_of(j * (LANES // 2), LANES // 2), LANES // 2), :], BF16)
            return acc + jnp.dot(a, wd_t, preferred_element_type=F32)

        yf = lax.fori_loop(0, F // LANES, ffn_tile, jnp.zeros((16, D), F32))
        finish([yf[0:8, :], yf[8:16, :]])

    if tail_copy is not None:
        tail_copy.wait()
    for c in range(2):
        @pl.when(fix_needed[c])
        def _():
            fix_copy(c).wait()


@jax.jit
def pallas_sequential_preLN__linear_attn_block__moe_arch_mod__prompt_kernel(
    A_x: jax.Array,
    A_wqkv: jax.Array,
    A_wo: jax.Array,
    B_x: jax.Array,
    B_w_r: jax.Array,
    B_w_gate: jax.Array,
    B_w_up: jax.Array,
    B_w_down: jax.Array,
):
    del B_x
    x = A_x.reshape(S, D)
    wr = B_w_r.reshape(NC, LANES)
    any_spec = pl.BlockSpec(memory_space=pl.ANY)
    out = pl.pallas_call(
        _kernel,
        out_shape=jax.ShapeDtypeStruct((S, D), BF16),
        in_specs=[any_spec] * 7,
        out_specs=any_spec,
        scratch_shapes=[
            pltpu.VMEM((S + DEF, D), BF16),
            pltpu.VMEM((D // 2, D), U32),
            pltpu.VMEM((3, D // 2, D), U32),
            pltpu.VMEM((NC, LANES), BF16),
            pltpu.VMEM((2, D // 2, F), U32),
            pltpu.VMEM((F // 2, D), U32),
            pltpu.VMEM(((S + TB) // 2, D), U32),
            pltpu.VMEM((D // 2, max(TB, P0)), U32),
            pltpu.VMEM((H * ZP, LANES), F32),
            pltpu.VMEM((D, D), F32),
            pltpu.VMEM((NC, DH * PSTR, LANES), U32),
            pltpu.VMEM((NC, DH * PSTR, LANES), U32),
            pltpu.VMEM((max(TB2, RL) // 2, D), U32),
            pltpu.VMEM((DEF, D), F32),
            pltpu.VMEM((2, S + DEF, D), BF16),
            pltpu.VMEM((8, LANES), U32),
            pltpu.SemaphoreType.DMA((NSEM,)),
        ],
        compiler_params=pltpu.CompilerParams(vmem_limit_bytes=110 * 1024 * 1024, **CPX),
    )(x, A_wqkv, A_wo, wr, B_w_gate, B_w_up, B_w_down)
    return out.reshape(1, S, D)
```

```python
import jax
import jax.numpy as jnp
from jax import lax
import jax.experimental.pallas as pl
import jax.experimental.pallas.tpu as pltpu

S = 2048
D = 1024
F = 3584
H = 32
DH = D // H
LANES = 128
NC = D // LANES

P0 = 512
TB = 384
NB1 = (S - P0) // TB
TX = 256
TB2 = 544
NB2 = 3
L0 = NB2 * TB2
RL = S - L0
OCL = (32, 64, 64, 64, 64, 64, 64)
QS = (224, 128, 64)
ONT = 2
NPRE = 20
NGAP = 7
GLAG = (None, None, None, None, None, 20, 8)
LAG_L = 3
OUT_AT = (160, 288, 352)
OCH = (64, 64, 64, 64, 64, 64, 64, 32, 64)
DEF = OCH[-1]
LNU = 8
LAG = 5
L1U = 8
L1LAG = 2
L1LAG0 = 4
ZP = 36
KVLAG = 1
KVGATE = ((), (), (0,), (1,), (2,), (3,), (4,), (5,))
MGATE = ((), (), (), (), (), (), (6,), (7,))
PSTR = 20

F32 = jnp.float32
BF16 = jnp.bfloat16
U32 = jnp.uint32
I32 = jnp.int32

XP = ((0, 128), (128, 128), (256, 768), (1024, 1024))
WKP = ((0, 128), (128, 128), (256, 256), (512, 512))

SEM_X = 0
SEM_WK = SEM_X + len(XP)
SEM_W3 = SEM_WK + len(WKP)
SEM_WR = SEM_W3 + 1
SEM_WGU = SEM_WR + 1
SEM_WD = SEM_WGU + 1
SEM_OUT = SEM_WD + 1
NSEM = SEM_OUT + 5

INT_MIN = -(2 ** 31)
CPX = dict(disable_bounds_checks=True, disable_semaphore_checks=True)


def _layernorm(x, tok=None, w=None):
    s0 = x[:, 0:LANES]
    if tok is not None:
        s0 = s0 + jnp.concatenate([tok] * (x.shape[0] // 8), axis=0)
    for c in range(1, NC):
        s0 = s0 + x[:, c * LANES:(c + 1) * LANES]
    mu = jnp.sum(s0, axis=-1, keepdims=True) * (1.0 / D)
    xc = x - mu
    var = jnp.sum(xc * xc, axis=-1, keepdims=True) * (1.0 / D)
    rstd = lax.rsqrt(var + 1e-5)
    if w is None:
        return xc * rstd
    return xc * rstd, jnp.sum(xc * w, axis=-1, keepdims=True) * rstd


def _phi(t):
    return jnp.where(t > 0, t + 1.0, jnp.exp(t)) + 1e-6


def _pack_rows(a, b):
    return (pltpu.bitcast(a, U32) >> 16) | pltpu.bitcast(b, U32)


def _load_packed(ref):
    cols = []
    for c in range(NC):
        w = jnp.concatenate([ref[c, d * PSTR:d * PSTR + H // 2, :] for d in range(DH)], axis=0)
        cols.append(pltpu.bitcast(w, BF16))
    return jnp.concatenate(cols, axis=1)


def _store_interleaved(ref, val, head0):
    acc = None
    for hp in range(val.shape[0] // (2 * DH)):
        w = _pack_rows(val[hp * 2 * DH:hp * 2 * DH + DH, :], val[hp * 2 * DH + DH:(hp + 1) * 2 * DH, :])
        for c in range(NC):
            ref[c, pl.ds(head0 // 2 + hp, DH, stride=PSTR), :] = w[:, c * LANES:(c + 1) * LANES]
            for g in range(DH // 8):
                piece = w[g * 8:(g + 1) * 8, c * LANES:(c + 1) * LANES]
                acc = piece if acc is None else acc | piece
    return acc


def _kernel(x_hbm, wqkv_hbm, wo_hbm, wr_hbm, wg_hbm, wu_hbm, wd_hbm, out_hbm,
            x_v, wk_v, w3_v, wr_v, wgu_v, wd_v,
            ln1_v, pkt_v, zacc_v, g_v, wqp_v, mp_v, pqn_v, attn_v, lo_v, zero_v, sems):

    ln2_v, out_v = lo_v.at[0], lo_v.at[1]

    wqkv_hbm, wo_hbm, wg_hbm, wu_hbm, wd_hbm = (r.bitcast(U32) for r in (wqkv_hbm, wo_hbm, wg_hbm, wu_hbm, wd_hbm))

    def wload(ref, r0, nr, cols):
        rows = pl.ds(r0 // 2, nr // 2) if isinstance(r0, int) else pl.ds(pl.multiple_of(r0 // 2, nr // 2), nr // 2)
        return pltpu.bitcast(ref[rows, cols], BF16)

    wq_v, wv_v, wo_v = w3_v.at[0], w3_v.at[1], w3_v.at[2]
    wg_v, wu_v = wgu_v.at[0], wgu_v.at[1]

    def x_copy(i):
        r0, n = XP[i]
        return pltpu.make_async_copy(x_hbm.at[pl.ds(r0, n), :], x_v.at[pl.ds(DEF + r0, n), :], sems.at[SEM_X + i])

    def out_copy(r0, n, s):
        return pltpu.make_async_copy(out_v.at[pl.ds(DEF + r0, n), :], out_hbm.at[pl.ds(r0, n), :],
                                     sems.at[SEM_OUT + s])

    def wk_copy(j):
        c0, n = WKP[j]
        return pltpu.make_async_copy(wqkv_hbm.at[:, pl.ds(D + c0, n)], wk_v.at[:, pl.ds(c0, n)],
                                     sems.at[SEM_WK + j])

    wr_copy = pltpu.make_async_copy(wr_hbm, wr_v, sems.at[SEM_WR])
    wd_copy = pltpu.make_async_copy(wd_hbm, wd_v, sems.at[SEM_WD])

    x_copy(0).start()
    wk_copy(0).start()
    x_copy(1).start()
    wr_copy.start()
    for j in range(1, len(WKP)):
        wk_copy(j).start()
    x_copy(2).start()
    x_copy(3).start()
    pltpu.make_async_copy(wqkv_hbm.at[:, pl.ds(0, D)], wq_v, sems.at[SEM_W3]).start()
    pltpu.make_async_copy(wqkv_hbm.at[:, pl.ds(2 * D, D)], wv_v, sems.at[SEM_W3]).start()
    pltpu.make_async_copy(wo_hbm, wo_v, sems.at[SEM_W3]).start()
    pltpu.make_async_copy(wg_hbm, wg_v, sems.at[SEM_WGU]).start()
    pltpu.make_async_copy(wu_hbm, wu_v, sems.at[SEM_WGU]).start()
    wd_copy.start()

    def ln1_rows(xr, xr0, lnr, r0, n):
        ln = _layernorm(xr[xr0:xr0 + n, :].astype(F32)).astype(BF16)
        lnr[r0 // 2:(r0 + n) // 2, :] = pltpu.bitcast(ln, U32)

    def ln1_rows_paced(xr, xr0, lnr, r0, n, L1LAG=L1LAG):
        zero_u = zero_v[...]
        toks = []
        lns = []
        for j in range(n // L1U):
            x = xr[xr0 + j * L1U:xr0 + (j + 1) * L1U, :].astype(F32)
            tok = toks[-L1LAG] if len(toks) >= L1LAG else None
            ln = _layernorm(x, tok)
            toks.append(pltpu.bitcast(pltpu.bitcast(ln[L1U - 8:L1U, 0:LANES], U32) & zero_u, F32))
            lns.append(ln)
            if (j + 1) * L1U % 16 == 0:
                grp = jnp.concatenate(lns, axis=0).astype(BF16)
                e = r0 + (j + 1) * L1U
                lnr[(e - grp.shape[0]) // 2:e // 2, :] = pltpu.bitcast(grp, U32)
                lns = []

    def ln1_load(lnr, r0, n):
        return pltpu.bitcast(lnr[r0 // 2:(r0 + n) // 2, :], BF16)

    def k_mm(lnr, r0, n, c0, nc):
        return jnp.dot(ln1_load(lnr, r0, n), wload(wk_v, 0, D, slice(c0, c0 + nc)), preferred_element_type=F32)

    def k_post(k, p0, c0, first=False):
        n, nc = k.shape
        pkt = _phi(k).T
        pkt_v[c0 // 2:(c0 + nc) // 2, p0:p0 + n] = pltpu.bitcast(pkt.astype(BF16), U32)
        zs = pkt[:, 0:LANES]
        for j in range(1, n // LANES):
            zs = zs + pkt[:, j * LANES:(j + 1) * LANES]
        for hh in range(nc // DH):
            z0 = (c0 // DH + hh) * ZP
            if first:
                zacc_v[z0:z0 + DH, :] = zs[hh * DH:(hh + 1) * DH, :]
            else:
                zacc_v[z0:z0 + DH, :] += zs[hh * DH:(hh + 1) * DH, :]

    def g_acc(lnr, r0, n, c0, nc, first=False):
        g = jnp.dot(pltpu.bitcast(pkt_v[c0 // 2:(c0 + nc) // 2, r0:r0 + n], BF16), ln1_load(lnr, r0, n),
                    preferred_element_type=F32)
        if first:
            g_v[c0:c0 + nc, :] = g
        else:
            g_v[c0:c0 + nc, :] += g

    attn_v[...] = jnp.zeros_like(attn_v)
    x_v[0:DEF, :] = jnp.zeros((DEF, D), BF16)
    zero_v[...] = jnp.zeros_like(zero_v)

    def k0(c0, nc):
        k_post(k_mm(ln1_v, 0, TX, c0, nc), 0, c0, first=True)

    def g0(c0, nc):
        g_acc(ln1_v, 0, TX, c0, nc, first=True)

    x_copy(0).wait()
    ln1_rows(x_v, DEF, ln1_v, 0, 128)
    wk_copy(0).wait()
    ka = k_mm(ln1_v, 0, 128, 0, 128)
    x_copy(1).wait()
    wr_copy.wait()
    ln1_rows(x_v, DEF + 128, ln1_v, 128, 128)
    k_post(ka, 0, 0, first=True)
    g_acc(ln1_v, 0, 128, 0, 128, first=True)
    wk_copy(1).wait()
    k_post(k_mm(ln1_v, 128, 128, 0, 128), 128, 0)
    k0(128, 128)
    g_acc(ln1_v, 128, 128, 0, 128)
    wk_copy(2).wait()
    k0(256, 256)
    g0(128, 128)
    g0(256, 256)
    wk_copy(3).wait()
    k0(512, 256)
    k0(768, 256)
    g0(512, 256)
    x_copy(2).wait()
    ln1_rows(x_v, DEF + TX, ln1_v, TX, TX)
    g0(768, 256)
    HD = D // 2
    k_post(k_mm(ln1_v, TX, TX, 0, HD), TX, 0)
    k_post(k_mm(ln1_v, TX, TX, HD, HD), TX, HD)
    ln1_rows_paced(x_v, DEF + P0, ln1_v, P0, TB, L1LAG0)
    g_acc(ln1_v, TX, TX, 0, HD)
    g_acc(ln1_v, TX, TX, HD, HD)

    def p1(i, carry):
        lnr = ln1_v.at[pl.ds(pl.multiple_of(P0 // 2 + i * (TB // 2), 64), TB), :]
        xr = x_v.at[pl.ds(pl.multiple_of(P0 + jnp.minimum(i + 1, NB1 - 1) * TB, 128), TB + DEF), :]
        k_post(k_mm(lnr, 0, TB, 0, HD), 0, 0)
        k_post(k_mm(lnr, 0, TB, HD, HD), 0, HD)
        ln1_rows_paced(xr, DEF, lnr, TB, TB)
        g_acc(lnr, 0, TB, 0, HD)
        g_acc(lnr, 0, TB, HD, HD)
        return carry

    x_copy(3).wait()
    lax.fori_loop(0, NB1, p1, 0)

    pltpu.make_async_copy(w3_v, w3_v, sems.at[SEM_W3]).wait()
    zero_u = zero_v[...]
    wtok = []
    for c in range(NC):
        wtok.append(zero_u & _store_interleaved(wqp_v, wload(wq_v, 0, D, slice(c * LANES, (c + 1) * LANES)).astype(F32).T,
                                                c * (LANES // DH)))
    zp = jnp.concatenate([zacc_v[pl.ds(d, H, stride=ZP), :] for d in range(DH)], axis=0)
    zrow = jnp.sum(zp.T, axis=0, keepdims=True)
    wr8 = wr_v[...].astype(F32)
    wr_row = jnp.concatenate([wr8[c:c + 1, :] for c in range(NC)], axis=1)

    row_h = lax.broadcasted_iota(I32, (LANES, LANES), 0) // DH
    col_h = lax.broadcasted_iota(I32, (LANES, LANES), 1) // DH
    diag = row_h == col_h
    def kv_part(c):
        cs = slice(c * LANES, (c + 1) * LANES)
        gb = g_v[cs, :]
        tk = None
        for cc in KVGATE[c]:
            tk = wtok[cc] if tk is None else tk | wtok[cc]
        if tk is not None:
            gb = jnp.concatenate([jnp.concatenate([gb[0:8, 0:LANES] + pltpu.bitcast(tk, F32), gb[0:8, LANES:]], axis=1),
                                  gb[8:, :]], axis=0)
        kv = jnp.dot(gb.astype(BF16), wload(wv_v, 0, D, cs), preferred_element_type=F32)
        return jnp.where(diag, kv, 0.0)

    def m_part(c, kv):
        cs = slice(c * LANES, (c + 1) * LANES)
        tk = None
        for cc in MGATE[c]:
            tk = wtok[cc] if tk is None else tk | wtok[cc]
        if tk is not None:
            kv = jnp.concatenate([kv[0:8, :] + pltpu.bitcast(tk, F32), kv[8:, :]], axis=0)
        m = jnp.dot(kv.astype(BF16), wload(wo_v, c * LANES, LANES, slice(None)), preferred_element_type=F32)
        _store_interleaved(mp_v, m.astype(BF16).astype(F32), c * (LANES // DH))

    kvs = {}
    for c in range(NC + KVLAG):
        if c < NC:
            kvs[c] = kv_part(c)
        if c >= KVLAG:
            m_part(c - KVLAG, kvs[c - KVLAG])

    def make_key(score, row):
        b = pltpu.bitcast(score, I32)
        srt = b ^ ((b >> 31) & 0x7FFFFFFF)
        return (srt & jnp.int32(-65536)) | (0xFFFF - row)

    def push_keys(key, top1, top2):
        for gidx in range(key.shape[0] // 8):
            kx = key[gidx * 8:(gidx + 1) * 8, :]
            top2 = jnp.maximum(top2, jnp.minimum(top1, kx))
            top1 = jnp.maximum(top1, kx)
        return top1, top2

    def colsum(t):
        acc = t[:, 0:LANES]
        for c in range(1, NC):
            acc = acc + t[:, c * LANES:(c + 1) * LANES]
        return acc

    def q_part(lnr, l0, r0, n, hint=None):
        q = lax.dot_general(ln1_load(lnr, l0 + r0, n), _load_packed(wqp_v),
                            (((1,), (1,)), ((), ())), preferred_element_type=F32)
        pq = _phi(q)
        den = colsum(pq * zrow)
        den = den + pltpu.roll(den, DH, 1)
        den = den + pltpu.roll(den, 2 * DH, 1)
        inv = 1.0 / (den + 1e-6)
        pqn = pq * jnp.concatenate([inv] * NC, axis=1)
        pqn_v[r0 // 2:(r0 + n) // 2, :] = pltpu.bitcast(pqn.astype(BF16), U32)
        if hint is None:
            return None
        urow, wrc, p1, p2 = hint
        xb = x_v[DEF + l0 + r0:DEF + l0 + r0 + n, :].astype(F32)
        num = jnp.sum(colsum(xb * wrc) + colsum(pq * urow) * inv, axis=-1, keepdims=True)
        return push_keys(make_key(num, (l0 + r0) + lax.broadcasted_iota(I32, (n, 1), 0)), p1, p2)

    def o_part(r0, n):
        return jnp.dot(pltpu.bitcast(pqn_v[r0 // 2:(r0 + n) // 2, :], BF16), _load_packed(mp_v),
                       preferred_element_type=F32)

    def ln2_unit(attn, xr, l2r, outr, r0, row0, valid, top1, top2, tok, fast=False, is_h=False):
        n = attn.shape[0]
        h = attn if is_h else xr[r0:r0 + n, :].astype(F32) + attn
        if fast:
            ln2, r = _layernorm(h, tok, wr_row)
        else:
            ln2 = _layernorm(h, tok)
            r = jnp.sum(ln2 * wr_row, axis=-1, keepdims=True)
        l2r[r0:r0 + n, :] = ln2.astype(BF16)
        res = h + ln2
        outr[r0:r0 + n, :] = res.astype(BF16)
        r = r.astype(BF16).astype(F32) + 0.0
        key = make_key(r, (row0 + r0) + lax.broadcasted_iota(I32, (n, 1), 0))
        if valid is not None:
            key = jnp.where(valid, key, INT_MIN)
        top1, top2 = push_keys(key, top1, top2)
        ntok = pltpu.bitcast(pltpu.bitcast(jnp.broadcast_to(r[n - 8:n, :], (8, LANES)), U32) & zero_u, F32)
        return top1, top2, ntok

    def ln2_part(attn, xr, l2r, outr, r0, row0, valid, top1, top2, toks, lag=LAG, **kw):
        n = attn.shape[0]
        u = min(LNU, n)
        for j in range(n // u):
            tok = toks[-lag] if len(toks) >= lag else None
            top1, top2, tok = ln2_unit(attn[j * u:(j + 1) * u, :], xr, l2r, outr, r0 + j * u, row0, valid,
                                       top1, top2, tok, **kw)
            toks.append(tok)
        return top1, top2

    def p2(i, carry):
        top1, top2 = carry
        b0 = pl.multiple_of(i * TB2, 16)
        lnr = ln1_v.at[pl.ds(pl.multiple_of(i * (TB2 // 2), 8), TB2 // 2), :]
        xr = x_v.at[pl.ds(b0, TB2 + DEF), :]
        l2r = ln2_v.at[pl.ds(b0, TB2 + DEF), :]
        outr = out_v.at[pl.ds(b0, TB2 + DEF), :]
        row0 = b0 - DEF
        toks = []
        top1, top2 = ln2_part(attn_v[...], xr, l2r, outr, 0, row0, i > 0, top1, top2, toks)

        @pl.when(i > 0)
        def _():
            out_copy(pl.multiple_of((i - 1) * TB2, 16), TB2, 0).start()

        qa = (TB2 // 32) * 16
        q_part(lnr, 0, 0, qa)
        q_part(lnr, 0, qa, TB2 - qa)
        r0 = 0
        for n in OCH[:-1]:
            top1, top2 = ln2_part(o_part(r0, n), xr, l2r, outr, DEF + r0, row0, None, top1, top2, toks)
            r0 += n
        attn_v[...] = o_part(r0, DEF)
        return top1, top2

    init = jnp.full((8, 1), INT_MIN, I32)
    top1, top2 = lax.fori_loop(0, NB2, p2, (init, init))

    pltpu.make_async_copy(wgu_v, wgu_v, sems.at[SEM_WGU]).wait()
    wd_copy.wait()
    sub8 = lax.broadcasted_iota(I32, (8, LANES), 0)

    def submax(v):
        for sh in (4, 2, 1):
            v = jnp.maximum(v, pltpu.roll(v, sh, 0))
        return v

    def subsum(v):
        for sh in (4, 2, 1):
            v = v + pltpu.roll(v, sh, 0)
        return v

    def best2(t1, t2):
        t1 = jnp.broadcast_to(t1, (8, LANES))
        t2 = jnp.broadcast_to(t2, (8, LANES))
        k1v = submax(t1)
        return k1v, submax(jnp.where(t1 == k1v, t2, t1))

    def key_row(k):
        return 0xFFFF - (k & 0xFFFF)

    def wide(m):
        return jnp.concatenate([m] * NC, axis=1)

    def m_tile(c, k0, nk):
        w = jnp.concatenate([mp_v[c, d * PSTR:d * PSTR + H // 2, :] for d in range(k0 // H, (k0 + nk) // H)], axis=0)
        return pltpu.bitcast(w, BF16)

    toks = []
    top1, top2 = ln2_part(attn_v[...], x_v, ln2_v, out_v, L0, -DEF, None, top1, top2, toks, lag=LAG_L)
    out_copy(L0 - TB2, TB2, 0).start()
    oldk = best2(top1, top2)
    oldx = []
    for kk in oldk:
        g8 = pl.multiple_of(((key_row(kk[0, 0]) >> 3) << 3) + DEF, 8)
        rows = ln2_v[pl.ds(g8, 8), :].astype(F32)
        oldx.append(subsum(jnp.where(wide((key_row(kk) & 7) == sub8), rows, 0.0)))

    wrc = wr_row - jnp.sum(wr_row, axis=-1, keepdims=True) * (1.0 / D)
    uparts = []
    for k0 in range(0, D, LANES):
        mrows = jnp.concatenate([m_tile(c, k0, LANES) for c in range(NC)], axis=1).astype(F32)
        part = colsum(mrows * wrc)
        if uparts:
            tok = pltpu.bitcast(pltpu.bitcast(jnp.broadcast_to(uparts[-1], (8, LANES)), U32) & zero_u, F32)
            mrows = jnp.concatenate([mrows[:, 0:LANES] + jnp.concatenate([tok] * (LANES // 8), axis=0),
                                     mrows[:, LANES:]], axis=1)
            part = colsum(mrows * wrc)
        uparts.append(jnp.sum(part.T, axis=0, keepdims=True))
    urow = jnp.concatenate(uparts, axis=1)
    p1, p2_, r0 = init, init, 0
    for n in QS:
        p1, p2_ = q_part(ln1_v, L0, r0, n, (urow, wrc, p1, p2_))
        r0 += n

    cand_p, cand_x = [], []
    for pk_ in (p1, p2_):
        cp = jnp.zeros((8, D), F32)
        cx = jnp.zeros((8, D), F32)
        for s in range(8):
            row = key_row(pk_[s, 0])
            g8 = pl.multiple_of((row >> 3) << 3, 8)
            m = wide(sub8 == s)
            pair = jnp.broadcast_to(pqn_v[pl.ds((row - L0) >> 1, 1), :], (8, D))
            half = pair & jnp.uint32(0xFFFF0000) if s % 2 else pair << 16
            cp = jnp.where(m, pltpu.bitcast(half, F32), cp)
            cx = jnp.where(m, x_v[pl.ds(g8 + DEF, 8), :].astype(F32), cx)
        cand_p.append(cp)
        cand_x.append(cx)
    cand_p = jnp.concatenate(cand_p, axis=0).astype(BF16)
    cand_x = jnp.concatenate(cand_x, axis=0)
    ids_lo = key_row(jnp.broadcast_to(p1, (8, LANES)))
    ids_hi = jnp.where(sub8 < 6, key_row(jnp.broadcast_to(p2_, (8, LANES))),
                       jnp.where(sub8 == 6, key_row(oldk[0]), key_row(oldk[1])))

    st = dict(top1=top1, top2=top2, pend=[], step=0, sent=0)

    def gated(v):
        tok = None
        while st["pend"] and st["pend"][0][0] <= st["step"]:
            t = st["pend"].pop(0)[1]
            tok = t if tok is None else tok | t
        if tok is None:
            return v
        u = pltpu.bitcast(v, U32)
        return pltpu.bitcast(jnp.concatenate([u[:, 0:LANES] | tok, u[:, LANES:]], axis=1), BF16)

    def o_units():
        r0 = -OCL[0]
        for ci, n in enumerate(OCL):
            r0 += OCL[ci - 1] if ci else OCL[0]
            lhs = pltpu.bitcast(pqn_v[r0 // 2:(r0 + n) // 2, :], BF16)
            halves = []
            for c0 in range(0, NC, ONT):
                acc = x_v[DEF + L0 + r0:DEF + L0 + r0 + n, c0 * LANES:(c0 + ONT) * LANES].astype(F32)
                ks = (4 // ONT) * LANES
                for k0 in range(0, D, ks):
                    w = jnp.concatenate([m_tile(c, k0, ks) for c in range(c0, c0 + ONT)], axis=1)
                    acc = acc + jnp.dot(lhs[:, k0:k0 + ks], w, preferred_element_type=F32)
                    if k0 + ks == D:
                        halves.append(acc)
                        if len(halves) == NC // ONT:
                            last = r0 + n == RL
                            tk = [] if last else toks
                            st["top1"], st["top2"] = ln2_part(
                                jnp.concatenate(halves, axis=1), x_v, ln2_v, out_v, DEF + L0 + r0, -DEF, None,
                                st["top1"], st["top2"], tk, lag=n if last else LAG_L, is_h=True, fast=last)
                            if GLAG[ci] is not None:
                                st["pend"].append((st["step"] + GLAG[ci],
                                                   pltpu.bitcast(jnp.broadcast_to(st["top1"], (8, LANES)), U32) & zero_u))
                            if last:
                                out_copy(L0 + st["sent"], r0 + n - st["sent"], 2).start()
                            elif r0 + n in OUT_AT:
                                out_copy(L0 + st["sent"], r0 + n - st["sent"], 1).start()
                                st["sent"] = r0 + n
                    yield

    res = {}

    def c_units():
        parts = []
        for c in range(NC):
            parts.append(jnp.dot(cand_p, m_tile(c, 0, D), preferred_element_type=F32))
            yield
        xs = _layernorm(cand_x + jnp.concatenate(parts, axis=1))
        hi = jnp.where(wide(sub8 < 6), xs[8:16, :], jnp.where(wide(sub8 == 6), oldx[0], oldx[1]))
        res["xs"] = jnp.concatenate([xs[0:8, :], hi], axis=0).astype(BF16)

    def f_units():
        xs = res["xs"]
        acts = []
        for j in range(F // LANES):
            cs = slice(j * LANES, (j + 1) * LANES)
            g = jnp.dot(gated(xs), wload(wg_v, 0, D, cs), preferred_element_type=F32)
            yield
            u = jnp.dot(xs, wload(wu_v, 0, D, cs), preferred_element_type=F32)
            acts.append((g * jax.nn.sigmoid(g) * u).astype(BF16))
            yield
        act = jnp.concatenate(acts, axis=1)
        zf = pltpu.bitcast(zero_u, F32)
        ys = []
        KF = (F // D) * D
        for c in range(0, NC, 2):
            acc = jnp.concatenate([jnp.concatenate([zf, zf], axis=0)] * 2, axis=1)
            acc = acc + jnp.dot(gated(act[:, KF:]), wload(wd_v, KF, F - KF, slice(c * LANES, (c + 2) * LANES)),
                                preferred_element_type=F32)
            yield
            for cc in range(2):
                y = acc[:, cc * LANES:(cc + 1) * LANES]
                for k0 in range(0, KF, D):
                    y = y + jnp.dot(gated(act[:, k0:k0 + D]),
                                    wload(wd_v, k0, D, slice((c + cc) * LANES, (c + cc + 1) * LANES)),
                                    preferred_element_type=F32)
                    yield
                ys.append(y)
        res["y"] = jnp.concatenate(ys, axis=1)

    ou = o_units()

    def o_step():
        next(ou, None)
        st["step"] += 1

    for _ in range(NPRE):
        o_step()
    for _ in c_units():
        o_step()
    for _ in range(NGAP):
        o_step()
    for _ in f_units():
        o_step()
    for _ in ou:
        pass

    keyv = best2(st["top1"], st["top2"])
    idx = [key_row(kk[0, 0]) for kk in keyv]
    grp = [pl.multiple_of((ii >> 3) << 3, 8) for ii in idx]
    vgrp = [pl.multiple_of(gg + DEF, 8) for gg in grp]
    y = res["y"]
    hits = None
    yrows = []
    for c in range(2):
        m_lo = ids_lo == key_row(keyv[c])
        m_hi = ids_hi == key_row(keyv[c])
        yrows.append(subsum(jnp.where(wide(m_lo), y[0:8, :], 0.0) + jnp.where(wide(m_hi), y[8:16, :], 0.0)))
        hit = submax(jnp.where(m_lo | m_hi, 1, 0))
        hits = hit if hits is None else hits + hit
    hit_all = hits[0, 0] == 2

    tail0 = L0 + st["sent"]
    tail_copy = out_copy(tail0, S - tail0, 2)
    in_tail = jnp.maximum(grp[0], grp[1]) >= tail0
    two_groups = grp[1] != grp[0]

    def fix_copy(c):
        return out_copy(grp[c], 8, 3 + c)

    def finish(ysel):
        for c in range(2):
            hi = keyv[c] & jnp.int32(-65536)
            score = pltpu.bitcast(hi ^ ((hi >> 31) & 0x7FFF0000), F32)
            sel = (key_row(keyv[c]) & 7) == sub8
            upd = jnp.where(wide(sel), ysel[c] * wide(jax.nn.sigmoid(score)), 0.0)
            out_v[pl.ds(vgrp[c], 8), :] = (out_v[pl.ds(vgrp[c], 8), :].astype(F32) + upd).astype(BF16)
        fix_copy(0).start()

        @pl.when(two_groups)
        def _():
            fix_copy(1).start()

    out_copy(0, L0, 0).wait()
    out_copy(L0, tail0 - L0, 1).wait()

    @pl.when(in_tail)
    def _():
        tail_copy.wait()

    @pl.when(hit_all)
    def _():
        finish(yrows)

    @pl.when(jnp.logical_not(hit_all))
    def _():
        xsel = jnp.concatenate([ln2_v[pl.ds(vgrp[c], 8), :] for c in range(2)], axis=0)

        def ffn_tile(j, acc):
            cs = pl.ds(pl.multiple_of(j * LANES, LANES), LANES)
            g = jnp.dot(xsel, wload(wg_v, 0, D, cs), preferred_element_type=F32)
            u = jnp.dot(xsel, wload(wu_v, 0, D, cs), preferred_element_type=F32)
            a = (g * jax.nn.sigmoid(g) * u).astype(BF16)
            wd_t = pltpu.bitcast(wd_v[pl.ds(pl.multiple_of(j * (LANES // 2), LANES // 2), LANES // 2), :], BF16)
            return acc + jnp.dot(a, wd_t, preferred_element_type=F32)

        yf = lax.fori_loop(0, F // LANES, ffn_tile, jnp.zeros((16, D), F32))
        finish([yf[0:8, :], yf[8:16, :]])

    @pl.when(jnp.logical_not(in_tail))
    def _():
        tail_copy.wait()

    fix_copy(0).wait()

    @pl.when(two_groups)
    def _():
        fix_copy(1).wait()


@jax.jit
def pallas_sequential_preLN__linear_attn_block__moe_arch_mod__prompt_kernel(
    A_x: jax.Array,
    A_wqkv: jax.Array,
    A_wo: jax.Array,
    B_x: jax.Array,
    B_w_r: jax.Array,
    B_w_gate: jax.Array,
    B_w_up: jax.Array,
    B_w_down: jax.Array,
):
    del B_x
    x = A_x.reshape(S, D)
    wr = B_w_r.reshape(NC, LANES)
    any_spec = pl.BlockSpec(memory_space=pl.ANY)
    out = pl.pallas_call(
        _kernel,
        out_shape=jax.ShapeDtypeStruct((S, D), BF16),
        in_specs=[any_spec] * 7,
        out_specs=any_spec,
        scratch_shapes=[
            pltpu.VMEM((S + DEF, D), BF16),
            pltpu.VMEM((D // 2, D), U32),
            pltpu.VMEM((3, D // 2, D), U32),
            pltpu.VMEM((NC, LANES), BF16),
            pltpu.VMEM((2, D // 2, F), U32),
            pltpu.VMEM((F // 2, D), U32),
            pltpu.VMEM(((S + TB) // 2, D), U32),
            pltpu.VMEM((D // 2, max(TB, P0)), U32),
            pltpu.VMEM((H * ZP, LANES), F32),
            pltpu.VMEM((D, D), F32),
            pltpu.VMEM((NC, DH * PSTR, LANES), U32),
            pltpu.VMEM((NC, DH * PSTR, LANES), U32),
            pltpu.VMEM((max(TB2, RL) // 2, D), U32),
            pltpu.VMEM((DEF, D), F32),
            pltpu.VMEM((2, S + DEF, D), BF16),
            pltpu.VMEM((8, LANES), U32),
            pltpu.SemaphoreType.DMA((NSEM,)),
        ],
        compiler_params=pltpu.CompilerParams(vmem_limit_bytes=110 * 1024 * 1024, **CPX),
    )(x, A_wqkv, A_wo, wr, B_w_gate, B_w_up, B_w_down)
    return out.reshape(1, S, D)
```

```python
import jax
import jax.numpy as jnp
from jax import lax
import jax.experimental.pallas as pl
import jax.experimental.pallas.tpu as pltpu

S = 2048
D = 1024
F = 3584
H = 32
DH = D // H
LANES = 128
NC = D // LANES

P0 = 512
TB = 384
NB1 = (S - P0) // TB
TX = 256
TB2 = 544
NB2 = 3
L0 = NB2 * TB2
RL = S - L0
OCL = (32, 64, 64, 64, 64, 64, 64)
QS = (224, 128, 64)
ONT = 2
NPRE = 20
NGAP = 7
GLAG = (None, None, None, None, None, 20, 8)
LAG_L = 3
OUT_AT = (160, 288, 352)
OCH = (64, 64, 64, 64, 64, 64, 64, 32, 64)
DEF = OCH[-1]
LNU = 8
LAG = 5
L1U = 8
L1LAG = 2
L1LAG0 = 3
ZP = 36
KVLAG = 1
KVGATE = ((), (), (0,), (1,), (2,), (3,), (4,), (5,))
MGATE = ((), (), (), (), (), (), (6,), (7,))
PSTR = 20

F32 = jnp.float32
BF16 = jnp.bfloat16
U32 = jnp.uint32
I32 = jnp.int32

XP = ((0, 128), (128, 128), (256, 768), (1024, 1024))
WKP = ((0, 128), (128, 128), (256, 256), (512, 512))

SEM_X = 0
SEM_WK = SEM_X + len(XP)
SEM_W3 = SEM_WK + len(WKP)
SEM_WR = SEM_W3 + 1
SEM_WGU = SEM_WR + 1
SEM_WD = SEM_WGU + 1
SEM_OUT = SEM_WD + 1
NSEM = SEM_OUT + 5

INT_MIN = -(2 ** 31)
CPX = dict(disable_bounds_checks=True, disable_semaphore_checks=True)


def _layernorm(x, tok=None, w=None):
    s0 = x[:, 0:LANES]
    if tok is not None:
        s0 = s0 + jnp.concatenate([tok] * (x.shape[0] // 8), axis=0)
    for c in range(1, NC):
        s0 = s0 + x[:, c * LANES:(c + 1) * LANES]
    mu = jnp.sum(s0, axis=-1, keepdims=True) * (1.0 / D)
    xc = x - mu
    var = jnp.sum(xc * xc, axis=-1, keepdims=True) * (1.0 / D)
    rstd = lax.rsqrt(var + 1e-5)
    if w is None:
        return xc * rstd
    return xc * rstd, jnp.sum(xc * w, axis=-1, keepdims=True) * rstd


def _phi(t):
    return jnp.where(t > 0, t + 1.0, jnp.exp(t)) + 1e-6


def _pack_rows(a, b):
    return (pltpu.bitcast(a, U32) >> 16) | pltpu.bitcast(b, U32)


def _load_packed(ref):
    cols = []
    for c in range(NC):
        w = jnp.concatenate([ref[c, d * PSTR:d * PSTR + H // 2, :] for d in range(DH)], axis=0)
        cols.append(pltpu.bitcast(w, BF16))
    return jnp.concatenate(cols, axis=1)


def _store_interleaved(ref, val, head0):
    acc = None
    for hp in range(val.shape[0] // (2 * DH)):
        w = _pack_rows(val[hp * 2 * DH:hp * 2 * DH + DH, :], val[hp * 2 * DH + DH:(hp + 1) * 2 * DH, :])
        for c in range(NC):
            ref[c, pl.ds(head0 // 2 + hp, DH, stride=PSTR), :] = w[:, c * LANES:(c + 1) * LANES]
            for g in range(DH // 8):
                piece = w[g * 8:(g + 1) * 8, c * LANES:(c + 1) * LANES]
                acc = piece if acc is None else acc | piece
    return acc


def _kernel(x_hbm, wqkv_hbm, wo_hbm, wr_hbm, wg_hbm, wu_hbm, wd_hbm, out_hbm,
            x_v, wk_v, w3_v, wr_v, wgu_v, wd_v,
            ln1_v, pkt_v, zacc_v, g_v, wqp_v, mp_v, pqn_v, attn_v, lo_v, zero_v, sems):

    ln2_v, out_v = lo_v.at[0], lo_v.at[1]

    wqkv_hbm, wo_hbm, wg_hbm, wu_hbm, wd_hbm = (r.bitcast(U32) for r in (wqkv_hbm, wo_hbm, wg_hbm, wu_hbm, wd_hbm))

    def wload(ref, r0, nr, cols):
        rows = pl.ds(r0 // 2, nr // 2) if isinstance(r0, int) else pl.ds(pl.multiple_of(r0 // 2, nr // 2), nr // 2)
        return pltpu.bitcast(ref[rows, cols], BF16)

    wq_v, wv_v, wo_v = w3_v.at[0], w3_v.at[1], w3_v.at[2]
    wg_v, wu_v = wgu_v.at[0], wgu_v.at[1]

    def x_copy(i):
        r0, n = XP[i]
        return pltpu.make_async_copy(x_hbm.at[pl.ds(r0, n), :], x_v.at[pl.ds(DEF + r0, n), :], sems.at[SEM_X + i])

    def out_copy(r0, n, s):
        return pltpu.make_async_copy(out_v.at[pl.ds(DEF + r0, n), :], out_hbm.at[pl.ds(r0, n), :],
                                     sems.at[SEM_OUT + s])

    def wk_copy(j):
        c0, n = WKP[j]
        return pltpu.make_async_copy(wqkv_hbm.at[:, pl.ds(D + c0, n)], wk_v.at[:, pl.ds(c0, n)],
                                     sems.at[SEM_WK + j])

    wr_copy = pltpu.make_async_copy(wr_hbm, wr_v, sems.at[SEM_WR])
    wd_copy = pltpu.make_async_copy(wd_hbm, wd_v.at[:, pl.ds(0, D)], sems.at[SEM_WD])
    wg_copy = pltpu.make_async_copy(wg_hbm, wg_v.at[:, pl.ds(0, F)], sems.at[SEM_WGU])
    wu_copy = pltpu.make_async_copy(wu_hbm, wu_v.at[:, pl.ds(0, F)], sems.at[SEM_WGU])

    x_copy(0).start()
    wk_copy(0).start()
    x_copy(1).start()
    wr_copy.start()
    for j in range(1, len(WKP)):
        wk_copy(j).start()
    x_copy(2).start()
    x_copy(3).start()
    pltpu.make_async_copy(wqkv_hbm.at[:, pl.ds(0, D)], wq_v, sems.at[SEM_W3]).start()
    pltpu.make_async_copy(wqkv_hbm.at[:, pl.ds(2 * D, D)], wv_v, sems.at[SEM_W3]).start()
    pltpu.make_async_copy(wo_hbm, wo_v, sems.at[SEM_W3]).start()
    wg_copy.start()
    wu_copy.start()
    wd_copy.start()

    def ln1_rows(xr, xr0, lnr, r0, n):
        ln = _layernorm(xr[xr0:xr0 + n, :].astype(F32)).astype(BF16)
        lnr[r0 // 2:(r0 + n) // 2, :] = pltpu.bitcast(ln, U32)

    def ln1_rows_paced(xr, xr0, lnr, r0, n, L1LAG=L1LAG):
        zero_u = zero_v[...]
        toks = []
        lns = []
        for j in range(n // L1U):
            x = xr[xr0 + j * L1U:xr0 + (j + 1) * L1U, :].astype(F32)
            tok = toks[-L1LAG] if len(toks) >= L1LAG else None
            ln = _layernorm(x, tok)
            toks.append(pltpu.bitcast(pltpu.bitcast(ln[L1U - 8:L1U, 0:LANES], U32) & zero_u, F32))
            lns.append(ln)
            if (j + 1) * L1U % 16 == 0:
                grp = jnp.concatenate(lns, axis=0).astype(BF16)
                e = r0 + (j + 1) * L1U
                lnr[(e - grp.shape[0]) // 2:e // 2, :] = pltpu.bitcast(grp, U32)
                lns = []

    def ln1_load(lnr, r0, n):
        return pltpu.bitcast(lnr[r0 // 2:(r0 + n) // 2, :], BF16)

    def k_mm(lnr, r0, n, c0, nc):
        return jnp.dot(ln1_load(lnr, r0, n), wload(wk_v, 0, D, slice(c0, c0 + nc)), preferred_element_type=F32)

    def k_post(k, p0, c0, first=False):
        n, nc = k.shape
        pkt = _phi(k).T
        pkt_v[c0 // 2:(c0 + nc) // 2, p0:p0 + n] = pltpu.bitcast(pkt.astype(BF16), U32)
        zs = pkt[:, 0:LANES]
        for j in range(1, n // LANES):
            zs = zs + pkt[:, j * LANES:(j + 1) * LANES]
        for hh in range(nc // DH):
            z0 = (c0 // DH + hh) * ZP
            if first:
                zacc_v[z0:z0 + DH, :] = zs[hh * DH:(hh + 1) * DH, :]
            else:
                zacc_v[z0:z0 + DH, :] += zs[hh * DH:(hh + 1) * DH, :]

    def g_acc(lnr, r0, n, c0, nc, first=False):
        g = jnp.dot(pltpu.bitcast(pkt_v[c0 // 2:(c0 + nc) // 2, r0:r0 + n], BF16), ln1_load(lnr, r0, n),
                    preferred_element_type=F32)
        if first:
            g_v[c0:c0 + nc, :] = g
        else:
            g_v[c0:c0 + nc, :] += g

    attn_v[...] = jnp.zeros_like(attn_v)
    x_v[0:DEF, :] = jnp.zeros((DEF, D), BF16)
    zero_v[...] = jnp.zeros_like(zero_v)

    def k0(c0, nc):
        k_post(k_mm(ln1_v, 0, TX, c0, nc), 0, c0, first=True)

    def g0(c0, nc):
        g_acc(ln1_v, 0, TX, c0, nc, first=True)

    x_copy(0).wait()
    ln1_rows(x_v, DEF, ln1_v, 0, 128)
    wk_copy(0).wait()
    ka = k_mm(ln1_v, 0, 128, 0, 128)
    x_copy(1).wait()
    wr_copy.wait()
    ln1_rows(x_v, DEF + 128, ln1_v, 128, 128)
    k_post(ka, 0, 0, first=True)
    g_acc(ln1_v, 0, 128, 0, 128, first=True)
    wk_copy(1).wait()
    k_post(k_mm(ln1_v, 128, 128, 0, 128), 128, 0)
    k0(128, 128)
    g_acc(ln1_v, 128, 128, 0, 128)
    wk_copy(2).wait()
    k0(256, 256)
    g0(128, 128)
    g0(256, 256)
    wk_copy(3).wait()
    k0(512, 256)
    k0(768, 256)
    g0(512, 256)
    x_copy(2).wait()
    ln1_rows(x_v, DEF + TX, ln1_v, TX, TX)
    g0(768, 256)
    HD = D // 2
    k_post(k_mm(ln1_v, TX, TX, 0, HD), TX, 0)
    k_post(k_mm(ln1_v, TX, TX, HD, HD), TX, HD)
    ln1_rows_paced(x_v, DEF + P0, ln1_v, P0, TB, L1LAG0)
    g_acc(ln1_v, TX, TX, 0, HD)
    g_acc(ln1_v, TX, TX, HD, HD)

    def p1(i, carry):
        lnr = ln1_v.at[pl.ds(pl.multiple_of(P0 // 2 + i * (TB // 2), 64), TB), :]
        xr = x_v.at[pl.ds(pl.multiple_of(P0 + jnp.minimum(i + 1, NB1 - 1) * TB, 128), TB + DEF), :]
        k_post(k_mm(lnr, 0, TB, 0, HD), 0, 0)
        k_post(k_mm(lnr, 0, TB, HD, HD), 0, HD)
        ln1_rows_paced(xr, DEF, lnr, TB, TB)
        g_acc(lnr, 0, TB, 0, HD)
        g_acc(lnr, 0, TB, HD, HD)
        return carry

    x_copy(3).wait()
    lax.fori_loop(0, NB1, p1, 0)

    pltpu.make_async_copy(w3_v, w3_v, sems.at[SEM_W3]).wait()
    zero_u = zero_v[...]
    wtok = []
    for c in range(NC):
        wtok.append(zero_u & _store_interleaved(wqp_v, wload(wq_v, 0, D, slice(c * LANES, (c + 1) * LANES)).astype(F32).T,
                                                c * (LANES // DH)))
    zp = jnp.concatenate([zacc_v[pl.ds(d, H, stride=ZP), :] for d in range(DH)], axis=0)
    zrow = jnp.sum(zp.T, axis=0, keepdims=True)
    wr8 = wr_v[...].astype(F32)
    wr_row = jnp.concatenate([wr8[c:c + 1, :] for c in range(NC)], axis=1)

    row_h = lax.broadcasted_iota(I32, (LANES, LANES), 0) // DH
    col_h = lax.broadcasted_iota(I32, (LANES, LANES), 1) // DH
    diag = row_h == col_h
    def kv_part(c):
        cs = slice(c * LANES, (c + 1) * LANES)
        gb = g_v[cs, :]
        tk = None
        for cc in KVGATE[c]:
            tk = wtok[cc] if tk is None else tk | wtok[cc]
        if tk is not None:
            gb = jnp.concatenate([jnp.concatenate([gb[0:8, 0:LANES] + pltpu.bitcast(tk, F32), gb[0:8, LANES:]], axis=1),
                                  gb[8:, :]], axis=0)
        kv = jnp.dot(gb.astype(BF16), wload(wv_v, 0, D, cs), preferred_element_type=F32)
        return jnp.where(diag, kv, 0.0)

    def m_part(c, kv):
        cs = slice(c * LANES, (c + 1) * LANES)
        tk = None
        for cc in MGATE[c]:
            tk = wtok[cc] if tk is None else tk | wtok[cc]
        if tk is not None:
            kv = jnp.concatenate([kv[0:8, :] + pltpu.bitcast(tk, F32), kv[8:, :]], axis=0)
        m = jnp.dot(kv.astype(BF16), wload(wo_v, c * LANES, LANES, slice(None)), preferred_element_type=F32)
        _store_interleaved(mp_v, m.astype(BF16).astype(F32), c * (LANES // DH))

    kvs = {}
    for c in range(NC + KVLAG):
        if c < NC:
            kvs[c] = kv_part(c)
        if c >= KVLAG:
            m_part(c - KVLAG, kvs[c - KVLAG])

    def make_key(score, row):
        b = pltpu.bitcast(score, I32)
        srt = b ^ ((b >> 31) & 0x7FFFFFFF)
        return (srt & jnp.int32(-65536)) | (0xFFFF - row)

    def push_keys(key, top1, top2):
        for gidx in range(key.shape[0] // 8):
            kx = key[gidx * 8:(gidx + 1) * 8, :]
            top2 = jnp.maximum(top2, jnp.minimum(top1, kx))
            top1 = jnp.maximum(top1, kx)
        return top1, top2

    def colsum(t):
        acc = t[:, 0:LANES]
        for c in range(1, NC):
            acc = acc + t[:, c * LANES:(c + 1) * LANES]
        return acc

    def q_part(lnr, l0, r0, n, hint=None):
        q = lax.dot_general(ln1_load(lnr, l0 + r0, n), _load_packed(wqp_v),
                            (((1,), (1,)), ((), ())), preferred_element_type=F32)
        pq = _phi(q)
        den = colsum(pq * zrow)
        den = den + pltpu.roll(den, DH, 1)
        den = den + pltpu.roll(den, 2 * DH, 1)
        inv = 1.0 / (den + 1e-6)
        pqn = pq * jnp.concatenate([inv] * NC, axis=1)
        pqn_v[r0 // 2:(r0 + n) // 2, :] = pltpu.bitcast(pqn.astype(BF16), U32)
        if hint is None:
            return None
        urow, wrc, p1, p2 = hint
        xb = x_v[DEF + l0 + r0:DEF + l0 + r0 + n, :].astype(F32)
        num = jnp.sum(colsum(xb * wrc) + colsum(pq * urow) * inv, axis=-1, keepdims=True)
        return push_keys(make_key(num, (l0 + r0) + lax.broadcasted_iota(I32, (n, 1), 0)), p1, p2)

    def o_part(r0, n):
        return jnp.dot(pltpu.bitcast(pqn_v[r0 // 2:(r0 + n) // 2, :], BF16), _load_packed(mp_v),
                       preferred_element_type=F32)

    def ln2_unit(attn, xr, l2r, outr, r0, row0, valid, top1, top2, tok, fast=False, is_h=False):
        n = attn.shape[0]
        h = attn if is_h else xr[r0:r0 + n, :].astype(F32) + attn
        if fast:
            ln2, r = _layernorm(h, tok, wr_row)
        else:
            ln2 = _layernorm(h, tok)
            r = jnp.sum(ln2 * wr_row, axis=-1, keepdims=True)
        l2r[r0:r0 + n, :] = ln2.astype(BF16)
        res = h + ln2
        outr[r0:r0 + n, :] = res.astype(BF16)
        r = r.astype(BF16).astype(F32) + 0.0
        key = make_key(r, (row0 + r0) + lax.broadcasted_iota(I32, (n, 1), 0))
        if valid is not None:
            key = jnp.where(valid, key, INT_MIN)
        top1, top2 = push_keys(key, top1, top2)
        ntok = pltpu.bitcast(pltpu.bitcast(jnp.broadcast_to(r[n - 8:n, :], (8, LANES)), U32) & zero_u, F32)
        return top1, top2, ntok

    def ln2_part(attn, xr, l2r, outr, r0, row0, valid, top1, top2, toks, lag=LAG, **kw):
        n = attn.shape[0]
        u = min(LNU, n)
        for j in range(n // u):
            tok = toks[-lag] if len(toks) >= lag else None
            top1, top2, tok = ln2_unit(attn[j * u:(j + 1) * u, :], xr, l2r, outr, r0 + j * u, row0, valid,
                                       top1, top2, tok, **kw)
            toks.append(tok)
        return top1, top2

    def p2(i, carry):
        top1, top2 = carry
        b0 = pl.multiple_of(i * TB2, 16)
        lnr = ln1_v.at[pl.ds(pl.multiple_of(i * (TB2 // 2), 8), TB2 // 2), :]
        xr = x_v.at[pl.ds(b0, TB2 + DEF), :]
        l2r = ln2_v.at[pl.ds(b0, TB2 + DEF), :]
        outr = out_v.at[pl.ds(b0, TB2 + DEF), :]
        row0 = b0 - DEF
        toks = []
        top1, top2 = ln2_part(attn_v[...], xr, l2r, outr, 0, row0, i > 0, top1, top2, toks)

        @pl.when(i > 0)
        def _():
            out_copy(pl.multiple_of((i - 1) * TB2, 16), TB2, 0).start()

        qa = (TB2 // 32) * 16
        q_part(lnr, 0, 0, qa)
        q_part(lnr, 0, qa, TB2 - qa)
        r0 = 0
        for n in OCH[:-1]:
            top1, top2 = ln2_part(o_part(r0, n), xr, l2r, outr, DEF + r0, row0, None, top1, top2, toks)
            r0 += n
        attn_v[...] = o_part(r0, DEF)
        return top1, top2

    init = jnp.full((8, 1), INT_MIN, I32)
    top1, top2 = lax.fori_loop(0, NB2, p2, (init, init))

    wg_copy.wait()
    wu_copy.wait()
    wd_copy.wait()
    sub8 = lax.broadcasted_iota(I32, (8, LANES), 0)

    def submax(v):
        for sh in (4, 2, 1):
            v = jnp.maximum(v, pltpu.roll(v, sh, 0))
        return v

    def subsum(v):
        for sh in (4, 2, 1):
            v = v + pltpu.roll(v, sh, 0)
        return v

    def best2(t1, t2):
        t1 = jnp.broadcast_to(t1, (8, LANES))
        t2 = jnp.broadcast_to(t2, (8, LANES))
        k1v = submax(t1)
        return k1v, submax(jnp.where(t1 == k1v, t2, t1))

    def key_row(k):
        return 0xFFFF - (k & 0xFFFF)

    def wide(m):
        return jnp.concatenate([m] * NC, axis=1)

    def m_tile(c, k0, nk):
        w = jnp.concatenate([mp_v[c, d * PSTR:d * PSTR + H // 2, :] for d in range(k0 // H, (k0 + nk) // H)], axis=0)
        return pltpu.bitcast(w, BF16)

    toks = []
    top1, top2 = ln2_part(attn_v[...], x_v, ln2_v, out_v, L0, -DEF, None, top1, top2, toks, lag=LAG_L)
    out_copy(L0 - TB2, TB2, 0).start()
    oldk = best2(top1, top2)
    oldx = []
    for kk in oldk:
        g8 = pl.multiple_of(((key_row(kk[0, 0]) >> 3) << 3) + DEF, 8)
        rows = ln2_v[pl.ds(g8, 8), :].astype(F32)
        oldx.append(subsum(jnp.where(wide((key_row(kk) & 7) == sub8), rows, 0.0)))

    wrc = wr_row - jnp.sum(wr_row, axis=-1, keepdims=True) * (1.0 / D)
    uparts = []
    for k0 in range(0, D, LANES):
        mrows = jnp.concatenate([m_tile(c, k0, LANES) for c in range(NC)], axis=1).astype(F32)
        part = colsum(mrows * wrc)
        if uparts:
            tok = pltpu.bitcast(pltpu.bitcast(jnp.broadcast_to(uparts[-1], (8, LANES)), U32) & zero_u, F32)
            mrows = jnp.concatenate([mrows[:, 0:LANES] + jnp.concatenate([tok] * (LANES // 8), axis=0),
                                     mrows[:, LANES:]], axis=1)
            part = colsum(mrows * wrc)
        uparts.append(jnp.sum(part.T, axis=0, keepdims=True))
    urow = jnp.concatenate(uparts, axis=1)
    p1, p2_, r0 = init, init, 0
    for n in QS:
        p1, p2_ = q_part(ln1_v, L0, r0, n, (urow, wrc, p1, p2_))
        r0 += n

    cand_p, cand_x = [], []
    for pk_ in (p1, p2_):
        cp = jnp.zeros((8, D), F32)
        cx = jnp.zeros((8, D), F32)
        for s in range(8):
            row = key_row(pk_[s, 0])
            g8 = pl.multiple_of((row >> 3) << 3, 8)
            m = wide(sub8 == s)
            pair = jnp.broadcast_to(pqn_v[pl.ds((row - L0) >> 1, 1), :], (8, D))
            half = pair & jnp.uint32(0xFFFF0000) if s % 2 else pair << 16
            cp = jnp.where(m, pltpu.bitcast(half, F32), cp)
            cx = jnp.where(m, x_v[pl.ds(g8 + DEF, 8), :].astype(F32), cx)
        cand_p.append(cp)
        cand_x.append(cx)
    cand_p = jnp.concatenate(cand_p, axis=0).astype(BF16)
    cand_x = jnp.concatenate(cand_x, axis=0)
    ids_lo = key_row(jnp.broadcast_to(p1, (8, LANES)))
    ids_hi = jnp.where(sub8 < 6, key_row(jnp.broadcast_to(p2_, (8, LANES))),
                       jnp.where(sub8 == 6, key_row(oldk[0]), key_row(oldk[1])))

    st = dict(top1=top1, top2=top2, pend=[], step=0, sent=0)

    def gated(v):
        tok = None
        while st["pend"] and st["pend"][0][0] <= st["step"]:
            t = st["pend"].pop(0)[1]
            tok = t if tok is None else tok | t
        if tok is None:
            return v
        u = pltpu.bitcast(v, U32)
        return pltpu.bitcast(jnp.concatenate([u[:, 0:LANES] | tok, u[:, LANES:]], axis=1), BF16)

    def o_units():
        r0 = -OCL[0]
        for ci, n in enumerate(OCL):
            r0 += OCL[ci - 1] if ci else OCL[0]
            lhs = pltpu.bitcast(pqn_v[r0 // 2:(r0 + n) // 2, :], BF16)
            halves = []
            for c0 in range(0, NC, ONT):
                acc = x_v[DEF + L0 + r0:DEF + L0 + r0 + n, c0 * LANES:(c0 + ONT) * LANES].astype(F32)
                ks = (4 // ONT) * LANES
                for k0 in range(0, D, ks):
                    w = jnp.concatenate([m_tile(c, k0, ks) for c in range(c0, c0 + ONT)], axis=1)
                    acc = acc + jnp.dot(lhs[:, k0:k0 + ks], w, preferred_element_type=F32)
                    if k0 + ks == D:
                        halves.append(acc)
                        if len(halves) == NC // ONT:
                            last = r0 + n == RL
                            tk = [] if last else toks
                            st["top1"], st["top2"] = ln2_part(
                                jnp.concatenate(halves, axis=1), x_v, ln2_v, out_v, DEF + L0 + r0, -DEF, None,
                                st["top1"], st["top2"], tk, lag=n if last else LAG_L, is_h=True, fast=last)
                            if GLAG[ci] is not None:
                                st["pend"].append((st["step"] + GLAG[ci],
                                                   pltpu.bitcast(jnp.broadcast_to(st["top1"], (8, LANES)), U32) & zero_u))
                            if last:
                                out_copy(L0 + st["sent"], r0 + n - st["sent"], 2).start()
                            elif r0 + n in OUT_AT:
                                out_copy(L0 + st["sent"], r0 + n - st["sent"], 1).start()
                                st["sent"] = r0 + n
                    yield

    res = {}

    def c_units():
        parts = []
        for c in range(NC):
            parts.append(jnp.dot(cand_p, m_tile(c, 0, D), preferred_element_type=F32))
            yield
        xs = _layernorm(cand_x + jnp.concatenate(parts, axis=1))
        hi = jnp.where(wide(sub8 < 6), xs[8:16, :], jnp.where(wide(sub8 == 6), oldx[0], oldx[1]))
        res["xs"] = jnp.concatenate([xs[0:8, :], hi], axis=0).astype(BF16)

    def f_units():
        xs = res["xs"]
        acts = []
        for j in range(F // LANES):
            cs = slice(j * LANES, (j + 1) * LANES)
            g = jnp.dot(gated(xs), wload(wg_v, 0, D, cs), preferred_element_type=F32)
            yield
            u = jnp.dot(xs, wload(wu_v, 0, D, cs), preferred_element_type=F32)
            acts.append((g * jax.nn.sigmoid(g) * u).astype(BF16))
            yield
        act = jnp.concatenate(acts, axis=1)
        zf = pltpu.bitcast(zero_u, F32)
        ys = []
        KF = (F // D) * D
        for c in range(0, NC, 2):
            acc = jnp.concatenate([jnp.concatenate([zf, zf], axis=0)] * 2, axis=1)
            acc = acc + jnp.dot(gated(act[:, KF:]), wload(wd_v, KF, F - KF, slice(c * LANES, (c + 2) * LANES)),
                                preferred_element_type=F32)
            yield
            for cc in range(2):
                y = acc[:, cc * LANES:(cc + 1) * LANES]
                for k0 in range(0, KF, D):
                    y = y + jnp.dot(gated(act[:, k0:k0 + D]),
                                    wload(wd_v, k0, D, slice((c + cc) * LANES, (c + cc + 1) * LANES)),
                                    preferred_element_type=F32)
                    yield
                ys.append(y)
        res["y"] = jnp.concatenate(ys, axis=1)

    ou = o_units()

    def o_step():
        next(ou, None)
        st["step"] += 1

    for _ in range(NPRE):
        o_step()
    for _ in c_units():
        o_step()
    for _ in range(NGAP):
        o_step()
    for _ in f_units():
        o_step()
    for _ in ou:
        pass

    keyv = best2(st["top1"], st["top2"])
    idx = [key_row(kk[0, 0]) for kk in keyv]
    grp = [pl.multiple_of((ii >> 3) << 3, 8) for ii in idx]
    vgrp = [pl.multiple_of(gg + DEF, 8) for gg in grp]
    y = res["y"]
    hits = None
    yrows = []
    for c in range(2):
        m_lo = ids_lo == key_row(keyv[c])
        m_hi = ids_hi == key_row(keyv[c])
        yrows.append(subsum(jnp.where(wide(m_lo), y[0:8, :], 0.0) + jnp.where(wide(m_hi), y[8:16, :], 0.0)))
        hit = submax(jnp.where(m_lo | m_hi, 1, 0))
        hits = hit if hits is None else hits + hit
    hit_all = hits[0, 0] == 2

    tail0 = L0 + st["sent"]
    tail_copy = out_copy(tail0, S - tail0, 2)
    in_tail = jnp.maximum(grp[0], grp[1]) >= tail0
    two_groups = grp[1] != grp[0]

    def fix_copy(c):
        return out_copy(grp[c], 8, 3 + c)

    def finish(ysel):
        for c in range(2):
            hi = keyv[c] & jnp.int32(-65536)
            score = pltpu.bitcast(hi ^ ((hi >> 31) & 0x7FFF0000), F32)
            sel = (key_row(keyv[c]) & 7) == sub8
            upd = jnp.where(wide(sel), ysel[c] * wide(jax.nn.sigmoid(score)), 0.0)
            out_v[pl.ds(vgrp[c], 8), :] = (out_v[pl.ds(vgrp[c], 8), :].astype(F32) + upd).astype(BF16)
        fix_copy(0).start()

        @pl.when(two_groups)
        def _():
            fix_copy(1).start()

    out_copy(0, L0, 0).wait()
    out_copy(L0, tail0 - L0, 1).wait()

    @pl.when(in_tail)
    def _():
        tail_copy.wait()

    @pl.when(hit_all)
    def _():
        finish(yrows)

    @pl.when(jnp.logical_not(hit_all))
    def _():
        xsel = jnp.concatenate([ln2_v[pl.ds(vgrp[c], 8), :] for c in range(2)], axis=0)

        def ffn_tile(j, acc):
            cs = pl.ds(pl.multiple_of(j * LANES, LANES), LANES)
            g = jnp.dot(xsel, wload(wg_v, 0, D, cs), preferred_element_type=F32)
            u = jnp.dot(xsel, wload(wu_v, 0, D, cs), preferred_element_type=F32)
            a = (g * jax.nn.sigmoid(g) * u).astype(BF16)
            wd_t = pltpu.bitcast(wd_v[pl.ds(pl.multiple_of(j * (LANES // 2), LANES // 2), LANES // 2), 0:D], BF16)
            return acc + jnp.dot(a, wd_t, preferred_element_type=F32)

        yf = lax.fori_loop(0, F // LANES, ffn_tile, jnp.zeros((16, D), F32))
        finish([yf[0:8, :], yf[8:16, :]])

    @pl.when(jnp.logical_not(in_tail))
    def _():
        tail_copy.wait()

    fix_copy(0).wait()

    @pl.when(two_groups)
    def _():
        fix_copy(1).wait()


@jax.jit
def pallas_sequential_preLN__linear_attn_block__moe_arch_mod__prompt_kernel(
    A_x: jax.Array,
    A_wqkv: jax.Array,
    A_wo: jax.Array,
    B_x: jax.Array,
    B_w_r: jax.Array,
    B_w_gate: jax.Array,
    B_w_up: jax.Array,
    B_w_down: jax.Array,
):
    del B_x
    x = A_x.reshape(S, D)
    wr = B_w_r.reshape(NC, LANES)
    any_spec = pl.BlockSpec(memory_space=pl.ANY)
    out = pl.pallas_call(
        _kernel,
        out_shape=jax.ShapeDtypeStruct((S, D), BF16),
        in_specs=[any_spec] * 7,
        out_specs=any_spec,
        scratch_shapes=[
            pltpu.VMEM((S + DEF, D), BF16),
            pltpu.VMEM((D // 2, D), U32),
            pltpu.VMEM((3, D // 2, D), U32),
            pltpu.VMEM((NC, LANES), BF16),
            pltpu.VMEM((2, D // 2, F + LANES), U32),
            pltpu.VMEM((F // 2, D + LANES), U32),
            pltpu.VMEM(((S + TB) // 2, D), U32),
            pltpu.VMEM((D // 2, max(TB, P0)), U32),
            pltpu.VMEM((H * ZP, LANES), F32),
            pltpu.VMEM((D, D), F32),
            pltpu.VMEM((NC, DH * PSTR, LANES), U32),
            pltpu.VMEM((NC, DH * PSTR, LANES), U32),
            pltpu.VMEM((max(TB2, RL) // 2, D), U32),
            pltpu.VMEM((DEF, D), F32),
            pltpu.VMEM((2, S + DEF, D), BF16),
            pltpu.VMEM((8, LANES), U32),
            pltpu.SemaphoreType.DMA((NSEM,)),
        ],
        compiler_params=pltpu.CompilerParams(vmem_limit_bytes=110 * 1024 * 1024, **CPX),
    )(x, A_wqkv, A_wo, wr, B_w_gate, B_w_up, B_w_down)
    return out.reshape(1, S, D)
```

```python
import jax
import jax.numpy as jnp
from jax import lax
import jax.experimental.pallas as pl
import jax.experimental.pallas.tpu as pltpu


S = 2048
D = 1024
F = 3584
H = 32
DH = D // H
LANES = 128
NC = D // LANES
HD = D // 2

P0 = 512
TX = 256
TB = 384
NB1 = (S - P0) // TB
TB2 = 544
NB2 = 3
OCH = (64, 64, 64, 64, 64, 64, 64, 32, 64)
DEF = OCH[-1]
L0 = NB2 * TB2
RL = S - L0
QS = (256, 96, 64)
OCL = (32, 64, 64, 64, 64, 64, 64)
ONT = 2
NPRE = 20
NGAP = 8
OUT_AT = (160, 288, 352)
LNU = 8
LAG = 5
LAG_L = 3
L1LAG = 2
L1LAG0 = 3
GLAG = (None, None, None, None, None, 20, 8)
KVGATE = ((), (), (0,), (1,), (2,), (3,), (4,), (5,))
MGATE = ((), (), (), (), (), (), (6,), (7,))
ZP = 36
PSTR = 20

F32 = jnp.float32
BF16 = jnp.bfloat16
U32 = jnp.uint32
I32 = jnp.int32

XP = ((0, 128), (128, 128), (256, 768), (1024, 1024))
WKP = ((0, 128), (128, 128), (256, 256), (512, 512))

SEM_X = 0
SEM_WK = SEM_X + len(XP)
SEM_W3 = SEM_WK + len(WKP)
SEM_WR = SEM_W3 + 1
SEM_WGU = SEM_WR + 1
SEM_WD = SEM_WGU + 1
SEM_OUT = SEM_WD + 1
NSEM = SEM_OUT + 5

INT_MIN = -(2 ** 31)


def _layernorm(x, tok=None, w=None):
    s0 = x[:, 0:LANES]
    if tok is not None:
        s0 = s0 + jnp.concatenate([tok] * (x.shape[0] // 8), axis=0)
    for c in range(1, NC):
        s0 = s0 + x[:, c * LANES:(c + 1) * LANES]
    mu = jnp.sum(s0, axis=-1, keepdims=True) * (1.0 / D)
    xc = x - mu
    var = jnp.sum(xc * xc, axis=-1, keepdims=True) * (1.0 / D)
    rstd = lax.rsqrt(var + 1e-5)
    if w is None:
        return xc * rstd
    return xc * rstd, jnp.sum(xc * w, axis=-1, keepdims=True) * rstd


def _phi(t):
    return jnp.where(t > 0, t + 1.0, jnp.exp(t)) + 1e-6


def _pack_rows(a, b):
    return (pltpu.bitcast(a, U32) >> 16) | pltpu.bitcast(b, U32)


def _load_packed(ref, n0=0, n1=D):
    cols = []
    for c in range(NC):
        w = jnp.concatenate([ref[c, d * PSTR:d * PSTR + H // 2, :] for d in range(n0 // H, n1 // H)], axis=0)
        cols.append(pltpu.bitcast(w, BF16))
    return jnp.concatenate(cols, axis=1)


def _store_interleaved(ref, val, head0):
    acc = None
    for hp in range(val.shape[0] // (2 * DH)):
        w = _pack_rows(val[hp * 2 * DH:hp * 2 * DH + DH, :], val[hp * 2 * DH + DH:(hp + 1) * 2 * DH, :])
        for c in range(NC):
            ref[c, pl.ds(head0 // 2 + hp, DH, stride=PSTR), :] = w[:, c * LANES:(c + 1) * LANES]
            for g in range(DH // 8):
                piece = w[g * 8:(g + 1) * 8, c * LANES:(c + 1) * LANES]
                acc = piece if acc is None else acc | piece
    return acc


def _kernel(x_hbm, wqkv_hbm, wo_hbm, wr_hbm, wg_hbm, wu_hbm, wd_hbm, out_hbm,
            x_v, wk_v, w3_v, wr_v, wgu_v, wd_v,
            ln1_v, pkt_v, zacc_v, g_v, wqp_v, wq0_v, mp_v, pqn_v, attn_v, lo_v, zero_v, sems):

    ln2_v, out_v = lo_v.at[0], lo_v.at[1]

    wqkv_hbm, wo_hbm, wg_hbm, wu_hbm, wd_hbm = (r.bitcast(U32) for r in (wqkv_hbm, wo_hbm, wg_hbm, wu_hbm, wd_hbm))

    def wload(ref, r0, nr, cols):
        return pltpu.bitcast(ref[r0 // 2:(r0 + nr) // 2, cols], BF16)

    wq_v, wv_v, wo_v = w3_v.at[0], w3_v.at[1], w3_v.at[2]
    wg_v, wu_v = wgu_v.at[0], wgu_v.at[1]

    def x_copy(i):
        r0, n = XP[i]
        return pltpu.make_async_copy(x_hbm.at[pl.ds(r0, n), :], x_v.at[pl.ds(DEF + r0, n), :], sems.at[SEM_X + i])

    def out_copy(r0, n, s):
        return pltpu.make_async_copy(out_v.at[pl.ds(DEF + r0, n), :], out_hbm.at[pl.ds(r0, n), :],
                                     sems.at[SEM_OUT + s])

    def wk_copy(j):
        c0, n = WKP[j]
        return pltpu.make_async_copy(wqkv_hbm.at[:, pl.ds(D + c0, n)], wk_v.at[:, pl.ds(c0, n)],
                                     sems.at[SEM_WK + j])

    wr_copy = pltpu.make_async_copy(wr_hbm, wr_v, sems.at[SEM_WR])
    wd_copy = pltpu.make_async_copy(wd_hbm, wd_v.at[:, pl.ds(0, D)], sems.at[SEM_WD])
    wg_copy = pltpu.make_async_copy(wg_hbm, wg_v.at[:, pl.ds(0, F)], sems.at[SEM_WGU])
    wu_copy = pltpu.make_async_copy(wu_hbm, wu_v.at[:, pl.ds(0, F)], sems.at[SEM_WGU])

    x_copy(0).start()
    wk_copy(0).start()
    x_copy(1).start()
    wr_copy.start()
    for j in range(1, len(WKP)):
        wk_copy(j).start()
    x_copy(2).start()
    x_copy(3).start()
    pltpu.make_async_copy(wqkv_hbm.at[:, pl.ds(0, D)], wq_v, sems.at[SEM_W3]).start()
    pltpu.make_async_copy(wqkv_hbm.at[:, pl.ds(2 * D, D)], wv_v, sems.at[SEM_W3]).start()
    pltpu.make_async_copy(wo_hbm, wo_v, sems.at[SEM_W3]).start()
    wg_copy.start()
    wu_copy.start()
    wd_copy.start()

    def ln1_rows(xr, xr0, lnr, r0, n):
        ln = _layernorm(xr[xr0:xr0 + n, :].astype(F32)).astype(BF16)
        lnr[r0 // 2:(r0 + n) // 2, :] = pltpu.bitcast(ln, U32)

    def ln1_rows_paced(xr, xr0, lnr, r0, n, lag):
        zero_u = zero_v[...]
        toks, lns = [], []
        for j in range(n // LNU):
            x = xr[xr0 + j * LNU:xr0 + (j + 1) * LNU, :].astype(F32)
            ln = _layernorm(x, toks[-lag] if len(toks) >= lag else None)
            toks.append(pltpu.bitcast(pltpu.bitcast(ln[:, 0:LANES], U32) & zero_u, F32))
            lns.append(ln)
            if j % 2:
                e = r0 + (j + 1) * LNU
                lnr[e // 2 - LNU:e // 2, :] = pltpu.bitcast(jnp.concatenate(lns, axis=0).astype(BF16), U32)
                lns = []

    def ln1_load(lnr, r0, n):
        return pltpu.bitcast(lnr[r0 // 2:(r0 + n) // 2, :], BF16)

    def k_mm(lnr, r0, n, c0, nc):
        return jnp.dot(ln1_load(lnr, r0, n), wload(wk_v, 0, D, slice(c0, c0 + nc)), preferred_element_type=F32)

    def k_post(k, p0, c0, first=False):
        n, nc = k.shape
        pkt = _phi(k).T
        pkt_v[c0 // 2:(c0 + nc) // 2, p0:p0 + n] = pltpu.bitcast(pkt.astype(BF16), U32)
        zs = pkt[:, 0:LANES]
        for j in range(1, n // LANES):
            zs = zs + pkt[:, j * LANES:(j + 1) * LANES]
        for hh in range(nc // DH):
            z0 = (c0 // DH + hh) * ZP
            if first:
                zacc_v[z0:z0 + DH, :] = zs[hh * DH:(hh + 1) * DH, :]
            else:
                zacc_v[z0:z0 + DH, :] += zs[hh * DH:(hh + 1) * DH, :]

    def g_acc(lnr, r0, n, c0, nc, first=False):
        g = jnp.dot(pltpu.bitcast(pkt_v[c0 // 2:(c0 + nc) // 2, r0:r0 + n], BF16), ln1_load(lnr, r0, n),
                    preferred_element_type=F32)
        if first:
            g_v[c0:c0 + nc, :] = g
        else:
            g_v[c0:c0 + nc, :] += g

    attn_v[...] = jnp.zeros_like(attn_v)
    x_v[0:DEF, :] = jnp.zeros((DEF, D), BF16)
    zero_v[...] = jnp.zeros_like(zero_v)

    def k0(c0, nc):
        k_post(k_mm(ln1_v, 0, TX, c0, nc), 0, c0, first=True)

    def g0(c0, nc):
        g_acc(ln1_v, 0, TX, c0, nc, first=True)

    x_copy(0).wait()
    ln1_rows(x_v, DEF, ln1_v, 0, 128)
    wk_copy(0).wait()
    ka = k_mm(ln1_v, 0, 128, 0, 128)
    x_copy(1).wait()
    wr_copy.wait()
    ln1_rows(x_v, DEF + 128, ln1_v, 128, 128)
    k_post(ka, 0, 0, first=True)
    g_acc(ln1_v, 0, 128, 0, 128, first=True)
    wk_copy(1).wait()
    k_post(k_mm(ln1_v, 128, 128, 0, 128), 128, 0)
    k0(128, 128)
    g_acc(ln1_v, 128, 128, 0, 128)
    wk_copy(2).wait()
    k0(256, 256)
    g0(128, 128)
    g0(256, 256)
    wk_copy(3).wait()
    k0(512, 256)
    k0(768, 256)
    g0(512, 256)
    x_copy(2).wait()
    ln1_rows(x_v, DEF + TX, ln1_v, TX, TX)
    g0(768, 256)
    k_post(k_mm(ln1_v, TX, TX, 0, HD), TX, 0)
    k_post(k_mm(ln1_v, TX, TX, HD, HD), TX, HD)
    ln1_rows_paced(x_v, DEF + P0, ln1_v, P0, TB, L1LAG0)
    g_acc(ln1_v, TX, TX, 0, HD)
    g_acc(ln1_v, TX, TX, HD, HD)

    def p1(i, carry):
        lnr = ln1_v.at[pl.ds(pl.multiple_of(P0 // 2 + i * (TB // 2), 64), TB), :]
        xr = x_v.at[pl.ds(pl.multiple_of(P0 + jnp.minimum(i + 1, NB1 - 1) * TB, 128), TB + DEF), :]
        k_post(k_mm(lnr, 0, TB, 0, HD), 0, 0)
        k_post(k_mm(lnr, 0, TB, HD, HD), 0, HD)
        ln1_rows_paced(xr, DEF, lnr, TB, TB, L1LAG)
        g_acc(lnr, 0, TB, 0, HD)
        g_acc(lnr, 0, TB, HD, HD)
        return carry

    x_copy(3).wait()
    lax.fori_loop(0, NB1, p1, 0)

    pltpu.make_async_copy(w3_v, w3_v, sems.at[SEM_W3]).wait()
    zero_u = zero_v[...]
    wtok = []
    for c in range(NC):
        wtok.append(zero_u & _store_interleaved(wqp_v, wload(wq_v, 0, D, slice(c * LANES, (c + 1) * LANES)).astype(F32).T,
                                                c * (LANES // DH)))
    wq0_v[...] = pltpu.bitcast(_load_packed(wqp_v, 0, LANES).astype(F32).T.astype(BF16), U32)
    zp = jnp.concatenate([zacc_v[pl.ds(d, H, stride=ZP), :] for d in range(DH)], axis=0)
    zrow = jnp.sum(zp.T, axis=0, keepdims=True)
    wr8 = wr_v[...].astype(F32)
    wr_row = jnp.concatenate([wr8[c:c + 1, :] for c in range(NC)], axis=1)

    row_h = lax.broadcasted_iota(I32, (LANES, LANES), 0) // DH
    col_h = lax.broadcasted_iota(I32, (LANES, LANES), 1) // DH
    diag = row_h == col_h

    def kv_part(c):
        cs = slice(c * LANES, (c + 1) * LANES)
        gb = g_v[cs, :]
        tk = None
        for cc in KVGATE[c]:
            tk = wtok[cc] if tk is None else tk | wtok[cc]
        if tk is not None:
            gb = jnp.concatenate([jnp.concatenate([gb[0:8, 0:LANES] + pltpu.bitcast(tk, F32), gb[0:8, LANES:]], axis=1),
                                  gb[8:, :]], axis=0)
        kv = jnp.dot(gb.astype(BF16), wload(wv_v, 0, D, cs), preferred_element_type=F32)
        return jnp.where(diag, kv, 0.0)

    def m_part(c, kv):
        tk = None
        for cc in MGATE[c]:
            tk = wtok[cc] if tk is None else tk | wtok[cc]
        if tk is not None:
            kv = jnp.concatenate([kv[0:8, :] + pltpu.bitcast(tk, F32), kv[8:, :]], axis=0)
        m = jnp.dot(kv.astype(BF16), wload(wo_v, c * LANES, LANES, slice(None)), preferred_element_type=F32)
        _store_interleaved(mp_v, m.astype(BF16).astype(F32), c * (LANES // DH))

    kv_prev = None
    for c in range(NC + 1):
        kv = kv_part(c) if c < NC else None
        if c:
            m_part(c - 1, kv_prev)
        kv_prev = kv

    def make_key(score, row):
        b = pltpu.bitcast(score, I32)
        srt = b ^ ((b >> 31) & 0x7FFFFFFF)
        return (srt & jnp.int32(-65536)) | (0xFFFF - row)

    def push_keys(key, top1, top2):
        for gidx in range(key.shape[0] // 8):
            kx = key[gidx * 8:(gidx + 1) * 8, :]
            top2 = jnp.maximum(top2, jnp.minimum(top1, kx))
            top1 = jnp.maximum(top1, kx)
        return top1, top2

    def colsum(t):
        acc = t[:, 0:LANES]
        for c in range(1, NC):
            acc = acc + t[:, c * LANES:(c + 1) * LANES]
        return acc

    def q_part(lnr, l0, r0, n, hint=None):
        lhs = ln1_load(lnr, l0 + r0, n)
        n0 = LANES if r0 == 0 else 0
        parts = [jnp.dot(lhs, pltpu.bitcast(wq0_v[...], BF16), preferred_element_type=F32)] if n0 else []
        parts.append(lax.dot_general(lhs, _load_packed(wqp_v, n0), (((1,), (1,)), ((), ())),
                                     preferred_element_type=F32))
        q = jnp.concatenate(parts, axis=1)
        pq = _phi(q)
        den = colsum(pq * zrow)
        den = den + pltpu.roll(den, DH, 1)
        den = den + pltpu.roll(den, 2 * DH, 1)
        inv = 1.0 / (den + 1e-6)
        pqn = pq * jnp.concatenate([inv] * NC, axis=1)
        pqn_v[r0 // 2:(r0 + n) // 2, :] = pltpu.bitcast(pqn.astype(BF16), U32)
        if hint is None:
            return None
        urow, wrc, p1, p2 = hint
        xb = x_v[DEF + l0 + r0:DEF + l0 + r0 + n, :].astype(F32)
        num = jnp.sum(colsum(xb * wrc) + colsum(pq * urow) * inv, axis=-1, keepdims=True)
        return push_keys(make_key(num, (l0 + r0) + lax.broadcasted_iota(I32, (n, 1), 0)), p1, p2)

    def o_part(r0, n):
        return jnp.dot(pltpu.bitcast(pqn_v[r0 // 2:(r0 + n) // 2, :], BF16), _load_packed(mp_v),
                       preferred_element_type=F32)

    def ln2_unit(attn, xr, l2r, outr, r0, row0, valid, top1, top2, tok, fast=False, is_h=False):
        n = attn.shape[0]
        h = attn if is_h else xr[r0:r0 + n, :].astype(F32) + attn
        if fast:
            ln2, r = _layernorm(h, tok, wr_row)
        else:
            ln2 = _layernorm(h, tok)
            r = jnp.sum(ln2 * wr_row, axis=-1, keepdims=True)
        l2r[r0:r0 + n, :] = ln2.astype(BF16)
        res = h + ln2
        outr[r0:r0 + n, :] = res.astype(BF16)
        r = r.astype(BF16).astype(F32) + 0.0
        key = make_key(r, (row0 + r0) + lax.broadcasted_iota(I32, (n, 1), 0))
        if valid is not None:
            key = jnp.where(valid, key, INT_MIN)
        top1, top2 = push_keys(key, top1, top2)
        ntok = pltpu.bitcast(pltpu.bitcast(jnp.broadcast_to(r[n - 8:n, :], (8, LANES)), U32) & zero_u, F32)
        return top1, top2, ntok

    def ln2_part(attn, xr, l2r, outr, r0, row0, valid, top1, top2, toks, lag=LAG, **kw):
        n = attn.shape[0]
        u = min(LNU, n)
        for j in range(n // u):
            tok = toks[-lag] if len(toks) >= lag else None
            top1, top2, tok = ln2_unit(attn[j * u:(j + 1) * u, :], xr, l2r, outr, r0 + j * u, row0, valid,
                                       top1, top2, tok, **kw)
            toks.append(tok)
        return top1, top2

    def p2(i, carry):
        top1, top2 = carry
        b0 = pl.multiple_of(i * TB2, 16)
        lnr = ln1_v.at[pl.ds(pl.multiple_of(i * (TB2 // 2), 8), TB2 // 2), :]
        xr = x_v.at[pl.ds(b0, TB2 + DEF), :]
        l2r = ln2_v.at[pl.ds(b0, TB2 + DEF), :]
        outr = out_v.at[pl.ds(b0, TB2 + DEF), :]
        row0 = b0 - DEF
        toks = []
        top1, top2 = ln2_part(attn_v[...], xr, l2r, outr, 0, row0, i > 0, top1, top2, toks)

        @pl.when(i > 0)
        def _():
            out_copy(pl.multiple_of((i - 1) * TB2, 16), TB2, 0).start()

        qa = (TB2 // 32) * 16
        q_part(lnr, 0, 0, qa)
        q_part(lnr, 0, qa, TB2 - qa)
        r0 = 0
        for n in OCH[:-1]:
            top1, top2 = ln2_part(o_part(r0, n), xr, l2r, outr, DEF + r0, row0, None, top1, top2, toks)
            r0 += n
        attn_v[...] = o_part(r0, DEF)
        return top1, top2

    init = jnp.full((8, 1), INT_MIN, I32)
    top1, top2 = lax.fori_loop(0, NB2, p2, (init, init))

    wg_copy.wait()
    wu_copy.wait()
    wd_copy.wait()
    sub8 = lax.broadcasted_iota(I32, (8, LANES), 0)

    def submax(v):
        for sh in (4, 2, 1):
            v = jnp.maximum(v, pltpu.roll(v, sh, 0))
        return v

    def subsum(v):
        for sh in (4, 2, 1):
            v = v + pltpu.roll(v, sh, 0)
        return v

    def best2(t1, t2):
        t1 = jnp.broadcast_to(t1, (8, LANES))
        t2 = jnp.broadcast_to(t2, (8, LANES))
        k1v = submax(t1)
        return k1v, submax(jnp.where(t1 == k1v, t2, t1))

    def key_row(k):
        return 0xFFFF - (k & 0xFFFF)

    def wide(m):
        return jnp.concatenate([m] * NC, axis=1)

    def m_tile(c, k0, nk):
        w = jnp.concatenate([mp_v[c, d * PSTR:d * PSTR + H // 2, :] for d in range(k0 // H, (k0 + nk) // H)], axis=0)
        return pltpu.bitcast(w, BF16)

    toks = []
    top1, top2 = ln2_part(attn_v[...], x_v, ln2_v, out_v, L0, -DEF, None, top1, top2, toks, lag=LAG_L)
    out_copy(L0 - TB2, TB2, 0).start()
    oldk = best2(top1, top2)
    oldx = []
    for kk in oldk:
        g8 = pl.multiple_of(((jnp.clip(key_row(kk[0, 0]), 0, S - 1) >> 3) << 3) + DEF, 8)
        rows = ln2_v[pl.ds(g8, 8), :].astype(F32)
        oldx.append(subsum(jnp.where(wide((key_row(kk) & 7) == sub8), rows, 0.0)))

    wrc = wr_row - jnp.sum(wr_row, axis=-1, keepdims=True) * (1.0 / D)
    uparts = []
    for k0 in range(0, D, LANES):
        mrows = _load_packed(mp_v, k0, k0 + LANES).astype(F32)
        if uparts:
            tok = pltpu.bitcast(pltpu.bitcast(jnp.broadcast_to(uparts[-1], (8, LANES)), U32) & zero_u, F32)
            mrows = jnp.concatenate([mrows[:, 0:LANES] + jnp.concatenate([tok] * (LANES // 8), axis=0),
                                     mrows[:, LANES:]], axis=1)
        uparts.append(jnp.sum(colsum(mrows * wrc).T, axis=0, keepdims=True))
    urow = jnp.concatenate(uparts, axis=1)
    p1, p2_, r0 = init, init, 0
    for n in QS:
        p1, p2_ = q_part(ln1_v, L0, r0, n, (urow, wrc, p1, p2_))
        r0 += n

    cp = jnp.zeros((8, D), U32)
    cx = [jnp.zeros((8, D), F32), jnp.zeros((8, D), F32)]
    for s in range(8):
        a1 = jnp.clip(key_row(p1[s, 0]) - L0, 0, RL - 1)
        a2 = jnp.clip(key_row(p2_[s, 0]) - L0, 0, RL - 1)
        b1, b2 = (a1 >> 3) & 1, (a2 >> 3) & 1
        w1 = pqn_v[pl.ds(pl.multiple_of((a1 >> 4) << 3, 8), 8), :]
        w2 = pqn_v[pl.ds(pl.multiple_of((a2 >> 4) << 3, 8), 8), :]
        w2 = jnp.where(b1 == b2, pltpu.roll(w2, 4, 0), w2)
        hm = jnp.uint32(0xFFFF0000 if s % 2 else 0x0000FFFF)
        m1 = wide(jnp.where(sub8 == s // 2 + 4 * b1, hm, jnp.uint32(0)))
        m2 = wide(jnp.where(sub8 == s // 2 + 4 * (1 - b1), hm, jnp.uint32(0)))
        cp = cp | (w1 & m1) | (w2 & m2)
        for hf, ar in enumerate((jnp.where(b1 == 1, a2, a1), jnp.where(b1 == 1, a1, a2))):
            g8 = pl.multiple_of(((ar >> 3) << 3) + (L0 + DEF), 8)
            cx[hf] = jnp.where(wide(sub8 == s), x_v[pl.ds(g8, 8), :].astype(F32), cx[hf])
    cand_p = pltpu.bitcast(cp, BF16)
    cand_x = jnp.concatenate(cx, axis=0)
    id1 = key_row(jnp.broadcast_to(p1, (8, LANES)))
    id2 = key_row(jnp.broadcast_to(p2_, (8, LANES)))
    up = (((id1 - L0) >> 3) & 1) == 1
    old_slot = (jnp.logical_and(sub8 >= 6, up), jnp.logical_and(sub8 >= 6, jnp.logical_not(up)))
    old_id = jnp.where(sub8 == 6, key_row(oldk[0]), key_row(oldk[1]))
    ids_lo = jnp.where(old_slot[0], old_id, jnp.where(up, id2, id1))
    ids_hi = jnp.where(old_slot[1], old_id, jnp.where(up, id1, id2))

    st = dict(top1=top1, top2=top2, pend=[], step=0, sent=0)

    def gated(v):
        tok = None
        while st["pend"] and st["pend"][0][0] <= st["step"]:
            t = st["pend"].pop(0)[1]
            tok = t if tok is None else tok | t
        if tok is None:
            return v
        u = pltpu.bitcast(v, U32)
        return pltpu.bitcast(jnp.concatenate([u[:, 0:LANES] | tok, u[:, LANES:]], axis=1), BF16)

    def o_units():
        for ci, n in enumerate(OCL):
            r0 = sum(OCL[:ci])
            lhs = pltpu.bitcast(pqn_v[r0 // 2:(r0 + n) // 2, :], BF16)
            halves = []
            for c0 in range(0, NC, ONT):
                acc = x_v[DEF + L0 + r0:DEF + L0 + r0 + n, c0 * LANES:(c0 + ONT) * LANES].astype(F32)
                ks = (4 // ONT) * LANES
                for k0 in range(0, D, ks):
                    w = jnp.concatenate([m_tile(c, k0, ks) for c in range(c0, c0 + ONT)], axis=1)
                    acc = acc + jnp.dot(lhs[:, k0:k0 + ks], w, preferred_element_type=F32)
                    if k0 + ks == D:
                        halves.append(acc)
                        if len(halves) == NC // ONT:
                            last = r0 + n == RL
                            tk = [] if last else toks
                            st["top1"], st["top2"] = ln2_part(
                                jnp.concatenate(halves, axis=1), x_v, ln2_v, out_v, DEF + L0 + r0, -DEF, None,
                                st["top1"], st["top2"], tk, lag=n if last else LAG_L, is_h=True, fast=last)
                            if GLAG[ci] is not None:
                                st["pend"].append((st["step"] + GLAG[ci],
                                                   pltpu.bitcast(jnp.broadcast_to(st["top1"], (8, LANES)), U32) & zero_u))
                            if last:
                                out_copy(L0 + st["sent"], r0 + n - st["sent"], 2).start()
                            elif r0 + n in OUT_AT:
                                out_copy(L0 + st["sent"], r0 + n - st["sent"], 1).start()
                                st["sent"] = r0 + n
                    yield

    res = {}

    def c_units():
        parts = []
        for c in range(NC):
            parts.append(jnp.dot(cand_p, m_tile(c, 0, D), preferred_element_type=F32))
            yield
        xs = _layernorm(cand_x + jnp.concatenate(parts, axis=1))
        old = jnp.where(wide(sub8 == 6), oldx[0], oldx[1])
        res["xs"] = jnp.concatenate([jnp.where(wide(old_slot[hf]), old, xs[hf * 8:(hf + 1) * 8, :])
                                     for hf in range(2)], axis=0).astype(BF16)

    def f_units():
        xs = res["xs"]
        acts = []
        for j in range(F // LANES):
            cs = slice(j * LANES, (j + 1) * LANES)
            g = jnp.dot(gated(xs), wload(wg_v, 0, D, cs), preferred_element_type=F32)
            yield
            u = jnp.dot(xs, wload(wu_v, 0, D, cs), preferred_element_type=F32)
            acts.append((g * jax.nn.sigmoid(g) * u).astype(BF16))
            yield
        act = jnp.concatenate(acts, axis=1)
        zf = pltpu.bitcast(zero_u, F32)
        ys = []
        KF = (F // D) * D
        for c in range(0, NC, 2):
            acc = jnp.concatenate([jnp.concatenate([zf, zf], axis=0)] * 2, axis=1)
            acc = acc + jnp.dot(gated(act[:, KF:]), wload(wd_v, KF, F - KF, slice(c * LANES, (c + 2) * LANES)),
                                preferred_element_type=F32)
            yield
            for cc in range(2):
                y = acc[:, cc * LANES:(cc + 1) * LANES]
                for k0 in range(0, KF, D):
                    y = y + jnp.dot(gated(act[:, k0:k0 + D]),
                                    wload(wd_v, k0, D, slice((c + cc) * LANES, (c + cc + 1) * LANES)),
                                    preferred_element_type=F32)
                    yield
                ys.append(y)
        res["y"] = jnp.concatenate(ys, axis=1)

    ou = o_units()

    def o_step():
        next(ou, None)
        st["step"] += 1

    for _ in range(NPRE):
        o_step()
    for _ in c_units():
        o_step()
    for _ in range(NGAP):
        o_step()
    for _ in f_units():
        o_step()
    for _ in ou:
        pass

    keyv = best2(st["top1"], st["top2"])
    idx = [jnp.clip(key_row(kk[0, 0]), 0, S - 1) for kk in keyv]
    grp = [pl.multiple_of((ii >> 3) << 3, 8) for ii in idx]
    vgrp = [pl.multiple_of(gg + DEF, 8) for gg in grp]
    y = res["y"]
    hits = None
    yrows = []
    for c in range(2):
        m_lo = ids_lo == key_row(keyv[c])
        m_hi = ids_hi == key_row(keyv[c])
        yrows.append(subsum(jnp.where(wide(m_lo), y[0:8, :], 0.0) + jnp.where(wide(m_hi), y[8:16, :], 0.0)))
        hit = submax(jnp.where(m_lo | m_hi, 1, 0))
        hits = hit if hits is None else hits + hit
    hit_all = hits[0, 0] == 2

    tail0 = L0 + st["sent"]
    tail_copy = out_copy(tail0, S - tail0, 2)
    in_tail = jnp.maximum(grp[0], grp[1]) >= tail0
    two_groups = grp[1] != grp[0]

    def fix_copy(c):
        return out_copy(grp[c], 8, 3 + c)

    def finish(ysel):
        for c in range(2):
            hi = keyv[c] & jnp.int32(-65536)
            score = pltpu.bitcast(hi ^ ((hi >> 31) & 0x7FFF0000), F32)
            sel = (key_row(keyv[c]) & 7) == sub8
            upd = jnp.where(wide(sel), ysel[c] * wide(jax.nn.sigmoid(score)), 0.0)
            out_v[pl.ds(vgrp[c], 8), :] = (out_v[pl.ds(vgrp[c], 8), :].astype(F32) + upd).astype(BF16)
        fix_copy(0).start()

        @pl.when(two_groups)
        def _():
            fix_copy(1).start()

    out_copy(0, L0, 0).wait()
    out_copy(L0, tail0 - L0, 1).wait()

    @pl.when(in_tail)
    def _():
        tail_copy.wait()

    @pl.when(hit_all)
    def _():
        finish(yrows)

    @pl.when(jnp.logical_not(hit_all))
    def _():
        xsel = jnp.concatenate([ln2_v[pl.ds(vgrp[c], 8), :] for c in range(2)], axis=0)

        def ffn_tile(j, acc):
            cs = pl.ds(pl.multiple_of(j * LANES, LANES), LANES)
            g = jnp.dot(xsel, wload(wg_v, 0, D, cs), preferred_element_type=F32)
            u = jnp.dot(xsel, wload(wu_v, 0, D, cs), preferred_element_type=F32)
            a = (g * jax.nn.sigmoid(g) * u).astype(BF16)
            wd_t = pltpu.bitcast(wd_v[pl.ds(pl.multiple_of(j * (LANES // 2), LANES // 2), LANES // 2), 0:D], BF16)
            return acc + jnp.dot(a, wd_t, preferred_element_type=F32)

        yf = lax.fori_loop(0, F // LANES, ffn_tile, jnp.zeros((16, D), F32))
        finish([yf[0:8, :], yf[8:16, :]])

    @pl.when(jnp.logical_not(in_tail))
    def _():
        tail_copy.wait()

    fix_copy(0).wait()

    @pl.when(two_groups)
    def _():
        fix_copy(1).wait()


@jax.jit
def pallas_sequential_preLN__linear_attn_block__moe_arch_mod__prompt_kernel(
    A_x: jax.Array,
    A_wqkv: jax.Array,
    A_wo: jax.Array,
    B_x: jax.Array,
    B_w_r: jax.Array,
    B_w_gate: jax.Array,
    B_w_up: jax.Array,
    B_w_down: jax.Array,
):
    del B_x
    x = A_x.reshape(S, D)
    wr = B_w_r.reshape(NC, LANES)
    any_spec = pl.BlockSpec(memory_space=pl.ANY)
    out = pl.pallas_call(
        _kernel,
        out_shape=jax.ShapeDtypeStruct((S, D), BF16),
        in_specs=[any_spec] * 7,
        out_specs=any_spec,
        scratch_shapes=[
            pltpu.VMEM((S + DEF, D), BF16),
            pltpu.VMEM((D // 2, D), U32),
            pltpu.VMEM((3, D // 2, D), U32),
            pltpu.VMEM((NC, LANES), BF16),
            pltpu.VMEM((2, D // 2, F + LANES), U32),
            pltpu.VMEM((F // 2, D + LANES), U32),
            pltpu.VMEM(((S + TB) // 2, D), U32),
            pltpu.VMEM((D // 2, max(TB, P0)), U32),
            pltpu.VMEM((H * ZP, LANES), F32),
            pltpu.VMEM((D, D), F32),
            pltpu.VMEM((NC, DH * PSTR, LANES), U32),
            pltpu.VMEM((D // 2, LANES), U32),
            pltpu.VMEM((NC, DH * PSTR, LANES), U32),
            pltpu.VMEM((max(TB2, RL) // 2, D), U32),
            pltpu.VMEM((DEF, D), F32),
            pltpu.VMEM((2, S + DEF, D), BF16),
            pltpu.VMEM((8, LANES), U32),
            pltpu.SemaphoreType.DMA((NSEM,)),
        ],
        compiler_params=pltpu.CompilerParams(vmem_limit_bytes=110 * 1024 * 1024, disable_bounds_checks=True,
                                             disable_semaphore_checks=True),
    )(x, A_wqkv, A_wo, wr, B_w_gate, B_w_up, B_w_down)
    return out.reshape(1, S, D)
```

```python
import jax
import jax.numpy as jnp
from jax import lax
import jax.experimental.pallas as pl
import jax.experimental.pallas.tpu as pltpu


S = 2048
D = 1024
F = 3584
H = 32
DH = D // H
LANES = 128
NC = D // LANES
HD = D // 2

LA = 1
LO = 1
NA, NO = 2 ** LA, 2 ** LO
DA, DO = D // NA, D // NO
P0 = 512
PB = S - P0
TX = 256
TB = 512
NB1 = PB // TB
TB2 = 544
NB2 = 3
QA = 288
OCH = (96, 128, 96, 96, 128)
DEF = OCH[-1]
L0 = NB2 * TB2
RL = S - L0
QS = (288, 128)
OCL = (32, 64, 64, 64, 64, 64, 64)
ONT = 2
NPRE = 20
NGAP = 8
OUT_AT = (160, 288, 352)
LNU = 8
LAG = 5
LAG_L = 3
L1LAG = 3
L1LAG0 = 4
WKLAG = 4
WK5 = 64
WKW = 128
KAT = 0
KGATE = 1
WKLAG6 = 3
KLN = (5, 16, 27, 38)
LNGATE = ((0, 44), (1, 55), (2, -1))
C6K = (None, None, 9, 19)
C6G = (31, 58)
WQ4 = 256
C6U = 10
P1U = 12
LNW = 128
WQLAG = 2
WQC = 2
ZG = 2
QGATE = True
GLAG = (None, None, None, None, None, 20, 8)
PSTR = 36

F32 = jnp.float32
BF16 = jnp.bfloat16
U32 = jnp.uint32
I32 = jnp.int32

XP = ((PB, 128), (PB + 128, 128), (PB + 256, 256), (0, TB), (TB, PB - TB))
WKP = ((0, 128), (128, 128), (256, 256), (512, 512))

SEM_X = 0
SEM_WK = SEM_X + len(XP)
SEM_WQ = SEM_WK + len(WKP)
SEM_W3 = SEM_WQ + 1
SEM_WR = SEM_W3 + 1
SEM_WGU = SEM_WR + 1
SEM_WD = SEM_WGU + 1
SEM_OUT = SEM_WD + 1
NSEM = SEM_OUT + 5

INT_MIN = -(2 ** 31)


def _layernorm(x, tok=None, w=None):
    s0 = x[:, 0:LANES]
    if tok is not None:
        s0 = s0 + jnp.concatenate([tok] * (x.shape[0] // 8), axis=0)
    for c in range(1, NC):
        s0 = s0 + x[:, c * LANES:(c + 1) * LANES]
    mu = jnp.sum(s0, axis=-1, keepdims=True) * (1.0 / D)
    xc = x - mu
    var = jnp.sum(xc * xc, axis=-1, keepdims=True) * (1.0 / D)
    rstd = lax.rsqrt(var + 1e-5)
    if w is None:
        return xc * rstd
    return xc * rstd, jnp.sum(xc * w, axis=-1, keepdims=True) * rstd


def _ln_stats(x, tok=None):
    s0 = x[:, 0:LANES]
    if tok is not None:
        s0 = s0 + tok
    for c in range(1, NC):
        s0 = s0 + x[:, c * LANES:(c + 1) * LANES]
    mu = jnp.sum(s0, axis=-1, keepdims=True) * (1.0 / D)
    xc = x - mu
    var = jnp.sum(xc * xc, axis=-1, keepdims=True) * (1.0 / D)
    return mu, lax.rsqrt(var + 1e-5)


def _phi(t):
    return jnp.where(t > 0, t + 1.0, jnp.exp(t)) + 1e-6


class _Stage:
    def __init__(self, ref):
        self.ref, self.r, self.c, self.h = ref, 0, 0, 0

    def pack(self, val):
        n, w = val.shape[0] // 2, val.shape[1]
        if self.c + w > self.ref.shape[1] or n != self.h:
            self.r, self.c, self.h = self.r + self.h, 0, n
        idx = (slice(self.r, self.r + n), slice(self.c, self.c + w))
        self.c += w
        self.ref[idx] = pltpu.bitcast(val.astype(BF16), U32)
        return self.ref[idx]


def _store_heads(ref, val, head0, stage):
    u = stage.pack(val)
    r = ref.shape[1] // PSTR
    for hh in range(u.shape[0] // r):
        for c in range(u.shape[1] // LANES):
            ref[c, pl.ds(head0 + hh, r, stride=PSTR), :] = u[hh * r:(hh + 1) * r, c * LANES:(c + 1) * LANES]
    return u


def _load_packed(ref, n0=0, n1=D, c0=0, c1=NC):
    cols = []
    for c in range(c0, c1):
        w = jnp.concatenate([ref[c, p * PSTR:p * PSTR + H, :] for p in range(n0 // (2 * H), n1 // (2 * H))], axis=0)
        cols.append(pltpu.bitcast(w, BF16))
    return jnp.concatenate(cols, axis=1)


def _quads(b):
    h = len(b) // 2
    return [[r[j * h:(j + 1) * h] for r in b[i * h:(i + 1) * h]] for i in range(2) for j in range(2)]


def _badd(x, y):
    return [[a + b for a, b in zip(rx, ry)] for rx, ry in zip(x, y)]


def _bsub(x, y):
    return [[a - b for a, b in zip(rx, ry)] for rx, ry in zip(x, y)]


def _a_set(b):
    if len(b) == 1:
        return [b[0][0]]
    q11, q12, q21, q22 = _quads(b)
    ops = (_badd(q11, q22), _badd(q21, q22), q11, q22, _badd(q11, q12), _bsub(q21, q11), _bsub(q12, q22))
    return [x for o in ops for x in _a_set(o)]


def _b_set(b):
    if len(b) == 1:
        return [b[0][0]]
    q11, q12, q21, q22 = _quads(b)
    ops = (_badd(q11, q22), q11, _bsub(q12, q22), _bsub(q21, q11), q22, _badd(q11, q12), _badd(q21, q22))
    return [x for o in ops for x in _b_set(o)]


def _b_in_a(i, levels):
    perm = (0, 2, 6, 5, 3, 4, 1)
    return sum(perm[(i // 7 ** l) % 7] * 7 ** l for l in range(levels))


def _strassen(prod, levels, base=0):
    if levels == 0:
        return [[prod(base)]]

    def m(i):
        return _strassen(prod, levels - 1, base * 7 + i)

    m2 = m(2)
    m4 = m(4)
    c12 = _badd(m2, m4)
    m3 = m(3)
    c11 = _bsub(m3, m4)
    m1 = m(1)
    c21 = _badd(m1, m3)
    c22 = _bsub(m2, m1)
    m0 = m(0)
    c11 = _badd(c11, m0)
    c22 = _badd(c22, m0)
    c11 = _badd(c11, m(6))
    c22 = _badd(c22, m(5))
    return [a + b for a, b in zip(c11, c12)] + [a + b for a, b in zip(c21, c22)]


def _goff(i, levels):
    return int(format(i, "0%db" % levels)[::-1], 2) if levels else 0


def _blocks(rows, n):
    w = rows[0].shape[1] // n
    return [[r[:, j * w:(j + 1) * w] for j in range(n)] for r in rows]


def _or_all(vals):
    acc = None
    for v in vals:
        v = v if v.dtype == U32 else pltpu.bitcast(v, U32)
        for g in range(v.shape[0] // 8):
            for c in range(v.shape[1] // LANES):
                p = v[g * 8:(g + 1) * 8, c * LANES:(c + 1) * LANES]
                acc = p if acc is None else acc | p
    return acc


def _raw_ops(levels):
    n = 2 ** levels
    names = [[_Tag((i, j)) for j in range(n)] for i in range(n)]
    return {op: t.ij for op, t in enumerate(_b_set(names)) if t.ij is not None}


class _Tag:
    def __init__(self, ij):
        self.ij = ij

    def __add__(self, other):
        return _Tag(None)

    __sub__ = __add__


def _store_set(ref, val, head, levels, transposed, stage, c0=0, nc=None, tok=None, skip=()):
    n = 2 ** levels
    dn, w = DH // n, D // n
    nc = NC // n if nc is None else nc
    b = [[val[i * dn:(i + 1) * dn, j * w + c0 * LANES:j * w + (c0 + nc) * LANES] for j in range(n)]
         for i in range(n)]
    if tok is not None:
        t = jnp.concatenate([jnp.concatenate([tok] * (dn // 8), axis=0)] * nc, axis=1)
        for i in range(n):
            b[i][i] = b[i][i] + t
    if transposed:
        b = [list(r) for r in zip(*b)]
    return _or_all([_store_heads(ref.at[op, c0:c0 + nc], x, head, stage)
                    for op, x in enumerate(_b_set(b)) if op not in skip])


def _kernel(x_hbm, wqkv_hbm, wo_hbm, wr_hbm, wg_hbm, wu_hbm, wd_hbm, out_hbm,
            x_v, wk_v, wq_v, w3_v, wr_v, wgu_v, wd_v,
            ln1_v, xs_v, wks_v, pkt_v, pks_v, zacc_v, zp_v, g_v, wqs_v, mp_v, ms_v, pqn_v, pqs_v, attn_v, lo_v, stg_v, zero_v,
            sems):

    ln2_v, out_v = lo_v.at[0], lo_v.at[1]

    wqkv_hbm, wo_hbm, wg_hbm, wu_hbm, wd_hbm = (r.bitcast(U32) for r in (wqkv_hbm, wo_hbm, wg_hbm, wu_hbm, wd_hbm))

    def wload(ref, r0, nr, cols):
        return pltpu.bitcast(ref[r0 // 2:(r0 + nr) // 2, cols], BF16)

    wv_v, wo_v = w3_v.at[0], w3_v.at[1]
    wg_v, wu_v = wgu_v.at[0], wgu_v.at[1]

    def x_copy(i):
        r0, n = XP[i]
        return pltpu.make_async_copy(x_hbm.at[pl.ds(r0, n), :], x_v.at[pl.ds(DEF + r0, n), :], sems.at[SEM_X + i])

    def out_copy(r0, n, s):
        return pltpu.make_async_copy(out_v.at[pl.ds(DEF + r0, n), :], out_hbm.at[pl.ds(r0, n), :],
                                     sems.at[SEM_OUT + s])

    def wk_copy(j):
        c0, n = WKP[j]
        return pltpu.make_async_copy(wqkv_hbm.at[:, pl.ds(D + c0, n)], wk_v.at[:, pl.ds(c0, n)],
                                     sems.at[SEM_WK + j])

    wq_copy = pltpu.make_async_copy(wqkv_hbm.at[:, pl.ds(0, D)], wq_v, sems.at[SEM_WQ])
    wr_copy = pltpu.make_async_copy(wr_hbm, wr_v, sems.at[SEM_WR])
    wd_copy = pltpu.make_async_copy(wd_hbm, wd_v.at[:, pl.ds(0, D)], sems.at[SEM_WD])
    wg_copy = pltpu.make_async_copy(wg_hbm, wg_v.at[:, pl.ds(0, F)], sems.at[SEM_WGU])
    wu_copy = pltpu.make_async_copy(wu_hbm, wu_v.at[:, pl.ds(0, F)], sems.at[SEM_WGU])

    x_copy(0).start()
    wk_copy(0).start()
    x_copy(1).start()
    wr_copy.start()
    for j in range(1, len(WKP)):
        wk_copy(j).start()
    for j in range(2, len(XP)):
        x_copy(j).start()
    wq_copy.start()
    pltpu.make_async_copy(wqkv_hbm.at[:, pl.ds(2 * D, D)], wv_v, sems.at[SEM_W3]).start()
    pltpu.make_async_copy(wo_hbm, wo_v, sems.at[SEM_W3]).start()
    wg_copy.start()
    wu_copy.start()
    wd_copy.start()

    def ln1_rows(xr, xr0, lnr, r0, n):
        ln = _layernorm(xr[xr0:xr0 + n, :].astype(F32)).astype(BF16)
        lnr[r0 // 2:(r0 + n) // 2, :] = pltpu.bitcast(ln, U32)

    def ln1_set(xr, xr0, xsr, a0, n, lag, done, extra=()):
        zero_u = zero_v[...]
        toks, stats, jobs = [], [], []
        extra = list(extra)
        per = -(-len(extra) // (n // LNU - lag))

        def piece(j0, st, c0):
            def job():
                blks = []
                for i in range(NA):
                    g = 2 * _goff(i, LA)
                    blks.append([jnp.concatenate(
                        [(xr[xr0 + (j0 + g + t) * LNU:xr0 + (j0 + g + t + 1) * LNU,
                             f * DA + c0:f * DA + c0 + LNW].astype(F32) - st[g + t][0]) * st[g + t][1]
                         for t in range(2)], axis=0) for f in range(NA)])
                r = (a0 + (j0 // (2 * NA)) * 16) // 2
                ops = _a_set(blks)
                for op, v in enumerate(ops):
                    xsr.at[op][r:r + 8, c0:c0 + LNW] = pltpu.bitcast(v.astype(BF16), U32)
                return _or_all([ops[0], ops[-1], ops[-2]])
            return job

        for j in range(n // LNU):
            x = xr[xr0 + j * LNU:xr0 + (j + 1) * LNU, :].astype(F32)
            mu, rstd = _ln_stats(x, toks[-lag] if len(toks) >= lag else None)
            dep = pltpu.bitcast(jnp.broadcast_to(rstd, (LNU, LANES)), U32)
            for _ in range(-(-(DA // LNW) // (2 * NA))):
                if jobs:
                    dep = dep | jobs.pop(0)()
            for _ in range(per):
                if extra and len(toks) >= lag:
                    dep = dep | extra.pop(0)(toks[-lag])
            toks.append(pltpu.bitcast(dep & zero_u, F32))
            stats.append((mu, rstd))
            if len(stats) == 2 * NA:
                jobs += [piece(j + 1 - 2 * NA, stats, c0) for c0 in range(0, DA, LNW)]
                stats = []
            done.append(pltpu.bitcast(toks[-1], U32))
            yield
        done.append(_or_all(done[-lag:] + [job() & zero_u for job in jobs]))

    def run_chained(jobs, lag):
        zero_u = zero_v[...]
        toks = []
        for job in jobs:
            dep = job(toks[-lag] if len(toks) >= lag else None)
            toks.append(pltpu.bitcast(pltpu.roll(dep & zero_u, 1, 1), F32))
            yield

    def advance(gen, n=None):
        while n is None or n > 0:
            if next(gen, gen) is gen:
                return
            n = None if n is None else n - 1

    def ln1_load(lnr, r0, n):
        return pltpu.bitcast(lnr[r0 // 2:(r0 + n) // 2, :], BF16)

    def gate(v, tok):
        if tok is None:
            return v
        u = pltpu.bitcast(v, U32)
        top = u[0:8, 0:LANES] | tok
        if u.shape[1] > LANES:
            top = jnp.concatenate([top, u[0:8, LANES:]], axis=1)
        return pltpu.bitcast(jnp.concatenate([top, u[8:, :]], axis=0) if u.shape[0] > 8 else top, BF16)

    def k_mm(lnr, r0, n, c0, nc, tok=None):
        return jnp.dot(gate(ln1_load(lnr, r0, n), tok), wload(wk_v, 0, D, slice(c0, c0 + nc)), preferred_element_type=F32)

    def z_acc(pkts, c0, first=False):
        zs = None
        for pkt in pkts:
            for j in range(pkt.shape[1] // LANES):
                p = pkt[:, j * LANES:(j + 1) * LANES]
                zs = p if zs is None else zs + p
        if first:
            zacc_v[c0:c0 + zs.shape[0], :] = zs
        else:
            zacc_v[c0:c0 + zs.shape[0], :] += zs

    def k_post(k, p0, c0, first=False):
        n, nc = k.shape
        pkt = _phi(k).T
        pkt_v[c0 // 2:(c0 + nc) // 2, p0:p0 + n] = pltpu.bitcast(pkt.astype(BF16), U32)
        z_acc([pkt], c0, first)

    def g_acc(lnr, r0, n, c0, nc, first=False, tok=None):
        g = jnp.dot(gate(pltpu.bitcast(pkt_v[c0 // 2:(c0 + nc) // 2, r0:r0 + n], BF16), tok), ln1_load(lnr, r0, n),
                    preferred_element_type=F32)
        if first:
            g_v[c0:c0 + nc, :] = g
        else:
            g_v[c0:c0 + nc, :] += g

    attn_v[...] = jnp.zeros_like(attn_v)
    x_v[0:DEF, :] = jnp.zeros((DEF, D), BF16)
    zero_v[...] = jnp.zeros_like(zero_v)

    def k0(c0, nc):
        k_post(k_mm(ln1_v, 0, TX, c0, nc), 0, c0, first=True)

    def g0(c0, nc):
        g_acc(ln1_v, 0, TX, c0, nc, first=True)

    x_copy(0).wait()
    ln1_rows(x_v, DEF + PB, ln1_v, 0, 128)
    wk_copy(0).wait()
    ka = k_mm(ln1_v, 0, 128, 0, 128)
    x_copy(1).wait()
    wr_copy.wait()
    ln1_rows(x_v, DEF + PB + 128, ln1_v, 128, 128)
    k_post(ka, 0, 0, first=True)
    g_acc(ln1_v, 0, 128, 0, 128, first=True)
    wk_copy(1).wait()
    k_post(k_mm(ln1_v, 128, 128, 0, 128), 128, 0)
    k0(128, 128)
    g_acc(ln1_v, 128, 128, 0, 128)
    wk_copy(2).wait()
    k0(256, 256)
    g0(128, 128)
    g0(256, 256)
    wk_copy(3).wait()

    wk_raw = _raw_ops(LA)

    def wk_job(r0, c0):
        def job(tok):
            def cut(i, j):
                return wk_v[(i * DA + r0) // 2:(i * DA + r0) // 2 + 8, j * DA + c0:j * DA + c0 + WKW]

            rows = [pltpu.bitcast(jnp.concatenate([cut(i, j) for j in range(NA)], axis=1), BF16).astype(F32)
                    for i in range(NA)]
            blks = _blocks(rows, NA)
            if tok is not None:
                t = jnp.concatenate([jnp.concatenate([tok, tok], axis=0)] * (WKW // LANES), axis=1)
                for i in range(NA):
                    blks[i][i] = blks[i][i] + t
            ops = [(op, v) for op, v in enumerate(_b_set(blks)) if op not in wk_raw]
            for op, v in ops:
                wks_v.at[op][r0 // 2:r0 // 2 + 8, c0:c0 + WKW] = pltpu.bitcast(v.astype(BF16), U32)
            for op, ij in wk_raw.items():
                wks_v[op, r0 // 2:r0 // 2 + 8, c0:c0 + WKW] = cut(*ij)
            return _or_all([ops[0][1], ops[1][1], ops[2][1]])
        return job

    wk_jobs = [wk_job(r0, c0) for r0 in range(0, DA, 16) for c0 in range(0, DA, WKW)]
    bg = run_chained(wk_jobs[:WK5], WKLAG)
    advance(bg, WK5 // 3)
    k0(512, 256)
    advance(bg, WK5 // 3)
    k0(768, 256)
    advance(bg)
    g0(512, 256)
    x_copy(2).wait()
    x_copy(3).wait()
    ln1_rows(x_v, DEF + PB + TX, ln1_v, TX, TX)
    g0(768, 256)
    done = []
    bg = ln1_set(x_v, DEF, xs_v, 0, TB, L1LAG0, done)
    for c0 in range(0, D, WQ4):
        advance(bg, C6U)
        u = C6K[c0 // WQ4]
        k_post(k_mm(ln1_v, TX, TX, c0, WQ4, None if u is None else done[u]), TX, c0)
    advance(bg)
    advance(run_chained(wk_jobs[WK5:], WKLAG6))
    g_acc(ln1_v, TX, TX, 0, HD, tok=done[C6G[0]])
    g_acc(ln1_v, TX, TX, HD, HD, tok=done[C6G[1]])

    MA = TB // NA
    NWK = LANES * NA // 2

    def xs_load(xsr, op, a0, m, cols=slice(None)):
        return pltpu.bitcast(xsr[op, a0 // 2:(a0 + m) // 2, cols], BF16)

    def k_step(xsr, j0, tok, at):
        cb = _strassen(lambda i: jnp.dot(gate(xs_load(xsr, i, 0, MA), tok if i == at else None),
                                         pltpu.bitcast(wks_v[i, :, j0:j0 + NWK], BF16),
                                         preferred_element_type=F32), LA)
        pt = [[_phi(cb[i][f]).T for i in range(NA)] for f in range(NA)]
        for f in range(NA):
            z_acc(pt[f], f * DA + j0)
        ops = _a_set(pt)
        for op, v in enumerate(ops):
            pks_v.at[op][j0 // 2:(j0 + NWK) // 2, :] = pltpu.bitcast(v.astype(BF16), U32)
        return _or_all([ops[0][0:8, :], ops[-1][NWK - 8:NWK, :], ops[-2][NWK - 8:NWK, :]]) & zero_v[...]

    def g_step(xsr, f0, nf, c0, nc, tok=None):
        cb = _strassen(lambda i: jnp.dot(gate(pltpu.bitcast(pks_v[i, f0 // 2:(f0 + nf) // 2, :], BF16),
                                              tok if i == (7 ** LA - 1) // 3 else None),
                                         xs_load(xsr, _b_in_a(i, LA), 0, MA, slice(c0, c0 + nc)),
                                         preferred_element_type=F32), LA)
        for f in range(NA):
            for c in range(NA):
                g_v[f * DA + f0:f * DA + f0 + nf, c * DA + c0:c * DA + c0 + nc] += cb[f][c]

    def p1(i, carry):
        xsr = xs_v.at[:, pl.ds(pl.multiple_of(i * (MA // 2), MA // 2), MA), :]
        xr = x_v.at[pl.ds(pl.multiple_of((i + 1) * TB, TB), TB + DEF), :]

        def wq_job(j, hh, c0):
            def job(tok):
                c = jnp.minimum(i * 3 + j, NC - 1)
                if j not in wqt:
                    w = pltpu.bitcast(wq_v[:, pl.ds(pl.multiple_of(c * LANES, LANES), LANES)], BF16)
                    wqt[j] = gate(w, None if tok is None else pltpu.bitcast(tok, U32)).astype(F32).T
                return _store_set(wqs_v, wqt[j][hh * DH:(hh + 1) * DH, :], c * (LANES // DH) + hh,
                                  LA, True, stage, c0, WQC, tok)
            return job

        wqt = {}
        stage = _Stage(stg_v)
        done = []
        bg = ln1_set(xr, DEF, xsr, MA, TB, L1LAG, done)
        kt = [None]
        for j0 in range(0, DA, NWK):
            advance(bg, P1U)
            tok = kt[-1]
            if KLN[j0 // NWK] is not None:
                tok = done[KLN[j0 // NWK]] if tok is None else tok | done[KLN[j0 // NWK]]
            kt.append(k_step(xsr, j0, tok, KAT))
        toks = {}
        advance(bg)
        advance(run_chained([wq_job(j, hh, c0) for j in range(3) for hh in range(LANES // DH)
                             for c0 in range(0, NC // NA, WQC)],
                            WQLAG))
        toks[KGATE] = kt[-1] if KGATE not in toks else toks[KGATE] | kt[-1]
        for pos, unit in LNGATE:
            toks[pos] = done[unit] if pos not in toks else toks[pos] | done[unit]
        gf = max(DA // 2, NWK)
        step = 0
        for f0 in range(0, DA, gf):
            for c0 in range(0, DA, 2 * LANES):
                g_step(xsr, f0, gf, c0, 2 * LANES, toks.get(step))
                step += 1
        return carry

    x_copy(4).wait()
    wq_copy.wait()
    lax.fori_loop(0, NB1, p1, 0)

    pltpu.make_async_copy(w3_v, w3_v, sems.at[SEM_W3]).wait()
    zero_u = zero_v[...]
    stage = _Stage(stg_v)
    za = zacc_v[...]
    zh = za.astype(BF16).astype(F32)
    _store_heads(zp_v, jnp.concatenate([zh, za - zh], axis=1), 0, stage)
    zp = _load_packed(zp_v, 0, D, 0, 2).astype(F32)
    zrow = jnp.sum((zp[:, 0:LANES] + zp[:, LANES:]).T, axis=0, keepdims=True)
    wr8 = wr_v[...].astype(F32)
    wr_row = jnp.concatenate([wr8[c:c + 1, :] for c in range(NC)], axis=1)

    row_h = lax.broadcasted_iota(I32, (LANES, LANES), 0) // DH
    col_h = lax.broadcasted_iota(I32, (LANES, LANES), 1) // DH
    diag = row_h == col_h

    m_raw = _raw_ops(LO)

    def kv_part(c):
        cs = slice(c * LANES, (c + 1) * LANES)
        tok = None
        if c == ZG:
            tok = _or_all([pltpu.bitcast(jnp.broadcast_to(zrow, (8, D)), U32)]) & zero_u
        kv = jnp.dot(gate(g_v[cs, :].astype(BF16), tok), wload(wv_v, 0, D, cs), preferred_element_type=F32)
        return jnp.where(diag, kv, 0.0)

    def m_part(c, kv):
        m = jnp.dot(kv.astype(BF16), wload(wo_v, c * LANES, LANES, slice(None)), preferred_element_type=F32)
        _store_heads(mp_v, m, c * (LANES // DH), stage)
        for hh in range(LANES // DH):
            _store_set(ms_v, m[hh * DH:(hh + 1) * DH, :], c * (LANES // DH) + hh, LO, False, stage, skip=m_raw)

    kv_prev = None
    for c in range(NC + 1):
        kv = kv_part(c) if c < NC else None
        if c:
            m_part(c - 1, kv_prev)
        kv_prev = kv

    def make_key(score, row):
        b = pltpu.bitcast(score, I32)
        srt = b ^ ((b >> 31) & 0x7FFFFFFF)
        return (srt & jnp.int32(-65536)) | (0xFFFF - row)

    def push_keys(key, top1, top2):
        for gidx in range(key.shape[0] // 8):
            kx = key[gidx * 8:(gidx + 1) * 8, :]
            top2 = jnp.maximum(top2, jnp.minimum(top1, kx))
            top1 = jnp.maximum(top1, kx)
        return top1, top2

    def colsum(t):
        acc = t[:, 0:LANES]
        for c in range(1, NC):
            acc = acc + t[:, c * LANES:(c + 1) * LANES]
        return acc

    even_lane = (lax.broadcasted_iota(I32, (1, LANES), 1) & 1) == 0

    def interleave(parts):
        return jnp.concatenate([p[g * 16:(g + 1) * 16, :] for g in range(parts[0].shape[0] // 16) for p in parts],
                               axis=0)

    def q_part(xsr, l0, r0, n, hint=None, tok=None):
        m = n // NA
        cols = [[[] for _ in range(NA)] for _ in range(NA)]
        for j0 in range(0, DA, NWK):
            cb = _strassen(lambda i: lax.dot_general(
                gate(xs_load(xsr, i, (l0 + r0) // NA, m), tok if (j0 == 0 and i == (7 ** LA - 1) // 3) else None),
                _load_packed(wqs_v.at[i], j0, j0 + NWK, 0, NC // NA),
                (((1,), (1,)), ((), ())), preferred_element_type=F32), LA)
            for i in range(NA):
                for f in range(NA):
                    cols[i][f].append(cb[i][f])
        pqns = [None] * NA
        for i in range(NA):
            pq = _phi(jnp.concatenate([c for f in range(NA) for c in cols[i][f]], axis=1))
            den = colsum(pq * zrow)
            den = den + pltpu.roll(den, 2 * H, 1)
            den = den + jnp.where(even_lane, pltpu.roll(den, LANES - 1, 1), pltpu.roll(den, 1, 1))
            inv = 1.0 / (den + 1e-6)
            pqns[_goff(i, LA)] = pq * jnp.concatenate([inv] * NC, axis=1)
            if hint is not None:
                urow, wrc, p1, p2 = hint
                starts = [l0 + r0 + (g * NA + _goff(i, LA)) * 16 for g in range(m // 16)]
                xb = jnp.concatenate([x_v[DEF + t:DEF + t + 16, :] for t in starts], axis=0).astype(F32)
                num = jnp.sum(colsum(xb * wrc) + colsum(pq * urow) * inv, axis=-1, keepdims=True)
                row = jnp.concatenate([t + lax.broadcasted_iota(I32, (16, 1), 0) for t in starts], axis=0)
                hint = (urow, wrc) + push_keys(make_key(num, row), p1, p2)
        if hint is not None:
            pqn_v[r0 // 2:(r0 + n) // 2, :] = pltpu.bitcast(interleave(pqns).astype(BF16), U32)
            return hint[2:]
        rows = [interleave(pqns[_goff(i, LO)::NO]) for i in range(NO)]
        for op, v in enumerate(_a_set(_blocks(rows, NO))):
            pqs_v.at[op][r0 // NO // 2:(r0 + n) // NO // 2, :] = pltpu.bitcast(v.astype(BF16), U32)
        return None

    def m_operand(i, c0, c1):
        if i not in m_raw:
            return _load_packed(ms_v.at[i], 0, DO, c0, c1)
        bi, bj = m_raw[i]
        return _load_packed(mp_v, bi * DO, (bi + 1) * DO, bj * (NC // NO) + c0, bj * (NC // NO) + c1)

    def o_part(r0, n):
        a0, m = r0 // NO, n // NO
        nw = LANES * NO // 2
        cols = [[[] for _ in range(NO)] for _ in range(NO)]
        for c0 in range(0, NC // NO, nw // LANES):
            cb = _strassen(lambda i: jnp.dot(
                pltpu.bitcast(pqs_v[i, a0 // 2:(a0 + m) // 2, :], BF16),
                m_operand(i, c0, c0 + nw // LANES), preferred_element_type=F32), LO)
            for i in range(NO):
                for f in range(NO):
                    cols[i][f].append(cb[i][f])
        parts = [None] * NO
        for i in range(NO):
            parts[_goff(i, LO)] = jnp.concatenate([c for f in range(NO) for c in cols[i][f]], axis=1)
        return interleave(parts)

    def ln2_unit(attn, xr, l2r, outr, r0, row0, valid, top1, top2, tok, fast=False, is_h=False):
        n = attn.shape[0]
        h = attn if is_h else xr[r0:r0 + n, :].astype(F32) + attn
        if fast:
            ln2, r = _layernorm(h, tok, wr_row)
        else:
            ln2 = _layernorm(h, tok)
            r = jnp.sum(ln2 * wr_row, axis=-1, keepdims=True)
        l2r[r0:r0 + n, :] = ln2.astype(BF16)
        res = h + ln2
        outr[r0:r0 + n, :] = res.astype(BF16)
        r = r.astype(BF16).astype(F32) + 0.0
        key = make_key(r, (row0 + r0) + lax.broadcasted_iota(I32, (n, 1), 0))
        if valid is not None:
            key = jnp.where(valid, key, INT_MIN)
        top1, top2 = push_keys(key, top1, top2)
        ntok = pltpu.bitcast(pltpu.bitcast(jnp.broadcast_to(r[n - 8:n, :], (8, LANES)), U32) & zero_u, F32)
        return top1, top2, ntok

    def ln2_part(attn, xr, l2r, outr, r0, row0, valid, top1, top2, toks, lag=LAG, **kw):
        n = attn.shape[0]
        u = min(LNU, n)
        for j in range(n // u):
            tok = toks[-lag] if len(toks) >= lag else None
            top1, top2, tok = ln2_unit(attn[j * u:(j + 1) * u, :], xr, l2r, outr, r0 + j * u, row0, valid,
                                       top1, top2, tok, **kw)
            toks.append(tok)
        return top1, top2

    def p2(i, carry):
        top1, top2 = carry
        b0 = pl.multiple_of(i * TB2, 16)
        xsr = xs_v.at[:, pl.ds(pl.multiple_of(i * (TB2 // NA // 2), 8), TB2 // NA // 2), :]
        xr = x_v.at[pl.ds(b0, TB2 + DEF), :]
        l2r = ln2_v.at[pl.ds(b0, TB2 + DEF), :]
        outr = out_v.at[pl.ds(b0, TB2 + DEF), :]
        row0 = b0 - DEF
        toks = []
        top1, top2 = ln2_part(attn_v[...], xr, l2r, outr, 0, row0, i > 0, top1, top2, toks)

        @pl.when(i > 0)
        def _():
            out_copy(pl.multiple_of((i - 1) * TB2, 16), TB2, 0).start()

        q_part(xsr, 0, 0, QA)
        q_part(xsr, 0, QA, TB2 - QA, tok=pltpu.bitcast(toks[-1], U32) if QGATE else None)
        r0 = 0
        for n in OCH[:-1]:
            top1, top2 = ln2_part(o_part(r0, n), xr, l2r, outr, DEF + r0, row0, None, top1, top2, toks)
            r0 += n
        attn_v[...] = o_part(r0, DEF)
        return top1, top2

    init = jnp.full((8, 1), INT_MIN, I32)
    top1, top2 = lax.fori_loop(0, NB2, p2, (init, init))

    wg_copy.wait()
    wu_copy.wait()
    wd_copy.wait()
    sub8 = lax.broadcasted_iota(I32, (8, LANES), 0)

    def submax(v):
        for sh in (4, 2, 1):
            v = jnp.maximum(v, pltpu.roll(v, sh, 0))
        return v

    def subsum(v):
        for sh in (4, 2, 1):
            v = v + pltpu.roll(v, sh, 0)
        return v

    def best2(t1, t2):
        t1 = jnp.broadcast_to(t1, (8, LANES))
        t2 = jnp.broadcast_to(t2, (8, LANES))
        k1v = submax(t1)
        return k1v, submax(jnp.where(t1 == k1v, t2, t1))

    def key_row(k):
        return 0xFFFF - (k & 0xFFFF)

    def wide(m):
        return jnp.concatenate([m] * NC, axis=1)

    def m_tile(c, k0, nk):
        return _load_packed(mp_v, k0, k0 + nk, c, c + 1)

    toks = []
    top1, top2 = ln2_part(attn_v[...], x_v, ln2_v, out_v, L0, -DEF, None, top1, top2, toks, lag=LAG_L)
    out_copy(L0 - TB2, TB2, 0).start()
    oldk = best2(top1, top2)
    oldx = []
    for kk in oldk:
        g8 = pl.multiple_of(((jnp.clip(key_row(kk[0, 0]), 0, S - 1) >> 3) << 3) + DEF, 8)
        rows = ln2_v[pl.ds(g8, 8), :].astype(F32)
        oldx.append(subsum(jnp.where(wide((key_row(kk) & 7) == sub8), rows, 0.0)))

    wrc = wr_row - jnp.sum(wr_row, axis=-1, keepdims=True) * (1.0 / D)
    uparts = []
    for k0 in range(0, D, LANES):
        mrows = _load_packed(mp_v, k0, k0 + LANES).astype(F32)
        if uparts:
            tok = pltpu.bitcast(pltpu.bitcast(jnp.broadcast_to(uparts[-1], (8, LANES)), U32) & zero_u, F32)
            mrows = jnp.concatenate([mrows[:, 0:LANES] + jnp.concatenate([tok] * (LANES // 8), axis=0),
                                     mrows[:, LANES:]], axis=1)
        uparts.append(jnp.sum(colsum(mrows * wrc).T, axis=0, keepdims=True))
    urow = jnp.concatenate(uparts, axis=1)
    p1, p2_, r0 = init, init, 0
    for n in QS:
        p1, p2_ = q_part(xs_v, L0, r0, n, (urow, wrc, p1, p2_))
        r0 += n

    cp = jnp.zeros((8, D), U32)
    cx = [jnp.zeros((8, D), F32), jnp.zeros((8, D), F32)]
    for s in range(8):
        a1 = jnp.clip(key_row(p1[s, 0]) - L0, 0, RL - 1)
        a2 = jnp.clip(key_row(p2_[s, 0]) - L0, 0, RL - 1)
        b1, b2 = (a1 >> 3) & 1, (a2 >> 3) & 1
        w1 = pqn_v[pl.ds(pl.multiple_of((a1 >> 4) << 3, 8), 8), :]
        w2 = pqn_v[pl.ds(pl.multiple_of((a2 >> 4) << 3, 8), 8), :]
        w2 = jnp.where(b1 == b2, pltpu.roll(w2, 4, 0), w2)
        hm = jnp.uint32(0xFFFF0000 if s % 2 else 0x0000FFFF)
        m1 = wide(jnp.where(sub8 == s // 2 + 4 * b1, hm, jnp.uint32(0)))
        m2 = wide(jnp.where(sub8 == s // 2 + 4 * (1 - b1), hm, jnp.uint32(0)))
        cp = cp | (w1 & m1) | (w2 & m2)
        for hf, ar in enumerate((jnp.where(b1 == 1, a2, a1), jnp.where(b1 == 1, a1, a2))):
            g8 = pl.multiple_of(((ar >> 3) << 3) + (L0 + DEF), 8)
            cx[hf] = jnp.where(wide(sub8 == s), x_v[pl.ds(g8, 8), :].astype(F32), cx[hf])
    cand_p = pltpu.bitcast(cp, BF16)
    cand_x = jnp.concatenate(cx, axis=0)
    id1 = key_row(jnp.broadcast_to(p1, (8, LANES)))
    id2 = key_row(jnp.broadcast_to(p2_, (8, LANES)))
    up = (((id1 - L0) >> 3) & 1) == 1
    old_slot = (jnp.logical_and(sub8 >= 6, up), jnp.logical_and(sub8 >= 6, jnp.logical_not(up)))
    old_id = jnp.where(sub8 == 6, key_row(oldk[0]), key_row(oldk[1]))
    ids_lo = jnp.where(old_slot[0], old_id, jnp.where(up, id2, id1))
    ids_hi = jnp.where(old_slot[1], old_id, jnp.where(up, id1, id2))

    st = dict(top1=top1, top2=top2, pend=[], step=0, sent=0)

    def gated(v):
        tok = None
        while st["pend"] and st["pend"][0][0] <= st["step"]:
            t = st["pend"].pop(0)[1]
            tok = t if tok is None else tok | t
        if tok is None:
            return v
        u = pltpu.bitcast(v, U32)
        return pltpu.bitcast(jnp.concatenate([u[:, 0:LANES] | tok, u[:, LANES:]], axis=1), BF16)

    def o_units():
        for ci, n in enumerate(OCL):
            r0 = sum(OCL[:ci])
            lhs = pltpu.bitcast(pqn_v[r0 // 2:(r0 + n) // 2, :], BF16)
            halves = []
            for c0 in range(0, NC, ONT):
                acc = x_v[DEF + L0 + r0:DEF + L0 + r0 + n, c0 * LANES:(c0 + ONT) * LANES].astype(F32)
                ks = (4 // ONT) * LANES
                for k0 in range(0, D, ks):
                    w = jnp.concatenate([m_tile(c, k0, ks) for c in range(c0, c0 + ONT)], axis=1)
                    acc = acc + jnp.dot(lhs[:, k0:k0 + ks], w, preferred_element_type=F32)
                    if k0 + ks == D:
                        halves.append(acc)
                        if len(halves) == NC // ONT:
                            last = r0 + n == RL
                            tk = [] if last else toks
                            st["top1"], st["top2"] = ln2_part(
                                jnp.concatenate(halves, axis=1), x_v, ln2_v, out_v, DEF + L0 + r0, -DEF, None,
                                st["top1"], st["top2"], tk, lag=n if last else LAG_L, is_h=True, fast=last)
                            if GLAG[ci] is not None:
                                st["pend"].append((st["step"] + GLAG[ci],
                                                   pltpu.bitcast(jnp.broadcast_to(st["top1"], (8, LANES)), U32) & zero_u))
                            if last:
                                out_copy(L0 + st["sent"], r0 + n - st["sent"], 2).start()
                            elif r0 + n in OUT_AT:
                                out_copy(L0 + st["sent"], r0 + n - st["sent"], 1).start()
                                st["sent"] = r0 + n
                    yield

    res = {}

    def c_units():
        parts = []
        for c in range(NC):
            parts.append(jnp.dot(cand_p, m_tile(c, 0, D), preferred_element_type=F32))
            yield
        xs = _layernorm(cand_x + jnp.concatenate(parts, axis=1))
        old = jnp.where(wide(sub8 == 6), oldx[0], oldx[1])
        res["xs"] = jnp.concatenate([jnp.where(wide(old_slot[hf]), old, xs[hf * 8:(hf + 1) * 8, :])
                                     for hf in range(2)], axis=0).astype(BF16)

    def f_units():
        xs = res["xs"]
        acts = []
        for j in range(F // LANES):
            cs = slice(j * LANES, (j + 1) * LANES)
            g = jnp.dot(gated(xs), wload(wg_v, 0, D, cs), preferred_element_type=F32)
            yield
            u = jnp.dot(xs, wload(wu_v, 0, D, cs), preferred_element_type=F32)
            acts.append((g * jax.nn.sigmoid(g) * u).astype(BF16))
            yield
        act = jnp.concatenate(acts, axis=1)
        zf = pltpu.bitcast(zero_u, F32)
        ys = []
        KF = (F // D) * D
        for c in range(0, NC, 2):
            acc = jnp.concatenate([jnp.concatenate([zf, zf], axis=0)] * 2, axis=1)
            acc = acc + jnp.dot(gated(act[:, KF:]), wload(wd_v, KF, F - KF, slice(c * LANES, (c + 2) * LANES)),
                                preferred_element_type=F32)
            yield
            for cc in range(2):
                y = acc[:, cc * LANES:(cc + 1) * LANES]
                for k0 in range(0, KF, D):
                    y = y + jnp.dot(gated(act[:, k0:k0 + D]),
                                    wload(wd_v, k0, D, slice((c + cc) * LANES, (c + cc + 1) * LANES)),
                                    preferred_element_type=F32)
                    yield
                ys.append(y)
        res["y"] = jnp.concatenate(ys, axis=1)

    ou = o_units()

    def o_step():
        next(ou, None)
        st["step"] += 1

    for _ in range(NPRE):
        o_step()
    for _ in c_units():
        o_step()
    for _ in range(NGAP):
        o_step()
    for _ in f_units():
        o_step()
    for _ in ou:
        pass

    keyv = best2(st["top1"], st["top2"])
    idx = [jnp.clip(key_row(kk[0, 0]), 0, S - 1) for kk in keyv]
    grp = [pl.multiple_of((ii >> 3) << 3, 8) for ii in idx]
    vgrp = [pl.multiple_of(gg + DEF, 8) for gg in grp]
    y = res["y"]
    hits = None
    yrows = []
    for c in range(2):
        m_lo = ids_lo == key_row(keyv[c])
        m_hi = ids_hi == key_row(keyv[c])
        yrows.append(subsum(jnp.where(wide(m_lo), y[0:8, :], 0.0) + jnp.where(wide(m_hi), y[8:16, :], 0.0)))
        hit = submax(jnp.where(m_lo | m_hi, 1, 0))
        hits = hit if hits is None else hits + hit
    hit_all = hits[0, 0] == 2

    tail0 = L0 + st["sent"]
    tail_copy = out_copy(tail0, S - tail0, 2)
    in_tail = jnp.maximum(grp[0], grp[1]) >= tail0
    two_groups = grp[1] != grp[0]

    def fix_copy(c):
        return out_copy(grp[c], 8, 3 + c)

    def finish(ysel):
        for c in range(2):
            hi = keyv[c] & jnp.int32(-65536)
            score = pltpu.bitcast(hi ^ ((hi >> 31) & 0x7FFF0000), F32)
            sel = (key_row(keyv[c]) & 7) == sub8
            upd = jnp.where(wide(sel), ysel[c] * wide(jax.nn.sigmoid(score)), 0.0)
            out_v[pl.ds(vgrp[c], 8), :] = (out_v[pl.ds(vgrp[c], 8), :].astype(F32) + upd).astype(BF16)
        fix_copy(0).start()

        @pl.when(two_groups)
        def _():
            fix_copy(1).start()

    out_copy(0, L0, 0).wait()
    out_copy(L0, tail0 - L0, 1).wait()

    @pl.when(in_tail)
    def _():
        tail_copy.wait()

    @pl.when(hit_all)
    def _():
        finish(yrows)

    @pl.when(jnp.logical_not(hit_all))
    def _():
        xsel = jnp.concatenate([ln2_v[pl.ds(vgrp[c], 8), :] for c in range(2)], axis=0)

        def ffn_tile(j, acc):
            cs = pl.ds(pl.multiple_of(j * LANES, LANES), LANES)
            g = jnp.dot(xsel, wload(wg_v, 0, D, cs), preferred_element_type=F32)
            u = jnp.dot(xsel, wload(wu_v, 0, D, cs), preferred_element_type=F32)
            a = (g * jax.nn.sigmoid(g) * u).astype(BF16)
            wd_t = pltpu.bitcast(wd_v[pl.ds(pl.multiple_of(j * (LANES // 2), LANES // 2), LANES // 2), 0:D], BF16)
            return acc + jnp.dot(a, wd_t, preferred_element_type=F32)

        yf = lax.fori_loop(0, F // LANES, ffn_tile, jnp.zeros((16, D), F32))
        finish([yf[0:8, :], yf[8:16, :]])

    @pl.when(jnp.logical_not(in_tail))
    def _():
        tail_copy.wait()

    fix_copy(0).wait()

    @pl.when(two_groups)
    def _():
        fix_copy(1).wait()


@jax.jit
def pallas_sequential_preLN__linear_attn_block__moe_arch_mod__prompt_kernel(
    A_x: jax.Array,
    A_wqkv: jax.Array,
    A_wo: jax.Array,
    B_x: jax.Array,
    B_w_r: jax.Array,
    B_w_gate: jax.Array,
    B_w_up: jax.Array,
    B_w_down: jax.Array,
):
    del B_x
    x = A_x.reshape(S, D)
    wr = B_w_r.reshape(NC, LANES)
    any_spec = pl.BlockSpec(memory_space=pl.ANY)
    out = pl.pallas_call(
        _kernel,
        out_shape=jax.ShapeDtypeStruct((S, D), BF16),
        in_specs=[any_spec] * 7,
        out_specs=any_spec,
        scratch_shapes=[
            pltpu.VMEM((S + DEF, D), BF16),
            pltpu.VMEM((D // 2, D), U32),
            pltpu.VMEM((D // 2, D), U32),
            pltpu.VMEM((2, D // 2, D), U32),
            pltpu.VMEM((NC, LANES), BF16),
            pltpu.VMEM((2, D // 2, F + LANES), U32),
            pltpu.VMEM((F // 2, D + LANES), U32),
            pltpu.VMEM((P0 // 2, D), U32),
            pltpu.VMEM((7 ** LA, S // NA // 2, DA), U32),
            pltpu.VMEM((7 ** LA, DA // 2, DA), U32),
            pltpu.VMEM((D // 2, P0), U32),
            pltpu.VMEM((7 ** LA, DA // 2, TB // NA), U32),
            pltpu.VMEM((D, LANES), F32),
            pltpu.VMEM((2, DH // 2 * PSTR, LANES), U32),
            pltpu.VMEM((D, D), F32),
            pltpu.VMEM((7 ** LA, NC // NA, DH // NA // 2 * PSTR, LANES), U32),
            pltpu.VMEM((NC, DH // 2 * PSTR, LANES), U32),
            pltpu.VMEM((7 ** LO, NC // NO, DH // NO // 2 * PSTR, LANES), U32),
            pltpu.VMEM((RL // 2, D), U32),
            pltpu.VMEM((7 ** LO, TB2 // NO // 2, DO), U32),
            pltpu.VMEM((DEF, D), F32),
            pltpu.VMEM((2, S + DEF, D), BF16),
            pltpu.VMEM((2048, D), U32),
            pltpu.VMEM((8, LANES), U32),
            pltpu.SemaphoreType.DMA((NSEM,)),
        ],
        compiler_params=pltpu.CompilerParams(vmem_limit_bytes=110 * 1024 * 1024, disable_bounds_checks=True,
                                             disable_semaphore_checks=True),
    )(x, A_wqkv, A_wo, wr, B_w_gate, B_w_up, B_w_down)
    return out.reshape(1, S, D)
```

```python
import jax
import jax.numpy as jnp
from jax import lax
import jax.experimental.pallas as pl
import jax.experimental.pallas.tpu as pltpu


S = 2048
D = 1024
F = 3584
H = 32
DH = D // H
LANES = 128
NC = D // LANES
HD = D // 2

LA = 2
LG = 1
LK = 2
LO = 1
NA, NG, NK, NO = 2 ** LA, 2 ** LG, 2 ** LK, 2 ** LO
DA, DG, DK, DO = D // NA, D // NG, D // NK, D // NO
XSN = 7 ** LA if LG == LA else 9 * 7 ** LG
P0 = 512
PB = S - P0
TX = 256
TB = 512
NB1 = PB // TB
TB2 = 512
NB2 = 3
QA = 256
OCH = (128, 128, 128, 128)
DEF = OCH[-1]
L0 = NB2 * TB2
RL = S - L0
QS = (256, 256)
OCL = ((128, False), (128, False), (128, False), (64, True), (64, True))
NPRE = 24
NGAP = 10
OUT_AT = (256, 384, 448)
LNU = 8
LAG_L = 4
LN_DELAY = 800
JOB_DELAY = 500
POST_DELAY = 800
GM = 128
PGM = 128
PGN = 128
PKM = 128
PKK = 256
EV0 = 0
EV1 = 0
EVT = 0
TRW = 256
TRM = 128
GN = 128
WK5 = 66
C6LN = (1000, 8900)
C6WK = (1500, 8900)
P1LN = (60, 12000)
P1WP = (6300, 11500)
P1WQ = (7500, 13100)
WQP = 5
EV2 = 300
P2U = (60, 2600)
P2X = (4300, 5900)
LAG = 5
QFIN = False
HFIN = True
EV3 = 0
LN2_DELAY = 900
QP_DELAY = 400
GLAG = (None, None, None, 20, 8)

F32 = jnp.float32
BF16 = jnp.bfloat16
U32 = jnp.uint32
I32 = jnp.int32

XP = ((PB, 128), (PB + 128, 128), (PB + 256, 256), (0, TB), (TB, PB - TB))
WKP = ((0, 128), (128, 128), (256, 256), (512, 512))

SEM_X = 0
SEM_WK = SEM_X + len(XP)
SEM_WQ = SEM_WK + len(WKP)
SEM_W3 = SEM_WQ + 1
SEM_WR = SEM_W3 + 1
SEM_WGU = SEM_WR + 1
SEM_WD = SEM_WGU + 1
SEM_OUT = SEM_WD + 1
NSEM = SEM_OUT + 5

INT_MIN = -(2 ** 31)


def _layernorm(x, tok=None, w=None):
    s0 = x[:, 0:LANES]
    if tok is not None:
        s0 = s0 + jnp.concatenate([tok] * (x.shape[0] // 8), axis=0)
    for c in range(1, NC):
        s0 = s0 + x[:, c * LANES:(c + 1) * LANES]
    mu = jnp.sum(s0, axis=-1, keepdims=True) * (1.0 / D)
    xc = x - mu
    var = jnp.sum(xc * xc, axis=-1, keepdims=True) * (1.0 / D)
    rstd = lax.rsqrt(var + 1e-5)
    if w is None:
        return xc * rstd
    return xc * rstd, jnp.sum(xc * w, axis=-1, keepdims=True) * rstd


def _phi(t):
    return jnp.where(t > 0, t + 1.0, jnp.exp(t)) + 1e-6


def _n_off(a, b):
    return 32 * a + 8 * b


def _n_groups():
    pos = {(2 * o + e) * LANES + _n_off(a, b): (16 * e + 4 * b + a) * DH + 8 * o
           for o in range(4) for e in range(2) for a in range(4) for b in range(4)}
    return [pos[n] for n in sorted(pos)]


def _quads(b):
    h = len(b) // 2
    return [[r[j * h:(j + 1) * h] for r in b[i * h:(i + 1) * h]] for i in range(2) for j in range(2)]


def _badd(x, y):
    return [[a + b for a, b in zip(rx, ry)] for rx, ry in zip(x, y)]


def _bsub(x, y):
    return [[a - b for a, b in zip(rx, ry)] for rx, ry in zip(x, y)]


def _a_set(b):
    if len(b) == 1:
        return [b[0][0]]
    return [x for o in _a_ops(b) for x in _a_set(o)]


def _b_set(b):
    if len(b) == 1:
        return [b[0][0]]
    q11, q12, q21, q22 = _quads(b)
    ops = (_badd(q11, q22), q11, _bsub(q12, q22), _bsub(q21, q11), q22, _badd(q11, q12), _badd(q21, q22))
    return [x for o in ops for x in _b_set(o)]


def _b_in_a(i, levels):
    perm = (0, 2, 6, 5, 3, 4, 1)
    return sum(perm[(i // 7 ** l) % 7] * 7 ** l for l in range(levels))


def _strassen(prod, levels, base=0, fin=lambda k, q: q, init=None):
    if levels == 0:
        return [[prod(base)]]

    def m(i):
        return _strassen(prod, levels - 1, base * 7 + i)

    def seed(q, x):
        return x if init is None else _badd(_quads(init)[q], x)

    m2 = m(2)
    c22 = seed(3, m2)
    m4 = m(4)
    c12 = fin(1, _badd(seed(1, m2), m4))
    c11 = m4 if init is None else _bsub(_quads(init)[0], m4)
    m3 = m(3)
    c11 = _bsub(m3, c11) if init is None else _badd(c11, m3)
    m1 = m(1)
    c21 = fin(2, _badd(seed(2, m3), m1))
    c22 = _bsub(c22, m1)
    m0 = m(0)
    c11 = _badd(c11, m0)
    c22 = _badd(c22, m0)
    c11 = fin(0, _badd(c11, m(6)))
    c22 = fin(3, _badd(c22, m(5)))
    return [a + b for a, b in zip(c11, c12)] + [a + b for a, b in zip(c21, c22)]


def _goff(i, levels):
    return int(format(i, "0%db" % levels)[::-1], 2) if levels else 0


def _blocks(rows, n):
    w = rows[0].shape[1] // n
    return [[r[:, j * w:(j + 1) * w] for j in range(n)] for r in rows]


def _or_all(vals):
    acc = None
    for v in vals:
        v = pltpu.bitcast(v, U32)
        for g in range(v.shape[0] // 8):
            for c in range(v.shape[1] // LANES):
                p = v[g * 8:(g + 1) * 8, c * LANES:(c + 1) * LANES]
                acc = p if acc is None else acc | p
    return acc


def _raw_ops(levels):
    n = 2 ** levels
    names = [[_Tag((i, j)) for j in range(n)] for i in range(n)]
    return {op: t.ij for op, t in enumerate(_b_set(names)) if t.ij is not None}


class _Tag:
    def __init__(self, ij):
        self.ij = ij

    def __add__(self, other):
        return _Tag(None)

    __sub__ = __add__


def _a_ops(b):
    q11, q12, q21, q22 = _quads(b)
    return (_badd(q11, q22), _badd(q21, q22), q11, q22, _badd(q11, q12), _bsub(q21, q11), _bsub(q12, q22))


def _x_set(o):
    return _a_set(o) + ([] if LG == LA else [o[0][1], o[1][0]])


_A_FORM = (((0, 0), (1, 1), 1), ((1, 0), (1, 1), 1), ((0, 0),), ((1, 1),), ((0, 0), (0, 1), 1),
           ((1, 0), (0, 0), -1), ((0, 1), (1, 1), -1))
_B_FORM = (((0, 0), (1, 1), 1), ((0, 0),), ((0, 1), (1, 1), -1), ((1, 0), (0, 0), -1), ((1, 1),),
           ((0, 0), (0, 1), 1), ((1, 0), (1, 1), 1))


def _outer(form, get, n):
    h = n // 2

    def quad(q):
        return [[get(q[0] * h + i, q[1] * h + j) for j in range(h)] for i in range(h)]

    if len(form) == 1:
        return quad(form[0])
    return (_badd if form[2] > 0 else _bsub)(quad(form[0]), quad(form[1]))


def _x_slot(i):
    return i if LG == LA else (i // 7) * 9 + i % 7


def _merge(b):
    return jnp.concatenate([jnp.concatenate(r, axis=1) for r in b], axis=0)


def _gate(v, tok):
    u = pltpu.bitcast(v, U32)
    top = u[0:8, 0:LANES] | tok
    if u.shape[1] > LANES:
        top = jnp.concatenate([top, u[0:8, LANES:]], axis=1)
    return pltpu.bitcast(jnp.concatenate([top, u[8:, :]], axis=0) if u.shape[0] > 8 else top, BF16)


class _Pacer:
    def __init__(self, zero, every=0):
        self.zero, self.t, self.jobs, self.pend, self.tok = zero, 0, [], [], None
        self.every, self.last = every, -every

    def add(self, jobs, t0, t1, delay):
        for k, job in enumerate(jobs):
            self.jobs.append((t0 + k * (t1 - t0) // len(jobs), len(self.jobs), job, delay))
        self.jobs.sort(key=lambda e: e[:2])

    def due(self, dep, delay):
        if dep is not None:
            self.pend.append((self.t + delay, _or_all([dep])))

    def release(self, upto):
        while self.jobs and self.jobs[0][0] <= upto:
            _, _, job, delay = self.jobs.pop(0)
            self.due(job(self.tok), delay)

    def dot(self, lhs, rhs):
        self.release(self.t)
        ready = [d for t, d in self.pend if t <= self.t]
        if ready and self.t - self.last >= self.every:
            self.pend = [e for e in self.pend if e[0] > self.t]
            self.last = self.t
            lhs = _gate(lhs, _or_all(ready) & self.zero)
        res = jnp.dot(lhs, rhs, preferred_element_type=F32)
        self.t += lhs.shape[0] * (lhs.shape[1] // LANES) * (res.shape[1] // LANES) // 4
        self.tok = pltpu.bitcast(pltpu.bitcast(res[0:8, 0:LANES], U32) & self.zero, F32)
        return res

    def flush(self):
        self.release(1 << 30)


def _kernel(x_hbm, wqkv_hbm, wo_hbm, wr_hbm, wg_hbm, wu_hbm, wd_hbm, out_hbm,
            x_v, wk_v, wq_v, w3_v, wr_v, wgu_v, wd_v,
            ln1_v, xs_v, wks_v, pkt_v, pks_v, zacc_v, uacc_v, xw_v, g_v, wqp_v, wqs_v, mp_v, ms_v, pq_v, pqn_v, pqs_v, attn_v, lo_v, lnf_v, zero_v,
            sems):

    ln2_v, out_v = lo_v.at[0], lo_v.at[1]

    wqkv_hbm, wo_hbm, wg_hbm, wu_hbm, wd_hbm = (r.bitcast(U32) for r in (wqkv_hbm, wo_hbm, wg_hbm, wu_hbm, wd_hbm))

    def wload(ref, r0, nr, cols):
        return pltpu.bitcast(ref[r0 // 2:(r0 + nr) // 2, cols], BF16)

    wv_v, wo_v = w3_v.at[0], w3_v.at[1]
    wg_v, wu_v = wgu_v.at[0], wgu_v.at[1]

    def x_copy(i):
        r0, n = XP[i]
        return pltpu.make_async_copy(x_hbm.at[pl.ds(r0, n), :], x_v.at[pl.ds(DEF + r0, n), :], sems.at[SEM_X + i])

    def out_copy(r0, n, s):
        return pltpu.make_async_copy(out_v.at[pl.ds(DEF + r0, n), :], out_hbm.at[pl.ds(r0, n), :],
                                     sems.at[SEM_OUT + s])

    def wk_copy(j):
        c0, n = WKP[j]
        return pltpu.make_async_copy(wqkv_hbm.at[:, pl.ds(D + c0, n)], wk_v.at[:, pl.ds(c0, n)],
                                     sems.at[SEM_WK + j])

    wq_copy = pltpu.make_async_copy(wqkv_hbm.at[:, pl.ds(0, D)], wq_v, sems.at[SEM_WQ])
    wr_copy = pltpu.make_async_copy(wr_hbm, wr_v, sems.at[SEM_WR])
    wd_copy = pltpu.make_async_copy(wd_hbm, wd_v.at[:, pl.ds(0, D)], sems.at[SEM_WD])
    wg_copy = pltpu.make_async_copy(wg_hbm, wg_v.at[:, pl.ds(0, F)], sems.at[SEM_WGU])
    wu_copy = pltpu.make_async_copy(wu_hbm, wu_v.at[:, pl.ds(0, F)], sems.at[SEM_WGU])

    x_copy(0).start()
    wk_copy(0).start()
    x_copy(1).start()
    wr_copy.start()
    for j in range(1, len(WKP)):
        wk_copy(j).start()
    for j in range(2, len(XP)):
        x_copy(j).start()
    wq_copy.start()
    pltpu.make_async_copy(wqkv_hbm.at[:, pl.ds(2 * D, D)], wv_v, sems.at[SEM_W3]).start()
    pltpu.make_async_copy(wo_hbm, wo_v, sems.at[SEM_W3]).start()
    wg_copy.start()
    wu_copy.start()
    wd_copy.start()

    def ln1_rows(xr, xr0, lnr, r0, n):
        ln = _layernorm(xr[xr0:xr0 + n, :].astype(F32)).astype(BF16)
        lnr[r0 // 2:(r0 + n) // 2, :] = pltpu.bitcast(ln, U32)

    def ln1_set(pc, xr, xr0, xsr, a0, n, t0, t1):
        def unit(j):
            def job(tok):
                ln = _layernorm(xr[xr0 + j * LNU:xr0 + (j + 1) * LNU, :].astype(F32), tok)
                lnf_v[j * LNU:(j + 1) * LNU, :] = ln
                return _or_all([ln[:, 0:LANES], ln[:, D - LANES:D]])
            return job

        def piece(j0, c0, o):
            def job(tok):
                def get(i, f):
                    r = (j0 + 2 * _goff(i, LA)) * LNU
                    v = lnf_v[r:r + 16, f * DA + c0:f * DA + c0 + LANES]
                    return v + jnp.concatenate([tok, tok], axis=0) if (i + f) % (NA // 2 + 1) == 0 else v

                r = (a0 + (j0 // (2 * NA)) * 16) // 2
                ops = _x_set(_outer(_A_FORM[o], get, NA))
                for op, v in enumerate(ops):
                    xsr.at[o * len(ops) + op][r:r + 8, c0:c0 + LANES] = pltpu.bitcast(v.astype(BF16), U32)
                return _or_all([v[0:8, :] for v in [ops[0]] + ops[5:7]])
            return job

        grp = 2 * NA
        ng = n // LNU // grp
        dt = (t1 - t0 - LN_DELAY) // (ng + 1)
        for g in range(ng):
            pc.add([unit(g * grp + j) for j in range(grp)], t0 + g * dt, t0 + (g + 1) * dt, LN_DELAY)
            s = t0 + (g + 1) * dt + LN_DELAY
            pc.add([piece(g * grp, c0, o) for c0 in range(0, DA, LANES) for o in range(7)], s, s + dt, JOB_DELAY)

    def ln1_load(lnr, r0, n):
        return pltpu.bitcast(lnr[r0 // 2:(r0 + n) // 2, :], BF16)

    def gate(v, tok):
        return v if tok is None else _gate(v, tok)

    def k_mm(r0, n, c0, nc):
        return jnp.dot(ln1_load(ln1_v, r0, n), wload(wk_v, 0, D, slice(c0, c0 + nc)), preferred_element_type=F32)

    def z_acc(pkts, c0, first=False):
        zs = None
        for pkt in pkts:
            for j in range(pkt.shape[1] // LANES):
                p = pkt[:, j * LANES:(j + 1) * LANES]
                zs = p if zs is None else zs + p
        if first:
            zacc_v[c0:c0 + zs.shape[0], :] = zs
        else:
            zacc_v[c0:c0 + zs.shape[0], :] += zs

    def k_post(k, p0, c0, first=False):
        n, nc = k.shape
        pkt = _phi(k).T
        pkt_v[c0 // 2:(c0 + nc) // 2, p0:p0 + n] = pltpu.bitcast(pkt.astype(BF16), U32)
        z_acc([pkt], c0, first)
        return pkt[nc - 8:nc, n - LANES:n]

    def g_acc(r0, n, c0, nc, first=False, pc=None):
        h, w = (nc, D) if pc is None else (min(nc, PGM), PGN)
        for f0 in range(c0, c0 + nc, h):
            for j0 in range(0, D, w):
                lhs = pltpu.bitcast(pkt_v[f0 // 2:(f0 + h) // 2, r0:r0 + n], BF16)
                rhs = pltpu.bitcast(ln1_v[r0 // 2:(r0 + n) // 2, j0:j0 + w], BF16)
                g = jnp.dot(lhs, rhs, preferred_element_type=F32) if pc is None else pc.dot(lhs, rhs)
                if first:
                    g_v[f0:f0 + h, j0:j0 + w] = g
                else:
                    g_v[f0:f0 + h, j0:j0 + w] += g

    def k_paced(pc, r0, c0, nc, first):
        for j0 in range(c0, c0 + nc, LANES):
            for t0 in range(r0, r0 + TX, PKM):
                k = None
                for k0 in range(0, D, PKK):
                    p = pc.dot(ln1_load(ln1_v, t0, PKM)[:, k0:k0 + PKK], wload(wk_v, k0, PKK, slice(j0, j0 + LANES)))
                    k = p if k is None else k + p
                pc.due(k_post(k, t0, j0, first and t0 == r0), POST_DELAY)

    attn_v[...] = jnp.zeros_like(attn_v)
    zero_v[...] = jnp.zeros_like(zero_v)

    x_copy(0).wait()
    ln1_rows(x_v, DEF + PB, ln1_v, 0, 128)
    wk_copy(0).wait()
    ka = k_mm(0, 128, 0, 128)
    x_copy(1).wait()
    wr_copy.wait()
    ln1_rows(x_v, DEF + PB + 128, ln1_v, 128, 128)
    k_post(ka, 0, 0, first=True)
    g_acc(0, 128, 0, 128, first=True)
    wk_copy(1).wait()
    k_post(k_mm(128, 128, 0, 128), 128, 0)
    k_post(k_mm(0, TX, 128, 128), 0, 128, first=True)
    g_acc(128, 128, 0, 128)
    def w_job(src_ref, dst_ref, levels, r0, c0, o):
        n = 2 ** levels
        w, raw, inner = D // n, _raw_ops(levels), 7 ** (levels - 1)

        def job(tok):
            def cut(i, j):
                return src_ref[(i * w + r0) // 2:(i * w + r0) // 2 + 8, j * w + c0:j * w + c0 + LANES]

            def get(i, j):
                u = cut(i, j)
                return pltpu.bitcast(u if tok is None else u | pltpu.bitcast(tok, U32), BF16).astype(F32)

            ops = []
            for op, v in enumerate(_b_set(_outer(_B_FORM[o], get, n))):
                dst = dst_ref.at[o * inner + op]
                if o * inner + op in raw:
                    dst[r0 // 2:r0 // 2 + 8, c0:c0 + LANES] = cut(*raw[o * inner + op])
                else:
                    dst[r0 // 2:r0 // 2 + 8, c0:c0 + LANES] = pltpu.bitcast(v.astype(BF16), U32)
                    ops.append(v)
            return _or_all(ops[0:1] + ops[-2:]) if ops else None
        return job

    def wk_jobs_of(outer):
        return [w_job(wk_v, wks_v, LK, r0, c0, o) for r0 in range(0, DK, 16) for c0 in range(0, DK, LANES)
                for o in outer]

    wk_copy(2).wait()
    pc = _Pacer(zero_v[...], EV0)
    pc.add(wk_jobs_of((1, 3)), 500, 2200, JOB_DELAY)
    k_paced(pc, 0, 256, 256, True)
    g_acc(0, TX, 128, 128, True, pc)
    g_acc(0, TX, 256, 256, True, pc)
    pc.flush()
    wk_copy(3).wait()
    wk_jobs = wk_jobs_of((0, 2, 4, 5, 6))
    pc = _Pacer(zero_v[...], EV0)
    pc.add(wk_jobs[:WK5], 500, 2700, JOB_DELAY)
    k_paced(pc, 0, 512, 512, True)
    g_acc(0, TX, 512, 256, True, pc)
    pc.flush()
    x_copy(2).wait()
    x_copy(3).wait()
    pc = _Pacer(zero_v[...], EV0)
    ln1_set(pc, x_v, DEF, xs_v, 0, TB, *C6LN)
    pc.add(wk_jobs[WK5:], *C6WK, JOB_DELAY)
    ln1_rows(x_v, DEF + PB + TX, ln1_v, TX, TX)
    g_acc(0, TX, 768, 256, True, pc)
    k_paced(pc, TX, 0, D, False)
    for c0 in range(0, D, 256):
        g_acc(TX, TX, c0, 256, False, pc)
    pc.flush()

    MA = TB // NA
    NS = NK // NG

    def xs_load(xsr, op, a0, m, cols=slice(None)):
        return pltpu.bitcast(xsr[op, a0 // 2:(a0 + m) // 2, cols], BF16)

    def k_step(pc, xsr, j0):
        def fin(_, q):
            if NS > 1:
                q = [[jnp.concatenate([_phi(jnp.concatenate([r[f] for r in q], axis=0)).T for f in range(NS)],
                                      axis=0)]]
            else:
                q = [[_phi(v).T for v in r] for r in q]
            pc.due(_or_all([v[t - 8:t, :] for r in q for v in r for t in range(LANES, v.shape[0] + 1, LANES)]),
                   POST_DELAY)
            return q

        def lhs(i):
            if LK == LA:
                return xs_load(xsr, _x_slot(i), 0, MA)
            return _merge([[xs_load(xsr, i * 9 + s, 0, MA) for s in r] for r in ((2, 7), (8, 3))])

        cb = _strassen(lambda i: pc.dot(lhs(i), pltpu.bitcast(wks_v[i, :, j0:j0 + LANES], BF16)), LK, fin=fin)
        ops = _a_ops([[cb[i][f] for i in range(NG)] for f in range(NG)])
        for half, o in ((0, ops[4]), (1, ops[1])):
            for f, rowb in enumerate(o):
                for s in range(NS):
                    z_acc([v[s * LANES:(s + 1) * LANES, :] for v in rowb], half * HD + f * DG + s * DK + j0)
        for _ in range(LG - 1):
            ops = [o for x in ops for o in _a_ops(x)]
        for op, o in enumerate(ops):
            r = j0 * NS
            pks_v.at[op][r // 2:(r + NS * LANES) // 2, :] = pltpu.bitcast(o[0][0].astype(BF16), U32)
        pc.due(_or_all([o[0][0][NS * LANES - 8:NS * LANES, :] for o in (ops[0], ops[-1], ops[-2])]), 2 * POST_DELAY)

    def g_rhs(xsr, i, c0, nc):
        o = _b_in_a(i, LG)
        if LG == LA:
            return xs_load(xsr, o, 0, MA, slice(c0, c0 + nc))
        j, cs = c0 // DA, slice(c0 % DA, c0 % DA + nc)
        return jnp.concatenate([xs_load(xsr, o * 9 + s, 0, MA, cs) for s in ((2, 8), (7, 3))[j]], axis=0)

    def g_step(pc, xsr, r0, nr, c0, nc):
        cb = _strassen(lambda i: pc.dot(pltpu.bitcast(pks_v[i, r0 // 2:(r0 + nr) // 2, :], BF16),
                                        g_rhs(xsr, i, c0, nc)), LG)
        for f in range(NG):
            for c in range(NG):
                h = min(nr, LANES)
                for t in range(nr // h):
                    step, sub = divmod((r0 + t * h) // LANES, NS)
                    g0_ = f * DG + sub * DK + step * LANES + (r0 + t * h) % LANES
                    g_v[g0_:g0_ + h, c * DG + c0:c * DG + c0 + nc] += cb[f][c][t * h:(t + 1) * h, :]

    def wq_jobs(u0, nr):
        span = (NA - 1) * DA + 16 * nr
        u0 = u0 if isinstance(u0, int) else pl.multiple_of(u0, 8)
        srcr, permr = wq_v.at[pl.ds(u0, span // 2), :], wqp_v.at[pl.ds(u0, span // 2), :]
        dstr = wqs_v.at[:, pl.ds(u0, 8 * nr), :]
        oct_ = (lax.broadcasted_iota(I32, (8, LANES), 1) % DH) // 8

        def perm(r, e):
            def job(tok):
                blk = [srcr[r // 2:r // 2 + 8, (4 * e + b) * LANES:(4 * e + b + 1) * LANES] | pltpu.bitcast(tok, U32)
                       for b in range(4)]
                outs = []
                for o in range(4):
                    v = blk[o]
                    for b in range(4):
                        if b != o:
                            v = jnp.where(oct_ == b, pltpu.roll(blk[b], (8 * (b - o)) % LANES, 1), v)
                    permr[r // 2:r // 2 + 8, (2 * o + e) * LANES:(2 * o + e + 1) * LANES] = v
                    outs.append(v)
                return _or_all(outs)
            return job

        return ([perm(i * DA + r0, e) for r0 in range(0, 16 * nr, 16) for i in range(NA) for e in range(2)],
                [w_job(permr, dstr, LA, r0, c0, o) for r0 in range(0, 16 * nr, 16)
                 for c0 in range(0, DA, LANES) for o in range(7)])

    def p1(i, carry):
        xsr = xs_v.at[:, pl.ds(pl.multiple_of(i * (MA // 2), MA // 2), MA), :]
        xr = x_v.at[pl.ds(pl.multiple_of((i + 1) * TB, TB), TB + DEF), :]

        pc = _Pacer(zero_v[...], EV1)
        ln1_set(pc, xr, DEF, xsr, MA, TB, *P1LN)
        perms, sets = wq_jobs(i * (8 * WQP), WQP)
        pc.add(perms, *P1WP, JOB_DELAY)
        pc.add(sets, *P1WQ, JOB_DELAY)
        for j0 in range(0, DK, LANES):
            k_step(pc, xsr, j0)
        for f0 in range(0, DG, GM):
            for c0 in range(0, DG, GN):
                g_step(pc, xsr, f0, GM, c0, GN)
        pc.flush()
        return carry

    x_copy(4).wait()
    wq_copy.wait()
    lax.fori_loop(0, NB1, p1, 0)

    pltpu.make_async_copy(w3_v, w3_v, sems.at[SEM_W3]).wait()
    zero_u = zero_v[...]
    def row_vector(acc_ref):
        return jnp.sum(jnp.concatenate([acc_ref[r:r + 8, :] for r in _n_groups()], axis=0).T, axis=0, keepdims=True)

    zrow = row_vector(zacc_v)
    wr8 = wr_v[...].astype(F32)
    wr_row = jnp.concatenate([wr8[c:c + 1, :] for c in range(NC)], axis=1)

    row_h = lax.broadcasted_iota(I32, (LANES, LANES), 0) // DH
    col_h = lax.broadcasted_iota(I32, (LANES, LANES), 1) // DH
    diag = row_h == col_h

    def colsum(t):
        acc = t[:, 0:LANES]
        for c in range(1, NC):
            acc = acc + t[:, c * LANES:(c + 1) * LANES]
        return acc

    wrc = wr_row - jnp.sum(wr_row, axis=-1, keepdims=True) * (1.0 / D)
    m_raw = _raw_ops(LO)

    def kv_part(c):
        cs = slice(c * LANES, (c + 1) * LANES)
        kv = None
        for k0 in range(0, D, TRW):
            p = pc.dot(g_v[cs, k0:k0 + TRW].astype(BF16), wload(wv_v, k0, TRW, cs))
            kv = p if kv is None else kv + p
        return jnp.where(diag, kv, 0.0)

    def m_part(c, kvs):
        e, b = c // 4, c % 4
        for j0 in range(0, DO, TRM):
            ms = [jnp.concatenate(
                [pc.dot(kv, wload(wo_v, (c + k) * LANES, LANES, slice(f * DO + j0, f * DO + j0 + TRM)))
                 for f in range(NO)], axis=1) for k, kv in enumerate(kvs)]
            deps = []
            for a in range(4):
                rows = [jnp.concatenate([m[a * DH + 8 * o:a * DH + 8 * o + 8, :] for m in ms], axis=0)
                        for o in range(4)]
                for o in range(4):
                    r = ((2 * o + e) * LANES + _n_off(a, b)) // 2
                    for f in range(NO):
                        mp_v[r:r + 8, f * DO + j0:f * DO + j0 + TRM] = pltpu.bitcast(
                            rows[o][:, f * TRM:(f + 1) * TRM].astype(BF16), U32)
                for t in range(4 // NO):
                    r = ((2 * t + e) * LANES + _n_off(a, b)) // 2
                    for op, v in enumerate(_b_set(_blocks(rows[t::4 // NO], NO))):
                        if op not in m_raw:
                            ms_v.at[op][r:r + 8, j0:j0 + TRM] = pltpu.bitcast(v.astype(BF16), U32)
                            deps.append(v[0:8, 0:LANES])
            pc.due(_or_all(deps[::4]), POST_DELAY)

    pc = _Pacer(zero_u, EVT)
    pc.due(jnp.broadcast_to(zrow, (8, D)), 1000)
    perms, sets = wq_jobs(NB1 * 8 * WQP, DA // 16 - NB1 * WQP)
    pc.add(perms, 60, 700, JOB_DELAY)
    pc.add(sets, 1300, 3400, JOB_DELAY)
    kv_prev = None
    for c in range(0, NC + 2, 2):
        kvs = [kv_part(c).astype(BF16), kv_part(c + 1).astype(BF16)] if c < NC else None
        if c:
            m_part(c - 2, kv_prev)
        kv_prev = kvs
    pc.flush()

    def make_key(score, row):
        b = pltpu.bitcast(score, I32)
        srt = b ^ ((b >> 31) & 0x7FFFFFFF)
        return (srt & jnp.int32(-65536)) | (0xFFFF - row)

    def push_keys(key, top1, top2):
        for gidx in range(key.shape[0] // 8):
            kx = key[gidx * 8:(gidx + 1) * 8, :]
            top2 = jnp.maximum(top2, jnp.minimum(top1, kx))
            top1 = jnp.maximum(top1, kx)
        return top1, top2

    lane = lax.broadcasted_iota(I32, (1, LANES), 1)

    def interleave(parts):
        return jnp.concatenate([p[g * 16:(g + 1) * 16, :] for g in range(parts[0].shape[0] // 16) for p in parts],
                               axis=0)

    def q_part(pc, xsr, l0, r0, n, hint=None):
        m = n // NA
        sums = {}

        def park(v, g, c):
            for t in range(m // 16):
                r = r0 + (t * NA + g) * 16
                pq_v[r:r + 16, c * LANES:(c + 1) * LANES] = v[t * 16:(t + 1) * 16, :]

        def fin(k, q):
            q = [[_phi(v) for v in r] for r in q]
            deps = []
            for a, r in enumerate(q):
                for b, v in enumerate(r):
                    i, c = (k // 2) * (NA // 2) + a, (((k % 2) * (NA // 2) + b) * DA + j0) // LANES
                    park(v, _goff(i, LA), c)
                    for name, row in (("z", zrow),) + ((("u", hint["u"]),) if hint else ()):
                        t = v * row[:, c * LANES:(c + 1) * LANES]
                        key = (name, _goff(i, LA), c % 2)
                        sums[key] = t if key not in sums else sums[key] + t
                deps.append(sums[key])
            if (r0 + n < RL or HFIN) if hint else QFIN:
                pc.due(_or_all(deps), POST_DELAY)
            return q

        for j0 in range(0, DA, LANES):
            _strassen(lambda i: pc.dot(xs_load(xsr, _x_slot(i), (l0 + r0) // NA, m),
                                       pltpu.bitcast(wqs_v[i, :, j0:j0 + LANES], BF16)), LA, fin=fin)
        if hint:
            pc.flush()
        den = jnp.concatenate([sums["z", g, e] for g in range(NA) for e in range(2)], axis=0)
        for s in (1, 2, 4):
            den = den + jnp.where((lane & s) == 0, pltpu.roll(den, LANES - s, 1), pltpu.roll(den, s, 1))
        inv_all = 1.0 / (den + 1e-6)

        def inv_of(g):
            return [inv_all[(g * 2 + e) * m:(g * 2 + e + 1) * m, :] for e in range(2)]

        for g in range(NA):
            for e in range(2):
                park(inv_of(g)[e], g, NC + e)
        if hint:
            for g in range(NA):
                starts = [r0 + (t * NA + g) * 16 for t in range(m // 16)]
                num = jnp.sum(jnp.concatenate([xw_v[t:t + 16, :] for t in starts], axis=0)
                              + sums["u", g, 0] * inv_of(g)[0] + sums["u", g, 1] * inv_of(g)[1],
                              axis=-1, keepdims=True)
                row = jnp.concatenate([(l0 + t) + lax.broadcasted_iota(I32, (16, 1), 0) for t in starts], axis=0)
                hint["p1"], hint["p2"] = push_keys(make_key(num, row), hint["p1"], hint["p2"])
            pc.due(jnp.broadcast_to(hint["p1"], (8, LANES)), 1200)


    def scaled(rows, tok=None):
        inv = pq_v[rows, D:D + 2 * LANES]
        if tok is not None:
            inv = inv + jnp.concatenate([jnp.concatenate([tok, tok], axis=0)] * 2, axis=1)
        return pq_v[rows, 0:D] * jnp.concatenate([inv] * (NC // 2), axis=1)

    def post_jobs(r0, n, plain=False):
        def post(t0):
            def job(tok):
                rows = [scaled(slice(t0 + g * 16, t0 + (g + 1) * 16), tok) for g in range(NO)]
                if plain:
                    pqn_v[t0 // 2:t0 // 2 + 8 * NO, :] = pltpu.bitcast(
                        jnp.concatenate(rows, axis=0).astype(BF16), U32)
                    return rows[0][0:8, 0:LANES]
                ops = _a_set(_blocks([rows[_goff(i, LO)] for i in range(NO)], NO))
                r = t0 // NO // 2
                for op, v in enumerate(ops):
                    pqs_v.at[op][r:r + 8, :] = pltpu.bitcast(v.astype(BF16), U32)
                return _or_all([v[0:8, 0:LANES] for v in (ops[0], ops[-1], ops[-2])])
            return job

        return [post(t0) for t0 in range(r0, r0 + n, 16 * NO)]

    def m_operand(i, c0, c1):
        if i not in m_raw:
            return pltpu.bitcast(ms_v[i, :, c0 * LANES:c1 * LANES], BF16)
        bi, bj = m_raw[i]
        return wload(mp_v, bi * DO, DO, slice(bj * DO + c0 * LANES, bj * DO + c1 * LANES))

    def o_part(dot, xr, x0, r0, n):
        a0, m = r0 // NO, n // NO
        nw = LANES * NO // 2
        cols = [[[] for _ in range(NO)] for _ in range(NO)]
        for c0 in range(0, DO, nw):
            init = [[jnp.concatenate(
                [xr[x0 + r0 + (g * NO + _goff(i, LO)) * 16:x0 + r0 + (g * NO + _goff(i, LO) + 1) * 16,
                    f * DO + c0:f * DO + c0 + nw] for g in range(m // 16)], axis=0).astype(F32)
                for f in range(NO)] for i in range(NO)]
            cb = _strassen(lambda i: dot(pltpu.bitcast(pqs_v[i, a0 // 2:(a0 + m) // 2, :], BF16),
                                         m_operand(i, c0 // LANES, (c0 + nw) // LANES)), LO, init=init)
            for i in range(NO):
                for f in range(NO):
                    cols[i][f].append(cb[i][f])
        parts = [None] * NO
        for i in range(NO):
            parts[_goff(i, LO)] = jnp.concatenate([c for f in range(NO) for c in cols[i][f]], axis=1)
        return interleave(parts)

    def ln2_unit(h, l2r, outr, r0, row0, valid, top1, top2, tok, fast=False):
        n = h.shape[0]
        if fast:
            ln2, r = _layernorm(h, tok, wr_row)
        else:
            ln2 = _layernorm(h, tok)
            r = jnp.sum(ln2 * wr_row, axis=-1, keepdims=True)
        l2r[r0:r0 + n, :] = ln2.astype(BF16)
        res = h + ln2
        outr[r0:r0 + n, :] = res.astype(BF16)
        r = r.astype(BF16).astype(F32) + 0.0
        key = make_key(r, (row0 + r0) + lax.broadcasted_iota(I32, (n, 1), 0))
        if valid is not None:
            key = jnp.where(valid, key, INT_MIN)
        top1, top2 = push_keys(key, top1, top2)
        ntok = pltpu.bitcast(pltpu.bitcast(jnp.broadcast_to(r[n - 8:n, :], (8, LANES)), U32) & zero_u, F32)
        return top1, top2, ntok

    def ln2_jobs(h, l2r, outr, r0, row0, valid, st, fast=False):
        def unit(j):
            def job(tok):
                st["top1"], st["top2"], dep = ln2_unit(h[j * LNU:(j + 1) * LNU, :], l2r, outr, r0 + j * LNU, row0,
                                                       valid, st["top1"], st["top2"], tok, fast)
                return dep
            return job
        return [unit(j) for j in range(h.shape[0] // LNU)]

    QC = 16 * 7 ** LA / 8 ** LA
    OC = 16 * 7 ** LO / 8 ** LO

    def p2(i, carry):
        st = dict(top1=carry[0], top2=carry[1])
        b0 = pl.multiple_of(i * TB2, 16)
        xsr = xs_v.at[:, pl.ds(pl.multiple_of(i * (TB2 // NA // 2), 8), TB2 // NA // 2), :]
        xr = x_v.at[pl.ds(b0, TB2 + DEF), :]
        l2r = ln2_v.at[pl.ds(b0, TB2 + DEF), :]
        outr = out_v.at[pl.ds(b0, TB2 + DEF), :]
        row0 = b0 - DEF
        pc = _Pacer(zero_u)
        toks = []

        def chain(jobs):
            for job in jobs:
                toks.append(job(toks[-LAG] if len(toks) >= LAG else None))

        chain(ln2_jobs(attn_v, l2r, outr, 0, row0, i > 0, st))

        @pl.when(i > 0)
        def _():
            out_copy(pl.multiple_of((i - 1) * TB2, 16), TB2, 0).start()

        pc.due(toks[-1], QA * QC)

        def u_job(r):
            def job(tok):
                t = colsum(gate(wload(mp_v, r, 32, slice(None)), pltpu.bitcast(tok, U32)).astype(F32) * wrc)
                uacc_v[r:r + 32, :] = t
                return t
            return job

        def xw_job(t):
            def job(tok):
                v = colsum(x_v[DEF + L0 + t:DEF + L0 + t + 16, :].astype(F32) * wrc)
                v = v + jnp.concatenate([tok, tok], axis=0)
                xw_v[t:t + 16, :] = v
                return v
            return job

        pc.add([u_job(r) for r in range(0, D, 32)], *P2U, JOB_DELAY)
        pc.add([xw_job(t) for t in range(0, RL, 16)], *P2X, JOB_DELAY)
        for r0, n in ((0, QA), (QA, TB2 - QA)):
            q_part(pc, xsr, 0, r0, n)
            for job in post_jobs(r0, n):
                job(None)
        r0 = 0
        for n in OCH[:-1]:
            chain(ln2_jobs(o_part(pc.dot, xr, DEF, r0, n), l2r, outr, DEF + r0, row0, None, st))
            r0 += n
        attn_v[...] = o_part(pc.dot, xr, DEF, r0, DEF)
        return st["top1"], st["top2"]

    init = jnp.full((8, 1), INT_MIN, I32)
    top1, top2 = lax.fori_loop(0, NB2, p2, (init, init))

    wg_copy.wait()
    wu_copy.wait()
    wd_copy.wait()
    sub8 = lax.broadcasted_iota(I32, (8, LANES), 0)
    urow = jnp.sum(uacc_v[...].T, axis=0, keepdims=True)

    def submax(v):
        for sh in (4, 2, 1):
            v = jnp.maximum(v, pltpu.roll(v, sh, 0))
        return v

    def subsum(v):
        for sh in (4, 2, 1):
            v = v + pltpu.roll(v, sh, 0)
        return v

    def best2(t1, t2):
        t1 = jnp.broadcast_to(t1, (8, LANES))
        t2 = jnp.broadcast_to(t2, (8, LANES))
        k1v = submax(t1)
        return k1v, submax(jnp.where(t1 == k1v, t2, t1))

    def key_row(k):
        return 0xFFFF - (k & 0xFFFF)

    def wide(m):
        return jnp.concatenate([m] * NC, axis=1)

    st = dict(top1=top1, top2=top2, pend=[], step=0, sent=0)
    pc = _Pacer(zero_u, EV2)
    hint = dict(u=urow, p1=init, p2=init)

    pc.add(ln2_jobs(attn_v, ln2_v, out_v, L0, -DEF, None, st), 60, QS[0] * QC - 600, LN2_DELAY)
    r0 = 0
    for k, n in enumerate(QS):
        q_part(pc, xs_v, L0, r0, n, hint)
        if k == 0:
            out_copy(L0 - TB2, TB2, 0).start()
            top1, top2 = st["top1"], st["top2"]
            pc.add(post_jobs(0, OCL[0][0], OCL[0][1]), pc.t + 600, pc.t + (RL - n) * QC - 300, QP_DELAY)
        r0 += n
    pc.every = EV3
    oldk = best2(top1, top2)
    oldx = []
    for kk in oldk:
        g8 = pl.multiple_of(((jnp.clip(key_row(kk[0, 0]), 0, S - 1) >> 3) << 3) + DEF, 8)
        rows = ln2_v[pl.ds(g8, 8), :].astype(F32)
        oldx.append(subsum(jnp.where(wide((key_row(kk) & 7) == sub8), rows, 0.0)))

    def gated(v):
        tok = None
        while st["pend"] and st["pend"][0][0] <= st["step"]:
            t = st["pend"].pop(0)[1]
            tok = t if tok is None else tok | t
        if tok is None:
            return v
        u = pltpu.bitcast(v, U32)
        return pltpu.bitcast(jnp.concatenate([u[:, 0:LANES] | tok, u[:, LANES:]], axis=1), BF16)

    res = {}

    def c_units():
        pc.flush()
        p1, p2_ = hint["p1"], hint["p2"]
        cand_p, cand_x = [], []
        for pk_ in (p1, p2_):
            cp, cx = None, None
            for s in range(8):
                g8 = pl.multiple_of((jnp.clip(key_row(pk_[s, 0]) - L0, 0, RL - 1) >> 3) << 3, 8)
                vp = pq_v[pl.ds(g8, 8), :]
                vx = x_v[pl.ds(pl.multiple_of(g8 + (L0 + DEF), 8), 8), :].astype(F32)
                cp = vp if cp is None else jnp.where(jnp.concatenate([sub8 == s] * (NC + 2), axis=1), vp, cp)
                cx = vx if cx is None else jnp.where(wide(sub8 == s), vx, cx)
            cand_p.append(cp[:, 0:D] * jnp.concatenate([cp[:, D:]] * (NC // 2), axis=1))
            cand_x.append(cx)
        cand_p = jnp.concatenate(cand_p, axis=0).astype(BF16)
        cand_x = jnp.concatenate(cand_x, axis=0)
        ids_lo = key_row(jnp.broadcast_to(p1, (8, LANES)))
        ids_hi = jnp.where(sub8 < 6, key_row(jnp.broadcast_to(p2_, (8, LANES))),
                           jnp.where(sub8 == 6, key_row(oldk[0]), key_row(oldk[1])))
        res["ids"] = (ids_lo, ids_hi)
        parts = []
        for c in range(NC):
            parts.append(jnp.dot(cand_p, wload(mp_v, 0, D, slice(c * LANES, (c + 1) * LANES)), preferred_element_type=F32))
            yield
        xs = _layernorm(cand_x + jnp.concatenate(parts, axis=1))
        hi = jnp.where(wide(sub8 < 6), xs[8:16, :], jnp.where(wide(sub8 == 6), oldx[0], oldx[1]))
        res["xs"] = jnp.concatenate([xs[0:8, :], hi], axis=0).astype(BF16)

    def f_units():
        xs = res["xs"]
        acts = []
        for j in range(F // LANES):
            cs = slice(j * LANES, (j + 1) * LANES)
            g = jnp.dot(gated(xs), wload(wg_v, 0, D, cs), preferred_element_type=F32)
            yield
            u = jnp.dot(xs, wload(wu_v, 0, D, cs), preferred_element_type=F32)
            acts.append((g * jax.nn.sigmoid(g) * u).astype(BF16))
            yield
        act = jnp.concatenate(acts, axis=1)
        zf = pltpu.bitcast(zero_u, F32)
        ys = []
        KF = (F // D) * D
        for c in range(0, NC, 2):
            acc = jnp.concatenate([jnp.concatenate([zf, zf], axis=0)] * 2, axis=1)
            acc = acc + jnp.dot(gated(act[:, KF:]), wload(wd_v, KF, F - KF, slice(c * LANES, (c + 2) * LANES)),
                                preferred_element_type=F32)
            yield
            for cc in range(2):
                y = acc[:, cc * LANES:(cc + 1) * LANES]
                for k0 in range(0, KF, D):
                    y = y + jnp.dot(gated(act[:, k0:k0 + D]),
                                    wload(wd_v, k0, D, slice((c + cc) * LANES, (c + cc + 1) * LANES)),
                                    preferred_element_type=F32)
                    yield
                ys.append(y)
        res["y"] = jnp.concatenate(ys, axis=1)

    def side_units():
        yield from range(NPRE)
        yield from c_units()
        yield from range(NGAP)
        yield from f_units()

    side = side_units()

    def o_dot(lhs, rhs):
        p = pc.dot(lhs, rhs) if st["step"] < NPRE else jnp.dot(lhs, rhs, preferred_element_type=F32)
        next(side, None)
        st["step"] += 1
        return p

    def o_plain(r0, n):
        lhs = pltpu.bitcast(pqn_v[r0 // 2:(r0 + n) // 2, :], BF16)
        parts = []
        for c0 in range(0, NC, 2):
            acc = x_v[DEF + L0 + r0:DEF + L0 + r0 + n, c0 * LANES:(c0 + 2) * LANES].astype(F32)
            for k0 in range(0, D, 2 * LANES):
                acc = acc + o_dot(lhs[:, k0:k0 + 2 * LANES], wload(mp_v, k0, 2 * LANES, slice(c0 * LANES, (c0 + 2) * LANES)))
            parts.append(acc)
        return jnp.concatenate(parts, axis=1)

    toks = []
    r0 = 0
    pc.add(post_jobs(OCL[0][0], *OCL[1]), pc.t + 200, pc.t + 1000, QP_DELAY)
    for ci, (n, plain) in enumerate(OCL):
        h = o_plain(r0, n) if plain else o_part(o_dot, x_v, DEF + L0, r0, n)
        last = r0 + n == RL
        units = ln2_jobs(h, ln2_v, out_v, DEF + L0 + r0, -DEF, None, st, fast=last)
        posts = post_jobs(r0 + n + OCL[ci + 1][0], *OCL[ci + 2]) if ci + 2 < len(OCL) else []
        for k, job in enumerate(units):
            toks.append(job(toks[-LAG_L] if len(toks) >= LAG_L and not last else None))
            if posts and k % 2:
                posts.pop(0)(toks[-1])
        if GLAG[ci] is not None:
            st["pend"].append((st["step"] + GLAG[ci],
                               pltpu.bitcast(jnp.broadcast_to(st["top1"], (8, LANES)), U32) & zero_u))
        r0 += n
        if last or r0 in OUT_AT:
            out_copy(L0 + st["sent"], r0 - st["sent"], 2 if last else 1).start()
            if not last:
                st["sent"] = r0
    for _ in side:
        st["step"] += 1

    keyv = best2(st["top1"], st["top2"])
    idx = [jnp.clip(key_row(kk[0, 0]), 0, S - 1) for kk in keyv]
    grp = [pl.multiple_of((ii >> 3) << 3, 8) for ii in idx]
    vgrp = [pl.multiple_of(gg + DEF, 8) for gg in grp]
    y = res["y"]
    ids_lo, ids_hi = res["ids"]
    hits = None
    yrows = []
    for c in range(2):
        m_lo = ids_lo == key_row(keyv[c])
        m_hi = ids_hi == key_row(keyv[c])
        yrows.append(subsum(jnp.where(wide(m_lo), y[0:8, :], 0.0) + jnp.where(wide(m_hi), y[8:16, :], 0.0)))
        hit = submax(jnp.where(m_lo | m_hi, 1, 0))
        hits = hit if hits is None else hits + hit
    hit_all = hits[0, 0] == 2

    tail0 = L0 + st["sent"]
    tail_copy = out_copy(tail0, S - tail0, 2)
    in_tail = jnp.maximum(grp[0], grp[1]) >= tail0
    two_groups = grp[1] != grp[0]

    def fix_copy(c):
        return out_copy(grp[c], 8, 3 + c)

    def finish(ysel):
        for c in range(2):
            hi = keyv[c] & jnp.int32(-65536)
            score = pltpu.bitcast(hi ^ ((hi >> 31) & 0x7FFF0000), F32)
            sel = (key_row(keyv[c]) & 7) == sub8
            upd = jnp.where(wide(sel), ysel[c] * wide(jax.nn.sigmoid(score)), 0.0)
            out_v[pl.ds(vgrp[c], 8), :] = (out_v[pl.ds(vgrp[c], 8), :].astype(F32) + upd).astype(BF16)
        fix_copy(0).start()

        @pl.when(two_groups)
        def _():
            fix_copy(1).start()

    out_copy(0, L0, 0).wait()
    out_copy(L0, tail0 - L0, 1).wait()

    @pl.when(in_tail)
    def _():
        tail_copy.wait()

    @pl.when(hit_all)
    def _():
        finish(yrows)

    @pl.when(jnp.logical_not(hit_all))
    def _():
        xsel = jnp.concatenate([ln2_v[pl.ds(vgrp[c], 8), :] for c in range(2)], axis=0)

        def ffn_tile(j, acc):
            cs = pl.ds(pl.multiple_of(j * LANES, LANES), LANES)
            g = jnp.dot(xsel, wload(wg_v, 0, D, cs), preferred_element_type=F32)
            u = jnp.dot(xsel, wload(wu_v, 0, D, cs), preferred_element_type=F32)
            a = (g * jax.nn.sigmoid(g) * u).astype(BF16)
            wd_t = pltpu.bitcast(wd_v[pl.ds(pl.multiple_of(j * (LANES // 2), LANES // 2), LANES // 2), 0:D], BF16)
            return acc + jnp.dot(a, wd_t, preferred_element_type=F32)

        yf = lax.fori_loop(0, F // LANES, ffn_tile, jnp.zeros((16, D), F32))
        finish([yf[0:8, :], yf[8:16, :]])

    @pl.when(jnp.logical_not(in_tail))
    def _():
        tail_copy.wait()

    fix_copy(0).wait()

    @pl.when(two_groups)
    def _():
        fix_copy(1).wait()


@jax.jit
def pallas_sequential_preLN__linear_attn_block__moe_arch_mod__prompt_kernel(
    A_x: jax.Array,
    A_wqkv: jax.Array,
    A_wo: jax.Array,
    B_x: jax.Array,
    B_w_r: jax.Array,
    B_w_gate: jax.Array,
    B_w_up: jax.Array,
    B_w_down: jax.Array,
):
    del B_x
    x = A_x.reshape(S, D)
    wr = B_w_r.reshape(NC, LANES)
    any_spec = pl.BlockSpec(memory_space=pl.ANY)
    out = pl.pallas_call(
        _kernel,
        out_shape=jax.ShapeDtypeStruct((S, D), BF16),
        in_specs=[any_spec] * 7,
        out_specs=any_spec,
        scratch_shapes=[
            pltpu.VMEM((S + DEF, D), BF16),
            pltpu.VMEM((D // 2, D), U32),
            pltpu.VMEM((D // 2, D), U32),
            pltpu.VMEM((2, D // 2, D), U32),
            pltpu.VMEM((NC, LANES), BF16),
            pltpu.VMEM((2, D // 2, F + LANES), U32),
            pltpu.VMEM((F // 2, D + LANES), U32),
            pltpu.VMEM((P0 // 2, D), U32),
            pltpu.VMEM((XSN, S // NA // 2, DA), U32),
            pltpu.VMEM((7 ** LK, DK // 2, DK), U32),
            pltpu.VMEM((D // 2, P0), U32),
            pltpu.VMEM((7 ** LG, DG // 2, TB // NG), U32),
            pltpu.VMEM((D, LANES), F32),
            pltpu.VMEM((D, LANES), F32),
            pltpu.VMEM((RL, LANES), F32),
            pltpu.VMEM((D, D), F32),
            pltpu.VMEM((D // 2, D), U32),
            pltpu.VMEM((7 ** LA, DA // 2, DA), U32),
            pltpu.VMEM((D // 2, D), U32),
            pltpu.VMEM((7 ** LO, DO // 2, DO), U32),
            pltpu.VMEM((max(TB2, RL), D + 2 * LANES), F32),
            pltpu.VMEM((RL // 2, D), U32),
            pltpu.VMEM((7 ** LO, max(TB2, RL) // NO // 2, DO), U32),
            pltpu.VMEM((DEF, D), F32),
            pltpu.VMEM((2, S + DEF, D), BF16),
            pltpu.VMEM((TB, D), F32),
            pltpu.VMEM((8, LANES), U32),
            pltpu.SemaphoreType.DMA((NSEM,)),
        ],
        compiler_params=pltpu.CompilerParams(vmem_limit_bytes=110 * 1024 * 1024, disable_bounds_checks=True,
                                             disable_semaphore_checks=True),
    )(x, A_wqkv, A_wo, wr, B_w_gate, B_w_up, B_w_down)
    return out.reshape(1, S, D)
```

```python
import jax
import jax.numpy as jnp
from jax import lax
import jax.experimental.pallas as pl
import jax.experimental.pallas.tpu as pltpu


S = 2048
D = 1024
F = 3584
H = 32
DH = D // H
LANES = 128
NC = D // LANES
HD = D // 2

LA = 2
LG = 1
LK = 2
LO = 1
NA, NG, NK, NO = 2 ** LA, 2 ** LG, 2 ** LK, 2 ** LO
DA, DG, DK, DO = D // NA, D // NG, D // NK, D // NO
XSN = 7 ** LA if LG == LA else 9 * 7 ** LG
P0 = 512
PB = S - P0
TX = 256
TB = 512
NB1 = PB // TB
TB2 = 512
NB2 = 3
QA = 256
OCH = (128, 128, 128, 128)
DEF = OCH[-1]
L0 = NB2 * TB2
RL = S - L0
QS = (256, 256)
OCL = ((128, False), (128, False), (128, False), (64, True), (64, True))
NPRE = 24
NGAP = 10
OUT_AT = (256, 384, 448)
LNU = 8
LAG_L = 4
LN_DELAY = 800
JOB_DELAY = 500
POST_DELAY = 800
GM = 128
PGM = 128
PGN = 128
PKM = 128
PKK = 256
EV0 = 0
EV1 = 0
EVT = 0
TRW = 256
TRM = 128
GN = 128
WK5 = 66
C6LN = (1000, 8900)
C6WK = (1500, 8900)
P1LN = (60, 12000)
P1WP = (6300, 11500)
P1WQ = (7500, 13100)
WQP = 5
EV2 = 300
P2U = (60, 2600)
P2X = (4300, 5900)
LAG = 5
QFIN = False
HFIN = True
EV3 = 0
LN2_DELAY = 900
QP_DELAY = 400
GLAG = (None, None, None, 20, 8)

F32 = jnp.float32
BF16 = jnp.bfloat16
U32 = jnp.uint32
I32 = jnp.int32

XP = ((PB, 128), (PB + 128, 128), (PB + 256, 256), (0, TB), (TB, PB - TB))
WKP = ((0, 128), (128, 128), (256, 256), (512, 512))

SEM_X = 0
SEM_WK = SEM_X + len(XP)
SEM_WQ = SEM_WK + len(WKP)
SEM_W3 = SEM_WQ + 1
SEM_WR = SEM_W3 + 1
SEM_WGU = SEM_WR + 1
SEM_WD = SEM_WGU + 1
SEM_OUT = SEM_WD + 1
NSEM = SEM_OUT + 5

INT_MIN = -(2 ** 31)


def _layernorm(x, tok=None, w=None):
    s0 = x[:, 0:LANES]
    if tok is not None:
        s0 = s0 + jnp.concatenate([tok] * (x.shape[0] // 8), axis=0)
    for c in range(1, NC):
        s0 = s0 + x[:, c * LANES:(c + 1) * LANES]
    mu = jnp.sum(s0, axis=-1, keepdims=True) * (1.0 / D)
    xc = x - mu
    var = jnp.sum(xc * xc, axis=-1, keepdims=True) * (1.0 / D)
    rstd = lax.rsqrt(var + 1e-5)
    if w is None:
        return xc * rstd
    return xc * rstd, jnp.sum(xc * w, axis=-1, keepdims=True) * rstd


def _phi(t):
    return jnp.where(t > 0, t + 1.0, jnp.exp(t)) + 1e-6


def _n_off(a, b):
    return 32 * a + 8 * b


def _n_groups():
    pos = {(2 * o + e) * LANES + _n_off(a, b): (16 * e + 4 * b + a) * DH + 8 * o
           for o in range(4) for e in range(2) for a in range(4) for b in range(4)}
    return [pos[n] for n in sorted(pos)]


def _quads(b):
    h = len(b) // 2
    return [[r[j * h:(j + 1) * h] for r in b[i * h:(i + 1) * h]] for i in range(2) for j in range(2)]


def _badd(x, y):
    return [[a + b for a, b in zip(rx, ry)] for rx, ry in zip(x, y)]


def _bsub(x, y):
    return [[a - b for a, b in zip(rx, ry)] for rx, ry in zip(x, y)]


def _a_set(b):
    if len(b) == 1:
        return [b[0][0]]
    return [x for o in _a_ops(b) for x in _a_set(o)]


def _b_set(b):
    if len(b) == 1:
        return [b[0][0]]
    q11, q12, q21, q22 = _quads(b)
    ops = (_badd(q11, q22), q11, _bsub(q12, q22), _bsub(q21, q11), q22, _badd(q11, q12), _badd(q21, q22))
    return [x for o in ops for x in _b_set(o)]


def _b_in_a(i, levels):
    perm = (0, 2, 6, 5, 3, 4, 1)
    return sum(perm[(i // 7 ** l) % 7] * 7 ** l for l in range(levels))


def _strassen(prod, levels, base=0, fin=lambda k, q: q, init=None):
    if levels == 0:
        return [[prod(base)]]

    def m(i):
        return _strassen(prod, levels - 1, base * 7 + i)

    def seed(q, x):
        return x if init is None else _badd(_quads(init)[q], x)

    m2 = m(2)
    c22 = seed(3, m2)
    m4 = m(4)
    c12 = fin(1, _badd(seed(1, m2), m4))
    c11 = m4 if init is None else _bsub(_quads(init)[0], m4)
    m3 = m(3)
    c11 = _bsub(m3, c11) if init is None else _badd(c11, m3)
    m1 = m(1)
    c21 = fin(2, _badd(seed(2, m3), m1))
    c22 = _bsub(c22, m1)
    m0 = m(0)
    c11 = _badd(c11, m0)
    c22 = _badd(c22, m0)
    c11 = fin(0, _badd(c11, m(6)))
    c22 = fin(3, _badd(c22, m(5)))
    return [a + b for a, b in zip(c11, c12)] + [a + b for a, b in zip(c21, c22)]


def _goff(i, levels):
    return int(format(i, "0%db" % levels)[::-1], 2) if levels else 0


def _blocks(rows, n):
    w = rows[0].shape[1] // n
    return [[r[:, j * w:(j + 1) * w] for j in range(n)] for r in rows]


def _or_all(vals):
    acc = None
    for v in vals:
        v = pltpu.bitcast(v, U32)
        for g in range(v.shape[0] // 8):
            for c in range(v.shape[1] // LANES):
                p = v[g * 8:(g + 1) * 8, c * LANES:(c + 1) * LANES]
                acc = p if acc is None else acc | p
    return acc


def _raw_ops(levels):
    n = 2 ** levels
    names = [[_Tag((i, j)) for j in range(n)] for i in range(n)]
    return {op: t.ij for op, t in enumerate(_b_set(names)) if t.ij is not None}


class _Tag:
    def __init__(self, ij):
        self.ij = ij

    def __add__(self, other):
        return _Tag(None)

    __sub__ = __add__


def _a_ops(b):
    q11, q12, q21, q22 = _quads(b)
    return (_badd(q11, q22), _badd(q21, q22), q11, q22, _badd(q11, q12), _bsub(q21, q11), _bsub(q12, q22))


def _x_set(o):
    return _a_set(o) + ([] if LG == LA else [o[0][1], o[1][0]])


_A_FORM = (((0, 0), (1, 1), 1), ((1, 0), (1, 1), 1), ((0, 0),), ((1, 1),), ((0, 0), (0, 1), 1),
           ((1, 0), (0, 0), -1), ((0, 1), (1, 1), -1))
_B_FORM = (((0, 0), (1, 1), 1), ((0, 0),), ((0, 1), (1, 1), -1), ((1, 0), (0, 0), -1), ((1, 1),),
           ((0, 0), (0, 1), 1), ((1, 0), (1, 1), 1))


def _outer(form, get, n):
    h = n // 2

    def quad(q):
        return [[get(q[0] * h + i, q[1] * h + j) for j in range(h)] for i in range(h)]

    if len(form) == 1:
        return quad(form[0])
    return (_badd if form[2] > 0 else _bsub)(quad(form[0]), quad(form[1]))


def _x_slot(i):
    return i if LG == LA else (i // 7) * 9 + i % 7


def _merge(b):
    return jnp.concatenate([jnp.concatenate(r, axis=1) for r in b], axis=0)


def _gate(v, tok):
    u = pltpu.bitcast(v, U32)
    top = u[0:8, 0:LANES] | tok
    if u.shape[1] > LANES:
        top = jnp.concatenate([top, u[0:8, LANES:]], axis=1)
    return pltpu.bitcast(jnp.concatenate([top, u[8:, :]], axis=0) if u.shape[0] > 8 else top, BF16)


class _Pacer:
    def __init__(self, zero, every=0):
        self.zero, self.t, self.jobs, self.pend, self.tok = zero, 0, [], [], None
        self.every, self.last = every, -every

    def add(self, jobs, t0, t1, delay):
        for k, job in enumerate(jobs):
            self.jobs.append((t0 + k * (t1 - t0) // len(jobs), len(self.jobs), job, delay))
        self.jobs.sort(key=lambda e: e[:2])

    def due(self, dep, delay):
        if dep is not None:
            self.pend.append((self.t + delay, _or_all([dep])))

    def release(self, upto):
        while self.jobs and self.jobs[0][0] <= upto:
            _, _, job, delay = self.jobs.pop(0)
            self.due(job(self.tok), delay)

    def dot(self, lhs, rhs):
        self.release(self.t)
        ready = [d for t, d in self.pend if t <= self.t]
        if ready and self.t - self.last >= self.every:
            self.pend = [e for e in self.pend if e[0] > self.t]
            self.last = self.t
            lhs = _gate(lhs, _or_all(ready) & self.zero)
        res = jnp.dot(lhs, rhs, preferred_element_type=F32)
        self.t += lhs.shape[0] * (lhs.shape[1] // LANES) * (res.shape[1] // LANES) // 4
        self.tok = pltpu.bitcast(pltpu.bitcast(res[0:8, 0:LANES], U32) & self.zero, F32)
        return res

    def flush(self):
        self.release(1 << 30)


def _kernel(x_hbm, wqkv_hbm, wo_hbm, wr_hbm, wg_hbm, wu_hbm, wd_hbm, out_hbm,
            x_v, wk_v, wq_v, w3_v, wr_v, wgu_v, wd_v,
            ln1_v, xs_v, wks_v, pkt_v, pks_v, zacc_v, uacc_v, xw_v, g_v, wqp_v, wqs_v, mp_v, ms_v, pq_v, pqn_v, pqs_v, attn_v, lo_v, lnf_v, zero_v,
            sems):

    ln2_v, out_v = lo_v.at[0], lo_v.at[1]

    wqkv_hbm, wo_hbm, wg_hbm, wu_hbm, wd_hbm = (r.bitcast(U32) for r in (wqkv_hbm, wo_hbm, wg_hbm, wu_hbm, wd_hbm))

    def wload(ref, r0, nr, cols):
        return pltpu.bitcast(ref[r0 // 2:(r0 + nr) // 2, cols], BF16)

    wv_v, wo_v = w3_v.at[0], w3_v.at[1]
    wg_v, wu_v = wgu_v.at[0], wgu_v.at[1]

    def x_copy(i):
        r0, n = XP[i]
        return pltpu.make_async_copy(x_hbm.at[pl.ds(r0, n), :], x_v.at[pl.ds(DEF + r0, n), :], sems.at[SEM_X + i])

    def out_copy(r0, n, s):
        return pltpu.make_async_copy(out_v.at[pl.ds(DEF + r0, n), :], out_hbm.at[pl.ds(r0, n), :],
                                     sems.at[SEM_OUT + s])

    def wk_copy(j):
        c0, n = WKP[j]
        return pltpu.make_async_copy(wqkv_hbm.at[:, pl.ds(D + c0, n)], wk_v.at[:, pl.ds(c0, n)],
                                     sems.at[SEM_WK + j])

    wq_copy = pltpu.make_async_copy(wqkv_hbm.at[:, pl.ds(0, D)], wq_v, sems.at[SEM_WQ])
    wr_copy = pltpu.make_async_copy(wr_hbm, wr_v, sems.at[SEM_WR])
    wd_copy = pltpu.make_async_copy(wd_hbm, wd_v.at[:, pl.ds(0, D)], sems.at[SEM_WD])
    wg_copy = pltpu.make_async_copy(wg_hbm, wg_v.at[:, pl.ds(0, F)], sems.at[SEM_WGU])
    wu_copy = pltpu.make_async_copy(wu_hbm, wu_v.at[:, pl.ds(0, F)], sems.at[SEM_WGU])

    x_copy(0).start()
    wk_copy(0).start()
    x_copy(1).start()
    wr_copy.start()
    for j in range(1, len(WKP)):
        wk_copy(j).start()
    for j in range(2, len(XP)):
        x_copy(j).start()
    wq_copy.start()
    pltpu.make_async_copy(wqkv_hbm.at[:, pl.ds(2 * D, D)], wv_v, sems.at[SEM_W3]).start()
    pltpu.make_async_copy(wo_hbm, wo_v, sems.at[SEM_W3]).start()
    wg_copy.start()
    wu_copy.start()
    wd_copy.start()

    def ln1_rows(xr, xr0, lnr, r0, n):
        ln = _layernorm(xr[xr0:xr0 + n, :].astype(F32)).astype(BF16)
        lnr[r0 // 2:(r0 + n) // 2, :] = pltpu.bitcast(ln, U32)

    def ln1_set(pc, xr, xr0, xsr, a0, n, t0, t1):
        def unit(j):
            def job(tok):
                ln = _layernorm(xr[xr0 + j * LNU:xr0 + (j + 1) * LNU, :].astype(F32), tok)
                lnf_v[j * LNU:(j + 1) * LNU, :] = ln
                return _or_all([ln[:, 0:LANES], ln[:, D - LANES:D]])
            return job

        def piece(j0, c0, o):
            def job(tok):
                def get(i, f):
                    r = (j0 + 2 * _goff(i, LA)) * LNU
                    v = lnf_v[r:r + 16, f * DA + c0:f * DA + c0 + LANES]
                    return v + jnp.concatenate([tok, tok], axis=0) if (i + f) % (NA // 2 + 1) == 0 else v

                r = (a0 + (j0 // (2 * NA)) * 16) // 2
                ops = _x_set(_outer(_A_FORM[o], get, NA))
                for op, v in enumerate(ops):
                    xsr.at[o * len(ops) + op][r:r + 8, c0:c0 + LANES] = pltpu.bitcast(v.astype(BF16), U32)
                return _or_all([v[0:8, :] for v in [ops[0]] + ops[5:7]])
            return job

        grp = 2 * NA
        ng = n // LNU // grp
        dt = (t1 - t0 - LN_DELAY) // (ng + 1)
        for g in range(ng):
            pc.add([unit(g * grp + j) for j in range(grp)], t0 + g * dt, t0 + (g + 1) * dt, LN_DELAY)
            s = t0 + (g + 1) * dt + LN_DELAY
            pc.add([piece(g * grp, c0, o) for c0 in range(0, DA, LANES) for o in range(7)], s, s + dt, JOB_DELAY)

    def ln1_load(lnr, r0, n):
        return pltpu.bitcast(lnr[r0 // 2:(r0 + n) // 2, :], BF16)

    def gate(v, tok):
        return v if tok is None else _gate(v, tok)

    def k_mm(r0, n, c0, nc):
        return jnp.dot(ln1_load(ln1_v, r0, n), wload(wk_v, 0, D, slice(c0, c0 + nc)), preferred_element_type=F32)

    def z_acc(pkts, c0, first=False):
        zs = None
        for pkt in pkts:
            for j in range(pkt.shape[1] // LANES):
                p = pkt[:, j * LANES:(j + 1) * LANES]
                zs = p if zs is None else zs + p
        if first:
            zacc_v[c0:c0 + zs.shape[0], :] = zs
        else:
            zacc_v[c0:c0 + zs.shape[0], :] += zs

    def k_post(k, p0, c0, first=False):
        n, nc = k.shape
        pkt = _phi(k).T
        pkt_v[c0 // 2:(c0 + nc) // 2, p0:p0 + n] = pltpu.bitcast(pkt.astype(BF16), U32)
        z_acc([pkt], c0, first)
        return pkt[nc - 8:nc, n - LANES:n]

    def g_acc(r0, n, c0, nc, first=False, pc=None):
        h, w = (nc, D) if pc is None else (min(nc, PGM), PGN)
        for f0 in range(c0, c0 + nc, h):
            for j0 in range(0, D, w):
                lhs = pltpu.bitcast(pkt_v[f0 // 2:(f0 + h) // 2, r0:r0 + n], BF16)
                rhs = pltpu.bitcast(ln1_v[r0 // 2:(r0 + n) // 2, j0:j0 + w], BF16)
                g = jnp.dot(lhs, rhs, preferred_element_type=F32) if pc is None else pc.dot(lhs, rhs)
                if first:
                    g_v[f0:f0 + h, j0:j0 + w] = g
                else:
                    g_v[f0:f0 + h, j0:j0 + w] += g

    def k_paced(pc, r0, c0, nc, first):
        for j0 in range(c0, c0 + nc, LANES):
            for t0 in range(r0, r0 + TX, PKM):
                k = None
                for k0 in range(0, D, PKK):
                    p = pc.dot(ln1_load(ln1_v, t0, PKM)[:, k0:k0 + PKK], wload(wk_v, k0, PKK, slice(j0, j0 + LANES)))
                    k = p if k is None else k + p
                pc.due(k_post(k, t0, j0, first and t0 == r0), POST_DELAY)

    attn_v[...] = jnp.zeros_like(attn_v)
    zero_v[...] = jnp.zeros_like(zero_v)

    x_copy(0).wait()
    ln1_rows(x_v, DEF + PB, ln1_v, 0, 128)
    wk_copy(0).wait()
    ka = k_mm(0, 128, 0, 128)
    x_copy(1).wait()
    wr_copy.wait()
    ln1_rows(x_v, DEF + PB + 128, ln1_v, 128, 128)
    k_post(ka, 0, 0, first=True)
    g_acc(0, 128, 0, 128, first=True)
    wk_copy(1).wait()
    k_post(k_mm(128, 128, 0, 128), 128, 0)
    k_post(k_mm(0, TX, 128, 128), 0, 128, first=True)
    g_acc(128, 128, 0, 128)
    def w_job(src_ref, dst_ref, levels, r0, c0, o):
        n = 2 ** levels
        w, raw, inner = D // n, _raw_ops(levels), 7 ** (levels - 1)

        def job(tok):
            def cut(i, j):
                return src_ref[(i * w + r0) // 2:(i * w + r0) // 2 + 8, j * w + c0:j * w + c0 + LANES]

            def get(i, j):
                u = cut(i, j)
                return pltpu.bitcast(u if tok is None else u | pltpu.bitcast(tok, U32), BF16).astype(F32)

            ops = []
            for op, v in enumerate(_b_set(_outer(_B_FORM[o], get, n))):
                dst = dst_ref.at[o * inner + op]
                if o * inner + op in raw:
                    dst[r0 // 2:r0 // 2 + 8, c0:c0 + LANES] = cut(*raw[o * inner + op])
                else:
                    dst[r0 // 2:r0 // 2 + 8, c0:c0 + LANES] = pltpu.bitcast(v.astype(BF16), U32)
                    ops.append(v)
            return _or_all(ops[0:1] + ops[-2:]) if ops else None
        return job

    def wk_jobs_of(outer):
        return [w_job(wk_v, wks_v, LK, r0, c0, o) for r0 in range(0, DK, 16) for c0 in range(0, DK, LANES)
                for o in outer]

    wk_copy(2).wait()
    pc = _Pacer(zero_v[...], EV0)
    pc.add(wk_jobs_of((1, 3)), 500, 2200, JOB_DELAY)
    k_paced(pc, 0, 256, 256, True)
    g_acc(0, TX, 128, 128, True, pc)
    g_acc(0, TX, 256, 256, True, pc)
    pc.flush()
    wk_copy(3).wait()
    wk_jobs = wk_jobs_of((0, 2, 4, 5, 6))
    pc = _Pacer(zero_v[...], EV0)
    pc.add(wk_jobs[:WK5], 500, 2700, JOB_DELAY)
    k_paced(pc, 0, 512, 512, True)
    g_acc(0, TX, 512, 256, True, pc)
    pc.flush()
    x_copy(2).wait()
    x_copy(3).wait()
    pc = _Pacer(zero_v[...], EV0)
    ln1_set(pc, x_v, DEF, xs_v, 0, TB, *C6LN)
    pc.add(wk_jobs[WK5:], *C6WK, JOB_DELAY)
    ln1_rows(x_v, DEF + PB + TX, ln1_v, TX, TX)
    g_acc(0, TX, 768, 256, True, pc)
    k_paced(pc, TX, 0, D, False)
    for c0 in range(0, D, 256):
        g_acc(TX, TX, c0, 256, False, pc)
    pc.flush()

    MA = TB // NA
    NS = NK // NG

    def xs_load(xsr, op, a0, m, cols=slice(None)):
        return pltpu.bitcast(xsr[op, a0 // 2:(a0 + m) // 2, cols], BF16)

    def k_step(pc, xsr, j0):
        def fin(_, q):
            if NS > 1:
                q = [[jnp.concatenate([_phi(jnp.concatenate([r[f] for r in q], axis=0)).T for f in range(NS)],
                                      axis=0)]]
            else:
                q = [[_phi(v).T for v in r] for r in q]
            pc.due(_or_all([v[t - 8:t, :] for r in q for v in r for t in range(LANES, v.shape[0] + 1, LANES)]),
                   POST_DELAY)
            return q

        def lhs(i):
            if LK == LA:
                return xs_load(xsr, _x_slot(i), 0, MA)
            return _merge([[xs_load(xsr, i * 9 + s, 0, MA) for s in r] for r in ((2, 7), (8, 3))])

        cb = _strassen(lambda i: pc.dot(lhs(i), pltpu.bitcast(wks_v[i, :, j0:j0 + LANES], BF16)), LK, fin=fin)
        ops = _a_ops([[cb[i][f] for i in range(NG)] for f in range(NG)])
        for half, o in ((0, ops[4]), (1, ops[1])):
            for f, rowb in enumerate(o):
                for s in range(NS):
                    z_acc([v[s * LANES:(s + 1) * LANES, :] for v in rowb], half * HD + f * DG + s * DK + j0)
        for _ in range(LG - 1):
            ops = [o for x in ops for o in _a_ops(x)]
        for op, o in enumerate(ops):
            r = j0 * NS
            pks_v.at[op][r // 2:(r + NS * LANES) // 2, :] = pltpu.bitcast(o[0][0].astype(BF16), U32)
        pc.due(_or_all([o[0][0][NS * LANES - 8:NS * LANES, :] for o in (ops[0], ops[-1], ops[-2])]), 2 * POST_DELAY)

    def g_rhs(xsr, i, c0, nc):
        o = _b_in_a(i, LG)
        if LG == LA:
            return xs_load(xsr, o, 0, MA, slice(c0, c0 + nc))
        j, cs = c0 // DA, slice(c0 % DA, c0 % DA + nc)
        return jnp.concatenate([xs_load(xsr, o * 9 + s, 0, MA, cs) for s in ((2, 8), (7, 3))[j]], axis=0)

    def g_step(pc, xsr, r0, nr, c0, nc):
        cb = _strassen(lambda i: pc.dot(pltpu.bitcast(pks_v[i, r0 // 2:(r0 + nr) // 2, :], BF16),
                                        g_rhs(xsr, i, c0, nc)), LG)
        for f in range(NG):
            for c in range(NG):
                h = min(nr, LANES)
                for t in range(nr // h):
                    step, sub = divmod((r0 + t * h) // LANES, NS)
                    g0_ = f * DG + sub * DK + step * LANES + (r0 + t * h) % LANES
                    g_v[g0_:g0_ + h, c * DG + c0:c * DG + c0 + nc] += cb[f][c][t * h:(t + 1) * h, :]

    def wq_jobs(u0, nr):
        span = (NA - 1) * DA + 16 * nr
        u0 = u0 if isinstance(u0, int) else pl.multiple_of(u0, 8)
        srcr, permr = wq_v.at[pl.ds(u0, span // 2), :], wqp_v.at[pl.ds(u0, span // 2), :]
        dstr = wqs_v.at[:, pl.ds(u0, 8 * nr), :]
        oct_ = (lax.broadcasted_iota(I32, (8, LANES), 1) % DH) // 8

        def perm(r, e):
            def job(tok):
                blk = [srcr[r // 2:r // 2 + 8, (4 * e + b) * LANES:(4 * e + b + 1) * LANES] | pltpu.bitcast(tok, U32)
                       for b in range(4)]
                outs = []
                for o in range(4):
                    v = blk[o]
                    for b in range(4):
                        if b != o:
                            v = jnp.where(oct_ == b, pltpu.roll(blk[b], (8 * (b - o)) % LANES, 1), v)
                    permr[r // 2:r // 2 + 8, (2 * o + e) * LANES:(2 * o + e + 1) * LANES] = v
                    outs.append(v)
                return _or_all(outs)
            return job

        return ([perm(i * DA + r0, e) for r0 in range(0, 16 * nr, 16) for i in range(NA) for e in range(2)],
                [w_job(permr, dstr, LA, r0, c0, o) for r0 in range(0, 16 * nr, 16)
                 for c0 in range(0, DA, LANES) for o in range(7)])

    def p1(i, carry):
        xsr = xs_v.at[:, pl.ds(pl.multiple_of(i * (MA // 2), MA // 2), MA), :]
        xr = x_v.at[pl.ds(pl.multiple_of((i + 1) * TB, TB), TB + DEF), :]

        pc = _Pacer(zero_v[...], EV1)
        ln1_set(pc, xr, DEF, xsr, MA, TB, *P1LN)
        perms, sets = wq_jobs(i * (8 * WQP), WQP)
        pc.add(perms, *P1WP, JOB_DELAY)
        pc.add(sets, *P1WQ, JOB_DELAY)
        for j0 in range(0, DK, LANES):
            k_step(pc, xsr, j0)
        for f0 in range(0, DG, GM):
            for c0 in range(0, DG, GN):
                g_step(pc, xsr, f0, GM, c0, GN)
        pc.flush()
        return carry

    x_copy(4).wait()
    wq_copy.wait()
    lax.fori_loop(0, NB1, p1, 0)

    pltpu.make_async_copy(w3_v, w3_v, sems.at[SEM_W3]).wait()
    zero_u = zero_v[...]
    def row_vector(acc_ref):
        return jnp.sum(jnp.concatenate([acc_ref[r:r + 8, :] for r in _n_groups()], axis=0).T, axis=0, keepdims=True)

    zrow = row_vector(zacc_v)
    wr8 = wr_v[...].astype(F32)
    wr_row = jnp.concatenate([wr8[c:c + 1, :] for c in range(NC)], axis=1)

    row_h = lax.broadcasted_iota(I32, (LANES, LANES), 0) // DH
    col_h = lax.broadcasted_iota(I32, (LANES, LANES), 1) // DH
    diag = row_h == col_h

    def colsum(t):
        acc = t[:, 0:LANES]
        for c in range(1, NC):
            acc = acc + t[:, c * LANES:(c + 1) * LANES]
        return acc

    wrc = wr_row - jnp.sum(wr_row, axis=-1, keepdims=True) * (1.0 / D)
    m_raw = _raw_ops(LO)

    def kv_part(c):
        cs = slice(c * LANES, (c + 1) * LANES)
        kv = None
        for k0 in range(0, D, TRW):
            p = pc.dot(g_v[cs, k0:k0 + TRW].astype(BF16), wload(wv_v, k0, TRW, cs))
            kv = p if kv is None else kv + p
        return jnp.where(diag, kv, 0.0)

    def m_part(c, kvs):
        e, b = c // 4, c % 4
        for j0 in range(0, DO, TRM):
            ms = [jnp.concatenate(
                [pc.dot(kv, wload(wo_v, (c + k) * LANES, LANES, slice(f * DO + j0, f * DO + j0 + TRM)))
                 for f in range(NO)], axis=1) for k, kv in enumerate(kvs)]
            deps = []
            for a in range(4):
                rows = [jnp.concatenate([m[a * DH + 8 * o:a * DH + 8 * o + 8, :] for m in ms], axis=0)
                        for o in range(4)]
                for o in range(4):
                    r = ((2 * o + e) * LANES + _n_off(a, b)) // 2
                    for f in range(NO):
                        mp_v[r:r + 8, f * DO + j0:f * DO + j0 + TRM] = pltpu.bitcast(
                            rows[o][:, f * TRM:(f + 1) * TRM].astype(BF16), U32)
                for t in range(4 // NO):
                    r = ((2 * t + e) * LANES + _n_off(a, b)) // 2
                    for op, v in enumerate(_b_set(_blocks(rows[t::4 // NO], NO))):
                        if op not in m_raw:
                            ms_v.at[op][r:r + 8, j0:j0 + TRM] = pltpu.bitcast(v.astype(BF16), U32)
                            deps.append(v[0:8, 0:LANES])
            pc.due(_or_all(deps[::4]), POST_DELAY)

    pc = _Pacer(zero_u, EVT)
    pc.due(jnp.broadcast_to(zrow, (8, D)), 1000)
    perms, sets = wq_jobs(NB1 * 8 * WQP, DA // 16 - NB1 * WQP)
    pc.add(perms, 60, 700, JOB_DELAY)
    pc.add(sets, 1300, 3400, JOB_DELAY)
    kv_prev = None
    for c in range(0, NC + 2, 2):
        kvs = [kv_part(c).astype(BF16), kv_part(c + 1).astype(BF16)] if c < NC else None
        if c:
            m_part(c - 2, kv_prev)
        kv_prev = kvs
    pc.flush()

    def make_key(score, row):
        b = pltpu.bitcast(score, I32)
        srt = b ^ ((b >> 31) & 0x7FFFFFFF)
        return (srt & jnp.int32(-65536)) | (0xFFFF - row)

    def push_keys(key, top1, top2):
        for gidx in range(key.shape[0] // 8):
            kx = key[gidx * 8:(gidx + 1) * 8, :]
            top2 = jnp.maximum(top2, jnp.minimum(top1, kx))
            top1 = jnp.maximum(top1, kx)
        return top1, top2

    lane = lax.broadcasted_iota(I32, (1, LANES), 1)

    def interleave(parts):
        return jnp.concatenate([p[g * 16:(g + 1) * 16, :] for g in range(parts[0].shape[0] // 16) for p in parts],
                               axis=0)

    def q_part(pc, xsr, l0, r0, n, hint=None):
        m = n // NA
        sums = {}

        def park(v, g, c):
            for t in range(m // 16):
                r = r0 + (t * NA + g) * 16
                pq_v[r:r + 16, c * LANES:(c + 1) * LANES] = v[t * 16:(t + 1) * 16, :]

        def fin(k, q):
            q = [[_phi(v) for v in r] for r in q]
            deps = []
            for a, r in enumerate(q):
                for b, v in enumerate(r):
                    i, c = (k // 2) * (NA // 2) + a, (((k % 2) * (NA // 2) + b) * DA + j0) // LANES
                    park(v, _goff(i, LA), c)
                    for name, row in (("z", zrow),) + ((("u", hint["u"]),) if hint else ()):
                        t = v * row[:, c * LANES:(c + 1) * LANES]
                        key = (name, _goff(i, LA), c % 2)
                        sums[key] = t if key not in sums else sums[key] + t
                deps.append(sums[key])
            if (r0 + n < RL or HFIN) if hint else QFIN:
                pc.due(_or_all(deps), POST_DELAY)
            return q

        for j0 in range(0, DA, LANES):
            _strassen(lambda i: pc.dot(xs_load(xsr, _x_slot(i), (l0 + r0) // NA, m),
                                       pltpu.bitcast(wqs_v[i, :, j0:j0 + LANES], BF16)), LA, fin=fin)
        if hint:
            pc.flush()
        den = jnp.concatenate([sums["z", g, e] for g in range(NA) for e in range(2)], axis=0)
        for s in (1, 2, 4):
            den = den + jnp.where((lane & s) == 0, pltpu.roll(den, LANES - s, 1), pltpu.roll(den, s, 1))
        inv_all = 1.0 / (den + 1e-6)

        def inv_of(g):
            return [inv_all[(g * 2 + e) * m:(g * 2 + e + 1) * m, :] for e in range(2)]

        for g in range(NA):
            for e in range(2):
                park(inv_of(g)[e], g, NC + e)
        if hint:
            for g in range(NA):
                starts = [r0 + (t * NA + g) * 16 for t in range(m // 16)]
                num = jnp.sum(jnp.concatenate([xw_v[t:t + 16, :] for t in starts], axis=0)
                              + sums["u", g, 0] * inv_of(g)[0] + sums["u", g, 1] * inv_of(g)[1],
                              axis=-1, keepdims=True)
                row = jnp.concatenate([(l0 + t) + lax.broadcasted_iota(I32, (16, 1), 0) for t in starts], axis=0)
                hint["p1"], hint["p2"] = push_keys(make_key(num, row), hint["p1"], hint["p2"])
            pc.due(jnp.broadcast_to(hint["p1"], (8, LANES)), 1200)


    def post_jobs(r0, n, plain=False):
        def scaled(t, c0, w, tok):
            inv = pq_v[t:t + 16, D:D + 2 * LANES]
            if tok is not None:
                inv = inv + jnp.concatenate([jnp.concatenate([tok, tok], axis=0)] * 2, axis=1)
            return pq_v[t:t + 16, c0:c0 + w] * jnp.concatenate([inv] * (w // (2 * LANES)), axis=1)

        def post_plain(t):
            def job(tok):
                v = scaled(t, 0, D, tok)
                pqn_v[t // 2:t // 2 + 8, :] = pltpu.bitcast(v.astype(BF16), U32)
                return v[0:8, 0:LANES]
            return job

        def post(t0, outer):
            def job(tok):
                deps = []
                for c0 in range(0, DO, 2 * LANES):
                    blk = {}

                    def get(i, f):
                        if (i, f) not in blk:
                            blk[i, f] = scaled(t0 + _goff(i, LO) * 16, f * DO + c0, 2 * LANES, tok)
                        return blk[i, f]

                    for o in outer:
                        ops = _a_set(_outer(_A_FORM[o], get, NO))
                        for op, v in enumerate(ops):
                            pqs_v.at[o * len(ops) + op][t0 // NO // 2:t0 // NO // 2 + 8, c0:c0 + 2 * LANES] = (
                                pltpu.bitcast(v.astype(BF16), U32))
                        deps.append(ops[0][0:8, 0:LANES])
                return _or_all(deps)
            return job

        if plain:
            return [post_plain(t) for t in range(r0, r0 + n, 16)]
        outers = [range(7)] if LO == 1 else [(o,) for o in range(7)]
        return [post(t0, outer) for t0 in range(r0, r0 + n, 16 * NO) for outer in outers]

    def m_operand(i, c0, c1):
        if i not in m_raw:
            return pltpu.bitcast(ms_v[i, :, c0 * LANES:c1 * LANES], BF16)
        bi, bj = m_raw[i]
        return wload(mp_v, bi * DO, DO, slice(bj * DO + c0 * LANES, bj * DO + c1 * LANES))

    def o_part(dot, xr, x0, r0, n):
        a0, m = r0 // NO, n // NO
        nw = LANES * NO // 2
        cols = [[[] for _ in range(NO)] for _ in range(NO)]
        for c0 in range(0, DO, nw):
            init = [[jnp.concatenate(
                [xr[x0 + r0 + (g * NO + _goff(i, LO)) * 16:x0 + r0 + (g * NO + _goff(i, LO) + 1) * 16,
                    f * DO + c0:f * DO + c0 + nw] for g in range(m // 16)], axis=0).astype(F32)
                for f in range(NO)] for i in range(NO)]
            cb = _strassen(lambda i: dot(pltpu.bitcast(pqs_v[i, a0 // 2:(a0 + m) // 2, :], BF16),
                                         m_operand(i, c0 // LANES, (c0 + nw) // LANES)), LO, init=init)
            for i in range(NO):
                for f in range(NO):
                    cols[i][f].append(cb[i][f])
        parts = [None] * NO
        for i in range(NO):
            parts[_goff(i, LO)] = jnp.concatenate([c for f in range(NO) for c in cols[i][f]], axis=1)
        return interleave(parts)

    def ln2_unit(h, l2r, outr, r0, row0, valid, top1, top2, tok, fast=False):
        n = h.shape[0]
        if fast:
            ln2, r = _layernorm(h, tok, wr_row)
        else:
            ln2 = _layernorm(h, tok)
            r = jnp.sum(ln2 * wr_row, axis=-1, keepdims=True)
        l2r[r0:r0 + n, :] = ln2.astype(BF16)
        res = h + ln2
        outr[r0:r0 + n, :] = res.astype(BF16)
        r = r.astype(BF16).astype(F32) + 0.0
        key = make_key(r, (row0 + r0) + lax.broadcasted_iota(I32, (n, 1), 0))
        if valid is not None:
            key = jnp.where(valid, key, INT_MIN)
        top1, top2 = push_keys(key, top1, top2)
        ntok = pltpu.bitcast(pltpu.bitcast(jnp.broadcast_to(r[n - 8:n, :], (8, LANES)), U32) & zero_u, F32)
        return top1, top2, ntok

    def ln2_jobs(h, l2r, outr, r0, row0, valid, st, fast=False):
        def unit(j):
            def job(tok):
                st["top1"], st["top2"], dep = ln2_unit(h[j * LNU:(j + 1) * LNU, :], l2r, outr, r0 + j * LNU, row0,
                                                       valid, st["top1"], st["top2"], tok, fast)
                return dep
            return job
        return [unit(j) for j in range(h.shape[0] // LNU)]

    QC = 16 * 7 ** LA / 8 ** LA
    OC = 16 * 7 ** LO / 8 ** LO

    def p2(i, carry):
        st = dict(top1=carry[0], top2=carry[1])
        b0 = pl.multiple_of(i * TB2, 16)
        xsr = xs_v.at[:, pl.ds(pl.multiple_of(i * (TB2 // NA // 2), 8), TB2 // NA // 2), :]
        xr = x_v.at[pl.ds(b0, TB2 + DEF), :]
        l2r = ln2_v.at[pl.ds(b0, TB2 + DEF), :]
        outr = out_v.at[pl.ds(b0, TB2 + DEF), :]
        row0 = b0 - DEF
        pc = _Pacer(zero_u)
        toks = []

        def chain(jobs):
            for job in jobs:
                toks.append(job(toks[-LAG] if len(toks) >= LAG else None))

        chain(ln2_jobs(attn_v, l2r, outr, 0, row0, i > 0, st))

        @pl.when(i > 0)
        def _():
            out_copy(pl.multiple_of((i - 1) * TB2, 16), TB2, 0).start()

        pc.due(toks[-1], QA * QC)

        def u_job(r):
            def job(tok):
                t = colsum(gate(wload(mp_v, r, 32, slice(None)), pltpu.bitcast(tok, U32)).astype(F32) * wrc)
                uacc_v[r:r + 32, :] = t
                return t
            return job

        def xw_job(t):
            def job(tok):
                v = colsum(x_v[DEF + L0 + t:DEF + L0 + t + 16, :].astype(F32) * wrc)
                v = v + jnp.concatenate([tok, tok], axis=0)
                xw_v[t:t + 16, :] = v
                return v
            return job

        pc.add([u_job(r) for r in range(0, D, 32)], *P2U, JOB_DELAY)
        pc.add([xw_job(t) for t in range(0, RL, 16)], *P2X, JOB_DELAY)
        for r0, n in ((0, QA), (QA, TB2 - QA)):
            q_part(pc, xsr, 0, r0, n)
            for job in post_jobs(r0, n):
                job(None)
        r0 = 0
        for n in OCH[:-1]:
            chain(ln2_jobs(o_part(pc.dot, xr, DEF, r0, n), l2r, outr, DEF + r0, row0, None, st))
            r0 += n
        attn_v[...] = o_part(pc.dot, xr, DEF, r0, DEF)
        return st["top1"], st["top2"]

    init = jnp.full((8, 1), INT_MIN, I32)
    top1, top2 = lax.fori_loop(0, NB2, p2, (init, init))

    wg_copy.wait()
    wu_copy.wait()
    wd_copy.wait()
    sub8 = lax.broadcasted_iota(I32, (8, LANES), 0)
    urow = jnp.sum(uacc_v[...].T, axis=0, keepdims=True)

    def submax(v):
        for sh in (4, 2, 1):
            v = jnp.maximum(v, pltpu.roll(v, sh, 0))
        return v

    def subsum(v):
        for sh in (4, 2, 1):
            v = v + pltpu.roll(v, sh, 0)
        return v

    def best2(t1, t2):
        t1 = jnp.broadcast_to(t1, (8, LANES))
        t2 = jnp.broadcast_to(t2, (8, LANES))
        k1v = submax(t1)
        return k1v, submax(jnp.where(t1 == k1v, t2, t1))

    def key_row(k):
        return 0xFFFF - (k & 0xFFFF)

    def wide(m):
        return jnp.concatenate([m] * NC, axis=1)

    st = dict(top1=top1, top2=top2, pend=[], step=0, sent=0)
    pc = _Pacer(zero_u, EV2)
    hint = dict(u=urow, p1=init, p2=init)

    pc.add(ln2_jobs(attn_v, ln2_v, out_v, L0, -DEF, None, st), 60, QS[0] * QC - 600, LN2_DELAY)
    r0 = 0
    for k, n in enumerate(QS):
        q_part(pc, xs_v, L0, r0, n, hint)
        if k == 0:
            out_copy(L0 - TB2, TB2, 0).start()
            top1, top2 = st["top1"], st["top2"]
            pc.add(post_jobs(0, OCL[0][0], OCL[0][1]), pc.t + 600, pc.t + (RL - n) * QC - 300, QP_DELAY)
        r0 += n
    pc.every = EV3
    oldk = best2(top1, top2)
    oldx = []
    for kk in oldk:
        g8 = pl.multiple_of(((jnp.clip(key_row(kk[0, 0]), 0, S - 1) >> 3) << 3) + DEF, 8)
        rows = ln2_v[pl.ds(g8, 8), :].astype(F32)
        oldx.append(subsum(jnp.where(wide((key_row(kk) & 7) == sub8), rows, 0.0)))

    def gated(v):
        tok = None
        while st["pend"] and st["pend"][0][0] <= st["step"]:
            t = st["pend"].pop(0)[1]
            tok = t if tok is None else tok | t
        if tok is None:
            return v
        u = pltpu.bitcast(v, U32)
        return pltpu.bitcast(jnp.concatenate([u[:, 0:LANES] | tok, u[:, LANES:]], axis=1), BF16)

    res = {}

    def c_units():
        pc.flush()
        p1, p2_ = hint["p1"], hint["p2"]
        cand_p, cand_x = [], []
        for pk_ in (p1, p2_):
            cp, cx = None, None
            for s in range(8):
                g8 = pl.multiple_of((jnp.clip(key_row(pk_[s, 0]) - L0, 0, RL - 1) >> 3) << 3, 8)
                vp = pq_v[pl.ds(g8, 8), :]
                vx = x_v[pl.ds(pl.multiple_of(g8 + (L0 + DEF), 8), 8), :].astype(F32)
                cp = vp if cp is None else jnp.where(jnp.concatenate([sub8 == s] * (NC + 2), axis=1), vp, cp)
                cx = vx if cx is None else jnp.where(wide(sub8 == s), vx, cx)
            cand_p.append(cp[:, 0:D] * jnp.concatenate([cp[:, D:]] * (NC // 2), axis=1))
            cand_x.append(cx)
        cand_p = jnp.concatenate(cand_p, axis=0).astype(BF16)
        cand_x = jnp.concatenate(cand_x, axis=0)
        ids_lo = key_row(jnp.broadcast_to(p1, (8, LANES)))
        ids_hi = jnp.where(sub8 < 6, key_row(jnp.broadcast_to(p2_, (8, LANES))),
                           jnp.where(sub8 == 6, key_row(oldk[0]), key_row(oldk[1])))
        res["ids"] = (ids_lo, ids_hi)
        parts = []
        for c in range(NC):
            parts.append(jnp.dot(cand_p, wload(mp_v, 0, D, slice(c * LANES, (c + 1) * LANES)), preferred_element_type=F32))
            yield
        xs = _layernorm(cand_x + jnp.concatenate(parts, axis=1))
        hi = jnp.where(wide(sub8 < 6), xs[8:16, :], jnp.where(wide(sub8 == 6), oldx[0], oldx[1]))
        res["xs"] = jnp.concatenate([xs[0:8, :], hi], axis=0).astype(BF16)

    def f_units():
        xs = res["xs"]
        acts = []
        for j in range(F // LANES):
            cs = slice(j * LANES, (j + 1) * LANES)
            g = jnp.dot(gated(xs), wload(wg_v, 0, D, cs), preferred_element_type=F32)
            yield
            u = jnp.dot(xs, wload(wu_v, 0, D, cs), preferred_element_type=F32)
            acts.append((g * jax.nn.sigmoid(g) * u).astype(BF16))
            yield
        act = jnp.concatenate(acts, axis=1)
        zf = pltpu.bitcast(zero_u, F32)
        ys = []
        KF = (F // D) * D
        for c in range(0, NC, 2):
            acc = jnp.concatenate([jnp.concatenate([zf, zf], axis=0)] * 2, axis=1)
            acc = acc + jnp.dot(gated(act[:, KF:]), wload(wd_v, KF, F - KF, slice(c * LANES, (c + 2) * LANES)),
                                preferred_element_type=F32)
            yield
            for cc in range(2):
                y = acc[:, cc * LANES:(cc + 1) * LANES]
                for k0 in range(0, KF, D):
                    y = y + jnp.dot(gated(act[:, k0:k0 + D]),
                                    wload(wd_v, k0, D, slice((c + cc) * LANES, (c + cc + 1) * LANES)),
                                    preferred_element_type=F32)
                    yield
                ys.append(y)
        res["y"] = jnp.concatenate(ys, axis=1)

    def side_units():
        yield from range(NPRE)
        yield from c_units()
        yield from range(NGAP)
        yield from f_units()

    side = side_units()

    def o_dot(lhs, rhs):
        p = pc.dot(lhs, rhs) if st["step"] < NPRE else jnp.dot(lhs, rhs, preferred_element_type=F32)
        next(side, None)
        st["step"] += 1
        return p

    def o_plain(r0, n):
        lhs = pltpu.bitcast(pqn_v[r0 // 2:(r0 + n) // 2, :], BF16)
        parts = []
        for c0 in range(0, NC, 2):
            acc = x_v[DEF + L0 + r0:DEF + L0 + r0 + n, c0 * LANES:(c0 + 2) * LANES].astype(F32)
            for k0 in range(0, D, 2 * LANES):
                acc = acc + o_dot(lhs[:, k0:k0 + 2 * LANES], wload(mp_v, k0, 2 * LANES, slice(c0 * LANES, (c0 + 2) * LANES)))
            parts.append(acc)
        return jnp.concatenate(parts, axis=1)

    toks = []
    r0 = 0
    pc.add(post_jobs(OCL[0][0], *OCL[1]), pc.t + 200, pc.t + 1000, QP_DELAY)
    for ci, (n, plain) in enumerate(OCL):
        h = o_plain(r0, n) if plain else o_part(o_dot, x_v, DEF + L0, r0, n)
        last = r0 + n == RL
        units = ln2_jobs(h, ln2_v, out_v, DEF + L0 + r0, -DEF, None, st, fast=last)
        posts = post_jobs(r0 + n + OCL[ci + 1][0], *OCL[ci + 2]) if ci + 2 < len(OCL) else []
        for k, job in enumerate(units):
            toks.append(job(toks[-LAG_L] if len(toks) >= LAG_L and not last else None))
            if posts:
                posts.pop(0)(toks[-1])
        if GLAG[ci] is not None:
            st["pend"].append((st["step"] + GLAG[ci],
                               pltpu.bitcast(jnp.broadcast_to(st["top1"], (8, LANES)), U32) & zero_u))
        r0 += n
        if last or r0 in OUT_AT:
            out_copy(L0 + st["sent"], r0 - st["sent"], 2 if last else 1).start()
            if not last:
                st["sent"] = r0
    for _ in side:
        st["step"] += 1

    keyv = best2(st["top1"], st["top2"])
    idx = [jnp.clip(key_row(kk[0, 0]), 0, S - 1) for kk in keyv]
    grp = [pl.multiple_of((ii >> 3) << 3, 8) for ii in idx]
    vgrp = [pl.multiple_of(gg + DEF, 8) for gg in grp]
    y = res["y"]
    ids_lo, ids_hi = res["ids"]
    hits = None
    yrows = []
    for c in range(2):
        m_lo = ids_lo == key_row(keyv[c])
        m_hi = ids_hi == key_row(keyv[c])
        yrows.append(subsum(jnp.where(wide(m_lo), y[0:8, :], 0.0) + jnp.where(wide(m_hi), y[8:16, :], 0.0)))
        hit = submax(jnp.where(m_lo | m_hi, 1, 0))
        hits = hit if hits is None else hits + hit
    hit_all = hits[0, 0] == 2

    tail0 = L0 + st["sent"]
    tail_copy = out_copy(tail0, S - tail0, 2)
    in_tail = jnp.maximum(grp[0], grp[1]) >= tail0
    two_groups = grp[1] != grp[0]

    def fix_copy(c):
        return out_copy(grp[c], 8, 3 + c)

    def finish(ysel):
        for c in range(2):
            hi = keyv[c] & jnp.int32(-65536)
            score = pltpu.bitcast(hi ^ ((hi >> 31) & 0x7FFF0000), F32)
            sel = (key_row(keyv[c]) & 7) == sub8
            upd = jnp.where(wide(sel), ysel[c] * wide(jax.nn.sigmoid(score)), 0.0)
            out_v[pl.ds(vgrp[c], 8), :] = (out_v[pl.ds(vgrp[c], 8), :].astype(F32) + upd).astype(BF16)
        fix_copy(0).start()

        @pl.when(two_groups)
        def _():
            fix_copy(1).start()

    out_copy(0, L0, 0).wait()
    out_copy(L0, tail0 - L0, 1).wait()

    @pl.when(in_tail)
    def _():
        tail_copy.wait()

    @pl.when(hit_all)
    def _():
        finish(yrows)

    @pl.when(jnp.logical_not(hit_all))
    def _():
        xsel = jnp.concatenate([ln2_v[pl.ds(vgrp[c], 8), :] for c in range(2)], axis=0)

        def ffn_tile(j, acc):
            cs = pl.ds(pl.multiple_of(j * LANES, LANES), LANES)
            g = jnp.dot(xsel, wload(wg_v, 0, D, cs), preferred_element_type=F32)
            u = jnp.dot(xsel, wload(wu_v, 0, D, cs), preferred_element_type=F32)
            a = (g * jax.nn.sigmoid(g) * u).astype(BF16)
            wd_t = pltpu.bitcast(wd_v[pl.ds(pl.multiple_of(j * (LANES // 2), LANES // 2), LANES // 2), 0:D], BF16)
            return acc + jnp.dot(a, wd_t, preferred_element_type=F32)

        yf = lax.fori_loop(0, F // LANES, ffn_tile, jnp.zeros((16, D), F32))
        finish([yf[0:8, :], yf[8:16, :]])

    @pl.when(jnp.logical_not(in_tail))
    def _():
        tail_copy.wait()

    fix_copy(0).wait()

    @pl.when(two_groups)
    def _():
        fix_copy(1).wait()


@jax.jit
def pallas_sequential_preLN__linear_attn_block__moe_arch_mod__prompt_kernel(
    A_x: jax.Array,
    A_wqkv: jax.Array,
    A_wo: jax.Array,
    B_x: jax.Array,
    B_w_r: jax.Array,
    B_w_gate: jax.Array,
    B_w_up: jax.Array,
    B_w_down: jax.Array,
):
    del B_x
    x = A_x.reshape(S, D)
    wr = B_w_r.reshape(NC, LANES)
    any_spec = pl.BlockSpec(memory_space=pl.ANY)
    out = pl.pallas_call(
        _kernel,
        out_shape=jax.ShapeDtypeStruct((S, D), BF16),
        in_specs=[any_spec] * 7,
        out_specs=any_spec,
        scratch_shapes=[
            pltpu.VMEM((S + DEF, D), BF16),
            pltpu.VMEM((D // 2, D), U32),
            pltpu.VMEM((D // 2, D), U32),
            pltpu.VMEM((2, D // 2, D), U32),
            pltpu.VMEM((NC, LANES), BF16),
            pltpu.VMEM((2, D // 2, F + LANES), U32),
            pltpu.VMEM((F // 2, D + LANES), U32),
            pltpu.VMEM((P0 // 2, D), U32),
            pltpu.VMEM((XSN, S // NA // 2, DA), U32),
            pltpu.VMEM((7 ** LK, DK // 2, DK), U32),
            pltpu.VMEM((D // 2, P0), U32),
            pltpu.VMEM((7 ** LG, DG // 2, TB // NG), U32),
            pltpu.VMEM((D, LANES), F32),
            pltpu.VMEM((D, LANES), F32),
            pltpu.VMEM((RL, LANES), F32),
            pltpu.VMEM((D, D), F32),
            pltpu.VMEM((D // 2, D), U32),
            pltpu.VMEM((7 ** LA, DA // 2, DA), U32),
            pltpu.VMEM((D // 2, D), U32),
            pltpu.VMEM((7 ** LO, DO // 2, DO), U32),
            pltpu.VMEM((max(TB2, RL), D + 2 * LANES), F32),
            pltpu.VMEM((RL // 2, D), U32),
            pltpu.VMEM((7 ** LO, max(TB2, RL) // NO // 2, DO), U32),
            pltpu.VMEM((DEF, D), F32),
            pltpu.VMEM((2, S + DEF, D), BF16),
            pltpu.VMEM((TB, D), F32),
            pltpu.VMEM((8, LANES), U32),
            pltpu.SemaphoreType.DMA((NSEM,)),
        ],
        compiler_params=pltpu.CompilerParams(vmem_limit_bytes=110 * 1024 * 1024, disable_bounds_checks=True,
                                             disable_semaphore_checks=True),
    )(x, A_wqkv, A_wo, wr, B_w_gate, B_w_up, B_w_down)
    return out.reshape(1, S, D)
```

```python
import jax
import jax.numpy as jnp
from jax import lax
import jax.experimental.pallas as pl
import jax.experimental.pallas.tpu as pltpu


S = 2048
D = 1024
F = 3584
H = 32
DH = D // H
LANES = 128
NC = D // LANES
HD = D // 2

LA = 2
LG = 1
LK = 2
LO = 1
NA, NG, NK, NO = 2 ** LA, 2 ** LG, 2 ** LK, 2 ** LO
DA, DG, DK, DO = D // NA, D // NG, D // NK, D // NO
XSN = 7 ** LA if LG == LA else 9 * 7 ** LG
P0 = 512
PB = S - P0
TX = 256
TB = 512
NB1 = PB // TB
TB2 = 384
NB2 = 4
QA = 192
OCH = (128, 128, 128)
DEF = OCH[-1]
L0 = NB2 * TB2
RL = S - L0
QS = (256, 256)
OCL = ((128, False), (128, False), (128, False), (64, True), (64, True))
NPRE = 24
NGAP = 10
OUT_AT = (256, 384, 448)
LNU = 8
LAG_L = 4
LN_DELAY = 800
JOB_DELAY = 500
POST_DELAY = 800
GM = 128
PGM = 128
PGN = 128
PKM = 128
PKK = 256
EV0 = 0
EV1 = 0
EVT = 0
TRW = 256
TRM = 128
GN = 128
WK5 = 66
C6LN = (1000, 8900)
C6WK = (1500, 8900)
P1LN = (60, 12000)
P1WP = (6300, 11500)
P1WQ = (7500, 13100)
WQP = 5
EV2 = 300
P2U = (60, 2000)
P2X = (2900, 4500)
LAG = 5
QFIN = False
HFIN = True
EV3 = 0
LN2_DELAY = 900
QP_DELAY = 400
GLAG = (None, None, None, 20, 8)

F32 = jnp.float32
BF16 = jnp.bfloat16
U32 = jnp.uint32
I32 = jnp.int32

XP = ((PB, 128), (PB + 128, 128), (PB + 256, 256), (0, TB), (TB, PB - TB))
WKP = ((0, 128), (128, 128), (256, 256), (512, 512))

SEM_X = 0
SEM_WK = SEM_X + len(XP)
SEM_WQ = SEM_WK + len(WKP)
SEM_W3 = SEM_WQ + 1
SEM_WR = SEM_W3 + 1
SEM_WGU = SEM_WR + 1
SEM_WD = SEM_WGU + 1
SEM_OUT = SEM_WD + 1
NSEM = SEM_OUT + 5

INT_MIN = -(2 ** 31)


def _layernorm(x, tok=None, w=None):
    s0 = x[:, 0:LANES]
    if tok is not None:
        s0 = s0 + jnp.concatenate([tok] * (x.shape[0] // 8), axis=0)
    for c in range(1, NC):
        s0 = s0 + x[:, c * LANES:(c + 1) * LANES]
    mu = jnp.sum(s0, axis=-1, keepdims=True) * (1.0 / D)
    xc = x - mu
    var = jnp.sum(xc * xc, axis=-1, keepdims=True) * (1.0 / D)
    rstd = lax.rsqrt(var + 1e-5)
    if w is None:
        return xc * rstd
    return xc * rstd, jnp.sum(xc * w, axis=-1, keepdims=True) * rstd


def _phi(t):
    return jnp.where(t > 0, t + 1.0, jnp.exp(t)) + 1e-6


def _n_off(a, b):
    return 32 * a + 8 * b


def _n_groups():
    pos = {(2 * o + e) * LANES + _n_off(a, b): (16 * e + 4 * b + a) * DH + 8 * o
           for o in range(4) for e in range(2) for a in range(4) for b in range(4)}
    return [pos[n] for n in sorted(pos)]


def _quads(b):
    h = len(b) // 2
    return [[r[j * h:(j + 1) * h] for r in b[i * h:(i + 1) * h]] for i in range(2) for j in range(2)]


def _badd(x, y):
    return [[a + b for a, b in zip(rx, ry)] for rx, ry in zip(x, y)]


def _bsub(x, y):
    return [[a - b for a, b in zip(rx, ry)] for rx, ry in zip(x, y)]


def _a_set(b):
    if len(b) == 1:
        return [b[0][0]]
    return [x for o in _a_ops(b) for x in _a_set(o)]


def _b_set(b):
    if len(b) == 1:
        return [b[0][0]]
    q11, q12, q21, q22 = _quads(b)
    ops = (_badd(q11, q22), q11, _bsub(q12, q22), _bsub(q21, q11), q22, _badd(q11, q12), _badd(q21, q22))
    return [x for o in ops for x in _b_set(o)]


def _b_in_a(i, levels):
    perm = (0, 2, 6, 5, 3, 4, 1)
    return sum(perm[(i // 7 ** l) % 7] * 7 ** l for l in range(levels))


def _strassen(prod, levels, base=0, fin=lambda k, q: q, init=None):
    if levels == 0:
        return [[prod(base)]]

    def m(i):
        return _strassen(prod, levels - 1, base * 7 + i)

    def seed(q, x):
        return x if init is None else _badd(_quads(init)[q], x)

    m2 = m(2)
    c22 = seed(3, m2)
    m4 = m(4)
    c12 = fin(1, _badd(seed(1, m2), m4))
    c11 = m4 if init is None else _bsub(_quads(init)[0], m4)
    m3 = m(3)
    c11 = _bsub(m3, c11) if init is None else _badd(c11, m3)
    m1 = m(1)
    c21 = fin(2, _badd(seed(2, m3), m1))
    c22 = _bsub(c22, m1)
    m0 = m(0)
    c11 = _badd(c11, m0)
    c22 = _badd(c22, m0)
    c11 = fin(0, _badd(c11, m(6)))
    c22 = fin(3, _badd(c22, m(5)))
    return [a + b for a, b in zip(c11, c12)] + [a + b for a, b in zip(c21, c22)]


def _goff(i, levels):
    return int(format(i, "0%db" % levels)[::-1], 2) if levels else 0


def _blocks(rows, n):
    w = rows[0].shape[1] // n
    return [[r[:, j * w:(j + 1) * w] for j in range(n)] for r in rows]


def _or_all(vals):
    acc = None
    for v in vals:
        v = pltpu.bitcast(v, U32)
        for g in range(v.shape[0] // 8):
            for c in range(v.shape[1] // LANES):
                p = v[g * 8:(g + 1) * 8, c * LANES:(c + 1) * LANES]
                acc = p if acc is None else acc | p
    return acc


def _raw_ops(levels):
    n = 2 ** levels
    names = [[_Tag((i, j)) for j in range(n)] for i in range(n)]
    return {op: t.ij for op, t in enumerate(_b_set(names)) if t.ij is not None}


class _Tag:
    def __init__(self, ij):
        self.ij = ij

    def __add__(self, other):
        return _Tag(None)

    __sub__ = __add__


def _a_ops(b):
    q11, q12, q21, q22 = _quads(b)
    return (_badd(q11, q22), _badd(q21, q22), q11, q22, _badd(q11, q12), _bsub(q21, q11), _bsub(q12, q22))


def _x_set(o):
    return _a_set(o) + ([] if LG == LA else [o[0][1], o[1][0]])


_A_FORM = (((0, 0), (1, 1), 1), ((1, 0), (1, 1), 1), ((0, 0),), ((1, 1),), ((0, 0), (0, 1), 1),
           ((1, 0), (0, 0), -1), ((0, 1), (1, 1), -1))
_B_FORM = (((0, 0), (1, 1), 1), ((0, 0),), ((0, 1), (1, 1), -1), ((1, 0), (0, 0), -1), ((1, 1),),
           ((0, 0), (0, 1), 1), ((1, 0), (1, 1), 1))


def _outer(form, get, n):
    h = n // 2

    def quad(q):
        return [[get(q[0] * h + i, q[1] * h + j) for j in range(h)] for i in range(h)]

    if len(form) == 1:
        return quad(form[0])
    return (_badd if form[2] > 0 else _bsub)(quad(form[0]), quad(form[1]))


def _x_slot(i):
    return i if LG == LA else (i // 7) * 9 + i % 7


def _merge(b):
    return jnp.concatenate([jnp.concatenate(r, axis=1) for r in b], axis=0)


def _gate(v, tok):
    u = pltpu.bitcast(v, U32)
    top = u[0:8, 0:LANES] | tok
    if u.shape[1] > LANES:
        top = jnp.concatenate([top, u[0:8, LANES:]], axis=1)
    return pltpu.bitcast(jnp.concatenate([top, u[8:, :]], axis=0) if u.shape[0] > 8 else top, BF16)


class _Pacer:
    def __init__(self, zero, every=0):
        self.zero, self.t, self.jobs, self.pend, self.tok = zero, 0, [], [], None
        self.every, self.last = every, -every

    def add(self, jobs, t0, t1, delay):
        for k, job in enumerate(jobs):
            self.jobs.append((t0 + k * (t1 - t0) // len(jobs), len(self.jobs), job, delay))
        self.jobs.sort(key=lambda e: e[:2])

    def due(self, dep, delay):
        if dep is not None:
            self.pend.append((self.t + delay, _or_all([dep])))

    def release(self, upto):
        while self.jobs and self.jobs[0][0] <= upto:
            _, _, job, delay = self.jobs.pop(0)
            self.due(job(self.tok), delay)

    def dot(self, lhs, rhs):
        self.release(self.t)
        ready = [d for t, d in self.pend if t <= self.t]
        if ready and self.t - self.last >= self.every:
            self.pend = [e for e in self.pend if e[0] > self.t]
            self.last = self.t
            lhs = _gate(lhs, _or_all(ready) & self.zero)
        res = jnp.dot(lhs, rhs, preferred_element_type=F32)
        self.t += lhs.shape[0] * (lhs.shape[1] // LANES) * (res.shape[1] // LANES) // 4
        self.tok = pltpu.bitcast(pltpu.bitcast(res[0:8, 0:LANES], U32) & self.zero, F32)
        return res

    def flush(self):
        self.release(1 << 30)


def _kernel(x_hbm, wqkv_hbm, wo_hbm, wr_hbm, wg_hbm, wu_hbm, wd_hbm, out_hbm,
            x_v, wk_v, wq_v, w3_v, wr_v, wgu_v, wd_v,
            ln1_v, xs_v, wks_v, pkt_v, pks_v, zacc_v, uacc_v, xw_v, g_v, wqp_v, wqs_v, mp_v, ms_v, pq_v, pqn_v, pqs_v, attn_v, lo_v, lnf_v, zero_v,
            sems):

    ln2_v, out_v = lo_v.at[0], lo_v.at[1]

    wqkv_hbm, wo_hbm, wg_hbm, wu_hbm, wd_hbm = (r.bitcast(U32) for r in (wqkv_hbm, wo_hbm, wg_hbm, wu_hbm, wd_hbm))

    def wload(ref, r0, nr, cols):
        return pltpu.bitcast(ref[r0 // 2:(r0 + nr) // 2, cols], BF16)

    wv_v, wo_v = w3_v.at[0], w3_v.at[1]
    wg_v, wu_v = wgu_v.at[0], wgu_v.at[1]

    def x_copy(i):
        r0, n = XP[i]
        return pltpu.make_async_copy(x_hbm.at[pl.ds(r0, n), :], x_v.at[pl.ds(DEF + r0, n), :], sems.at[SEM_X + i])

    def out_copy(r0, n, s):
        return pltpu.make_async_copy(out_v.at[pl.ds(DEF + r0, n), :], out_hbm.at[pl.ds(r0, n), :],
                                     sems.at[SEM_OUT + s])

    def wk_copy(j):
        c0, n = WKP[j]
        return pltpu.make_async_copy(wqkv_hbm.at[:, pl.ds(D + c0, n)], wk_v.at[:, pl.ds(c0, n)],
                                     sems.at[SEM_WK + j])

    wq_copy = pltpu.make_async_copy(wqkv_hbm.at[:, pl.ds(0, D)], wq_v, sems.at[SEM_WQ])
    wr_copy = pltpu.make_async_copy(wr_hbm, wr_v, sems.at[SEM_WR])
    wd_copy = pltpu.make_async_copy(wd_hbm, wd_v.at[:, pl.ds(0, D)], sems.at[SEM_WD])
    wg_copy = pltpu.make_async_copy(wg_hbm, wg_v.at[:, pl.ds(0, F)], sems.at[SEM_WGU])
    wu_copy = pltpu.make_async_copy(wu_hbm, wu_v.at[:, pl.ds(0, F)], sems.at[SEM_WGU])

    x_copy(0).start()
    wk_copy(0).start()
    x_copy(1).start()
    wr_copy.start()
    for j in range(1, len(WKP)):
        wk_copy(j).start()
    for j in range(2, len(XP)):
        x_copy(j).start()
    wq_copy.start()
    pltpu.make_async_copy(wqkv_hbm.at[:, pl.ds(2 * D, D)], wv_v, sems.at[SEM_W3]).start()
    pltpu.make_async_copy(wo_hbm, wo_v, sems.at[SEM_W3]).start()
    wg_copy.start()
    wu_copy.start()
    wd_copy.start()

    def ln1_rows(xr, xr0, lnr, r0, n):
        ln = _layernorm(xr[xr0:xr0 + n, :].astype(F32)).astype(BF16)
        lnr[r0 // 2:(r0 + n) // 2, :] = pltpu.bitcast(ln, U32)

    def ln1_set(pc, xr, xr0, xsr, a0, n, t0, t1):
        def unit(j):
            def job(tok):
                ln = _layernorm(xr[xr0 + j * LNU:xr0 + (j + 1) * LNU, :].astype(F32), tok)
                lnf_v[j * LNU:(j + 1) * LNU, :] = ln
                return _or_all([ln[:, 0:LANES], ln[:, D - LANES:D]])
            return job

        def piece(j0, c0, o):
            def job(tok):
                def get(i, f):
                    r = (j0 + 2 * _goff(i, LA)) * LNU
                    v = lnf_v[r:r + 16, f * DA + c0:f * DA + c0 + LANES]
                    return v + jnp.concatenate([tok, tok], axis=0) if (i + f) % (NA // 2 + 1) == 0 else v

                r = (a0 + (j0 // (2 * NA)) * 16) // 2
                ops = _x_set(_outer(_A_FORM[o], get, NA))
                for op, v in enumerate(ops):
                    xsr.at[o * len(ops) + op][r:r + 8, c0:c0 + LANES] = pltpu.bitcast(v.astype(BF16), U32)
                return _or_all([v[0:8, :] for v in [ops[0]] + ops[5:7]])
            return job

        grp = 2 * NA
        ng = n // LNU // grp
        dt = (t1 - t0 - LN_DELAY) // (ng + 1)
        for g in range(ng):
            pc.add([unit(g * grp + j) for j in range(grp)], t0 + g * dt, t0 + (g + 1) * dt, LN_DELAY)
            s = t0 + (g + 1) * dt + LN_DELAY
            pc.add([piece(g * grp, c0, o) for c0 in range(0, DA, LANES) for o in range(7)], s, s + dt, JOB_DELAY)

    def ln1_load(lnr, r0, n):
        return pltpu.bitcast(lnr[r0 // 2:(r0 + n) // 2, :], BF16)

    def gate(v, tok):
        return v if tok is None else _gate(v, tok)

    def k_mm(r0, n, c0, nc):
        return jnp.dot(ln1_load(ln1_v, r0, n), wload(wk_v, 0, D, slice(c0, c0 + nc)), preferred_element_type=F32)

    def z_acc(pkts, c0, first=False):
        zs = None
        for pkt in pkts:
            for j in range(pkt.shape[1] // LANES):
                p = pkt[:, j * LANES:(j + 1) * LANES]
                zs = p if zs is None else zs + p
        if first:
            zacc_v[c0:c0 + zs.shape[0], :] = zs
        else:
            zacc_v[c0:c0 + zs.shape[0], :] += zs

    def k_post(k, p0, c0, first=False):
        n, nc = k.shape
        pkt = _phi(k).T
        pkt_v[c0 // 2:(c0 + nc) // 2, p0:p0 + n] = pltpu.bitcast(pkt.astype(BF16), U32)
        z_acc([pkt], c0, first)
        return pkt[nc - 8:nc, n - LANES:n]

    def g_acc(r0, n, c0, nc, first=False, pc=None):
        h, w = (nc, D) if pc is None else (min(nc, PGM), PGN)
        for f0 in range(c0, c0 + nc, h):
            for j0 in range(0, D, w):
                lhs = pltpu.bitcast(pkt_v[f0 // 2:(f0 + h) // 2, r0:r0 + n], BF16)
                rhs = pltpu.bitcast(ln1_v[r0 // 2:(r0 + n) // 2, j0:j0 + w], BF16)
                g = jnp.dot(lhs, rhs, preferred_element_type=F32) if pc is None else pc.dot(lhs, rhs)
                if first:
                    g_v[f0:f0 + h, j0:j0 + w] = g
                else:
                    g_v[f0:f0 + h, j0:j0 + w] += g

    def k_paced(pc, r0, c0, nc, first):
        for j0 in range(c0, c0 + nc, LANES):
            for t0 in range(r0, r0 + TX, PKM):
                k = None
                for k0 in range(0, D, PKK):
                    p = pc.dot(ln1_load(ln1_v, t0, PKM)[:, k0:k0 + PKK], wload(wk_v, k0, PKK, slice(j0, j0 + LANES)))
                    k = p if k is None else k + p
                pc.due(k_post(k, t0, j0, first and t0 == r0), POST_DELAY)

    attn_v[...] = jnp.zeros_like(attn_v)
    zero_v[...] = jnp.zeros_like(zero_v)

    x_copy(0).wait()
    ln1_rows(x_v, DEF + PB, ln1_v, 0, 128)
    wk_copy(0).wait()
    ka = k_mm(0, 128, 0, 128)
    x_copy(1).wait()
    wr_copy.wait()
    ln1_rows(x_v, DEF + PB + 128, ln1_v, 128, 128)
    k_post(ka, 0, 0, first=True)
    g_acc(0, 128, 0, 128, first=True)
    wk_copy(1).wait()
    k_post(k_mm(128, 128, 0, 128), 128, 0)
    k_post(k_mm(0, TX, 128, 128), 0, 128, first=True)
    g_acc(128, 128, 0, 128)
    def w_job(src_ref, dst_ref, levels, r0, c0, o):
        n = 2 ** levels
        w, raw, inner = D // n, _raw_ops(levels), 7 ** (levels - 1)

        def job(tok):
            def cut(i, j):
                return src_ref[(i * w + r0) // 2:(i * w + r0) // 2 + 8, j * w + c0:j * w + c0 + LANES]

            def get(i, j):
                u = cut(i, j)
                return pltpu.bitcast(u if tok is None else u | pltpu.bitcast(tok, U32), BF16).astype(F32)

            ops = []
            for op, v in enumerate(_b_set(_outer(_B_FORM[o], get, n))):
                dst = dst_ref.at[o * inner + op]
                if o * inner + op in raw:
                    dst[r0 // 2:r0 // 2 + 8, c0:c0 + LANES] = cut(*raw[o * inner + op])
                else:
                    dst[r0 // 2:r0 // 2 + 8, c0:c0 + LANES] = pltpu.bitcast(v.astype(BF16), U32)
                    ops.append(v)
            return _or_all(ops[0:1] + ops[-2:]) if ops else None
        return job

    def wk_jobs_of(outer):
        return [w_job(wk_v, wks_v, LK, r0, c0, o) for r0 in range(0, DK, 16) for c0 in range(0, DK, LANES)
                for o in outer]

    wk_copy(2).wait()
    pc = _Pacer(zero_v[...], EV0)
    pc.add(wk_jobs_of((1, 3)), 500, 2200, JOB_DELAY)
    k_paced(pc, 0, 256, 256, True)
    g_acc(0, TX, 128, 128, True, pc)
    g_acc(0, TX, 256, 256, True, pc)
    pc.flush()
    wk_copy(3).wait()
    wk_jobs = wk_jobs_of((0, 2, 4, 5, 6))
    pc = _Pacer(zero_v[...], EV0)
    pc.add(wk_jobs[:WK5], 500, 2700, JOB_DELAY)
    k_paced(pc, 0, 512, 512, True)
    g_acc(0, TX, 512, 256, True, pc)
    pc.flush()
    x_copy(2).wait()
    x_copy(3).wait()
    pc = _Pacer(zero_v[...], EV0)
    ln1_set(pc, x_v, DEF, xs_v, 0, TB, *C6LN)
    pc.add(wk_jobs[WK5:], *C6WK, JOB_DELAY)
    ln1_rows(x_v, DEF + PB + TX, ln1_v, TX, TX)
    g_acc(0, TX, 768, 256, True, pc)
    k_paced(pc, TX, 0, D, False)
    for c0 in range(0, D, 256):
        g_acc(TX, TX, c0, 256, False, pc)
    pc.flush()

    MA = TB // NA
    NS = NK // NG

    def xs_load(xsr, op, a0, m, cols=slice(None)):
        return pltpu.bitcast(xsr[op, a0 // 2:(a0 + m) // 2, cols], BF16)

    def k_step(pc, xsr, j0):
        def fin(_, q):
            if NS > 1:
                q = [[jnp.concatenate([_phi(jnp.concatenate([r[f] for r in q], axis=0)).T for f in range(NS)],
                                      axis=0)]]
            else:
                q = [[_phi(v).T for v in r] for r in q]
            pc.due(_or_all([v[t - 8:t, :] for r in q for v in r for t in range(LANES, v.shape[0] + 1, LANES)]),
                   POST_DELAY)
            return q

        def lhs(i):
            if LK == LA:
                return xs_load(xsr, _x_slot(i), 0, MA)
            return _merge([[xs_load(xsr, i * 9 + s, 0, MA) for s in r] for r in ((2, 7), (8, 3))])

        cb = _strassen(lambda i: pc.dot(lhs(i), pltpu.bitcast(wks_v[i, :, j0:j0 + LANES], BF16)), LK, fin=fin)
        ops = _a_ops([[cb[i][f] for i in range(NG)] for f in range(NG)])
        for half, o in ((0, ops[4]), (1, ops[1])):
            for f, rowb in enumerate(o):
                for s in range(NS):
                    z_acc([v[s * LANES:(s + 1) * LANES, :] for v in rowb], half * HD + f * DG + s * DK + j0)
        for _ in range(LG - 1):
            ops = [o for x in ops for o in _a_ops(x)]
        for op, o in enumerate(ops):
            r = j0 * NS
            pks_v.at[op][r // 2:(r + NS * LANES) // 2, :] = pltpu.bitcast(o[0][0].astype(BF16), U32)
        pc.due(_or_all([o[0][0][NS * LANES - 8:NS * LANES, :] for o in (ops[0], ops[-1], ops[-2])]), 2 * POST_DELAY)

    def g_rhs(xsr, i, c0, nc):
        o = _b_in_a(i, LG)
        if LG == LA:
            return xs_load(xsr, o, 0, MA, slice(c0, c0 + nc))
        j, cs = c0 // DA, slice(c0 % DA, c0 % DA + nc)
        return jnp.concatenate([xs_load(xsr, o * 9 + s, 0, MA, cs) for s in ((2, 8), (7, 3))[j]], axis=0)

    def g_step(pc, xsr, r0, nr, c0, nc):
        cb = _strassen(lambda i: pc.dot(pltpu.bitcast(pks_v[i, r0 // 2:(r0 + nr) // 2, :], BF16),
                                        g_rhs(xsr, i, c0, nc)), LG)
        for f in range(NG):
            for c in range(NG):
                h = min(nr, LANES)
                for t in range(nr // h):
                    step, sub = divmod((r0 + t * h) // LANES, NS)
                    g0_ = f * DG + sub * DK + step * LANES + (r0 + t * h) % LANES
                    g_v[g0_:g0_ + h, c * DG + c0:c * DG + c0 + nc] += cb[f][c][t * h:(t + 1) * h, :]

    def wq_jobs(u0, nr):
        span = (NA - 1) * DA + 16 * nr
        u0 = u0 if isinstance(u0, int) else pl.multiple_of(u0, 8)
        srcr, permr = wq_v.at[pl.ds(u0, span // 2), :], wqp_v.at[pl.ds(u0, span // 2), :]
        dstr = wqs_v.at[:, pl.ds(u0, 8 * nr), :]
        oct_ = (lax.broadcasted_iota(I32, (8, LANES), 1) % DH) // 8

        def perm(r, e):
            def job(tok):
                blk = [srcr[r // 2:r // 2 + 8, (4 * e + b) * LANES:(4 * e + b + 1) * LANES] | pltpu.bitcast(tok, U32)
                       for b in range(4)]
                outs = []
                for o in range(4):
                    v = blk[o]
                    for b in range(4):
                        if b != o:
                            v = jnp.where(oct_ == b, pltpu.roll(blk[b], (8 * (b - o)) % LANES, 1), v)
                    permr[r // 2:r // 2 + 8, (2 * o + e) * LANES:(2 * o + e + 1) * LANES] = v
                    outs.append(v)
                return _or_all(outs)
            return job

        return ([perm(i * DA + r0, e) for r0 in range(0, 16 * nr, 16) for i in range(NA) for e in range(2)],
                [w_job(permr, dstr, LA, r0, c0, o) for r0 in range(0, 16 * nr, 16)
                 for c0 in range(0, DA, LANES) for o in range(7)])

    def p1(i, carry):
        xsr = xs_v.at[:, pl.ds(pl.multiple_of(i * (MA // 2), MA // 2), MA), :]
        xr = x_v.at[pl.ds(pl.multiple_of((i + 1) * TB, TB), TB + DEF), :]

        pc = _Pacer(zero_v[...], EV1)
        ln1_set(pc, xr, DEF, xsr, MA, TB, *P1LN)
        perms, sets = wq_jobs(i * (8 * WQP), WQP)
        pc.add(perms, *P1WP, JOB_DELAY)
        pc.add(sets, *P1WQ, JOB_DELAY)
        for j0 in range(0, DK, LANES):
            k_step(pc, xsr, j0)
        for f0 in range(0, DG, GM):
            for c0 in range(0, DG, GN):
                g_step(pc, xsr, f0, GM, c0, GN)
        pc.flush()
        return carry

    x_copy(4).wait()
    wq_copy.wait()
    lax.fori_loop(0, NB1, p1, 0)

    pltpu.make_async_copy(w3_v, w3_v, sems.at[SEM_W3]).wait()
    zero_u = zero_v[...]
    def row_vector(acc_ref):
        return jnp.sum(jnp.concatenate([acc_ref[r:r + 8, :] for r in _n_groups()], axis=0).T, axis=0, keepdims=True)

    zrow = row_vector(zacc_v)
    wr8 = wr_v[...].astype(F32)
    wr_row = jnp.concatenate([wr8[c:c + 1, :] for c in range(NC)], axis=1)

    row_h = lax.broadcasted_iota(I32, (LANES, LANES), 0) // DH
    col_h = lax.broadcasted_iota(I32, (LANES, LANES), 1) // DH
    diag = row_h == col_h

    def colsum(t):
        acc = t[:, 0:LANES]
        for c in range(1, NC):
            acc = acc + t[:, c * LANES:(c + 1) * LANES]
        return acc

    wrc = wr_row - jnp.sum(wr_row, axis=-1, keepdims=True) * (1.0 / D)
    m_raw = _raw_ops(LO)

    def kv_part(c):
        cs = slice(c * LANES, (c + 1) * LANES)
        kv = None
        for k0 in range(0, D, TRW):
            p = pc.dot(g_v[cs, k0:k0 + TRW].astype(BF16), wload(wv_v, k0, TRW, cs))
            kv = p if kv is None else kv + p
        return jnp.where(diag, kv, 0.0)

    def m_part(c, kvs):
        e, b = c // 4, c % 4
        for j0 in range(0, DO, TRM):
            ms = [jnp.concatenate(
                [pc.dot(kv, wload(wo_v, (c + k) * LANES, LANES, slice(f * DO + j0, f * DO + j0 + TRM)))
                 for f in range(NO)], axis=1) for k, kv in enumerate(kvs)]
            deps = []
            for a in range(4):
                rows = [jnp.concatenate([m[a * DH + 8 * o:a * DH + 8 * o + 8, :] for m in ms], axis=0)
                        for o in range(4)]
                for o in range(4):
                    r = ((2 * o + e) * LANES + _n_off(a, b)) // 2
                    for f in range(NO):
                        mp_v[r:r + 8, f * DO + j0:f * DO + j0 + TRM] = pltpu.bitcast(
                            rows[o][:, f * TRM:(f + 1) * TRM].astype(BF16), U32)
                for t in range(4 // NO):
                    r = ((2 * t + e) * LANES + _n_off(a, b)) // 2
                    for op, v in enumerate(_b_set(_blocks(rows[t::4 // NO], NO))):
                        if op not in m_raw:
                            ms_v.at[op][r:r + 8, j0:j0 + TRM] = pltpu.bitcast(v.astype(BF16), U32)
                            deps.append(v[0:8, 0:LANES])
            pc.due(_or_all(deps[::4]), POST_DELAY)

    pc = _Pacer(zero_u, EVT)
    pc.due(jnp.broadcast_to(zrow, (8, D)), 1000)
    perms, sets = wq_jobs(NB1 * 8 * WQP, DA // 16 - NB1 * WQP)
    pc.add(perms, 60, 700, JOB_DELAY)
    pc.add(sets, 1300, 3400, JOB_DELAY)
    kv_prev = None
    for c in range(0, NC + 2, 2):
        kvs = [kv_part(c).astype(BF16), kv_part(c + 1).astype(BF16)] if c < NC else None
        if c:
            m_part(c - 2, kv_prev)
        kv_prev = kvs
    pc.flush()

    def make_key(score, row):
        b = pltpu.bitcast(score, I32)
        srt = b ^ ((b >> 31) & 0x7FFFFFFF)
        return (srt & jnp.int32(-65536)) | (0xFFFF - row)

    def push_keys(key, top1, top2):
        for gidx in range(key.shape[0] // 8):
            kx = key[gidx * 8:(gidx + 1) * 8, :]
            top2 = jnp.maximum(top2, jnp.minimum(top1, kx))
            top1 = jnp.maximum(top1, kx)
        return top1, top2

    lane = lax.broadcasted_iota(I32, (1, LANES), 1)

    def interleave(parts):
        return jnp.concatenate([p[g * 16:(g + 1) * 16, :] for g in range(parts[0].shape[0] // 16) for p in parts],
                               axis=0)

    def q_part(pc, xsr, l0, r0, n, hint=None):
        m = n // NA
        sums = {}

        def park(v, g, c):
            for t in range(m // 16):
                r = r0 + (t * NA + g) * 16
                pq_v[r:r + 16, c * LANES:(c + 1) * LANES] = v[t * 16:(t + 1) * 16, :]

        def fin(k, q):
            q = [[_phi(v) for v in r] for r in q]
            deps = []
            for a, r in enumerate(q):
                for b, v in enumerate(r):
                    i, c = (k // 2) * (NA // 2) + a, (((k % 2) * (NA // 2) + b) * DA + j0) // LANES
                    park(v, _goff(i, LA), c)
                    for name, row in (("z", zrow),) + ((("u", hint["u"]),) if hint else ()):
                        t = v * row[:, c * LANES:(c + 1) * LANES]
                        key = (name, _goff(i, LA), c % 2)
                        sums[key] = t if key not in sums else sums[key] + t
                deps.append(sums[key])
            if (r0 + n < RL or HFIN) if hint else QFIN:
                pc.due(_or_all(deps), POST_DELAY)
            return q

        for j0 in range(0, DA, LANES):
            _strassen(lambda i: pc.dot(xs_load(xsr, _x_slot(i), (l0 + r0) // NA, m),
                                       pltpu.bitcast(wqs_v[i, :, j0:j0 + LANES], BF16)), LA, fin=fin)
        if hint:
            pc.flush()
        den = jnp.concatenate([sums["z", g, e] for g in range(NA) for e in range(2)], axis=0)
        for s in (1, 2, 4):
            den = den + jnp.where((lane & s) == 0, pltpu.roll(den, LANES - s, 1), pltpu.roll(den, s, 1))
        inv_all = 1.0 / (den + 1e-6)

        def inv_of(g):
            return [inv_all[(g * 2 + e) * m:(g * 2 + e + 1) * m, :] for e in range(2)]

        for g in range(NA):
            for e in range(2):
                park(inv_of(g)[e], g, NC + e)
        if hint:
            for g in range(NA):
                starts = [r0 + (t * NA + g) * 16 for t in range(m // 16)]
                num = jnp.sum(jnp.concatenate([xw_v[t:t + 16, :] for t in starts], axis=0)
                              + sums["u", g, 0] * inv_of(g)[0] + sums["u", g, 1] * inv_of(g)[1],
                              axis=-1, keepdims=True)
                row = jnp.concatenate([(l0 + t) + lax.broadcasted_iota(I32, (16, 1), 0) for t in starts], axis=0)
                hint["p1"], hint["p2"] = push_keys(make_key(num, row), hint["p1"], hint["p2"])
            pc.due(jnp.broadcast_to(hint["p1"], (8, LANES)), 1200)


    def post_jobs(r0, n, plain=False):
        def scaled(t, c0, w, tok):
            inv = pq_v[t:t + 16, D:D + 2 * LANES]
            if tok is not None:
                inv = inv + jnp.concatenate([jnp.concatenate([tok, tok], axis=0)] * 2, axis=1)
            return pq_v[t:t + 16, c0:c0 + w] * jnp.concatenate([inv] * (w // (2 * LANES)), axis=1)

        def post_plain(t):
            def job(tok):
                v = scaled(t, 0, D, tok)
                pqn_v[t // 2:t // 2 + 8, :] = pltpu.bitcast(v.astype(BF16), U32)
                return v[0:8, 0:LANES]
            return job

        def post(t0, outer):
            def job(tok):
                deps = []
                for c0 in range(0, DO, 2 * LANES):
                    blk = {}

                    def get(i, f):
                        if (i, f) not in blk:
                            blk[i, f] = scaled(t0 + _goff(i, LO) * 16, f * DO + c0, 2 * LANES, tok)
                        return blk[i, f]

                    for o in outer:
                        ops = _a_set(_outer(_A_FORM[o], get, NO))
                        for op, v in enumerate(ops):
                            pqs_v.at[o * len(ops) + op][t0 // NO // 2:t0 // NO // 2 + 8, c0:c0 + 2 * LANES] = (
                                pltpu.bitcast(v.astype(BF16), U32))
                        deps.append(ops[0][0:8, 0:LANES])
                return _or_all(deps)
            return job

        if plain:
            return [post_plain(t) for t in range(r0, r0 + n, 16)]
        outers = [range(7)] if LO == 1 else [(o,) for o in range(7)]
        return [post(t0, outer) for t0 in range(r0, r0 + n, 16 * NO) for outer in outers]

    def m_operand(i, c0, c1):
        if i not in m_raw:
            return pltpu.bitcast(ms_v[i, :, c0 * LANES:c1 * LANES], BF16)
        bi, bj = m_raw[i]
        return wload(mp_v, bi * DO, DO, slice(bj * DO + c0 * LANES, bj * DO + c1 * LANES))

    def o_part(dot, xr, x0, r0, n):
        a0, m = r0 // NO, n // NO
        nw = LANES * NO // 2
        cols = [[[] for _ in range(NO)] for _ in range(NO)]
        for c0 in range(0, DO, nw):
            init = [[jnp.concatenate(
                [xr[x0 + r0 + (g * NO + _goff(i, LO)) * 16:x0 + r0 + (g * NO + _goff(i, LO) + 1) * 16,
                    f * DO + c0:f * DO + c0 + nw] for g in range(m // 16)], axis=0).astype(F32)
                for f in range(NO)] for i in range(NO)]
            cb = _strassen(lambda i: dot(pltpu.bitcast(pqs_v[i, a0 // 2:(a0 + m) // 2, :], BF16),
                                         m_operand(i, c0 // LANES, (c0 + nw) // LANES)), LO, init=init)
            for i in range(NO):
                for f in range(NO):
                    cols[i][f].append(cb[i][f])
        parts = [None] * NO
        for i in range(NO):
            parts[_goff(i, LO)] = jnp.concatenate([c for f in range(NO) for c in cols[i][f]], axis=1)
        return interleave(parts)

    def ln2_unit(h, l2r, outr, r0, row0, valid, top1, top2, tok, fast=False):
        n = h.shape[0]
        if fast:
            ln2, r = _layernorm(h, tok, wr_row)
        else:
            ln2 = _layernorm(h, tok)
            r = jnp.sum(ln2 * wr_row, axis=-1, keepdims=True)
        l2r[r0:r0 + n, :] = ln2.astype(BF16)
        res = h + ln2
        outr[r0:r0 + n, :] = res.astype(BF16)
        r = r.astype(BF16).astype(F32) + 0.0
        key = make_key(r, (row0 + r0) + lax.broadcasted_iota(I32, (n, 1), 0))
        if valid is not None:
            key = jnp.where(valid, key, INT_MIN)
        top1, top2 = push_keys(key, top1, top2)
        ntok = pltpu.bitcast(pltpu.bitcast(jnp.broadcast_to(r[n - 8:n, :], (8, LANES)), U32) & zero_u, F32)
        return top1, top2, ntok

    def ln2_jobs(h, l2r, outr, r0, row0, valid, st, fast=False):
        def unit(j):
            def job(tok):
                st["top1"], st["top2"], dep = ln2_unit(h[j * LNU:(j + 1) * LNU, :], l2r, outr, r0 + j * LNU, row0,
                                                       valid, st["top1"], st["top2"], tok, fast)
                return dep
            return job
        return [unit(j) for j in range(h.shape[0] // LNU)]

    QC = 16 * 7 ** LA / 8 ** LA
    OC = 16 * 7 ** LO / 8 ** LO

    def p2(i, carry):
        st = dict(top1=carry[0], top2=carry[1])
        b0 = pl.multiple_of(i * TB2, 16)
        xsr = xs_v.at[:, pl.ds(pl.multiple_of(i * (TB2 // NA // 2), 8), TB2 // NA // 2), :]
        xr = x_v.at[pl.ds(b0, TB2 + DEF), :]
        l2r = ln2_v.at[pl.ds(b0, TB2 + DEF), :]
        outr = out_v.at[pl.ds(b0, TB2 + DEF), :]
        row0 = b0 - DEF
        pc = _Pacer(zero_u)
        toks = []

        def chain(jobs):
            for job in jobs:
                toks.append(job(toks[-LAG] if len(toks) >= LAG else None))

        chain(ln2_jobs(attn_v, l2r, outr, 0, row0, i > 0, st))

        @pl.when(i > 0)
        def _():
            out_copy(pl.multiple_of((i - 1) * TB2, 16), TB2, 0).start()

        pc.due(toks[-1], QA * QC)

        def u_job(r):
            def job(tok):
                t = colsum(gate(wload(mp_v, r, 32, slice(None)), pltpu.bitcast(tok, U32)).astype(F32) * wrc)
                uacc_v[r:r + 32, :] = t
                return t
            return job

        def xw_job(t):
            def job(tok):
                v = colsum(x_v[DEF + L0 + t:DEF + L0 + t + 16, :].astype(F32) * wrc)
                v = v + jnp.concatenate([tok, tok], axis=0)
                xw_v[t:t + 16, :] = v
                return v
            return job

        pc.add([u_job(r) for r in range(0, D, 32)], *P2U, JOB_DELAY)
        pc.add([xw_job(t) for t in range(0, RL, 16)], *P2X, JOB_DELAY)
        for r0, n in ((0, QA), (QA, TB2 - QA)):
            q_part(pc, xsr, 0, r0, n)
            for job in post_jobs(r0, n):
                job(None)
        r0 = 0
        for n in OCH[:-1]:
            chain(ln2_jobs(o_part(pc.dot, xr, DEF, r0, n), l2r, outr, DEF + r0, row0, None, st))
            r0 += n
        attn_v[...] = o_part(pc.dot, xr, DEF, r0, DEF)
        return st["top1"], st["top2"]

    init = jnp.full((8, 1), INT_MIN, I32)
    top1, top2 = lax.fori_loop(0, NB2, p2, (init, init))

    wg_copy.wait()
    wu_copy.wait()
    wd_copy.wait()
    sub8 = lax.broadcasted_iota(I32, (8, LANES), 0)
    urow = jnp.sum(uacc_v[...].T, axis=0, keepdims=True)

    def submax(v):
        for sh in (4, 2, 1):
            v = jnp.maximum(v, pltpu.roll(v, sh, 0))
        return v

    def subsum(v):
        for sh in (4, 2, 1):
            v = v + pltpu.roll(v, sh, 0)
        return v

    def best2(t1, t2):
        t1 = jnp.broadcast_to(t1, (8, LANES))
        t2 = jnp.broadcast_to(t2, (8, LANES))
        k1v = submax(t1)
        return k1v, submax(jnp.where(t1 == k1v, t2, t1))

    def key_row(k):
        return 0xFFFF - (k & 0xFFFF)

    def wide(m):
        return jnp.concatenate([m] * NC, axis=1)

    st = dict(top1=top1, top2=top2, pend=[], step=0, sent=0)
    pc = _Pacer(zero_u, EV2)
    hint = dict(u=urow, p1=init, p2=init)

    pc.add(ln2_jobs(attn_v, ln2_v, out_v, L0, -DEF, None, st), 60, QS[0] * QC - 600, LN2_DELAY)
    r0 = 0
    for k, n in enumerate(QS):
        q_part(pc, xs_v, L0, r0, n, hint)
        if k == 0:
            out_copy(L0 - TB2, TB2, 0).start()
            top1, top2 = st["top1"], st["top2"]
            pc.add(post_jobs(0, OCL[0][0], OCL[0][1]), pc.t + 600, pc.t + (RL - n) * QC - 300, QP_DELAY)
        r0 += n
    pc.every = EV3
    oldk = best2(top1, top2)
    oldx = []
    for kk in oldk:
        g8 = pl.multiple_of(((jnp.clip(key_row(kk[0, 0]), 0, S - 1) >> 3) << 3) + DEF, 8)
        rows = ln2_v[pl.ds(g8, 8), :].astype(F32)
        oldx.append(subsum(jnp.where(wide((key_row(kk) & 7) == sub8), rows, 0.0)))

    def gated(v):
        tok = None
        while st["pend"] and st["pend"][0][0] <= st["step"]:
            t = st["pend"].pop(0)[1]
            tok = t if tok is None else tok | t
        if tok is None:
            return v
        u = pltpu.bitcast(v, U32)
        return pltpu.bitcast(jnp.concatenate([u[:, 0:LANES] | tok, u[:, LANES:]], axis=1), BF16)

    res = {}

    def c_units():
        pc.flush()
        p1, p2_ = hint["p1"], hint["p2"]
        cand_p, cand_x = [], []
        for pk_ in (p1, p2_):
            cp, cx = None, None
            for s in range(8):
                g8 = pl.multiple_of((jnp.clip(key_row(pk_[s, 0]) - L0, 0, RL - 1) >> 3) << 3, 8)
                vp = pq_v[pl.ds(g8, 8), :]
                vx = x_v[pl.ds(pl.multiple_of(g8 + (L0 + DEF), 8), 8), :].astype(F32)
                cp = vp if cp is None else jnp.where(jnp.concatenate([sub8 == s] * (NC + 2), axis=1), vp, cp)
                cx = vx if cx is None else jnp.where(wide(sub8 == s), vx, cx)
            cand_p.append(cp[:, 0:D] * jnp.concatenate([cp[:, D:]] * (NC // 2), axis=1))
            cand_x.append(cx)
        cand_p = jnp.concatenate(cand_p, axis=0).astype(BF16)
        cand_x = jnp.concatenate(cand_x, axis=0)
        ids_lo = key_row(jnp.broadcast_to(p1, (8, LANES)))
        ids_hi = jnp.where(sub8 < 6, key_row(jnp.broadcast_to(p2_, (8, LANES))),
                           jnp.where(sub8 == 6, key_row(oldk[0]), key_row(oldk[1])))
        res["ids"] = (ids_lo, ids_hi)
        parts = []
        for c in range(NC):
            parts.append(jnp.dot(cand_p, wload(mp_v, 0, D, slice(c * LANES, (c + 1) * LANES)), preferred_element_type=F32))
            yield
        xs = _layernorm(cand_x + jnp.concatenate(parts, axis=1))
        hi = jnp.where(wide(sub8 < 6), xs[8:16, :], jnp.where(wide(sub8 == 6), oldx[0], oldx[1]))
        res["xs"] = jnp.concatenate([xs[0:8, :], hi], axis=0).astype(BF16)

    def f_units():
        xs = res["xs"]
        acts = []
        for j in range(F // LANES):
            cs = slice(j * LANES, (j + 1) * LANES)
            g = jnp.dot(gated(xs), wload(wg_v, 0, D, cs), preferred_element_type=F32)
            yield
            u = jnp.dot(xs, wload(wu_v, 0, D, cs), preferred_element_type=F32)
            acts.append((g * jax.nn.sigmoid(g) * u).astype(BF16))
            yield
        act = jnp.concatenate(acts, axis=1)
        zf = pltpu.bitcast(zero_u, F32)
        ys = []
        KF = (F // D) * D
        for c in range(0, NC, 2):
            acc = jnp.concatenate([jnp.concatenate([zf, zf], axis=0)] * 2, axis=1)
            acc = acc + jnp.dot(gated(act[:, KF:]), wload(wd_v, KF, F - KF, slice(c * LANES, (c + 2) * LANES)),
                                preferred_element_type=F32)
            yield
            for cc in range(2):
                y = acc[:, cc * LANES:(cc + 1) * LANES]
                for k0 in range(0, KF, D):
                    y = y + jnp.dot(gated(act[:, k0:k0 + D]),
                                    wload(wd_v, k0, D, slice((c + cc) * LANES, (c + cc + 1) * LANES)),
                                    preferred_element_type=F32)
                    yield
                ys.append(y)
        res["y"] = jnp.concatenate(ys, axis=1)

    def side_units():
        yield from range(NPRE)
        yield from c_units()
        yield from range(NGAP)
        yield from f_units()

    side = side_units()

    def o_dot(lhs, rhs):
        p = pc.dot(lhs, rhs) if st["step"] < NPRE else jnp.dot(lhs, rhs, preferred_element_type=F32)
        next(side, None)
        st["step"] += 1
        return p

    def o_plain(r0, n):
        lhs = pltpu.bitcast(pqn_v[r0 // 2:(r0 + n) // 2, :], BF16)
        parts = []
        for c0 in range(0, NC, 2):
            acc = x_v[DEF + L0 + r0:DEF + L0 + r0 + n, c0 * LANES:(c0 + 2) * LANES].astype(F32)
            for k0 in range(0, D, 2 * LANES):
                acc = acc + o_dot(lhs[:, k0:k0 + 2 * LANES], wload(mp_v, k0, 2 * LANES, slice(c0 * LANES, (c0 + 2) * LANES)))
            parts.append(acc)
        return jnp.concatenate(parts, axis=1)

    toks = []
    r0 = 0
    pc.add(post_jobs(OCL[0][0], *OCL[1]), pc.t + 200, pc.t + 1000, QP_DELAY)
    for ci, (n, plain) in enumerate(OCL):
        h = o_plain(r0, n) if plain else o_part(o_dot, x_v, DEF + L0, r0, n)
        last = r0 + n == RL
        units = ln2_jobs(h, ln2_v, out_v, DEF + L0 + r0, -DEF, None, st, fast=last)
        posts = post_jobs(r0 + n + OCL[ci + 1][0], *OCL[ci + 2]) if ci + 2 < len(OCL) else []
        for k, job in enumerate(units):
            toks.append(job(toks[-LAG_L] if len(toks) >= LAG_L and not last else None))
            if posts:
                posts.pop(0)(toks[-1])
        if GLAG[ci] is not None:
            st["pend"].append((st["step"] + GLAG[ci],
                               pltpu.bitcast(jnp.broadcast_to(st["top1"], (8, LANES)), U32) & zero_u))
        r0 += n
        if last or r0 in OUT_AT:
            out_copy(L0 + st["sent"], r0 - st["sent"], 2 if last else 1).start()
            if not last:
                st["sent"] = r0
    for _ in side:
        st["step"] += 1

    keyv = best2(st["top1"], st["top2"])
    idx = [jnp.clip(key_row(kk[0, 0]), 0, S - 1) for kk in keyv]
    grp = [pl.multiple_of((ii >> 3) << 3, 8) for ii in idx]
    vgrp = [pl.multiple_of(gg + DEF, 8) for gg in grp]
    y = res["y"]
    ids_lo, ids_hi = res["ids"]
    hits = None
    yrows = []
    for c in range(2):
        m_lo = ids_lo == key_row(keyv[c])
        m_hi = ids_hi == key_row(keyv[c])
        yrows.append(subsum(jnp.where(wide(m_lo), y[0:8, :], 0.0) + jnp.where(wide(m_hi), y[8:16, :], 0.0)))
        hit = submax(jnp.where(m_lo | m_hi, 1, 0))
        hits = hit if hits is None else hits + hit
    hit_all = hits[0, 0] == 2

    tail0 = L0 + st["sent"]
    tail_copy = out_copy(tail0, S - tail0, 2)
    in_tail = jnp.maximum(grp[0], grp[1]) >= tail0
    two_groups = grp[1] != grp[0]

    def fix_copy(c):
        return out_copy(grp[c], 8, 3 + c)

    def finish(ysel):
        for c in range(2):
            hi = keyv[c] & jnp.int32(-65536)
            score = pltpu.bitcast(hi ^ ((hi >> 31) & 0x7FFF0000), F32)
            sel = (key_row(keyv[c]) & 7) == sub8
            upd = jnp.where(wide(sel), ysel[c] * wide(jax.nn.sigmoid(score)), 0.0)
            out_v[pl.ds(vgrp[c], 8), :] = (out_v[pl.ds(vgrp[c], 8), :].astype(F32) + upd).astype(BF16)
        fix_copy(0).start()

        @pl.when(two_groups)
        def _():
            fix_copy(1).start()

    out_copy(0, L0, 0).wait()
    out_copy(L0, tail0 - L0, 1).wait()

    @pl.when(in_tail)
    def _():
        tail_copy.wait()

    @pl.when(hit_all)
    def _():
        finish(yrows)

    @pl.when(jnp.logical_not(hit_all))
    def _():
        xsel = jnp.concatenate([ln2_v[pl.ds(vgrp[c], 8), :] for c in range(2)], axis=0)

        def ffn_tile(j, acc):
            cs = pl.ds(pl.multiple_of(j * LANES, LANES), LANES)
            g = jnp.dot(xsel, wload(wg_v, 0, D, cs), preferred_element_type=F32)
            u = jnp.dot(xsel, wload(wu_v, 0, D, cs), preferred_element_type=F32)
            a = (g * jax.nn.sigmoid(g) * u).astype(BF16)
            wd_t = pltpu.bitcast(wd_v[pl.ds(pl.multiple_of(j * (LANES // 2), LANES // 2), LANES // 2), 0:D], BF16)
            return acc + jnp.dot(a, wd_t, preferred_element_type=F32)

        yf = lax.fori_loop(0, F // LANES, ffn_tile, jnp.zeros((16, D), F32))
        finish([yf[0:8, :], yf[8:16, :]])

    @pl.when(jnp.logical_not(in_tail))
    def _():
        tail_copy.wait()

    fix_copy(0).wait()

    @pl.when(two_groups)
    def _():
        fix_copy(1).wait()


@jax.jit
def pallas_sequential_preLN__linear_attn_block__moe_arch_mod__prompt_kernel(
    A_x: jax.Array,
    A_wqkv: jax.Array,
    A_wo: jax.Array,
    B_x: jax.Array,
    B_w_r: jax.Array,
    B_w_gate: jax.Array,
    B_w_up: jax.Array,
    B_w_down: jax.Array,
):
    del B_x
    x = A_x.reshape(S, D)
    wr = B_w_r.reshape(NC, LANES)
    any_spec = pl.BlockSpec(memory_space=pl.ANY)
    out = pl.pallas_call(
        _kernel,
        out_shape=jax.ShapeDtypeStruct((S, D), BF16),
        in_specs=[any_spec] * 7,
        out_specs=any_spec,
        scratch_shapes=[
            pltpu.VMEM((S + DEF, D), BF16),
            pltpu.VMEM((D // 2, D), U32),
            pltpu.VMEM((D // 2, D), U32),
            pltpu.VMEM((2, D // 2, D), U32),
            pltpu.VMEM((NC, LANES), BF16),
            pltpu.VMEM((2, D // 2, F + LANES), U32),
            pltpu.VMEM((F // 2, D + LANES), U32),
            pltpu.VMEM((P0 // 2, D), U32),
            pltpu.VMEM((XSN, S // NA // 2, DA), U32),
            pltpu.VMEM((7 ** LK, DK // 2, DK), U32),
            pltpu.VMEM((D // 2, P0), U32),
            pltpu.VMEM((7 ** LG, DG // 2, TB // NG), U32),
            pltpu.VMEM((D, LANES), F32),
            pltpu.VMEM((D, LANES), F32),
            pltpu.VMEM((RL, LANES), F32),
            pltpu.VMEM((D, D), F32),
            pltpu.VMEM((D // 2, D), U32),
            pltpu.VMEM((7 ** LA, DA // 2, DA), U32),
            pltpu.VMEM((D // 2, D), U32),
            pltpu.VMEM((7 ** LO, DO // 2, DO), U32),
            pltpu.VMEM((max(TB2, RL), D + 2 * LANES), F32),
            pltpu.VMEM((RL // 2, D), U32),
            pltpu.VMEM((7 ** LO, max(TB2, RL) // NO // 2, DO), U32),
            pltpu.VMEM((DEF, D), F32),
            pltpu.VMEM((2, S + DEF, D), BF16),
            pltpu.VMEM((TB, D), F32),
            pltpu.VMEM((8, LANES), U32),
            pltpu.SemaphoreType.DMA((NSEM,)),
        ],
        compiler_params=pltpu.CompilerParams(vmem_limit_bytes=110 * 1024 * 1024, disable_bounds_checks=True,
                                             disable_semaphore_checks=True),
    )(x, A_wqkv, A_wo, wr, B_w_gate, B_w_up, B_w_down)
    return out.reshape(1, S, D)
```

```python
import jax
import jax.numpy as jnp
from jax import lax
import jax.experimental.pallas as pl
import jax.experimental.pallas.tpu as pltpu


S = 2048
D = 1024
F = 3584
H = 32
DH = D // H
LANES = 128
NC = D // LANES
HD = D // 2

LA = 2
LG = 1
LK = 2
LO = 1
NA, NG, NK, NO = 2 ** LA, 2 ** LG, 2 ** LK, 2 ** LO
DA, DG, DK, DO = D // NA, D // NG, D // NK, D // NO
XSN = 7 ** LA if LG == LA else 9 * 7 ** LG
P0 = 512
PB = S - P0
TX = 256
TB = 512
NB1 = PB // TB
TB2 = 384
NB2 = 4
QA = 192
OCH = (128, 128, 128)
DEF = OCH[-1]
L0 = NB2 * TB2
RL = S - L0
QS = (256, 256)
OCL = ((128, False), (128, False), (128, False), (64, True), (64, True))
NPRE = 24
NGAP = 10
OUT_AT = (256, 384, 448)
LNU = 8
LAG_L = 4
LN_DELAY = 800
JOB_DELAY = 500
POST_DELAY = 800
GM = 128
PGM = 128
PGN = 128
PKM = 128
PKK = 256
EV0 = 0
EV1 = 0
EVT = 0
TRW = 256
TRM = 128
GN = 128
WK5 = 66
C6LN = (1000, 8900)
C6WK = (1500, 8900)
P1LN = (60, 12000)
P1WP = (6300, 11500)
P1WQ = (7500, 13100)
WQP = 5
EV2 = 300
P2U = (60, 2000)
LAG = 5
QFIN = False
HFIN = True
EV3 = 0
LN2_DELAY = 900
QP_DELAY = 400
GLAG = (None, None, None, 20, 8)

F32 = jnp.float32
BF16 = jnp.bfloat16
U32 = jnp.uint32
I32 = jnp.int32

XP = ((PB, 128), (PB + 128, 128), (PB + 256, 256), (0, TB), (TB, PB - TB))
WKP = ((0, 128), (128, 128), (256, 256), (512, 512))

SEM_X = 0
SEM_WK = SEM_X + len(XP)
SEM_WQ = SEM_WK + len(WKP)
SEM_W3 = SEM_WQ + 1
SEM_WR = SEM_W3 + 1
SEM_WGU = SEM_WR + 1
SEM_WD = SEM_WGU + 1
SEM_OUT = SEM_WD + 1
NSEM = SEM_OUT + 5

INT_MIN = -(2 ** 31)


def _layernorm(x, tok=None, w=None):
    s0 = x[:, 0:LANES]
    if tok is not None:
        s0 = s0 + jnp.concatenate([tok] * (x.shape[0] // 8), axis=0)
    for c in range(1, NC):
        s0 = s0 + x[:, c * LANES:(c + 1) * LANES]
    mu = jnp.sum(s0, axis=-1, keepdims=True) * (1.0 / D)
    xc = x - mu
    var = jnp.sum(xc * xc, axis=-1, keepdims=True) * (1.0 / D)
    rstd = lax.rsqrt(var + 1e-5)
    if w is None:
        return xc * rstd
    return xc * rstd, jnp.sum(xc * w, axis=-1, keepdims=True) * rstd


def _phi(t):
    return jnp.where(t > 0, t + 1.0, jnp.exp(t)) + 1e-6


def _n_off(a, b):
    return 32 * a + 8 * b


def _n_groups():
    pos = {(2 * o + e) * LANES + _n_off(a, b): (16 * e + 4 * b + a) * DH + 8 * o
           for o in range(4) for e in range(2) for a in range(4) for b in range(4)}
    return [pos[n] for n in sorted(pos)]


def _quads(b):
    h = len(b) // 2
    return [[r[j * h:(j + 1) * h] for r in b[i * h:(i + 1) * h]] for i in range(2) for j in range(2)]


def _badd(x, y):
    return [[a + b for a, b in zip(rx, ry)] for rx, ry in zip(x, y)]


def _bsub(x, y):
    return [[a - b for a, b in zip(rx, ry)] for rx, ry in zip(x, y)]


def _a_set(b):
    if len(b) == 1:
        return [b[0][0]]
    return [x for o in _a_ops(b) for x in _a_set(o)]


def _b_set(b):
    if len(b) == 1:
        return [b[0][0]]
    q11, q12, q21, q22 = _quads(b)
    ops = (_badd(q11, q22), q11, _bsub(q12, q22), _bsub(q21, q11), q22, _badd(q11, q12), _badd(q21, q22))
    return [x for o in ops for x in _b_set(o)]


def _b_in_a(i, levels):
    perm = (0, 2, 6, 5, 3, 4, 1)
    return sum(perm[(i // 7 ** l) % 7] * 7 ** l for l in range(levels))


def _strassen(prod, levels, base=0, fin=lambda k, q: q, init=None):
    if levels == 0:
        return [[prod(base)]]

    def m(i):
        return _strassen(prod, levels - 1, base * 7 + i)

    def seed(q, x):
        return x if init is None else _badd(_quads(init)[q], x)

    m2 = m(2)
    c22 = seed(3, m2)
    m4 = m(4)
    c12 = fin(1, _badd(seed(1, m2), m4))
    c11 = m4 if init is None else _bsub(_quads(init)[0], m4)
    m3 = m(3)
    c11 = _bsub(m3, c11) if init is None else _badd(c11, m3)
    m1 = m(1)
    c21 = fin(2, _badd(seed(2, m3), m1))
    c22 = _bsub(c22, m1)
    m0 = m(0)
    c11 = _badd(c11, m0)
    c22 = _badd(c22, m0)
    c11 = fin(0, _badd(c11, m(6)))
    c22 = fin(3, _badd(c22, m(5)))
    return [a + b for a, b in zip(c11, c12)] + [a + b for a, b in zip(c21, c22)]


def _goff(i, levels):
    return int(format(i, "0%db" % levels)[::-1], 2) if levels else 0


def _blocks(rows, n):
    w = rows[0].shape[1] // n
    return [[r[:, j * w:(j + 1) * w] for j in range(n)] for r in rows]


def _or_all(vals):
    acc = None
    for v in vals:
        v = pltpu.bitcast(v, U32)
        for g in range(v.shape[0] // 8):
            for c in range(v.shape[1] // LANES):
                p = v[g * 8:(g + 1) * 8, c * LANES:(c + 1) * LANES]
                acc = p if acc is None else acc | p
    return acc


def _raw_ops(levels):
    n = 2 ** levels
    names = [[_Tag((i, j)) for j in range(n)] for i in range(n)]
    return {op: t.ij for op, t in enumerate(_b_set(names)) if t.ij is not None}


class _Tag:
    def __init__(self, ij):
        self.ij = ij

    def __add__(self, other):
        return _Tag(None)

    __sub__ = __add__


def _a_ops(b):
    q11, q12, q21, q22 = _quads(b)
    return (_badd(q11, q22), _badd(q21, q22), q11, q22, _badd(q11, q12), _bsub(q21, q11), _bsub(q12, q22))


def _x_set(o):
    return _a_set(o) + ([] if LG == LA else [o[0][1], o[1][0]])


_A_FORM = (((0, 0), (1, 1), 1), ((1, 0), (1, 1), 1), ((0, 0),), ((1, 1),), ((0, 0), (0, 1), 1),
           ((1, 0), (0, 0), -1), ((0, 1), (1, 1), -1))
_B_FORM = (((0, 0), (1, 1), 1), ((0, 0),), ((0, 1), (1, 1), -1), ((1, 0), (0, 0), -1), ((1, 1),),
           ((0, 0), (0, 1), 1), ((1, 0), (1, 1), 1))


def _outer(form, get, n):
    h = n // 2

    def quad(q):
        return [[get(q[0] * h + i, q[1] * h + j) for j in range(h)] for i in range(h)]

    if len(form) == 1:
        return quad(form[0])
    return (_badd if form[2] > 0 else _bsub)(quad(form[0]), quad(form[1]))


def _x_slot(i):
    return i if LG == LA else (i // 7) * 9 + i % 7


def _merge(b):
    return jnp.concatenate([jnp.concatenate(r, axis=1) for r in b], axis=0)


def _gate(v, tok):
    u = pltpu.bitcast(v, U32)
    top = u[0:8, 0:LANES] | tok
    if u.shape[1] > LANES:
        top = jnp.concatenate([top, u[0:8, LANES:]], axis=1)
    return pltpu.bitcast(jnp.concatenate([top, u[8:, :]], axis=0) if u.shape[0] > 8 else top, BF16)


class _Pacer:
    def __init__(self, zero, every=0):
        self.zero, self.t, self.jobs, self.pend, self.tok = zero, 0, [], [], None
        self.every, self.last = every, -every

    def add(self, jobs, t0, t1, delay):
        for k, job in enumerate(jobs):
            self.jobs.append((t0 + k * (t1 - t0) // len(jobs), len(self.jobs), job, delay))
        self.jobs.sort(key=lambda e: e[:2])

    def due(self, dep, delay):
        if dep is not None:
            self.pend.append((self.t + delay, _or_all([dep])))

    def release(self, upto):
        while self.jobs and self.jobs[0][0] <= upto:
            _, _, job, delay = self.jobs.pop(0)
            self.due(job(self.tok), delay)

    def dot(self, lhs, rhs):
        self.release(self.t)
        ready = [d for t, d in self.pend if t <= self.t]
        if ready and self.t - self.last >= self.every:
            self.pend = [e for e in self.pend if e[0] > self.t]
            self.last = self.t
            lhs = _gate(lhs, _or_all(ready) & self.zero)
        res = jnp.dot(lhs, rhs, preferred_element_type=F32)
        self.t += lhs.shape[0] * (lhs.shape[1] // LANES) * (res.shape[1] // LANES) // 4
        self.tok = pltpu.bitcast(pltpu.bitcast(res[0:8, 0:LANES], U32) & self.zero, F32)
        return res

    def flush(self):
        self.release(1 << 30)


def _kernel(x_hbm, wqkv_hbm, wo_hbm, wr_hbm, wg_hbm, wu_hbm, wd_hbm, out_hbm,
            x_v, wk_v, wq_v, w3_v, wr_v, wgu_v, wd_v,
            ln1_v, xs_v, wks_v, pkt_v, pks_v, zacc_v, uacc_v, xw_v, g_v, wqp_v, wqs_v, mp_v, ms_v, pq_v, pqn_v, pqs_v, attn_v, lo_v, lnf_v, zero_v,
            sems):

    ln2_v, out_v = lo_v.at[0], lo_v.at[1]

    wqkv_hbm, wo_hbm, wg_hbm, wu_hbm, wd_hbm = (r.bitcast(U32) for r in (wqkv_hbm, wo_hbm, wg_hbm, wu_hbm, wd_hbm))

    def wload(ref, r0, nr, cols):
        return pltpu.bitcast(ref[r0 // 2:(r0 + nr) // 2, cols], BF16)

    wv_v, wo_v = w3_v.at[0], w3_v.at[1]
    wg_v, wu_v = wgu_v.at[0], wgu_v.at[1]

    def x_copy(i):
        r0, n = XP[i]
        return pltpu.make_async_copy(x_hbm.at[pl.ds(r0, n), :], x_v.at[pl.ds(DEF + r0, n), :], sems.at[SEM_X + i])

    def out_copy(r0, n, s):
        return pltpu.make_async_copy(out_v.at[pl.ds(DEF + r0, n), :], out_hbm.at[pl.ds(r0, n), :],
                                     sems.at[SEM_OUT + s])

    def wk_copy(j):
        c0, n = WKP[j]
        return pltpu.make_async_copy(wqkv_hbm.at[:, pl.ds(D + c0, n)], wk_v.at[:, pl.ds(c0, n)],
                                     sems.at[SEM_WK + j])

    wq_copy = pltpu.make_async_copy(wqkv_hbm.at[:, pl.ds(0, D)], wq_v, sems.at[SEM_WQ])
    wr_copy = pltpu.make_async_copy(wr_hbm, wr_v, sems.at[SEM_WR])
    wd_copy = pltpu.make_async_copy(wd_hbm, wd_v.at[:, pl.ds(0, D)], sems.at[SEM_WD])
    wg_copy = pltpu.make_async_copy(wg_hbm, wg_v.at[:, pl.ds(0, F)], sems.at[SEM_WGU])
    wu_copy = pltpu.make_async_copy(wu_hbm, wu_v.at[:, pl.ds(0, F)], sems.at[SEM_WGU])

    x_copy(0).start()
    wk_copy(0).start()
    x_copy(1).start()
    wr_copy.start()
    for j in range(1, len(WKP)):
        wk_copy(j).start()
    for j in range(2, len(XP)):
        x_copy(j).start()
    wq_copy.start()
    pltpu.make_async_copy(wqkv_hbm.at[:, pl.ds(2 * D, D)], wv_v, sems.at[SEM_W3]).start()
    pltpu.make_async_copy(wo_hbm, wo_v, sems.at[SEM_W3]).start()
    wg_copy.start()
    wu_copy.start()
    wd_copy.start()

    def ln1_rows(xr, xr0, lnr, r0, n):
        ln = _layernorm(xr[xr0:xr0 + n, :].astype(F32)).astype(BF16)
        lnr[r0 // 2:(r0 + n) // 2, :] = pltpu.bitcast(ln, U32)

    def ln1_set(pc, xr, xr0, xsr, a0, n, t0, t1):
        def unit(j):
            def job(tok):
                ln = _layernorm(xr[xr0 + j * LNU:xr0 + (j + 1) * LNU, :].astype(F32), tok)
                lnf_v[j * LNU:(j + 1) * LNU, :] = ln
                return _or_all([ln[:, 0:LANES], ln[:, D - LANES:D]])
            return job

        def piece(j0, c0, o):
            def job(tok):
                def get(i, f):
                    r = (j0 + 2 * _goff(i, LA)) * LNU
                    v = lnf_v[r:r + 16, f * DA + c0:f * DA + c0 + LANES]
                    return v + jnp.concatenate([tok, tok], axis=0) if (i + f) % (NA // 2 + 1) == 0 else v

                r = (a0 + (j0 // (2 * NA)) * 16) // 2
                ops = _x_set(_outer(_A_FORM[o], get, NA))
                for op, v in enumerate(ops):
                    xsr.at[o * len(ops) + op][r:r + 8, c0:c0 + LANES] = pltpu.bitcast(v.astype(BF16), U32)
                return _or_all([v[0:8, :] for v in [ops[0]] + ops[5:7]])
            return job

        grp = 2 * NA
        ng = n // LNU // grp
        dt = (t1 - t0 - LN_DELAY) // (ng + 1)
        for g in range(ng):
            pc.add([unit(g * grp + j) for j in range(grp)], t0 + g * dt, t0 + (g + 1) * dt, LN_DELAY)
            s = t0 + (g + 1) * dt + LN_DELAY
            pc.add([piece(g * grp, c0, o) for c0 in range(0, DA, LANES) for o in range(7)], s, s + dt, JOB_DELAY)

    def ln1_load(lnr, r0, n):
        return pltpu.bitcast(lnr[r0 // 2:(r0 + n) // 2, :], BF16)

    def gate(v, tok):
        return v if tok is None else _gate(v, tok)

    def k_mm(r0, n, c0, nc):
        return jnp.dot(ln1_load(ln1_v, r0, n), wload(wk_v, 0, D, slice(c0, c0 + nc)), preferred_element_type=F32)

    def z_acc(pkts, c0, first=False):
        zs = None
        for pkt in pkts:
            for j in range(pkt.shape[1] // LANES):
                p = pkt[:, j * LANES:(j + 1) * LANES]
                zs = p if zs is None else zs + p
        if first:
            zacc_v[c0:c0 + zs.shape[0], :] = zs
        else:
            zacc_v[c0:c0 + zs.shape[0], :] += zs

    def k_post(k, p0, c0, first=False):
        n, nc = k.shape
        pkt = _phi(k).T
        pkt_v[c0 // 2:(c0 + nc) // 2, p0:p0 + n] = pltpu.bitcast(pkt.astype(BF16), U32)
        z_acc([pkt], c0, first)
        return pkt[nc - 8:nc, n - LANES:n]

    def g_acc(r0, n, c0, nc, first=False, pc=None):
        h, w = (nc, D) if pc is None else (min(nc, PGM), PGN)
        for f0 in range(c0, c0 + nc, h):
            for j0 in range(0, D, w):
                lhs = pltpu.bitcast(pkt_v[f0 // 2:(f0 + h) // 2, r0:r0 + n], BF16)
                rhs = pltpu.bitcast(ln1_v[r0 // 2:(r0 + n) // 2, j0:j0 + w], BF16)
                g = jnp.dot(lhs, rhs, preferred_element_type=F32) if pc is None else pc.dot(lhs, rhs)
                if first:
                    g_v[f0:f0 + h, j0:j0 + w] = g
                else:
                    g_v[f0:f0 + h, j0:j0 + w] += g

    def k_paced(pc, r0, c0, nc, first):
        for j0 in range(c0, c0 + nc, LANES):
            for t0 in range(r0, r0 + TX, PKM):
                k = None
                for k0 in range(0, D, PKK):
                    p = pc.dot(ln1_load(ln1_v, t0, PKM)[:, k0:k0 + PKK], wload(wk_v, k0, PKK, slice(j0, j0 + LANES)))
                    k = p if k is None else k + p
                pc.due(k_post(k, t0, j0, first and t0 == r0), POST_DELAY)

    attn_v[...] = jnp.zeros_like(attn_v)
    zero_v[...] = jnp.zeros_like(zero_v)

    x_copy(0).wait()
    ln1_rows(x_v, DEF + PB, ln1_v, 0, 128)
    wk_copy(0).wait()
    ka = k_mm(0, 128, 0, 128)
    x_copy(1).wait()
    wr_copy.wait()
    ln1_rows(x_v, DEF + PB + 128, ln1_v, 128, 128)
    k_post(ka, 0, 0, first=True)
    g_acc(0, 128, 0, 128, first=True)
    wk_copy(1).wait()
    k_post(k_mm(128, 128, 0, 128), 128, 0)
    k_post(k_mm(0, TX, 128, 128), 0, 128, first=True)
    g_acc(128, 128, 0, 128)
    def w_job(src_ref, dst_ref, levels, r0, c0, o):
        n = 2 ** levels
        w, raw, inner = D // n, _raw_ops(levels), 7 ** (levels - 1)

        def job(tok):
            def cut(i, j):
                return src_ref[(i * w + r0) // 2:(i * w + r0) // 2 + 8, j * w + c0:j * w + c0 + LANES]

            def get(i, j):
                u = cut(i, j)
                return pltpu.bitcast(u if tok is None else u | pltpu.bitcast(tok, U32), BF16).astype(F32)

            ops = []
            for op, v in enumerate(_b_set(_outer(_B_FORM[o], get, n))):
                dst = dst_ref.at[o * inner + op]
                if o * inner + op in raw:
                    dst[r0 // 2:r0 // 2 + 8, c0:c0 + LANES] = cut(*raw[o * inner + op])
                else:
                    dst[r0 // 2:r0 // 2 + 8, c0:c0 + LANES] = pltpu.bitcast(v.astype(BF16), U32)
                    ops.append(v)
            return _or_all(ops[0:1] + ops[-2:]) if ops else None
        return job

    def wk_jobs_of(outer):
        return [w_job(wk_v, wks_v, LK, r0, c0, o) for r0 in range(0, DK, 16) for c0 in range(0, DK, LANES)
                for o in outer]

    wk_copy(2).wait()
    pc = _Pacer(zero_v[...], EV0)
    pc.add(wk_jobs_of((1, 3)), 500, 2200, JOB_DELAY)
    k_paced(pc, 0, 256, 256, True)
    g_acc(0, TX, 128, 128, True, pc)
    g_acc(0, TX, 256, 256, True, pc)
    pc.flush()
    wk_copy(3).wait()
    wk_jobs = wk_jobs_of((0, 2, 4, 5, 6))
    pc = _Pacer(zero_v[...], EV0)
    pc.add(wk_jobs[:WK5], 500, 2700, JOB_DELAY)
    k_paced(pc, 0, 512, 512, True)
    g_acc(0, TX, 512, 256, True, pc)
    pc.flush()
    x_copy(2).wait()
    x_copy(3).wait()
    pc = _Pacer(zero_v[...], EV0)
    ln1_set(pc, x_v, DEF, xs_v, 0, TB, *C6LN)
    pc.add(wk_jobs[WK5:], *C6WK, JOB_DELAY)
    ln1_rows(x_v, DEF + PB + TX, ln1_v, TX, TX)
    g_acc(0, TX, 768, 256, True, pc)
    k_paced(pc, TX, 0, D, False)
    for c0 in range(0, D, 256):
        g_acc(TX, TX, c0, 256, False, pc)
    pc.flush()

    MA = TB // NA
    NS = NK // NG

    def xs_load(xsr, op, a0, m, cols=slice(None)):
        return pltpu.bitcast(xsr[op, a0 // 2:(a0 + m) // 2, cols], BF16)

    def k_step(pc, xsr, j0):
        def fin(_, q):
            if NS > 1:
                q = [[jnp.concatenate([_phi(jnp.concatenate([r[f] for r in q], axis=0)).T for f in range(NS)],
                                      axis=0)]]
            else:
                q = [[_phi(v).T for v in r] for r in q]
            pc.due(_or_all([v[t - 8:t, :] for r in q for v in r for t in range(LANES, v.shape[0] + 1, LANES)]),
                   POST_DELAY)
            return q

        def lhs(i):
            if LK == LA:
                return xs_load(xsr, _x_slot(i), 0, MA)
            return _merge([[xs_load(xsr, i * 9 + s, 0, MA) for s in r] for r in ((2, 7), (8, 3))])

        cb = _strassen(lambda i: pc.dot(lhs(i), pltpu.bitcast(wks_v[i, :, j0:j0 + LANES], BF16)), LK, fin=fin)
        ops = _a_ops([[cb[i][f] for i in range(NG)] for f in range(NG)])
        for half, o in ((0, ops[4]), (1, ops[1])):
            for f, rowb in enumerate(o):
                for s in range(NS):
                    z_acc([v[s * LANES:(s + 1) * LANES, :] for v in rowb], half * HD + f * DG + s * DK + j0)
        for _ in range(LG - 1):
            ops = [o for x in ops for o in _a_ops(x)]
        for op, o in enumerate(ops):
            r = j0 * NS
            pks_v.at[op][r // 2:(r + NS * LANES) // 2, :] = pltpu.bitcast(o[0][0].astype(BF16), U32)
        pc.due(_or_all([o[0][0][NS * LANES - 8:NS * LANES, :] for o in (ops[0], ops[-1], ops[-2])]), 2 * POST_DELAY)

    def g_rhs(xsr, i, c0, nc):
        o = _b_in_a(i, LG)
        if LG == LA:
            return xs_load(xsr, o, 0, MA, slice(c0, c0 + nc))
        j, cs = c0 // DA, slice(c0 % DA, c0 % DA + nc)
        return jnp.concatenate([xs_load(xsr, o * 9 + s, 0, MA, cs) for s in ((2, 8), (7, 3))[j]], axis=0)

    def g_step(pc, xsr, r0, nr, c0, nc):
        cb = _strassen(lambda i: pc.dot(pltpu.bitcast(pks_v[i, r0 // 2:(r0 + nr) // 2, :], BF16),
                                        g_rhs(xsr, i, c0, nc)), LG)
        for f in range(NG):
            for c in range(NG):
                h = min(nr, LANES)
                for t in range(nr // h):
                    step, sub = divmod((r0 + t * h) // LANES, NS)
                    g0_ = f * DG + sub * DK + step * LANES + (r0 + t * h) % LANES
                    g_v[g0_:g0_ + h, c * DG + c0:c * DG + c0 + nc] += cb[f][c][t * h:(t + 1) * h, :]

    def wq_jobs(u0, nr):
        span = (NA - 1) * DA + 16 * nr
        u0 = u0 if isinstance(u0, int) else pl.multiple_of(u0, 8)
        srcr, permr = wq_v.at[pl.ds(u0, span // 2), :], wqp_v.at[pl.ds(u0, span // 2), :]
        dstr = wqs_v.at[:, pl.ds(u0, 8 * nr), :]
        oct_ = (lax.broadcasted_iota(I32, (8, LANES), 1) % DH) // 8

        def perm(r, e):
            def job(tok):
                blk = [srcr[r // 2:r // 2 + 8, (4 * e + b) * LANES:(4 * e + b + 1) * LANES] | pltpu.bitcast(tok, U32)
                       for b in range(4)]
                outs = []
                for o in range(4):
                    v = blk[o]
                    for b in range(4):
                        if b != o:
                            v = jnp.where(oct_ == b, pltpu.roll(blk[b], (8 * (b - o)) % LANES, 1), v)
                    permr[r // 2:r // 2 + 8, (2 * o + e) * LANES:(2 * o + e + 1) * LANES] = v
                    outs.append(v)
                return _or_all(outs)
            return job

        return ([perm(i * DA + r0, e) for r0 in range(0, 16 * nr, 16) for i in range(NA) for e in range(2)],
                [w_job(permr, dstr, LA, r0, c0, o) for r0 in range(0, 16 * nr, 16)
                 for c0 in range(0, DA, LANES) for o in range(7)])

    def p1(i, carry):
        xsr = xs_v.at[:, pl.ds(pl.multiple_of(i * (MA // 2), MA // 2), MA), :]
        xr = x_v.at[pl.ds(pl.multiple_of((i + 1) * TB, TB), TB + DEF), :]

        pc = _Pacer(zero_v[...], EV1)
        ln1_set(pc, xr, DEF, xsr, MA, TB, *P1LN)
        perms, sets = wq_jobs(i * (8 * WQP), WQP)
        pc.add(perms, *P1WP, JOB_DELAY)
        pc.add(sets, *P1WQ, JOB_DELAY)
        for j0 in range(0, DK, LANES):
            k_step(pc, xsr, j0)
        for f0 in range(0, DG, GM):
            for c0 in range(0, DG, GN):
                g_step(pc, xsr, f0, GM, c0, GN)
        pc.flush()
        return carry

    x_copy(4).wait()
    wq_copy.wait()
    lax.fori_loop(0, NB1, p1, 0)

    pltpu.make_async_copy(w3_v, w3_v, sems.at[SEM_W3]).wait()
    zero_u = zero_v[...]
    def row_vector(acc_ref):
        return jnp.sum(jnp.concatenate([acc_ref[r:r + 8, :] for r in _n_groups()], axis=0).T, axis=0, keepdims=True)

    zrow = row_vector(zacc_v)
    wr8 = wr_v[...].astype(F32)
    wr_row = jnp.concatenate([wr8[c:c + 1, :] for c in range(NC)], axis=1)

    row_h = lax.broadcasted_iota(I32, (LANES, LANES), 0) // DH
    col_h = lax.broadcasted_iota(I32, (LANES, LANES), 1) // DH
    diag = row_h == col_h

    def colsum(t):
        acc = t[:, 0:LANES]
        for c in range(1, NC):
            acc = acc + t[:, c * LANES:(c + 1) * LANES]
        return acc

    wrc = wr_row - jnp.sum(wr_row, axis=-1, keepdims=True) * (1.0 / D)
    m_raw = _raw_ops(LO)

    def kv_part(c):
        cs = slice(c * LANES, (c + 1) * LANES)
        kv = None
        for k0 in range(0, D, TRW):
            p = pc.dot(g_v[cs, k0:k0 + TRW].astype(BF16), wload(wv_v, k0, TRW, cs))
            kv = p if kv is None else kv + p
        return jnp.where(diag, kv, 0.0)

    def m_part(c, kvs):
        e, b = c // 4, c % 4
        for j0 in range(0, DO, TRM):
            ms = [jnp.concatenate(
                [pc.dot(kv, wload(wo_v, (c + k) * LANES, LANES, slice(f * DO + j0, f * DO + j0 + TRM)))
                 for f in range(NO)], axis=1) for k, kv in enumerate(kvs)]
            deps = []
            for a in range(4):
                rows = [jnp.concatenate([m[a * DH + 8 * o:a * DH + 8 * o + 8, :] for m in ms], axis=0)
                        for o in range(4)]
                for o in range(4):
                    r = ((2 * o + e) * LANES + _n_off(a, b)) // 2
                    for f in range(NO):
                        mp_v[r:r + 8, f * DO + j0:f * DO + j0 + TRM] = pltpu.bitcast(
                            rows[o][:, f * TRM:(f + 1) * TRM].astype(BF16), U32)
                for t in range(4 // NO):
                    r = ((2 * t + e) * LANES + _n_off(a, b)) // 2
                    for op, v in enumerate(_b_set(_blocks(rows[t::4 // NO], NO))):
                        if op not in m_raw:
                            ms_v.at[op][r:r + 8, j0:j0 + TRM] = pltpu.bitcast(v.astype(BF16), U32)
                            deps.append(v[0:8, 0:LANES])
            pc.due(_or_all(deps[::4]), POST_DELAY)

    pc = _Pacer(zero_u, EVT)
    pc.due(jnp.broadcast_to(zrow, (8, D)), 1000)
    perms, sets = wq_jobs(NB1 * 8 * WQP, DA // 16 - NB1 * WQP)
    pc.add(perms, 60, 700, JOB_DELAY)
    pc.add(sets, 1300, 3400, JOB_DELAY)
    kv_prev = None
    for c in range(0, NC + 2, 2):
        kvs = [kv_part(c).astype(BF16), kv_part(c + 1).astype(BF16)] if c < NC else None
        if c:
            m_part(c - 2, kv_prev)
        kv_prev = kvs
    pc.flush()

    def make_key(score, row):
        b = pltpu.bitcast(score, I32)
        srt = b ^ ((b >> 31) & 0x7FFFFFFF)
        return (srt & jnp.int32(-65536)) | (0xFFFF - row)

    def push_keys(key, top1, top2):
        for gidx in range(key.shape[0] // 8):
            kx = key[gidx * 8:(gidx + 1) * 8, :]
            top2 = jnp.maximum(top2, jnp.minimum(top1, kx))
            top1 = jnp.maximum(top1, kx)
        return top1, top2

    lane = lax.broadcasted_iota(I32, (1, LANES), 1)

    def interleave(parts):
        return jnp.concatenate([p[g * 16:(g + 1) * 16, :] for g in range(parts[0].shape[0] // 16) for p in parts],
                               axis=0)

    def q_part(pc, xsr, l0, r0, n, hint=None):
        m = n // NA
        sums = {}

        def park(v, g, c):
            for t in range(m // 16):
                r = r0 + (t * NA + g) * 16
                pq_v[r:r + 16, c * LANES:(c + 1) * LANES] = v[t * 16:(t + 1) * 16, :]

        def fin(k, q):
            q = [[_phi(v) for v in r] for r in q]
            deps = []
            for a, r in enumerate(q):
                for b, v in enumerate(r):
                    i, c = (k // 2) * (NA // 2) + a, (((k % 2) * (NA // 2) + b) * DA + j0) // LANES
                    park(v, _goff(i, LA), c)
                    for name, row in (("z", zrow),) + ((("u", hint["u"]),) if hint else ()):
                        t = v * row[:, c * LANES:(c + 1) * LANES]
                        key = (name, _goff(i, LA), c % 2)
                        sums[key] = t if key not in sums else sums[key] + t
                deps.append(sums[key])
            if (r0 + n < RL or HFIN) if hint else QFIN:
                pc.due(_or_all(deps), POST_DELAY)
            return q

        for j0 in range(0, DA, LANES):
            _strassen(lambda i: pc.dot(xs_load(xsr, _x_slot(i), (l0 + r0) // NA, m),
                                       pltpu.bitcast(wqs_v[i, :, j0:j0 + LANES], BF16)), LA, fin=fin)
        if hint:
            pc.flush()
        den = jnp.concatenate([sums["z", g, e] for g in range(NA) for e in range(2)], axis=0)
        for s in (1, 2, 4):
            den = den + jnp.where((lane & s) == 0, pltpu.roll(den, LANES - s, 1), pltpu.roll(den, s, 1))
        inv_all = 1.0 / (den + 1e-6)

        def inv_of(g):
            return [inv_all[(g * 2 + e) * m:(g * 2 + e + 1) * m, :] for e in range(2)]

        for g in range(NA):
            for e in range(2):
                park(inv_of(g)[e], g, NC + e)
        if hint:
            for g in range(NA):
                starts = [r0 + (t * NA + g) * 16 for t in range(m // 16)]
                num = jnp.sum(jnp.concatenate([xw_v[t:t + 16, :] for t in starts], axis=0)
                              + sums["u", g, 0] * inv_of(g)[0] + sums["u", g, 1] * inv_of(g)[1],
                              axis=-1, keepdims=True)
                row = jnp.concatenate([(l0 + t) + lax.broadcasted_iota(I32, (16, 1), 0) for t in starts], axis=0)
                hint["p1"], hint["p2"] = push_keys(make_key(num, row), hint["p1"], hint["p2"])
            pc.due(jnp.broadcast_to(hint["p1"], (8, LANES)), 1200)


    def post_jobs(r0, n, plain=False):
        def scaled(t, c0, w, tok):
            inv = pq_v[t:t + 16, D:D + 2 * LANES]
            if tok is not None:
                inv = inv + jnp.concatenate([jnp.concatenate([tok, tok], axis=0)] * 2, axis=1)
            return pq_v[t:t + 16, c0:c0 + w] * jnp.concatenate([inv] * (w // (2 * LANES)), axis=1)

        def post_plain(t):
            def job(tok):
                v = scaled(t, 0, D, tok)
                pqn_v[t // 2:t // 2 + 8, :] = pltpu.bitcast(v.astype(BF16), U32)
                return v[0:8, 0:LANES]
            return job

        def post(t0, outer):
            def job(tok):
                deps = []
                for c0 in range(0, DO, 2 * LANES):
                    blk = {}

                    def get(i, f):
                        if (i, f) not in blk:
                            blk[i, f] = scaled(t0 + _goff(i, LO) * 16, f * DO + c0, 2 * LANES, tok)
                        return blk[i, f]

                    for o in outer:
                        ops = _a_set(_outer(_A_FORM[o], get, NO))
                        for op, v in enumerate(ops):
                            pqs_v.at[o * len(ops) + op][t0 // NO // 2:t0 // NO // 2 + 8, c0:c0 + 2 * LANES] = (
                                pltpu.bitcast(v.astype(BF16), U32))
                        deps.append(ops[0][0:8, 0:LANES])
                return _or_all(deps)
            return job

        if plain:
            return [post_plain(t) for t in range(r0, r0 + n, 16)]
        outers = [range(7)] if LO == 1 else [(o,) for o in range(7)]
        return [post(t0, outer) for t0 in range(r0, r0 + n, 16 * NO) for outer in outers]

    def m_operand(i, c0, c1):
        if i not in m_raw:
            return pltpu.bitcast(ms_v[i, :, c0 * LANES:c1 * LANES], BF16)
        bi, bj = m_raw[i]
        return wload(mp_v, bi * DO, DO, slice(bj * DO + c0 * LANES, bj * DO + c1 * LANES))

    def o_part(dot, xr, x0, r0, n):
        a0, m = r0 // NO, n // NO
        nw = LANES * NO // 2
        cols = [[[] for _ in range(NO)] for _ in range(NO)]
        for c0 in range(0, DO, nw):
            init = [[jnp.concatenate(
                [xr[x0 + r0 + (g * NO + _goff(i, LO)) * 16:x0 + r0 + (g * NO + _goff(i, LO) + 1) * 16,
                    f * DO + c0:f * DO + c0 + nw] for g in range(m // 16)], axis=0).astype(F32)
                for f in range(NO)] for i in range(NO)]
            cb = _strassen(lambda i: dot(pltpu.bitcast(pqs_v[i, a0 // 2:(a0 + m) // 2, :], BF16),
                                         m_operand(i, c0 // LANES, (c0 + nw) // LANES)), LO, init=init)
            for i in range(NO):
                for f in range(NO):
                    cols[i][f].append(cb[i][f])
        parts = [None] * NO
        for i in range(NO):
            parts[_goff(i, LO)] = jnp.concatenate([c for f in range(NO) for c in cols[i][f]], axis=1)
        return interleave(parts)

    def ln2_unit(h, l2r, outr, r0, row0, valid, top1, top2, tok, fast=False):
        n = h.shape[0]
        if fast:
            ln2, r = _layernorm(h, tok, wr_row)
        else:
            ln2 = _layernorm(h, tok)
            r = jnp.sum(ln2 * wr_row, axis=-1, keepdims=True)
        l2r[r0:r0 + n, :] = ln2.astype(BF16)
        res = h + ln2
        outr[r0:r0 + n, :] = res.astype(BF16)
        r = r.astype(BF16).astype(F32) + 0.0
        key = make_key(r, (row0 + r0) + lax.broadcasted_iota(I32, (n, 1), 0))
        if valid is not None:
            key = jnp.where(valid, key, INT_MIN)
        top1, top2 = push_keys(key, top1, top2)
        ntok = pltpu.bitcast(pltpu.bitcast(jnp.broadcast_to(r[n - 8:n, :], (8, LANES)), U32) & zero_u, F32)
        return top1, top2, ntok

    def ln2_jobs(h, l2r, outr, r0, row0, valid, st, fast=False):
        def unit(j):
            def job(tok):
                st["top1"], st["top2"], dep = ln2_unit(h[j * LNU:(j + 1) * LNU, :], l2r, outr, r0 + j * LNU, row0,
                                                       valid, st["top1"], st["top2"], tok, fast)
                return dep
            return job
        return [unit(j) for j in range(h.shape[0] // LNU)]

    QC = 16 * 7 ** LA / 8 ** LA
    OC = 16 * 7 ** LO / 8 ** LO

    def p2(i, carry):
        st = dict(top1=carry[0], top2=carry[1])
        b0 = pl.multiple_of(i * TB2, 16)
        xsr = xs_v.at[:, pl.ds(pl.multiple_of(i * (TB2 // NA // 2), 8), TB2 // NA // 2), :]
        xr = x_v.at[pl.ds(b0, TB2 + DEF), :]
        l2r = ln2_v.at[pl.ds(b0, TB2 + DEF), :]
        outr = out_v.at[pl.ds(b0, TB2 + DEF), :]
        row0 = b0 - DEF
        pc = _Pacer(zero_u)
        toks = []

        def chain(jobs):
            for job in jobs:
                toks.append(job(toks[-LAG] if len(toks) >= LAG else None))

        chain(ln2_jobs(attn_v, l2r, outr, 0, row0, i > 0, st))

        @pl.when(i > 0)
        def _():
            out_copy(pl.multiple_of((i - 1) * TB2, 16), TB2, 0).start()

        pc.due(toks[-1], QA * QC)

        nu, nx = D // NB2, RL // NB2
        mr = mp_v.at[pl.ds(pl.multiple_of(i * (nu // 2), 8), nu // 2), :]
        ur = uacc_v.at[pl.ds(pl.multiple_of(i * nu, 8), nu), :]
        xl = x_v.at[pl.ds(pl.multiple_of(DEF + L0 + i * nx, 16), nx), :]
        xwr = xw_v.at[pl.ds(pl.multiple_of(i * nx, 8), nx), :]

        def hint_job(load, dst, r):
            def job(tok):
                v = colsum(load(r).astype(F32) * wrc) + jnp.concatenate([tok, tok], axis=0)
                dst[r:r + 16, :] = v
                return v
            return job

        pc.add([hint_job(lambda r: wload(mr, r, 16, slice(None)), ur, r) for r in range(0, nu, 16)]
               + [hint_job(lambda r: xl[r:r + 16, :], xwr, r) for r in range(0, nx, 16)], *P2U, JOB_DELAY)
        for r0, n in ((0, QA), (QA, TB2 - QA)):
            q_part(pc, xsr, 0, r0, n)
            for job in post_jobs(r0, n):
                job(None)
        r0 = 0
        for n in OCH[:-1]:
            chain(ln2_jobs(o_part(pc.dot, xr, DEF, r0, n), l2r, outr, DEF + r0, row0, None, st))
            r0 += n
        attn_v[...] = o_part(pc.dot, xr, DEF, r0, DEF)
        return st["top1"], st["top2"]

    init = jnp.full((8, 1), INT_MIN, I32)
    top1, top2 = lax.fori_loop(0, NB2, p2, (init, init))

    wg_copy.wait()
    wu_copy.wait()
    wd_copy.wait()
    sub8 = lax.broadcasted_iota(I32, (8, LANES), 0)
    urow = jnp.sum(uacc_v[...].T, axis=0, keepdims=True)

    def submax(v):
        for sh in (4, 2, 1):
            v = jnp.maximum(v, pltpu.roll(v, sh, 0))
        return v

    def subsum(v):
        for sh in (4, 2, 1):
            v = v + pltpu.roll(v, sh, 0)
        return v

    def best2(t1, t2):
        t1 = jnp.broadcast_to(t1, (8, LANES))
        t2 = jnp.broadcast_to(t2, (8, LANES))
        k1v = submax(t1)
        return k1v, submax(jnp.where(t1 == k1v, t2, t1))

    def key_row(k):
        return 0xFFFF - (k & 0xFFFF)

    def wide(m):
        return jnp.concatenate([m] * NC, axis=1)

    st = dict(top1=top1, top2=top2, pend=[], step=0, sent=0)
    pc = _Pacer(zero_u, EV2)
    hint = dict(u=urow, p1=init, p2=init)

    pc.add(ln2_jobs(attn_v, ln2_v, out_v, L0, -DEF, None, st), 60, QS[0] * QC - 600, LN2_DELAY)
    r0 = 0
    for k, n in enumerate(QS):
        q_part(pc, xs_v, L0, r0, n, hint)
        if k == 0:
            out_copy(L0 - TB2, TB2, 0).start()
            top1, top2 = st["top1"], st["top2"]
            pc.add(post_jobs(0, OCL[0][0], OCL[0][1]), pc.t + 600, pc.t + (RL - n) * QC - 300, QP_DELAY)
        r0 += n
    pc.every = EV3
    oldk = best2(top1, top2)
    oldx = []
    for kk in oldk:
        g8 = pl.multiple_of(((jnp.clip(key_row(kk[0, 0]), 0, S - 1) >> 3) << 3) + DEF, 8)
        rows = ln2_v[pl.ds(g8, 8), :].astype(F32)
        oldx.append(subsum(jnp.where(wide((key_row(kk) & 7) == sub8), rows, 0.0)))

    def gated(v):
        tok = None
        while st["pend"] and st["pend"][0][0] <= st["step"]:
            t = st["pend"].pop(0)[1]
            tok = t if tok is None else tok | t
        if tok is None:
            return v
        u = pltpu.bitcast(v, U32)
        return pltpu.bitcast(jnp.concatenate([u[:, 0:LANES] | tok, u[:, LANES:]], axis=1), BF16)

    res = {}

    def c_units():
        pc.flush()
        p1, p2_ = hint["p1"], hint["p2"]
        cand_p, cand_x = [], []
        for pk_ in (p1, p2_):
            cp, cx = None, None
            for s in range(8):
                g8 = pl.multiple_of((jnp.clip(key_row(pk_[s, 0]) - L0, 0, RL - 1) >> 3) << 3, 8)
                vp = pq_v[pl.ds(g8, 8), :]
                vx = x_v[pl.ds(pl.multiple_of(g8 + (L0 + DEF), 8), 8), :].astype(F32)
                cp = vp if cp is None else jnp.where(jnp.concatenate([sub8 == s] * (NC + 2), axis=1), vp, cp)
                cx = vx if cx is None else jnp.where(wide(sub8 == s), vx, cx)
            cand_p.append(cp[:, 0:D] * jnp.concatenate([cp[:, D:]] * (NC // 2), axis=1))
            cand_x.append(cx)
        cand_p = jnp.concatenate(cand_p, axis=0).astype(BF16)
        cand_x = jnp.concatenate(cand_x, axis=0)
        ids_lo = key_row(jnp.broadcast_to(p1, (8, LANES)))
        ids_hi = jnp.where(sub8 < 6, key_row(jnp.broadcast_to(p2_, (8, LANES))),
                           jnp.where(sub8 == 6, key_row(oldk[0]), key_row(oldk[1])))
        res["ids"] = (ids_lo, ids_hi)
        parts = []
        for c in range(NC):
            parts.append(jnp.dot(cand_p, wload(mp_v, 0, D, slice(c * LANES, (c + 1) * LANES)), preferred_element_type=F32))
            yield
        xs = _layernorm(cand_x + jnp.concatenate(parts, axis=1))
        hi = jnp.where(wide(sub8 < 6), xs[8:16, :], jnp.where(wide(sub8 == 6), oldx[0], oldx[1]))
        res["xs"] = jnp.concatenate([xs[0:8, :], hi], axis=0).astype(BF16)

    def f_units():
        xs = res["xs"]
        acts = []
        for j in range(F // LANES):
            cs = slice(j * LANES, (j + 1) * LANES)
            g = jnp.dot(gated(xs), wload(wg_v, 0, D, cs), preferred_element_type=F32)
            yield
            u = jnp.dot(xs, wload(wu_v, 0, D, cs), preferred_element_type=F32)
            acts.append((g * jax.nn.sigmoid(g) * u).astype(BF16))
            yield
        act = jnp.concatenate(acts, axis=1)
        zf = pltpu.bitcast(zero_u, F32)
        ys = []
        KF = (F // D) * D
        for c in range(0, NC, 2):
            acc = jnp.concatenate([jnp.concatenate([zf, zf], axis=0)] * 2, axis=1)
            acc = acc + jnp.dot(gated(act[:, KF:]), wload(wd_v, KF, F - KF, slice(c * LANES, (c + 2) * LANES)),
                                preferred_element_type=F32)
            yield
            for cc in range(2):
                y = acc[:, cc * LANES:(cc + 1) * LANES]
                for k0 in range(0, KF, D):
                    y = y + jnp.dot(gated(act[:, k0:k0 + D]),
                                    wload(wd_v, k0, D, slice((c + cc) * LANES, (c + cc + 1) * LANES)),
                                    preferred_element_type=F32)
                    yield
                ys.append(y)
        res["y"] = jnp.concatenate(ys, axis=1)

    def side_units():
        yield from range(NPRE)
        yield from c_units()
        yield from range(NGAP)
        yield from f_units()

    side = side_units()

    def o_dot(lhs, rhs):
        p = pc.dot(lhs, rhs) if st["step"] < NPRE else jnp.dot(lhs, rhs, preferred_element_type=F32)
        next(side, None)
        st["step"] += 1
        return p

    def o_plain(r0, n):
        lhs = pltpu.bitcast(pqn_v[r0 // 2:(r0 + n) // 2, :], BF16)
        parts = []
        for c0 in range(0, NC, 2):
            acc = x_v[DEF + L0 + r0:DEF + L0 + r0 + n, c0 * LANES:(c0 + 2) * LANES].astype(F32)
            for k0 in range(0, D, 2 * LANES):
                acc = acc + o_dot(lhs[:, k0:k0 + 2 * LANES], wload(mp_v, k0, 2 * LANES, slice(c0 * LANES, (c0 + 2) * LANES)))
            parts.append(acc)
        return jnp.concatenate(parts, axis=1)

    toks = []
    r0 = 0
    pc.add(post_jobs(OCL[0][0], *OCL[1]), pc.t + 200, pc.t + 1000, QP_DELAY)
    for ci, (n, plain) in enumerate(OCL):
        h = o_plain(r0, n) if plain else o_part(o_dot, x_v, DEF + L0, r0, n)
        last = r0 + n == RL
        units = ln2_jobs(h, ln2_v, out_v, DEF + L0 + r0, -DEF, None, st, fast=last)
        posts = post_jobs(r0 + n + OCL[ci + 1][0], *OCL[ci + 2]) if ci + 2 < len(OCL) else []
        for k, job in enumerate(units):
            toks.append(job(toks[-LAG_L] if len(toks) >= LAG_L and not last else None))
            if posts:
                posts.pop(0)(toks[-1])
        if GLAG[ci] is not None:
            st["pend"].append((st["step"] + GLAG[ci],
                               pltpu.bitcast(jnp.broadcast_to(st["top1"], (8, LANES)), U32) & zero_u))
        r0 += n
        if last or r0 in OUT_AT:
            out_copy(L0 + st["sent"], r0 - st["sent"], 2 if last else 1).start()
            if not last:
                st["sent"] = r0
    for _ in side:
        st["step"] += 1

    keyv = best2(st["top1"], st["top2"])
    idx = [jnp.clip(key_row(kk[0, 0]), 0, S - 1) for kk in keyv]
    grp = [pl.multiple_of((ii >> 3) << 3, 8) for ii in idx]
    vgrp = [pl.multiple_of(gg + DEF, 8) for gg in grp]
    y = res["y"]
    ids_lo, ids_hi = res["ids"]
    hits = None
    yrows = []
    for c in range(2):
        m_lo = ids_lo == key_row(keyv[c])
        m_hi = ids_hi == key_row(keyv[c])
        yrows.append(subsum(jnp.where(wide(m_lo), y[0:8, :], 0.0) + jnp.where(wide(m_hi), y[8:16, :], 0.0)))
        hit = submax(jnp.where(m_lo | m_hi, 1, 0))
        hits = hit if hits is None else hits + hit
    hit_all = hits[0, 0] == 2

    tail0 = L0 + st["sent"]
    tail_copy = out_copy(tail0, S - tail0, 2)
    in_tail = jnp.maximum(grp[0], grp[1]) >= tail0
    two_groups = grp[1] != grp[0]

    def fix_copy(c):
        return out_copy(grp[c], 8, 3 + c)

    def finish(ysel):
        for c in range(2):
            hi = keyv[c] & jnp.int32(-65536)
            score = pltpu.bitcast(hi ^ ((hi >> 31) & 0x7FFF0000), F32)
            sel = (key_row(keyv[c]) & 7) == sub8
            upd = jnp.where(wide(sel), ysel[c] * wide(jax.nn.sigmoid(score)), 0.0)
            out_v[pl.ds(vgrp[c], 8), :] = (out_v[pl.ds(vgrp[c], 8), :].astype(F32) + upd).astype(BF16)
        fix_copy(0).start()

        @pl.when(two_groups)
        def _():
            fix_copy(1).start()

    out_copy(0, L0, 0).wait()
    out_copy(L0, tail0 - L0, 1).wait()

    @pl.when(in_tail)
    def _():
        tail_copy.wait()

    @pl.when(hit_all)
    def _():
        finish(yrows)

    @pl.when(jnp.logical_not(hit_all))
    def _():
        xsel = jnp.concatenate([ln2_v[pl.ds(vgrp[c], 8), :] for c in range(2)], axis=0)

        def ffn_tile(j, acc):
            cs = pl.ds(pl.multiple_of(j * LANES, LANES), LANES)
            g = jnp.dot(xsel, wload(wg_v, 0, D, cs), preferred_element_type=F32)
            u = jnp.dot(xsel, wload(wu_v, 0, D, cs), preferred_element_type=F32)
            a = (g * jax.nn.sigmoid(g) * u).astype(BF16)
            wd_t = pltpu.bitcast(wd_v[pl.ds(pl.multiple_of(j * (LANES // 2), LANES // 2), LANES // 2), 0:D], BF16)
            return acc + jnp.dot(a, wd_t, preferred_element_type=F32)

        yf = lax.fori_loop(0, F // LANES, ffn_tile, jnp.zeros((16, D), F32))
        finish([yf[0:8, :], yf[8:16, :]])

    @pl.when(jnp.logical_not(in_tail))
    def _():
        tail_copy.wait()

    fix_copy(0).wait()

    @pl.when(two_groups)
    def _():
        fix_copy(1).wait()


@jax.jit
def pallas_sequential_preLN__linear_attn_block__moe_arch_mod__prompt_kernel(
    A_x: jax.Array,
    A_wqkv: jax.Array,
    A_wo: jax.Array,
    B_x: jax.Array,
    B_w_r: jax.Array,
    B_w_gate: jax.Array,
    B_w_up: jax.Array,
    B_w_down: jax.Array,
):
    del B_x
    x = A_x.reshape(S, D)
    wr = B_w_r.reshape(NC, LANES)
    any_spec = pl.BlockSpec(memory_space=pl.ANY)
    out = pl.pallas_call(
        _kernel,
        out_shape=jax.ShapeDtypeStruct((S, D), BF16),
        in_specs=[any_spec] * 7,
        out_specs=any_spec,
        scratch_shapes=[
            pltpu.VMEM((S + DEF, D), BF16),
            pltpu.VMEM((D // 2, D), U32),
            pltpu.VMEM((D // 2, D), U32),
            pltpu.VMEM((2, D // 2, D), U32),
            pltpu.VMEM((NC, LANES), BF16),
            pltpu.VMEM((2, D // 2, F + LANES), U32),
            pltpu.VMEM((F // 2, D + LANES), U32),
            pltpu.VMEM((P0 // 2, D), U32),
            pltpu.VMEM((XSN, S // NA // 2, DA), U32),
            pltpu.VMEM((7 ** LK, DK // 2, DK), U32),
            pltpu.VMEM((D // 2, P0), U32),
            pltpu.VMEM((7 ** LG, DG // 2, TB // NG), U32),
            pltpu.VMEM((D, LANES), F32),
            pltpu.VMEM((D, LANES), F32),
            pltpu.VMEM((RL, LANES), F32),
            pltpu.VMEM((D, D), F32),
            pltpu.VMEM((D // 2, D), U32),
            pltpu.VMEM((7 ** LA, DA // 2, DA), U32),
            pltpu.VMEM((D // 2, D), U32),
            pltpu.VMEM((7 ** LO, DO // 2, DO), U32),
            pltpu.VMEM((max(TB2, RL), D + 2 * LANES), F32),
            pltpu.VMEM((RL // 2, D), U32),
            pltpu.VMEM((7 ** LO, max(TB2, RL) // NO // 2, DO), U32),
            pltpu.VMEM((DEF, D), F32),
            pltpu.VMEM((2, S + DEF, D), BF16),
            pltpu.VMEM((TB, D), F32),
            pltpu.VMEM((8, LANES), U32),
            pltpu.SemaphoreType.DMA((NSEM,)),
        ],
        compiler_params=pltpu.CompilerParams(vmem_limit_bytes=110 * 1024 * 1024, disable_bounds_checks=True,
                                             disable_semaphore_checks=True),
    )(x, A_wqkv, A_wo, wr, B_w_gate, B_w_up, B_w_down)
    return out.reshape(1, S, D)
```

```python
import jax
import jax.numpy as jnp
from jax import lax
import jax.experimental.pallas as pl
import jax.experimental.pallas.tpu as pltpu


S = 2048
D = 1024
F = 3584
H = 32
DH = D // H
LANES = 128
NC = D // LANES
HD = D // 2

LA = 2
LG = 2
LK = 2
LO = 1
NA, NG, NK, NO = 2 ** LA, 2 ** LG, 2 ** LK, 2 ** LO
DA, DG, DK, DO = D // NA, D // NG, D // NK, D // NO
XSN = 7 ** LA if LG == LA else 9 * 7 ** LG
P0 = 512
PB = S - P0
TX = 256
TB = 512
NB1 = PB // TB
TB2 = 384
NB2 = 4
QA = 192
OCH = (128, 128, 128)
DEF = OCH[-1]
L0 = NB2 * TB2
RL = S - L0
QS = (256, 256)
OCL = ((128, False), (128, False), (128, False), (64, True), (64, True))
NPRE = 24
NGAP = 10
OUT_AT = (256, 384, 448)
LNU = 8
LAG_L = 4
LN_DELAY = 800
JOB_DELAY = 500
POST_DELAY = 800
GM = 64
NZ = 5
PGM = 128
PGN = 128
PKM = 128
PKK = 256
EV0 = 0
EV1 = 0
EVT = 0
TRW = 256
TRM = 128
GN = 256
WK5 = 66
C6LN = (1000, 8900)
C6WK = (1500, 8900)
P1LN = (60, 11200)
P1WP = (6300, 10700)
P1WQ = (7300, 12200)
WQP = 5
EV2 = 300
P2U = (60, 2000)
LAG = 5
QFIN = False
HFIN = True
EV3 = 0
LN2_DELAY = 900
QP_DELAY = 400
GLAG = (None, None, None, 20, 8)

F32 = jnp.float32
BF16 = jnp.bfloat16
U32 = jnp.uint32
I32 = jnp.int32

XP = ((PB, 128), (PB + 128, 128), (PB + 256, 256), (0, TB), (TB, PB - TB))
WKP = ((0, 128), (128, 128), (256, 256), (512, 512))

SEM_X = 0
SEM_WK = SEM_X + len(XP)
SEM_WQ = SEM_WK + len(WKP)
SEM_W3 = SEM_WQ + 1
SEM_WR = SEM_W3 + 1
SEM_WGU = SEM_WR + 1
SEM_WD = SEM_WGU + 1
SEM_OUT = SEM_WD + 1
NSEM = SEM_OUT + 5

INT_MIN = -(2 ** 31)


def _layernorm(x, tok=None, w=None):
    s0 = x[:, 0:LANES]
    if tok is not None:
        s0 = s0 + jnp.concatenate([tok] * (x.shape[0] // 8), axis=0)
    for c in range(1, NC):
        s0 = s0 + x[:, c * LANES:(c + 1) * LANES]
    mu = jnp.sum(s0, axis=-1, keepdims=True) * (1.0 / D)
    xc = x - mu
    var = jnp.sum(xc * xc, axis=-1, keepdims=True) * (1.0 / D)
    rstd = lax.rsqrt(var + 1e-5)
    if w is None:
        return xc * rstd
    return xc * rstd, jnp.sum(xc * w, axis=-1, keepdims=True) * rstd


def _phi(t):
    return jnp.where(t > 0, t + 1.0, jnp.exp(t)) + 1e-6


def _n_off(a, b):
    return 32 * a + 8 * b


def _n_groups():
    pos = {(2 * o + e) * LANES + _n_off(a, b): (16 * e + 4 * b + a) * DH + 8 * o
           for o in range(4) for e in range(2) for a in range(4) for b in range(4)}
    return [pos[n] for n in sorted(pos)]


def _quads(b):
    h = len(b) // 2
    return [[r[j * h:(j + 1) * h] for r in b[i * h:(i + 1) * h]] for i in range(2) for j in range(2)]


def _badd(x, y):
    return [[a + b for a, b in zip(rx, ry)] for rx, ry in zip(x, y)]


def _bsub(x, y):
    return [[a - b for a, b in zip(rx, ry)] for rx, ry in zip(x, y)]


def _a_set(b):
    if len(b) == 1:
        return [b[0][0]]
    return [x for o in _a_ops(b) for x in _a_set(o)]


def _b_set(b):
    if len(b) == 1:
        return [b[0][0]]
    q11, q12, q21, q22 = _quads(b)
    ops = (_badd(q11, q22), q11, _bsub(q12, q22), _bsub(q21, q11), q22, _badd(q11, q12), _badd(q21, q22))
    return [x for o in ops for x in _b_set(o)]


def _b_in_a(i, levels):
    perm = (0, 2, 6, 5, 3, 4, 1)
    return sum(perm[(i // 7 ** l) % 7] * 7 ** l for l in range(levels))


def _strassen(prod, levels, base=0, fin=lambda k, q: q, init=None):
    if levels == 0:
        return [[prod(base)]]

    def m(i):
        return _strassen(prod, levels - 1, base * 7 + i)

    def seed(q, x):
        return x if init is None else _badd(_quads(init)[q], x)

    m2 = m(2)
    c22 = seed(3, m2)
    m4 = m(4)
    c12 = fin(1, _badd(seed(1, m2), m4))
    c11 = m4 if init is None else _bsub(_quads(init)[0], m4)
    m3 = m(3)
    c11 = _bsub(m3, c11) if init is None else _badd(c11, m3)
    m1 = m(1)
    c21 = fin(2, _badd(seed(2, m3), m1))
    c22 = _bsub(c22, m1)
    m0 = m(0)
    c11 = _badd(c11, m0)
    c22 = _badd(c22, m0)
    c11 = fin(0, _badd(c11, m(6)))
    c22 = fin(3, _badd(c22, m(5)))
    return [a + b for a, b in zip(c11, c12)] + [a + b for a, b in zip(c21, c22)]


def _goff(i, levels):
    return int(format(i, "0%db" % levels)[::-1], 2) if levels else 0


def _blocks(rows, n):
    w = rows[0].shape[1] // n
    return [[r[:, j * w:(j + 1) * w] for j in range(n)] for r in rows]


def _or_all(vals):
    acc = None
    for v in vals:
        v = pltpu.bitcast(v, U32)
        for g in range(v.shape[0] // 8):
            for c in range(v.shape[1] // LANES):
                p = v[g * 8:(g + 1) * 8, c * LANES:(c + 1) * LANES]
                acc = p if acc is None else acc | p
    return acc


def _raw_ops(levels):
    n = 2 ** levels
    names = [[_Tag((i, j)) for j in range(n)] for i in range(n)]
    return {op: t.ij for op, t in enumerate(_b_set(names)) if t.ij is not None}


class _Tag:
    def __init__(self, ij):
        self.ij = ij

    def __add__(self, other):
        return _Tag(None)

    __sub__ = __add__


def _a_ops(b):
    q11, q12, q21, q22 = _quads(b)
    return (_badd(q11, q22), _badd(q21, q22), q11, q22, _badd(q11, q12), _bsub(q21, q11), _bsub(q12, q22))


def _x_set(o):
    return _a_set(o) + ([] if LG == LA else [o[0][1], o[1][0]])


_A_FORM = (((0, 0), (1, 1), 1), ((1, 0), (1, 1), 1), ((0, 0),), ((1, 1),), ((0, 0), (0, 1), 1),
           ((1, 0), (0, 0), -1), ((0, 1), (1, 1), -1))
_B_FORM = (((0, 0), (1, 1), 1), ((0, 0),), ((0, 1), (1, 1), -1), ((1, 0), (0, 0), -1), ((1, 1),),
           ((0, 0), (0, 1), 1), ((1, 0), (1, 1), 1))


_C_FORM = (((0, 1), (3, 1), (4, -1), (6, 1)), ((2, 1), (4, 1)), ((1, 1), (3, 1)), ((0, 1), (1, -1), (2, 1), (5, 1)))


def _outer(form, get, n):
    h = n // 2

    def quad(q):
        return [[get(q[0] * h + i, q[1] * h + j) for j in range(h)] for i in range(h)]

    if len(form) == 1:
        return quad(form[0])
    return (_badd if form[2] > 0 else _bsub)(quad(form[0]), quad(form[1]))


def _x_slot(i):
    return i if LG == LA else (i // 7) * 9 + i % 7


def _merge(b):
    return jnp.concatenate([jnp.concatenate(r, axis=1) for r in b], axis=0)


def _gate(v, tok):
    u = pltpu.bitcast(v, U32)
    top = u[0:8, 0:LANES] | tok
    if u.shape[1] > LANES:
        top = jnp.concatenate([top, u[0:8, LANES:]], axis=1)
    return pltpu.bitcast(jnp.concatenate([top, u[8:, :]], axis=0) if u.shape[0] > 8 else top, BF16)


class _Pacer:
    def __init__(self, zero, every=0):
        self.zero, self.t, self.jobs, self.pend, self.tok = zero, 0, [], [], None
        self.every, self.last = every, -every

    def add(self, jobs, t0, t1, delay):
        for k, job in enumerate(jobs):
            self.jobs.append((t0 + k * (t1 - t0) // len(jobs), len(self.jobs), job, delay))
        self.jobs.sort(key=lambda e: e[:2])

    def due(self, dep, delay):
        if dep is not None:
            self.pend.append((self.t + delay, _or_all([dep])))

    def release(self, upto):
        while self.jobs and self.jobs[0][0] <= upto:
            _, _, job, delay = self.jobs.pop(0)
            self.due(job(self.tok), delay)

    def dot(self, lhs, rhs):
        self.release(self.t)
        ready = [d for t, d in self.pend if t <= self.t]
        if ready and self.t - self.last >= self.every:
            self.pend = [e for e in self.pend if e[0] > self.t]
            self.last = self.t
            lhs = _gate(lhs, _or_all(ready) & self.zero)
        res = jnp.dot(lhs, rhs, preferred_element_type=F32)
        self.t += lhs.shape[0] * (lhs.shape[1] // LANES) * (res.shape[1] // LANES) // 4
        self.tok = pltpu.bitcast(pltpu.bitcast(res[0:8, 0:LANES], U32) & self.zero, F32)
        return res

    def flush(self):
        self.release(1 << 30)


def _kernel(x_hbm, wqkv_hbm, wo_hbm, wr_hbm, wg_hbm, wu_hbm, wd_hbm, out_hbm,
            x_v, wk_v, wq_v, w3_v, wr_v, wgu_v, wd_v,
            ln1_v, xs_v, wks_v, pkt_v, pks_v, zacc_v, uacc_v, xw_v, g_v, gs_v, wqp_v, wqs_v, mp_v, ms_v, pq_v, pqn_v, pqs_v, attn_v, lo_v, lnf_v, zero_v,
            sems):

    ln2_v, out_v = lo_v.at[0], lo_v.at[1]

    wqkv_hbm, wo_hbm, wg_hbm, wu_hbm, wd_hbm = (r.bitcast(U32) for r in (wqkv_hbm, wo_hbm, wg_hbm, wu_hbm, wd_hbm))

    def wload(ref, r0, nr, cols):
        return pltpu.bitcast(ref[r0 // 2:(r0 + nr) // 2, cols], BF16)

    wv_v, wo_v = w3_v.at[0], w3_v.at[1]
    wg_v, wu_v = wgu_v.at[0], wgu_v.at[1]

    def x_copy(i):
        r0, n = XP[i]
        return pltpu.make_async_copy(x_hbm.at[pl.ds(r0, n), :], x_v.at[pl.ds(DEF + r0, n), :], sems.at[SEM_X + i])

    def out_copy(r0, n, s):
        return pltpu.make_async_copy(out_v.at[pl.ds(DEF + r0, n), :], out_hbm.at[pl.ds(r0, n), :],
                                     sems.at[SEM_OUT + s])

    def wk_copy(j):
        c0, n = WKP[j]
        return pltpu.make_async_copy(wqkv_hbm.at[:, pl.ds(D + c0, n)], wk_v.at[:, pl.ds(c0, n)],
                                     sems.at[SEM_WK + j])

    wq_copy = pltpu.make_async_copy(wqkv_hbm.at[:, pl.ds(0, D)], wq_v, sems.at[SEM_WQ])
    wr_copy = pltpu.make_async_copy(wr_hbm, wr_v, sems.at[SEM_WR])
    wd_copy = pltpu.make_async_copy(wd_hbm, wd_v.at[:, pl.ds(0, D)], sems.at[SEM_WD])
    wg_copy = pltpu.make_async_copy(wg_hbm, wg_v.at[:, pl.ds(0, F)], sems.at[SEM_WGU])
    wu_copy = pltpu.make_async_copy(wu_hbm, wu_v.at[:, pl.ds(0, F)], sems.at[SEM_WGU])

    x_copy(0).start()
    wk_copy(0).start()
    x_copy(1).start()
    wr_copy.start()
    for j in range(1, len(WKP)):
        wk_copy(j).start()
    for j in range(2, len(XP)):
        x_copy(j).start()
    wq_copy.start()
    pltpu.make_async_copy(wqkv_hbm.at[:, pl.ds(2 * D, D)], wv_v, sems.at[SEM_W3]).start()
    pltpu.make_async_copy(wo_hbm, wo_v, sems.at[SEM_W3]).start()
    wg_copy.start()
    wu_copy.start()
    wd_copy.start()

    def ln1_rows(xr, xr0, lnr, r0, n):
        ln = _layernorm(xr[xr0:xr0 + n, :].astype(F32)).astype(BF16)
        lnr[r0 // 2:(r0 + n) // 2, :] = pltpu.bitcast(ln, U32)

    def ln1_set(pc, xr, xr0, xsr, a0, n, t0, t1):
        def unit(j):
            def job(tok):
                ln = _layernorm(xr[xr0 + j * LNU:xr0 + (j + 1) * LNU, :].astype(F32), tok)
                lnf_v[j * LNU:(j + 1) * LNU, :] = ln
                return _or_all([ln[:, 0:LANES], ln[:, D - LANES:D]])
            return job

        def piece(j0, c0, o):
            def job(tok):
                def get(i, f):
                    r = (j0 + 2 * _goff(i, LA)) * LNU
                    v = lnf_v[r:r + 16, f * DA + c0:f * DA + c0 + LANES]
                    return v + jnp.concatenate([tok, tok], axis=0) if (i + f) % (NA // 2 + 1) == 0 else v

                r = (a0 + (j0 // (2 * NA)) * 16) // 2
                ops = _x_set(_outer(_A_FORM[o], get, NA))
                for op, v in enumerate(ops):
                    xsr.at[o * len(ops) + op][r:r + 8, c0:c0 + LANES] = pltpu.bitcast(v.astype(BF16), U32)
                return _or_all([v[0:8, :] for v in [ops[0]] + ops[5:7]])
            return job

        grp = 2 * NA
        ng = n // LNU // grp
        dt = (t1 - t0 - LN_DELAY) // (ng + 1)
        for g in range(ng):
            pc.add([unit(g * grp + j) for j in range(grp)], t0 + g * dt, t0 + (g + 1) * dt, LN_DELAY)
            s = t0 + (g + 1) * dt + LN_DELAY
            pc.add([piece(g * grp, c0, o) for c0 in range(0, DA, LANES) for o in range(7)], s, s + dt, JOB_DELAY)

    def ln1_load(lnr, r0, n):
        return pltpu.bitcast(lnr[r0 // 2:(r0 + n) // 2, :], BF16)

    def gate(v, tok):
        return v if tok is None else _gate(v, tok)

    def k_mm(r0, n, c0, nc):
        return jnp.dot(ln1_load(ln1_v, r0, n), wload(wk_v, 0, D, slice(c0, c0 + nc)), preferred_element_type=F32)

    def z_acc(pkts, c0, first=False):
        zs = None
        for pkt in pkts:
            for j in range(pkt.shape[1] // LANES):
                p = pkt[:, j * LANES:(j + 1) * LANES]
                zs = p if zs is None else zs + p
        if first:
            zacc_v[c0:c0 + zs.shape[0], :] = zs
        else:
            zacc_v[c0:c0 + zs.shape[0], :] += zs

    def k_post(k, p0, c0, first=False):
        n, nc = k.shape
        pkt = _phi(k).T
        pkt_v[c0 // 2:(c0 + nc) // 2, p0:p0 + n] = pltpu.bitcast(pkt.astype(BF16), U32)
        z_acc([pkt], c0, first)
        return pkt[nc - 8:nc, n - LANES:n]

    def g_acc(r0, n, c0, nc, first=False, pc=None):
        h, w = (nc, D) if pc is None else (min(nc, PGM), PGN)
        for f0 in range(c0, c0 + nc, h):
            for j0 in range(0, D, w):
                lhs = pltpu.bitcast(pkt_v[f0 // 2:(f0 + h) // 2, r0:r0 + n], BF16)
                rhs = pltpu.bitcast(ln1_v[r0 // 2:(r0 + n) // 2, j0:j0 + w], BF16)
                g = jnp.dot(lhs, rhs, preferred_element_type=F32) if pc is None else pc.dot(lhs, rhs)
                if first:
                    g_v[f0:f0 + h, j0:j0 + w] = g
                else:
                    g_v[f0:f0 + h, j0:j0 + w] += g

    def k_paced(pc, r0, c0, nc, first):
        for j0 in range(c0, c0 + nc, LANES):
            for t0 in range(r0, r0 + TX, PKM):
                k = None
                for k0 in range(0, D, PKK):
                    p = pc.dot(ln1_load(ln1_v, t0, PKM)[:, k0:k0 + PKK], wload(wk_v, k0, PKK, slice(j0, j0 + LANES)))
                    k = p if k is None else k + p
                pc.due(k_post(k, t0, j0, first and t0 == r0), POST_DELAY)

    attn_v[...] = jnp.zeros_like(attn_v)
    zero_v[...] = jnp.zeros_like(zero_v)

    def gs_zero(o0, o1):
        gs_v[o0:o1] = jnp.zeros((o1 - o0, HD, HD), F32)

    x_copy(0).wait()
    ln1_rows(x_v, DEF + PB, ln1_v, 0, 128)
    gs_zero(0, 1)
    wk_copy(0).wait()
    ka = k_mm(0, 128, 0, 128)
    gs_zero(1, 2)
    x_copy(1).wait()
    wr_copy.wait()
    gs_zero(2, 3)
    ln1_rows(x_v, DEF + PB + 128, ln1_v, 128, 128)
    k_post(ka, 0, 0, first=True)
    g_acc(0, 128, 0, 128, first=True)
    wk_copy(1).wait()
    gs_zero(3, NZ)
    k_post(k_mm(128, 128, 0, 128), 128, 0)
    k_post(k_mm(0, TX, 128, 128), 0, 128, first=True)
    g_acc(128, 128, 0, 128)
    def w_job(src_ref, dst_ref, levels, r0, c0, o):
        n = 2 ** levels
        w, raw, inner = D // n, _raw_ops(levels), 7 ** (levels - 1)

        def job(tok):
            def cut(i, j):
                return src_ref[(i * w + r0) // 2:(i * w + r0) // 2 + 8, j * w + c0:j * w + c0 + LANES]

            def get(i, j):
                u = cut(i, j)
                return pltpu.bitcast(u if tok is None else u | pltpu.bitcast(tok, U32), BF16).astype(F32)

            ops = []
            for op, v in enumerate(_b_set(_outer(_B_FORM[o], get, n))):
                dst = dst_ref.at[o * inner + op]
                if o * inner + op in raw:
                    dst[r0 // 2:r0 // 2 + 8, c0:c0 + LANES] = cut(*raw[o * inner + op])
                else:
                    dst[r0 // 2:r0 // 2 + 8, c0:c0 + LANES] = pltpu.bitcast(v.astype(BF16), U32)
                    ops.append(v)
            return _or_all(ops[0:1] + ops[-2:]) if ops else None
        return job

    def wk_jobs_of(outer):
        return [w_job(wk_v, wks_v, LK, r0, c0, o) for r0 in range(0, DK, 16) for c0 in range(0, DK, LANES)
                for o in outer]

    wk_copy(2).wait()
    pc = _Pacer(zero_v[...], EV0)
    pc.add(wk_jobs_of((1, 3)), 500, 2200, JOB_DELAY)
    k_paced(pc, 0, 256, 256, True)
    g_acc(0, TX, 128, 128, True, pc)
    g_acc(0, TX, 256, 256, True, pc)
    pc.flush()
    wk_copy(3).wait()
    wk_jobs = wk_jobs_of((0, 2, 4, 5, 6))
    pc = _Pacer(zero_v[...], EV0)
    pc.add(wk_jobs[:WK5], 500, 2700, JOB_DELAY)
    k_paced(pc, 0, 512, 512, True)
    g_acc(0, TX, 512, 256, True, pc)
    pc.flush()
    x_copy(2).wait()
    x_copy(3).wait()
    pc = _Pacer(zero_v[...], EV0)
    ln1_set(pc, x_v, DEF, xs_v, 0, TB, *C6LN)
    pc.add(wk_jobs[WK5:], *C6WK, JOB_DELAY)
    ln1_rows(x_v, DEF + PB + TX, ln1_v, TX, TX)
    g_acc(0, TX, 768, 256, True, pc)
    k_paced(pc, TX, 0, D, False)
    for c0 in range(0, D, 256):
        g_acc(TX, TX, c0, 256, False, pc)
    pc.flush()

    MA = TB // NA
    MG = TB // NG
    NS = NK // NG

    def xs_load(xsr, op, a0, m, cols=slice(None)):
        return pltpu.bitcast(xsr[op, a0 // 2:(a0 + m) // 2, cols], BF16)

    def k_step(pc, xsr, j0):
        def fin(_, q):
            if NS > 1:
                q = [[jnp.concatenate([_phi(jnp.concatenate([r[f] for r in q], axis=0)).T for f in range(NS)],
                                      axis=0)]]
            else:
                q = [[_phi(v).T for v in r] for r in q]
            pc.due(_or_all([v[t - 8:t, :] for r in q for v in r for t in range(LANES, v.shape[0] + 1, LANES)]),
                   POST_DELAY)
            return q

        def lhs(i):
            if LK == LA:
                return xs_load(xsr, _x_slot(i), 0, MA)
            return _merge([[xs_load(xsr, i * 9 + s, 0, MA) for s in r] for r in ((2, 7), (8, 3))])

        cb = _strassen(lambda i: pc.dot(lhs(i), pltpu.bitcast(wks_v[i, :, j0:j0 + LANES], BF16)), LK, fin=fin)
        ops = _a_ops([[cb[i][f] for i in range(NG)] for f in range(NG)])
        for half, o in ((0, ops[4]), (1, ops[1])):
            for f, rowb in enumerate(o):
                for s in range(NS):
                    z_acc([v[s * LANES:(s + 1) * LANES, :] for v in rowb], half * HD + f * DG + s * DK + j0)
        for _ in range(LG - 1):
            ops = [o for x in ops for o in _a_ops(x)]
        for op, o in enumerate(ops):
            r = j0 * NS
            pks_v[r // 2:(r + NS * LANES) // 2, op * MG:(op + 1) * MG] = pltpu.bitcast(o[0][0].astype(BF16), U32)
        pc.due(_or_all([o[0][0][NS * LANES - 8:NS * LANES, :] for o in (ops[0], ops[-1], ops[-2])]), 2 * POST_DELAY)

    def g_rhs(xsr, i, c0, nc):
        o = _b_in_a(i, LG)
        if LG == LA:
            return xs_load(xsr, o, 0, MA, slice(c0, c0 + nc))
        j, cs = c0 // DA, slice(c0 % DA, c0 % DA + nc)
        return jnp.concatenate([xs_load(xsr, o * 9 + s, 0, MA, cs) for s in ((2, 8), (7, 3))[j]], axis=0)

    def g_step(pc, xsr, r0, nr, c0, nc, later):
        def old(o, f, c):
            v = gs_v[o, f * DG + r0:f * DG + r0 + nr, c * DG + c0:c * DG + c0 + nc]
            return v if o < NZ else jnp.where(later, v, 0.0)

        for o in range(7):
            cb = _strassen(lambda i: pc.dot(pltpu.bitcast(pks_v[r0 // 2:(r0 + nr) // 2, i * MG:(i + 1) * MG], BF16),
                                            g_rhs(xsr, i, c0, nc)), LG - 1, base=o,
                           init=[[old(o, f, c) for c in range(NG // 2)] for f in range(NG // 2)])
            for f in range(NG // 2):
                for c in range(NG // 2):
                    gs_v[o, f * DG + r0:f * DG + r0 + nr, c * DG + c0:c * DG + c0 + nc] = cb[f][c]

    def wq_jobs(u0, nr):
        span = (NA - 1) * DA + 16 * nr
        u0 = u0 if isinstance(u0, int) else pl.multiple_of(u0, 8)
        srcr, permr = wq_v.at[pl.ds(u0, span // 2), :], wqp_v.at[pl.ds(u0, span // 2), :]
        dstr = wqs_v.at[:, pl.ds(u0, 8 * nr), :]
        oct_ = (lax.broadcasted_iota(I32, (8, LANES), 1) % DH) // 8

        def perm(r, e):
            def job(tok):
                blk = [srcr[r // 2:r // 2 + 8, (4 * e + b) * LANES:(4 * e + b + 1) * LANES] | pltpu.bitcast(tok, U32)
                       for b in range(4)]
                outs = []
                for o in range(4):
                    v = blk[o]
                    for b in range(4):
                        if b != o:
                            v = jnp.where(oct_ == b, pltpu.roll(blk[b], (8 * (b - o)) % LANES, 1), v)
                    permr[r // 2:r // 2 + 8, (2 * o + e) * LANES:(2 * o + e + 1) * LANES] = v
                    outs.append(v)
                return _or_all(outs)
            return job

        return ([perm(i * DA + r0, e) for r0 in range(0, 16 * nr, 16) for i in range(NA) for e in range(2)],
                [w_job(permr, dstr, LA, r0, c0, o) for r0 in range(0, 16 * nr, 16)
                 for c0 in range(0, DA, LANES) for o in range(7)])

    def p1(i, carry):
        xsr = xs_v.at[:, pl.ds(pl.multiple_of(i * (MA // 2), MA // 2), MA), :]
        xr = x_v.at[pl.ds(pl.multiple_of((i + 1) * TB, TB), TB + DEF), :]

        pc = _Pacer(zero_v[...], EV1)
        ln1_set(pc, xr, DEF, xsr, MA, TB, *P1LN)
        perms, sets = wq_jobs(i * (8 * WQP), WQP)
        pc.add(perms, *P1WP, JOB_DELAY)
        pc.add(sets, *P1WQ, JOB_DELAY)
        for j0 in range(0, DK, LANES):
            k_step(pc, xsr, j0)
        for f0 in range(0, DG, GM):
            for c0 in range(0, DG, GN):
                g_step(pc, xsr, f0, GM, c0, GN, i > 0)
        pc.flush()
        return carry

    x_copy(4).wait()
    wq_copy.wait()
    lax.fori_loop(0, NB1, p1, 0)

    pltpu.make_async_copy(w3_v, w3_v, sems.at[SEM_W3]).wait()
    zero_u = zero_v[...]
    def row_vector(acc_ref):
        return jnp.sum(jnp.concatenate([acc_ref[r:r + 8, :] for r in _n_groups()], axis=0).T, axis=0, keepdims=True)

    zrow = row_vector(zacc_v)
    wr8 = wr_v[...].astype(F32)
    wr_row = jnp.concatenate([wr8[c:c + 1, :] for c in range(NC)], axis=1)

    row_h = lax.broadcasted_iota(I32, (LANES, LANES), 0) // DH
    col_h = lax.broadcasted_iota(I32, (LANES, LANES), 1) // DH
    diag = row_h == col_h

    def colsum(t):
        acc = t[:, 0:LANES]
        for c in range(1, NC):
            acc = acc + t[:, c * LANES:(c + 1) * LANES]
        return acc

    wrc = wr_row - jnp.sum(wr_row, axis=-1, keepdims=True) * (1.0 / D)
    m_raw = _raw_ops(LO)

    def kv_part(c):
        cs = slice(c * LANES, (c + 1) * LANES)
        kv = None
        for k0 in range(0, D, TRW):
            g = g_v[cs, k0:k0 + TRW]
            for o, sign in _C_FORM[(c * LANES // HD) * 2 + k0 // HD]:
                t = gs_v[o, c * LANES % HD:c * LANES % HD + LANES, k0 % HD:k0 % HD + TRW]
                g = g + t if sign > 0 else g - t
            p = pc.dot(g.astype(BF16), wload(wv_v, k0, TRW, cs))
            kv = p if kv is None else kv + p
        return jnp.where(diag, kv, 0.0)

    def m_part(c, kvs):
        e, b = c // 4, c % 4
        for j0 in range(0, DO, TRM):
            ms = [jnp.concatenate(
                [pc.dot(kv, wload(wo_v, (c + k) * LANES, LANES, slice(f * DO + j0, f * DO + j0 + TRM)))
                 for f in range(NO)], axis=1) for k, kv in enumerate(kvs)]
            deps = []
            for a in range(4):
                rows = [jnp.concatenate([m[a * DH + 8 * o:a * DH + 8 * o + 8, :] for m in ms], axis=0)
                        for o in range(4)]
                for o in range(4):
                    r = ((2 * o + e) * LANES + _n_off(a, b)) // 2
                    for f in range(NO):
                        mp_v[r:r + 8, f * DO + j0:f * DO + j0 + TRM] = pltpu.bitcast(
                            rows[o][:, f * TRM:(f + 1) * TRM].astype(BF16), U32)
                for t in range(4 // NO):
                    r = ((2 * t + e) * LANES + _n_off(a, b)) // 2
                    for op, v in enumerate(_b_set(_blocks(rows[t::4 // NO], NO))):
                        if op not in m_raw:
                            ms_v.at[op][r:r + 8, j0:j0 + TRM] = pltpu.bitcast(v.astype(BF16), U32)
                            deps.append(v[0:8, 0:LANES])
            pc.due(_or_all(deps[::4]), POST_DELAY)

    pc = _Pacer(zero_u, EVT)
    pc.due(jnp.broadcast_to(zrow, (8, D)), 1000)
    perms, sets = wq_jobs(NB1 * 8 * WQP, DA // 16 - NB1 * WQP)
    pc.add(perms, 60, 700, JOB_DELAY)
    pc.add(sets, 1300, 3400, JOB_DELAY)
    kv_prev = None
    for c in range(0, NC + 2, 2):
        kvs = [kv_part(c).astype(BF16), kv_part(c + 1).astype(BF16)] if c < NC else None
        if c:
            m_part(c - 2, kv_prev)
        kv_prev = kvs
    pc.flush()

    def make_key(score, row):
        b = pltpu.bitcast(score, I32)
        srt = b ^ ((b >> 31) & 0x7FFFFFFF)
        return (srt & jnp.int32(-65536)) | (0xFFFF - row)

    def push_keys(key, top1, top2):
        for gidx in range(key.shape[0] // 8):
            kx = key[gidx * 8:(gidx + 1) * 8, :]
            top2 = jnp.maximum(top2, jnp.minimum(top1, kx))
            top1 = jnp.maximum(top1, kx)
        return top1, top2

    lane = lax.broadcasted_iota(I32, (1, LANES), 1)

    def interleave(parts):
        return jnp.concatenate([p[g * 16:(g + 1) * 16, :] for g in range(parts[0].shape[0] // 16) for p in parts],
                               axis=0)

    def q_part(pc, xsr, l0, r0, n, hint=None):
        m = n // NA
        sums = {}

        def park(v, g, c):
            for t in range(m // 16):
                r = r0 + (t * NA + g) * 16
                pq_v[r:r + 16, c * LANES:(c + 1) * LANES] = v[t * 16:(t + 1) * 16, :]

        def fin(k, q):
            q = [[_phi(v) for v in r] for r in q]
            deps = []
            for a, r in enumerate(q):
                for b, v in enumerate(r):
                    i, c = (k // 2) * (NA // 2) + a, (((k % 2) * (NA // 2) + b) * DA + j0) // LANES
                    park(v, _goff(i, LA), c)
                    for name, row in (("z", zrow),) + ((("u", hint["u"]),) if hint else ()):
                        t = v * row[:, c * LANES:(c + 1) * LANES]
                        key = (name, _goff(i, LA), c % 2)
                        sums[key] = t if key not in sums else sums[key] + t
                deps.append(sums[key])
            if (r0 + n < RL or HFIN) if hint else QFIN:
                pc.due(_or_all(deps), POST_DELAY)
            return q

        for j0 in range(0, DA, LANES):
            _strassen(lambda i: pc.dot(xs_load(xsr, _x_slot(i), (l0 + r0) // NA, m),
                                       pltpu.bitcast(wqs_v[i, :, j0:j0 + LANES], BF16)), LA, fin=fin)
        if hint:
            pc.flush()
        den = jnp.concatenate([sums["z", g, e] for g in range(NA) for e in range(2)], axis=0)
        for s in (1, 2, 4):
            den = den + jnp.where((lane & s) == 0, pltpu.roll(den, LANES - s, 1), pltpu.roll(den, s, 1))
        inv_all = 1.0 / (den + 1e-6)

        def inv_of(g):
            return [inv_all[(g * 2 + e) * m:(g * 2 + e + 1) * m, :] for e in range(2)]

        for g in range(NA):
            for e in range(2):
                park(inv_of(g)[e], g, NC + e)
        if hint:
            for g in range(NA):
                starts = [r0 + (t * NA + g) * 16 for t in range(m // 16)]
                num = jnp.sum(jnp.concatenate([xw_v[t:t + 16, :] for t in starts], axis=0)
                              + sums["u", g, 0] * inv_of(g)[0] + sums["u", g, 1] * inv_of(g)[1],
                              axis=-1, keepdims=True)
                row = jnp.concatenate([(l0 + t) + lax.broadcasted_iota(I32, (16, 1), 0) for t in starts], axis=0)
                hint["p1"], hint["p2"] = push_keys(make_key(num, row), hint["p1"], hint["p2"])
            pc.due(jnp.broadcast_to(hint["p1"], (8, LANES)), 1200)


    def post_jobs(r0, n, plain=False):
        def scaled(t, c0, w, tok):
            inv = pq_v[t:t + 16, D:D + 2 * LANES]
            if tok is not None:
                inv = inv + jnp.concatenate([jnp.concatenate([tok, tok], axis=0)] * 2, axis=1)
            return pq_v[t:t + 16, c0:c0 + w] * jnp.concatenate([inv] * (w // (2 * LANES)), axis=1)

        def post_plain(t):
            def job(tok):
                v = scaled(t, 0, D, tok)
                pqn_v[t // 2:t // 2 + 8, :] = pltpu.bitcast(v.astype(BF16), U32)
                return v[0:8, 0:LANES]
            return job

        def post(t0, outer):
            def job(tok):
                deps = []
                for c0 in range(0, DO, 2 * LANES):
                    blk = {}

                    def get(i, f):
                        if (i, f) not in blk:
                            blk[i, f] = scaled(t0 + _goff(i, LO) * 16, f * DO + c0, 2 * LANES, tok)
                        return blk[i, f]

                    for o in outer:
                        ops = _a_set(_outer(_A_FORM[o], get, NO))
                        for op, v in enumerate(ops):
                            pqs_v.at[o * len(ops) + op][t0 // NO // 2:t0 // NO // 2 + 8, c0:c0 + 2 * LANES] = (
                                pltpu.bitcast(v.astype(BF16), U32))
                        deps.append(ops[0][0:8, 0:LANES])
                return _or_all(deps)
            return job

        if plain:
            return [post_plain(t) for t in range(r0, r0 + n, 16)]
        outers = [range(7)] if LO == 1 else [(o,) for o in range(7)]
        return [post(t0, outer) for t0 in range(r0, r0 + n, 16 * NO) for outer in outers]

    def m_operand(i, c0, c1):
        if i not in m_raw:
            return pltpu.bitcast(ms_v[i, :, c0 * LANES:c1 * LANES], BF16)
        bi, bj = m_raw[i]
        return wload(mp_v, bi * DO, DO, slice(bj * DO + c0 * LANES, bj * DO + c1 * LANES))

    def o_part(dot, xr, x0, r0, n):
        a0, m = r0 // NO, n // NO
        nw = LANES * NO // 2
        cols = [[[] for _ in range(NO)] for _ in range(NO)]
        for c0 in range(0, DO, nw):
            init = [[jnp.concatenate(
                [xr[x0 + r0 + (g * NO + _goff(i, LO)) * 16:x0 + r0 + (g * NO + _goff(i, LO) + 1) * 16,
                    f * DO + c0:f * DO + c0 + nw] for g in range(m // 16)], axis=0).astype(F32)
                for f in range(NO)] for i in range(NO)]
            cb = _strassen(lambda i: dot(pltpu.bitcast(pqs_v[i, a0 // 2:(a0 + m) // 2, :], BF16),
                                         m_operand(i, c0 // LANES, (c0 + nw) // LANES)), LO, init=init)
            for i in range(NO):
                for f in range(NO):
                    cols[i][f].append(cb[i][f])
        parts = [None] * NO
        for i in range(NO):
            parts[_goff(i, LO)] = jnp.concatenate([c for f in range(NO) for c in cols[i][f]], axis=1)
        return interleave(parts)

    def ln2_unit(h, l2r, outr, r0, row0, valid, top1, top2, tok, fast=False):
        n = h.shape[0]
        if fast:
            ln2, r = _layernorm(h, tok, wr_row)
        else:
            ln2 = _layernorm(h, tok)
            r = jnp.sum(ln2 * wr_row, axis=-1, keepdims=True)
        l2r[r0:r0 + n, :] = ln2.astype(BF16)
        res = h + ln2
        outr[r0:r0 + n, :] = res.astype(BF16)
        r = r.astype(BF16).astype(F32) + 0.0
        key = make_key(r, (row0 + r0) + lax.broadcasted_iota(I32, (n, 1), 0))
        if valid is not None:
            key = jnp.where(valid, key, INT_MIN)
        top1, top2 = push_keys(key, top1, top2)
        ntok = pltpu.bitcast(pltpu.bitcast(jnp.broadcast_to(r[n - 8:n, :], (8, LANES)), U32) & zero_u, F32)
        return top1, top2, ntok

    def ln2_jobs(h, l2r, outr, r0, row0, valid, st, fast=False):
        def unit(j):
            def job(tok):
                st["top1"], st["top2"], dep = ln2_unit(h[j * LNU:(j + 1) * LNU, :], l2r, outr, r0 + j * LNU, row0,
                                                       valid, st["top1"], st["top2"], tok, fast)
                return dep
            return job
        return [unit(j) for j in range(h.shape[0] // LNU)]

    QC = 16 * 7 ** LA / 8 ** LA
    OC = 16 * 7 ** LO / 8 ** LO

    def p2(i, carry):
        st = dict(top1=carry[0], top2=carry[1])
        b0 = pl.multiple_of(i * TB2, 16)
        xsr = xs_v.at[:, pl.ds(pl.multiple_of(i * (TB2 // NA // 2), 8), TB2 // NA // 2), :]
        xr = x_v.at[pl.ds(b0, TB2 + DEF), :]
        l2r = ln2_v.at[pl.ds(b0, TB2 + DEF), :]
        outr = out_v.at[pl.ds(b0, TB2 + DEF), :]
        row0 = b0 - DEF
        pc = _Pacer(zero_u)
        toks = []

        def chain(jobs):
            for job in jobs:
                toks.append(job(toks[-LAG] if len(toks) >= LAG else None))

        chain(ln2_jobs(attn_v, l2r, outr, 0, row0, i > 0, st))

        @pl.when(i > 0)
        def _():
            out_copy(pl.multiple_of((i - 1) * TB2, 16), TB2, 0).start()

        pc.due(toks[-1], QA * QC)

        nu, nx = D // NB2, RL // NB2
        mr = mp_v.at[pl.ds(pl.multiple_of(i * (nu // 2), 8), nu // 2), :]
        ur = uacc_v.at[pl.ds(pl.multiple_of(i * nu, 8), nu), :]
        xl = x_v.at[pl.ds(pl.multiple_of(DEF + L0 + i * nx, 16), nx), :]
        xwr = xw_v.at[pl.ds(pl.multiple_of(i * nx, 8), nx), :]

        def hint_job(load, dst, r):
            def job(tok):
                v = colsum(load(r).astype(F32) * wrc) + jnp.concatenate([tok, tok], axis=0)
                dst[r:r + 16, :] = v
                return v
            return job

        pc.add([hint_job(lambda r: wload(mr, r, 16, slice(None)), ur, r) for r in range(0, nu, 16)]
               + [hint_job(lambda r: xl[r:r + 16, :], xwr, r) for r in range(0, nx, 16)], *P2U, JOB_DELAY)
        for r0, n in ((0, QA), (QA, TB2 - QA)):
            q_part(pc, xsr, 0, r0, n)
            for job in post_jobs(r0, n):
                job(None)
        r0 = 0
        for n in OCH[:-1]:
            chain(ln2_jobs(o_part(pc.dot, xr, DEF, r0, n), l2r, outr, DEF + r0, row0, None, st))
            r0 += n
        attn_v[...] = o_part(pc.dot, xr, DEF, r0, DEF)
        return st["top1"], st["top2"]

    init = jnp.full((8, 1), INT_MIN, I32)
    top1, top2 = lax.fori_loop(0, NB2, p2, (init, init))

    wg_copy.wait()
    wu_copy.wait()
    wd_copy.wait()
    sub8 = lax.broadcasted_iota(I32, (8, LANES), 0)
    urow = jnp.sum(uacc_v[...].T, axis=0, keepdims=True)

    def submax(v):
        for sh in (4, 2, 1):
            v = jnp.maximum(v, pltpu.roll(v, sh, 0))
        return v

    def subsum(v):
        for sh in (4, 2, 1):
            v = v + pltpu.roll(v, sh, 0)
        return v

    def best2(t1, t2):
        t1 = jnp.broadcast_to(t1, (8, LANES))
        t2 = jnp.broadcast_to(t2, (8, LANES))
        k1v = submax(t1)
        return k1v, submax(jnp.where(t1 == k1v, t2, t1))

    def key_row(k):
        return 0xFFFF - (k & 0xFFFF)

    def wide(m):
        return jnp.concatenate([m] * NC, axis=1)

    st = dict(top1=top1, top2=top2, pend=[], step=0, sent=0)
    pc = _Pacer(zero_u, EV2)
    hint = dict(u=urow, p1=init, p2=init)

    pc.add(ln2_jobs(attn_v, ln2_v, out_v, L0, -DEF, None, st), 60, QS[0] * QC - 600, LN2_DELAY)
    r0 = 0
    for k, n in enumerate(QS):
        q_part(pc, xs_v, L0, r0, n, hint)
        if k == 0:
            out_copy(L0 - TB2, TB2, 0).start()
            top1, top2 = st["top1"], st["top2"]
            pc.add(post_jobs(0, OCL[0][0], OCL[0][1]), pc.t + 600, pc.t + (RL - n) * QC - 300, QP_DELAY)
        r0 += n
    pc.every = EV3
    oldk = best2(top1, top2)
    oldx = []
    for kk in oldk:
        g8 = pl.multiple_of(((jnp.clip(key_row(kk[0, 0]), 0, S - 1) >> 3) << 3) + DEF, 8)
        rows = ln2_v[pl.ds(g8, 8), :].astype(F32)
        oldx.append(subsum(jnp.where(wide((key_row(kk) & 7) == sub8), rows, 0.0)))

    def gated(v):
        tok = None
        while st["pend"] and st["pend"][0][0] <= st["step"]:
            t = st["pend"].pop(0)[1]
            tok = t if tok is None else tok | t
        if tok is None:
            return v
        u = pltpu.bitcast(v, U32)
        return pltpu.bitcast(jnp.concatenate([u[:, 0:LANES] | tok, u[:, LANES:]], axis=1), BF16)

    res = {}

    def c_units():
        pc.flush()
        p1, p2_ = hint["p1"], hint["p2"]
        cand_p, cand_x = [], []
        for pk_ in (p1, p2_):
            cp, cx = None, None
            for s in range(8):
                g8 = pl.multiple_of((jnp.clip(key_row(pk_[s, 0]) - L0, 0, RL - 1) >> 3) << 3, 8)
                vp = pq_v[pl.ds(g8, 8), :]
                vx = x_v[pl.ds(pl.multiple_of(g8 + (L0 + DEF), 8), 8), :].astype(F32)
                cp = vp if cp is None else jnp.where(jnp.concatenate([sub8 == s] * (NC + 2), axis=1), vp, cp)
                cx = vx if cx is None else jnp.where(wide(sub8 == s), vx, cx)
            cand_p.append(cp[:, 0:D] * jnp.concatenate([cp[:, D:]] * (NC // 2), axis=1))
            cand_x.append(cx)
        cand_p = jnp.concatenate(cand_p, axis=0).astype(BF16)
        cand_x = jnp.concatenate(cand_x, axis=0)
        ids_lo = key_row(jnp.broadcast_to(p1, (8, LANES)))
        ids_hi = jnp.where(sub8 < 6, key_row(jnp.broadcast_to(p2_, (8, LANES))),
                           jnp.where(sub8 == 6, key_row(oldk[0]), key_row(oldk[1])))
        res["ids"] = (ids_lo, ids_hi)
        parts = []
        for c in range(NC):
            parts.append(jnp.dot(cand_p, wload(mp_v, 0, D, slice(c * LANES, (c + 1) * LANES)), preferred_element_type=F32))
            yield
        xs = _layernorm(cand_x + jnp.concatenate(parts, axis=1))
        hi = jnp.where(wide(sub8 < 6), xs[8:16, :], jnp.where(wide(sub8 == 6), oldx[0], oldx[1]))
        res["xs"] = jnp.concatenate([xs[0:8, :], hi], axis=0).astype(BF16)

    def f_units():
        xs = res["xs"]
        acts = []
        for j in range(F // LANES):
            cs = slice(j * LANES, (j + 1) * LANES)
            g = jnp.dot(gated(xs), wload(wg_v, 0, D, cs), preferred_element_type=F32)
            yield
            u = jnp.dot(xs, wload(wu_v, 0, D, cs), preferred_element_type=F32)
            acts.append((g * jax.nn.sigmoid(g) * u).astype(BF16))
            yield
        act = jnp.concatenate(acts, axis=1)
        zf = pltpu.bitcast(zero_u, F32)
        ys = []
        KF = (F // D) * D
        for c in range(0, NC, 2):
            acc = jnp.concatenate([jnp.concatenate([zf, zf], axis=0)] * 2, axis=1)
            acc = acc + jnp.dot(gated(act[:, KF:]), wload(wd_v, KF, F - KF, slice(c * LANES, (c + 2) * LANES)),
                                preferred_element_type=F32)
            yield
            for cc in range(2):
                y = acc[:, cc * LANES:(cc + 1) * LANES]
                for k0 in range(0, KF, D):
                    y = y + jnp.dot(gated(act[:, k0:k0 + D]),
                                    wload(wd_v, k0, D, slice((c + cc) * LANES, (c + cc + 1) * LANES)),
                                    preferred_element_type=F32)
                    yield
                ys.append(y)
        res["y"] = jnp.concatenate(ys, axis=1)

    def side_units():
        yield from range(NPRE)
        yield from c_units()
        yield from range(NGAP)
        yield from f_units()

    side = side_units()

    def o_dot(lhs, rhs):
        p = pc.dot(lhs, rhs) if st["step"] < NPRE else jnp.dot(lhs, rhs, preferred_element_type=F32)
        next(side, None)
        st["step"] += 1
        return p

    def o_plain(r0, n):
        lhs = pltpu.bitcast(pqn_v[r0 // 2:(r0 + n) // 2, :], BF16)
        parts = []
        for c0 in range(0, NC, 2):
            acc = x_v[DEF + L0 + r0:DEF + L0 + r0 + n, c0 * LANES:(c0 + 2) * LANES].astype(F32)
            for k0 in range(0, D, 2 * LANES):
                acc = acc + o_dot(lhs[:, k0:k0 + 2 * LANES], wload(mp_v, k0, 2 * LANES, slice(c0 * LANES, (c0 + 2) * LANES)))
            parts.append(acc)
        return jnp.concatenate(parts, axis=1)

    toks = []
    r0 = 0
    pc.add(post_jobs(OCL[0][0], *OCL[1]), pc.t + 200, pc.t + 1000, QP_DELAY)
    for ci, (n, plain) in enumerate(OCL):
        h = o_plain(r0, n) if plain else o_part(o_dot, x_v, DEF + L0, r0, n)
        last = r0 + n == RL
        units = ln2_jobs(h, ln2_v, out_v, DEF + L0 + r0, -DEF, None, st, fast=last)
        posts = post_jobs(r0 + n + OCL[ci + 1][0], *OCL[ci + 2]) if ci + 2 < len(OCL) else []
        for k, job in enumerate(units):
            toks.append(job(toks[-LAG_L] if len(toks) >= LAG_L and not last else None))
            if posts:
                posts.pop(0)(toks[-1])
        if GLAG[ci] is not None:
            st["pend"].append((st["step"] + GLAG[ci],
                               pltpu.bitcast(jnp.broadcast_to(st["top1"], (8, LANES)), U32) & zero_u))
        r0 += n
        if last or r0 in OUT_AT:
            out_copy(L0 + st["sent"], r0 - st["sent"], 2 if last else 1).start()
            if not last:
                st["sent"] = r0
    for _ in side:
        st["step"] += 1

    keyv = best2(st["top1"], st["top2"])
    idx = [jnp.clip(key_row(kk[0, 0]), 0, S - 1) for kk in keyv]
    grp = [pl.multiple_of((ii >> 3) << 3, 8) for ii in idx]
    vgrp = [pl.multiple_of(gg + DEF, 8) for gg in grp]
    y = res["y"]
    ids_lo, ids_hi = res["ids"]
    hits = None
    yrows = []
    for c in range(2):
        m_lo = ids_lo == key_row(keyv[c])
        m_hi = ids_hi == key_row(keyv[c])
        yrows.append(subsum(jnp.where(wide(m_lo), y[0:8, :], 0.0) + jnp.where(wide(m_hi), y[8:16, :], 0.0)))
        hit = submax(jnp.where(m_lo | m_hi, 1, 0))
        hits = hit if hits is None else hits + hit
    hit_all = hits[0, 0] == 2

    tail0 = L0 + st["sent"]
    tail_copy = out_copy(tail0, S - tail0, 2)
    in_tail = jnp.maximum(grp[0], grp[1]) >= tail0
    two_groups = grp[1] != grp[0]

    def fix_copy(c):
        return out_copy(grp[c], 8, 3 + c)

    def finish(ysel):
        for c in range(2):
            hi = keyv[c] & jnp.int32(-65536)
            score = pltpu.bitcast(hi ^ ((hi >> 31) & 0x7FFF0000), F32)
            sel = (key_row(keyv[c]) & 7) == sub8
            upd = jnp.where(wide(sel), ysel[c] * wide(jax.nn.sigmoid(score)), 0.0)
            out_v[pl.ds(vgrp[c], 8), :] = (out_v[pl.ds(vgrp[c], 8), :].astype(F32) + upd).astype(BF16)
        fix_copy(0).start()

        @pl.when(two_groups)
        def _():
            fix_copy(1).start()

    out_copy(0, L0, 0).wait()
    out_copy(L0, tail0 - L0, 1).wait()

    @pl.when(in_tail)
    def _():
        tail_copy.wait()

    @pl.when(hit_all)
    def _():
        finish(yrows)

    @pl.when(jnp.logical_not(hit_all))
    def _():
        xsel = jnp.concatenate([ln2_v[pl.ds(vgrp[c], 8), :] for c in range(2)], axis=0)

        def ffn_tile(j, acc):
            cs = pl.ds(pl.multiple_of(j * LANES, LANES), LANES)
            g = jnp.dot(xsel, wload(wg_v, 0, D, cs), preferred_element_type=F32)
            u = jnp.dot(xsel, wload(wu_v, 0, D, cs), preferred_element_type=F32)
            a = (g * jax.nn.sigmoid(g) * u).astype(BF16)
            wd_t = pltpu.bitcast(wd_v[pl.ds(pl.multiple_of(j * (LANES // 2), LANES // 2), LANES // 2), 0:D], BF16)
            return acc + jnp.dot(a, wd_t, preferred_element_type=F32)

        yf = lax.fori_loop(0, F // LANES, ffn_tile, jnp.zeros((16, D), F32))
        finish([yf[0:8, :], yf[8:16, :]])

    @pl.when(jnp.logical_not(in_tail))
    def _():
        tail_copy.wait()

    fix_copy(0).wait()

    @pl.when(two_groups)
    def _():
        fix_copy(1).wait()


@jax.jit
def pallas_sequential_preLN__linear_attn_block__moe_arch_mod__prompt_kernel(
    A_x: jax.Array,
    A_wqkv: jax.Array,
    A_wo: jax.Array,
    B_x: jax.Array,
    B_w_r: jax.Array,
    B_w_gate: jax.Array,
    B_w_up: jax.Array,
    B_w_down: jax.Array,
):
    del B_x
    x = A_x.reshape(S, D)
    wr = B_w_r.reshape(NC, LANES)
    any_spec = pl.BlockSpec(memory_space=pl.ANY)
    out = pl.pallas_call(
        _kernel,
        out_shape=jax.ShapeDtypeStruct((S, D), BF16),
        in_specs=[any_spec] * 7,
        out_specs=any_spec,
        scratch_shapes=[
            pltpu.VMEM((S + DEF, D), BF16),
            pltpu.VMEM((D // 2, D), U32),
            pltpu.VMEM((D // 2, D), U32),
            pltpu.VMEM((2, D // 2, D), U32),
            pltpu.VMEM((NC, LANES), BF16),
            pltpu.VMEM((2, D // 2, F + LANES), U32),
            pltpu.VMEM((F // 2, D + LANES), U32),
            pltpu.VMEM((P0 // 2, D), U32),
            pltpu.VMEM((XSN, S // NA // 2, DA), U32),
            pltpu.VMEM((7 ** LK, DK // 2, DK), U32),
            pltpu.VMEM((D // 2, P0), U32),
            pltpu.VMEM((DG // 2, 7 ** LG * (TB // NG)), U32),
            pltpu.VMEM((D, LANES), F32),
            pltpu.VMEM((D, LANES), F32),
            pltpu.VMEM((RL, LANES), F32),
            pltpu.VMEM((D, D), F32),
            pltpu.VMEM((7, HD, HD), F32),
            pltpu.VMEM((D // 2, D), U32),
            pltpu.VMEM((7 ** LA, DA // 2, DA), U32),
            pltpu.VMEM((D // 2, D), U32),
            pltpu.VMEM((7 ** LO, DO // 2, DO), U32),
            pltpu.VMEM((max(TB2, RL), D + 2 * LANES), F32),
            pltpu.VMEM((RL // 2, D), U32),
            pltpu.VMEM((7 ** LO, max(TB2, RL) // NO // 2, DO), U32),
            pltpu.VMEM((DEF, D), F32),
            pltpu.VMEM((2, S + DEF, D), BF16),
            pltpu.VMEM((TB, D), F32),
            pltpu.VMEM((8, LANES), U32),
            pltpu.SemaphoreType.DMA((NSEM,)),
        ],
        compiler_params=pltpu.CompilerParams(vmem_limit_bytes=110 * 1024 * 1024, disable_bounds_checks=True,
                                             disable_semaphore_checks=True),
    )(x, A_wqkv, A_wo, wr, B_w_gate, B_w_up, B_w_down)
    return out.reshape(1, S, D)
```

```python
import jax
import jax.numpy as jnp
from jax import lax
import jax.experimental.pallas as pl
import jax.experimental.pallas.tpu as pltpu


S = 2048
D = 1024
F = 3584
H = 32
DH = D // H
LANES = 128
NC = D // LANES
HD = D // 2

LA = 2
LG = 2
LK = 2
LO = 1
NA, NG, NK, NO = 2 ** LA, 2 ** LG, 2 ** LK, 2 ** LO
DA, DG, DK, DO = D // NA, D // NG, D // NK, D // NO
XSN = 7 ** LA if LG == LA else 9 * 7 ** LG
P0 = 512
PB = S - P0
TX = 256
TB = 512
NB1 = PB // TB
TB2 = 384
NB2 = 4
QA = 192
OCH = (128, 128, 128)
DEF = OCH[-1]
L0 = NB2 * TB2
RL = S - L0
QS = (256, 256)
OCL = ((128, False), (128, False), (128, False), (64, True), (64, True))
NPRE = 24
NGAP = 10
OUT_AT = (256, 384, 448)
LNU = 8
LAG_L = 4
LN_DELAY = 800
JOB_DELAY = 500
POST_DELAY = 800
GM = 32
KM = 128
NZ = 5
PGM = 128
PGN = 128
PKM = 128
PKK = 256
EV0 = 0
EV1 = 0
EVT = 0
TRP = 700
TRS = 1300
TRW = 256
TRM = 128
GN = 256
WK5 = 66
C6LN = (1000, 8900)
C6WK = (1500, 8900)
P1LN = (60, 11200)
P1WP = (6300, 10700)
P1WQ = (7300, 12200)
WQP = 5
EV2 = 300
P2U = (60, 2000)
LAG = 5
QFIN = False
HFIN = True
EV3 = 0
LN2_DELAY = 900
QP_DELAY = 400
GLAG = (None, None, None, 20, 8)

F32 = jnp.float32
BF16 = jnp.bfloat16
U32 = jnp.uint32
I32 = jnp.int32

XP = ((PB, 128), (PB + 128, 128), (PB + 256, 256), (0, TB), (TB, PB - TB))
WKP = ((0, 128), (128, 128), (256, 256), (512, 512))

SEM_X = 0
SEM_WK = SEM_X + len(XP)
SEM_WQ = SEM_WK + len(WKP)
SEM_W3 = SEM_WQ + 1
SEM_WR = SEM_W3 + 1
SEM_WGU = SEM_WR + 1
SEM_WD = SEM_WGU + 1
SEM_OUT = SEM_WD + 1
NSEM = SEM_OUT + 5

INT_MIN = -(2 ** 31)


def _layernorm(x, tok=None, w=None):
    s0 = x[:, 0:LANES]
    if tok is not None:
        s0 = s0 + jnp.concatenate([tok] * (x.shape[0] // 8), axis=0)
    for c in range(1, NC):
        s0 = s0 + x[:, c * LANES:(c + 1) * LANES]
    mu = jnp.sum(s0, axis=-1, keepdims=True) * (1.0 / D)
    xc = x - mu
    var = jnp.sum(xc * xc, axis=-1, keepdims=True) * (1.0 / D)
    rstd = lax.rsqrt(var + 1e-5)
    if w is None:
        return xc * rstd
    return xc * rstd, jnp.sum(xc * w, axis=-1, keepdims=True) * rstd


def _phi(t):
    return jnp.where(t > 0, t + 1.0, jnp.exp(t)) + 1e-6


def _n_off(a, b):
    return 32 * a + 8 * b


def _n_groups():
    pos = {(2 * o + e) * LANES + _n_off(a, b): (16 * e + 4 * b + a) * DH + 8 * o
           for o in range(4) for e in range(2) for a in range(4) for b in range(4)}
    return [pos[n] for n in sorted(pos)]


def _quads(b):
    h = len(b) // 2
    return [[r[j * h:(j + 1) * h] for r in b[i * h:(i + 1) * h]] for i in range(2) for j in range(2)]


def _badd(x, y):
    return [[a + b for a, b in zip(rx, ry)] for rx, ry in zip(x, y)]


def _bsub(x, y):
    return [[a - b for a, b in zip(rx, ry)] for rx, ry in zip(x, y)]


def _a_set(b):
    if len(b) == 1:
        return [b[0][0]]
    return [x for o in _a_ops(b) for x in _a_set(o)]


def _b_set(b):
    if len(b) == 1:
        return [b[0][0]]
    q11, q12, q21, q22 = _quads(b)
    ops = (_badd(q11, q22), q11, _bsub(q12, q22), _bsub(q21, q11), q22, _badd(q11, q12), _badd(q21, q22))
    return [x for o in ops for x in _b_set(o)]


def _b_in_a(i, levels):
    perm = (0, 2, 6, 5, 3, 4, 1)
    return sum(perm[(i // 7 ** l) % 7] * 7 ** l for l in range(levels))


def _strassen(prod, levels, base=0, fin=lambda k, q: q, init=None, parts=None):
    if levels == 0:
        return [[prod(base)]]

    def m(i):
        if parts is not None:
            rs = [_strassen(lambda j, p=p: prod(j, p), levels - 1, base * 7 + i) for p in parts]
            return [[jnp.concatenate(v, axis=0) for v in zip(*r)] for r in zip(*rs)]
        return _strassen(prod, levels - 1, base * 7 + i)

    def seed(q, x):
        return x if init is None else _badd(_quads(init)[q], x)

    m2 = m(2)
    c22 = seed(3, m2)
    m4 = m(4)
    c12 = fin(1, _badd(seed(1, m2), m4))
    c11 = m4 if init is None else _bsub(_quads(init)[0], m4)
    m3 = m(3)
    c11 = _bsub(m3, c11) if init is None else _badd(c11, m3)
    m1 = m(1)
    c21 = fin(2, _badd(seed(2, m3), m1))
    c22 = _bsub(c22, m1)
    m0 = m(0)
    c11 = _badd(c11, m0)
    c22 = _badd(c22, m0)
    c11 = fin(0, _badd(c11, m(6)))
    c22 = fin(3, _badd(c22, m(5)))
    return [a + b for a, b in zip(c11, c12)] + [a + b for a, b in zip(c21, c22)]


def _goff(i, levels):
    return int(format(i, "0%db" % levels)[::-1], 2) if levels else 0


def _blocks(rows, n):
    w = rows[0].shape[1] // n
    return [[r[:, j * w:(j + 1) * w] for j in range(n)] for r in rows]


def _or_all(vals):
    acc = None
    for v in vals:
        v = pltpu.bitcast(v, U32)
        for g in range(v.shape[0] // 8):
            for c in range(v.shape[1] // LANES):
                p = v[g * 8:(g + 1) * 8, c * LANES:(c + 1) * LANES]
                acc = p if acc is None else acc | p
    return acc


def _raw_ops(levels):
    n = 2 ** levels
    names = [[_Tag((i, j)) for j in range(n)] for i in range(n)]
    return {op: t.ij for op, t in enumerate(_b_set(names)) if t.ij is not None}


class _Tag:
    def __init__(self, ij):
        self.ij = ij

    def __add__(self, other):
        return _Tag(None)

    __sub__ = __add__


def _a_ops(b):
    q11, q12, q21, q22 = _quads(b)
    return (_badd(q11, q22), _badd(q21, q22), q11, q22, _badd(q11, q12), _bsub(q21, q11), _bsub(q12, q22))


def _x_set(o):
    return _a_set(o) + ([] if LG == LA else [o[0][1], o[1][0]])


_A_FORM = (((0, 0), (1, 1), 1), ((1, 0), (1, 1), 1), ((0, 0),), ((1, 1),), ((0, 0), (0, 1), 1),
           ((1, 0), (0, 0), -1), ((0, 1), (1, 1), -1))
_B_FORM = (((0, 0), (1, 1), 1), ((0, 0),), ((0, 1), (1, 1), -1), ((1, 0), (0, 0), -1), ((1, 1),),
           ((0, 0), (0, 1), 1), ((1, 0), (1, 1), 1))


_C_FORM = (((0, 1), (3, 1), (4, -1), (6, 1)), ((2, 1), (4, 1)), ((1, 1), (3, 1)), ((0, 1), (1, -1), (2, 1), (5, 1)))


def _outer(form, get, n):
    h = n // 2

    def quad(q):
        return [[get(q[0] * h + i, q[1] * h + j) for j in range(h)] for i in range(h)]

    if len(form) == 1:
        return quad(form[0])
    return (_badd if form[2] > 0 else _bsub)(quad(form[0]), quad(form[1]))


def _x_slot(i):
    return i if LG == LA else (i // 7) * 9 + i % 7


def _merge(b):
    return jnp.concatenate([jnp.concatenate(r, axis=1) for r in b], axis=0)


def _gate(v, tok):
    u = pltpu.bitcast(v, U32)
    top = u[0:8, 0:LANES] | tok
    if u.shape[1] > LANES:
        top = jnp.concatenate([top, u[0:8, LANES:]], axis=1)
    return pltpu.bitcast(jnp.concatenate([top, u[8:, :]], axis=0) if u.shape[0] > 8 else top, BF16)


class _Pacer:
    def __init__(self, zero, every=0):
        self.zero, self.t, self.jobs, self.pend, self.tok = zero, 0, [], [], None
        self.every, self.last = every, -every

    def add(self, jobs, t0, t1, delay):
        for k, job in enumerate(jobs):
            self.jobs.append((t0 + k * (t1 - t0) // len(jobs), len(self.jobs), job, delay))
        self.jobs.sort(key=lambda e: e[:2])

    def due(self, dep, delay):
        if dep is not None:
            self.pend.append((self.t + delay, _or_all([dep])))

    def release(self, upto):
        while self.jobs and self.jobs[0][0] <= upto:
            _, _, job, delay = self.jobs.pop(0)
            self.due(job(self.tok), delay)

    def dot(self, lhs, rhs):
        self.release(self.t)
        ready = [d for t, d in self.pend if t <= self.t]
        if ready and self.t - self.last >= self.every:
            self.pend = [e for e in self.pend if e[0] > self.t]
            self.last = self.t
            lhs = _gate(lhs, _or_all(ready) & self.zero)
        res = jnp.dot(lhs, rhs, preferred_element_type=F32)
        self.t += lhs.shape[0] * (lhs.shape[1] // LANES) * (res.shape[1] // LANES) // 4
        self.tok = pltpu.bitcast(pltpu.bitcast(res[0:8, 0:LANES], U32) & self.zero, F32)
        return res

    def flush(self):
        self.release(1 << 30)


def _kernel(x_hbm, wqkv_hbm, wo_hbm, wr_hbm, wg_hbm, wu_hbm, wd_hbm, out_hbm,
            x_v, wk_v, wq_v, w3_v, wr_v, wgu_v, wd_v,
            ln1_v, xs_v, wks_v, pkt_v, pks_v, zacc_v, uacc_v, xw_v, g_v, gs_v, wqp_v, wqs_v, mp_v, ms_v, pq_v, pqn_v, pqs_v, attn_v, lo_v, lnf_v, zero_v,
            sems):

    ln2_v, out_v = lo_v.at[0], lo_v.at[1]

    wqkv_hbm, wo_hbm, wg_hbm, wu_hbm, wd_hbm = (r.bitcast(U32) for r in (wqkv_hbm, wo_hbm, wg_hbm, wu_hbm, wd_hbm))

    def wload(ref, r0, nr, cols):
        return pltpu.bitcast(ref[r0 // 2:(r0 + nr) // 2, cols], BF16)

    wv_v, wo_v = w3_v.at[0], w3_v.at[1]
    wg_v, wu_v = wgu_v.at[0], wgu_v.at[1]

    def x_copy(i):
        r0, n = XP[i]
        return pltpu.make_async_copy(x_hbm.at[pl.ds(r0, n), :], x_v.at[pl.ds(DEF + r0, n), :], sems.at[SEM_X + i])

    def out_copy(r0, n, s):
        return pltpu.make_async_copy(out_v.at[pl.ds(DEF + r0, n), :], out_hbm.at[pl.ds(r0, n), :],
                                     sems.at[SEM_OUT + s])

    def wk_copy(j):
        c0, n = WKP[j]
        return pltpu.make_async_copy(wqkv_hbm.at[:, pl.ds(D + c0, n)], wk_v.at[:, pl.ds(c0, n)],
                                     sems.at[SEM_WK + j])

    wq_copy = pltpu.make_async_copy(wqkv_hbm.at[:, pl.ds(0, D)], wq_v, sems.at[SEM_WQ])
    wr_copy = pltpu.make_async_copy(wr_hbm, wr_v, sems.at[SEM_WR])
    wd_copy = pltpu.make_async_copy(wd_hbm, wd_v.at[:, pl.ds(0, D)], sems.at[SEM_WD])
    wg_copy = pltpu.make_async_copy(wg_hbm, wg_v.at[:, pl.ds(0, F)], sems.at[SEM_WGU])
    wu_copy = pltpu.make_async_copy(wu_hbm, wu_v.at[:, pl.ds(0, F)], sems.at[SEM_WGU])

    x_copy(0).start()
    wk_copy(0).start()
    x_copy(1).start()
    wr_copy.start()
    for j in range(1, len(WKP)):
        wk_copy(j).start()
    for j in range(2, len(XP)):
        x_copy(j).start()
    wq_copy.start()
    pltpu.make_async_copy(wqkv_hbm.at[:, pl.ds(2 * D, D)], wv_v, sems.at[SEM_W3]).start()
    pltpu.make_async_copy(wo_hbm, wo_v, sems.at[SEM_W3]).start()
    wg_copy.start()
    wu_copy.start()
    wd_copy.start()

    def ln1_rows(xr, xr0, lnr, r0, n):
        ln = _layernorm(xr[xr0:xr0 + n, :].astype(F32)).astype(BF16)
        lnr[r0 // 2:(r0 + n) // 2, :] = pltpu.bitcast(ln, U32)

    def ln1_set(pc, xr, xr0, xsr, a0, n, t0, t1):
        def unit(j):
            def job(tok):
                ln = _layernorm(xr[xr0 + j * LNU:xr0 + (j + 1) * LNU, :].astype(F32), tok)
                lnf_v[j * LNU:(j + 1) * LNU, :] = ln
                return _or_all([ln[:, 0:LANES], ln[:, D - LANES:D]])
            return job

        def piece(j0, c0, o):
            def job(tok):
                def get(i, f):
                    r = (j0 + 2 * _goff(i, LA)) * LNU
                    v = lnf_v[r:r + 16, f * DA + c0:f * DA + c0 + LANES]
                    return v + jnp.concatenate([tok, tok], axis=0) if (i + f) % (NA // 2 + 1) == 0 else v

                r = (a0 + (j0 // (2 * NA)) * 16) // 2
                ops = _x_set(_outer(_A_FORM[o], get, NA))
                for op, v in enumerate(ops):
                    xsr.at[o * len(ops) + op][r:r + 8, c0:c0 + LANES] = pltpu.bitcast(v.astype(BF16), U32)
                return _or_all([v[0:8, :] for v in [ops[0]] + ops[5:7]])
            return job

        grp = 2 * NA
        ng = n // LNU // grp
        dt = (t1 - t0 - LN_DELAY) // (ng + 1)
        for g in range(ng):
            pc.add([unit(g * grp + j) for j in range(grp)], t0 + g * dt, t0 + (g + 1) * dt, LN_DELAY)
            s = t0 + (g + 1) * dt + LN_DELAY
            pc.add([piece(g * grp, c0, o) for c0 in range(0, DA, LANES) for o in range(7)], s, s + dt, JOB_DELAY)

    def ln1_load(lnr, r0, n):
        return pltpu.bitcast(lnr[r0 // 2:(r0 + n) // 2, :], BF16)

    def gate(v, tok):
        return v if tok is None else _gate(v, tok)

    def k_mm(r0, n, c0, nc):
        return jnp.dot(ln1_load(ln1_v, r0, n), wload(wk_v, 0, D, slice(c0, c0 + nc)), preferred_element_type=F32)

    def z_acc(pkts, c0, first=False):
        zs = None
        for pkt in pkts:
            for j in range(pkt.shape[1] // LANES):
                p = pkt[:, j * LANES:(j + 1) * LANES]
                zs = p if zs is None else zs + p
        if first:
            zacc_v[c0:c0 + zs.shape[0], :] = zs
        else:
            zacc_v[c0:c0 + zs.shape[0], :] += zs

    def k_post(k, p0, c0, first=False):
        n, nc = k.shape
        pkt = _phi(k).T
        pkt_v[c0 // 2:(c0 + nc) // 2, p0:p0 + n] = pltpu.bitcast(pkt.astype(BF16), U32)
        z_acc([pkt], c0, first)
        return pkt[nc - 8:nc, n - LANES:n]

    def g_acc(r0, n, c0, nc, first=False, pc=None):
        h, w = (nc, D) if pc is None else (min(nc, PGM), PGN)
        for f0 in range(c0, c0 + nc, h):
            for j0 in range(0, D, w):
                lhs = pltpu.bitcast(pkt_v[f0 // 2:(f0 + h) // 2, r0:r0 + n], BF16)
                rhs = pltpu.bitcast(ln1_v[r0 // 2:(r0 + n) // 2, j0:j0 + w], BF16)
                g = jnp.dot(lhs, rhs, preferred_element_type=F32) if pc is None else pc.dot(lhs, rhs)
                if first:
                    g_v[f0:f0 + h, j0:j0 + w] = g
                else:
                    g_v[f0:f0 + h, j0:j0 + w] += g

    def k_paced(pc, r0, c0, nc, first):
        for j0 in range(c0, c0 + nc, LANES):
            for t0 in range(r0, r0 + TX, PKM):
                k = None
                for k0 in range(0, D, PKK):
                    p = pc.dot(ln1_load(ln1_v, t0, PKM)[:, k0:k0 + PKK], wload(wk_v, k0, PKK, slice(j0, j0 + LANES)))
                    k = p if k is None else k + p
                pc.due(k_post(k, t0, j0, first and t0 == r0), POST_DELAY)

    attn_v[...] = jnp.zeros_like(attn_v)
    zero_v[...] = jnp.zeros_like(zero_v)

    def gs_zero(o0, o1):
        gs_v[o0:o1] = jnp.zeros((o1 - o0, HD, HD), F32)

    x_copy(0).wait()
    ln1_rows(x_v, DEF + PB, ln1_v, 0, 128)
    gs_zero(0, 1)
    wk_copy(0).wait()
    ka = k_mm(0, 128, 0, 128)
    gs_zero(1, 2)
    x_copy(1).wait()
    wr_copy.wait()
    gs_zero(2, 3)
    ln1_rows(x_v, DEF + PB + 128, ln1_v, 128, 128)
    k_post(ka, 0, 0, first=True)
    g_acc(0, 128, 0, 128, first=True)
    wk_copy(1).wait()
    gs_zero(3, NZ)
    k_post(k_mm(128, 128, 0, 128), 128, 0)
    k_post(k_mm(0, TX, 128, 128), 0, 128, first=True)
    g_acc(128, 128, 0, 128)
    def w_job(src_ref, dst_ref, levels, r0, c0, o):
        n = 2 ** levels
        w, raw, inner = D // n, _raw_ops(levels), 7 ** (levels - 1)

        def job(tok):
            def cut(i, j):
                return src_ref[(i * w + r0) // 2:(i * w + r0) // 2 + 8, j * w + c0:j * w + c0 + LANES]

            def get(i, j):
                u = cut(i, j)
                return pltpu.bitcast(u if tok is None else u | pltpu.bitcast(tok, U32), BF16).astype(F32)

            ops = []
            for op, v in enumerate(_b_set(_outer(_B_FORM[o], get, n))):
                dst = dst_ref.at[o * inner + op]
                if o * inner + op in raw:
                    dst[r0 // 2:r0 // 2 + 8, c0:c0 + LANES] = cut(*raw[o * inner + op])
                else:
                    dst[r0 // 2:r0 // 2 + 8, c0:c0 + LANES] = pltpu.bitcast(v.astype(BF16), U32)
                    ops.append(v)
            return _or_all(ops[0:1] + ops[-2:]) if ops else None
        return job

    def wk_jobs_of(outer):
        return [w_job(wk_v, wks_v, LK, r0, c0, o) for r0 in range(0, DK, 16) for c0 in range(0, DK, LANES)
                for o in outer]

    wk_copy(2).wait()
    pc = _Pacer(zero_v[...], EV0)
    pc.add(wk_jobs_of((1, 3)), 500, 2200, JOB_DELAY)
    k_paced(pc, 0, 256, 256, True)
    g_acc(0, TX, 128, 128, True, pc)
    g_acc(0, TX, 256, 256, True, pc)
    pc.flush()
    wk_copy(3).wait()
    wk_jobs = wk_jobs_of((0, 2, 4, 5, 6))
    pc = _Pacer(zero_v[...], EV0)
    pc.add(wk_jobs[:WK5], 500, 2700, JOB_DELAY)
    k_paced(pc, 0, 512, 512, True)
    g_acc(0, TX, 512, 256, True, pc)
    pc.flush()
    x_copy(2).wait()
    x_copy(3).wait()
    pc = _Pacer(zero_v[...], EV0)
    ln1_set(pc, x_v, DEF, xs_v, 0, TB, *C6LN)
    pc.add(wk_jobs[WK5:], *C6WK, JOB_DELAY)
    ln1_rows(x_v, DEF + PB + TX, ln1_v, TX, TX)
    g_acc(0, TX, 768, 256, True, pc)
    k_paced(pc, TX, 0, D, False)
    for c0 in range(0, D, 256):
        g_acc(TX, TX, c0, 256, False, pc)
    pc.flush()

    MA = TB // NA
    MG = TB // NG
    NS = NK // NG

    def xs_load(xsr, op, a0, m, cols=slice(None)):
        return pltpu.bitcast(xsr[op, a0 // 2:(a0 + m) // 2, cols], BF16)

    def k_step(pc, xsr, j0):
        def fin(_, q):
            if NS > 1:
                q = [[jnp.concatenate([_phi(jnp.concatenate([r[f] for r in q], axis=0)).T for f in range(NS)],
                                      axis=0)]]
            else:
                q = [[_phi(v).T for v in r] for r in q]
            pc.due(_or_all([v[t - 8:t, :] for r in q for v in r for t in range(LANES, v.shape[0] + 1, LANES)]),
                   POST_DELAY)
            return q

        cb = _strassen(lambda i, p: pc.dot(xs_load(xsr, _x_slot(i), p, KM),
                                           pltpu.bitcast(wks_v[i, :, j0:j0 + LANES], BF16)), LK, fin=fin,
                       parts=range(0, MA, KM))
        ops = _a_ops([[cb[i][f] for i in range(NG)] for f in range(NG)])
        for half, o in ((0, ops[4]), (1, ops[1])):
            for f, rowb in enumerate(o):
                for s in range(NS):
                    z_acc([v[s * LANES:(s + 1) * LANES, :] for v in rowb], half * HD + f * DG + s * DK + j0)
        for _ in range(LG - 1):
            ops = [o for x in ops for o in _a_ops(x)]
        for op, o in enumerate(ops):
            r = j0 * NS
            pks_v[r // 2:(r + NS * LANES) // 2, op * MG:(op + 1) * MG] = pltpu.bitcast(o[0][0].astype(BF16), U32)
        pc.due(_or_all([o[0][0][NS * LANES - 8:NS * LANES, :] for o in (ops[0], ops[-1], ops[-2])]), 2 * POST_DELAY)

    def g_rhs(xsr, i, c0, nc):
        o = _b_in_a(i, LG)
        if LG == LA:
            return xs_load(xsr, o, 0, MA, slice(c0, c0 + nc))
        j, cs = c0 // DA, slice(c0 % DA, c0 % DA + nc)
        return jnp.concatenate([xs_load(xsr, o * 9 + s, 0, MA, cs) for s in ((2, 8), (7, 3))[j]], axis=0)

    def g_step(pc, xsr, r0, nr, c0, nc, later):
        def old(o, f, c):
            v = gs_v[o, f * DG + r0:f * DG + r0 + nr, c * DG + c0:c * DG + c0 + nc]
            return v if o < NZ else jnp.where(later, v, 0.0)

        for o in range(7):
            cb = _strassen(lambda i: pc.dot(pltpu.bitcast(pks_v[r0 // 2:(r0 + nr) // 2, i * MG:(i + 1) * MG], BF16),
                                            g_rhs(xsr, i, c0, nc)), LG - 1, base=o,
                           init=[[old(o, f, c) for c in range(NG // 2)] for f in range(NG // 2)])
            for f in range(NG // 2):
                for c in range(NG // 2):
                    gs_v[o, f * DG + r0:f * DG + r0 + nr, c * DG + c0:c * DG + c0 + nc] = cb[f][c]

    def wq_jobs(u0, nr):
        span = (NA - 1) * DA + 16 * nr
        u0 = u0 if isinstance(u0, int) else pl.multiple_of(u0, 8)
        srcr, permr = wq_v.at[pl.ds(u0, span // 2), :], wqp_v.at[pl.ds(u0, span // 2), :]
        dstr = wqs_v.at[:, pl.ds(u0, 8 * nr), :]
        oct_ = (lax.broadcasted_iota(I32, (8, LANES), 1) % DH) // 8

        def perm(r, e):
            def job(tok):
                blk = [srcr[r // 2:r // 2 + 8, (4 * e + b) * LANES:(4 * e + b + 1) * LANES] | pltpu.bitcast(tok, U32)
                       for b in range(4)]
                outs = []
                for o in range(4):
                    v = blk[o]
                    for b in range(4):
                        if b != o:
                            v = jnp.where(oct_ == b, pltpu.roll(blk[b], (8 * (b - o)) % LANES, 1), v)
                    permr[r // 2:r // 2 + 8, (2 * o + e) * LANES:(2 * o + e + 1) * LANES] = v
                    outs.append(v)
                return _or_all(outs)
            return job

        return ([perm(i * DA + r0, e) for r0 in range(0, 16 * nr, 16) for i in range(NA) for e in range(2)],
                [w_job(permr, dstr, LA, r0, c0, o) for r0 in range(0, 16 * nr, 16)
                 for c0 in range(0, DA, LANES) for o in range(7)])

    def p1(i, carry):
        xsr = xs_v.at[:, pl.ds(pl.multiple_of(i * (MA // 2), MA // 2), MA), :]
        xr = x_v.at[pl.ds(pl.multiple_of((i + 1) * TB, TB), TB + DEF), :]

        pc = _Pacer(zero_v[...], EV1)
        ln1_set(pc, xr, DEF, xsr, MA, TB, *P1LN)
        perms, sets = wq_jobs(i * (8 * WQP), WQP)
        pc.add(perms, *P1WP, JOB_DELAY)
        pc.add(sets, *P1WQ, JOB_DELAY)
        for j0 in range(0, DK, LANES):
            k_step(pc, xsr, j0)
        for f0 in range(0, DG, GM):
            for c0 in range(0, DG, GN):
                g_step(pc, xsr, f0, GM, c0, GN, i > 0)
        pc.flush()
        return carry

    x_copy(4).wait()
    wq_copy.wait()
    lax.fori_loop(0, NB1, p1, 0)

    pltpu.make_async_copy(w3_v, w3_v, sems.at[SEM_W3]).wait()
    zero_u = zero_v[...]
    def row_vector(acc_ref):
        return jnp.sum(jnp.concatenate([acc_ref[r:r + 8, :] for r in _n_groups()], axis=0).T, axis=0, keepdims=True)

    zrow = row_vector(zacc_v)
    wr8 = wr_v[...].astype(F32)
    wr_row = jnp.concatenate([wr8[c:c + 1, :] for c in range(NC)], axis=1)

    row_h = lax.broadcasted_iota(I32, (LANES, LANES), 0) // DH
    col_h = lax.broadcasted_iota(I32, (LANES, LANES), 1) // DH
    diag = row_h == col_h

    def colsum(t):
        acc = t[:, 0:LANES]
        for c in range(1, NC):
            acc = acc + t[:, c * LANES:(c + 1) * LANES]
        return acc

    wrc = wr_row - jnp.sum(wr_row, axis=-1, keepdims=True) * (1.0 / D)
    m_raw = _raw_ops(LO)

    def kv_part(c):
        cs = slice(c * LANES, (c + 1) * LANES)
        kv = None
        for k0 in range(0, D, TRW):
            g = g_v[cs, k0:k0 + TRW]
            for o, sign in _C_FORM[(c * LANES // HD) * 2 + k0 // HD]:
                t = gs_v[o, c * LANES % HD:c * LANES % HD + LANES, k0 % HD:k0 % HD + TRW]
                g = g + t if sign > 0 else g - t
            p = pc.dot(g.astype(BF16), wload(wv_v, k0, TRW, cs))
            kv = p if kv is None else kv + p
        return jnp.where(diag, kv, 0.0)

    def m_part(c, kvs):
        e, b = c // 4, c % 4
        for j0 in range(0, DO, TRM):
            ms = [jnp.concatenate(
                [pc.dot(kv, wload(wo_v, (c + k) * LANES, LANES, slice(f * DO + j0, f * DO + j0 + TRM)))
                 for f in range(NO)], axis=1) for k, kv in enumerate(kvs)]
            deps = []
            for a in range(4):
                rows = [jnp.concatenate([m[a * DH + 8 * o:a * DH + 8 * o + 8, :] for m in ms], axis=0)
                        for o in range(4)]
                for o in range(4):
                    r = ((2 * o + e) * LANES + _n_off(a, b)) // 2
                    for f in range(NO):
                        mp_v[r:r + 8, f * DO + j0:f * DO + j0 + TRM] = pltpu.bitcast(
                            rows[o][:, f * TRM:(f + 1) * TRM].astype(BF16), U32)
                for t in range(4 // NO):
                    r = ((2 * t + e) * LANES + _n_off(a, b)) // 2
                    for op, v in enumerate(_b_set(_blocks(rows[t::4 // NO], NO))):
                        if op not in m_raw:
                            ms_v.at[op][r:r + 8, j0:j0 + TRM] = pltpu.bitcast(v.astype(BF16), U32)
                            deps.append(v[0:8, 0:LANES])
            pc.due(_or_all(deps[::4]), POST_DELAY)

    pc = _Pacer(zero_u, EVT)
    pc.due(jnp.broadcast_to(zrow, (8, D)), 1000)
    perms, sets = wq_jobs(NB1 * 8 * WQP, DA // 16 - NB1 * WQP)
    pc.add(perms, 60, TRP, JOB_DELAY)
    pc.add(sets, TRS, 3500, JOB_DELAY)
    kv_prev = None
    for c in range(0, NC + 2, 2):
        kvs = [kv_part(c).astype(BF16), kv_part(c + 1).astype(BF16)] if c < NC else None
        if c:
            m_part(c - 2, kv_prev)
        kv_prev = kvs
    pc.flush()

    def make_key(score, row):
        b = pltpu.bitcast(score, I32)
        srt = b ^ ((b >> 31) & 0x7FFFFFFF)
        return (srt & jnp.int32(-65536)) | (0xFFFF - row)

    def push_keys(key, top1, top2):
        for gidx in range(key.shape[0] // 8):
            kx = key[gidx * 8:(gidx + 1) * 8, :]
            top2 = jnp.maximum(top2, jnp.minimum(top1, kx))
            top1 = jnp.maximum(top1, kx)
        return top1, top2

    lane = lax.broadcasted_iota(I32, (1, LANES), 1)

    def interleave(parts):
        return jnp.concatenate([p[g * 16:(g + 1) * 16, :] for g in range(parts[0].shape[0] // 16) for p in parts],
                               axis=0)

    def q_part(pc, xsr, l0, r0, n, hint=None):
        m = n // NA
        sums = {}

        def park(v, g, c):
            for t in range(m // 16):
                r = r0 + (t * NA + g) * 16
                pq_v[r:r + 16, c * LANES:(c + 1) * LANES] = v[t * 16:(t + 1) * 16, :]

        def fin(k, q):
            q = [[_phi(v) for v in r] for r in q]
            deps = []
            for a, r in enumerate(q):
                for b, v in enumerate(r):
                    i, c = (k // 2) * (NA // 2) + a, (((k % 2) * (NA // 2) + b) * DA + j0) // LANES
                    park(v, _goff(i, LA), c)
                    for name, row in (("z", zrow),) + ((("u", hint["u"]),) if hint else ()):
                        t = v * row[:, c * LANES:(c + 1) * LANES]
                        key = (name, _goff(i, LA), c % 2)
                        sums[key] = t if key not in sums else sums[key] + t
                deps.append(sums[key])
            if (r0 + n < RL or HFIN) if hint else QFIN:
                pc.due(_or_all(deps), POST_DELAY)
            return q

        for j0 in range(0, DA, LANES):
            _strassen(lambda i: pc.dot(xs_load(xsr, _x_slot(i), (l0 + r0) // NA, m),
                                       pltpu.bitcast(wqs_v[i, :, j0:j0 + LANES], BF16)), LA, fin=fin)
        if hint:
            pc.flush()
        den = jnp.concatenate([sums["z", g, e] for g in range(NA) for e in range(2)], axis=0)
        for s in (1, 2, 4):
            den = den + jnp.where((lane & s) == 0, pltpu.roll(den, LANES - s, 1), pltpu.roll(den, s, 1))
        inv_all = 1.0 / (den + 1e-6)

        def inv_of(g):
            return [inv_all[(g * 2 + e) * m:(g * 2 + e + 1) * m, :] for e in range(2)]

        for g in range(NA):
            for e in range(2):
                park(inv_of(g)[e], g, NC + e)
        if hint:
            for g in range(NA):
                starts = [r0 + (t * NA + g) * 16 for t in range(m // 16)]
                num = jnp.sum(jnp.concatenate([xw_v[t:t + 16, :] for t in starts], axis=0)
                              + sums["u", g, 0] * inv_of(g)[0] + sums["u", g, 1] * inv_of(g)[1],
                              axis=-1, keepdims=True)
                row = jnp.concatenate([(l0 + t) + lax.broadcasted_iota(I32, (16, 1), 0) for t in starts], axis=0)
                hint["p1"], hint["p2"] = push_keys(make_key(num, row), hint["p1"], hint["p2"])
            pc.due(jnp.broadcast_to(hint["p1"], (8, LANES)), 1200)


    def post_jobs(r0, n, plain=False):
        def scaled(t, c0, w, tok):
            inv = pq_v[t:t + 16, D:D + 2 * LANES]
            if tok is not None:
                inv = inv + jnp.concatenate([jnp.concatenate([tok, tok], axis=0)] * 2, axis=1)
            return pq_v[t:t + 16, c0:c0 + w] * jnp.concatenate([inv] * (w // (2 * LANES)), axis=1)

        def post_plain(t):
            def job(tok):
                v = scaled(t, 0, D, tok)
                pqn_v[t // 2:t // 2 + 8, :] = pltpu.bitcast(v.astype(BF16), U32)
                return v[0:8, 0:LANES]
            return job

        def post(t0, outer):
            def job(tok):
                deps = []
                for c0 in range(0, DO, 2 * LANES):
                    blk = {}

                    def get(i, f):
                        if (i, f) not in blk:
                            blk[i, f] = scaled(t0 + _goff(i, LO) * 16, f * DO + c0, 2 * LANES, tok)
                        return blk[i, f]

                    for o in outer:
                        ops = _a_set(_outer(_A_FORM[o], get, NO))
                        for op, v in enumerate(ops):
                            pqs_v.at[o * len(ops) + op][t0 // NO // 2:t0 // NO // 2 + 8, c0:c0 + 2 * LANES] = (
                                pltpu.bitcast(v.astype(BF16), U32))
                        deps.append(ops[0][0:8, 0:LANES])
                return _or_all(deps)
            return job

        if plain:
            return [post_plain(t) for t in range(r0, r0 + n, 16)]
        outers = [range(7)] if LO == 1 else [(o,) for o in range(7)]
        return [post(t0, outer) for t0 in range(r0, r0 + n, 16 * NO) for outer in outers]

    def m_operand(i, c0, c1):
        if i not in m_raw:
            return pltpu.bitcast(ms_v[i, :, c0 * LANES:c1 * LANES], BF16)
        bi, bj = m_raw[i]
        return wload(mp_v, bi * DO, DO, slice(bj * DO + c0 * LANES, bj * DO + c1 * LANES))

    def o_part(dot, xr, x0, r0, n):
        a0, m = r0 // NO, n // NO
        nw = LANES * NO // 2
        cols = [[[] for _ in range(NO)] for _ in range(NO)]
        for c0 in range(0, DO, nw):
            init = [[jnp.concatenate(
                [xr[x0 + r0 + (g * NO + _goff(i, LO)) * 16:x0 + r0 + (g * NO + _goff(i, LO) + 1) * 16,
                    f * DO + c0:f * DO + c0 + nw] for g in range(m // 16)], axis=0).astype(F32)
                for f in range(NO)] for i in range(NO)]
            cb = _strassen(lambda i: dot(pltpu.bitcast(pqs_v[i, a0 // 2:(a0 + m) // 2, :], BF16),
                                         m_operand(i, c0 // LANES, (c0 + nw) // LANES)), LO, init=init)
            for i in range(NO):
                for f in range(NO):
                    cols[i][f].append(cb[i][f])
        parts = [None] * NO
        for i in range(NO):
            parts[_goff(i, LO)] = jnp.concatenate([c for f in range(NO) for c in cols[i][f]], axis=1)
        return interleave(parts)

    def ln2_unit(h, l2r, outr, r0, row0, valid, top1, top2, tok, fast=False):
        n = h.shape[0]
        if fast:
            ln2, r = _layernorm(h, tok, wr_row)
        else:
            ln2 = _layernorm(h, tok)
            r = jnp.sum(ln2 * wr_row, axis=-1, keepdims=True)
        l2r[r0:r0 + n, :] = ln2.astype(BF16)
        res = h + ln2
        outr[r0:r0 + n, :] = res.astype(BF16)
        r = r.astype(BF16).astype(F32) + 0.0
        key = make_key(r, (row0 + r0) + lax.broadcasted_iota(I32, (n, 1), 0))
        if valid is not None:
            key = jnp.where(valid, key, INT_MIN)
        top1, top2 = push_keys(key, top1, top2)
        ntok = pltpu.bitcast(pltpu.bitcast(jnp.broadcast_to(r[n - 8:n, :], (8, LANES)), U32) & zero_u, F32)
        return top1, top2, ntok

    def ln2_jobs(h, l2r, outr, r0, row0, valid, st, fast=False):
        def unit(j):
            def job(tok):
                st["top1"], st["top2"], dep = ln2_unit(h[j * LNU:(j + 1) * LNU, :], l2r, outr, r0 + j * LNU, row0,
                                                       valid, st["top1"], st["top2"], tok, fast)
                return dep
            return job
        return [unit(j) for j in range(h.shape[0] // LNU)]

    QC = 16 * 7 ** LA / 8 ** LA
    OC = 16 * 7 ** LO / 8 ** LO

    def p2(i, carry):
        st = dict(top1=carry[0], top2=carry[1])
        b0 = pl.multiple_of(i * TB2, 16)
        xsr = xs_v.at[:, pl.ds(pl.multiple_of(i * (TB2 // NA // 2), 8), TB2 // NA // 2), :]
        xr = x_v.at[pl.ds(b0, TB2 + DEF), :]
        l2r = ln2_v.at[pl.ds(b0, TB2 + DEF), :]
        outr = out_v.at[pl.ds(b0, TB2 + DEF), :]
        row0 = b0 - DEF
        pc = _Pacer(zero_u)
        toks = []

        def chain(jobs):
            for job in jobs:
                toks.append(job(toks[-LAG] if len(toks) >= LAG else None))

        chain(ln2_jobs(attn_v, l2r, outr, 0, row0, i > 0, st))

        @pl.when(i > 0)
        def _():
            out_copy(pl.multiple_of((i - 1) * TB2, 16), TB2, 0).start()

        pc.due(toks[-1], QA * QC)

        nu, nx = D // NB2, RL // NB2
        mr = mp_v.at[pl.ds(pl.multiple_of(i * (nu // 2), 8), nu // 2), :]
        ur = uacc_v.at[pl.ds(pl.multiple_of(i * nu, 8), nu), :]
        xl = x_v.at[pl.ds(pl.multiple_of(DEF + L0 + i * nx, 16), nx), :]
        xwr = xw_v.at[pl.ds(pl.multiple_of(i * nx, 8), nx), :]

        def hint_job(load, dst, r):
            def job(tok):
                v = colsum(load(r).astype(F32) * wrc) + jnp.concatenate([tok, tok], axis=0)
                dst[r:r + 16, :] = v
                return v
            return job

        pc.add([hint_job(lambda r: wload(mr, r, 16, slice(None)), ur, r) for r in range(0, nu, 16)]
               + [hint_job(lambda r: xl[r:r + 16, :], xwr, r) for r in range(0, nx, 16)], *P2U, JOB_DELAY)
        for r0, n in ((0, QA), (QA, TB2 - QA)):
            q_part(pc, xsr, 0, r0, n)
            for job in post_jobs(r0, n):
                job(None)
        r0 = 0
        for n in OCH[:-1]:
            chain(ln2_jobs(o_part(pc.dot, xr, DEF, r0, n), l2r, outr, DEF + r0, row0, None, st))
            r0 += n
        attn_v[...] = o_part(pc.dot, xr, DEF, r0, DEF)
        return st["top1"], st["top2"]

    init = jnp.full((8, 1), INT_MIN, I32)
    top1, top2 = lax.fori_loop(0, NB2, p2, (init, init))

    wg_copy.wait()
    wu_copy.wait()
    wd_copy.wait()
    sub8 = lax.broadcasted_iota(I32, (8, LANES), 0)
    urow = jnp.sum(uacc_v[...].T, axis=0, keepdims=True)

    def submax(v):
        for sh in (4, 2, 1):
            v = jnp.maximum(v, pltpu.roll(v, sh, 0))
        return v

    def subsum(v):
        for sh in (4, 2, 1):
            v = v + pltpu.roll(v, sh, 0)
        return v

    def best2(t1, t2):
        t1 = jnp.broadcast_to(t1, (8, LANES))
        t2 = jnp.broadcast_to(t2, (8, LANES))
        k1v = submax(t1)
        return k1v, submax(jnp.where(t1 == k1v, t2, t1))

    def key_row(k):
        return 0xFFFF - (k & 0xFFFF)

    def wide(m):
        return jnp.concatenate([m] * NC, axis=1)

    st = dict(top1=top1, top2=top2, pend=[], step=0, sent=0)
    pc = _Pacer(zero_u, EV2)
    hint = dict(u=urow, p1=init, p2=init)

    pc.add(ln2_jobs(attn_v, ln2_v, out_v, L0, -DEF, None, st), 60, QS[0] * QC - 600, LN2_DELAY)
    r0 = 0
    for k, n in enumerate(QS):
        q_part(pc, xs_v, L0, r0, n, hint)
        if k == 0:
            out_copy(L0 - TB2, TB2, 0).start()
            top1, top2 = st["top1"], st["top2"]
            pc.add(post_jobs(0, OCL[0][0], OCL[0][1]), pc.t + 600, pc.t + (RL - n) * QC - 300, QP_DELAY)
        r0 += n
    pc.every = EV3
    oldk = best2(top1, top2)
    oldx = []
    for kk in oldk:
        g8 = pl.multiple_of(((jnp.clip(key_row(kk[0, 0]), 0, S - 1) >> 3) << 3) + DEF, 8)
        rows = ln2_v[pl.ds(g8, 8), :].astype(F32)
        oldx.append(subsum(jnp.where(wide((key_row(kk) & 7) == sub8), rows, 0.0)))

    def gated(v):
        tok = None
        while st["pend"] and st["pend"][0][0] <= st["step"]:
            t = st["pend"].pop(0)[1]
            tok = t if tok is None else tok | t
        if tok is None:
            return v
        u = pltpu.bitcast(v, U32)
        return pltpu.bitcast(jnp.concatenate([u[:, 0:LANES] | tok, u[:, LANES:]], axis=1), BF16)

    res = {}

    def c_units():
        pc.flush()
        p1, p2_ = hint["p1"], hint["p2"]
        cand_p, cand_x = [], []
        for pk_ in (p1, p2_):
            cp, cx = None, None
            for s in range(8):
                g8 = pl.multiple_of((jnp.clip(key_row(pk_[s, 0]) - L0, 0, RL - 1) >> 3) << 3, 8)
                vp = pq_v[pl.ds(g8, 8), :]
                vx = x_v[pl.ds(pl.multiple_of(g8 + (L0 + DEF), 8), 8), :].astype(F32)
                cp = vp if cp is None else jnp.where(jnp.concatenate([sub8 == s] * (NC + 2), axis=1), vp, cp)
                cx = vx if cx is None else jnp.where(wide(sub8 == s), vx, cx)
            cand_p.append(cp[:, 0:D] * jnp.concatenate([cp[:, D:]] * (NC // 2), axis=1))
            cand_x.append(cx)
        cand_p = jnp.concatenate(cand_p, axis=0).astype(BF16)
        cand_x = jnp.concatenate(cand_x, axis=0)
        ids_lo = key_row(jnp.broadcast_to(p1, (8, LANES)))
        ids_hi = jnp.where(sub8 < 6, key_row(jnp.broadcast_to(p2_, (8, LANES))),
                           jnp.where(sub8 == 6, key_row(oldk[0]), key_row(oldk[1])))
        res["ids"] = (ids_lo, ids_hi)
        parts = []
        for c in range(NC):
            parts.append(jnp.dot(cand_p, wload(mp_v, 0, D, slice(c * LANES, (c + 1) * LANES)), preferred_element_type=F32))
            yield
        xs = _layernorm(cand_x + jnp.concatenate(parts, axis=1))
        hi = jnp.where(wide(sub8 < 6), xs[8:16, :], jnp.where(wide(sub8 == 6), oldx[0], oldx[1]))
        res["xs"] = jnp.concatenate([xs[0:8, :], hi], axis=0).astype(BF16)

    def f_units():
        xs = res["xs"]
        acts = []
        for j in range(F // LANES):
            cs = slice(j * LANES, (j + 1) * LANES)
            g = jnp.dot(gated(xs), wload(wg_v, 0, D, cs), preferred_element_type=F32)
            yield
            u = jnp.dot(xs, wload(wu_v, 0, D, cs), preferred_element_type=F32)
            acts.append((g * jax.nn.sigmoid(g) * u).astype(BF16))
            yield
        act = jnp.concatenate(acts, axis=1)
        zf = pltpu.bitcast(zero_u, F32)
        ys = []
        KF = (F // D) * D
        for c in range(0, NC, 2):
            acc = jnp.concatenate([jnp.concatenate([zf, zf], axis=0)] * 2, axis=1)
            acc = acc + jnp.dot(gated(act[:, KF:]), wload(wd_v, KF, F - KF, slice(c * LANES, (c + 2) * LANES)),
                                preferred_element_type=F32)
            yield
            for cc in range(2):
                y = acc[:, cc * LANES:(cc + 1) * LANES]
                for k0 in range(0, KF, D):
                    y = y + jnp.dot(gated(act[:, k0:k0 + D]),
                                    wload(wd_v, k0, D, slice((c + cc) * LANES, (c + cc + 1) * LANES)),
                                    preferred_element_type=F32)
                    yield
                ys.append(y)
        res["y"] = jnp.concatenate(ys, axis=1)

    def side_units():
        yield from range(NPRE)
        yield from c_units()
        yield from range(NGAP)
        yield from f_units()

    side = side_units()

    def o_dot(lhs, rhs):
        p = pc.dot(lhs, rhs) if st["step"] < NPRE else jnp.dot(lhs, rhs, preferred_element_type=F32)
        next(side, None)
        st["step"] += 1
        return p

    def o_plain(r0, n):
        lhs = pltpu.bitcast(pqn_v[r0 // 2:(r0 + n) // 2, :], BF16)
        parts = []
        for c0 in range(0, NC, 2):
            acc = x_v[DEF + L0 + r0:DEF + L0 + r0 + n, c0 * LANES:(c0 + 2) * LANES].astype(F32)
            for k0 in range(0, D, 2 * LANES):
                acc = acc + o_dot(lhs[:, k0:k0 + 2 * LANES], wload(mp_v, k0, 2 * LANES, slice(c0 * LANES, (c0 + 2) * LANES)))
            parts.append(acc)
        return jnp.concatenate(parts, axis=1)

    toks = []
    r0 = 0
    pc.add(post_jobs(OCL[0][0], *OCL[1]), pc.t + 200, pc.t + 1000, QP_DELAY)
    for ci, (n, plain) in enumerate(OCL):
        h = o_plain(r0, n) if plain else o_part(o_dot, x_v, DEF + L0, r0, n)
        last = r0 + n == RL
        units = ln2_jobs(h, ln2_v, out_v, DEF + L0 + r0, -DEF, None, st, fast=last)
        posts = post_jobs(r0 + n + OCL[ci + 1][0], *OCL[ci + 2]) if ci + 2 < len(OCL) else []
        for k, job in enumerate(units):
            toks.append(job(toks[-LAG_L] if len(toks) >= LAG_L and not last else None))
            if posts:
                posts.pop(0)(toks[-1])
        if GLAG[ci] is not None:
            st["pend"].append((st["step"] + GLAG[ci],
                               pltpu.bitcast(jnp.broadcast_to(st["top1"], (8, LANES)), U32) & zero_u))
        r0 += n
        if last or r0 in OUT_AT:
            out_copy(L0 + st["sent"], r0 - st["sent"], 2 if last else 1).start()
            if not last:
                st["sent"] = r0
    for _ in side:
        st["step"] += 1

    keyv = best2(st["top1"], st["top2"])
    idx = [jnp.clip(key_row(kk[0, 0]), 0, S - 1) for kk in keyv]
    grp = [pl.multiple_of((ii >> 3) << 3, 8) for ii in idx]
    vgrp = [pl.multiple_of(gg + DEF, 8) for gg in grp]
    y = res["y"]
    ids_lo, ids_hi = res["ids"]
    hits = None
    yrows = []
    for c in range(2):
        m_lo = ids_lo == key_row(keyv[c])
        m_hi = ids_hi == key_row(keyv[c])
        yrows.append(subsum(jnp.where(wide(m_lo), y[0:8, :], 0.0) + jnp.where(wide(m_hi), y[8:16, :], 0.0)))
        hit = submax(jnp.where(m_lo | m_hi, 1, 0))
        hits = hit if hits is None else hits + hit
    hit_all = hits[0, 0] == 2

    tail0 = L0 + st["sent"]
    tail_copy = out_copy(tail0, S - tail0, 2)
    in_tail = jnp.maximum(grp[0], grp[1]) >= tail0
    two_groups = grp[1] != grp[0]

    def fix_copy(c):
        return out_copy(grp[c], 8, 3 + c)

    def finish(ysel):
        for c in range(2):
            hi = keyv[c] & jnp.int32(-65536)
            score = pltpu.bitcast(hi ^ ((hi >> 31) & 0x7FFF0000), F32)
            sel = (key_row(keyv[c]) & 7) == sub8
            upd = jnp.where(wide(sel), ysel[c] * wide(jax.nn.sigmoid(score)), 0.0)
            out_v[pl.ds(vgrp[c], 8), :] = (out_v[pl.ds(vgrp[c], 8), :].astype(F32) + upd).astype(BF16)
        fix_copy(0).start()

        @pl.when(two_groups)
        def _():
            fix_copy(1).start()

    out_copy(0, L0, 0).wait()
    out_copy(L0, tail0 - L0, 1).wait()

    @pl.when(in_tail)
    def _():
        tail_copy.wait()

    @pl.when(hit_all)
    def _():
        finish(yrows)

    @pl.when(jnp.logical_not(hit_all))
    def _():
        xsel = jnp.concatenate([ln2_v[pl.ds(vgrp[c], 8), :] for c in range(2)], axis=0)

        def ffn_tile(j, acc):
            cs = pl.ds(pl.multiple_of(j * LANES, LANES), LANES)
            g = jnp.dot(xsel, wload(wg_v, 0, D, cs), preferred_element_type=F32)
            u = jnp.dot(xsel, wload(wu_v, 0, D, cs), preferred_element_type=F32)
            a = (g * jax.nn.sigmoid(g) * u).astype(BF16)
            wd_t = pltpu.bitcast(wd_v[pl.ds(pl.multiple_of(j * (LANES // 2), LANES // 2), LANES // 2), 0:D], BF16)
            return acc + jnp.dot(a, wd_t, preferred_element_type=F32)

        yf = lax.fori_loop(0, F // LANES, ffn_tile, jnp.zeros((16, D), F32))
        finish([yf[0:8, :], yf[8:16, :]])

    @pl.when(jnp.logical_not(in_tail))
    def _():
        tail_copy.wait()

    fix_copy(0).wait()

    @pl.when(two_groups)
    def _():
        fix_copy(1).wait()


@jax.jit
def pallas_sequential_preLN__linear_attn_block__moe_arch_mod__prompt_kernel(
    A_x: jax.Array,
    A_wqkv: jax.Array,
    A_wo: jax.Array,
    B_x: jax.Array,
    B_w_r: jax.Array,
    B_w_gate: jax.Array,
    B_w_up: jax.Array,
    B_w_down: jax.Array,
):
    del B_x
    x = A_x.reshape(S, D)
    wr = B_w_r.reshape(NC, LANES)
    any_spec = pl.BlockSpec(memory_space=pl.ANY)
    out = pl.pallas_call(
        _kernel,
        out_shape=jax.ShapeDtypeStruct((S, D), BF16),
        in_specs=[any_spec] * 7,
        out_specs=any_spec,
        scratch_shapes=[
            pltpu.VMEM((S + DEF, D), BF16),
            pltpu.VMEM((D // 2, D), U32),
            pltpu.VMEM((D // 2, D), U32),
            pltpu.VMEM((2, D // 2, D), U32),
            pltpu.VMEM((NC, LANES), BF16),
            pltpu.VMEM((2, D // 2, F + LANES), U32),
            pltpu.VMEM((F // 2, D + LANES), U32),
            pltpu.VMEM((P0 // 2, D), U32),
            pltpu.VMEM((XSN, S // NA // 2, DA), U32),
            pltpu.VMEM((7 ** LK, DK // 2, DK), U32),
            pltpu.VMEM((D // 2, P0), U32),
            pltpu.VMEM((DG // 2, 7 ** LG * (TB // NG)), U32),
            pltpu.VMEM((D, LANES), F32),
            pltpu.VMEM((D, LANES), F32),
            pltpu.VMEM((RL, LANES), F32),
            pltpu.VMEM((D, D), F32),
            pltpu.VMEM((7, HD, HD), F32),
            pltpu.VMEM((D // 2, D), U32),
            pltpu.VMEM((7 ** LA, DA // 2, DA), U32),
            pltpu.VMEM((D // 2, D), U32),
            pltpu.VMEM((7 ** LO, DO // 2, DO), U32),
            pltpu.VMEM((max(TB2, RL), D + 2 * LANES), F32),
            pltpu.VMEM((RL // 2, D), U32),
            pltpu.VMEM((7 ** LO, max(TB2, RL) // NO // 2, DO), U32),
            pltpu.VMEM((DEF, D), F32),
            pltpu.VMEM((2, S + DEF, D), BF16),
            pltpu.VMEM((TB, D), F32),
            pltpu.VMEM((8, LANES), U32),
            pltpu.SemaphoreType.DMA((NSEM,)),
        ],
        compiler_params=pltpu.CompilerParams(vmem_limit_bytes=110 * 1024 * 1024, disable_bounds_checks=True,
                                             disable_semaphore_checks=True),
    )(x, A_wqkv, A_wo, wr, B_w_gate, B_w_up, B_w_down)
    return out.reshape(1, S, D)
```

```python
import jax
import jax.numpy as jnp
from jax import lax
import jax.experimental.pallas as pl
import jax.experimental.pallas.tpu as pltpu


S = 2048
D = 1024
F = 3584
H = 32
DH = D // H
LANES = 128
NC = D // LANES
HD = D // 2

LA = 2
LO = 1
NA, NO = 2 ** LA, 2 ** LO
DA, DO = D // NA, D // NO
P0 = 512
PB = S - P0
TX = 256
TB = 512
NB1 = PB // TB
MA = TB // NA
TB2 = 384
NB2 = 4
QA = 192
OCH = (128, 128, 128)
DEF = OCH[-1]
L0 = NB2 * TB2
RL = S - L0
QS = (256, 256)
OCL = ((128, False), (128, False), (128, False), (64, True), (64, True))
NPRE = 24
NGAP = 10
OUT_AT = (256, 384, 448)
GM = 32
NZ = 5
WQP = 5
LNU = 8
LAG = 5
LAG_L = 4
LN_DELAY = 800
LN2_DELAY = 900
JOB_DELAY = 500
POST_DELAY = 800
QP_DELAY = 400
WK5 = 66
C6LN = (1000, 8900)
C6WK = (1500, 8900)
P1LN = (60, 11200)
P1WP = (6300, 10700)
P1WQ = (7300, 12200)
P2U = (60, 2000)
EV2 = 300
GLAG = (None, None, None, 20, 8)

F32 = jnp.float32
BF16 = jnp.bfloat16
U32 = jnp.uint32
I32 = jnp.int32

XP = ((PB, 128), (PB + 128, 128), (PB + 256, 256), (0, TB), (TB, PB - TB))
WKP = ((0, 128), (128, 128), (256, 256), (512, 512))

SEM_X = 0
SEM_WK = SEM_X + len(XP)
SEM_WQ = SEM_WK + len(WKP)
SEM_W3 = SEM_WQ + 1
SEM_WR = SEM_W3 + 1
SEM_WGU = SEM_WR + 1
SEM_WD = SEM_WGU + 1
SEM_OUT = SEM_WD + 1
NSEM = SEM_OUT + 5

INT_MIN = -(2 ** 31)


def _layernorm(x, tok=None, w=None):
    s0 = x[:, 0:LANES]
    if tok is not None:
        s0 = s0 + jnp.concatenate([tok] * (x.shape[0] // 8), axis=0)
    for c in range(1, NC):
        s0 = s0 + x[:, c * LANES:(c + 1) * LANES]
    mu = jnp.sum(s0, axis=-1, keepdims=True) * (1.0 / D)
    xc = x - mu
    var = jnp.sum(xc * xc, axis=-1, keepdims=True) * (1.0 / D)
    rstd = lax.rsqrt(var + 1e-5)
    if w is None:
        return xc * rstd
    return xc * rstd, jnp.sum(xc * w, axis=-1, keepdims=True) * rstd


def _phi(t):
    return jnp.where(t > 0, t + 1.0, jnp.exp(t)) + 1e-6


def _n_off(a, b):
    return 32 * a + 8 * b


def _n_groups():
    pos = {(2 * o + e) * LANES + _n_off(a, b): (16 * e + 4 * b + a) * DH + 8 * o
           for o in range(4) for e in range(2) for a in range(4) for b in range(4)}
    return [pos[n] for n in sorted(pos)]


def _quads(b):
    h = len(b) // 2
    return [[r[j * h:(j + 1) * h] for r in b[i * h:(i + 1) * h]] for i in range(2) for j in range(2)]


def _badd(x, y):
    return [[a + b for a, b in zip(rx, ry)] for rx, ry in zip(x, y)]


def _bsub(x, y):
    return [[a - b for a, b in zip(rx, ry)] for rx, ry in zip(x, y)]


def _a_set(b):
    if len(b) == 1:
        return [b[0][0]]
    return [x for o in _a_ops(b) for x in _a_set(o)]


def _b_set(b):
    if len(b) == 1:
        return [b[0][0]]
    q11, q12, q21, q22 = _quads(b)
    ops = (_badd(q11, q22), q11, _bsub(q12, q22), _bsub(q21, q11), q22, _badd(q11, q12), _badd(q21, q22))
    return [x for o in ops for x in _b_set(o)]


def _b_in_a(i, levels):
    perm = (0, 2, 6, 5, 3, 4, 1)
    return sum(perm[(i // 7 ** l) % 7] * 7 ** l for l in range(levels))


def _strassen(prod, levels, base=0, fin=lambda k, q: q, init=None):
    if levels == 0:
        return [[prod(base)]]

    def m(i):
        return _strassen(prod, levels - 1, base * 7 + i)

    def seed(q, x):
        return x if init is None else _badd(_quads(init)[q], x)

    m2 = m(2)
    c22 = seed(3, m2)
    m4 = m(4)
    c12 = fin(1, _badd(seed(1, m2), m4))
    c11 = m4 if init is None else _bsub(_quads(init)[0], m4)
    m3 = m(3)
    c11 = _bsub(m3, c11) if init is None else _badd(c11, m3)
    m1 = m(1)
    c21 = fin(2, _badd(seed(2, m3), m1))
    c22 = _bsub(c22, m1)
    m0 = m(0)
    c11 = _badd(c11, m0)
    c22 = _badd(c22, m0)
    c11 = fin(0, _badd(c11, m(6)))
    c22 = fin(3, _badd(c22, m(5)))
    return [a + b for a, b in zip(c11, c12)] + [a + b for a, b in zip(c21, c22)]


def _goff(i, levels):
    return int(format(i, "0%db" % levels)[::-1], 2) if levels else 0


def _blocks(rows, n):
    w = rows[0].shape[1] // n
    return [[r[:, j * w:(j + 1) * w] for j in range(n)] for r in rows]


def _or_all(vals):
    acc = None
    for v in vals:
        v = pltpu.bitcast(v, U32)
        for g in range(v.shape[0] // 8):
            for c in range(v.shape[1] // LANES):
                p = v[g * 8:(g + 1) * 8, c * LANES:(c + 1) * LANES]
                acc = p if acc is None else acc | p
    return acc


def _raw_ops(levels):
    n = 2 ** levels
    names = [[_Tag((i, j)) for j in range(n)] for i in range(n)]
    return {op: t.ij for op, t in enumerate(_b_set(names)) if t.ij is not None}


class _Tag:
    def __init__(self, ij):
        self.ij = ij

    def __add__(self, other):
        return _Tag(None)

    __sub__ = __add__


def _a_ops(b):
    q11, q12, q21, q22 = _quads(b)
    return (_badd(q11, q22), _badd(q21, q22), q11, q22, _badd(q11, q12), _bsub(q21, q11), _bsub(q12, q22))


_A_FORM = (((0, 0), (1, 1), 1), ((1, 0), (1, 1), 1), ((0, 0),), ((1, 1),), ((0, 0), (0, 1), 1),
           ((1, 0), (0, 0), -1), ((0, 1), (1, 1), -1))
_B_FORM = (((0, 0), (1, 1), 1), ((0, 0),), ((0, 1), (1, 1), -1), ((1, 0), (0, 0), -1), ((1, 1),),
           ((0, 0), (0, 1), 1), ((1, 0), (1, 1), 1))
_C_FORM = (((0, 1), (3, 1), (4, -1), (6, 1)), ((2, 1), (4, 1)), ((1, 1), (3, 1)), ((0, 1), (1, -1), (2, 1), (5, 1)))


def _outer(form, get, n):
    h = n // 2

    def quad(q):
        return [[get(q[0] * h + i, q[1] * h + j) for j in range(h)] for i in range(h)]

    if len(form) == 1:
        return quad(form[0])
    return (_badd if form[2] > 0 else _bsub)(quad(form[0]), quad(form[1]))


def _gate(v, tok):
    u = pltpu.bitcast(v, U32)
    top = u[0:8, 0:LANES] | tok
    if u.shape[1] > LANES:
        top = jnp.concatenate([top, u[0:8, LANES:]], axis=1)
    return pltpu.bitcast(jnp.concatenate([top, u[8:, :]], axis=0) if u.shape[0] > 8 else top, BF16)


class _Pacer:
    def __init__(self, zero, every=0):
        self.zero, self.t, self.jobs, self.pend, self.tok = zero, 0, [], [], None
        self.every, self.last = every, -every

    def add(self, jobs, t0, t1, delay):
        for k, job in enumerate(jobs):
            self.jobs.append((t0 + k * (t1 - t0) // len(jobs), len(self.jobs), job, delay))
        self.jobs.sort(key=lambda e: e[:2])

    def due(self, dep, delay):
        if dep is not None:
            self.pend.append((self.t + delay, _or_all([dep])))

    def release(self, upto):
        while self.jobs and self.jobs[0][0] <= upto:
            _, _, job, delay = self.jobs.pop(0)
            self.due(job(self.tok), delay)

    def dot(self, lhs, rhs):
        self.release(self.t)
        ready = [d for t, d in self.pend if t <= self.t]
        if ready and self.t - self.last >= self.every:
            self.pend = [e for e in self.pend if e[0] > self.t]
            self.last = self.t
            lhs = _gate(lhs, _or_all(ready) & self.zero)
        res = jnp.dot(lhs, rhs, preferred_element_type=F32)
        self.t += lhs.shape[0] * (lhs.shape[1] // LANES) * (res.shape[1] // LANES) // 4
        self.tok = pltpu.bitcast(pltpu.bitcast(res[0:8, 0:LANES], U32) & self.zero, F32)
        return res

    def flush(self):
        self.release(1 << 30)


def _kernel(x_hbm, wqkv_hbm, wo_hbm, wr_hbm, wg_hbm, wu_hbm, wd_hbm, out_hbm,
            x_v, wk_v, wq_v, w3_v, wr_v, wgu_v, wd_v,
            ln1_v, xs_v, wks_v, pkt_v, pks_v, zacc_v, uacc_v, xw_v, g_v, gs_v, wqp_v, wqs_v, mp_v, ms_v,
            pq_v, pqn_v, pqs_v, attn_v, lo_v, lnf_v, zero_v, sems):

    ln2_v, out_v = lo_v.at[0], lo_v.at[1]

    wqkv_hbm, wo_hbm, wg_hbm, wu_hbm, wd_hbm = (r.bitcast(U32) for r in (wqkv_hbm, wo_hbm, wg_hbm, wu_hbm, wd_hbm))

    def wload(ref, r0, nr, cols):
        return pltpu.bitcast(ref[r0 // 2:(r0 + nr) // 2, cols], BF16)

    wv_v, wo_v = w3_v.at[0], w3_v.at[1]
    wg_v, wu_v = wgu_v.at[0], wgu_v.at[1]

    def x_copy(i):
        r0, n = XP[i]
        return pltpu.make_async_copy(x_hbm.at[pl.ds(r0, n), :], x_v.at[pl.ds(DEF + r0, n), :], sems.at[SEM_X + i])

    def out_copy(r0, n, s):
        return pltpu.make_async_copy(out_v.at[pl.ds(DEF + r0, n), :], out_hbm.at[pl.ds(r0, n), :],
                                     sems.at[SEM_OUT + s])

    def wk_copy(j):
        c0, n = WKP[j]
        return pltpu.make_async_copy(wqkv_hbm.at[:, pl.ds(D + c0, n)], wk_v.at[:, pl.ds(c0, n)],
                                     sems.at[SEM_WK + j])

    wq_copy = pltpu.make_async_copy(wqkv_hbm.at[:, pl.ds(0, D)], wq_v, sems.at[SEM_WQ])
    wr_copy = pltpu.make_async_copy(wr_hbm, wr_v, sems.at[SEM_WR])
    wd_copy = pltpu.make_async_copy(wd_hbm, wd_v.at[:, pl.ds(0, D)], sems.at[SEM_WD])
    wg_copy = pltpu.make_async_copy(wg_hbm, wg_v.at[:, pl.ds(0, F)], sems.at[SEM_WGU])
    wu_copy = pltpu.make_async_copy(wu_hbm, wu_v.at[:, pl.ds(0, F)], sems.at[SEM_WGU])

    x_copy(0).start()
    wk_copy(0).start()
    x_copy(1).start()
    wr_copy.start()
    for j in range(1, len(WKP)):
        wk_copy(j).start()
    for j in range(2, len(XP)):
        x_copy(j).start()
    wq_copy.start()
    pltpu.make_async_copy(wqkv_hbm.at[:, pl.ds(2 * D, D)], wv_v, sems.at[SEM_W3]).start()
    pltpu.make_async_copy(wo_hbm, wo_v, sems.at[SEM_W3]).start()
    wg_copy.start()
    wu_copy.start()
    wd_copy.start()

    def ln1_rows(xr, xr0, lnr, r0, n):
        ln = _layernorm(xr[xr0:xr0 + n, :].astype(F32)).astype(BF16)
        lnr[r0 // 2:(r0 + n) // 2, :] = pltpu.bitcast(ln, U32)

    def ln1_set(pc, xr, xr0, xsr, a0, n, t0, t1):
        def unit(j):
            def job(tok):
                ln = _layernorm(xr[xr0 + j * LNU:xr0 + (j + 1) * LNU, :].astype(F32), tok)
                lnf_v[j * LNU:(j + 1) * LNU, :] = ln
                return _or_all([ln[:, 0:LANES], ln[:, D - LANES:D]])
            return job

        def piece(j0, c0, o):
            def job(tok):
                def get(i, f):
                    r = (j0 + 2 * _goff(i, LA)) * LNU
                    v = lnf_v[r:r + 16, f * DA + c0:f * DA + c0 + LANES]
                    return v + jnp.concatenate([tok, tok], axis=0) if (i + f) % (NA // 2 + 1) == 0 else v

                r = (a0 + (j0 // (2 * NA)) * 16) // 2
                ops = _a_set(_outer(_A_FORM[o], get, NA))
                for op, v in enumerate(ops):
                    xsr.at[o * len(ops) + op][r:r + 8, c0:c0 + LANES] = pltpu.bitcast(v.astype(BF16), U32)
                return _or_all([v[0:8, :] for v in [ops[0]] + ops[5:7]])
            return job

        grp = 2 * NA
        ng = n // LNU // grp
        dt = (t1 - t0 - LN_DELAY) // (ng + 1)
        for g in range(ng):
            pc.add([unit(g * grp + j) for j in range(grp)], t0 + g * dt, t0 + (g + 1) * dt, LN_DELAY)
            s = t0 + (g + 1) * dt + LN_DELAY
            pc.add([piece(g * grp, c0, o) for c0 in range(0, DA, LANES) for o in range(7)], s, s + dt, JOB_DELAY)

    def ln1_load(lnr, r0, n):
        return pltpu.bitcast(lnr[r0 // 2:(r0 + n) // 2, :], BF16)

    def k_mm(r0, n, c0, nc):
        return jnp.dot(ln1_load(ln1_v, r0, n), wload(wk_v, 0, D, slice(c0, c0 + nc)), preferred_element_type=F32)

    def z_acc(pkts, c0, first=False):
        zs = None
        for pkt in pkts:
            for j in range(pkt.shape[1] // LANES):
                p = pkt[:, j * LANES:(j + 1) * LANES]
                zs = p if zs is None else zs + p
        if first:
            zacc_v[c0:c0 + zs.shape[0], :] = zs
        else:
            zacc_v[c0:c0 + zs.shape[0], :] += zs

    def k_post(k, p0, c0, first=False):
        n, nc = k.shape
        pkt = _phi(k).T
        pkt_v[c0 // 2:(c0 + nc) // 2, p0:p0 + n] = pltpu.bitcast(pkt.astype(BF16), U32)
        z_acc([pkt], c0, first)
        return pkt[nc - 8:nc, n - LANES:n]

    def g_acc(r0, n, c0, nc, first=False, pc=None):
        h, w = (nc, D) if pc is None else (LANES, LANES)
        for f0 in range(c0, c0 + nc, h):
            for j0 in range(0, D, w):
                lhs = pltpu.bitcast(pkt_v[f0 // 2:(f0 + h) // 2, r0:r0 + n], BF16)
                rhs = pltpu.bitcast(ln1_v[r0 // 2:(r0 + n) // 2, j0:j0 + w], BF16)
                g = jnp.dot(lhs, rhs, preferred_element_type=F32) if pc is None else pc.dot(lhs, rhs)
                if first:
                    g_v[f0:f0 + h, j0:j0 + w] = g
                else:
                    g_v[f0:f0 + h, j0:j0 + w] += g

    def k_paced(pc, r0, c0, nc, first):
        for j0 in range(c0, c0 + nc, LANES):
            for t0 in range(r0, r0 + TX, LANES):
                k = None
                for k0 in range(0, D, TX):
                    p = pc.dot(ln1_load(ln1_v, t0, LANES)[:, k0:k0 + TX], wload(wk_v, k0, TX, slice(j0, j0 + LANES)))
                    k = p if k is None else k + p
                pc.due(k_post(k, t0, j0, first and t0 == r0), POST_DELAY)

    attn_v[...] = jnp.zeros_like(attn_v)
    zero_v[...] = jnp.zeros_like(zero_v)

    def gs_zero(o0, o1):
        gs_v[o0:o1] = jnp.zeros((o1 - o0, HD, HD), F32)

    x_copy(0).wait()
    ln1_rows(x_v, DEF + PB, ln1_v, 0, 128)
    gs_zero(0, 1)
    wk_copy(0).wait()
    ka = k_mm(0, 128, 0, 128)
    gs_zero(1, 2)
    x_copy(1).wait()
    wr_copy.wait()
    gs_zero(2, 3)
    ln1_rows(x_v, DEF + PB + 128, ln1_v, 128, 128)
    k_post(ka, 0, 0, first=True)
    g_acc(0, 128, 0, 128, first=True)
    wk_copy(1).wait()
    gs_zero(3, NZ)
    k_post(k_mm(128, 128, 0, 128), 128, 0)
    k_post(k_mm(0, TX, 128, 128), 0, 128, first=True)
    g_acc(128, 128, 0, 128)

    def w_job(src_ref, dst_ref, levels, r0, c0, o):
        n = 2 ** levels
        w, raw, inner = D // n, _raw_ops(levels), 7 ** (levels - 1)

        def job(tok):
            def cut(i, j):
                return src_ref[(i * w + r0) // 2:(i * w + r0) // 2 + 8, j * w + c0:j * w + c0 + LANES]

            def get(i, j):
                u = cut(i, j)
                return pltpu.bitcast(u if tok is None else u | pltpu.bitcast(tok, U32), BF16).astype(F32)

            ops = []
            for op, v in enumerate(_b_set(_outer(_B_FORM[o], get, n))):
                dst = dst_ref.at[o * inner + op]
                if o * inner + op in raw:
                    dst[r0 // 2:r0 // 2 + 8, c0:c0 + LANES] = cut(*raw[o * inner + op])
                else:
                    dst[r0 // 2:r0 // 2 + 8, c0:c0 + LANES] = pltpu.bitcast(v.astype(BF16), U32)
                    ops.append(v)
            return _or_all(ops[0:1] + ops[-2:]) if ops else None
        return job

    def wk_jobs_of(outer):
        return [w_job(wk_v, wks_v, LA, r0, c0, o) for r0 in range(0, DA, 16) for c0 in range(0, DA, LANES)
                for o in outer]

    wk_copy(2).wait()
    pc = _Pacer(zero_v[...])
    pc.add(wk_jobs_of((1, 3)), 500, 2200, JOB_DELAY)
    k_paced(pc, 0, 256, 256, True)
    g_acc(0, TX, 128, 128, True, pc)
    g_acc(0, TX, 256, 256, True, pc)
    pc.flush()
    wk_copy(3).wait()
    wk_jobs = wk_jobs_of((0, 2, 4, 5, 6))
    pc = _Pacer(zero_v[...])
    pc.add(wk_jobs[:WK5], 500, 2700, JOB_DELAY)
    k_paced(pc, 0, 512, 512, True)
    g_acc(0, TX, 512, 256, True, pc)
    pc.flush()
    x_copy(2).wait()
    x_copy(3).wait()
    pc = _Pacer(zero_v[...])
    ln1_set(pc, x_v, DEF, xs_v, 0, TB, *C6LN)
    pc.add(wk_jobs[WK5:], *C6WK, JOB_DELAY)
    ln1_rows(x_v, DEF + PB + TX, ln1_v, TX, TX)
    g_acc(0, TX, 768, 256, True, pc)
    k_paced(pc, TX, 0, D, False)
    for c0 in range(0, D, 256):
        g_acc(TX, TX, c0, 256, False, pc)
    pc.flush()

    def xs_load(xsr, op, a0, m):
        return pltpu.bitcast(xsr[op, a0 // 2:(a0 + m) // 2, :], BF16)

    def k_step(pc, xsr, j0):
        def fin(_, q):
            q = [[_phi(v).T for v in r] for r in q]
            pc.due(_or_all([v[LANES - 8:LANES, :] for r in q for v in r]), POST_DELAY)
            return q

        cb = _strassen(lambda i: pc.dot(xs_load(xsr, i, 0, MA), pltpu.bitcast(wks_v[i, :, j0:j0 + LANES], BF16)),
                       LA, fin=fin)
        outer = _a_ops([[cb[i][f] for i in range(NA)] for f in range(NA)])
        for half, o in ((0, outer[4]), (1, outer[1])):
            for f, rowb in enumerate(o):
                z_acc(rowb, half * HD + f * DA + j0)
        ops = [v for o in outer for v in _a_set(o)]
        for op, v in enumerate(ops):
            pks_v[j0 // 2:(j0 + LANES) // 2, op * MA:(op + 1) * MA] = pltpu.bitcast(v.astype(BF16), U32)
        pc.due(_or_all([v[LANES - 8:LANES, :] for v in (ops[0], ops[-1], ops[-2])]), 2 * POST_DELAY)

    def g_step(pc, xsr, r0, later):
        def old(o, f, c):
            v = gs_v[o, f * DA + r0:f * DA + r0 + GM, c * DA:(c + 1) * DA]
            return v if o < NZ else jnp.where(later, v, 0.0)

        for o in range(7):
            cb = _strassen(lambda i: pc.dot(pltpu.bitcast(pks_v[r0 // 2:(r0 + GM) // 2, i * MA:(i + 1) * MA], BF16),
                                            xs_load(xsr, _b_in_a(i, LA), 0, MA)), LA - 1, base=o,
                           init=[[old(o, f, c) for c in range(NA // 2)] for f in range(NA // 2)])
            for f in range(NA // 2):
                for c in range(NA // 2):
                    gs_v[o, f * DA + r0:f * DA + r0 + GM, c * DA:(c + 1) * DA] = cb[f][c]

    def wq_jobs(u0, nr):
        span = (NA - 1) * DA + 16 * nr
        u0 = u0 if isinstance(u0, int) else pl.multiple_of(u0, 8)
        srcr, permr = wq_v.at[pl.ds(u0, span // 2), :], wqp_v.at[pl.ds(u0, span // 2), :]
        dstr = wqs_v.at[:, pl.ds(u0, 8 * nr), :]
        oct_ = (lax.broadcasted_iota(I32, (8, LANES), 1) % DH) // 8

        def perm(r, e):
            def job(tok):
                blk = [srcr[r // 2:r // 2 + 8, (4 * e + b) * LANES:(4 * e + b + 1) * LANES] | pltpu.bitcast(tok, U32)
                       for b in range(4)]
                outs = []
                for o in range(4):
                    v = blk[o]
                    for b in range(4):
                        if b != o:
                            v = jnp.where(oct_ == b, pltpu.roll(blk[b], (8 * (b - o)) % LANES, 1), v)
                    permr[r // 2:r // 2 + 8, (2 * o + e) * LANES:(2 * o + e + 1) * LANES] = v
                    outs.append(v)
                return _or_all(outs)
            return job

        return ([perm(i * DA + r0, e) for r0 in range(0, 16 * nr, 16) for i in range(NA) for e in range(2)],
                [w_job(permr, dstr, LA, r0, c0, o) for r0 in range(0, 16 * nr, 16)
                 for c0 in range(0, DA, LANES) for o in range(7)])

    def p1(i, carry):
        xsr = xs_v.at[:, pl.ds(pl.multiple_of(i * (MA // 2), MA // 2), MA), :]
        xr = x_v.at[pl.ds(pl.multiple_of((i + 1) * TB, TB), TB + DEF), :]

        pc = _Pacer(zero_v[...])
        ln1_set(pc, xr, DEF, xsr, MA, TB, *P1LN)
        perms, sets = wq_jobs(i * (8 * WQP), WQP)
        pc.add(perms, *P1WP, JOB_DELAY)
        pc.add(sets, *P1WQ, JOB_DELAY)
        for j0 in range(0, DA, LANES):
            k_step(pc, xsr, j0)
        for r0 in range(0, DA, GM):
            g_step(pc, xsr, r0, i > 0)
        pc.flush()
        return carry

    x_copy(4).wait()
    wq_copy.wait()
    lax.fori_loop(0, NB1, p1, 0)

    pltpu.make_async_copy(w3_v, w3_v, sems.at[SEM_W3]).wait()
    zero_u = zero_v[...]
    zrow = jnp.sum(jnp.concatenate([zacc_v[r:r + 8, :] for r in _n_groups()], axis=0).T, axis=0, keepdims=True)
    wr8 = wr_v[...].astype(F32)
    wr_row = jnp.concatenate([wr8[c:c + 1, :] for c in range(NC)], axis=1)

    row_h = lax.broadcasted_iota(I32, (LANES, LANES), 0) // DH
    col_h = lax.broadcasted_iota(I32, (LANES, LANES), 1) // DH
    diag = row_h == col_h

    def colsum(t):
        acc = t[:, 0:LANES]
        for c in range(1, NC):
            acc = acc + t[:, c * LANES:(c + 1) * LANES]
        return acc

    wrc = wr_row - jnp.sum(wr_row, axis=-1, keepdims=True) * (1.0 / D)
    m_raw = _raw_ops(LO)

    def kv_part(c):
        cs = slice(c * LANES, (c + 1) * LANES)
        kv = None
        for k0 in range(0, D, TX):
            g = g_v[cs, k0:k0 + TX]
            for o, sign in _C_FORM[(c * LANES // HD) * 2 + k0 // HD]:
                t = gs_v[o, c * LANES % HD:c * LANES % HD + LANES, k0 % HD:k0 % HD + TX]
                g = g + t if sign > 0 else g - t
            p = pc.dot(g.astype(BF16), wload(wv_v, k0, TX, cs))
            kv = p if kv is None else kv + p
        return jnp.where(diag, kv, 0.0)

    def m_part(c, kvs):
        e, b = c // 4, c % 4
        for j0 in range(0, DO, LANES):
            ms = [jnp.concatenate(
                [pc.dot(kv, wload(wo_v, (c + k) * LANES, LANES, slice(f * DO + j0, f * DO + j0 + LANES)))
                 for f in range(NO)], axis=1) for k, kv in enumerate(kvs)]
            deps = []
            for a in range(4):
                rows = [jnp.concatenate([m[a * DH + 8 * o:a * DH + 8 * o + 8, :] for m in ms], axis=0)
                        for o in range(4)]
                for o in range(4):
                    r = ((2 * o + e) * LANES + _n_off(a, b)) // 2
                    for f in range(NO):
                        mp_v[r:r + 8, f * DO + j0:f * DO + j0 + LANES] = pltpu.bitcast(
                            rows[o][:, f * LANES:(f + 1) * LANES].astype(BF16), U32)
                for t in range(4 // NO):
                    r = ((2 * t + e) * LANES + _n_off(a, b)) // 2
                    for op, v in enumerate(_b_set(_blocks(rows[t::4 // NO], NO))):
                        if op not in m_raw:
                            ms_v.at[op][r:r + 8, j0:j0 + LANES] = pltpu.bitcast(v.astype(BF16), U32)
                            deps.append(v[0:8, 0:LANES])
            pc.due(_or_all(deps[::4]), POST_DELAY)

    pc = _Pacer(zero_u)
    pc.due(jnp.broadcast_to(zrow, (8, D)), 1000)
    perms, sets = wq_jobs(NB1 * 8 * WQP, DA // 16 - NB1 * WQP)
    pc.add(perms, 60, 700, JOB_DELAY)
    pc.add(sets, 1300, 3500, JOB_DELAY)
    kv_prev = None
    for c in range(0, NC + 2, 2):
        kvs = [kv_part(c).astype(BF16), kv_part(c + 1).astype(BF16)] if c < NC else None
        if c:
            m_part(c - 2, kv_prev)
        kv_prev = kvs
    pc.flush()

    def make_key(score, row):
        b = pltpu.bitcast(score, I32)
        srt = b ^ ((b >> 31) & 0x7FFFFFFF)
        return (srt & jnp.int32(-65536)) | (0xFFFF - row)

    def push_keys(key, top1, top2):
        for gidx in range(key.shape[0] // 8):
            kx = key[gidx * 8:(gidx + 1) * 8, :]
            top2 = jnp.maximum(top2, jnp.minimum(top1, kx))
            top1 = jnp.maximum(top1, kx)
        return top1, top2

    lane = lax.broadcasted_iota(I32, (1, LANES), 1)

    def interleave(parts):
        return jnp.concatenate([p[g * 16:(g + 1) * 16, :] for g in range(parts[0].shape[0] // 16) for p in parts],
                               axis=0)

    def q_part(pc, xsr, l0, r0, n, hint=None):
        m = n // NA
        sums = {}

        def park(v, g, c):
            for t in range(m // 16):
                r = r0 + (t * NA + g) * 16
                pq_v[r:r + 16, c * LANES:(c + 1) * LANES] = v[t * 16:(t + 1) * 16, :]

        def fin(k, q):
            q = [[_phi(v) for v in r] for r in q]
            deps = []
            for a, r in enumerate(q):
                for b, v in enumerate(r):
                    i, c = (k // 2) * (NA // 2) + a, (((k % 2) * (NA // 2) + b) * DA + j0) // LANES
                    park(v, _goff(i, LA), c)
                    for name, row in (("z", zrow),) + ((("u", hint["u"]),) if hint else ()):
                        t = v * row[:, c * LANES:(c + 1) * LANES]
                        key = (name, _goff(i, LA), c % 2)
                        sums[key] = t if key not in sums else sums[key] + t
                deps.append(sums[key])
            if hint:
                pc.due(_or_all(deps), POST_DELAY)
            return q

        for j0 in range(0, DA, LANES):
            _strassen(lambda i: pc.dot(xs_load(xsr, i, (l0 + r0) // NA, m),
                                       pltpu.bitcast(wqs_v[i, :, j0:j0 + LANES], BF16)), LA, fin=fin)
        if hint:
            pc.flush()
        den = jnp.concatenate([sums["z", g, e] for g in range(NA) for e in range(2)], axis=0)
        for s in (1, 2, 4):
            den = den + jnp.where((lane & s) == 0, pltpu.roll(den, LANES - s, 1), pltpu.roll(den, s, 1))
        inv_all = 1.0 / (den + 1e-6)

        def inv_of(g):
            return [inv_all[(g * 2 + e) * m:(g * 2 + e + 1) * m, :] for e in range(2)]

        for g in range(NA):
            for e in range(2):
                park(inv_of(g)[e], g, NC + e)
        if hint:
            for g in range(NA):
                starts = [r0 + (t * NA + g) * 16 for t in range(m // 16)]
                num = jnp.sum(jnp.concatenate([xw_v[t:t + 16, :] for t in starts], axis=0)
                              + sums["u", g, 0] * inv_of(g)[0] + sums["u", g, 1] * inv_of(g)[1],
                              axis=-1, keepdims=True)
                row = jnp.concatenate([(l0 + t) + lax.broadcasted_iota(I32, (16, 1), 0) for t in starts], axis=0)
                hint["p1"], hint["p2"] = push_keys(make_key(num, row), hint["p1"], hint["p2"])
            pc.due(jnp.broadcast_to(hint["p1"], (8, LANES)), 1200)


    def post_jobs(r0, n, plain=False):
        def scaled(t, c0, w, tok):
            inv = pq_v[t:t + 16, D:D + 2 * LANES]
            if tok is not None:
                inv = inv + jnp.concatenate([jnp.concatenate([tok, tok], axis=0)] * 2, axis=1)
            return pq_v[t:t + 16, c0:c0 + w] * jnp.concatenate([inv] * (w // (2 * LANES)), axis=1)

        def post_plain(t):
            def job(tok):
                v = scaled(t, 0, D, tok)
                pqn_v[t // 2:t // 2 + 8, :] = pltpu.bitcast(v.astype(BF16), U32)
                return v[0:8, 0:LANES]
            return job

        def post(t0, outer):
            def job(tok):
                deps = []
                for c0 in range(0, DO, 2 * LANES):
                    blk = {}

                    def get(i, f):
                        if (i, f) not in blk:
                            blk[i, f] = scaled(t0 + _goff(i, LO) * 16, f * DO + c0, 2 * LANES, tok)
                        return blk[i, f]

                    for o in outer:
                        ops = _a_set(_outer(_A_FORM[o], get, NO))
                        for op, v in enumerate(ops):
                            pqs_v.at[o * len(ops) + op][t0 // NO // 2:t0 // NO // 2 + 8, c0:c0 + 2 * LANES] = (
                                pltpu.bitcast(v.astype(BF16), U32))
                        deps.append(ops[0][0:8, 0:LANES])
                return _or_all(deps)
            return job

        if plain:
            return [post_plain(t) for t in range(r0, r0 + n, 16)]
        outers = [range(7)] if LO == 1 else [(o,) for o in range(7)]
        return [post(t0, outer) for t0 in range(r0, r0 + n, 16 * NO) for outer in outers]

    def m_operand(i, c0, c1):
        if i not in m_raw:
            return pltpu.bitcast(ms_v[i, :, c0 * LANES:c1 * LANES], BF16)
        bi, bj = m_raw[i]
        return wload(mp_v, bi * DO, DO, slice(bj * DO + c0 * LANES, bj * DO + c1 * LANES))

    def o_part(dot, xr, x0, r0, n):
        a0, m = r0 // NO, n // NO
        nw = LANES * NO // 2
        cols = [[[] for _ in range(NO)] for _ in range(NO)]
        for c0 in range(0, DO, nw):
            init = [[jnp.concatenate(
                [xr[x0 + r0 + (g * NO + _goff(i, LO)) * 16:x0 + r0 + (g * NO + _goff(i, LO) + 1) * 16,
                    f * DO + c0:f * DO + c0 + nw] for g in range(m // 16)], axis=0).astype(F32)
                for f in range(NO)] for i in range(NO)]
            cb = _strassen(lambda i: dot(pltpu.bitcast(pqs_v[i, a0 // 2:(a0 + m) // 2, :], BF16),
                                         m_operand(i, c0 // LANES, (c0 + nw) // LANES)), LO, init=init)
            for i in range(NO):
                for f in range(NO):
                    cols[i][f].append(cb[i][f])
        parts = [None] * NO
        for i in range(NO):
            parts[_goff(i, LO)] = jnp.concatenate([c for f in range(NO) for c in cols[i][f]], axis=1)
        return interleave(parts)

    def ln2_unit(h, l2r, outr, r0, row0, valid, top1, top2, tok, fast=False):
        n = h.shape[0]
        if fast:
            ln2, r = _layernorm(h, tok, wr_row)
        else:
            ln2 = _layernorm(h, tok)
            r = jnp.sum(ln2 * wr_row, axis=-1, keepdims=True)
        l2r[r0:r0 + n, :] = ln2.astype(BF16)
        res = h + ln2
        outr[r0:r0 + n, :] = res.astype(BF16)
        r = r.astype(BF16).astype(F32) + 0.0
        key = make_key(r, (row0 + r0) + lax.broadcasted_iota(I32, (n, 1), 0))
        if valid is not None:
            key = jnp.where(valid, key, INT_MIN)
        top1, top2 = push_keys(key, top1, top2)
        ntok = pltpu.bitcast(pltpu.bitcast(jnp.broadcast_to(r[n - 8:n, :], (8, LANES)), U32) & zero_u, F32)
        return top1, top2, ntok

    def ln2_jobs(h, l2r, outr, r0, row0, valid, st, fast=False):
        def unit(j):
            def job(tok):
                st["top1"], st["top2"], dep = ln2_unit(h[j * LNU:(j + 1) * LNU, :], l2r, outr, r0 + j * LNU, row0,
                                                       valid, st["top1"], st["top2"], tok, fast)
                return dep
            return job
        return [unit(j) for j in range(h.shape[0] // LNU)]

    QC = 16 * 7 ** LA / 8 ** LA

    def p2(i, carry):
        st = dict(top1=carry[0], top2=carry[1])
        b0 = pl.multiple_of(i * TB2, 16)
        xsr = xs_v.at[:, pl.ds(pl.multiple_of(i * (TB2 // NA // 2), 8), TB2 // NA // 2), :]
        xr = x_v.at[pl.ds(b0, TB2 + DEF), :]
        l2r = ln2_v.at[pl.ds(b0, TB2 + DEF), :]
        outr = out_v.at[pl.ds(b0, TB2 + DEF), :]
        row0 = b0 - DEF
        pc = _Pacer(zero_u)
        toks = []

        def chain(jobs):
            for job in jobs:
                toks.append(job(toks[-LAG] if len(toks) >= LAG else None))

        chain(ln2_jobs(attn_v, l2r, outr, 0, row0, i > 0, st))

        @pl.when(i > 0)
        def _():
            out_copy(pl.multiple_of((i - 1) * TB2, 16), TB2, 0).start()

        pc.due(toks[-1], QA * QC)

        nu, nx = D // NB2, RL // NB2
        mr = mp_v.at[pl.ds(pl.multiple_of(i * (nu // 2), 8), nu // 2), :]
        ur = uacc_v.at[pl.ds(pl.multiple_of(i * nu, 8), nu), :]
        xl = x_v.at[pl.ds(pl.multiple_of(DEF + L0 + i * nx, 16), nx), :]
        xwr = xw_v.at[pl.ds(pl.multiple_of(i * nx, 8), nx), :]

        def hint_job(load, dst, r):
            def job(tok):
                v = colsum(load(r).astype(F32) * wrc) + jnp.concatenate([tok, tok], axis=0)
                dst[r:r + 16, :] = v
                return v
            return job

        pc.add([hint_job(lambda r: wload(mr, r, 16, slice(None)), ur, r) for r in range(0, nu, 16)]
               + [hint_job(lambda r: xl[r:r + 16, :], xwr, r) for r in range(0, nx, 16)], *P2U, JOB_DELAY)
        for r0, n in ((0, QA), (QA, TB2 - QA)):
            q_part(pc, xsr, 0, r0, n)
            for job in post_jobs(r0, n):
                job(None)
        r0 = 0
        for n in OCH[:-1]:
            chain(ln2_jobs(o_part(pc.dot, xr, DEF, r0, n), l2r, outr, DEF + r0, row0, None, st))
            r0 += n
        attn_v[...] = o_part(pc.dot, xr, DEF, r0, DEF)
        return st["top1"], st["top2"]

    init = jnp.full((8, 1), INT_MIN, I32)
    top1, top2 = lax.fori_loop(0, NB2, p2, (init, init))

    wg_copy.wait()
    wu_copy.wait()
    wd_copy.wait()
    sub8 = lax.broadcasted_iota(I32, (8, LANES), 0)
    urow = jnp.sum(uacc_v[...].T, axis=0, keepdims=True)

    def submax(v):
        for sh in (4, 2, 1):
            v = jnp.maximum(v, pltpu.roll(v, sh, 0))
        return v

    def subsum(v):
        for sh in (4, 2, 1):
            v = v + pltpu.roll(v, sh, 0)
        return v

    def best2(t1, t2):
        t1 = jnp.broadcast_to(t1, (8, LANES))
        t2 = jnp.broadcast_to(t2, (8, LANES))
        k1v = submax(t1)
        return k1v, submax(jnp.where(t1 == k1v, t2, t1))

    def key_row(k):
        return 0xFFFF - (k & 0xFFFF)

    def wide(m):
        return jnp.concatenate([m] * NC, axis=1)

    st = dict(top1=top1, top2=top2, pend=[], step=0, sent=0)
    pc = _Pacer(zero_u, EV2)
    hint = dict(u=urow, p1=init, p2=init)

    pc.add(ln2_jobs(attn_v, ln2_v, out_v, L0, -DEF, None, st), 60, QS[0] * QC - 600, LN2_DELAY)
    r0 = 0
    for k, n in enumerate(QS):
        q_part(pc, xs_v, L0, r0, n, hint)
        if k == 0:
            out_copy(L0 - TB2, TB2, 0).start()
            top1, top2 = st["top1"], st["top2"]
            pc.add(post_jobs(0, OCL[0][0], OCL[0][1]), pc.t + 600, pc.t + (RL - n) * QC - 300, QP_DELAY)
        r0 += n
    pc.every = 0
    oldk = best2(top1, top2)
    oldx = []
    for kk in oldk:
        g8 = pl.multiple_of(((jnp.clip(key_row(kk[0, 0]), 0, S - 1) >> 3) << 3) + DEF, 8)
        rows = ln2_v[pl.ds(g8, 8), :].astype(F32)
        oldx.append(subsum(jnp.where(wide((key_row(kk) & 7) == sub8), rows, 0.0)))

    def gated(v):
        tok = None
        while st["pend"] and st["pend"][0][0] <= st["step"]:
            t = st["pend"].pop(0)[1]
            tok = t if tok is None else tok | t
        if tok is None:
            return v
        u = pltpu.bitcast(v, U32)
        return pltpu.bitcast(jnp.concatenate([u[:, 0:LANES] | tok, u[:, LANES:]], axis=1), BF16)

    res = {}

    def c_units():
        pc.flush()
        p1, p2_ = hint["p1"], hint["p2"]
        cand_p, cand_x = [], []
        for pk_ in (p1, p2_):
            cp, cx = None, None
            for s in range(8):
                g8 = pl.multiple_of((jnp.clip(key_row(pk_[s, 0]) - L0, 0, RL - 1) >> 3) << 3, 8)
                vp = pq_v[pl.ds(g8, 8), :]
                vx = x_v[pl.ds(pl.multiple_of(g8 + (L0 + DEF), 8), 8), :].astype(F32)
                cp = vp if cp is None else jnp.where(jnp.concatenate([sub8 == s] * (NC + 2), axis=1), vp, cp)
                cx = vx if cx is None else jnp.where(wide(sub8 == s), vx, cx)
            cand_p.append(cp[:, 0:D] * jnp.concatenate([cp[:, D:]] * (NC // 2), axis=1))
            cand_x.append(cx)
        cand_p = jnp.concatenate(cand_p, axis=0).astype(BF16)
        cand_x = jnp.concatenate(cand_x, axis=0)
        ids_lo = key_row(jnp.broadcast_to(p1, (8, LANES)))
        ids_hi = jnp.where(sub8 < 6, key_row(jnp.broadcast_to(p2_, (8, LANES))),
                           jnp.where(sub8 == 6, key_row(oldk[0]), key_row(oldk[1])))
        res["ids"] = (ids_lo, ids_hi)
        parts = []
        for c in range(NC):
            parts.append(jnp.dot(cand_p, wload(mp_v, 0, D, slice(c * LANES, (c + 1) * LANES)), preferred_element_type=F32))
            yield
        xs = _layernorm(cand_x + jnp.concatenate(parts, axis=1))
        hi = jnp.where(wide(sub8 < 6), xs[8:16, :], jnp.where(wide(sub8 == 6), oldx[0], oldx[1]))
        res["xs"] = jnp.concatenate([xs[0:8, :], hi], axis=0).astype(BF16)

    def f_units():
        xs = res["xs"]
        acts = []
        for j in range(F // LANES):
            cs = slice(j * LANES, (j + 1) * LANES)
            g = jnp.dot(gated(xs), wload(wg_v, 0, D, cs), preferred_element_type=F32)
            yield
            u = jnp.dot(xs, wload(wu_v, 0, D, cs), preferred_element_type=F32)
            acts.append((g * jax.nn.sigmoid(g) * u).astype(BF16))
            yield
        act = jnp.concatenate(acts, axis=1)
        zf = pltpu.bitcast(zero_u, F32)
        ys = []
        KF = (F // D) * D
        for c in range(0, NC, 2):
            acc = jnp.concatenate([jnp.concatenate([zf, zf], axis=0)] * 2, axis=1)
            acc = acc + jnp.dot(gated(act[:, KF:]), wload(wd_v, KF, F - KF, slice(c * LANES, (c + 2) * LANES)),
                                preferred_element_type=F32)
            yield
            for cc in range(2):
                y = acc[:, cc * LANES:(cc + 1) * LANES]
                for k0 in range(0, KF, D):
                    y = y + jnp.dot(gated(act[:, k0:k0 + D]),
                                    wload(wd_v, k0, D, slice((c + cc) * LANES, (c + cc + 1) * LANES)),
                                    preferred_element_type=F32)
                    yield
                ys.append(y)
        res["y"] = jnp.concatenate(ys, axis=1)

    def side_units():
        yield from range(NPRE)
        yield from c_units()
        yield from range(NGAP)
        yield from f_units()

    side = side_units()

    def o_dot(lhs, rhs):
        p = pc.dot(lhs, rhs) if st["step"] < NPRE else jnp.dot(lhs, rhs, preferred_element_type=F32)
        next(side, None)
        st["step"] += 1
        return p

    def o_plain(r0, n):
        lhs = pltpu.bitcast(pqn_v[r0 // 2:(r0 + n) // 2, :], BF16)
        parts = []
        for c0 in range(0, NC, 2):
            acc = x_v[DEF + L0 + r0:DEF + L0 + r0 + n, c0 * LANES:(c0 + 2) * LANES].astype(F32)
            for k0 in range(0, D, 2 * LANES):
                acc = acc + o_dot(lhs[:, k0:k0 + 2 * LANES], wload(mp_v, k0, 2 * LANES, slice(c0 * LANES, (c0 + 2) * LANES)))
            parts.append(acc)
        return jnp.concatenate(parts, axis=1)

    toks = []
    r0 = 0
    pc.add(post_jobs(OCL[0][0], *OCL[1]), pc.t + 200, pc.t + 1000, QP_DELAY)
    for ci, (n, plain) in enumerate(OCL):
        h = o_plain(r0, n) if plain else o_part(o_dot, x_v, DEF + L0, r0, n)
        last = r0 + n == RL
        units = ln2_jobs(h, ln2_v, out_v, DEF + L0 + r0, -DEF, None, st, fast=last)
        posts = post_jobs(r0 + n + OCL[ci + 1][0], *OCL[ci + 2]) if ci + 2 < len(OCL) else []
        for k, job in enumerate(units):
            toks.append(job(toks[-LAG_L] if len(toks) >= LAG_L and not last else None))
            if posts:
                posts.pop(0)(toks[-1])
        if GLAG[ci] is not None:
            st["pend"].append((st["step"] + GLAG[ci],
                               pltpu.bitcast(jnp.broadcast_to(st["top1"], (8, LANES)), U32) & zero_u))
        r0 += n
        if last or r0 in OUT_AT:
            out_copy(L0 + st["sent"], r0 - st["sent"], 2 if last else 1).start()
            if not last:
                st["sent"] = r0
    for _ in side:
        st["step"] += 1

    keyv = best2(st["top1"], st["top2"])
    idx = [jnp.clip(key_row(kk[0, 0]), 0, S - 1) for kk in keyv]
    grp = [pl.multiple_of((ii >> 3) << 3, 8) for ii in idx]
    vgrp = [pl.multiple_of(gg + DEF, 8) for gg in grp]
    y = res["y"]
    ids_lo, ids_hi = res["ids"]
    hits = None
    yrows = []
    for c in range(2):
        m_lo = ids_lo == key_row(keyv[c])
        m_hi = ids_hi == key_row(keyv[c])
        yrows.append(subsum(jnp.where(wide(m_lo), y[0:8, :], 0.0) + jnp.where(wide(m_hi), y[8:16, :], 0.0)))
        hit = submax(jnp.where(m_lo | m_hi, 1, 0))
        hits = hit if hits is None else hits + hit
    hit_all = hits[0, 0] == 2

    tail0 = L0 + st["sent"]
    tail_copy = out_copy(tail0, S - tail0, 2)
    in_tail = jnp.maximum(grp[0], grp[1]) >= tail0
    two_groups = grp[1] != grp[0]

    def fix_copy(c):
        return out_copy(grp[c], 8, 3 + c)

    def finish(ysel):
        for c in range(2):
            hi = keyv[c] & jnp.int32(-65536)
            score = pltpu.bitcast(hi ^ ((hi >> 31) & 0x7FFF0000), F32)
            sel = (key_row(keyv[c]) & 7) == sub8
            upd = jnp.where(wide(sel), ysel[c] * wide(jax.nn.sigmoid(score)), 0.0)
            out_v[pl.ds(vgrp[c], 8), :] = (out_v[pl.ds(vgrp[c], 8), :].astype(F32) + upd).astype(BF16)
        fix_copy(0).start()

        @pl.when(two_groups)
        def _():
            fix_copy(1).start()

    out_copy(0, L0, 0).wait()
    out_copy(L0, tail0 - L0, 1).wait()

    @pl.when(in_tail)
    def _():
        tail_copy.wait()

    @pl.when(hit_all)
    def _():
        finish(yrows)

    @pl.when(jnp.logical_not(hit_all))
    def _():
        xsel = jnp.concatenate([ln2_v[pl.ds(vgrp[c], 8), :] for c in range(2)], axis=0)

        def ffn_tile(j, acc):
            cs = pl.ds(pl.multiple_of(j * LANES, LANES), LANES)
            g = jnp.dot(xsel, wload(wg_v, 0, D, cs), preferred_element_type=F32)
            u = jnp.dot(xsel, wload(wu_v, 0, D, cs), preferred_element_type=F32)
            a = (g * jax.nn.sigmoid(g) * u).astype(BF16)
            wd_t = pltpu.bitcast(wd_v[pl.ds(pl.multiple_of(j * (LANES // 2), LANES // 2), LANES // 2), 0:D], BF16)
            return acc + jnp.dot(a, wd_t, preferred_element_type=F32)

        yf = lax.fori_loop(0, F // LANES, ffn_tile, jnp.zeros((16, D), F32))
        finish([yf[0:8, :], yf[8:16, :]])

    @pl.when(jnp.logical_not(in_tail))
    def _():
        tail_copy.wait()

    fix_copy(0).wait()

    @pl.when(two_groups)
    def _():
        fix_copy(1).wait()


@jax.jit
def pallas_sequential_preLN__linear_attn_block__moe_arch_mod__prompt_kernel(
    A_x: jax.Array,
    A_wqkv: jax.Array,
    A_wo: jax.Array,
    B_x: jax.Array,
    B_w_r: jax.Array,
    B_w_gate: jax.Array,
    B_w_up: jax.Array,
    B_w_down: jax.Array,
):
    del B_x
    x = A_x.reshape(S, D)
    wr = B_w_r.reshape(NC, LANES)
    any_spec = pl.BlockSpec(memory_space=pl.ANY)
    out = pl.pallas_call(
        _kernel,
        out_shape=jax.ShapeDtypeStruct((S, D), BF16),
        in_specs=[any_spec] * 7,
        out_specs=any_spec,
        scratch_shapes=[
            pltpu.VMEM((S + DEF, D), BF16),
            pltpu.VMEM((D // 2, D), U32),
            pltpu.VMEM((D // 2, D), U32),
            pltpu.VMEM((2, D // 2, D), U32),
            pltpu.VMEM((NC, LANES), BF16),
            pltpu.VMEM((2, D // 2, F + LANES), U32),
            pltpu.VMEM((F // 2, D + LANES), U32),
            pltpu.VMEM((P0 // 2, D), U32),
            pltpu.VMEM((7 ** LA, S // NA // 2, DA), U32),
            pltpu.VMEM((7 ** LA, DA // 2, DA), U32),
            pltpu.VMEM((D // 2, P0), U32),
            pltpu.VMEM((DA // 2, 7 ** LA * MA), U32),
            pltpu.VMEM((D, LANES), F32),
            pltpu.VMEM((D, LANES), F32),
            pltpu.VMEM((RL, LANES), F32),
            pltpu.VMEM((D, D), F32),
            pltpu.VMEM((7, HD, HD), F32),
            pltpu.VMEM((D // 2, D), U32),
            pltpu.VMEM((7 ** LA, DA // 2, DA), U32),
            pltpu.VMEM((D // 2, D), U32),
            pltpu.VMEM((7 ** LO, DO // 2, DO), U32),
            pltpu.VMEM((max(TB2, RL), D + 2 * LANES), F32),
            pltpu.VMEM((RL // 2, D), U32),
            pltpu.VMEM((7 ** LO, max(TB2, RL) // NO // 2, DO), U32),
            pltpu.VMEM((DEF, D), F32),
            pltpu.VMEM((2, S + DEF, D), BF16),
            pltpu.VMEM((TB, D), F32),
            pltpu.VMEM((8, LANES), U32),
            pltpu.SemaphoreType.DMA((NSEM,)),
        ],
        compiler_params=pltpu.CompilerParams(vmem_limit_bytes=110 * 1024 * 1024, disable_bounds_checks=True,
                                             disable_semaphore_checks=True),
    )(x, A_wqkv, A_wo, wr, B_w_gate, B_w_up, B_w_down)
    return out.reshape(1, S, D)
```

```python
import jax
import jax.numpy as jnp
from jax import lax
import jax.experimental.pallas as pl
import jax.experimental.pallas.tpu as pltpu


S = 2048
D = 1024
F = 3584
H = 32
DH = D // H
LANES = 128
NC = D // LANES
HD = D // 2

LA = 2
LO = 1
NA, NO = 2 ** LA, 2 ** LO
DA, DO = D // NA, D // NO
P0 = 512
PB = S - P0
TX = 256
TB = 512
NB1 = PB // TB
MA = TB // NA
TB2 = 384
NB2 = 4
QA = 192
OCH = (128, 128, 128)
DEF = OCH[-1]
L0 = NB2 * TB2
RL = S - L0
QS = (256, 256)
OCL = ((128, False), (128, False), (128, False), (64, True), (64, True))
NPRE = 22
NGAP = 9
OUT_AT = (256, 384, 448)
GM = 32
NZ = 5
WQP = 5
LNU = 8
LAG = 5
LAG_L = 5
LN_DELAY = 800
LN2_DELAY = 900
JOB_DELAY = 500
POST_DELAY = 800
QP_DELAY = 400
WK5 = 66
C6LN = (1000, 8900)
C6WK = (1500, 8900)
P1LN = (60, 10500)
P1WP = (6800, 11000)
P1WQ = (8000, 12300)
P2U = (60, 2000)
EV2 = 300
GLAG = (None, None, None, 20, 8)

F32 = jnp.float32
BF16 = jnp.bfloat16
U32 = jnp.uint32
I32 = jnp.int32

XP = ((PB, 128), (PB + 128, 128), (PB + 256, 256), (0, TB), (TB, PB - TB))
WKP = ((0, 128), (128, 128), (256, 256), (512, 512))

SEM_X = 0
SEM_WK = SEM_X + len(XP)
SEM_WQ = SEM_WK + len(WKP)
SEM_W3 = SEM_WQ + 1
SEM_WR = SEM_W3 + 1
SEM_WGU = SEM_WR + 1
SEM_WD = SEM_WGU + 1
SEM_OUT = SEM_WD + 1
NSEM = SEM_OUT + 5

INT_MIN = -(2 ** 31)


def _layernorm(x, tok=None, w=None):
    s0 = x[:, 0:LANES]
    if tok is not None:
        s0 = s0 + jnp.concatenate([tok] * (x.shape[0] // 8), axis=0)
    for c in range(1, NC):
        s0 = s0 + x[:, c * LANES:(c + 1) * LANES]
    mu = jnp.sum(s0, axis=-1, keepdims=True) * (1.0 / D)
    xc = x - mu
    var = jnp.sum(xc * xc, axis=-1, keepdims=True) * (1.0 / D)
    rstd = lax.rsqrt(var + 1e-5)
    if w is None:
        return xc * rstd
    return xc * rstd, jnp.sum(xc * w, axis=-1, keepdims=True) * rstd


def _phi(t):
    return jnp.where(t > 0, t + 1.0, jnp.exp(t)) + 1e-6


def _n_off(a, b):
    return 32 * a + 8 * b


def _n_groups():
    pos = {(2 * o + e) * LANES + _n_off(a, b): (16 * e + 4 * b + a) * DH + 8 * o
           for o in range(4) for e in range(2) for a in range(4) for b in range(4)}
    return [pos[n] for n in sorted(pos)]


def _quads(b):
    h = len(b) // 2
    return [[r[j * h:(j + 1) * h] for r in b[i * h:(i + 1) * h]] for i in range(2) for j in range(2)]


def _badd(x, y):
    return [[a + b for a, b in zip(rx, ry)] for rx, ry in zip(x, y)]


def _bsub(x, y):
    return [[a - b for a, b in zip(rx, ry)] for rx, ry in zip(x, y)]


def _a_set(b):
    if len(b) == 1:
        return [b[0][0]]
    return [x for o in _a_ops(b) for x in _a_set(o)]


def _b_set(b):
    if len(b) == 1:
        return [b[0][0]]
    q11, q12, q21, q22 = _quads(b)
    ops = (_badd(q11, q22), q11, _bsub(q12, q22), _bsub(q21, q11), q22, _badd(q11, q12), _badd(q21, q22))
    return [x for o in ops for x in _b_set(o)]


def _b_in_a(i, levels):
    perm = (0, 2, 6, 5, 3, 4, 1)
    return sum(perm[(i // 7 ** l) % 7] * 7 ** l for l in range(levels))


def _strassen(prod, levels, base=0, fin=lambda k, q: q, init=None):
    if levels == 0:
        return [[prod(base)]]

    def m(i):
        return _strassen(prod, levels - 1, base * 7 + i)

    def seed(q, x):
        return x if init is None else _badd(_quads(init)[q], x)

    m2 = m(2)
    c22 = seed(3, m2)
    m4 = m(4)
    c12 = fin(1, _badd(seed(1, m2), m4))
    c11 = m4 if init is None else _bsub(_quads(init)[0], m4)
    m3 = m(3)
    c11 = _bsub(m3, c11) if init is None else _badd(c11, m3)
    m1 = m(1)
    c21 = fin(2, _badd(seed(2, m3), m1))
    c22 = _bsub(c22, m1)
    m0 = m(0)
    c11 = _badd(c11, m0)
    c22 = _badd(c22, m0)
    c11 = fin(0, _badd(c11, m(6)))
    c22 = fin(3, _badd(c22, m(5)))
    return [a + b for a, b in zip(c11, c12)] + [a + b for a, b in zip(c21, c22)]


def _goff(i, levels):
    return int(format(i, "0%db" % levels)[::-1], 2) if levels else 0


def _blocks(rows, n):
    w = rows[0].shape[1] // n
    return [[r[:, j * w:(j + 1) * w] for j in range(n)] for r in rows]


def _or_all(vals):
    acc = None
    for v in vals:
        v = pltpu.bitcast(v, U32)
        for g in range(v.shape[0] // 8):
            for c in range(v.shape[1] // LANES):
                p = v[g * 8:(g + 1) * 8, c * LANES:(c + 1) * LANES]
                acc = p if acc is None else acc | p
    return acc


def _raw_ops(levels):
    n = 2 ** levels
    names = [[_Tag((i, j)) for j in range(n)] for i in range(n)]
    return {op: t.ij for op, t in enumerate(_b_set(names)) if t.ij is not None}


class _Tag:
    def __init__(self, ij):
        self.ij = ij

    def __add__(self, other):
        return _Tag(None)

    __sub__ = __add__


def _a_ops(b):
    q11, q12, q21, q22 = _quads(b)
    return (_badd(q11, q22), _badd(q21, q22), q11, q22, _badd(q11, q12), _bsub(q21, q11), _bsub(q12, q22))


_A_FORM = (((0, 0), (1, 1), 1), ((1, 0), (1, 1), 1), ((0, 0),), ((1, 1),), ((0, 0), (0, 1), 1),
           ((1, 0), (0, 0), -1), ((0, 1), (1, 1), -1))
_B_FORM = (((0, 0), (1, 1), 1), ((0, 0),), ((0, 1), (1, 1), -1), ((1, 0), (0, 0), -1), ((1, 1),),
           ((0, 0), (0, 1), 1), ((1, 0), (1, 1), 1))
_C_FORM = (((0, 1), (3, 1), (4, -1), (6, 1)), ((2, 1), (4, 1)), ((1, 1), (3, 1)), ((0, 1), (1, -1), (2, 1), (5, 1)))


def _outer(form, get, n):
    h = n // 2

    def quad(q):
        return [[get(q[0] * h + i, q[1] * h + j) for j in range(h)] for i in range(h)]

    if len(form) == 1:
        return quad(form[0])
    return (_badd if form[2] > 0 else _bsub)(quad(form[0]), quad(form[1]))


def _gate(v, tok):
    u = pltpu.bitcast(v, U32)
    top = u[0:8, 0:LANES] | tok
    if u.shape[1] > LANES:
        top = jnp.concatenate([top, u[0:8, LANES:]], axis=1)
    return pltpu.bitcast(jnp.concatenate([top, u[8:, :]], axis=0) if u.shape[0] > 8 else top, BF16)


class _Pacer:
    def __init__(self, zero, every=0):
        self.zero, self.t, self.jobs, self.pend, self.tok = zero, 0, [], [], None
        self.every, self.last = every, -every

    def add(self, jobs, t0, t1, delay):
        for k, job in enumerate(jobs):
            self.jobs.append((t0 + k * (t1 - t0) // len(jobs), len(self.jobs), job, delay))
        self.jobs.sort(key=lambda e: e[:2])

    def due(self, dep, delay):
        if dep is not None:
            self.pend.append((self.t + delay, _or_all([dep])))

    def release(self, upto):
        while self.jobs and self.jobs[0][0] <= upto:
            _, _, job, delay = self.jobs.pop(0)
            self.due(job(self.tok), delay)

    def dot(self, lhs, rhs):
        self.release(self.t)
        ready = [d for t, d in self.pend if t <= self.t]
        if ready and self.t - self.last >= self.every:
            self.pend = [e for e in self.pend if e[0] > self.t]
            self.last = self.t
            lhs = _gate(lhs, _or_all(ready) & self.zero)
        res = jnp.dot(lhs, rhs, preferred_element_type=F32)
        self.t += lhs.shape[0] * (lhs.shape[1] // LANES) * (res.shape[1] // LANES) // 4
        self.tok = pltpu.bitcast(pltpu.bitcast(res[0:8, 0:LANES], U32) & self.zero, F32)
        return res

    def flush(self):
        self.release(1 << 30)


def _kernel(x_hbm, wqkv_hbm, wo_hbm, wr_hbm, wg_hbm, wu_hbm, wd_hbm, out_hbm,
            x_v, wk_v, wq_v, w3_v, wr_v, wgu_v, wd_v,
            ln1_v, xs_v, wks_v, pkt_v, pks_v, zacc_v, uacc_v, xw_v, g_v, gs_v, wqp_v, wqs_v, mp_v, ms_v,
            pq_v, pqn_v, pqs_v, attn_v, lo_v, lnf_v, zero_v, sems):

    ln2_v, out_v = lo_v.at[0], lo_v.at[1]

    wqkv_hbm, wo_hbm, wg_hbm, wu_hbm, wd_hbm = (r.bitcast(U32) for r in (wqkv_hbm, wo_hbm, wg_hbm, wu_hbm, wd_hbm))

    def wload(ref, r0, nr, cols):
        return pltpu.bitcast(ref[r0 // 2:(r0 + nr) // 2, cols], BF16)

    wv_v, wo_v = w3_v.at[0], w3_v.at[1]
    wg_v, wu_v = wgu_v.at[0], wgu_v.at[1]

    def x_copy(i):
        r0, n = XP[i]
        return pltpu.make_async_copy(x_hbm.at[pl.ds(r0, n), :], x_v.at[pl.ds(DEF + r0, n), :], sems.at[SEM_X + i])

    def out_copy(r0, n, s):
        return pltpu.make_async_copy(out_v.at[pl.ds(DEF + r0, n), :], out_hbm.at[pl.ds(r0, n), :],
                                     sems.at[SEM_OUT + s])

    def wk_copy(j):
        c0, n = WKP[j]
        return pltpu.make_async_copy(wqkv_hbm.at[:, pl.ds(D + c0, n)], wk_v.at[:, pl.ds(c0, n)],
                                     sems.at[SEM_WK + j])

    wq_copy = pltpu.make_async_copy(wqkv_hbm.at[:, pl.ds(0, D)], wq_v, sems.at[SEM_WQ])
    wr_copy = pltpu.make_async_copy(wr_hbm, wr_v, sems.at[SEM_WR])
    wd_copy = pltpu.make_async_copy(wd_hbm, wd_v.at[:, pl.ds(0, D)], sems.at[SEM_WD])
    wg_copy = pltpu.make_async_copy(wg_hbm, wg_v.at[:, pl.ds(0, F)], sems.at[SEM_WGU])
    wu_copy = pltpu.make_async_copy(wu_hbm, wu_v.at[:, pl.ds(0, F)], sems.at[SEM_WGU])

    x_copy(0).start()
    wk_copy(0).start()
    x_copy(1).start()
    wr_copy.start()
    for j in range(1, len(WKP)):
        wk_copy(j).start()
    for j in range(2, len(XP)):
        x_copy(j).start()
    wq_copy.start()
    pltpu.make_async_copy(wqkv_hbm.at[:, pl.ds(2 * D, D)], wv_v, sems.at[SEM_W3]).start()
    pltpu.make_async_copy(wo_hbm, wo_v, sems.at[SEM_W3]).start()
    wg_copy.start()
    wu_copy.start()
    wd_copy.start()

    def ln1_rows(xr, xr0, lnr, r0, n):
        ln = _layernorm(xr[xr0:xr0 + n, :].astype(F32)).astype(BF16)
        lnr[r0 // 2:(r0 + n) // 2, :] = pltpu.bitcast(ln, U32)

    def ln1_set(pc, xr, xr0, xsr, a0, n, t0, t1):
        def unit(j):
            def job(tok):
                ln = _layernorm(xr[xr0 + j * LNU:xr0 + (j + 1) * LNU, :].astype(F32), tok)
                lnf_v[j * LNU:(j + 1) * LNU, :] = ln
                return _or_all([ln[:, 0:LANES], ln[:, D - LANES:D]])
            return job

        def piece(j0, c0, o):
            def job(tok):
                def get(i, f):
                    r = (j0 + 2 * _goff(i, LA)) * LNU
                    v = lnf_v[r:r + 16, f * DA + c0:f * DA + c0 + LANES]
                    return v + jnp.concatenate([tok, tok], axis=0) if (i + f) % (NA // 2 + 1) == 0 else v

                r = (a0 + (j0 // (2 * NA)) * 16) // 2
                ops = _a_set(_outer(_A_FORM[o], get, NA))
                for op, v in enumerate(ops):
                    xsr.at[o * len(ops) + op][r:r + 8, c0:c0 + LANES] = pltpu.bitcast(v.astype(BF16), U32)
                return _or_all([v[0:8, :] for v in [ops[0]] + ops[5:7]])
            return job

        grp = 2 * NA
        ng = n // LNU // grp
        dt = (t1 - t0 - LN_DELAY) // (ng + 1)
        for g in range(ng):
            pc.add([unit(g * grp + j) for j in range(grp)], t0 + g * dt, t0 + (g + 1) * dt, LN_DELAY)
            s = t0 + (g + 1) * dt + LN_DELAY
            pc.add([piece(g * grp, c0, o) for c0 in range(0, DA, LANES) for o in range(7)], s, s + dt, JOB_DELAY)

    def ln1_load(lnr, r0, n):
        return pltpu.bitcast(lnr[r0 // 2:(r0 + n) // 2, :], BF16)

    def k_mm(r0, n, c0, nc):
        return jnp.dot(ln1_load(ln1_v, r0, n), wload(wk_v, 0, D, slice(c0, c0 + nc)), preferred_element_type=F32)

    def z_acc(pkts, c0, first=False):
        zs = None
        for pkt in pkts:
            for j in range(pkt.shape[1] // LANES):
                p = pkt[:, j * LANES:(j + 1) * LANES]
                zs = p if zs is None else zs + p
        if first:
            zacc_v[c0:c0 + zs.shape[0], :] = zs
        else:
            zacc_v[c0:c0 + zs.shape[0], :] += zs

    def k_post(k, p0, c0, first=False):
        n, nc = k.shape
        pkt = _phi(k).T
        pkt_v[c0 // 2:(c0 + nc) // 2, p0:p0 + n] = pltpu.bitcast(pkt.astype(BF16), U32)
        z_acc([pkt], c0, first)
        return pkt[nc - 8:nc, n - LANES:n]

    def g_acc(r0, n, c0, nc, first=False, pc=None):
        h, w = (nc, D) if pc is None else (LANES, LANES)
        for f0 in range(c0, c0 + nc, h):
            for j0 in range(0, D, w):
                lhs = pltpu.bitcast(pkt_v[f0 // 2:(f0 + h) // 2, r0:r0 + n], BF16)
                rhs = pltpu.bitcast(ln1_v[r0 // 2:(r0 + n) // 2, j0:j0 + w], BF16)
                g = jnp.dot(lhs, rhs, preferred_element_type=F32) if pc is None else pc.dot(lhs, rhs)
                if first:
                    g_v[f0:f0 + h, j0:j0 + w] = g
                else:
                    g_v[f0:f0 + h, j0:j0 + w] += g

    def k_paced(pc, r0, c0, nc, first):
        for j0 in range(c0, c0 + nc, LANES):
            for t0 in range(r0, r0 + TX, LANES):
                k = None
                for k0 in range(0, D, TX):
                    p = pc.dot(ln1_load(ln1_v, t0, LANES)[:, k0:k0 + TX], wload(wk_v, k0, TX, slice(j0, j0 + LANES)))
                    k = p if k is None else k + p
                pc.due(k_post(k, t0, j0, first and t0 == r0), POST_DELAY)

    attn_v[...] = jnp.zeros_like(attn_v)
    zero_v[...] = jnp.zeros_like(zero_v)

    def gs_zero(o0, o1):
        gs_v[o0:o1] = jnp.zeros((o1 - o0, HD, HD), F32)

    x_copy(0).wait()
    ln1_rows(x_v, DEF + PB, ln1_v, 0, 128)
    gs_zero(0, 1)
    wk_copy(0).wait()
    ka = k_mm(0, 128, 0, 128)
    gs_zero(1, 2)
    x_copy(1).wait()
    wr_copy.wait()
    gs_zero(2, 3)
    ln1_rows(x_v, DEF + PB + 128, ln1_v, 128, 128)
    k_post(ka, 0, 0, first=True)
    g_acc(0, 128, 0, 128, first=True)
    wk_copy(1).wait()
    gs_zero(3, NZ)
    k_post(k_mm(128, 128, 0, 128), 128, 0)
    k_post(k_mm(0, TX, 128, 128), 0, 128, first=True)
    g_acc(128, 128, 0, 128)

    def w_job(src_ref, dst_ref, levels, r0, c0, o):
        n = 2 ** levels
        w, raw, inner = D // n, _raw_ops(levels), 7 ** (levels - 1)

        def job(tok):
            def cut(i, j):
                return src_ref[(i * w + r0) // 2:(i * w + r0) // 2 + 8, j * w + c0:j * w + c0 + LANES]

            def get(i, j):
                u = cut(i, j)
                return pltpu.bitcast(u if tok is None else u | pltpu.bitcast(tok, U32), BF16).astype(F32)

            ops = []
            for op, v in enumerate(_b_set(_outer(_B_FORM[o], get, n))):
                dst = dst_ref.at[o * inner + op]
                if o * inner + op in raw:
                    dst[r0 // 2:r0 // 2 + 8, c0:c0 + LANES] = cut(*raw[o * inner + op])
                else:
                    dst[r0 // 2:r0 // 2 + 8, c0:c0 + LANES] = pltpu.bitcast(v.astype(BF16), U32)
                    ops.append(v)
            return _or_all(ops[0:1] + ops[-2:]) if ops else None
        return job

    def wk_jobs_of(outer):
        return [w_job(wk_v, wks_v, LA, r0, c0, o) for r0 in range(0, DA, 16) for c0 in range(0, DA, LANES)
                for o in outer]

    wk_copy(2).wait()
    pc = _Pacer(zero_v[...])
    pc.add(wk_jobs_of((1, 3)), 500, 2200, JOB_DELAY)
    k_paced(pc, 0, 256, 256, True)
    g_acc(0, TX, 128, 128, True, pc)
    g_acc(0, TX, 256, 256, True, pc)
    pc.flush()
    wk_copy(3).wait()
    wk_jobs = wk_jobs_of((0, 2, 4, 5, 6))
    pc = _Pacer(zero_v[...])
    pc.add(wk_jobs[:WK5], 500, 2700, JOB_DELAY)
    k_paced(pc, 0, 512, 512, True)
    g_acc(0, TX, 512, 256, True, pc)
    pc.flush()
    x_copy(2).wait()
    x_copy(3).wait()
    pc = _Pacer(zero_v[...])
    ln1_set(pc, x_v, DEF, xs_v, 0, TB, *C6LN)
    pc.add(wk_jobs[WK5:], *C6WK, JOB_DELAY)
    ln1_rows(x_v, DEF + PB + TX, ln1_v, TX, TX)
    g_acc(0, TX, 768, 256, True, pc)
    k_paced(pc, TX, 0, D, False)
    for c0 in range(0, D, 256):
        g_acc(TX, TX, c0, 256, False, pc)
    pc.flush()

    def xs_load(xsr, op, a0, m):
        return pltpu.bitcast(xsr[op, a0 // 2:(a0 + m) // 2, :], BF16)

    def k_step(pc, xsr, j0):
        def fin(_, q):
            q = [[_phi(v).T for v in r] for r in q]
            pc.due(_or_all([v[LANES - 8:LANES, :] for r in q for v in r]), POST_DELAY)
            return q

        cb = _strassen(lambda i: pc.dot(xs_load(xsr, i, 0, MA), pltpu.bitcast(wks_v[i, :, j0:j0 + LANES], BF16)),
                       LA, fin=fin)
        outer = _a_ops([[cb[i][f] for i in range(NA)] for f in range(NA)])
        for half, o in ((0, outer[4]), (1, outer[1])):
            for f, rowb in enumerate(o):
                z_acc(rowb, half * HD + f * DA + j0)
        ops = [v for o in outer for v in _a_set(o)]
        for op, v in enumerate(ops):
            pks_v[j0 // 2:(j0 + LANES) // 2, op * MA:(op + 1) * MA] = pltpu.bitcast(v.astype(BF16), U32)
        pc.due(_or_all([v[LANES - 8:LANES, :] for v in (ops[0], ops[-1], ops[-2])]), 2 * POST_DELAY)

    def g_step(pc, xsr, r0, later):
        def old(o, f, c):
            v = gs_v[o, f * DA + r0:f * DA + r0 + GM, c * DA:(c + 1) * DA]
            return v if o < NZ else jnp.where(later, v, 0.0)

        for o in range(7):
            cb = _strassen(lambda i: pc.dot(pltpu.bitcast(pks_v[r0 // 2:(r0 + GM) // 2, i * MA:(i + 1) * MA], BF16),
                                            xs_load(xsr, _b_in_a(i, LA), 0, MA)), LA - 1, base=o,
                           init=[[old(o, f, c) for c in range(NA // 2)] for f in range(NA // 2)])
            for f in range(NA // 2):
                for c in range(NA // 2):
                    gs_v[o, f * DA + r0:f * DA + r0 + GM, c * DA:(c + 1) * DA] = cb[f][c]

    def wq_jobs(u0, nr):
        span = (NA - 1) * DA + 16 * nr
        u0 = u0 if isinstance(u0, int) else pl.multiple_of(u0, 8)
        srcr, permr = wq_v.at[pl.ds(u0, span // 2), :], wqp_v.at[pl.ds(u0, span // 2), :]
        dstr = wqs_v.at[:, pl.ds(u0, 8 * nr), :]
        oct_ = (lax.broadcasted_iota(I32, (8, LANES), 1) % DH) // 8

        def perm(r, e):
            def job(tok):
                blk = [srcr[r // 2:r // 2 + 8, (4 * e + b) * LANES:(4 * e + b + 1) * LANES] | pltpu.bitcast(tok, U32)
                       for b in range(4)]
                outs = []
                for o in range(4):
                    v = blk[o]
                    for b in range(4):
                        if b != o:
                            v = jnp.where(oct_ == b, pltpu.roll(blk[b], (8 * (b - o)) % LANES, 1), v)
                    permr[r // 2:r // 2 + 8, (2 * o + e) * LANES:(2 * o + e + 1) * LANES] = v
                    outs.append(v)
                return _or_all(outs)
            return job

        return ([perm(i * DA + r0, e) for r0 in range(0, 16 * nr, 16) for i in range(NA) for e in range(2)],
                [w_job(permr, dstr, LA, r0, c0, o) for r0 in range(0, 16 * nr, 16)
                 for c0 in range(0, DA, LANES) for o in range(7)])

    def p1(i, carry):
        xsr = xs_v.at[:, pl.ds(pl.multiple_of(i * (MA // 2), MA // 2), MA), :]
        xr = x_v.at[pl.ds(pl.multiple_of((i + 1) * TB, TB), TB + DEF), :]

        pc = _Pacer(zero_v[...])
        ln1_set(pc, xr, DEF, xsr, MA, TB, *P1LN)
        perms, sets = wq_jobs(i * (8 * WQP), WQP)
        pc.add(perms, *P1WP, JOB_DELAY)
        pc.add(sets, *P1WQ, JOB_DELAY)
        for j0 in range(0, DA, LANES):
            k_step(pc, xsr, j0)
        for r0 in range(0, DA, GM):
            g_step(pc, xsr, r0, i > 0)
        pc.flush()
        return carry

    x_copy(4).wait()
    wq_copy.wait()
    lax.fori_loop(0, NB1, p1, 0)

    pltpu.make_async_copy(w3_v, w3_v, sems.at[SEM_W3]).wait()
    zero_u = zero_v[...]
    zrow = jnp.sum(jnp.concatenate([zacc_v[r:r + 8, :] for r in _n_groups()], axis=0).T, axis=0, keepdims=True)
    wr8 = wr_v[...].astype(F32)
    wr_row = jnp.concatenate([wr8[c:c + 1, :] for c in range(NC)], axis=1)

    row_h = lax.broadcasted_iota(I32, (LANES, LANES), 0) // DH
    col_h = lax.broadcasted_iota(I32, (LANES, LANES), 1) // DH
    diag = row_h == col_h

    def colsum(t):
        acc = t[:, 0:LANES]
        for c in range(1, NC):
            acc = acc + t[:, c * LANES:(c + 1) * LANES]
        return acc

    wrc = wr_row - jnp.sum(wr_row, axis=-1, keepdims=True) * (1.0 / D)
    m_raw = _raw_ops(LO)

    def kv_part(c):
        cs = slice(c * LANES, (c + 1) * LANES)
        kv = None
        for k0 in range(0, D, TX):
            g = g_v[cs, k0:k0 + TX]
            for o, sign in _C_FORM[(c * LANES // HD) * 2 + k0 // HD]:
                t = gs_v[o, c * LANES % HD:c * LANES % HD + LANES, k0 % HD:k0 % HD + TX]
                g = g + t if sign > 0 else g - t
            p = pc.dot(g.astype(BF16), wload(wv_v, k0, TX, cs))
            kv = p if kv is None else kv + p
        return jnp.where(diag, kv, 0.0)

    def m_part(c, kvs):
        e, b = c // 4, c % 4
        for j0 in range(0, DO, LANES):
            ms = [jnp.concatenate(
                [pc.dot(kv, wload(wo_v, (c + k) * LANES, LANES, slice(f * DO + j0, f * DO + j0 + LANES)))
                 for f in range(NO)], axis=1) for k, kv in enumerate(kvs)]
            deps = []
            for a in range(4):
                rows = [jnp.concatenate([m[a * DH + 8 * o:a * DH + 8 * o + 8, :] for m in ms], axis=0)
                        for o in range(4)]
                for o in range(4):
                    r = ((2 * o + e) * LANES + _n_off(a, b)) // 2
                    for f in range(NO):
                        mp_v[r:r + 8, f * DO + j0:f * DO + j0 + LANES] = pltpu.bitcast(
                            rows[o][:, f * LANES:(f + 1) * LANES].astype(BF16), U32)
                for t in range(4 // NO):
                    r = ((2 * t + e) * LANES + _n_off(a, b)) // 2
                    for op, v in enumerate(_b_set(_blocks(rows[t::4 // NO], NO))):
                        if op not in m_raw:
                            ms_v.at[op][r:r + 8, j0:j0 + LANES] = pltpu.bitcast(v.astype(BF16), U32)
                            deps.append(v[0:8, 0:LANES])
            pc.due(_or_all(deps[::4]), POST_DELAY)

    pc = _Pacer(zero_u)
    pc.due(jnp.broadcast_to(zrow, (8, D)), 1000)
    perms, sets = wq_jobs(NB1 * 8 * WQP, DA // 16 - NB1 * WQP)
    pc.add(perms, 60, 700, JOB_DELAY)
    pc.add(sets, 1300, 3500, JOB_DELAY)
    kv_prev = None
    for c in range(0, NC + 2, 2):
        kvs = [kv_part(c).astype(BF16), kv_part(c + 1).astype(BF16)] if c < NC else None
        if c:
            m_part(c - 2, kv_prev)
        kv_prev = kvs
    pc.flush()

    def make_key(score, row):
        b = pltpu.bitcast(score, I32)
        srt = b ^ ((b >> 31) & 0x7FFFFFFF)
        return (srt & jnp.int32(-65536)) | (0xFFFF - row)

    def push_keys(key, top1, top2):
        for gidx in range(key.shape[0] // 8):
            kx = key[gidx * 8:(gidx + 1) * 8, :]
            top2 = jnp.maximum(top2, jnp.minimum(top1, kx))
            top1 = jnp.maximum(top1, kx)
        return top1, top2

    lane = lax.broadcasted_iota(I32, (1, LANES), 1)

    def interleave(parts):
        return jnp.concatenate([p[g * 16:(g + 1) * 16, :] for g in range(parts[0].shape[0] // 16) for p in parts],
                               axis=0)

    def q_part(pc, xsr, l0, r0, n, hint=None):
        m = n // NA
        sums = {}

        def park(v, g, c):
            for t in range(m // 16):
                r = r0 + (t * NA + g) * 16
                pq_v[r:r + 16, c * LANES:(c + 1) * LANES] = v[t * 16:(t + 1) * 16, :]

        def fin(k, q):
            q = [[_phi(v) for v in r] for r in q]
            deps = []
            for a, r in enumerate(q):
                for b, v in enumerate(r):
                    i, c = (k // 2) * (NA // 2) + a, (((k % 2) * (NA // 2) + b) * DA + j0) // LANES
                    park(v, _goff(i, LA), c)
                    for name, row in (("z", zrow),) + ((("u", hint["u"]),) if hint else ()):
                        t = v * row[:, c * LANES:(c + 1) * LANES]
                        key = (name, _goff(i, LA), c % 2)
                        sums[key] = t if key not in sums else sums[key] + t
                deps.append(sums[key])
            if hint:
                pc.due(_or_all(deps), POST_DELAY)
            return q

        for j0 in range(0, DA, LANES):
            _strassen(lambda i: pc.dot(xs_load(xsr, i, (l0 + r0) // NA, m),
                                       pltpu.bitcast(wqs_v[i, :, j0:j0 + LANES], BF16)), LA, fin=fin)
        if hint:
            pc.flush()
        den = jnp.concatenate([sums["z", g, e] for g in range(NA) for e in range(2)], axis=0)
        for s in (1, 2, 4):
            den = den + jnp.where((lane & s) == 0, pltpu.roll(den, LANES - s, 1), pltpu.roll(den, s, 1))
        inv_all = 1.0 / (den + 1e-6)

        def inv_of(g):
            return [inv_all[(g * 2 + e) * m:(g * 2 + e + 1) * m, :] for e in range(2)]

        for g in range(NA):
            for e in range(2):
                park(inv_of(g)[e], g, NC + e)
        if hint:
            for g in range(NA):
                starts = [r0 + (t * NA + g) * 16 for t in range(m // 16)]
                num = jnp.sum(jnp.concatenate([xw_v[t:t + 16, :] for t in starts], axis=0)
                              + sums["u", g, 0] * inv_of(g)[0] + sums["u", g, 1] * inv_of(g)[1],
                              axis=-1, keepdims=True)
                row = jnp.concatenate([(l0 + t) + lax.broadcasted_iota(I32, (16, 1), 0) for t in starts], axis=0)
                hint["p1"], hint["p2"] = push_keys(make_key(num, row), hint["p1"], hint["p2"])
            pc.due(jnp.broadcast_to(hint["p1"], (8, LANES)), 1200)


    def post_jobs(r0, n, plain=False):
        def scaled(t, c0, w, tok):
            inv = pq_v[t:t + 16, D:D + 2 * LANES]
            if tok is not None:
                inv = inv + jnp.concatenate([jnp.concatenate([tok, tok], axis=0)] * 2, axis=1)
            return pq_v[t:t + 16, c0:c0 + w] * jnp.concatenate([inv] * (w // (2 * LANES)), axis=1)

        def post_plain(t):
            def job(tok):
                v = scaled(t, 0, D, tok)
                pqn_v[t // 2:t // 2 + 8, :] = pltpu.bitcast(v.astype(BF16), U32)
                return v[0:8, 0:LANES]
            return job

        def post(t0, outer):
            def job(tok):
                deps = []
                for c0 in range(0, DO, 2 * LANES):
                    blk = {}

                    def get(i, f):
                        if (i, f) not in blk:
                            blk[i, f] = scaled(t0 + _goff(i, LO) * 16, f * DO + c0, 2 * LANES, tok)
                        return blk[i, f]

                    for o in outer:
                        ops = _a_set(_outer(_A_FORM[o], get, NO))
                        for op, v in enumerate(ops):
                            pqs_v.at[o * len(ops) + op][t0 // NO // 2:t0 // NO // 2 + 8, c0:c0 + 2 * LANES] = (
                                pltpu.bitcast(v.astype(BF16), U32))
                        deps.append(ops[0][0:8, 0:LANES])
                return _or_all(deps)
            return job

        if plain:
            return [post_plain(t) for t in range(r0, r0 + n, 16)]
        outers = [range(7)] if LO == 1 else [(o,) for o in range(7)]
        return [post(t0, outer) for t0 in range(r0, r0 + n, 16 * NO) for outer in outers]

    def m_operand(i, c0, c1):
        if i not in m_raw:
            return pltpu.bitcast(ms_v[i, :, c0 * LANES:c1 * LANES], BF16)
        bi, bj = m_raw[i]
        return wload(mp_v, bi * DO, DO, slice(bj * DO + c0 * LANES, bj * DO + c1 * LANES))

    def o_part(dot, xr, x0, r0, n):
        a0, m = r0 // NO, n // NO
        nw = LANES * NO // 2
        cols = [[[] for _ in range(NO)] for _ in range(NO)]
        for c0 in range(0, DO, nw):
            init = [[jnp.concatenate(
                [xr[x0 + r0 + (g * NO + _goff(i, LO)) * 16:x0 + r0 + (g * NO + _goff(i, LO) + 1) * 16,
                    f * DO + c0:f * DO + c0 + nw] for g in range(m // 16)], axis=0).astype(F32)
                for f in range(NO)] for i in range(NO)]
            cb = _strassen(lambda i: dot(pltpu.bitcast(pqs_v[i, a0 // 2:(a0 + m) // 2, :], BF16),
                                         m_operand(i, c0 // LANES, (c0 + nw) // LANES)), LO, init=init)
            for i in range(NO):
                for f in range(NO):
                    cols[i][f].append(cb[i][f])
        parts = [None] * NO
        for i in range(NO):
            parts[_goff(i, LO)] = jnp.concatenate([c for f in range(NO) for c in cols[i][f]], axis=1)
        return interleave(parts)

    def ln2_unit(h, l2r, outr, r0, row0, valid, top1, top2, tok, fast=False):
        n = h.shape[0]
        if fast:
            ln2, r = _layernorm(h, tok, wr_row)
        else:
            ln2 = _layernorm(h, tok)
            r = jnp.sum(ln2 * wr_row, axis=-1, keepdims=True)
        l2r[r0:r0 + n, :] = ln2.astype(BF16)
        res = h + ln2
        outr[r0:r0 + n, :] = res.astype(BF16)
        r = r.astype(BF16).astype(F32) + 0.0
        key = make_key(r, (row0 + r0) + lax.broadcasted_iota(I32, (n, 1), 0))
        if valid is not None:
            key = jnp.where(valid, key, INT_MIN)
        top1, top2 = push_keys(key, top1, top2)
        ntok = pltpu.bitcast(pltpu.bitcast(jnp.broadcast_to(r[n - 8:n, :], (8, LANES)), U32) & zero_u, F32)
        return top1, top2, ntok

    def ln2_jobs(h, l2r, outr, r0, row0, valid, st, fast=False):
        def unit(j):
            def job(tok):
                st["top1"], st["top2"], dep = ln2_unit(h[j * LNU:(j + 1) * LNU, :], l2r, outr, r0 + j * LNU, row0,
                                                       valid, st["top1"], st["top2"], tok, fast)
                return dep
            return job
        return [unit(j) for j in range(h.shape[0] // LNU)]

    QC = 16 * 7 ** LA / 8 ** LA

    def p2(i, carry):
        st = dict(top1=carry[0], top2=carry[1])
        b0 = pl.multiple_of(i * TB2, 16)
        xsr = xs_v.at[:, pl.ds(pl.multiple_of(i * (TB2 // NA // 2), 8), TB2 // NA // 2), :]
        xr = x_v.at[pl.ds(b0, TB2 + DEF), :]
        l2r = ln2_v.at[pl.ds(b0, TB2 + DEF), :]
        outr = out_v.at[pl.ds(b0, TB2 + DEF), :]
        row0 = b0 - DEF
        pc = _Pacer(zero_u)
        toks = []

        def chain(jobs):
            for job in jobs:
                toks.append(job(toks[-LAG] if len(toks) >= LAG else None))

        chain(ln2_jobs(attn_v, l2r, outr, 0, row0, i > 0, st))

        @pl.when(i > 0)
        def _():
            out_copy(pl.multiple_of((i - 1) * TB2, 16), TB2, 0).start()

        pc.due(toks[-1], QA * QC)

        nu, nx = D // NB2, RL // NB2
        mr = mp_v.at[pl.ds(pl.multiple_of(i * (nu // 2), 8), nu // 2), :]
        ur = uacc_v.at[pl.ds(pl.multiple_of(i * nu, 8), nu), :]
        xl = x_v.at[pl.ds(pl.multiple_of(DEF + L0 + i * nx, 16), nx), :]
        xwr = xw_v.at[pl.ds(pl.multiple_of(i * nx, 8), nx), :]

        def hint_job(load, dst, r):
            def job(tok):
                v = colsum(load(r).astype(F32) * wrc) + jnp.concatenate([tok, tok], axis=0)
                dst[r:r + 16, :] = v
                return v
            return job

        pc.add([hint_job(lambda r: wload(mr, r, 16, slice(None)), ur, r) for r in range(0, nu, 16)]
               + [hint_job(lambda r: xl[r:r + 16, :], xwr, r) for r in range(0, nx, 16)], *P2U, JOB_DELAY)
        for r0, n in ((0, QA), (QA, TB2 - QA)):
            q_part(pc, xsr, 0, r0, n)
            for job in post_jobs(r0, n):
                job(None)
        r0 = 0
        for n in OCH[:-1]:
            chain(ln2_jobs(o_part(pc.dot, xr, DEF, r0, n), l2r, outr, DEF + r0, row0, None, st))
            r0 += n
        attn_v[...] = o_part(pc.dot, xr, DEF, r0, DEF)
        return st["top1"], st["top2"]

    init = jnp.full((8, 1), INT_MIN, I32)
    top1, top2 = lax.fori_loop(0, NB2, p2, (init, init))

    wg_copy.wait()
    wu_copy.wait()
    wd_copy.wait()
    sub8 = lax.broadcasted_iota(I32, (8, LANES), 0)
    urow = jnp.sum(uacc_v[...].T, axis=0, keepdims=True)

    def submax(v):
        for sh in (4, 2, 1):
            v = jnp.maximum(v, pltpu.roll(v, sh, 0))
        return v

    def subsum(v):
        for sh in (4, 2, 1):
            v = v + pltpu.roll(v, sh, 0)
        return v

    def best2(t1, t2):
        t1 = jnp.broadcast_to(t1, (8, LANES))
        t2 = jnp.broadcast_to(t2, (8, LANES))
        k1v = submax(t1)
        return k1v, submax(jnp.where(t1 == k1v, t2, t1))

    def key_row(k):
        return 0xFFFF - (k & 0xFFFF)

    def wide(m):
        return jnp.concatenate([m] * NC, axis=1)

    st = dict(top1=top1, top2=top2, pend=[], step=0, sent=0)
    pc = _Pacer(zero_u, EV2)
    hint = dict(u=urow, p1=init, p2=init)

    pc.add(ln2_jobs(attn_v, ln2_v, out_v, L0, -DEF, None, st), 60, QS[0] * QC - 600, LN2_DELAY)
    r0 = 0
    for k, n in enumerate(QS):
        q_part(pc, xs_v, L0, r0, n, hint)
        if k == 0:
            out_copy(L0 - TB2, TB2, 0).start()
            top1, top2 = st["top1"], st["top2"]
            pc.add(post_jobs(0, OCL[0][0], OCL[0][1]), pc.t + 600, pc.t + (RL - n) * QC - 300, QP_DELAY)
        r0 += n
    pc.every = 0
    oldk = best2(top1, top2)
    oldx = []
    for kk in oldk:
        g8 = pl.multiple_of(((jnp.clip(key_row(kk[0, 0]), 0, S - 1) >> 3) << 3) + DEF, 8)
        rows = ln2_v[pl.ds(g8, 8), :].astype(F32)
        oldx.append(subsum(jnp.where(wide((key_row(kk) & 7) == sub8), rows, 0.0)))

    def gated(v):
        tok = None
        while st["pend"] and st["pend"][0][0] <= st["step"]:
            t = st["pend"].pop(0)[1]
            tok = t if tok is None else tok | t
        if tok is None:
            return v
        u = pltpu.bitcast(v, U32)
        return pltpu.bitcast(jnp.concatenate([u[:, 0:LANES] | tok, u[:, LANES:]], axis=1), BF16)

    res = {}

    def c_units():
        pc.flush()
        p1, p2_ = hint["p1"], hint["p2"]
        cand_p, cand_x = [], []
        for pk_ in (p1, p2_):
            cp, cx = None, None
            for s in range(8):
                g8 = pl.multiple_of((jnp.clip(key_row(pk_[s, 0]) - L0, 0, RL - 1) >> 3) << 3, 8)
                vp = pq_v[pl.ds(g8, 8), :]
                vx = x_v[pl.ds(pl.multiple_of(g8 + (L0 + DEF), 8), 8), :].astype(F32)
                cp = vp if cp is None else jnp.where(jnp.concatenate([sub8 == s] * (NC + 2), axis=1), vp, cp)
                cx = vx if cx is None else jnp.where(wide(sub8 == s), vx, cx)
            cand_p.append(cp[:, 0:D] * jnp.concatenate([cp[:, D:]] * (NC // 2), axis=1))
            cand_x.append(cx)
        cand_p = jnp.concatenate(cand_p, axis=0).astype(BF16)
        cand_x = jnp.concatenate(cand_x, axis=0)
        ids_lo = key_row(jnp.broadcast_to(p1, (8, LANES)))
        ids_hi = jnp.where(sub8 < 6, key_row(jnp.broadcast_to(p2_, (8, LANES))),
                           jnp.where(sub8 == 6, key_row(oldk[0]), key_row(oldk[1])))
        res["ids"] = (ids_lo, ids_hi)
        parts = []
        for c in range(NC):
            parts.append(jnp.dot(cand_p, wload(mp_v, 0, D, slice(c * LANES, (c + 1) * LANES)), preferred_element_type=F32))
            yield
        xs = _layernorm(cand_x + jnp.concatenate(parts, axis=1))
        hi = jnp.where(wide(sub8 < 6), xs[8:16, :], jnp.where(wide(sub8 == 6), oldx[0], oldx[1]))
        res["xs"] = jnp.concatenate([xs[0:8, :], hi], axis=0).astype(BF16)

    def f_units():
        xs = res["xs"]
        acts = []
        for j in range(F // LANES):
            cs = slice(j * LANES, (j + 1) * LANES)
            g = jnp.dot(gated(xs), wload(wg_v, 0, D, cs), preferred_element_type=F32)
            yield
            u = jnp.dot(xs, wload(wu_v, 0, D, cs), preferred_element_type=F32)
            acts.append((g * jax.nn.sigmoid(g) * u).astype(BF16))
            yield
        act = jnp.concatenate(acts, axis=1)
        zf = pltpu.bitcast(zero_u, F32)
        ys = []
        KF = (F // D) * D
        for c in range(0, NC, 2):
            acc = jnp.concatenate([jnp.concatenate([zf, zf], axis=0)] * 2, axis=1)
            acc = acc + jnp.dot(gated(act[:, KF:]), wload(wd_v, KF, F - KF, slice(c * LANES, (c + 2) * LANES)),
                                preferred_element_type=F32)
            yield
            for cc in range(2):
                y = acc[:, cc * LANES:(cc + 1) * LANES]
                for k0 in range(0, KF, D):
                    y = y + jnp.dot(gated(act[:, k0:k0 + D]),
                                    wload(wd_v, k0, D, slice((c + cc) * LANES, (c + cc + 1) * LANES)),
                                    preferred_element_type=F32)
                    yield
                ys.append(y)
        res["y"] = jnp.concatenate(ys, axis=1)

    def side_units():
        yield from range(NPRE)
        yield from c_units()
        yield from range(NGAP)
        yield from f_units()

    side = side_units()

    def o_dot(lhs, rhs):
        p = pc.dot(lhs, rhs) if st["step"] < NPRE else jnp.dot(lhs, rhs, preferred_element_type=F32)
        next(side, None)
        st["step"] += 1
        return p

    def o_plain(r0, n):
        lhs = pltpu.bitcast(pqn_v[r0 // 2:(r0 + n) // 2, :], BF16)
        parts = []
        for c0 in range(0, NC, 2):
            acc = x_v[DEF + L0 + r0:DEF + L0 + r0 + n, c0 * LANES:(c0 + 2) * LANES].astype(F32)
            for k0 in range(0, D, 2 * LANES):
                acc = acc + o_dot(lhs[:, k0:k0 + 2 * LANES], wload(mp_v, k0, 2 * LANES, slice(c0 * LANES, (c0 + 2) * LANES)))
            parts.append(acc)
        return jnp.concatenate(parts, axis=1)

    toks = []
    r0 = 0
    pc.add(post_jobs(OCL[0][0], *OCL[1]), pc.t + 200, pc.t + 1000, QP_DELAY)
    for ci, (n, plain) in enumerate(OCL):
        h = o_plain(r0, n) if plain else o_part(o_dot, x_v, DEF + L0, r0, n)
        last = r0 + n == RL
        units = ln2_jobs(h, ln2_v, out_v, DEF + L0 + r0, -DEF, None, st, fast=last)
        posts = post_jobs(r0 + n + OCL[ci + 1][0], *OCL[ci + 2]) if ci + 2 < len(OCL) else []
        for k, job in enumerate(units):
            toks.append(job(toks[-LAG_L] if len(toks) >= LAG_L and not last else None))
            if posts:
                posts.pop(0)(toks[-1])
        if GLAG[ci] is not None:
            st["pend"].append((st["step"] + GLAG[ci],
                               pltpu.bitcast(jnp.broadcast_to(st["top1"], (8, LANES)), U32) & zero_u))
        r0 += n
        if last or r0 in OUT_AT:
            out_copy(L0 + st["sent"], r0 - st["sent"], 2 if last else 1).start()
            if not last:
                st["sent"] = r0
    for _ in side:
        st["step"] += 1

    keyv = best2(st["top1"], st["top2"])
    idx = [jnp.clip(key_row(kk[0, 0]), 0, S - 1) for kk in keyv]
    grp = [pl.multiple_of((ii >> 3) << 3, 8) for ii in idx]
    vgrp = [pl.multiple_of(gg + DEF, 8) for gg in grp]
    y = res["y"]
    ids_lo, ids_hi = res["ids"]
    hits = None
    yrows = []
    for c in range(2):
        m_lo = ids_lo == key_row(keyv[c])
        m_hi = ids_hi == key_row(keyv[c])
        yrows.append(subsum(jnp.where(wide(m_lo), y[0:8, :], 0.0) + jnp.where(wide(m_hi), y[8:16, :], 0.0)))
        hit = submax(jnp.where(m_lo | m_hi, 1, 0))
        hits = hit if hits is None else hits + hit
    hit_all = hits[0, 0] == 2

    tail0 = L0 + st["sent"]
    tail_copy = out_copy(tail0, S - tail0, 2)
    in_tail = jnp.maximum(grp[0], grp[1]) >= tail0
    two_groups = grp[1] != grp[0]

    def fix_copy(c):
        return out_copy(grp[c], 8, 3 + c)

    def finish(ysel):
        for c in range(2):
            hi = keyv[c] & jnp.int32(-65536)
            score = pltpu.bitcast(hi ^ ((hi >> 31) & 0x7FFF0000), F32)
            sel = (key_row(keyv[c]) & 7) == sub8
            upd = jnp.where(wide(sel), ysel[c] * wide(jax.nn.sigmoid(score)), 0.0)
            out_v[pl.ds(vgrp[c], 8), :] = (out_v[pl.ds(vgrp[c], 8), :].astype(F32) + upd).astype(BF16)
        fix_copy(0).start()

        @pl.when(two_groups)
        def _():
            fix_copy(1).start()

    out_copy(0, L0, 0).wait()
    out_copy(L0, tail0 - L0, 1).wait()

    @pl.when(in_tail)
    def _():
        tail_copy.wait()

    @pl.when(hit_all)
    def _():
        finish(yrows)

    @pl.when(jnp.logical_not(hit_all))
    def _():
        xsel = jnp.concatenate([ln2_v[pl.ds(vgrp[c], 8), :] for c in range(2)], axis=0)

        def ffn_tile(j, acc):
            cs = pl.ds(pl.multiple_of(j * LANES, LANES), LANES)
            g = jnp.dot(xsel, wload(wg_v, 0, D, cs), preferred_element_type=F32)
            u = jnp.dot(xsel, wload(wu_v, 0, D, cs), preferred_element_type=F32)
            a = (g * jax.nn.sigmoid(g) * u).astype(BF16)
            wd_t = pltpu.bitcast(wd_v[pl.ds(pl.multiple_of(j * (LANES // 2), LANES // 2), LANES // 2), 0:D], BF16)
            return acc + jnp.dot(a, wd_t, preferred_element_type=F32)

        yf = lax.fori_loop(0, F // LANES, ffn_tile, jnp.zeros((16, D), F32))
        finish([yf[0:8, :], yf[8:16, :]])

    @pl.when(jnp.logical_not(in_tail))
    def _():
        tail_copy.wait()

    fix_copy(0).wait()

    @pl.when(two_groups)
    def _():
        fix_copy(1).wait()


@jax.jit
def pallas_sequential_preLN__linear_attn_block__moe_arch_mod__prompt_kernel(
    A_x: jax.Array,
    A_wqkv: jax.Array,
    A_wo: jax.Array,
    B_x: jax.Array,
    B_w_r: jax.Array,
    B_w_gate: jax.Array,
    B_w_up: jax.Array,
    B_w_down: jax.Array,
):
    del B_x
    x = A_x.reshape(S, D)
    wr = B_w_r.reshape(NC, LANES)
    any_spec = pl.BlockSpec(memory_space=pl.ANY)
    out = pl.pallas_call(
        _kernel,
        out_shape=jax.ShapeDtypeStruct((S, D), BF16),
        in_specs=[any_spec] * 7,
        out_specs=any_spec,
        scratch_shapes=[
            pltpu.VMEM((S + DEF, D), BF16),
            pltpu.VMEM((D // 2, D), U32),
            pltpu.VMEM((D // 2, D), U32),
            pltpu.VMEM((2, D // 2, D), U32),
            pltpu.VMEM((NC, LANES), BF16),
            pltpu.VMEM((2, D // 2, F + LANES), U32),
            pltpu.VMEM((F // 2, D + LANES), U32),
            pltpu.VMEM((P0 // 2, D), U32),
            pltpu.VMEM((7 ** LA, S // NA // 2, DA), U32),
            pltpu.VMEM((7 ** LA, DA // 2, DA), U32),
            pltpu.VMEM((D // 2, P0), U32),
            pltpu.VMEM((DA // 2, 7 ** LA * MA), U32),
            pltpu.VMEM((D, LANES), F32),
            pltpu.VMEM((D, LANES), F32),
            pltpu.VMEM((RL, LANES), F32),
            pltpu.VMEM((D, D), F32),
            pltpu.VMEM((7, HD, HD), F32),
            pltpu.VMEM((D // 2, D), U32),
            pltpu.VMEM((7 ** LA, DA // 2, DA), U32),
            pltpu.VMEM((D // 2, D), U32),
            pltpu.VMEM((7 ** LO, DO // 2, DO), U32),
            pltpu.VMEM((max(TB2, RL), D + 2 * LANES), F32),
            pltpu.VMEM((RL // 2, D), U32),
            pltpu.VMEM((7 ** LO, max(TB2, RL) // NO // 2, DO), U32),
            pltpu.VMEM((DEF, D), F32),
            pltpu.VMEM((2, S + DEF, D), BF16),
            pltpu.VMEM((TB, D), F32),
            pltpu.VMEM((8, LANES), U32),
            pltpu.SemaphoreType.DMA((NSEM,)),
        ],
        compiler_params=pltpu.CompilerParams(vmem_limit_bytes=110 * 1024 * 1024, disable_bounds_checks=True,
                                             disable_semaphore_checks=True),
    )(x, A_wqkv, A_wo, wr, B_w_gate, B_w_up, B_w_down)
    return out.reshape(1, S, D)
```

```python
import jax
import jax.numpy as jnp
from jax import lax
import jax.experimental.pallas as pl
import jax.experimental.pallas.tpu as pltpu


S = 2048
D = 1024
F = 3584
H = 32
DH = D // H
LANES = 128
NC = D // LANES
HD = D // 2

LA = 2
LO = 1
NA, NO = 2 ** LA, 2 ** LO
DA, DO = D // NA, D // NO
P0 = 512
PB = S - P0
TX = 256
TB = 512
NB1 = PB // TB
MA = TB // NA
TB2 = 384
NB2 = 4
QA = 192
OCH = (128, 128, 128)
DEF = OCH[-1]
L0 = NB2 * TB2
RL = S - L0
QS = (256, 256)
OCL = ((128, False), (128, False), (128, False), (64, True), (64, True))
NPRE = 22
NGAP = 9
OUT_AT = (256, 384, 448)
GM = 32
NZ = 5
WQP = 5
LNU = 8
LAG = 5
LAG_L = 5
LN_DELAY = 800
LN2_DELAY = 900
JOB_DELAY = 500
POST_DELAY = 800
QP_DELAY = 400
WK5 = 66
C6LN = (1000, 8900)
C6WK = (1500, 8900)
P1LN = (60, 10500)
P1WP = (6800, 11000)
P1WQ = (8000, 12300)
P2U = (60, 2000)
EV2 = 300
GLAG = (None, None, None, 20, 8)

F32 = jnp.float32
BF16 = jnp.bfloat16
U32 = jnp.uint32
I32 = jnp.int32

XP = ((PB, 128), (PB + 128, 128), (PB + 256, 256), (0, TB), (TB, PB - TB))
WKP = ((0, 128), (128, 128), (256, 256), (512, 512))

SEM_X = 0
SEM_WK = SEM_X + len(XP)
SEM_WQ = SEM_WK + len(WKP)
SEM_W3 = SEM_WQ + 1
SEM_WR = SEM_W3 + 1
SEM_WGU = SEM_WR + 1
SEM_WD = SEM_WGU + 1
SEM_OUT = SEM_WD + 1
NSEM = SEM_OUT + 5

INT_MIN = -(2 ** 31)


def _layernorm(x, tok=None, w=None):
    s0 = x[:, 0:LANES]
    if tok is not None:
        s0 = s0 + jnp.concatenate([tok] * (x.shape[0] // 8), axis=0)
    for c in range(1, NC):
        s0 = s0 + x[:, c * LANES:(c + 1) * LANES]
    mu = jnp.sum(s0, axis=-1, keepdims=True) * (1.0 / D)
    xc = x - mu
    var = jnp.sum(xc * xc, axis=-1, keepdims=True) * (1.0 / D)
    rstd = lax.rsqrt(var + 1e-5)
    if w is None:
        return xc * rstd
    return xc * rstd, jnp.sum(xc * w, axis=-1, keepdims=True) * rstd


def _phi(t):
    return jnp.where(t > 0, t + 1.0, jnp.exp(t)) + 1e-6


def _n_off(a, b):
    return 32 * a + 8 * b


def _n_groups():
    pos = {(2 * o + e) * LANES + _n_off(a, b): (16 * e + 4 * b + a) * DH + 8 * o
           for o in range(4) for e in range(2) for a in range(4) for b in range(4)}
    return [pos[n] for n in sorted(pos)]


def _quads(b):
    h = len(b) // 2
    return [[r[j * h:(j + 1) * h] for r in b[i * h:(i + 1) * h]] for i in range(2) for j in range(2)]


def _badd(x, y):
    return [[a + b for a, b in zip(rx, ry)] for rx, ry in zip(x, y)]


def _bsub(x, y):
    return [[a - b for a, b in zip(rx, ry)] for rx, ry in zip(x, y)]


def _a_set(b):
    if len(b) == 1:
        return [b[0][0]]
    return [x for o in _a_ops(b) for x in _a_set(o)]


def _b_set(b):
    if len(b) == 1:
        return [b[0][0]]
    q11, q12, q21, q22 = _quads(b)
    ops = (_badd(q11, q22), q11, _bsub(q12, q22), _bsub(q21, q11), q22, _badd(q11, q12), _badd(q21, q22))
    return [x for o in ops for x in _b_set(o)]


def _b_in_a(i, levels):
    perm = (0, 2, 6, 5, 3, 4, 1)
    return sum(perm[(i // 7 ** l) % 7] * 7 ** l for l in range(levels))


def _strassen(prod, levels, base=0, fin=lambda k, q: q, init=None):
    if levels == 0:
        return [[prod(base)]]

    def m(i):
        return _strassen(prod, levels - 1, base * 7 + i)

    def seed(q, x):
        return x if init is None else _badd(_quads(init)[q], x)

    m2 = m(2)
    c22 = seed(3, m2)
    m4 = m(4)
    c12 = fin(1, _badd(seed(1, m2), m4))
    c11 = m4 if init is None else _bsub(_quads(init)[0], m4)
    m3 = m(3)
    c11 = _bsub(m3, c11) if init is None else _badd(c11, m3)
    m1 = m(1)
    c21 = fin(2, _badd(seed(2, m3), m1))
    c22 = _bsub(c22, m1)
    m0 = m(0)
    c11 = _badd(c11, m0)
    c22 = _badd(c22, m0)
    c11 = fin(0, _badd(c11, m(6)))
    c22 = fin(3, _badd(c22, m(5)))
    return [a + b for a, b in zip(c11, c12)] + [a + b for a, b in zip(c21, c22)]


def _goff(i, levels):
    return int(format(i, "0%db" % levels)[::-1], 2) if levels else 0


def _blocks(rows, n):
    w = rows[0].shape[1] // n
    return [[r[:, j * w:(j + 1) * w] for j in range(n)] for r in rows]


def _or_all(vals):
    acc = None
    for v in vals:
        v = v if v.dtype == U32 else pltpu.bitcast(v, U32)
        for g in range(v.shape[0] // 8):
            for c in range(v.shape[1] // LANES):
                p = v if v.shape == (8, LANES) else v[g * 8:(g + 1) * 8, c * LANES:(c + 1) * LANES]
                acc = p if acc is None else acc | p
    return acc


def _raw_ops(levels):
    n = 2 ** levels
    names = [[_Tag((i, j)) for j in range(n)] for i in range(n)]
    return {op: t.ij for op, t in enumerate(_b_set(names)) if t.ij is not None}


class _Tag:
    def __init__(self, ij):
        self.ij = ij

    def __add__(self, other):
        return _Tag(None)

    __sub__ = __add__


def _a_ops(b):
    q11, q12, q21, q22 = _quads(b)
    return (_badd(q11, q22), _badd(q21, q22), q11, q22, _badd(q11, q12), _bsub(q21, q11), _bsub(q12, q22))


_A_FORM = (((0, 0), (1, 1), 1), ((1, 0), (1, 1), 1), ((0, 0),), ((1, 1),), ((0, 0), (0, 1), 1),
           ((1, 0), (0, 0), -1), ((0, 1), (1, 1), -1))
_B_FORM = (((0, 0), (1, 1), 1), ((0, 0),), ((0, 1), (1, 1), -1), ((1, 0), (0, 0), -1), ((1, 1),),
           ((0, 0), (0, 1), 1), ((1, 0), (1, 1), 1))
_C_FORM = (((0, 1), (3, 1), (4, -1), (6, 1)), ((2, 1), (4, 1)), ((1, 1), (3, 1)), ((0, 1), (1, -1), (2, 1), (5, 1)))


def _outer(form, get, n):
    h = n // 2

    def quad(q):
        return [[get(q[0] * h + i, q[1] * h + j) for j in range(h)] for i in range(h)]

    if len(form) == 1:
        return quad(form[0])
    return (_badd if form[2] > 0 else _bsub)(quad(form[0]), quad(form[1]))


def _gate(v, tok):
    u = pltpu.bitcast(v, U32)
    top = u[0:8, 0:LANES] | tok
    if u.shape[1] > LANES:
        top = jnp.concatenate([top, u[0:8, LANES:]], axis=1)
    return pltpu.bitcast(jnp.concatenate([top, u[8:, :]], axis=0) if u.shape[0] > 8 else top, BF16)


class _Pacer:
    def __init__(self, zero, every=0):
        self.zero, self.t, self.jobs, self.pend, self.res, self.tok = zero, 0, [], [], None, None
        self.every, self.last = every, -every

    def add(self, jobs, t0, t1, delay):
        for k, job in enumerate(jobs):
            self.jobs.append((t0 + k * (t1 - t0) // len(jobs), len(self.jobs), job, delay))
        self.jobs.sort(key=lambda e: e[:2])

    def due(self, dep, delay):
        if dep is not None:
            self.pend.append((self.t + delay, _or_all([dep])))

    def release(self, upto):
        while self.jobs and self.jobs[0][0] <= upto:
            _, _, job, delay = self.jobs.pop(0)
            if self.res is not None:
                self.tok = pltpu.bitcast(pltpu.bitcast(self.res[0:8, 0:LANES], U32) & self.zero, F32)
                self.res = None
            self.due(job(self.tok), delay)

    def dot(self, lhs, rhs):
        self.release(self.t)
        ready = [d for t, d in self.pend if t <= self.t]
        if ready and self.t - self.last >= self.every:
            self.pend = [e for e in self.pend if e[0] > self.t]
            self.last = self.t
            lhs = _gate(lhs, _or_all(ready) & self.zero)
        res = jnp.dot(lhs, rhs, preferred_element_type=F32)
        self.t += lhs.shape[0] * (lhs.shape[1] // LANES) * (res.shape[1] // LANES) // 4
        self.res = res
        return res

    def flush(self):
        self.release(1 << 30)


def _kernel(x_hbm, wqkv_hbm, wo_hbm, wr_hbm, wg_hbm, wu_hbm, wd_hbm, out_hbm,
            x_v, wk_v, wq_v, w3_v, wr_v, wgu_v, wd_v,
            ln1_v, xs_v, wks_v, pkt_v, pks_v, zacc_v, uacc_v, xw_v, g_v, gs_v, wqp_v, wqs_v, mp_v, ms_v,
            pq_v, pqn_v, pqs_v, attn_v, lo_v, lnf_v, zero_v, sems):

    ln2_v, out_v = lo_v.at[0], lo_v.at[1]

    wqkv_hbm, wo_hbm, wg_hbm, wu_hbm, wd_hbm = (r.bitcast(U32) for r in (wqkv_hbm, wo_hbm, wg_hbm, wu_hbm, wd_hbm))

    def wload(ref, r0, nr, cols):
        return pltpu.bitcast(ref[r0 // 2:(r0 + nr) // 2, cols], BF16)

    wv_v, wo_v = w3_v.at[0], w3_v.at[1]
    wg_v, wu_v = wgu_v.at[0], wgu_v.at[1]

    def x_copy(i):
        r0, n = XP[i]
        return pltpu.make_async_copy(x_hbm.at[pl.ds(r0, n), :], x_v.at[pl.ds(DEF + r0, n), :], sems.at[SEM_X + i])

    def out_copy(r0, n, s):
        return pltpu.make_async_copy(out_v.at[pl.ds(DEF + r0, n), :], out_hbm.at[pl.ds(r0, n), :],
                                     sems.at[SEM_OUT + s])

    def wk_copy(j):
        c0, n = WKP[j]
        return pltpu.make_async_copy(wqkv_hbm.at[:, pl.ds(D + c0, n)], wk_v.at[:, pl.ds(c0, n)],
                                     sems.at[SEM_WK + j])

    wq_copy = pltpu.make_async_copy(wqkv_hbm.at[:, pl.ds(0, D)], wq_v, sems.at[SEM_WQ])
    wr_copy = pltpu.make_async_copy(wr_hbm, wr_v, sems.at[SEM_WR])
    wd_copy = pltpu.make_async_copy(wd_hbm, wd_v.at[:, pl.ds(0, D)], sems.at[SEM_WD])
    wg_copy = pltpu.make_async_copy(wg_hbm, wg_v.at[:, pl.ds(0, F)], sems.at[SEM_WGU])
    wu_copy = pltpu.make_async_copy(wu_hbm, wu_v.at[:, pl.ds(0, F)], sems.at[SEM_WGU])

    x_copy(0).start()
    wk_copy(0).start()
    x_copy(1).start()
    wr_copy.start()
    for j in range(1, len(WKP)):
        wk_copy(j).start()
    for j in range(2, len(XP)):
        x_copy(j).start()
    wq_copy.start()
    pltpu.make_async_copy(wqkv_hbm.at[:, pl.ds(2 * D, D)], wv_v, sems.at[SEM_W3]).start()
    pltpu.make_async_copy(wo_hbm, wo_v, sems.at[SEM_W3]).start()
    wg_copy.start()
    wu_copy.start()
    wd_copy.start()

    def ln1_rows(xr, xr0, lnr, r0, n):
        ln = _layernorm(xr[xr0:xr0 + n, :].astype(F32)).astype(BF16)
        lnr[r0 // 2:(r0 + n) // 2, :] = pltpu.bitcast(ln, U32)

    def ln1_set(pc, xr, xr0, xsr, a0, n, t0, t1):
        def unit(j):
            def job(tok):
                ln = _layernorm(xr[xr0 + j * LNU:xr0 + (j + 1) * LNU, :].astype(F32), tok)
                lnf_v[j * LNU:(j + 1) * LNU, :] = ln
                return _or_all([ln[:, 0:LANES], ln[:, D - LANES:D]])
            return job

        def piece(j0, c0, o):
            def job(tok):
                def get(i, f):
                    r = (j0 + 2 * _goff(i, LA)) * LNU
                    v = lnf_v[r:r + 16, f * DA + c0:f * DA + c0 + LANES]
                    return v + jnp.concatenate([tok, tok], axis=0) if (i + f) % (NA // 2 + 1) == 0 else v

                r = (a0 + (j0 // (2 * NA)) * 16) // 2
                ops = _a_set(_outer(_A_FORM[o], get, NA))
                for op, v in enumerate(ops):
                    xsr.at[o * len(ops) + op][r:r + 8, c0:c0 + LANES] = pltpu.bitcast(v.astype(BF16), U32)
                return _or_all([v[0:8, :] for v in [ops[0]] + ops[5:7]])
            return job

        grp = 2 * NA
        ng = n // LNU // grp
        dt = (t1 - t0 - LN_DELAY) // (ng + 1)
        for g in range(ng):
            pc.add([unit(g * grp + j) for j in range(grp)], t0 + g * dt, t0 + (g + 1) * dt, LN_DELAY)
            s = t0 + (g + 1) * dt + LN_DELAY
            pc.add([piece(g * grp, c0, o) for c0 in range(0, DA, LANES) for o in range(7)], s, s + dt, JOB_DELAY)

    def ln1_load(lnr, r0, n):
        return pltpu.bitcast(lnr[r0 // 2:(r0 + n) // 2, :], BF16)

    def k_mm(r0, n, c0, nc):
        return jnp.dot(ln1_load(ln1_v, r0, n), wload(wk_v, 0, D, slice(c0, c0 + nc)), preferred_element_type=F32)

    def z_acc(pkts, c0, first=False):
        zs = None
        for pkt in pkts:
            for j in range(pkt.shape[1] // LANES):
                p = pkt[:, j * LANES:(j + 1) * LANES]
                zs = p if zs is None else zs + p
        if first:
            zacc_v[c0:c0 + zs.shape[0], :] = zs
        else:
            zacc_v[c0:c0 + zs.shape[0], :] += zs

    def k_post(k, p0, c0, first=False):
        n, nc = k.shape
        pkt = _phi(k).T
        pkt_v[c0 // 2:(c0 + nc) // 2, p0:p0 + n] = pltpu.bitcast(pkt.astype(BF16), U32)
        z_acc([pkt], c0, first)
        return pkt[nc - 8:nc, n - LANES:n]

    def g_acc(r0, n, c0, nc, first=False, pc=None):
        h, w = (nc, D) if pc is None else (LANES, LANES)
        for f0 in range(c0, c0 + nc, h):
            for j0 in range(0, D, w):
                lhs = pltpu.bitcast(pkt_v[f0 // 2:(f0 + h) // 2, r0:r0 + n], BF16)
                rhs = pltpu.bitcast(ln1_v[r0 // 2:(r0 + n) // 2, j0:j0 + w], BF16)
                g = jnp.dot(lhs, rhs, preferred_element_type=F32) if pc is None else pc.dot(lhs, rhs)
                if first:
                    g_v[f0:f0 + h, j0:j0 + w] = g
                else:
                    g_v[f0:f0 + h, j0:j0 + w] += g

    def k_paced(pc, r0, c0, nc, first):
        for j0 in range(c0, c0 + nc, LANES):
            for t0 in range(r0, r0 + TX, LANES):
                k = None
                for k0 in range(0, D, TX):
                    p = pc.dot(ln1_load(ln1_v, t0, LANES)[:, k0:k0 + TX], wload(wk_v, k0, TX, slice(j0, j0 + LANES)))
                    k = p if k is None else k + p
                pc.due(k_post(k, t0, j0, first and t0 == r0), POST_DELAY)

    attn_v[...] = jnp.zeros_like(attn_v)
    zero_v[...] = jnp.zeros_like(zero_v)

    def gs_zero(o0, o1):
        gs_v[o0:o1] = jnp.zeros((o1 - o0, HD, HD), F32)

    x_copy(0).wait()
    ln1_rows(x_v, DEF + PB, ln1_v, 0, 128)
    gs_zero(0, 1)
    wk_copy(0).wait()
    ka = k_mm(0, 128, 0, 128)
    gs_zero(1, 2)
    x_copy(1).wait()
    wr_copy.wait()
    gs_zero(2, 3)
    ln1_rows(x_v, DEF + PB + 128, ln1_v, 128, 128)
    k_post(ka, 0, 0, first=True)
    g_acc(0, 128, 0, 128, first=True)
    wk_copy(1).wait()
    gs_zero(3, NZ)
    k_post(k_mm(128, 128, 0, 128), 128, 0)
    k_post(k_mm(0, TX, 128, 128), 0, 128, first=True)
    g_acc(128, 128, 0, 128)

    def w_job(src_ref, dst_ref, levels, r0, c0, o):
        n = 2 ** levels
        w, raw, inner = D // n, _raw_ops(levels), 7 ** (levels - 1)

        def job(tok):
            def cut(i, j):
                return src_ref[(i * w + r0) // 2:(i * w + r0) // 2 + 8, j * w + c0:j * w + c0 + LANES]

            def get(i, j):
                u = cut(i, j)
                return pltpu.bitcast(u if tok is None else u | pltpu.bitcast(tok, U32), BF16).astype(F32)

            ops = []
            for op, v in enumerate(_b_set(_outer(_B_FORM[o], get, n))):
                dst = dst_ref.at[o * inner + op]
                if o * inner + op in raw:
                    dst[r0 // 2:r0 // 2 + 8, c0:c0 + LANES] = cut(*raw[o * inner + op])
                else:
                    dst[r0 // 2:r0 // 2 + 8, c0:c0 + LANES] = pltpu.bitcast(v.astype(BF16), U32)
                    ops.append(v)
            return _or_all(ops[0:1] + ops[-2:]) if ops else None
        return job

    def wk_jobs_of(outer):
        return [w_job(wk_v, wks_v, LA, r0, c0, o) for r0 in range(0, DA, 16) for c0 in range(0, DA, LANES)
                for o in outer]

    wk_copy(2).wait()
    pc = _Pacer(zero_v[...])
    pc.add(wk_jobs_of((1, 3)), 500, 2200, JOB_DELAY)
    k_paced(pc, 0, 256, 256, True)
    g_acc(0, TX, 128, 128, True, pc)
    g_acc(0, TX, 256, 256, True, pc)
    pc.flush()
    wk_copy(3).wait()
    wk_jobs = wk_jobs_of((0, 2, 4, 5, 6))
    pc = _Pacer(zero_v[...])
    pc.add(wk_jobs[:WK5], 500, 2700, JOB_DELAY)
    k_paced(pc, 0, 512, 512, True)
    g_acc(0, TX, 512, 256, True, pc)
    pc.flush()
    x_copy(2).wait()
    x_copy(3).wait()
    pc = _Pacer(zero_v[...])
    ln1_set(pc, x_v, DEF, xs_v, 0, TB, *C6LN)
    pc.add(wk_jobs[WK5:], *C6WK, JOB_DELAY)
    ln1_rows(x_v, DEF + PB + TX, ln1_v, TX, TX)
    g_acc(0, TX, 768, 256, True, pc)
    k_paced(pc, TX, 0, D, False)
    for c0 in range(0, D, 256):
        g_acc(TX, TX, c0, 256, False, pc)
    pc.flush()

    def xs_load(xsr, op, a0, m):
        return pltpu.bitcast(xsr[op, a0 // 2:(a0 + m) // 2, :], BF16)

    def k_step(pc, xsr, j0):
        def fin(_, q):
            q = [[_phi(v).T for v in r] for r in q]
            pc.due(_or_all([v[LANES - 8:LANES, :] for r in q for v in r]), POST_DELAY)
            return q

        cb = _strassen(lambda i: pc.dot(xs_load(xsr, i, 0, MA), pltpu.bitcast(wks_v[i, :, j0:j0 + LANES], BF16)),
                       LA, fin=fin)
        outer = _a_ops([[cb[i][f] for i in range(NA)] for f in range(NA)])
        for half, o in ((0, outer[4]), (1, outer[1])):
            for f, rowb in enumerate(o):
                z_acc(rowb, half * HD + f * DA + j0)
        ops = [v for o in outer for v in _a_set(o)]
        for op, v in enumerate(ops):
            pks_v[j0 // 2:(j0 + LANES) // 2, op * MA:(op + 1) * MA] = pltpu.bitcast(v.astype(BF16), U32)
        pc.due(_or_all([v[LANES - 8:LANES, :] for v in (ops[0], ops[-1], ops[-2])]), 2 * POST_DELAY)

    def g_step(pc, xsr, r0, later):
        def old(o, f, c):
            v = gs_v[o, f * DA + r0:f * DA + r0 + GM, c * DA:(c + 1) * DA]
            return v if o < NZ else jnp.where(later, v, 0.0)

        for o in range(7):
            cb = _strassen(lambda i: pc.dot(pltpu.bitcast(pks_v[r0 // 2:(r0 + GM) // 2, i * MA:(i + 1) * MA], BF16),
                                            xs_load(xsr, _b_in_a(i, LA), 0, MA)), LA - 1, base=o,
                           init=[[old(o, f, c) for c in range(NA // 2)] for f in range(NA // 2)])
            for f in range(NA // 2):
                for c in range(NA // 2):
                    gs_v[o, f * DA + r0:f * DA + r0 + GM, c * DA:(c + 1) * DA] = cb[f][c]

    def wq_jobs(u0, nr):
        span = (NA - 1) * DA + 16 * nr
        u0 = u0 if isinstance(u0, int) else pl.multiple_of(u0, 8)
        srcr, permr = wq_v.at[pl.ds(u0, span // 2), :], wqp_v.at[pl.ds(u0, span // 2), :]
        dstr = wqs_v.at[:, pl.ds(u0, 8 * nr), :]
        oct_ = (lax.broadcasted_iota(I32, (8, LANES), 1) % DH) // 8

        def perm(r, e):
            def job(tok):
                blk = [srcr[r // 2:r // 2 + 8, (4 * e + b) * LANES:(4 * e + b + 1) * LANES] | pltpu.bitcast(tok, U32)
                       for b in range(4)]
                outs = []
                for o in range(4):
                    v = blk[o]
                    for b in range(4):
                        if b != o:
                            v = jnp.where(oct_ == b, pltpu.roll(blk[b], (8 * (b - o)) % LANES, 1), v)
                    permr[r // 2:r // 2 + 8, (2 * o + e) * LANES:(2 * o + e + 1) * LANES] = v
                    outs.append(v)
                return _or_all(outs)
            return job

        return ([perm(i * DA + r0, e) for r0 in range(0, 16 * nr, 16) for i in range(NA) for e in range(2)],
                [w_job(permr, dstr, LA, r0, c0, o) for r0 in range(0, 16 * nr, 16)
                 for c0 in range(0, DA, LANES) for o in range(7)])

    def p1(i, carry):
        xsr = xs_v.at[:, pl.ds(pl.multiple_of(i * (MA // 2), MA // 2), MA), :]
        xr = x_v.at[pl.ds(pl.multiple_of((i + 1) * TB, TB), TB + DEF), :]

        pc = _Pacer(zero_v[...])
        ln1_set(pc, xr, DEF, xsr, MA, TB, *P1LN)
        perms, sets = wq_jobs(i * (8 * WQP), WQP)
        pc.add(perms, *P1WP, JOB_DELAY)
        pc.add(sets, *P1WQ, JOB_DELAY)
        for j0 in range(0, DA, LANES):
            k_step(pc, xsr, j0)
        for r0 in range(0, DA, GM):
            g_step(pc, xsr, r0, i > 0)
        pc.flush()
        return carry

    x_copy(4).wait()
    wq_copy.wait()
    lax.fori_loop(0, NB1, p1, 0)

    pltpu.make_async_copy(w3_v, w3_v, sems.at[SEM_W3]).wait()
    zero_u = zero_v[...]
    zrow = jnp.sum(jnp.concatenate([zacc_v[r:r + 8, :] for r in _n_groups()], axis=0).T, axis=0, keepdims=True)
    wr8 = wr_v[...].astype(F32)
    wr_row = jnp.concatenate([wr8[c:c + 1, :] for c in range(NC)], axis=1)

    row_h = lax.broadcasted_iota(I32, (LANES, LANES), 0) // DH
    col_h = lax.broadcasted_iota(I32, (LANES, LANES), 1) // DH
    diag = row_h == col_h

    def colsum(t):
        acc = t[:, 0:LANES]
        for c in range(1, NC):
            acc = acc + t[:, c * LANES:(c + 1) * LANES]
        return acc

    wrc = wr_row - jnp.sum(wr_row, axis=-1, keepdims=True) * (1.0 / D)
    m_raw = _raw_ops(LO)

    def kv_part(c):
        cs = slice(c * LANES, (c + 1) * LANES)
        kv = None
        for k0 in range(0, D, TX):
            g = g_v[cs, k0:k0 + TX]
            for o, sign in _C_FORM[(c * LANES // HD) * 2 + k0 // HD]:
                t = gs_v[o, c * LANES % HD:c * LANES % HD + LANES, k0 % HD:k0 % HD + TX]
                g = g + t if sign > 0 else g - t
            p = pc.dot(g.astype(BF16), wload(wv_v, k0, TX, cs))
            kv = p if kv is None else kv + p
        return jnp.where(diag, kv, 0.0)

    def m_part(c, kvs):
        e, b = c // 4, c % 4
        for j0 in range(0, DO, LANES):
            ms = [jnp.concatenate(
                [pc.dot(kv, wload(wo_v, (c + k) * LANES, LANES, slice(f * DO + j0, f * DO + j0 + LANES)))
                 for f in range(NO)], axis=1) for k, kv in enumerate(kvs)]
            deps = []
            for a in range(4):
                rows = [jnp.concatenate([m[a * DH + 8 * o:a * DH + 8 * o + 8, :] for m in ms], axis=0)
                        for o in range(4)]
                for o in range(4):
                    r = ((2 * o + e) * LANES + _n_off(a, b)) // 2
                    for f in range(NO):
                        mp_v[r:r + 8, f * DO + j0:f * DO + j0 + LANES] = pltpu.bitcast(
                            rows[o][:, f * LANES:(f + 1) * LANES].astype(BF16), U32)
                for t in range(4 // NO):
                    r = ((2 * t + e) * LANES + _n_off(a, b)) // 2
                    for op, v in enumerate(_b_set(_blocks(rows[t::4 // NO], NO))):
                        if op not in m_raw:
                            ms_v.at[op][r:r + 8, j0:j0 + LANES] = pltpu.bitcast(v.astype(BF16), U32)
                            deps.append(v[0:8, 0:LANES])
            pc.due(_or_all(deps[::4]), POST_DELAY)

    pc = _Pacer(zero_u)
    pc.due(jnp.broadcast_to(zrow, (8, D)), 1000)
    perms, sets = wq_jobs(NB1 * 8 * WQP, DA // 16 - NB1 * WQP)
    pc.add(perms, 60, 700, JOB_DELAY)
    pc.add(sets, 1300, 3500, JOB_DELAY)
    kv_prev = None
    for c in range(0, NC + 2, 2):
        kvs = [kv_part(c).astype(BF16), kv_part(c + 1).astype(BF16)] if c < NC else None
        if c:
            m_part(c - 2, kv_prev)
        kv_prev = kvs
    pc.flush()

    def make_key(score, row):
        b = pltpu.bitcast(score, I32)
        srt = b ^ ((b >> 31) & 0x7FFFFFFF)
        return (srt & jnp.int32(-65536)) | (0xFFFF - row)

    def push_keys(key, top1, top2):
        for gidx in range(key.shape[0] // 8):
            kx = key[gidx * 8:(gidx + 1) * 8, :]
            top2 = jnp.maximum(top2, jnp.minimum(top1, kx))
            top1 = jnp.maximum(top1, kx)
        return top1, top2

    lane = lax.broadcasted_iota(I32, (1, LANES), 1)

    def interleave(parts):
        return jnp.concatenate([p[g * 16:(g + 1) * 16, :] for g in range(parts[0].shape[0] // 16) for p in parts],
                               axis=0)

    def q_part(pc, xsr, l0, r0, n, hint=None):
        m = n // NA
        sums = {}

        def park(v, g, c):
            for t in range(m // 16):
                r = r0 + (t * NA + g) * 16
                pq_v[r:r + 16, c * LANES:(c + 1) * LANES] = v[t * 16:(t + 1) * 16, :]

        def fin(k, q):
            q = [[_phi(v) for v in r] for r in q]
            deps = []
            for a, r in enumerate(q):
                for b, v in enumerate(r):
                    i, c = (k // 2) * (NA // 2) + a, (((k % 2) * (NA // 2) + b) * DA + j0) // LANES
                    park(v, _goff(i, LA), c)
                    for name, row in (("z", zrow),) + ((("u", hint["u"]),) if hint else ()):
                        t = v * row[:, c * LANES:(c + 1) * LANES]
                        key = (name, _goff(i, LA), c % 2)
                        sums[key] = t if key not in sums else sums[key] + t
                deps.append(sums[key])
            if hint:
                pc.due(_or_all(deps), POST_DELAY)
            return q

        for j0 in range(0, DA, LANES):
            _strassen(lambda i: pc.dot(xs_load(xsr, i, (l0 + r0) // NA, m),
                                       pltpu.bitcast(wqs_v[i, :, j0:j0 + LANES], BF16)), LA, fin=fin)
        if hint:
            pc.flush()
        den = jnp.concatenate([sums["z", g, e] for g in range(NA) for e in range(2)], axis=0)
        for s in (1, 2, 4):
            den = den + jnp.where((lane & s) == 0, pltpu.roll(den, LANES - s, 1), pltpu.roll(den, s, 1))
        inv_all = 1.0 / (den + 1e-6)

        def inv_of(g):
            return [inv_all[(g * 2 + e) * m:(g * 2 + e + 1) * m, :] for e in range(2)]

        for g in range(NA):
            for e in range(2):
                park(inv_of(g)[e], g, NC + e)
        if hint:
            for g in range(NA):
                starts = [r0 + (t * NA + g) * 16 for t in range(m // 16)]
                num = jnp.sum(jnp.concatenate([xw_v[t:t + 16, :] for t in starts], axis=0)
                              + sums["u", g, 0] * inv_of(g)[0] + sums["u", g, 1] * inv_of(g)[1],
                              axis=-1, keepdims=True)
                row = jnp.concatenate([(l0 + t) + lax.broadcasted_iota(I32, (16, 1), 0) for t in starts], axis=0)
                hint["p1"], hint["p2"] = push_keys(make_key(num, row), hint["p1"], hint["p2"])
            pc.due(jnp.broadcast_to(hint["p1"], (8, LANES)), 1200)


    def post_jobs(r0, n, plain=False):
        def scaled(t, c0, w, tok):
            inv = pq_v[t:t + 16, D:D + 2 * LANES]
            if tok is not None:
                inv = inv + jnp.concatenate([jnp.concatenate([tok, tok], axis=0)] * 2, axis=1)
            return pq_v[t:t + 16, c0:c0 + w] * jnp.concatenate([inv] * (w // (2 * LANES)), axis=1)

        def post_plain(t):
            def job(tok):
                v = scaled(t, 0, D, tok)
                pqn_v[t // 2:t // 2 + 8, :] = pltpu.bitcast(v.astype(BF16), U32)
                return v[0:8, 0:LANES]
            return job

        def post(t0, outer):
            def job(tok):
                deps = []
                for c0 in range(0, DO, 2 * LANES):
                    blk = {}

                    def get(i, f):
                        if (i, f) not in blk:
                            blk[i, f] = scaled(t0 + _goff(i, LO) * 16, f * DO + c0, 2 * LANES, tok)
                        return blk[i, f]

                    for o in outer:
                        ops = _a_set(_outer(_A_FORM[o], get, NO))
                        for op, v in enumerate(ops):
                            pqs_v.at[o * len(ops) + op][t0 // NO // 2:t0 // NO // 2 + 8, c0:c0 + 2 * LANES] = (
                                pltpu.bitcast(v.astype(BF16), U32))
                        deps.append(ops[0][0:8, 0:LANES])
                return _or_all(deps)
            return job

        if plain:
            return [post_plain(t) for t in range(r0, r0 + n, 16)]
        outers = [range(7)] if LO == 1 else [(o,) for o in range(7)]
        return [post(t0, outer) for t0 in range(r0, r0 + n, 16 * NO) for outer in outers]

    def m_operand(i, c0, c1):
        if i not in m_raw:
            return pltpu.bitcast(ms_v[i, :, c0 * LANES:c1 * LANES], BF16)
        bi, bj = m_raw[i]
        return wload(mp_v, bi * DO, DO, slice(bj * DO + c0 * LANES, bj * DO + c1 * LANES))

    def o_part(dot, xr, x0, r0, n):
        a0, m = r0 // NO, n // NO
        nw = LANES * NO // 2
        cols = [[[] for _ in range(NO)] for _ in range(NO)]
        for c0 in range(0, DO, nw):
            init = [[jnp.concatenate(
                [xr[x0 + r0 + (g * NO + _goff(i, LO)) * 16:x0 + r0 + (g * NO + _goff(i, LO) + 1) * 16,
                    f * DO + c0:f * DO + c0 + nw] for g in range(m // 16)], axis=0).astype(F32)
                for f in range(NO)] for i in range(NO)]
            cb = _strassen(lambda i: dot(pltpu.bitcast(pqs_v[i, a0 // 2:(a0 + m) // 2, :], BF16),
                                         m_operand(i, c0 // LANES, (c0 + nw) // LANES)), LO, init=init)
            for i in range(NO):
                for f in range(NO):
                    cols[i][f].append(cb[i][f])
        parts = [None] * NO
        for i in range(NO):
            parts[_goff(i, LO)] = jnp.concatenate([c for f in range(NO) for c in cols[i][f]], axis=1)
        return interleave(parts)

    def ln2_unit(h, l2r, outr, r0, row0, valid, top1, top2, tok, fast=False):
        n = h.shape[0]
        if fast:
            ln2, r = _layernorm(h, tok, wr_row)
        else:
            ln2 = _layernorm(h, tok)
            r = jnp.sum(ln2 * wr_row, axis=-1, keepdims=True)
        l2r[r0:r0 + n, :] = ln2.astype(BF16)
        res = h + ln2
        outr[r0:r0 + n, :] = res.astype(BF16)
        r = r.astype(BF16).astype(F32) + 0.0
        key = make_key(r, (row0 + r0) + lax.broadcasted_iota(I32, (n, 1), 0))
        if valid is not None:
            key = jnp.where(valid, key, INT_MIN)
        top1, top2 = push_keys(key, top1, top2)
        ntok = pltpu.bitcast(pltpu.bitcast(jnp.broadcast_to(r[n - 8:n, :], (8, LANES)), U32) & zero_u, F32)
        return top1, top2, ntok

    def ln2_jobs(h, l2r, outr, r0, row0, valid, st, fast=False):
        def unit(j):
            def job(tok):
                st["top1"], st["top2"], dep = ln2_unit(h[j * LNU:(j + 1) * LNU, :], l2r, outr, r0 + j * LNU, row0,
                                                       valid, st["top1"], st["top2"], tok, fast)
                return dep
            return job
        return [unit(j) for j in range(h.shape[0] // LNU)]

    QC = 16 * 7 ** LA / 8 ** LA

    def p2(i, carry):
        st = dict(top1=carry[0], top2=carry[1])
        b0 = pl.multiple_of(i * TB2, 16)
        xsr = xs_v.at[:, pl.ds(pl.multiple_of(i * (TB2 // NA // 2), 8), TB2 // NA // 2), :]
        xr = x_v.at[pl.ds(b0, TB2 + DEF), :]
        l2r = ln2_v.at[pl.ds(b0, TB2 + DEF), :]
        outr = out_v.at[pl.ds(b0, TB2 + DEF), :]
        row0 = b0 - DEF
        pc = _Pacer(zero_u)
        toks = []

        def chain(jobs):
            for job in jobs:
                toks.append(job(toks[-LAG] if len(toks) >= LAG else None))

        chain(ln2_jobs(attn_v, l2r, outr, 0, row0, i > 0, st))

        @pl.when(i > 0)
        def _():
            out_copy(pl.multiple_of((i - 1) * TB2, 16), TB2, 0).start()

        pc.due(toks[-1], QA * QC)

        nu, nx = D // NB2, RL // NB2
        mr = mp_v.at[pl.ds(pl.multiple_of(i * (nu // 2), 8), nu // 2), :]
        ur = uacc_v.at[pl.ds(pl.multiple_of(i * nu, 8), nu), :]
        xl = x_v.at[pl.ds(pl.multiple_of(DEF + L0 + i * nx, 16), nx), :]
        xwr = xw_v.at[pl.ds(pl.multiple_of(i * nx, 8), nx), :]

        def hint_job(load, dst, r):
            def job(tok):
                v = colsum(load(r).astype(F32) * wrc) + jnp.concatenate([tok, tok], axis=0)
                dst[r:r + 16, :] = v
                return v
            return job

        pc.add([hint_job(lambda r: wload(mr, r, 16, slice(None)), ur, r) for r in range(0, nu, 16)]
               + [hint_job(lambda r: xl[r:r + 16, :], xwr, r) for r in range(0, nx, 16)], *P2U, JOB_DELAY)
        for r0, n in ((0, QA), (QA, TB2 - QA)):
            q_part(pc, xsr, 0, r0, n)
            for job in post_jobs(r0, n):
                job(None)
        r0 = 0
        for n in OCH[:-1]:
            chain(ln2_jobs(o_part(pc.dot, xr, DEF, r0, n), l2r, outr, DEF + r0, row0, None, st))
            r0 += n
        attn_v[...] = o_part(pc.dot, xr, DEF, r0, DEF)
        return st["top1"], st["top2"]

    init = jnp.full((8, 1), INT_MIN, I32)
    top1, top2 = lax.fori_loop(0, NB2, p2, (init, init))

    wg_copy.wait()
    wu_copy.wait()
    wd_copy.wait()
    sub8 = lax.broadcasted_iota(I32, (8, LANES), 0)
    urow = jnp.sum(uacc_v[...].T, axis=0, keepdims=True)

    def submax(v):
        for sh in (4, 2, 1):
            v = jnp.maximum(v, pltpu.roll(v, sh, 0))
        return v

    def subsum(v):
        for sh in (4, 2, 1):
            v = v + pltpu.roll(v, sh, 0)
        return v

    def best2(t1, t2):
        t1 = jnp.broadcast_to(t1, (8, LANES))
        t2 = jnp.broadcast_to(t2, (8, LANES))
        k1v = submax(t1)
        return k1v, submax(jnp.where(t1 == k1v, t2, t1))

    def key_row(k):
        return 0xFFFF - (k & 0xFFFF)

    def wide(m):
        return jnp.concatenate([m] * NC, axis=1)

    st = dict(top1=top1, top2=top2, pend=[], step=0, sent=0)
    pc = _Pacer(zero_u, EV2)
    hint = dict(u=urow, p1=init, p2=init)

    pc.add(ln2_jobs(attn_v, ln2_v, out_v, L0, -DEF, None, st), 60, QS[0] * QC - 600, LN2_DELAY)
    r0 = 0
    for k, n in enumerate(QS):
        q_part(pc, xs_v, L0, r0, n, hint)
        if k == 0:
            out_copy(L0 - TB2, TB2, 0).start()
            top1, top2 = st["top1"], st["top2"]
            pc.add(post_jobs(0, OCL[0][0], OCL[0][1]), pc.t + 600, pc.t + (RL - n) * QC - 300, QP_DELAY)
        r0 += n
    pc.every = 0
    oldk = best2(top1, top2)
    oldx = []
    for kk in oldk:
        g8 = pl.multiple_of(((jnp.clip(key_row(kk[0, 0]), 0, S - 1) >> 3) << 3) + DEF, 8)
        rows = ln2_v[pl.ds(g8, 8), :].astype(F32)
        oldx.append(subsum(jnp.where(wide((key_row(kk) & 7) == sub8), rows, 0.0)))

    def gated(v):
        tok = None
        while st["pend"] and st["pend"][0][0] <= st["step"]:
            t = st["pend"].pop(0)[1]
            tok = t if tok is None else tok | t
        if tok is None:
            return v
        u = pltpu.bitcast(v, U32)
        return pltpu.bitcast(jnp.concatenate([u[:, 0:LANES] | tok, u[:, LANES:]], axis=1), BF16)

    res = {}

    def c_units():
        pc.flush()
        p1, p2_ = hint["p1"], hint["p2"]
        cand_p, cand_x = [], []
        for pk_ in (p1, p2_):
            cp, cx = None, None
            for s in range(8):
                g8 = pl.multiple_of((jnp.clip(key_row(pk_[s, 0]) - L0, 0, RL - 1) >> 3) << 3, 8)
                vp = pq_v[pl.ds(g8, 8), :]
                vx = x_v[pl.ds(pl.multiple_of(g8 + (L0 + DEF), 8), 8), :].astype(F32)
                cp = vp if cp is None else jnp.where(jnp.concatenate([sub8 == s] * (NC + 2), axis=1), vp, cp)
                cx = vx if cx is None else jnp.where(wide(sub8 == s), vx, cx)
            cand_p.append(cp[:, 0:D] * jnp.concatenate([cp[:, D:]] * (NC // 2), axis=1))
            cand_x.append(cx)
        cand_p = jnp.concatenate(cand_p, axis=0).astype(BF16)
        cand_x = jnp.concatenate(cand_x, axis=0)
        ids_lo = key_row(jnp.broadcast_to(p1, (8, LANES)))
        ids_hi = jnp.where(sub8 < 6, key_row(jnp.broadcast_to(p2_, (8, LANES))),
                           jnp.where(sub8 == 6, key_row(oldk[0]), key_row(oldk[1])))
        res["ids"] = (ids_lo, ids_hi)
        parts = []
        for c in range(NC):
            parts.append(jnp.dot(cand_p, wload(mp_v, 0, D, slice(c * LANES, (c + 1) * LANES)), preferred_element_type=F32))
            yield
        xs = _layernorm(cand_x + jnp.concatenate(parts, axis=1))
        hi = jnp.where(wide(sub8 < 6), xs[8:16, :], jnp.where(wide(sub8 == 6), oldx[0], oldx[1]))
        res["xs"] = jnp.concatenate([xs[0:8, :], hi], axis=0).astype(BF16)

    def f_units():
        xs = res["xs"]
        acts = []
        for j in range(F // LANES):
            cs = slice(j * LANES, (j + 1) * LANES)
            g = jnp.dot(gated(xs), wload(wg_v, 0, D, cs), preferred_element_type=F32)
            yield
            u = jnp.dot(xs, wload(wu_v, 0, D, cs), preferred_element_type=F32)
            acts.append((g * jax.nn.sigmoid(g) * u).astype(BF16))
            yield
        act = jnp.concatenate(acts, axis=1)
        zf = pltpu.bitcast(zero_u, F32)
        ys = []
        KF = (F // D) * D
        for c in range(0, NC, 2):
            acc = jnp.concatenate([jnp.concatenate([zf, zf], axis=0)] * 2, axis=1)
            acc = acc + jnp.dot(gated(act[:, KF:]), wload(wd_v, KF, F - KF, slice(c * LANES, (c + 2) * LANES)),
                                preferred_element_type=F32)
            yield
            for cc in range(2):
                y = acc[:, cc * LANES:(cc + 1) * LANES]
                for k0 in range(0, KF, D):
                    y = y + jnp.dot(gated(act[:, k0:k0 + D]),
                                    wload(wd_v, k0, D, slice((c + cc) * LANES, (c + cc + 1) * LANES)),
                                    preferred_element_type=F32)
                    yield
                ys.append(y)
        res["y"] = jnp.concatenate(ys, axis=1)

    def side_units():
        yield from range(NPRE)
        yield from c_units()
        yield from range(NGAP)
        yield from f_units()

    side = side_units()

    def o_dot(lhs, rhs):
        p = pc.dot(lhs, rhs) if st["step"] < NPRE else jnp.dot(lhs, rhs, preferred_element_type=F32)
        next(side, None)
        st["step"] += 1
        return p

    def o_plain(r0, n):
        lhs = pltpu.bitcast(pqn_v[r0 // 2:(r0 + n) // 2, :], BF16)
        parts = []
        for c0 in range(0, NC, 2):
            acc = x_v[DEF + L0 + r0:DEF + L0 + r0 + n, c0 * LANES:(c0 + 2) * LANES].astype(F32)
            for k0 in range(0, D, 2 * LANES):
                acc = acc + o_dot(lhs[:, k0:k0 + 2 * LANES], wload(mp_v, k0, 2 * LANES, slice(c0 * LANES, (c0 + 2) * LANES)))
            parts.append(acc)
        return jnp.concatenate(parts, axis=1)

    toks = []
    r0 = 0
    pc.add(post_jobs(OCL[0][0], *OCL[1]), pc.t + 200, pc.t + 1000, QP_DELAY)
    for ci, (n, plain) in enumerate(OCL):
        h = o_plain(r0, n) if plain else o_part(o_dot, x_v, DEF + L0, r0, n)
        last = r0 + n == RL
        units = ln2_jobs(h, ln2_v, out_v, DEF + L0 + r0, -DEF, None, st, fast=last)
        posts = post_jobs(r0 + n + OCL[ci + 1][0], *OCL[ci + 2]) if ci + 2 < len(OCL) else []
        for k, job in enumerate(units):
            toks.append(job(toks[-LAG_L] if len(toks) >= LAG_L and not last else None))
            if posts:
                posts.pop(0)(toks[-1])
        if GLAG[ci] is not None:
            st["pend"].append((st["step"] + GLAG[ci],
                               pltpu.bitcast(jnp.broadcast_to(st["top1"], (8, LANES)), U32) & zero_u))
        r0 += n
        if last or r0 in OUT_AT:
            out_copy(L0 + st["sent"], r0 - st["sent"], 2 if last else 1).start()
            if not last:
                st["sent"] = r0
    for _ in side:
        st["step"] += 1

    keyv = best2(st["top1"], st["top2"])
    idx = [jnp.clip(key_row(kk[0, 0]), 0, S - 1) for kk in keyv]
    grp = [pl.multiple_of((ii >> 3) << 3, 8) for ii in idx]
    vgrp = [pl.multiple_of(gg + DEF, 8) for gg in grp]
    y = res["y"]
    ids_lo, ids_hi = res["ids"]
    hits = None
    yrows = []
    for c in range(2):
        m_lo = ids_lo == key_row(keyv[c])
        m_hi = ids_hi == key_row(keyv[c])
        yrows.append(subsum(jnp.where(wide(m_lo), y[0:8, :], 0.0) + jnp.where(wide(m_hi), y[8:16, :], 0.0)))
        hit = submax(jnp.where(m_lo | m_hi, 1, 0))
        hits = hit if hits is None else hits + hit
    hit_all = hits[0, 0] == 2

    tail0 = L0 + st["sent"]
    tail_copy = out_copy(tail0, S - tail0, 2)
    in_tail = jnp.maximum(grp[0], grp[1]) >= tail0
    two_groups = grp[1] != grp[0]

    def fix_copy(c):
        return out_copy(grp[c], 8, 3 + c)

    def finish(ysel):
        for c in range(2):
            hi = keyv[c] & jnp.int32(-65536)
            score = pltpu.bitcast(hi ^ ((hi >> 31) & 0x7FFF0000), F32)
            sel = (key_row(keyv[c]) & 7) == sub8
            upd = jnp.where(wide(sel), ysel[c] * wide(jax.nn.sigmoid(score)), 0.0)
            out_v[pl.ds(vgrp[c], 8), :] = (out_v[pl.ds(vgrp[c], 8), :].astype(F32) + upd).astype(BF16)
        fix_copy(0).start()

        @pl.when(two_groups)
        def _():
            fix_copy(1).start()

    out_copy(0, L0, 0).wait()
    out_copy(L0, tail0 - L0, 1).wait()

    @pl.when(in_tail)
    def _():
        tail_copy.wait()

    @pl.when(hit_all)
    def _():
        finish(yrows)

    @pl.when(jnp.logical_not(hit_all))
    def _():
        xsel = jnp.concatenate([ln2_v[pl.ds(vgrp[c], 8), :] for c in range(2)], axis=0)

        def ffn_tile(j, acc):
            cs = pl.ds(pl.multiple_of(j * LANES, LANES), LANES)
            g = jnp.dot(xsel, wload(wg_v, 0, D, cs), preferred_element_type=F32)
            u = jnp.dot(xsel, wload(wu_v, 0, D, cs), preferred_element_type=F32)
            a = (g * jax.nn.sigmoid(g) * u).astype(BF16)
            wd_t = pltpu.bitcast(wd_v[pl.ds(pl.multiple_of(j * (LANES // 2), LANES // 2), LANES // 2), 0:D], BF16)
            return acc + jnp.dot(a, wd_t, preferred_element_type=F32)

        yf = lax.fori_loop(0, F // LANES, ffn_tile, jnp.zeros((16, D), F32))
        finish([yf[0:8, :], yf[8:16, :]])

    @pl.when(jnp.logical_not(in_tail))
    def _():
        tail_copy.wait()

    fix_copy(0).wait()

    @pl.when(two_groups)
    def _():
        fix_copy(1).wait()


@jax.jit
def pallas_sequential_preLN__linear_attn_block__moe_arch_mod__prompt_kernel(
    A_x: jax.Array,
    A_wqkv: jax.Array,
    A_wo: jax.Array,
    B_x: jax.Array,
    B_w_r: jax.Array,
    B_w_gate: jax.Array,
    B_w_up: jax.Array,
    B_w_down: jax.Array,
):
    del B_x
    x = A_x.reshape(S, D)
    wr = B_w_r.reshape(NC, LANES)
    any_spec = pl.BlockSpec(memory_space=pl.ANY)
    out = pl.pallas_call(
        _kernel,
        out_shape=jax.ShapeDtypeStruct((S, D), BF16),
        in_specs=[any_spec] * 7,
        out_specs=any_spec,
        scratch_shapes=[
            pltpu.VMEM((S + DEF, D), BF16),
            pltpu.VMEM((D // 2, D), U32),
            pltpu.VMEM((D // 2, D), U32),
            pltpu.VMEM((2, D // 2, D), U32),
            pltpu.VMEM((NC, LANES), BF16),
            pltpu.VMEM((2, D // 2, F + LANES), U32),
            pltpu.VMEM((F // 2, D + LANES), U32),
            pltpu.VMEM((P0 // 2, D), U32),
            pltpu.VMEM((7 ** LA, S // NA // 2, DA), U32),
            pltpu.VMEM((7 ** LA, DA // 2, DA), U32),
            pltpu.VMEM((D // 2, P0), U32),
            pltpu.VMEM((DA // 2, 7 ** LA * MA), U32),
            pltpu.VMEM((D, LANES), F32),
            pltpu.VMEM((D, LANES), F32),
            pltpu.VMEM((RL, LANES), F32),
            pltpu.VMEM((D, D), F32),
            pltpu.VMEM((7, HD, HD), F32),
            pltpu.VMEM((D // 2, D), U32),
            pltpu.VMEM((7 ** LA, DA // 2, DA), U32),
            pltpu.VMEM((D // 2, D), U32),
            pltpu.VMEM((7 ** LO, DO // 2, DO), U32),
            pltpu.VMEM((max(TB2, RL), D + 2 * LANES), F32),
            pltpu.VMEM((RL // 2, D), U32),
            pltpu.VMEM((7 ** LO, max(TB2, RL) // NO // 2, DO), U32),
            pltpu.VMEM((DEF, D), F32),
            pltpu.VMEM((2, S + DEF, D), BF16),
            pltpu.VMEM((TB, D), F32),
            pltpu.VMEM((8, LANES), U32),
            pltpu.SemaphoreType.DMA((NSEM,)),
        ],
        compiler_params=pltpu.CompilerParams(vmem_limit_bytes=110 * 1024 * 1024, disable_bounds_checks=True,
                                             disable_semaphore_checks=True),
    )(x, A_wqkv, A_wo, wr, B_w_gate, B_w_up, B_w_down)
    return out.reshape(1, S, D)
```

```python
import jax
import jax.numpy as jnp
from jax import lax
import jax.experimental.pallas as pl
import jax.experimental.pallas.tpu as pltpu


S = 2048
D = 1024
F = 3584
H = 32
DH = D // H
LANES = 128
NC = D // LANES
HD = D // 2

LA = 2
LO = 1
NA, NO = 2 ** LA, 2 ** LO
DA, DO = D // NA, D // NO
P0 = 512
PB = S - P0
TX = 256
TB = 512
NB1 = PB // TB
MA = TB // NA
TB2 = 384
NB2 = 4
QA = 192
OCH = (128, 128, 128)
DEF = OCH[-1]
L0 = NB2 * TB2
RL = S - L0
QS = (256, 256)
OCL = ((128, False), (128, False), (128, False), (64, True), (64, True))
NPRE = 22
NGAP = 9
OUT_AT = (256, 384, 448)
GM = 32
NZ = 5
WQP = 5
LNU = 8
LAG = 5
LAG_L = 5
LN_DELAY = 800
LN2_DELAY = 900
JOB_DELAY = 500
POST_DELAY = 800
QP_DELAY = 400
WK5 = 66
C6LN = (1000, 8900)
C6WK = (1500, 8900)
P1LN = (60, 10500)
P1WP = (6800, 11000)
P1WQ = (8000, 12300)
P2U = (60, 2000)
EV2 = 300
GLAG = (None, None, None, 20, 8)

F32 = jnp.float32
BF16 = jnp.bfloat16
U32 = jnp.uint32
I32 = jnp.int32

XP = ((PB, 128), (PB + 128, 128), (PB + 256, 256), (0, TB), (TB, PB - TB))
WKP = ((0, 128), (128, 128), (256, 256), (512, 512))

SEM_X = 0
SEM_WK = SEM_X + len(XP)
SEM_WQ = SEM_WK + len(WKP)
SEM_W3 = SEM_WQ + 1
SEM_WR = SEM_W3 + 1
SEM_WGU = SEM_WR + 1
SEM_WD = SEM_WGU + 1
SEM_OUT = SEM_WD + 1
NSEM = SEM_OUT + 5

INT_MIN = -(2 ** 31)


def _layernorm(x, tok=None, w=None):
    s0 = x[:, 0:LANES]
    if tok is not None:
        s0 = s0 + jnp.concatenate([tok] * (x.shape[0] // 8), axis=0)
    for c in range(1, NC):
        s0 = s0 + x[:, c * LANES:(c + 1) * LANES]
    mu = jnp.sum(s0, axis=-1, keepdims=True) * (1.0 / D)
    xc = x - mu
    var = jnp.sum(xc * xc, axis=-1, keepdims=True) * (1.0 / D)
    rstd = lax.rsqrt(var + 1e-5)
    if w is None:
        return xc * rstd
    return xc * rstd, jnp.sum(xc * w, axis=-1, keepdims=True) * rstd


def _phi(t):
    return jnp.where(t > 0, t + 1.0, jnp.exp(t)) + 1e-6


def _n_off(a, b):
    return 32 * a + 8 * b


def _n_groups():
    pos = {(2 * o + e) * LANES + _n_off(a, b): (16 * e + 4 * b + a) * DH + 8 * o
           for o in range(4) for e in range(2) for a in range(4) for b in range(4)}
    return [pos[n] for n in sorted(pos)]


def _quads(b):
    h = len(b) // 2
    return [[r[j * h:(j + 1) * h] for r in b[i * h:(i + 1) * h]] for i in range(2) for j in range(2)]


def _badd(x, y):
    return [[a + b for a, b in zip(rx, ry)] for rx, ry in zip(x, y)]


def _bsub(x, y):
    return [[a - b for a, b in zip(rx, ry)] for rx, ry in zip(x, y)]


def _a_set(b):
    if len(b) == 1:
        return [b[0][0]]
    return [x for o in _a_ops(b) for x in _a_set(o)]


def _b_set(b):
    if len(b) == 1:
        return [b[0][0]]
    q11, q12, q21, q22 = _quads(b)
    ops = (_badd(q11, q22), q11, _bsub(q12, q22), _bsub(q21, q11), q22, _badd(q11, q12), _badd(q21, q22))
    return [x for o in ops for x in _b_set(o)]


def _b_in_a(i, levels):
    perm = (0, 2, 6, 5, 3, 4, 1)
    return sum(perm[(i // 7 ** l) % 7] * 7 ** l for l in range(levels))


def _strassen(prod, levels, base=0, fin=lambda k, q: q, init=None):
    if levels == 0:
        return [[prod(base)]]

    def m(i):
        return _strassen(prod, levels - 1, base * 7 + i)

    def seed(q, x):
        return x if init is None else _badd(_quads(init)[q], x)

    m2 = m(2)
    c22 = seed(3, m2)
    m4 = m(4)
    c12 = fin(1, _badd(seed(1, m2), m4))
    c11 = m4 if init is None else _bsub(_quads(init)[0], m4)
    m3 = m(3)
    c11 = _bsub(m3, c11) if init is None else _badd(c11, m3)
    m1 = m(1)
    c21 = fin(2, _badd(seed(2, m3), m1))
    c22 = _bsub(c22, m1)
    m0 = m(0)
    c11 = _badd(c11, m0)
    c22 = _badd(c22, m0)
    c11 = fin(0, _badd(c11, m(6)))
    c22 = fin(3, _badd(c22, m(5)))
    return [a + b for a, b in zip(c11, c12)] + [a + b for a, b in zip(c21, c22)]


def _goff(i, levels):
    return int(format(i, "0%db" % levels)[::-1], 2) if levels else 0


def _blocks(rows, n):
    w = rows[0].shape[1] // n
    return [[r[:, j * w:(j + 1) * w] for j in range(n)] for r in rows]


def _or_all(vals):
    acc = None
    for v in vals:
        v = v if v.dtype == U32 else pltpu.bitcast(v, U32)
        for g in range(v.shape[0] // 8):
            for c in range(v.shape[1] // LANES):
                p = v if v.shape == (8, LANES) else v[g * 8:(g + 1) * 8, c * LANES:(c + 1) * LANES]
                acc = p if acc is None else acc | p
    return acc


def _raw_ops(levels):
    n = 2 ** levels
    names = [[_Tag((i, j)) for j in range(n)] for i in range(n)]
    return {op: t.ij for op, t in enumerate(_b_set(names)) if t.ij is not None}


class _Tag:
    def __init__(self, ij):
        self.ij = ij

    def __add__(self, other):
        return _Tag(None)

    __sub__ = __add__


def _a_ops(b):
    q11, q12, q21, q22 = _quads(b)
    return (_badd(q11, q22), _badd(q21, q22), q11, q22, _badd(q11, q12), _bsub(q21, q11), _bsub(q12, q22))


_A_FORM = (((0, 0), (1, 1), 1), ((1, 0), (1, 1), 1), ((0, 0),), ((1, 1),), ((0, 0), (0, 1), 1),
           ((1, 0), (0, 0), -1), ((0, 1), (1, 1), -1))
_B_FORM = (((0, 0), (1, 1), 1), ((0, 0),), ((0, 1), (1, 1), -1), ((1, 0), (0, 0), -1), ((1, 1),),
           ((0, 0), (0, 1), 1), ((1, 0), (1, 1), 1))
_C_FORM = (((0, 1), (3, 1), (4, -1), (6, 1)), ((2, 1), (4, 1)), ((1, 1), (3, 1)), ((0, 1), (1, -1), (2, 1), (5, 1)))


def _outer(form, get, n):
    h = n // 2

    def quad(q):
        return [[get(q[0] * h + i, q[1] * h + j) for j in range(h)] for i in range(h)]

    if len(form) == 1:
        return quad(form[0])
    return (_badd if form[2] > 0 else _bsub)(quad(form[0]), quad(form[1]))


def _gate(v, tok):
    u = pltpu.bitcast(v, U32)
    top = u[0:8, 0:LANES] | tok
    if u.shape[1] > LANES:
        top = jnp.concatenate([top, u[0:8, LANES:]], axis=1)
    return pltpu.bitcast(jnp.concatenate([top, u[8:, :]], axis=0) if u.shape[0] > 8 else top, BF16)


class _Pacer:
    def __init__(self, zero, every=0):
        self.zero, self.t, self.jobs, self.pend, self.res, self.tok = zero, 0, [], [], None, None
        self.every, self.last = every, -every

    def add(self, jobs, t0, t1, delay):
        for k, job in enumerate(jobs):
            self.jobs.append((t0 + k * (t1 - t0) // len(jobs), len(self.jobs), job, delay))
        self.jobs.sort(key=lambda e: e[:2])

    def due(self, dep, delay):
        if dep is not None:
            self.pend.append((self.t + delay, _or_all([dep])))

    def release(self, upto):
        while self.jobs and self.jobs[0][0] <= upto:
            _, _, job, delay = self.jobs.pop(0)
            if self.res is not None:
                self.tok = pltpu.bitcast(pltpu.bitcast(self.res[0:8, 0:LANES], U32) & self.zero, F32)
                self.res = None
            self.due(job(self.tok), delay)

    def dot(self, lhs, rhs):
        self.release(self.t)
        ready = [d for t, d in self.pend if t <= self.t]
        if ready and self.t - self.last >= self.every:
            self.pend = [e for e in self.pend if e[0] > self.t]
            self.last = self.t
            lhs = _gate(lhs, _or_all(ready) & self.zero)
        res = jnp.dot(lhs, rhs, preferred_element_type=F32)
        self.t += lhs.shape[0] * (lhs.shape[1] // LANES) * (res.shape[1] // LANES) // 4
        self.res = res
        return res

    def flush(self):
        self.release(1 << 30)


def _kernel(x_hbm, wqkv_hbm, wo_hbm, wr_hbm, wg_hbm, wu_hbm, wd_hbm, out_hbm,
            x_v, wk_v, wq_v, w3_v, wr_v, wgu_v, wd_v,
            ln1_v, xs_v, wks_v, pkt_v, pks_v, zacc_v, uacc_v, xw_v, g_v, gs_v, wqp_v, wqs_v, mp_v, ms_v,
            pq_v, pqn_v, pqs_v, attn_v, lo_v, lnf_v, zero_v, sems):

    ln2_v, out_v = lo_v.at[0], lo_v.at[1]

    def wload(ref, r0, nr, cols):
        if ref.dtype == BF16:
            return ref[r0:r0 + nr, cols]
        return pltpu.bitcast(ref[r0 // 2:(r0 + nr) // 2, cols], BF16)

    wv_v, wo_v = w3_v.at[0], w3_v.at[1]
    wg_v, wu_v = wgu_v.at[0], wgu_v.at[1]

    def x_copy(i):
        r0, n = XP[i]
        return pltpu.make_async_copy(x_hbm.at[pl.ds(r0, n), :], x_v.at[pl.ds(DEF + r0, n), :], sems.at[SEM_X + i])

    def out_copy(r0, n, s):
        return pltpu.make_async_copy(out_v.at[pl.ds(DEF + r0, n), :], out_hbm.at[pl.ds(r0, n), :],
                                     sems.at[SEM_OUT + s])

    def wk_copy(j):
        c0, n = WKP[j]
        return pltpu.make_async_copy(wqkv_hbm.at[:, pl.ds(D + c0, n)], wk_v.at[:, pl.ds(c0, n)],
                                     sems.at[SEM_WK + j])

    wq_copy = pltpu.make_async_copy(wqkv_hbm.at[:, pl.ds(0, D)], wq_v.at[:, pl.ds(0, D)], sems.at[SEM_WQ])
    wv_copy = pltpu.make_async_copy(wqkv_hbm.at[:, pl.ds(2 * D, D)], wv_v.at[:, pl.ds(0, D)], sems.at[SEM_W3])
    wo_copy = pltpu.make_async_copy(wo_hbm, wo_v.at[:, pl.ds(0, D)], sems.at[SEM_W3])
    wr_copy = pltpu.make_async_copy(wr_hbm, wr_v, sems.at[SEM_WR])
    wd_copy = pltpu.make_async_copy(wd_hbm, wd_v.at[:, pl.ds(0, D)], sems.at[SEM_WD])
    wg_copy = pltpu.make_async_copy(wg_hbm, wg_v, sems.at[SEM_WGU])
    wu_copy = pltpu.make_async_copy(wu_hbm, wu_v, sems.at[SEM_WGU])

    x_copy(0).start()
    wk_copy(0).start()
    x_copy(1).start()
    wr_copy.start()
    for j in range(1, len(WKP)):
        wk_copy(j).start()
    for j in range(2, len(XP)):
        x_copy(j).start()
    wq_copy.start()
    wv_copy.start()
    wo_copy.start()
    wg_copy.start()
    wu_copy.start()
    wd_copy.start()

    def ln1_rows(xr, xr0, lnr, r0, n):
        ln = _layernorm(xr[xr0:xr0 + n, :].astype(F32)).astype(BF16)
        lnr[r0 // 2:(r0 + n) // 2, :] = pltpu.bitcast(ln, U32)

    def ln1_set(pc, xr, xr0, xsr, a0, n, t0, t1):
        def unit(j):
            def job(tok):
                ln = _layernorm(xr[xr0 + j * LNU:xr0 + (j + 1) * LNU, :].astype(F32), tok)
                lnf_v[j * LNU:(j + 1) * LNU, :] = ln
                return _or_all([ln[:, 0:LANES], ln[:, D - LANES:D]])
            return job

        def piece(j0, c0, o):
            def job(tok):
                def get(i, f):
                    r = (j0 + 2 * _goff(i, LA)) * LNU
                    v = lnf_v[r:r + 16, f * DA + c0:f * DA + c0 + LANES]
                    return v + jnp.concatenate([tok, tok], axis=0) if (i + f) % (NA // 2 + 1) == 0 else v

                r = (a0 + (j0 // (2 * NA)) * 16) // 2
                ops = _a_set(_outer(_A_FORM[o], get, NA))
                for op, v in enumerate(ops):
                    xsr.at[o * len(ops) + op][r:r + 8, c0:c0 + LANES] = pltpu.bitcast(v.astype(BF16), U32)
                return _or_all([v[0:8, :] for v in [ops[0]] + ops[5:7]])
            return job

        grp = 2 * NA
        ng = n // LNU // grp
        dt = (t1 - t0 - LN_DELAY) // (ng + 1)
        for g in range(ng):
            pc.add([unit(g * grp + j) for j in range(grp)], t0 + g * dt, t0 + (g + 1) * dt, LN_DELAY)
            s = t0 + (g + 1) * dt + LN_DELAY
            pc.add([piece(g * grp, c0, o) for c0 in range(0, DA, LANES) for o in range(7)], s, s + dt, JOB_DELAY)

    def ln1_load(lnr, r0, n):
        return pltpu.bitcast(lnr[r0 // 2:(r0 + n) // 2, :], BF16)

    def k_mm(r0, n, c0, nc):
        return jnp.dot(ln1_load(ln1_v, r0, n), wload(wk_v, 0, D, slice(c0, c0 + nc)), preferred_element_type=F32)

    def z_acc(pkts, c0, first=False):
        zs = None
        for pkt in pkts:
            for j in range(pkt.shape[1] // LANES):
                p = pkt[:, j * LANES:(j + 1) * LANES]
                zs = p if zs is None else zs + p
        if first:
            zacc_v[c0:c0 + zs.shape[0], :] = zs
        else:
            zacc_v[c0:c0 + zs.shape[0], :] += zs

    def k_post(k, p0, c0, first=False):
        n, nc = k.shape
        pkt = _phi(k).T
        pkt_v[c0 // 2:(c0 + nc) // 2, p0:p0 + n] = pltpu.bitcast(pkt.astype(BF16), U32)
        z_acc([pkt], c0, first)
        return pkt[nc - 8:nc, n - LANES:n]

    def g_acc(r0, n, c0, nc, first=False, pc=None):
        h, w = (nc, D) if pc is None else (LANES, LANES)
        for f0 in range(c0, c0 + nc, h):
            for j0 in range(0, D, w):
                lhs = pltpu.bitcast(pkt_v[f0 // 2:(f0 + h) // 2, r0:r0 + n], BF16)
                rhs = pltpu.bitcast(ln1_v[r0 // 2:(r0 + n) // 2, j0:j0 + w], BF16)
                g = jnp.dot(lhs, rhs, preferred_element_type=F32) if pc is None else pc.dot(lhs, rhs)
                if first:
                    g_v[f0:f0 + h, j0:j0 + w] = g
                else:
                    g_v[f0:f0 + h, j0:j0 + w] += g

    def k_paced(pc, r0, c0, nc, first):
        for j0 in range(c0, c0 + nc, LANES):
            for t0 in range(r0, r0 + TX, LANES):
                k = None
                for k0 in range(0, D, TX):
                    p = pc.dot(ln1_load(ln1_v, t0, LANES)[:, k0:k0 + TX], wload(wk_v, k0, TX, slice(j0, j0 + LANES)))
                    k = p if k is None else k + p
                pc.due(k_post(k, t0, j0, first and t0 == r0), POST_DELAY)

    attn_v[...] = jnp.zeros_like(attn_v)
    zero_v[...] = jnp.zeros_like(zero_v)

    def gs_zero(o0, o1):
        gs_v[o0:o1] = jnp.zeros((o1 - o0, HD, HD), F32)

    x_copy(0).wait()
    ln1_rows(x_v, DEF + PB, ln1_v, 0, 128)
    gs_zero(0, 1)
    wk_copy(0).wait()
    ka = k_mm(0, 128, 0, 128)
    gs_zero(1, 2)
    x_copy(1).wait()
    wr_copy.wait()
    gs_zero(2, 3)
    ln1_rows(x_v, DEF + PB + 128, ln1_v, 128, 128)
    k_post(ka, 0, 0, first=True)
    g_acc(0, 128, 0, 128, first=True)
    wk_copy(1).wait()
    gs_zero(3, NZ)
    k_post(k_mm(128, 128, 0, 128), 128, 0)
    k_post(k_mm(0, TX, 128, 128), 0, 128, first=True)
    g_acc(128, 128, 0, 128)

    def w_job(src_ref, dst_ref, levels, r0, c0, o):
        n = 2 ** levels
        w, raw, inner = D // n, _raw_ops(levels), 7 ** (levels - 1)

        def job(tok):
            def cut(i, j):
                return wload(src_ref, i * w + r0, 16, slice(j * w + c0, j * w + c0 + LANES))

            def get(i, j):
                v = cut(i, j).astype(F32)
                return v + jnp.concatenate([tok, tok], axis=0) if (i + j) % (n // 2 + 1) == 0 else v

            ops = []
            for op, v in enumerate(_b_set(_outer(_B_FORM[o], get, n))):
                dst = dst_ref.at[o * inner + op]
                if o * inner + op in raw:
                    dst[r0 // 2:r0 // 2 + 8, c0:c0 + LANES] = pltpu.bitcast(cut(*raw[o * inner + op]), U32)
                else:
                    dst[r0 // 2:r0 // 2 + 8, c0:c0 + LANES] = pltpu.bitcast(v.astype(BF16), U32)
                    ops.append(v)
            return _or_all(ops[0:1] + ops[-2:]) if ops else None
        return job

    def wk_jobs_of(outer):
        return [w_job(wk_v, wks_v, LA, r0, c0, o) for r0 in range(0, DA, 16) for c0 in range(0, DA, LANES)
                for o in outer]

    wk_copy(2).wait()
    pc = _Pacer(zero_v[...])
    pc.add(wk_jobs_of((1, 3)), 500, 2200, JOB_DELAY)
    k_paced(pc, 0, 256, 256, True)
    g_acc(0, TX, 128, 128, True, pc)
    g_acc(0, TX, 256, 256, True, pc)
    pc.flush()
    wk_copy(3).wait()
    wk_jobs = wk_jobs_of((0, 2, 4, 5, 6))
    pc = _Pacer(zero_v[...])
    pc.add(wk_jobs[:WK5], 500, 2700, JOB_DELAY)
    k_paced(pc, 0, 512, 512, True)
    g_acc(0, TX, 512, 256, True, pc)
    pc.flush()
    x_copy(2).wait()
    x_copy(3).wait()
    pc = _Pacer(zero_v[...])
    ln1_set(pc, x_v, DEF, xs_v, 0, TB, *C6LN)
    pc.add(wk_jobs[WK5:], *C6WK, JOB_DELAY)
    ln1_rows(x_v, DEF + PB + TX, ln1_v, TX, TX)
    g_acc(0, TX, 768, 256, True, pc)
    k_paced(pc, TX, 0, D, False)
    for c0 in range(0, D, 256):
        g_acc(TX, TX, c0, 256, False, pc)
    pc.flush()

    def xs_load(xsr, op, a0, m):
        return pltpu.bitcast(xsr[op, a0 // 2:(a0 + m) // 2, :], BF16)

    def k_step(pc, xsr, j0):
        def fin(_, q):
            q = [[_phi(v).T for v in r] for r in q]
            pc.due(_or_all([v[LANES - 8:LANES, :] for r in q for v in r]), POST_DELAY)
            return q

        cb = _strassen(lambda i: pc.dot(xs_load(xsr, i, 0, MA), pltpu.bitcast(wks_v[i, :, j0:j0 + LANES], BF16)),
                       LA, fin=fin)
        outer = _a_ops([[cb[i][f] for i in range(NA)] for f in range(NA)])
        for half, o in ((0, outer[4]), (1, outer[1])):
            for f, rowb in enumerate(o):
                z_acc(rowb, half * HD + f * DA + j0)
        ops = [v for o in outer for v in _a_set(o)]
        for op, v in enumerate(ops):
            pks_v[j0 // 2:(j0 + LANES) // 2, op * MA:(op + 1) * MA] = pltpu.bitcast(v.astype(BF16), U32)
        pc.due(_or_all([v[LANES - 8:LANES, :] for v in (ops[0], ops[-1], ops[-2])]), 2 * POST_DELAY)

    def g_step(pc, xsr, r0, later):
        def old(o, f, c):
            v = gs_v[o, f * DA + r0:f * DA + r0 + GM, c * DA:(c + 1) * DA]
            return v if o < NZ else jnp.where(later, v, 0.0)

        for o in range(7):
            cb = _strassen(lambda i: pc.dot(pltpu.bitcast(pks_v[r0 // 2:(r0 + GM) // 2, i * MA:(i + 1) * MA], BF16),
                                            xs_load(xsr, _b_in_a(i, LA), 0, MA)), LA - 1, base=o,
                           init=[[old(o, f, c) for c in range(NA // 2)] for f in range(NA // 2)])
            for f in range(NA // 2):
                for c in range(NA // 2):
                    gs_v[o, f * DA + r0:f * DA + r0 + GM, c * DA:(c + 1) * DA] = cb[f][c]

    def wq_jobs(u0, nr):
        span = (NA - 1) * DA + 16 * nr
        u0 = u0 if isinstance(u0, int) else pl.multiple_of(u0, 8)
        r_first = 2 * u0 if isinstance(u0, int) else pl.multiple_of(2 * u0, 16)
        srcr, permr = wq_v.at[pl.ds(r_first, span), :], wqp_v.at[pl.ds(u0, span // 2), :]
        dstr = wqs_v.at[:, pl.ds(u0, 8 * nr), :]
        oct_ = (lax.broadcasted_iota(I32, (8, LANES), 1) % DH) // 8

        def perm(r, e):
            def job(tok):
                blk = [pltpu.bitcast(srcr[r:r + 16, (4 * e + b) * LANES:(4 * e + b + 1) * LANES], U32)
                       | pltpu.bitcast(tok, U32)
                       for b in range(4)]
                outs = []
                for o in range(4):
                    v = blk[o]
                    for b in range(4):
                        if b != o:
                            v = jnp.where(oct_ == b, pltpu.roll(blk[b], (8 * (b - o)) % LANES, 1), v)
                    permr[r // 2:r // 2 + 8, (2 * o + e) * LANES:(2 * o + e + 1) * LANES] = v
                    outs.append(v)
                return _or_all(outs)
            return job

        return ([perm(i * DA + r0, e) for r0 in range(0, 16 * nr, 16) for i in range(NA) for e in range(2)],
                [w_job(permr, dstr, LA, r0, c0, o) for r0 in range(0, 16 * nr, 16)
                 for c0 in range(0, DA, LANES) for o in range(7)])

    def p1(i, carry):
        xsr = xs_v.at[:, pl.ds(pl.multiple_of(i * (MA // 2), MA // 2), MA), :]
        xr = x_v.at[pl.ds(pl.multiple_of((i + 1) * TB, TB), TB + DEF), :]

        pc = _Pacer(zero_v[...])
        ln1_set(pc, xr, DEF, xsr, MA, TB, *P1LN)
        perms, sets = wq_jobs(i * (8 * WQP), WQP)
        pc.add(perms, *P1WP, JOB_DELAY)
        pc.add(sets, *P1WQ, JOB_DELAY)
        for j0 in range(0, DA, LANES):
            k_step(pc, xsr, j0)
        for r0 in range(0, DA, GM):
            g_step(pc, xsr, r0, i > 0)
        pc.flush()
        return carry

    x_copy(4).wait()
    wq_copy.wait()
    lax.fori_loop(0, NB1, p1, 0)

    wv_copy.wait()
    wo_copy.wait()
    zero_u = zero_v[...]
    zrow = jnp.sum(jnp.concatenate([zacc_v[r:r + 8, :] for r in _n_groups()], axis=0).T, axis=0, keepdims=True)
    wr8 = wr_v[...].astype(F32)
    wr_row = jnp.concatenate([wr8[c:c + 1, :] for c in range(NC)], axis=1)

    row_h = lax.broadcasted_iota(I32, (LANES, LANES), 0) // DH
    col_h = lax.broadcasted_iota(I32, (LANES, LANES), 1) // DH
    diag = row_h == col_h

    def colsum(t):
        acc = t[:, 0:LANES]
        for c in range(1, NC):
            acc = acc + t[:, c * LANES:(c + 1) * LANES]
        return acc

    wrc = wr_row - jnp.sum(wr_row, axis=-1, keepdims=True) * (1.0 / D)
    m_raw = _raw_ops(LO)

    def kv_part(c):
        cs = slice(c * LANES, (c + 1) * LANES)
        kv = None
        for k0 in range(0, D, TX):
            g = g_v[cs, k0:k0 + TX]
            for o, sign in _C_FORM[(c * LANES // HD) * 2 + k0 // HD]:
                t = gs_v[o, c * LANES % HD:c * LANES % HD + LANES, k0 % HD:k0 % HD + TX]
                g = g + t if sign > 0 else g - t
            p = pc.dot(g.astype(BF16), wload(wv_v, k0, TX, cs))
            kv = p if kv is None else kv + p
        return jnp.where(diag, kv, 0.0)

    def m_part(c, kvs):
        e, b = c // 4, c % 4
        for j0 in range(0, DO, LANES):
            ms = [jnp.concatenate(
                [pc.dot(kv, wload(wo_v, (c + k) * LANES, LANES, slice(f * DO + j0, f * DO + j0 + LANES)))
                 for f in range(NO)], axis=1) for k, kv in enumerate(kvs)]
            deps = []
            for a in range(4):
                rows = [jnp.concatenate([m[a * DH + 8 * o:a * DH + 8 * o + 8, :] for m in ms], axis=0)
                        for o in range(4)]
                for o in range(4):
                    r = ((2 * o + e) * LANES + _n_off(a, b)) // 2
                    for f in range(NO):
                        mp_v[r:r + 8, f * DO + j0:f * DO + j0 + LANES] = pltpu.bitcast(
                            rows[o][:, f * LANES:(f + 1) * LANES].astype(BF16), U32)
                for t in range(4 // NO):
                    r = ((2 * t + e) * LANES + _n_off(a, b)) // 2
                    for op, v in enumerate(_b_set(_blocks(rows[t::4 // NO], NO))):
                        if op not in m_raw:
                            ms_v.at[op][r:r + 8, j0:j0 + LANES] = pltpu.bitcast(v.astype(BF16), U32)
                            deps.append(v[0:8, 0:LANES])
            pc.due(_or_all(deps[::4]), POST_DELAY)

    pc = _Pacer(zero_u)
    pc.due(jnp.broadcast_to(zrow, (8, D)), 1000)
    perms, sets = wq_jobs(NB1 * 8 * WQP, DA // 16 - NB1 * WQP)
    pc.add(perms, 60, 700, JOB_DELAY)
    pc.add(sets, 1300, 3500, JOB_DELAY)
    kv_prev = None
    for c in range(0, NC + 2, 2):
        kvs = [kv_part(c).astype(BF16), kv_part(c + 1).astype(BF16)] if c < NC else None
        if c:
            m_part(c - 2, kv_prev)
        kv_prev = kvs
    pc.flush()

    def make_key(score, row):
        b = pltpu.bitcast(score, I32)
        srt = b ^ ((b >> 31) & 0x7FFFFFFF)
        return (srt & jnp.int32(-65536)) | (0xFFFF - row)

    def push_keys(key, top1, top2):
        for gidx in range(key.shape[0] // 8):
            kx = key[gidx * 8:(gidx + 1) * 8, :]
            top2 = jnp.maximum(top2, jnp.minimum(top1, kx))
            top1 = jnp.maximum(top1, kx)
        return top1, top2

    lane = lax.broadcasted_iota(I32, (1, LANES), 1)

    def interleave(parts):
        return jnp.concatenate([p[g * 16:(g + 1) * 16, :] for g in range(parts[0].shape[0] // 16) for p in parts],
                               axis=0)

    def q_part(pc, xsr, l0, r0, n, hint=None):
        m = n // NA
        sums = {}

        def park(v, g, c):
            for t in range(m // 16):
                r = r0 + (t * NA + g) * 16
                pq_v[r:r + 16, c * LANES:(c + 1) * LANES] = v[t * 16:(t + 1) * 16, :]

        def fin(k, q):
            q = [[_phi(v) for v in r] for r in q]
            deps = []
            for a, r in enumerate(q):
                for b, v in enumerate(r):
                    i, c = (k // 2) * (NA // 2) + a, (((k % 2) * (NA // 2) + b) * DA + j0) // LANES
                    park(v, _goff(i, LA), c)
                    for name, row in (("z", zrow),) + ((("u", hint["u"]),) if hint else ()):
                        t = v * row[:, c * LANES:(c + 1) * LANES]
                        key = (name, _goff(i, LA), c % 2)
                        sums[key] = t if key not in sums else sums[key] + t
                deps.append(sums[key])
            if hint:
                pc.due(_or_all(deps), POST_DELAY)
            return q

        for j0 in range(0, DA, LANES):
            _strassen(lambda i: pc.dot(xs_load(xsr, i, (l0 + r0) // NA, m),
                                       pltpu.bitcast(wqs_v[i, :, j0:j0 + LANES], BF16)), LA, fin=fin)
        if hint:
            pc.flush()
        den = jnp.concatenate([sums["z", g, e] for g in range(NA) for e in range(2)], axis=0)
        for s in (1, 2, 4):
            den = den + jnp.where((lane & s) == 0, pltpu.roll(den, LANES - s, 1), pltpu.roll(den, s, 1))
        inv_all = 1.0 / (den + 1e-6)

        def inv_of(g):
            return [inv_all[(g * 2 + e) * m:(g * 2 + e + 1) * m, :] for e in range(2)]

        for g in range(NA):
            for e in range(2):
                park(inv_of(g)[e], g, NC + e)
        if hint:
            for g in range(NA):
                starts = [r0 + (t * NA + g) * 16 for t in range(m // 16)]
                num = jnp.sum(jnp.concatenate([xw_v[t:t + 16, :] for t in starts], axis=0)
                              + sums["u", g, 0] * inv_of(g)[0] + sums["u", g, 1] * inv_of(g)[1],
                              axis=-1, keepdims=True)
                row = jnp.concatenate([(l0 + t) + lax.broadcasted_iota(I32, (16, 1), 0) for t in starts], axis=0)
                hint["p1"], hint["p2"] = push_keys(make_key(num, row), hint["p1"], hint["p2"])
            pc.due(jnp.broadcast_to(hint["p1"], (8, LANES)), 1200)


    def post_jobs(r0, n, plain=False):
        def scaled(t, c0, w, tok):
            inv = pq_v[t:t + 16, D:D + 2 * LANES]
            if tok is not None:
                inv = inv + jnp.concatenate([jnp.concatenate([tok, tok], axis=0)] * 2, axis=1)
            return pq_v[t:t + 16, c0:c0 + w] * jnp.concatenate([inv] * (w // (2 * LANES)), axis=1)

        def post_plain(t):
            def job(tok):
                v = scaled(t, 0, D, tok)
                pqn_v[t // 2:t // 2 + 8, :] = pltpu.bitcast(v.astype(BF16), U32)
                return v[0:8, 0:LANES]
            return job

        def post(t0, outer):
            def job(tok):
                deps = []
                for c0 in range(0, DO, 2 * LANES):
                    blk = {}

                    def get(i, f):
                        if (i, f) not in blk:
                            blk[i, f] = scaled(t0 + _goff(i, LO) * 16, f * DO + c0, 2 * LANES, tok)
                        return blk[i, f]

                    for o in outer:
                        ops = _a_set(_outer(_A_FORM[o], get, NO))
                        for op, v in enumerate(ops):
                            pqs_v.at[o * len(ops) + op][t0 // NO // 2:t0 // NO // 2 + 8, c0:c0 + 2 * LANES] = (
                                pltpu.bitcast(v.astype(BF16), U32))
                        deps.append(ops[0][0:8, 0:LANES])
                return _or_all(deps)
            return job

        if plain:
            return [post_plain(t) for t in range(r0, r0 + n, 16)]
        outers = [range(7)] if LO == 1 else [(o,) for o in range(7)]
        return [post(t0, outer) for t0 in range(r0, r0 + n, 16 * NO) for outer in outers]

    def m_operand(i, c0, c1):
        if i not in m_raw:
            return pltpu.bitcast(ms_v[i, :, c0 * LANES:c1 * LANES], BF16)
        bi, bj = m_raw[i]
        return wload(mp_v, bi * DO, DO, slice(bj * DO + c0 * LANES, bj * DO + c1 * LANES))

    def o_part(dot, xr, x0, r0, n):
        a0, m = r0 // NO, n // NO
        nw = LANES * NO // 2
        cols = [[[] for _ in range(NO)] for _ in range(NO)]
        for c0 in range(0, DO, nw):
            init = [[jnp.concatenate(
                [xr[x0 + r0 + (g * NO + _goff(i, LO)) * 16:x0 + r0 + (g * NO + _goff(i, LO) + 1) * 16,
                    f * DO + c0:f * DO + c0 + nw] for g in range(m // 16)], axis=0).astype(F32)
                for f in range(NO)] for i in range(NO)]
            cb = _strassen(lambda i: dot(pltpu.bitcast(pqs_v[i, a0 // 2:(a0 + m) // 2, :], BF16),
                                         m_operand(i, c0 // LANES, (c0 + nw) // LANES)), LO, init=init)
            for i in range(NO):
                for f in range(NO):
                    cols[i][f].append(cb[i][f])
        parts = [None] * NO
        for i in range(NO):
            parts[_goff(i, LO)] = jnp.concatenate([c for f in range(NO) for c in cols[i][f]], axis=1)
        return interleave(parts)

    def ln2_unit(h, l2r, outr, r0, row0, valid, top1, top2, tok, fast=False):
        n = h.shape[0]
        if fast:
            ln2, r = _layernorm(h, tok, wr_row)
        else:
            ln2 = _layernorm(h, tok)
            r = jnp.sum(ln2 * wr_row, axis=-1, keepdims=True)
        l2r[r0:r0 + n, :] = ln2.astype(BF16)
        res = h + ln2
        outr[r0:r0 + n, :] = res.astype(BF16)
        r = r.astype(BF16).astype(F32) + 0.0
        key = make_key(r, (row0 + r0) + lax.broadcasted_iota(I32, (n, 1), 0))
        if valid is not None:
            key = jnp.where(valid, key, INT_MIN)
        top1, top2 = push_keys(key, top1, top2)
        ntok = pltpu.bitcast(pltpu.bitcast(jnp.broadcast_to(r[n - 8:n, :], (8, LANES)), U32) & zero_u, F32)
        return top1, top2, ntok

    def ln2_jobs(h, l2r, outr, r0, row0, valid, st, fast=False):
        def unit(j):
            def job(tok):
                st["top1"], st["top2"], dep = ln2_unit(h[j * LNU:(j + 1) * LNU, :], l2r, outr, r0 + j * LNU, row0,
                                                       valid, st["top1"], st["top2"], tok, fast)
                return dep
            return job
        return [unit(j) for j in range(h.shape[0] // LNU)]

    QC = 16 * 7 ** LA / 8 ** LA

    def p2(i, carry):
        st = dict(top1=carry[0], top2=carry[1])
        b0 = pl.multiple_of(i * TB2, 16)
        xsr = xs_v.at[:, pl.ds(pl.multiple_of(i * (TB2 // NA // 2), 8), TB2 // NA // 2), :]
        xr = x_v.at[pl.ds(b0, TB2 + DEF), :]
        l2r = ln2_v.at[pl.ds(b0, TB2 + DEF), :]
        outr = out_v.at[pl.ds(b0, TB2 + DEF), :]
        row0 = b0 - DEF
        pc = _Pacer(zero_u)
        toks = []

        def chain(jobs):
            for job in jobs:
                toks.append(job(toks[-LAG] if len(toks) >= LAG else None))

        chain(ln2_jobs(attn_v, l2r, outr, 0, row0, i > 0, st))

        @pl.when(i > 0)
        def _():
            out_copy(pl.multiple_of((i - 1) * TB2, 16), TB2, 0).start()

        pc.due(toks[-1], QA * QC)

        nu, nx = D // NB2, RL // NB2
        mr = mp_v.at[pl.ds(pl.multiple_of(i * (nu // 2), 8), nu // 2), :]
        ur = uacc_v.at[pl.ds(pl.multiple_of(i * nu, 8), nu), :]
        xl = x_v.at[pl.ds(pl.multiple_of(DEF + L0 + i * nx, 16), nx), :]
        xwr = xw_v.at[pl.ds(pl.multiple_of(i * nx, 8), nx), :]

        def hint_job(load, dst, r):
            def job(tok):
                v = colsum(load(r).astype(F32) * wrc) + jnp.concatenate([tok, tok], axis=0)
                dst[r:r + 16, :] = v
                return v
            return job

        pc.add([hint_job(lambda r: wload(mr, r, 16, slice(None)), ur, r) for r in range(0, nu, 16)]
               + [hint_job(lambda r: xl[r:r + 16, :], xwr, r) for r in range(0, nx, 16)], *P2U, JOB_DELAY)
        for r0, n in ((0, QA), (QA, TB2 - QA)):
            q_part(pc, xsr, 0, r0, n)
            for job in post_jobs(r0, n):
                job(None)
        r0 = 0
        for n in OCH[:-1]:
            chain(ln2_jobs(o_part(pc.dot, xr, DEF, r0, n), l2r, outr, DEF + r0, row0, None, st))
            r0 += n
        attn_v[...] = o_part(pc.dot, xr, DEF, r0, DEF)
        return st["top1"], st["top2"]

    init = jnp.full((8, 1), INT_MIN, I32)
    top1, top2 = lax.fori_loop(0, NB2, p2, (init, init))

    wg_copy.wait()
    wu_copy.wait()
    wd_copy.wait()
    sub8 = lax.broadcasted_iota(I32, (8, LANES), 0)
    urow = jnp.sum(uacc_v[...].T, axis=0, keepdims=True)

    def submax(v):
        for sh in (4, 2, 1):
            v = jnp.maximum(v, pltpu.roll(v, sh, 0))
        return v

    def subsum(v):
        for sh in (4, 2, 1):
            v = v + pltpu.roll(v, sh, 0)
        return v

    def best2(t1, t2):
        t1 = jnp.broadcast_to(t1, (8, LANES))
        t2 = jnp.broadcast_to(t2, (8, LANES))
        k1v = submax(t1)
        return k1v, submax(jnp.where(t1 == k1v, t2, t1))

    def key_row(k):
        return 0xFFFF - (k & 0xFFFF)

    def wide(m):
        return jnp.concatenate([m] * NC, axis=1)

    st = dict(top1=top1, top2=top2, pend=[], step=0, sent=0)
    pc = _Pacer(zero_u, EV2)
    hint = dict(u=urow, p1=init, p2=init)

    pc.add(ln2_jobs(attn_v, ln2_v, out_v, L0, -DEF, None, st), 60, QS[0] * QC - 600, LN2_DELAY)
    r0 = 0
    for k, n in enumerate(QS):
        q_part(pc, xs_v, L0, r0, n, hint)
        if k == 0:
            out_copy(L0 - TB2, TB2, 0).start()
            top1, top2 = st["top1"], st["top2"]
            pc.add(post_jobs(0, OCL[0][0], OCL[0][1]), pc.t + 600, pc.t + (RL - n) * QC - 300, QP_DELAY)
        r0 += n
    pc.every = 0
    oldk = best2(top1, top2)
    oldx = []
    for kk in oldk:
        g8 = pl.multiple_of(((jnp.clip(key_row(kk[0, 0]), 0, S - 1) >> 3) << 3) + DEF, 8)
        rows = ln2_v[pl.ds(g8, 8), :].astype(F32)
        oldx.append(subsum(jnp.where(wide((key_row(kk) & 7) == sub8), rows, 0.0)))

    def gated(v):
        tok = None
        while st["pend"] and st["pend"][0][0] <= st["step"]:
            t = st["pend"].pop(0)[1]
            tok = t if tok is None else tok | t
        if tok is None:
            return v
        u = pltpu.bitcast(v, U32)
        return pltpu.bitcast(jnp.concatenate([u[:, 0:LANES] | tok, u[:, LANES:]], axis=1), BF16)

    res = {}

    def c_units():
        pc.flush()
        p1, p2_ = hint["p1"], hint["p2"]
        cand_p, cand_x = [], []
        for pk_ in (p1, p2_):
            cp, cx = None, None
            for s in range(8):
                g8 = pl.multiple_of((jnp.clip(key_row(pk_[s, 0]) - L0, 0, RL - 1) >> 3) << 3, 8)
                vp = pq_v[pl.ds(g8, 8), :]
                vx = x_v[pl.ds(pl.multiple_of(g8 + (L0 + DEF), 8), 8), :].astype(F32)
                cp = vp if cp is None else jnp.where(jnp.concatenate([sub8 == s] * (NC + 2), axis=1), vp, cp)
                cx = vx if cx is None else jnp.where(wide(sub8 == s), vx, cx)
            cand_p.append(cp[:, 0:D] * jnp.concatenate([cp[:, D:]] * (NC // 2), axis=1))
            cand_x.append(cx)
        cand_p = jnp.concatenate(cand_p, axis=0).astype(BF16)
        cand_x = jnp.concatenate(cand_x, axis=0)
        ids_lo = key_row(jnp.broadcast_to(p1, (8, LANES)))
        ids_hi = jnp.where(sub8 < 6, key_row(jnp.broadcast_to(p2_, (8, LANES))),
                           jnp.where(sub8 == 6, key_row(oldk[0]), key_row(oldk[1])))
        res["ids"] = (ids_lo, ids_hi)
        parts = []
        for c in range(NC):
            parts.append(jnp.dot(cand_p, wload(mp_v, 0, D, slice(c * LANES, (c + 1) * LANES)), preferred_element_type=F32))
            yield
        xs = _layernorm(cand_x + jnp.concatenate(parts, axis=1))
        hi = jnp.where(wide(sub8 < 6), xs[8:16, :], jnp.where(wide(sub8 == 6), oldx[0], oldx[1]))
        res["xs"] = jnp.concatenate([xs[0:8, :], hi], axis=0).astype(BF16)

    def f_units():
        xs = res["xs"]
        acts = []
        for j in range(F // LANES):
            cs = slice(j * LANES, (j + 1) * LANES)
            g = jnp.dot(gated(xs), wload(wg_v, 0, D, cs), preferred_element_type=F32)
            yield
            u = jnp.dot(xs, wload(wu_v, 0, D, cs), preferred_element_type=F32)
            acts.append((g * jax.nn.sigmoid(g) * u).astype(BF16))
            yield
        act = jnp.concatenate(acts, axis=1)
        zf = pltpu.bitcast(zero_u, F32)
        ys = []
        KF = (F // D) * D
        for c in range(0, NC, 2):
            acc = jnp.concatenate([jnp.concatenate([zf, zf], axis=0)] * 2, axis=1)
            acc = acc + jnp.dot(gated(act[:, KF:]), wload(wd_v, KF, F - KF, slice(c * LANES, (c + 2) * LANES)),
                                preferred_element_type=F32)
            yield
            for cc in range(2):
                y = acc[:, cc * LANES:(cc + 1) * LANES]
                for k0 in range(0, KF, D):
                    y = y + jnp.dot(gated(act[:, k0:k0 + D]),
                                    wload(wd_v, k0, D, slice((c + cc) * LANES, (c + cc + 1) * LANES)),
                                    preferred_element_type=F32)
                    yield
                ys.append(y)
        res["y"] = jnp.concatenate(ys, axis=1)

    def side_units():
        yield from range(NPRE)
        yield from c_units()
        yield from range(NGAP)
        yield from f_units()

    side = side_units()

    def o_dot(lhs, rhs):
        p = pc.dot(lhs, rhs) if st["step"] < NPRE else jnp.dot(lhs, rhs, preferred_element_type=F32)
        next(side, None)
        st["step"] += 1
        return p

    def o_plain(r0, n):
        lhs = pltpu.bitcast(pqn_v[r0 // 2:(r0 + n) // 2, :], BF16)
        parts = []
        for c0 in range(0, NC, 2):
            acc = x_v[DEF + L0 + r0:DEF + L0 + r0 + n, c0 * LANES:(c0 + 2) * LANES].astype(F32)
            for k0 in range(0, D, 2 * LANES):
                acc = acc + o_dot(lhs[:, k0:k0 + 2 * LANES], wload(mp_v, k0, 2 * LANES, slice(c0 * LANES, (c0 + 2) * LANES)))
            parts.append(acc)
        return jnp.concatenate(parts, axis=1)

    toks = []
    r0 = 0
    pc.add(post_jobs(OCL[0][0], *OCL[1]), pc.t + 200, pc.t + 1000, QP_DELAY)
    for ci, (n, plain) in enumerate(OCL):
        h = o_plain(r0, n) if plain else o_part(o_dot, x_v, DEF + L0, r0, n)
        last = r0 + n == RL
        units = ln2_jobs(h, ln2_v, out_v, DEF + L0 + r0, -DEF, None, st, fast=last)
        posts = post_jobs(r0 + n + OCL[ci + 1][0], *OCL[ci + 2]) if ci + 2 < len(OCL) else []
        for k, job in enumerate(units):
            toks.append(job(toks[-LAG_L] if len(toks) >= LAG_L and not last else None))
            if posts:
                posts.pop(0)(toks[-1])
        if GLAG[ci] is not None:
            st["pend"].append((st["step"] + GLAG[ci],
                               pltpu.bitcast(jnp.broadcast_to(st["top1"], (8, LANES)), U32) & zero_u))
        r0 += n
        if last or r0 in OUT_AT:
            out_copy(L0 + st["sent"], r0 - st["sent"], 2 if last else 1).start()
            if not last:
                st["sent"] = r0
    for _ in side:
        st["step"] += 1

    keyv = best2(st["top1"], st["top2"])
    idx = [jnp.clip(key_row(kk[0, 0]), 0, S - 1) for kk in keyv]
    grp = [pl.multiple_of((ii >> 3) << 3, 8) for ii in idx]
    vgrp = [pl.multiple_of(gg + DEF, 8) for gg in grp]
    y = res["y"]
    ids_lo, ids_hi = res["ids"]
    hits = None
    yrows = []
    for c in range(2):
        m_lo = ids_lo == key_row(keyv[c])
        m_hi = ids_hi == key_row(keyv[c])
        yrows.append(subsum(jnp.where(wide(m_lo), y[0:8, :], 0.0) + jnp.where(wide(m_hi), y[8:16, :], 0.0)))
        hit = submax(jnp.where(m_lo | m_hi, 1, 0))
        hits = hit if hits is None else hits + hit
    hit_all = hits[0, 0] == 2

    tail0 = L0 + st["sent"]
    tail_copy = out_copy(tail0, S - tail0, 2)
    in_tail = jnp.maximum(grp[0], grp[1]) >= tail0
    two_groups = grp[1] != grp[0]

    def fix_copy(c):
        return out_copy(grp[c], 8, 3 + c)

    def finish(ysel):
        for c in range(2):
            hi = keyv[c] & jnp.int32(-65536)
            score = pltpu.bitcast(hi ^ ((hi >> 31) & 0x7FFF0000), F32)
            sel = (key_row(keyv[c]) & 7) == sub8
            upd = jnp.where(wide(sel), ysel[c] * wide(jax.nn.sigmoid(score)), 0.0)
            out_v[pl.ds(vgrp[c], 8), :] = (out_v[pl.ds(vgrp[c], 8), :].astype(F32) + upd).astype(BF16)
        fix_copy(0).start()

        @pl.when(two_groups)
        def _():
            fix_copy(1).start()

    out_copy(0, L0, 0).wait()
    out_copy(L0, tail0 - L0, 1).wait()

    @pl.when(in_tail)
    def _():
        tail_copy.wait()

    @pl.when(hit_all)
    def _():
        finish(yrows)

    @pl.when(jnp.logical_not(hit_all))
    def _():
        xsel = jnp.concatenate([ln2_v[pl.ds(vgrp[c], 8), :] for c in range(2)], axis=0)

        def ffn_tile(j, acc):
            cs = pl.ds(pl.multiple_of(j * LANES, LANES), LANES)
            g = jnp.dot(xsel, wload(wg_v, 0, D, cs), preferred_element_type=F32)
            u = jnp.dot(xsel, wload(wu_v, 0, D, cs), preferred_element_type=F32)
            a = (g * jax.nn.sigmoid(g) * u).astype(BF16)
            return acc + jnp.dot(a, wd_v[cs, 0:D], preferred_element_type=F32)

        yf = lax.fori_loop(0, F // LANES, ffn_tile, jnp.zeros((16, D), F32))
        finish([yf[0:8, :], yf[8:16, :]])

    @pl.when(jnp.logical_not(in_tail))
    def _():
        tail_copy.wait()

    fix_copy(0).wait()

    @pl.when(two_groups)
    def _():
        fix_copy(1).wait()


@jax.jit
def pallas_sequential_preLN__linear_attn_block__moe_arch_mod__prompt_kernel(
    A_x: jax.Array,
    A_wqkv: jax.Array,
    A_wo: jax.Array,
    B_x: jax.Array,
    B_w_r: jax.Array,
    B_w_gate: jax.Array,
    B_w_up: jax.Array,
    B_w_down: jax.Array,
):
    del B_x
    x = A_x.reshape(S, D)
    wr = B_w_r.reshape(NC, LANES)
    any_spec = pl.BlockSpec(memory_space=pl.ANY)
    out = pl.pallas_call(
        _kernel,
        out_shape=jax.ShapeDtypeStruct((S, D), BF16),
        in_specs=[any_spec] * 7,
        out_specs=any_spec,
        scratch_shapes=[
            pltpu.VMEM((S + DEF, D), BF16),
            pltpu.VMEM((D, D + LANES), BF16),
            pltpu.VMEM((D, D + LANES), BF16),
            pltpu.VMEM((2, D, D + LANES), BF16),
            pltpu.VMEM((NC, LANES), BF16),
            pltpu.VMEM((2, D, F), BF16),
            pltpu.VMEM((F, D + LANES), BF16),
            pltpu.VMEM((P0 // 2, D), U32),
            pltpu.VMEM((7 ** LA, S // NA // 2, DA), U32),
            pltpu.VMEM((7 ** LA, DA // 2, DA), U32),
            pltpu.VMEM((D // 2, P0), U32),
            pltpu.VMEM((DA // 2, 7 ** LA * MA), U32),
            pltpu.VMEM((D, LANES), F32),
            pltpu.VMEM((D, LANES), F32),
            pltpu.VMEM((RL, LANES), F32),
            pltpu.VMEM((D, D), F32),
            pltpu.VMEM((7, HD, HD), F32),
            pltpu.VMEM((D // 2, D), U32),
            pltpu.VMEM((7 ** LA, DA // 2, DA), U32),
            pltpu.VMEM((D // 2, D), U32),
            pltpu.VMEM((7 ** LO, DO // 2, DO), U32),
            pltpu.VMEM((max(TB2, RL), D + 2 * LANES), F32),
            pltpu.VMEM((RL // 2, D), U32),
            pltpu.VMEM((7 ** LO, max(TB2, RL) // NO // 2, DO), U32),
            pltpu.VMEM((DEF, D), F32),
            pltpu.VMEM((2, S + DEF, D), BF16),
            pltpu.VMEM((TB, D), F32),
            pltpu.VMEM((8, LANES), U32),
            pltpu.SemaphoreType.DMA((NSEM,)),
        ],
        compiler_params=pltpu.CompilerParams(vmem_limit_bytes=110 * 1024 * 1024, disable_bounds_checks=True,
                                             disable_semaphore_checks=True),
    )(x, A_wqkv, A_wo, wr, B_w_gate, B_w_up, B_w_down)
    return out.reshape(1, S, D)
```

```python
import jax
import jax.numpy as jnp
from jax import lax
import jax.experimental.pallas as pl
import jax.experimental.pallas.tpu as pltpu


S = 2048
D = 1024
F = 3584
H = 32
DH = D // H
LANES = 128
NC = D // LANES
HD = D // 2

LA = 2
LO = 1
NA, NO = 2 ** LA, 2 ** LO
DA, DO = D // NA, D // NO
P0 = 512
PB = S - P0
TX = 256
TB = 512
NB1 = PB // TB
MA = TB // NA
TB2 = 384
NB2 = 4
QA = 192
OCH = (128, 128, 128)
DEF = OCH[-1]
L0 = NB2 * TB2
RL = S - L0
QS = (256, 256)
OCL = ((128, False), (128, False), (128, False), (64, True), (64, True))
NPRE = 22
NGAP = 9
OUT_AT = (256, 384, 448)
GM = 32
NZ = 5
WQP = 5
LNU = 8
LAG = 5
LAG_L = 6
LN_DELAY = 800
LN2_DELAY = 900
JOB_DELAY = 500
POST_DELAY = 800
QP_DELAY = 400
WK5 = 66
C6LN = (1000, 8900)
C6WK = (1500, 8900)
P1LN = (60, 10500)
P1WP = (6800, 11000)
P1WQ = (8000, 12300)
P2U = (60, 2000)
EV2 = 300
GLAG = (None, None, 26, 16, 7)

F32 = jnp.float32
BF16 = jnp.bfloat16
U32 = jnp.uint32
I32 = jnp.int32

XP = ((PB, 128), (PB + 128, 128), (PB + 256, 256), (0, TB), (TB, PB - TB))
WKP = ((0, 128), (128, 128), (256, 256), (512, 512))

SEM_X = 0
SEM_WK = SEM_X + len(XP)
SEM_WQ = SEM_WK + len(WKP)
SEM_W3 = SEM_WQ + 1
SEM_WR = SEM_W3 + 1
SEM_WGU = SEM_WR + 1
SEM_WD = SEM_WGU + 1
SEM_OUT = SEM_WD + 1
NSEM = SEM_OUT + 5

INT_MIN = -(2 ** 31)


def _layernorm(x, tok=None, w=None):
    s0 = x[:, 0:LANES]
    if tok is not None:
        s0 = s0 + jnp.concatenate([tok] * (x.shape[0] // 8), axis=0)
    for c in range(1, NC):
        s0 = s0 + x[:, c * LANES:(c + 1) * LANES]
    mu = jnp.sum(s0, axis=-1, keepdims=True) * (1.0 / D)
    xc = x - mu
    var = jnp.sum(xc * xc, axis=-1, keepdims=True) * (1.0 / D)
    rstd = lax.rsqrt(var + 1e-5)
    if w is None:
        return xc * rstd
    return xc * rstd, jnp.sum(xc * w, axis=-1, keepdims=True) * rstd


def _phi(t):
    return jnp.where(t > 0, t + 1.0, jnp.exp(t)) + 1e-6


def _n_off(a, b):
    return 32 * a + 8 * b


def _n_groups():
    pos = {(2 * o + e) * LANES + _n_off(a, b): (16 * e + 4 * b + a) * DH + 8 * o
           for o in range(4) for e in range(2) for a in range(4) for b in range(4)}
    return [pos[n] for n in sorted(pos)]


def _quads(b):
    h = len(b) // 2
    return [[r[j * h:(j + 1) * h] for r in b[i * h:(i + 1) * h]] for i in range(2) for j in range(2)]


def _badd(x, y):
    return [[a + b for a, b in zip(rx, ry)] for rx, ry in zip(x, y)]


def _bsub(x, y):
    return [[a - b for a, b in zip(rx, ry)] for rx, ry in zip(x, y)]


def _a_set(b):
    if len(b) == 1:
        return [b[0][0]]
    return [x for o in _a_ops(b) for x in _a_set(o)]


def _b_set(b):
    if len(b) == 1:
        return [b[0][0]]
    q11, q12, q21, q22 = _quads(b)
    ops = (_badd(q11, q22), q11, _bsub(q12, q22), _bsub(q21, q11), q22, _badd(q11, q12), _badd(q21, q22))
    return [x for o in ops for x in _b_set(o)]


def _b_in_a(i, levels):
    perm = (0, 2, 6, 5, 3, 4, 1)
    return sum(perm[(i // 7 ** l) % 7] * 7 ** l for l in range(levels))


def _strassen(prod, levels, base=0, fin=lambda k, q: q, init=None):
    if levels == 0:
        return [[prod(base)]]

    def m(i):
        return _strassen(prod, levels - 1, base * 7 + i)

    def seed(q, x):
        return x if init is None else _badd(_quads(init)[q], x)

    m2 = m(2)
    c22 = seed(3, m2)
    m4 = m(4)
    c12 = fin(1, _badd(seed(1, m2), m4))
    c11 = m4 if init is None else _bsub(_quads(init)[0], m4)
    m3 = m(3)
    c11 = _bsub(m3, c11) if init is None else _badd(c11, m3)
    m1 = m(1)
    c21 = fin(2, _badd(seed(2, m3), m1))
    c22 = _bsub(c22, m1)
    m0 = m(0)
    c11 = _badd(c11, m0)
    c22 = _badd(c22, m0)
    c11 = fin(0, _badd(c11, m(6)))
    c22 = fin(3, _badd(c22, m(5)))
    return [a + b for a, b in zip(c11, c12)] + [a + b for a, b in zip(c21, c22)]


def _goff(i, levels):
    return int(format(i, "0%db" % levels)[::-1], 2) if levels else 0


def _blocks(rows, n):
    w = rows[0].shape[1] // n
    return [[r[:, j * w:(j + 1) * w] for j in range(n)] for r in rows]


def _or_all(vals):
    acc = None
    for v in vals:
        v = v if v.dtype == U32 else pltpu.bitcast(v, U32)
        for g in range(v.shape[0] // 8):
            for c in range(v.shape[1] // LANES):
                p = v if v.shape == (8, LANES) else v[g * 8:(g + 1) * 8, c * LANES:(c + 1) * LANES]
                acc = p if acc is None else acc | p
    return acc


def _raw_ops(levels):
    n = 2 ** levels
    names = [[_Tag((i, j)) for j in range(n)] for i in range(n)]
    return {op: t.ij for op, t in enumerate(_b_set(names)) if t.ij is not None}


class _Tag:
    def __init__(self, ij):
        self.ij = ij

    def __add__(self, other):
        return _Tag(None)

    __sub__ = __add__


def _a_ops(b):
    q11, q12, q21, q22 = _quads(b)
    return (_badd(q11, q22), _badd(q21, q22), q11, q22, _badd(q11, q12), _bsub(q21, q11), _bsub(q12, q22))


_A_FORM = (((0, 0), (1, 1), 1), ((1, 0), (1, 1), 1), ((0, 0),), ((1, 1),), ((0, 0), (0, 1), 1),
           ((1, 0), (0, 0), -1), ((0, 1), (1, 1), -1))
_B_FORM = (((0, 0), (1, 1), 1), ((0, 0),), ((0, 1), (1, 1), -1), ((1, 0), (0, 0), -1), ((1, 1),),
           ((0, 0), (0, 1), 1), ((1, 0), (1, 1), 1))
_C_FORM = (((0, 1), (3, 1), (4, -1), (6, 1)), ((2, 1), (4, 1)), ((1, 1), (3, 1)), ((0, 1), (1, -1), (2, 1), (5, 1)))


def _outer(form, get, n):
    h = n // 2

    def quad(q):
        return [[get(q[0] * h + i, q[1] * h + j) for j in range(h)] for i in range(h)]

    if len(form) == 1:
        return quad(form[0])
    return (_badd if form[2] > 0 else _bsub)(quad(form[0]), quad(form[1]))


def _gate(v, tok):
    u = pltpu.bitcast(v, U32)
    top = u[0:8, 0:LANES] | tok
    if u.shape[1] > LANES:
        top = jnp.concatenate([top, u[0:8, LANES:]], axis=1)
    return pltpu.bitcast(jnp.concatenate([top, u[8:, :]], axis=0) if u.shape[0] > 8 else top, BF16)


class _Pacer:
    def __init__(self, zero, every=0):
        self.zero, self.t, self.jobs, self.pend, self.res, self.tok = zero, 0, [], [], None, None
        self.every, self.last = every, -every

    def add(self, jobs, t0, t1, delay):
        for k, job in enumerate(jobs):
            self.jobs.append((t0 + k * (t1 - t0) // len(jobs), len(self.jobs), job, delay))
        self.jobs.sort(key=lambda e: e[:2])

    def due(self, dep, delay):
        if dep is not None:
            self.pend.append((self.t + delay, _or_all([dep])))

    def release(self, upto):
        while self.jobs and self.jobs[0][0] <= upto:
            _, _, job, delay = self.jobs.pop(0)
            if self.res is not None:
                self.tok = pltpu.bitcast(pltpu.bitcast(self.res[0:8, 0:LANES], U32) & self.zero, F32)
                self.res = None
            self.due(job(self.tok), delay)

    def dot(self, lhs, rhs):
        self.release(self.t)
        ready = [d for t, d in self.pend if t <= self.t]
        if ready and self.t - self.last >= self.every:
            self.pend = [e for e in self.pend if e[0] > self.t]
            self.last = self.t
            lhs = _gate(lhs, _or_all(ready) & self.zero)
        res = jnp.dot(lhs, rhs, preferred_element_type=F32)
        self.t += lhs.shape[0] * (lhs.shape[1] // LANES) * (res.shape[1] // LANES) // 4
        self.res = res
        return res

    def flush(self):
        self.release(1 << 30)


def _kernel(x_hbm, wqkv_hbm, wo_hbm, wr_hbm, wg_hbm, wu_hbm, wd_hbm, out_hbm,
            x_v, wk_v, wq_v, w3_v, wr_v, wgu_v, wd_v,
            ln1_v, xs_v, wks_v, pkt_v, pks_v, zacc_v, uacc_v, xw_v, g_v, gs_v, wqp_v, wqs_v, mp_v, ms_v,
            pq_v, pqn_v, pqs_v, attn_v, lo_v, lnf_v, zero_v, sems):

    ln2_v, out_v = lo_v.at[0], lo_v.at[1]

    def wload(ref, r0, nr, cols):
        if ref.dtype == BF16:
            return ref[r0:r0 + nr, cols]
        return pltpu.bitcast(ref[r0 // 2:(r0 + nr) // 2, cols], BF16)

    wv_v, wo_v = w3_v.at[0], w3_v.at[1]
    wg_v, wu_v = wgu_v.at[0], wgu_v.at[1]

    def x_copy(i):
        r0, n = XP[i]
        return pltpu.make_async_copy(x_hbm.at[pl.ds(r0, n), :], x_v.at[pl.ds(DEF + r0, n), :], sems.at[SEM_X + i])

    def out_copy(r0, n, s):
        return pltpu.make_async_copy(out_v.at[pl.ds(DEF + r0, n), :], out_hbm.at[pl.ds(r0, n), :],
                                     sems.at[SEM_OUT + s])

    def wk_copy(j):
        c0, n = WKP[j]
        return pltpu.make_async_copy(wqkv_hbm.at[:, pl.ds(D + c0, n)], wk_v.at[:, pl.ds(c0, n)],
                                     sems.at[SEM_WK + j])

    wq_copy = pltpu.make_async_copy(wqkv_hbm.at[:, pl.ds(0, D)], wq_v, sems.at[SEM_WQ])
    wv_copy = pltpu.make_async_copy(wqkv_hbm.at[:, pl.ds(2 * D, D)], wv_v.at[:, pl.ds(0, D)], sems.at[SEM_W3])
    wo_copy = pltpu.make_async_copy(wo_hbm, wo_v.at[:, pl.ds(0, D)], sems.at[SEM_W3])
    wr_copy = pltpu.make_async_copy(wr_hbm, wr_v, sems.at[SEM_WR])
    wd_copy = pltpu.make_async_copy(wd_hbm, wd_v.at[:, pl.ds(0, D)], sems.at[SEM_WD])
    wg_copy = pltpu.make_async_copy(wg_hbm, wg_v, sems.at[SEM_WGU])
    wu_copy = pltpu.make_async_copy(wu_hbm, wu_v, sems.at[SEM_WGU])

    x_copy(0).start()
    wk_copy(0).start()
    x_copy(1).start()
    wr_copy.start()
    for j in range(1, len(WKP)):
        wk_copy(j).start()
    for j in range(2, len(XP)):
        x_copy(j).start()
    wq_copy.start()
    wv_copy.start()
    wo_copy.start()

    def ln1_rows(xr, xr0, lnr, r0, n):
        ln = _layernorm(xr[xr0:xr0 + n, :].astype(F32)).astype(BF16)
        lnr[r0 // 2:(r0 + n) // 2, :] = pltpu.bitcast(ln, U32)

    def ln1_set(pc, xr, xr0, xsr, a0, n, t0, t1):
        def unit(j):
            def job(tok):
                ln = _layernorm(xr[xr0 + j * LNU:xr0 + (j + 1) * LNU, :].astype(F32), tok)
                lnf_v[j * LNU:(j + 1) * LNU, :] = ln
                return _or_all([ln[:, 0:LANES], ln[:, D - LANES:D]])
            return job

        def piece(j0, c0, o):
            def job(tok):
                def get(i, f):
                    r = (j0 + 2 * _goff(i, LA)) * LNU
                    v = lnf_v[r:r + 16, f * DA + c0:f * DA + c0 + LANES]
                    return v + jnp.concatenate([tok, tok], axis=0) if (i + f) % (NA // 2 + 1) == 0 else v

                r = (a0 + (j0 // (2 * NA)) * 16) // 2
                ops = _a_set(_outer(_A_FORM[o], get, NA))
                for op, v in enumerate(ops):
                    xsr.at[o * len(ops) + op][r:r + 8, c0:c0 + LANES] = pltpu.bitcast(v.astype(BF16), U32)
                return _or_all([v[0:8, :] for v in [ops[0]] + ops[5:7]])
            return job

        grp = 2 * NA
        ng = n // LNU // grp
        dt = (t1 - t0 - LN_DELAY) // (ng + 1)
        for g in range(ng):
            pc.add([unit(g * grp + j) for j in range(grp)], t0 + g * dt, t0 + (g + 1) * dt, LN_DELAY)
            s = t0 + (g + 1) * dt + LN_DELAY
            pc.add([piece(g * grp, c0, o) for c0 in range(0, DA, LANES) for o in range(7)], s, s + dt, JOB_DELAY)

    def ln1_load(lnr, r0, n):
        return pltpu.bitcast(lnr[r0 // 2:(r0 + n) // 2, :], BF16)

    def k_mm(r0, n, c0, nc):
        return jnp.dot(ln1_load(ln1_v, r0, n), wload(wk_v, 0, D, slice(c0, c0 + nc)), preferred_element_type=F32)

    def z_acc(pkts, c0, first=False):
        zs = None
        for pkt in pkts:
            for j in range(pkt.shape[1] // LANES):
                p = pkt[:, j * LANES:(j + 1) * LANES]
                zs = p if zs is None else zs + p
        if first:
            zacc_v[c0:c0 + zs.shape[0], :] = zs
        else:
            zacc_v[c0:c0 + zs.shape[0], :] += zs

    def k_post(k, p0, c0, first=False):
        n, nc = k.shape
        pkt = _phi(k).T
        pkt_v[c0 // 2:(c0 + nc) // 2, p0:p0 + n] = pltpu.bitcast(pkt.astype(BF16), U32)
        z_acc([pkt], c0, first)
        return pkt[nc - 8:nc, n - LANES:n]

    def g_acc(r0, n, c0, nc, first=False, pc=None):
        h, w = (nc, D) if pc is None else (LANES, LANES)
        for f0 in range(c0, c0 + nc, h):
            for j0 in range(0, D, w):
                lhs = pltpu.bitcast(pkt_v[f0 // 2:(f0 + h) // 2, r0:r0 + n], BF16)
                rhs = pltpu.bitcast(ln1_v[r0 // 2:(r0 + n) // 2, j0:j0 + w], BF16)
                g = jnp.dot(lhs, rhs, preferred_element_type=F32) if pc is None else pc.dot(lhs, rhs)
                if first:
                    g_v[f0:f0 + h, j0:j0 + w] = g
                else:
                    g_v[f0:f0 + h, j0:j0 + w] += g

    def k_paced(pc, r0, c0, nc, first):
        for j0 in range(c0, c0 + nc, LANES):
            for t0 in range(r0, r0 + TX, LANES):
                k = None
                for k0 in range(0, D, TX):
                    p = pc.dot(ln1_load(ln1_v, t0, LANES)[:, k0:k0 + TX], wload(wk_v, k0, TX, slice(j0, j0 + LANES)))
                    k = p if k is None else k + p
                pc.due(k_post(k, t0, j0, first and t0 == r0), POST_DELAY)

    attn_v[...] = jnp.zeros_like(attn_v)
    zero_v[...] = jnp.zeros_like(zero_v)

    def gs_zero(o0, o1):
        gs_v[o0:o1] = jnp.zeros((o1 - o0, HD, HD), F32)

    x_copy(0).wait()
    ln1_rows(x_v, DEF + PB, ln1_v, 0, 128)
    gs_zero(0, 1)
    wk_copy(0).wait()
    ka = k_mm(0, 128, 0, 128)
    gs_zero(1, 2)
    x_copy(1).wait()
    wr_copy.wait()
    gs_zero(2, 3)
    ln1_rows(x_v, DEF + PB + 128, ln1_v, 128, 128)
    k_post(ka, 0, 0, first=True)
    g_acc(0, 128, 0, 128, first=True)
    wk_copy(1).wait()
    gs_zero(3, NZ)
    k_post(k_mm(128, 128, 0, 128), 128, 0)
    k_post(k_mm(0, TX, 128, 128), 0, 128, first=True)
    g_acc(128, 128, 0, 128)

    def w_job(src_ref, dst_ref, levels, r0, c0, o):
        n = 2 ** levels
        w, raw, inner = D // n, _raw_ops(levels), 7 ** (levels - 1)

        def job(tok):
            def cut(i, j):
                return wload(src_ref, i * w + r0, 16, slice(j * w + c0, j * w + c0 + LANES))

            def get(i, j):
                v = cut(i, j).astype(F32)
                return v + jnp.concatenate([tok, tok], axis=0) if (i + j) % (n // 2 + 1) == 0 else v

            ops = []
            for op, v in enumerate(_b_set(_outer(_B_FORM[o], get, n))):
                dst = dst_ref.at[o * inner + op]
                if o * inner + op in raw:
                    dst[r0 // 2:r0 // 2 + 8, c0:c0 + LANES] = pltpu.bitcast(cut(*raw[o * inner + op]), U32)
                else:
                    dst[r0 // 2:r0 // 2 + 8, c0:c0 + LANES] = pltpu.bitcast(v.astype(BF16), U32)
                    ops.append(v)
            return _or_all(ops[0:1] + ops[-2:]) if ops else None
        return job

    def wk_jobs_of(outer):
        return [w_job(wk_v, wks_v, LA, r0, c0, o) for r0 in range(0, DA, 16) for c0 in range(0, DA, LANES)
                for o in outer]

    wk_copy(2).wait()
    pc = _Pacer(zero_v[...])
    pc.add(wk_jobs_of((1, 3)), 500, 2200, JOB_DELAY)
    k_paced(pc, 0, 256, 256, True)
    g_acc(0, TX, 128, 128, True, pc)
    g_acc(0, TX, 256, 256, True, pc)
    pc.flush()
    wk_copy(3).wait()
    wk_jobs = wk_jobs_of((0, 2, 4, 5, 6))
    pc = _Pacer(zero_v[...])
    pc.add(wk_jobs[:WK5], 500, 2700, JOB_DELAY)
    k_paced(pc, 0, 512, 512, True)
    g_acc(0, TX, 512, 256, True, pc)
    pc.flush()
    x_copy(2).wait()
    x_copy(3).wait()
    pc = _Pacer(zero_v[...])
    ln1_set(pc, x_v, DEF, xs_v, 0, TB, *C6LN)
    pc.add(wk_jobs[WK5:], *C6WK, JOB_DELAY)
    ln1_rows(x_v, DEF + PB + TX, ln1_v, TX, TX)
    g_acc(0, TX, 768, 256, True, pc)
    k_paced(pc, TX, 0, D, False)
    for c0 in range(0, D, 256):
        g_acc(TX, TX, c0, 256, False, pc)
    pc.flush()

    def xs_load(xsr, op, a0, m):
        return pltpu.bitcast(xsr[op, a0 // 2:(a0 + m) // 2, :], BF16)

    def k_step(pc, xsr, j0):
        def fin(_, q):
            q = [[_phi(v).T for v in r] for r in q]
            pc.due(_or_all([v[LANES - 8:LANES, :] for r in q for v in r]), POST_DELAY)
            return q

        cb = _strassen(lambda i: pc.dot(xs_load(xsr, i, 0, MA), pltpu.bitcast(wks_v[i, :, j0:j0 + LANES], BF16)),
                       LA, fin=fin)
        outer = _a_ops([[cb[i][f] for i in range(NA)] for f in range(NA)])
        for half, o in ((0, outer[4]), (1, outer[1])):
            for f, rowb in enumerate(o):
                z_acc(rowb, half * HD + f * DA + j0)
        ops = [v for o in outer for v in _a_set(o)]
        for op, v in enumerate(ops):
            pks_v[j0 // 2:(j0 + LANES) // 2, op * MA:(op + 1) * MA] = pltpu.bitcast(v.astype(BF16), U32)
        pc.due(_or_all([v[LANES - 8:LANES, :] for v in (ops[0], ops[-1], ops[-2])]), 2 * POST_DELAY)

    def g_step(pc, xsr, r0, later):
        def old(o, f, c):
            v = gs_v[o, f * DA + r0:f * DA + r0 + GM, c * DA:(c + 1) * DA]
            return v if o < NZ else jnp.where(later, v, 0.0)

        for o in range(7):
            cb = _strassen(lambda i: pc.dot(pltpu.bitcast(pks_v[r0 // 2:(r0 + GM) // 2, i * MA:(i + 1) * MA], BF16),
                                            xs_load(xsr, _b_in_a(i, LA), 0, MA)), LA - 1, base=o,
                           init=[[old(o, f, c) for c in range(NA // 2)] for f in range(NA // 2)])
            for f in range(NA // 2):
                for c in range(NA // 2):
                    gs_v[o, f * DA + r0:f * DA + r0 + GM, c * DA:(c + 1) * DA] = cb[f][c]

    def wq_jobs(u0, nr):
        span = (NA - 1) * DA + 16 * nr
        u0 = u0 if isinstance(u0, int) else pl.multiple_of(u0, 8)
        r_first = 2 * u0 if isinstance(u0, int) else pl.multiple_of(2 * u0, 16)
        srcr, permr = wq_v.at[pl.ds(r_first, span), :], wqp_v.at[pl.ds(u0, span // 2), :]
        dstr = wqs_v.at[:, pl.ds(u0, 8 * nr), :]
        oct_ = (lax.broadcasted_iota(I32, (8, LANES), 1) % DH) // 8

        def perm(r, e):
            def job(tok):
                blk = [pltpu.bitcast(srcr[r:r + 16, (4 * e + b) * LANES:(4 * e + b + 1) * LANES], U32)
                       | pltpu.bitcast(tok, U32)
                       for b in range(4)]
                outs = []
                for o in range(4):
                    v = blk[o]
                    for b in range(4):
                        if b != o:
                            v = jnp.where(oct_ == b, pltpu.roll(blk[b], (8 * (b - o)) % LANES, 1), v)
                    permr[r // 2:r // 2 + 8, (2 * o + e) * LANES:(2 * o + e + 1) * LANES] = v
                    outs.append(v)
                return _or_all(outs)
            return job

        return ([perm(i * DA + r0, e) for r0 in range(0, 16 * nr, 16) for i in range(NA) for e in range(2)],
                [w_job(permr, dstr, LA, r0, c0, o) for r0 in range(0, 16 * nr, 16)
                 for c0 in range(0, DA, LANES) for o in range(7)])

    def p1(i, carry):
        xsr = xs_v.at[:, pl.ds(pl.multiple_of(i * (MA // 2), MA // 2), MA), :]
        xr = x_v.at[pl.ds(pl.multiple_of((i + 1) * TB, TB), TB + DEF), :]

        @pl.when(i == NB1 - 2)
        def _():
            wg_copy.start()
            wu_copy.start()
            wd_copy.start()

        pc = _Pacer(zero_v[...])
        ln1_set(pc, xr, DEF, xsr, MA, TB, *P1LN)
        perms, sets = wq_jobs(i * (8 * WQP), WQP)
        pc.add(perms, *P1WP, JOB_DELAY)
        pc.add(sets, *P1WQ, JOB_DELAY)
        for j0 in range(0, DA, LANES):
            k_step(pc, xsr, j0)
        for r0 in range(0, DA, GM):
            g_step(pc, xsr, r0, i > 0)
        pc.flush()
        return carry

    x_copy(4).wait()
    wq_copy.wait()
    lax.fori_loop(0, NB1, p1, 0)

    wv_copy.wait()
    wo_copy.wait()
    zero_u = zero_v[...]
    zrow = jnp.sum(jnp.concatenate([zacc_v[r:r + 8, :] for r in _n_groups()], axis=0).T, axis=0, keepdims=True)
    wr8 = wr_v[...].astype(F32)
    wr_row = jnp.concatenate([wr8[c:c + 1, :] for c in range(NC)], axis=1)

    row_h = lax.broadcasted_iota(I32, (LANES, LANES), 0) // DH
    col_h = lax.broadcasted_iota(I32, (LANES, LANES), 1) // DH
    diag = row_h == col_h

    def colsum(t):
        acc = t[:, 0:LANES]
        for c in range(1, NC):
            acc = acc + t[:, c * LANES:(c + 1) * LANES]
        return acc

    wrc = wr_row - jnp.sum(wr_row, axis=-1, keepdims=True) * (1.0 / D)
    m_raw = _raw_ops(LO)

    def kv_part(c):
        cs = slice(c * LANES, (c + 1) * LANES)
        kv = None
        for k0 in range(0, D, TX):
            g = g_v[cs, k0:k0 + TX]
            for o, sign in _C_FORM[(c * LANES // HD) * 2 + k0 // HD]:
                t = gs_v[o, c * LANES % HD:c * LANES % HD + LANES, k0 % HD:k0 % HD + TX]
                g = g + t if sign > 0 else g - t
            p = pc.dot(g.astype(BF16), wload(wv_v, k0, TX, cs))
            kv = p if kv is None else kv + p
        return jnp.where(diag, kv, 0.0)

    def m_part(c, kvs):
        e, b = c // 4, c % 4
        for j0 in range(0, DO, LANES):
            ms = [jnp.concatenate(
                [pc.dot(kv, wload(wo_v, (c + k) * LANES, LANES, slice(f * DO + j0, f * DO + j0 + LANES)))
                 for f in range(NO)], axis=1) for k, kv in enumerate(kvs)]
            deps = []
            for a in range(4):
                rows = [jnp.concatenate([m[a * DH + 8 * o:a * DH + 8 * o + 8, :] for m in ms], axis=0)
                        for o in range(4)]
                for o in range(4):
                    r = ((2 * o + e) * LANES + _n_off(a, b)) // 2
                    for f in range(NO):
                        mp_v[r:r + 8, f * DO + j0:f * DO + j0 + LANES] = pltpu.bitcast(
                            rows[o][:, f * LANES:(f + 1) * LANES].astype(BF16), U32)
                for t in range(4 // NO):
                    r = ((2 * t + e) * LANES + _n_off(a, b)) // 2
                    for op, v in enumerate(_b_set(_blocks(rows[t::4 // NO], NO))):
                        if op not in m_raw:
                            ms_v.at[op][r:r + 8, j0:j0 + LANES] = pltpu.bitcast(v.astype(BF16), U32)
                            deps.append(v[0:8, 0:LANES])
            pc.due(_or_all(deps[::4]), POST_DELAY)

    pc = _Pacer(zero_u)
    pc.due(jnp.broadcast_to(zrow, (8, D)), 1000)
    perms, sets = wq_jobs(NB1 * 8 * WQP, DA // 16 - NB1 * WQP)
    pc.add(perms, 60, 700, JOB_DELAY)
    pc.add(sets, 1300, 3500, JOB_DELAY)
    kv_prev = None
    for c in range(0, NC + 2, 2):
        kvs = [kv_part(c).astype(BF16), kv_part(c + 1).astype(BF16)] if c < NC else None
        if c:
            m_part(c - 2, kv_prev)
        kv_prev = kvs
    pc.flush()

    def make_key(score, row):
        b = pltpu.bitcast(score, I32)
        srt = b ^ ((b >> 31) & 0x7FFFFFFF)
        return (srt & jnp.int32(-65536)) | (0xFFFF - row)

    def push_keys(key, top1, top2):
        for gidx in range(key.shape[0] // 8):
            kx = key[gidx * 8:(gidx + 1) * 8, :]
            top2 = jnp.maximum(top2, jnp.minimum(top1, kx))
            top1 = jnp.maximum(top1, kx)
        return top1, top2

    lane = lax.broadcasted_iota(I32, (1, LANES), 1)

    def interleave(parts):
        return jnp.concatenate([p[g * 16:(g + 1) * 16, :] for g in range(parts[0].shape[0] // 16) for p in parts],
                               axis=0)

    def q_part(pc, xsr, l0, r0, n, hint=None):
        m = n // NA
        sums = {}

        def park(v, g, c):
            for t in range(m // 16):
                r = r0 + (t * NA + g) * 16
                pq_v[r:r + 16, c * LANES:(c + 1) * LANES] = v[t * 16:(t + 1) * 16, :]

        def fin(k, q):
            q = [[_phi(v) for v in r] for r in q]
            deps = []
            for a, r in enumerate(q):
                for b, v in enumerate(r):
                    i, c = (k // 2) * (NA // 2) + a, (((k % 2) * (NA // 2) + b) * DA + j0) // LANES
                    park(v, _goff(i, LA), c)
                    for name, row in (("z", zrow),) + ((("u", hint["u"]),) if hint else ()):
                        t = v * row[:, c * LANES:(c + 1) * LANES]
                        key = (name, _goff(i, LA), c % 2)
                        sums[key] = t if key not in sums else sums[key] + t
                deps.append(sums[key])
            if hint:
                pc.due(_or_all(deps), POST_DELAY)
            return q

        for j0 in range(0, DA, LANES):
            _strassen(lambda i: pc.dot(xs_load(xsr, i, (l0 + r0) // NA, m),
                                       pltpu.bitcast(wqs_v[i, :, j0:j0 + LANES], BF16)), LA, fin=fin)
        if hint:
            pc.flush()
        den = jnp.concatenate([sums["z", g, e] for g in range(NA) for e in range(2)], axis=0)
        for s in (1, 2, 4):
            den = den + jnp.where((lane & s) == 0, pltpu.roll(den, LANES - s, 1), pltpu.roll(den, s, 1))
        inv_all = 1.0 / (den + 1e-6)

        def inv_of(g):
            return [inv_all[(g * 2 + e) * m:(g * 2 + e + 1) * m, :] for e in range(2)]

        for g in range(NA):
            for e in range(2):
                park(inv_of(g)[e], g, NC + e)
        if hint:
            for g in range(NA):
                starts = [r0 + (t * NA + g) * 16 for t in range(m // 16)]
                num = jnp.sum(jnp.concatenate([xw_v[t:t + 16, :] for t in starts], axis=0)
                              + sums["u", g, 0] * inv_of(g)[0] + sums["u", g, 1] * inv_of(g)[1],
                              axis=-1, keepdims=True)
                row = jnp.concatenate([(l0 + t) + lax.broadcasted_iota(I32, (16, 1), 0) for t in starts], axis=0)
                hint["p1"], hint["p2"] = push_keys(make_key(num, row), hint["p1"], hint["p2"])
            pc.due(jnp.broadcast_to(hint["p1"], (8, LANES)), 1200)


    def post_jobs(r0, n, plain=False):
        def scaled(t, c0, w, tok):
            inv = pq_v[t:t + 16, D:D + 2 * LANES]
            if tok is not None:
                inv = inv + jnp.concatenate([jnp.concatenate([tok, tok], axis=0)] * 2, axis=1)
            return pq_v[t:t + 16, c0:c0 + w] * jnp.concatenate([inv] * (w // (2 * LANES)), axis=1)

        def post_plain(t):
            def job(tok):
                v = scaled(t, 0, D, tok)
                pqn_v[t // 2:t // 2 + 8, :] = pltpu.bitcast(v.astype(BF16), U32)
                return v[0:8, 0:LANES]
            return job

        def post(t0, outer):
            def job(tok):
                deps = []
                for c0 in range(0, DO, 2 * LANES):
                    blk = {}

                    def get(i, f):
                        if (i, f) not in blk:
                            blk[i, f] = scaled(t0 + _goff(i, LO) * 16, f * DO + c0, 2 * LANES, tok)
                        return blk[i, f]

                    for o in outer:
                        ops = _a_set(_outer(_A_FORM[o], get, NO))
                        for op, v in enumerate(ops):
                            pqs_v.at[o * len(ops) + op][t0 // NO // 2:t0 // NO // 2 + 8, c0:c0 + 2 * LANES] = (
                                pltpu.bitcast(v.astype(BF16), U32))
                        deps.append(ops[0][0:8, 0:LANES])
                return _or_all(deps)
            return job

        if plain:
            return [post_plain(t) for t in range(r0, r0 + n, 16)]
        outers = [range(7)] if LO == 1 else [(o,) for o in range(7)]
        return [post(t0, outer) for t0 in range(r0, r0 + n, 16 * NO) for outer in outers]

    def m_operand(i, c0, c1):
        if i not in m_raw:
            return pltpu.bitcast(ms_v[i, :, c0 * LANES:c1 * LANES], BF16)
        bi, bj = m_raw[i]
        return wload(mp_v, bi * DO, DO, slice(bj * DO + c0 * LANES, bj * DO + c1 * LANES))

    def o_part(dot, xr, x0, r0, n):
        a0, m = r0 // NO, n // NO
        nw = LANES * NO // 2
        cols = [[[] for _ in range(NO)] for _ in range(NO)]
        for c0 in range(0, DO, nw):
            init = [[jnp.concatenate(
                [xr[x0 + r0 + (g * NO + _goff(i, LO)) * 16:x0 + r0 + (g * NO + _goff(i, LO) + 1) * 16,
                    f * DO + c0:f * DO + c0 + nw] for g in range(m // 16)], axis=0).astype(F32)
                for f in range(NO)] for i in range(NO)]
            cb = _strassen(lambda i: dot(pltpu.bitcast(pqs_v[i, a0 // 2:(a0 + m) // 2, :], BF16),
                                         m_operand(i, c0 // LANES, (c0 + nw) // LANES)), LO, init=init)
            for i in range(NO):
                for f in range(NO):
                    cols[i][f].append(cb[i][f])
        parts = [None] * NO
        for i in range(NO):
            parts[_goff(i, LO)] = jnp.concatenate([c for f in range(NO) for c in cols[i][f]], axis=1)
        return interleave(parts)

    def ln2_unit(h, l2r, outr, r0, row0, valid, top1, top2, tok, fast=False):
        n = h.shape[0]
        if fast:
            ln2, r = _layernorm(h, tok, wr_row)
        else:
            ln2 = _layernorm(h, tok)
            r = jnp.sum(ln2 * wr_row, axis=-1, keepdims=True)
        l2r[r0:r0 + n, :] = ln2.astype(BF16)
        res = h + ln2
        outr[r0:r0 + n, :] = res.astype(BF16)
        r = r.astype(BF16).astype(F32) + 0.0
        key = make_key(r, (row0 + r0) + lax.broadcasted_iota(I32, (n, 1), 0))
        if valid is not None:
            key = jnp.where(valid, key, INT_MIN)
        top1, top2 = push_keys(key, top1, top2)
        ntok = pltpu.bitcast(pltpu.bitcast(jnp.broadcast_to(r[n - 8:n, :], (8, LANES)), U32) & zero_u, F32)
        return top1, top2, ntok

    def ln2_jobs(h, l2r, outr, r0, row0, valid, st, fast=False):
        def unit(j):
            def job(tok):
                st["top1"], st["top2"], dep = ln2_unit(h[j * LNU:(j + 1) * LNU, :], l2r, outr, r0 + j * LNU, row0,
                                                       valid, st["top1"], st["top2"], tok, fast)
                return dep
            return job
        return [unit(j) for j in range(h.shape[0] // LNU)]

    QC = 16 * 7 ** LA / 8 ** LA

    def p2(i, carry):
        st = dict(top1=carry[0], top2=carry[1])
        b0 = pl.multiple_of(i * TB2, 16)
        xsr = xs_v.at[:, pl.ds(pl.multiple_of(i * (TB2 // NA // 2), 8), TB2 // NA // 2), :]
        xr = x_v.at[pl.ds(b0, TB2 + DEF), :]
        l2r = ln2_v.at[pl.ds(b0, TB2 + DEF), :]
        outr = out_v.at[pl.ds(b0, TB2 + DEF), :]
        row0 = b0 - DEF
        pc = _Pacer(zero_u)
        toks = []

        def chain(jobs):
            for job in jobs:
                toks.append(job(toks[-LAG] if len(toks) >= LAG else None))

        chain(ln2_jobs(attn_v, l2r, outr, 0, row0, i > 0, st))

        @pl.when(i > 0)
        def _():
            out_copy(pl.multiple_of((i - 1) * TB2, 16), TB2, 0).start()

        pc.due(toks[-1], QA * QC)

        nu, nx = D // NB2, RL // NB2
        mr = mp_v.at[pl.ds(pl.multiple_of(i * (nu // 2), 8), nu // 2), :]
        ur = uacc_v.at[pl.ds(pl.multiple_of(i * nu, 8), nu), :]
        xl = x_v.at[pl.ds(pl.multiple_of(DEF + L0 + i * nx, 16), nx), :]
        xwr = xw_v.at[pl.ds(pl.multiple_of(i * nx, 8), nx), :]

        def hint_job(load, dst, r):
            def job(tok):
                v = colsum(load(r).astype(F32) * wrc) + jnp.concatenate([tok, tok], axis=0)
                dst[r:r + 16, :] = v
                return v
            return job

        pc.add([hint_job(lambda r: wload(mr, r, 16, slice(None)), ur, r) for r in range(0, nu, 16)]
               + [hint_job(lambda r: xl[r:r + 16, :], xwr, r) for r in range(0, nx, 16)], *P2U, JOB_DELAY)
        for r0, n in ((0, QA), (QA, TB2 - QA)):
            q_part(pc, xsr, 0, r0, n)
            for job in post_jobs(r0, n):
                job(None)
        r0 = 0
        for n in OCH[:-1]:
            chain(ln2_jobs(o_part(pc.dot, xr, DEF, r0, n), l2r, outr, DEF + r0, row0, None, st))
            r0 += n
        attn_v[...] = o_part(pc.dot, xr, DEF, r0, DEF)
        return st["top1"], st["top2"]

    init = jnp.full((8, 1), INT_MIN, I32)
    top1, top2 = lax.fori_loop(0, NB2, p2, (init, init))

    wg_copy.wait()
    wu_copy.wait()
    wd_copy.wait()
    sub8 = lax.broadcasted_iota(I32, (8, LANES), 0)
    urow = jnp.sum(uacc_v[...].T, axis=0, keepdims=True)

    def submax(v):
        for sh in (4, 2, 1):
            v = jnp.maximum(v, pltpu.roll(v, sh, 0))
        return v

    def subsum(v):
        for sh in (4, 2, 1):
            v = v + pltpu.roll(v, sh, 0)
        return v

    def best2(t1, t2):
        t1 = jnp.broadcast_to(t1, (8, LANES))
        t2 = jnp.broadcast_to(t2, (8, LANES))
        k1v = submax(t1)
        return k1v, submax(jnp.where(t1 == k1v, t2, t1))

    def key_row(k):
        return 0xFFFF - (k & 0xFFFF)

    def wide(m):
        return jnp.concatenate([m] * NC, axis=1)

    st = dict(top1=top1, top2=top2, pend=[], step=0, sent=0)
    pc = _Pacer(zero_u, EV2)
    hint = dict(u=urow, p1=init, p2=init)

    pc.add(ln2_jobs(attn_v, ln2_v, out_v, L0, -DEF, None, st), 60, QS[0] * QC - 600, LN2_DELAY)
    r0 = 0
    for k, n in enumerate(QS):
        q_part(pc, xs_v, L0, r0, n, hint)
        if k == 0:
            out_copy(L0 - TB2, TB2, 0).start()
            top1, top2 = st["top1"], st["top2"]
            pc.add(post_jobs(0, OCL[0][0], OCL[0][1]), pc.t + 600, pc.t + (RL - n) * QC - 300, QP_DELAY)
        r0 += n
    pc.every = 0
    oldk = best2(top1, top2)
    oldx = []
    for kk in oldk:
        g8 = pl.multiple_of(((jnp.clip(key_row(kk[0, 0]), 0, S - 1) >> 3) << 3) + DEF, 8)
        rows = ln2_v[pl.ds(g8, 8), :].astype(F32)
        oldx.append(subsum(jnp.where(wide((key_row(kk) & 7) == sub8), rows, 0.0)))

    def gated(v):
        tok = None
        while st["pend"] and st["pend"][0][0] <= st["step"]:
            t = st["pend"].pop(0)[1]
            tok = t if tok is None else tok | t
        if tok is None:
            return v
        u = pltpu.bitcast(v, U32)
        return pltpu.bitcast(jnp.concatenate([u[:, 0:LANES] | tok, u[:, LANES:]], axis=1), BF16)

    res = {}

    def c_units():
        pc.flush()
        p1, p2_ = hint["p1"], hint["p2"]
        cand_p, cand_x = [], []
        for pk_ in (p1, p2_):
            cp, cx = None, None
            for s in range(8):
                g8 = pl.multiple_of((jnp.clip(key_row(pk_[s, 0]) - L0, 0, RL - 1) >> 3) << 3, 8)
                vp = pq_v[pl.ds(g8, 8), :]
                vx = x_v[pl.ds(pl.multiple_of(g8 + (L0 + DEF), 8), 8), :].astype(F32)
                cp = vp if cp is None else jnp.where(jnp.concatenate([sub8 == s] * (NC + 2), axis=1), vp, cp)
                cx = vx if cx is None else jnp.where(wide(sub8 == s), vx, cx)
            cand_p.append(cp[:, 0:D] * jnp.concatenate([cp[:, D:]] * (NC // 2), axis=1))
            cand_x.append(cx)
        cand_p = jnp.concatenate(cand_p, axis=0).astype(BF16)
        cand_x = jnp.concatenate(cand_x, axis=0)
        ids_lo = key_row(jnp.broadcast_to(p1, (8, LANES)))
        ids_hi = jnp.where(sub8 < 6, key_row(jnp.broadcast_to(p2_, (8, LANES))),
                           jnp.where(sub8 == 6, key_row(oldk[0]), key_row(oldk[1])))
        res["ids"] = (ids_lo, ids_hi)
        parts = []
        for c in range(NC):
            parts.append(jnp.dot(cand_p, wload(mp_v, 0, D, slice(c * LANES, (c + 1) * LANES)), preferred_element_type=F32))
            yield
        xs = _layernorm(cand_x + jnp.concatenate(parts, axis=1))
        hi = jnp.where(wide(sub8 < 6), xs[8:16, :], jnp.where(wide(sub8 == 6), oldx[0], oldx[1]))
        res["xs"] = jnp.concatenate([xs[0:8, :], hi], axis=0).astype(BF16)

    def f_units():
        xs = res["xs"]
        acts = []
        for j in range(F // LANES):
            cs = slice(j * LANES, (j + 1) * LANES)
            g = jnp.dot(gated(xs), wload(wg_v, 0, D, cs), preferred_element_type=F32)
            yield
            u = jnp.dot(xs, wload(wu_v, 0, D, cs), preferred_element_type=F32)
            acts.append((g * jax.nn.sigmoid(g) * u).astype(BF16))
            yield
        act = jnp.concatenate(acts, axis=1)
        zf = pltpu.bitcast(zero_u, F32)
        ys = []
        KF = (F // D) * D
        for c in range(0, NC, 2):
            acc = jnp.concatenate([jnp.concatenate([zf, zf], axis=0)] * 2, axis=1)
            acc = acc + jnp.dot(gated(act[:, KF:]), wload(wd_v, KF, F - KF, slice(c * LANES, (c + 2) * LANES)),
                                preferred_element_type=F32)
            yield
            for cc in range(2):
                y = acc[:, cc * LANES:(cc + 1) * LANES]
                for k0 in range(0, KF, D):
                    y = y + jnp.dot(gated(act[:, k0:k0 + D]),
                                    wload(wd_v, k0, D, slice((c + cc) * LANES, (c + cc + 1) * LANES)),
                                    preferred_element_type=F32)
                    yield
                ys.append(y)
        res["y"] = jnp.concatenate(ys, axis=1)

    def side_units():
        yield from range(NPRE)
        yield from c_units()
        yield from range(NGAP)
        yield from f_units()

    side = side_units()

    def o_dot(lhs, rhs):
        p = pc.dot(lhs, rhs) if st["step"] < NPRE else jnp.dot(lhs, rhs, preferred_element_type=F32)
        next(side, None)
        st["step"] += 1
        return p

    def o_plain(r0, n):
        lhs = pltpu.bitcast(pqn_v[r0 // 2:(r0 + n) // 2, :], BF16)
        parts = []
        for c0 in range(0, NC, 2):
            acc = x_v[DEF + L0 + r0:DEF + L0 + r0 + n, c0 * LANES:(c0 + 2) * LANES].astype(F32)
            for k0 in range(0, D, 2 * LANES):
                acc = acc + o_dot(lhs[:, k0:k0 + 2 * LANES], wload(mp_v, k0, 2 * LANES, slice(c0 * LANES, (c0 + 2) * LANES)))
            parts.append(acc)
        return jnp.concatenate(parts, axis=1)

    toks = []
    r0 = 0
    pc.add(post_jobs(OCL[0][0], *OCL[1]), pc.t + 200, pc.t + 1000, QP_DELAY)
    for ci, (n, plain) in enumerate(OCL):
        h = o_plain(r0, n) if plain else o_part(o_dot, x_v, DEF + L0, r0, n)
        last = r0 + n == RL
        units = ln2_jobs(h, ln2_v, out_v, DEF + L0 + r0, -DEF, None, st, fast=last)
        posts = post_jobs(r0 + n + OCL[ci + 1][0], *OCL[ci + 2]) if ci + 2 < len(OCL) else []
        for k, job in enumerate(units):
            toks.append(job(toks[-LAG_L] if len(toks) >= LAG_L and not last else None))
            if posts:
                posts.pop(0)(toks[-1])
        if GLAG[ci] is not None:
            st["pend"].append((st["step"] + GLAG[ci],
                               pltpu.bitcast(jnp.broadcast_to(st["top1"], (8, LANES)), U32) & zero_u))
        r0 += n
        if last or r0 in OUT_AT:
            out_copy(L0 + st["sent"], r0 - st["sent"], 2 if last else 1).start()
            if not last:
                st["sent"] = r0
    for _ in side:
        st["step"] += 1

    keyv = best2(st["top1"], st["top2"])
    idx = [jnp.clip(key_row(kk[0, 0]), 0, S - 1) for kk in keyv]
    grp = [pl.multiple_of((ii >> 3) << 3, 8) for ii in idx]
    vgrp = [pl.multiple_of(gg + DEF, 8) for gg in grp]
    y = res["y"]
    ids_lo, ids_hi = res["ids"]
    hits = None
    yrows = []
    for c in range(2):
        m_lo = ids_lo == key_row(keyv[c])
        m_hi = ids_hi == key_row(keyv[c])
        yrows.append(subsum(jnp.where(wide(m_lo), y[0:8, :], 0.0) + jnp.where(wide(m_hi), y[8:16, :], 0.0)))
        hit = submax(jnp.where(m_lo | m_hi, 1, 0))
        hits = hit if hits is None else hits + hit
    hit_all = hits[0, 0] == 2

    tail0 = L0 + st["sent"]
    tail_copy = out_copy(tail0, S - tail0, 2)
    in_tail = jnp.maximum(grp[0], grp[1]) >= tail0
    two_groups = grp[1] != grp[0]

    def fix_copy(c):
        return out_copy(grp[c], 8, 3 + c)

    def finish(ysel):
        for c in range(2):
            hi = keyv[c] & jnp.int32(-65536)
            score = pltpu.bitcast(hi ^ ((hi >> 31) & 0x7FFF0000), F32)
            sel = (key_row(keyv[c]) & 7) == sub8
            upd = jnp.where(wide(sel), ysel[c] * wide(jax.nn.sigmoid(score)), 0.0)
            out_v[pl.ds(vgrp[c], 8), :] = (out_v[pl.ds(vgrp[c], 8), :].astype(F32) + upd).astype(BF16)
        fix_copy(0).start()

        @pl.when(two_groups)
        def _():
            fix_copy(1).start()

    out_copy(0, L0, 0).wait()
    out_copy(L0, tail0 - L0, 1).wait()

    @pl.when(in_tail)
    def _():
        tail_copy.wait()

    @pl.when(hit_all)
    def _():
        finish(yrows)

    @pl.when(jnp.logical_not(hit_all))
    def _():
        xsel = jnp.concatenate([ln2_v[pl.ds(vgrp[c], 8), :] for c in range(2)], axis=0)

        def ffn_tile(j, acc):
            cs = pl.ds(pl.multiple_of(j * LANES, LANES), LANES)
            g = jnp.dot(xsel, wload(wg_v, 0, D, cs), preferred_element_type=F32)
            u = jnp.dot(xsel, wload(wu_v, 0, D, cs), preferred_element_type=F32)
            a = (g * jax.nn.sigmoid(g) * u).astype(BF16)
            return acc + jnp.dot(a, wd_v[cs, 0:D], preferred_element_type=F32)

        yf = lax.fori_loop(0, F // LANES, ffn_tile, jnp.zeros((16, D), F32))
        finish([yf[0:8, :], yf[8:16, :]])

    @pl.when(jnp.logical_not(in_tail))
    def _():
        tail_copy.wait()

    fix_copy(0).wait()

    @pl.when(two_groups)
    def _():
        fix_copy(1).wait()


@jax.jit
def pallas_sequential_preLN__linear_attn_block__moe_arch_mod__prompt_kernel(
    A_x: jax.Array,
    A_wqkv: jax.Array,
    A_wo: jax.Array,
    B_x: jax.Array,
    B_w_r: jax.Array,
    B_w_gate: jax.Array,
    B_w_up: jax.Array,
    B_w_down: jax.Array,
):
    del B_x
    x = A_x.reshape(S, D)
    wr = B_w_r.reshape(NC, LANES)
    any_spec = pl.BlockSpec(memory_space=pl.ANY)
    out = pl.pallas_call(
        _kernel,
        out_shape=jax.ShapeDtypeStruct((S, D), BF16),
        in_specs=[any_spec] * 7,
        out_specs=any_spec,
        scratch_shapes=[
            pltpu.VMEM((S + DEF, D), BF16),
            pltpu.VMEM((D, D + LANES), BF16),
            pltpu.VMEM((D, D), BF16),
            pltpu.VMEM((2, D, D + LANES), BF16),
            pltpu.VMEM((NC, LANES), BF16),
            pltpu.VMEM((2, D, F), BF16),
            pltpu.VMEM((F, D + LANES), BF16),
            pltpu.VMEM((P0 // 2, D), U32),
            pltpu.VMEM((7 ** LA, S // NA // 2, DA), U32),
            pltpu.VMEM((7 ** LA, DA // 2, DA), U32),
            pltpu.VMEM((D // 2, P0), U32),
            pltpu.VMEM((DA // 2, 7 ** LA * MA), U32),
            pltpu.VMEM((D, LANES), F32),
            pltpu.VMEM((D, LANES), F32),
            pltpu.VMEM((RL, LANES), F32),
            pltpu.VMEM((D, D), F32),
            pltpu.VMEM((7, HD, HD), F32),
            pltpu.VMEM((D // 2, D), U32),
            pltpu.VMEM((7 ** LA, DA // 2, DA), U32),
            pltpu.VMEM((D // 2, D), U32),
            pltpu.VMEM((7 ** LO, DO // 2, DO), U32),
            pltpu.VMEM((max(TB2, RL), D + 2 * LANES), F32),
            pltpu.VMEM((RL // 2, D), U32),
            pltpu.VMEM((7 ** LO, max(TB2, RL) // NO // 2, DO), U32),
            pltpu.VMEM((DEF, D), F32),
            pltpu.VMEM((2, S + DEF, D), BF16),
            pltpu.VMEM((TB, D), F32),
            pltpu.VMEM((8, LANES), U32),
            pltpu.SemaphoreType.DMA((NSEM,)),
        ],
        compiler_params=pltpu.CompilerParams(vmem_limit_bytes=110 * 1024 * 1024, disable_bounds_checks=True,
                                             disable_semaphore_checks=True),
    )(x, A_wqkv, A_wo, wr, B_w_gate, B_w_up, B_w_down)
    return out.reshape(1, S, D)
```

```python
import jax
import jax.numpy as jnp
from jax import lax
import jax.experimental.pallas as pl
import jax.experimental.pallas.tpu as pltpu


S = 2048
D = 1024
F = 3584
H = 32
DH = D // H
LANES = 128
NC = D // LANES
HD = D // 2

LA = 2
LO = 1
NA, NO = 2 ** LA, 2 ** LO
DA, DO = D // NA, D // NO
P0 = 512
PB = S - P0
TX = 256
TB = 512
NB1 = PB // TB
MA = TB // NA
TB2 = 384
NB2 = 4
QA = 192
OCH = (128, 128, 128)
DEF = OCH[-1]
L0 = NB2 * TB2
RL = S - L0
QS = (256, 256)
OCL = ((128, False), (128, False), (128, False), (64, True), (64, True))
NPRE = 22
NGAP = 9
OUT_AT = (256, 384, 448)
GM = 64
GN = 128
NZ = 5
WQP = 5
LNU = 8
LAG = 5
LAG_L = 6
LN_DELAY = 800
LN2_DELAY = 900
JOB_DELAY = 500
POST_DELAY = 800
QP_DELAY = 400
WK5 = 66
C6LN = (1000, 8900)
C6WK = (1500, 8900)
P1LN = (60, 10500)
P1WP = (6800, 11000)
P1WQ = (8000, 12300)
P2U = (60, 2000)
EV2 = 300
GLAG = (None, None, 26, 16, 7)

F32 = jnp.float32
BF16 = jnp.bfloat16
U32 = jnp.uint32
I32 = jnp.int32

XP = ((PB, 128), (PB + 128, 128), (PB + 256, 256), (0, TB), (TB, PB - TB))
WKP = ((0, 128), (128, 128), (256, 256), (512, 512))

SEM_X = 0
SEM_WK = SEM_X + len(XP)
SEM_WQ = SEM_WK + len(WKP)
SEM_W3 = SEM_WQ + 1
SEM_WR = SEM_W3 + 1
SEM_WGU = SEM_WR + 1
SEM_WD = SEM_WGU + 1
SEM_OUT = SEM_WD + 1
NSEM = SEM_OUT + 5

INT_MIN = -(2 ** 31)


def _layernorm(x, tok=None, w=None):
    s0 = x[:, 0:LANES]
    if tok is not None:
        s0 = s0 + jnp.concatenate([tok] * (x.shape[0] // 8), axis=0)
    for c in range(1, NC):
        s0 = s0 + x[:, c * LANES:(c + 1) * LANES]
    mu = jnp.sum(s0, axis=-1, keepdims=True) * (1.0 / D)
    xc = x - mu
    var = jnp.sum(xc * xc, axis=-1, keepdims=True) * (1.0 / D)
    rstd = lax.rsqrt(var + 1e-5)
    if w is None:
        return xc * rstd
    return xc * rstd, jnp.sum(xc * w, axis=-1, keepdims=True) * rstd


def _phi(t):
    return jnp.where(t > 0, t + 1.0, jnp.exp(t)) + 1e-6


def _n_off(a, b):
    return 32 * a + 8 * b


def _n_groups():
    pos = {(2 * o + e) * LANES + _n_off(a, b): (16 * e + 4 * b + a) * DH + 8 * o
           for o in range(4) for e in range(2) for a in range(4) for b in range(4)}
    return [pos[n] for n in sorted(pos)]


def _quads(b):
    h = len(b) // 2
    return [[r[j * h:(j + 1) * h] for r in b[i * h:(i + 1) * h]] for i in range(2) for j in range(2)]


def _badd(x, y):
    return [[a + b for a, b in zip(rx, ry)] for rx, ry in zip(x, y)]


def _bsub(x, y):
    return [[a - b for a, b in zip(rx, ry)] for rx, ry in zip(x, y)]


def _a_set(b):
    if len(b) == 1:
        return [b[0][0]]
    return [x for o in _a_ops(b) for x in _a_set(o)]


def _b_set(b):
    if len(b) == 1:
        return [b[0][0]]
    q11, q12, q21, q22 = _quads(b)
    ops = (_badd(q11, q22), q11, _bsub(q12, q22), _bsub(q21, q11), q22, _badd(q11, q12), _badd(q21, q22))
    return [x for o in ops for x in _b_set(o)]


def _b_in_a(i, levels):
    perm = (0, 2, 6, 5, 3, 4, 1)
    return sum(perm[(i // 7 ** l) % 7] * 7 ** l for l in range(levels))


def _strassen(prod, levels, base=0, fin=lambda k, q: q, init=None):
    if levels == 0:
        return [[prod(base)]]

    def m(i):
        return _strassen(prod, levels - 1, base * 7 + i)

    def seed(q, x):
        return x if init is None else _badd(_quads(init)[q], x)

    m2 = m(2)
    c22 = seed(3, m2)
    m4 = m(4)
    c12 = fin(1, _badd(seed(1, m2), m4))
    c11 = m4 if init is None else _bsub(_quads(init)[0], m4)
    m3 = m(3)
    c11 = _bsub(m3, c11) if init is None else _badd(c11, m3)
    m1 = m(1)
    c21 = fin(2, _badd(seed(2, m3), m1))
    c22 = _bsub(c22, m1)
    m0 = m(0)
    c11 = _badd(c11, m0)
    c22 = _badd(c22, m0)
    c11 = fin(0, _badd(c11, m(6)))
    c22 = fin(3, _badd(c22, m(5)))
    return [a + b for a, b in zip(c11, c12)] + [a + b for a, b in zip(c21, c22)]


def _goff(i, levels):
    return int(format(i, "0%db" % levels)[::-1], 2) if levels else 0


def _blocks(rows, n):
    w = rows[0].shape[1] // n
    return [[r[:, j * w:(j + 1) * w] for j in range(n)] for r in rows]


def _or_all(vals):
    acc = None
    for v in vals:
        v = v if v.dtype == U32 else pltpu.bitcast(v, U32)
        for g in range(v.shape[0] // 8):
            for c in range(v.shape[1] // LANES):
                p = v if v.shape == (8, LANES) else v[g * 8:(g + 1) * 8, c * LANES:(c + 1) * LANES]
                acc = p if acc is None else acc | p
    return acc


def _raw_ops(levels):
    n = 2 ** levels
    names = [[_Tag((i, j)) for j in range(n)] for i in range(n)]
    return {op: t.ij for op, t in enumerate(_b_set(names)) if t.ij is not None}


class _Tag:
    def __init__(self, ij):
        self.ij = ij

    def __add__(self, other):
        return _Tag(None)

    __sub__ = __add__


def _a_ops(b):
    q11, q12, q21, q22 = _quads(b)
    return (_badd(q11, q22), _badd(q21, q22), q11, q22, _badd(q11, q12), _bsub(q21, q11), _bsub(q12, q22))


_A_FORM = (((0, 0), (1, 1), 1), ((1, 0), (1, 1), 1), ((0, 0),), ((1, 1),), ((0, 0), (0, 1), 1),
           ((1, 0), (0, 0), -1), ((0, 1), (1, 1), -1))
_B_FORM = (((0, 0), (1, 1), 1), ((0, 0),), ((0, 1), (1, 1), -1), ((1, 0), (0, 0), -1), ((1, 1),),
           ((0, 0), (0, 1), 1), ((1, 0), (1, 1), 1))
_C_FORM = (((0, 1), (3, 1), (4, -1), (6, 1)), ((2, 1), (4, 1)), ((1, 1), (3, 1)), ((0, 1), (1, -1), (2, 1), (5, 1)))


def _outer(form, get, n):
    h = n // 2

    def quad(q):
        return [[get(q[0] * h + i, q[1] * h + j) for j in range(h)] for i in range(h)]

    if len(form) == 1:
        return quad(form[0])
    return (_badd if form[2] > 0 else _bsub)(quad(form[0]), quad(form[1]))


def _gate(v, tok):
    u = pltpu.bitcast(v, U32)
    top = u[0:8, 0:LANES] | tok
    if u.shape[1] > LANES:
        top = jnp.concatenate([top, u[0:8, LANES:]], axis=1)
    return pltpu.bitcast(jnp.concatenate([top, u[8:, :]], axis=0) if u.shape[0] > 8 else top, BF16)


class _Pacer:
    def __init__(self, zero, every=0):
        self.zero, self.t, self.jobs, self.pend, self.res, self.tok = zero, 0, [], [], None, None
        self.every, self.last = every, -every

    def add(self, jobs, t0, t1, delay):
        for k, job in enumerate(jobs):
            self.jobs.append((t0 + k * (t1 - t0) // len(jobs), len(self.jobs), job, delay))
        self.jobs.sort(key=lambda e: e[:2])

    def due(self, dep, delay):
        if dep is not None:
            self.pend.append((self.t + delay, _or_all([dep])))

    def release(self, upto):
        while self.jobs and self.jobs[0][0] <= upto:
            _, _, job, delay = self.jobs.pop(0)
            if self.res is not None:
                self.tok = pltpu.bitcast(pltpu.bitcast(self.res[0:8, 0:LANES], U32) & self.zero, F32)
                self.res = None
            self.due(job(self.tok), delay)

    def dot(self, lhs, rhs):
        self.release(self.t)
        ready = [d for t, d in self.pend if t <= self.t]
        if ready and self.t - self.last >= self.every:
            self.pend = [e for e in self.pend if e[0] > self.t]
            self.last = self.t
            lhs = _gate(lhs, _or_all(ready) & self.zero)
        res = jnp.dot(lhs, rhs, preferred_element_type=F32)
        self.t += lhs.shape[0] * (lhs.shape[1] // LANES) * (res.shape[1] // LANES) // 4
        self.res = res
        return res

    def flush(self):
        self.release(1 << 30)


def _kernel(x_hbm, wqkv_hbm, wo_hbm, wr_hbm, wg_hbm, wu_hbm, wd_hbm, out_hbm,
            x_v, wk_v, wq_v, w3_v, wr_v, wgu_v, wd_v,
            ln1_v, xs_v, wks_v, pkt_v, pks_v, zacc_v, uacc_v, xw_v, g_v, gs_v, wqp_v, wqs_v, mp_v, ms_v,
            pq_v, pqn_v, pqs_v, attn_v, lo_v, lnf_v, zero_v, sems):

    ln2_v, out_v = lo_v.at[0], lo_v.at[1]

    def wload(ref, r0, nr, cols):
        if ref.dtype == BF16:
            return ref[r0:r0 + nr, cols]
        return pltpu.bitcast(ref[r0 // 2:(r0 + nr) // 2, cols], BF16)

    wv_v, wo_v = w3_v.at[0], w3_v.at[1]
    wg_v, wu_v = wgu_v.at[0], wgu_v.at[1]

    def x_copy(i):
        r0, n = XP[i]
        return pltpu.make_async_copy(x_hbm.at[pl.ds(r0, n), :], x_v.at[pl.ds(DEF + r0, n), :], sems.at[SEM_X + i])

    def out_copy(r0, n, s):
        return pltpu.make_async_copy(out_v.at[pl.ds(DEF + r0, n), :], out_hbm.at[pl.ds(r0, n), :],
                                     sems.at[SEM_OUT + s])

    def wk_copy(j):
        c0, n = WKP[j]
        return pltpu.make_async_copy(wqkv_hbm.at[:, pl.ds(D + c0, n)], wk_v.at[:, pl.ds(c0, n)],
                                     sems.at[SEM_WK + j])

    wq_copy = pltpu.make_async_copy(wqkv_hbm.at[:, pl.ds(0, D)], wq_v, sems.at[SEM_WQ])
    wv_copy = pltpu.make_async_copy(wqkv_hbm.at[:, pl.ds(2 * D, D)], wv_v.at[:, pl.ds(0, D)], sems.at[SEM_W3])
    wo_copy = pltpu.make_async_copy(wo_hbm, wo_v.at[:, pl.ds(0, D)], sems.at[SEM_W3])
    wr_copy = pltpu.make_async_copy(wr_hbm, wr_v, sems.at[SEM_WR])
    wd_copy = pltpu.make_async_copy(wd_hbm, wd_v.at[:, pl.ds(0, D)], sems.at[SEM_WD])
    wg_copy = pltpu.make_async_copy(wg_hbm, wg_v, sems.at[SEM_WGU])
    wu_copy = pltpu.make_async_copy(wu_hbm, wu_v, sems.at[SEM_WGU])

    x_copy(0).start()
    wk_copy(0).start()
    x_copy(1).start()
    wr_copy.start()
    for j in range(1, len(WKP)):
        wk_copy(j).start()
    for j in range(2, len(XP)):
        x_copy(j).start()
    wq_copy.start()
    wv_copy.start()
    wo_copy.start()

    def ln1_rows(xr, xr0, lnr, r0, n):
        ln = _layernorm(xr[xr0:xr0 + n, :].astype(F32)).astype(BF16)
        lnr[r0 // 2:(r0 + n) // 2, :] = pltpu.bitcast(ln, U32)

    def ln1_set(pc, xr, xr0, xsr, a0, n, t0, t1):
        def unit(j):
            def job(tok):
                ln = _layernorm(xr[xr0 + j * LNU:xr0 + (j + 1) * LNU, :].astype(F32), tok)
                lnf_v[j * LNU:(j + 1) * LNU, :] = ln
                return _or_all([ln[:, 0:LANES], ln[:, D - LANES:D]])
            return job

        def piece(j0, c0, o):
            def job(tok):
                def get(i, f):
                    r = (j0 + 2 * _goff(i, LA)) * LNU
                    v = lnf_v[r:r + 16, f * DA + c0:f * DA + c0 + LANES]
                    return v + jnp.concatenate([tok, tok], axis=0) if (i + f) % (NA // 2 + 1) == 0 else v

                r = (a0 + (j0 // (2 * NA)) * 16) // 2
                ops = _a_set(_outer(_A_FORM[o], get, NA))
                for op, v in enumerate(ops):
                    xsr.at[o * len(ops) + op][r:r + 8, c0:c0 + LANES] = pltpu.bitcast(v.astype(BF16), U32)
                return _or_all([v[0:8, :] for v in [ops[0]] + ops[5:7]])
            return job

        grp = 2 * NA
        ng = n // LNU // grp
        dt = (t1 - t0 - LN_DELAY) // (ng + 1)
        for g in range(ng):
            pc.add([unit(g * grp + j) for j in range(grp)], t0 + g * dt, t0 + (g + 1) * dt, LN_DELAY)
            s = t0 + (g + 1) * dt + LN_DELAY
            pc.add([piece(g * grp, c0, o) for c0 in range(0, DA, LANES) for o in range(7)], s, s + dt, JOB_DELAY)

    def ln1_load(lnr, r0, n):
        return pltpu.bitcast(lnr[r0 // 2:(r0 + n) // 2, :], BF16)

    def k_mm(r0, n, c0, nc):
        return jnp.dot(ln1_load(ln1_v, r0, n), wload(wk_v, 0, D, slice(c0, c0 + nc)), preferred_element_type=F32)

    def z_acc(pkts, c0, first=False):
        zs = None
        for pkt in pkts:
            for j in range(pkt.shape[1] // LANES):
                p = pkt[:, j * LANES:(j + 1) * LANES]
                zs = p if zs is None else zs + p
        if first:
            zacc_v[c0:c0 + zs.shape[0], :] = zs
        else:
            zacc_v[c0:c0 + zs.shape[0], :] += zs

    def k_post(k, p0, c0, first=False):
        n, nc = k.shape
        pkt = _phi(k).T
        pkt_v[c0 // 2:(c0 + nc) // 2, p0:p0 + n] = pltpu.bitcast(pkt.astype(BF16), U32)
        z_acc([pkt], c0, first)
        return pkt[nc - 8:nc, n - LANES:n]

    def g_acc(r0, n, c0, nc, first=False, pc=None):
        h, w = (nc, D) if pc is None else (LANES, LANES)
        for f0 in range(c0, c0 + nc, h):
            for j0 in range(0, D, w):
                lhs = pltpu.bitcast(pkt_v[f0 // 2:(f0 + h) // 2, r0:r0 + n], BF16)
                rhs = pltpu.bitcast(ln1_v[r0 // 2:(r0 + n) // 2, j0:j0 + w], BF16)
                g = jnp.dot(lhs, rhs, preferred_element_type=F32) if pc is None else pc.dot(lhs, rhs)
                if first:
                    g_v[f0:f0 + h, j0:j0 + w] = g
                else:
                    g_v[f0:f0 + h, j0:j0 + w] += g

    def k_paced(pc, r0, c0, nc, first):
        for j0 in range(c0, c0 + nc, LANES):
            for t0 in range(r0, r0 + TX, LANES):
                k = None
                for k0 in range(0, D, TX):
                    p = pc.dot(ln1_load(ln1_v, t0, LANES)[:, k0:k0 + TX], wload(wk_v, k0, TX, slice(j0, j0 + LANES)))
                    k = p if k is None else k + p
                pc.due(k_post(k, t0, j0, first and t0 == r0), POST_DELAY)

    attn_v[...] = jnp.zeros_like(attn_v)
    zero_v[...] = jnp.zeros_like(zero_v)

    def gs_zero(o0, o1):
        gs_v[o0:o1] = jnp.zeros((o1 - o0, HD, HD), F32)

    x_copy(0).wait()
    ln1_rows(x_v, DEF + PB, ln1_v, 0, 128)
    gs_zero(0, 1)
    wk_copy(0).wait()
    ka = k_mm(0, 128, 0, 128)
    gs_zero(1, 2)
    x_copy(1).wait()
    wr_copy.wait()
    gs_zero(2, 3)
    ln1_rows(x_v, DEF + PB + 128, ln1_v, 128, 128)
    k_post(ka, 0, 0, first=True)
    g_acc(0, 128, 0, 128, first=True)
    wk_copy(1).wait()
    gs_zero(3, NZ)
    k_post(k_mm(128, 128, 0, 128), 128, 0)
    k_post(k_mm(0, TX, 128, 128), 0, 128, first=True)
    g_acc(128, 128, 0, 128)

    def w_job(src_ref, dst_ref, levels, r0, c0, o):
        n = 2 ** levels
        w, raw, inner = D // n, _raw_ops(levels), 7 ** (levels - 1)

        def job(tok):
            def cut(i, j):
                return wload(src_ref, i * w + r0, 16, slice(j * w + c0, j * w + c0 + LANES))

            def get(i, j):
                v = cut(i, j).astype(F32)
                return v + jnp.concatenate([tok, tok], axis=0) if (i + j) % (n // 2 + 1) == 0 else v

            ops = []
            for op, v in enumerate(_b_set(_outer(_B_FORM[o], get, n))):
                dst = dst_ref.at[o * inner + op]
                if o * inner + op in raw:
                    dst[r0 // 2:r0 // 2 + 8, c0:c0 + LANES] = pltpu.bitcast(cut(*raw[o * inner + op]), U32)
                else:
                    dst[r0 // 2:r0 // 2 + 8, c0:c0 + LANES] = pltpu.bitcast(v.astype(BF16), U32)
                    ops.append(v)
            return _or_all(ops[0:1] + ops[-2:]) if ops else None
        return job

    def wk_jobs_of(outer):
        return [w_job(wk_v, wks_v, LA, r0, c0, o) for r0 in range(0, DA, 16) for c0 in range(0, DA, LANES)
                for o in outer]

    wk_copy(2).wait()
    pc = _Pacer(zero_v[...])
    pc.add(wk_jobs_of((1, 3)), 500, 2200, JOB_DELAY)
    k_paced(pc, 0, 256, 256, True)
    g_acc(0, TX, 128, 128, True, pc)
    g_acc(0, TX, 256, 256, True, pc)
    pc.flush()
    wk_copy(3).wait()
    wk_jobs = wk_jobs_of((0, 2, 4, 5, 6))
    pc = _Pacer(zero_v[...])
    pc.add(wk_jobs[:WK5], 500, 2700, JOB_DELAY)
    k_paced(pc, 0, 512, 512, True)
    g_acc(0, TX, 512, 256, True, pc)
    pc.flush()
    x_copy(2).wait()
    x_copy(3).wait()
    pc = _Pacer(zero_v[...])
    ln1_set(pc, x_v, DEF, xs_v, 0, TB, *C6LN)
    pc.add(wk_jobs[WK5:], *C6WK, JOB_DELAY)
    ln1_rows(x_v, DEF + PB + TX, ln1_v, TX, TX)
    g_acc(0, TX, 768, 256, True, pc)
    k_paced(pc, TX, 0, D, False)
    for c0 in range(0, D, 256):
        g_acc(TX, TX, c0, 256, False, pc)
    pc.flush()

    def xs_load(xsr, op, a0, m):
        return pltpu.bitcast(xsr[op, a0 // 2:(a0 + m) // 2, :], BF16)

    def k_step(pc, xsr, j0):
        def fin(_, q):
            q = [[_phi(v).T for v in r] for r in q]
            pc.due(_or_all([v[LANES - 8:LANES, :] for r in q for v in r]), POST_DELAY)
            return q

        cb = _strassen(lambda i: pc.dot(xs_load(xsr, i, 0, MA), pltpu.bitcast(wks_v[i, :, j0:j0 + LANES], BF16)),
                       LA, fin=fin)
        outer = _a_ops([[cb[i][f] for i in range(NA)] for f in range(NA)])
        for half, o in ((0, outer[4]), (1, outer[1])):
            for f, rowb in enumerate(o):
                z_acc(rowb, half * HD + f * DA + j0)
        ops = [v for o in outer for v in _a_set(o)]
        for op, v in enumerate(ops):
            pks_v[j0 // 2:(j0 + LANES) // 2, op * MA:(op + 1) * MA] = pltpu.bitcast(v.astype(BF16), U32)
        pc.due(_or_all([v[LANES - 8:LANES, :] for v in (ops[0], ops[-1], ops[-2])]), 2 * POST_DELAY)

    def g_step(pc, xsr, r0, c0, later):
        def old(o, f, c):
            v = gs_v[o, f * DA + r0:f * DA + r0 + GM, c * DA + c0:c * DA + c0 + GN]
            return v if o < NZ else jnp.where(later, v, 0.0)

        for o in range(7):
            cb = _strassen(lambda i: pc.dot(pltpu.bitcast(pks_v[r0 // 2:(r0 + GM) // 2, i * MA:(i + 1) * MA], BF16),
                                            xs_load(xsr, _b_in_a(i, LA), 0, MA)[:, c0:c0 + GN]), LA - 1, base=o,
                           init=[[old(o, f, c) for c in range(NA // 2)] for f in range(NA // 2)])
            for f in range(NA // 2):
                for c in range(NA // 2):
                    gs_v[o, f * DA + r0:f * DA + r0 + GM, c * DA + c0:c * DA + c0 + GN] = cb[f][c]

    def wq_jobs(u0, nr):
        span = (NA - 1) * DA + 16 * nr
        u0 = u0 if isinstance(u0, int) else pl.multiple_of(u0, 8)
        r_first = 2 * u0 if isinstance(u0, int) else pl.multiple_of(2 * u0, 16)
        srcr, permr = wq_v.at[pl.ds(r_first, span), :], wqp_v.at[pl.ds(u0, span // 2), :]
        dstr = wqs_v.at[:, pl.ds(u0, 8 * nr), :]
        oct_ = (lax.broadcasted_iota(I32, (8, LANES), 1) % DH) // 8

        def perm(r, e):
            def job(tok):
                blk = [pltpu.bitcast(srcr[r:r + 16, (4 * e + b) * LANES:(4 * e + b + 1) * LANES], U32)
                       | pltpu.bitcast(tok, U32)
                       for b in range(4)]
                outs = []
                for o in range(4):
                    v = blk[o]
                    for b in range(4):
                        if b != o:
                            v = jnp.where(oct_ == b, pltpu.roll(blk[b], (8 * (b - o)) % LANES, 1), v)
                    permr[r // 2:r // 2 + 8, (2 * o + e) * LANES:(2 * o + e + 1) * LANES] = v
                    outs.append(v)
                return _or_all(outs)
            return job

        return ([perm(i * DA + r0, e) for r0 in range(0, 16 * nr, 16) for i in range(NA) for e in range(2)],
                [w_job(permr, dstr, LA, r0, c0, o) for r0 in range(0, 16 * nr, 16)
                 for c0 in range(0, DA, LANES) for o in range(7)])

    def p1(i, carry):
        xsr = xs_v.at[:, pl.ds(pl.multiple_of(i * (MA // 2), MA // 2), MA), :]
        xr = x_v.at[pl.ds(pl.multiple_of((i + 1) * TB, TB), TB + DEF), :]

        @pl.when(i == NB1 - 2)
        def _():
            wg_copy.start()
            wu_copy.start()
            wd_copy.start()

        pc = _Pacer(zero_v[...])
        ln1_set(pc, xr, DEF, xsr, MA, TB, *P1LN)
        perms, sets = wq_jobs(i * (8 * WQP), WQP)
        pc.add(perms, *P1WP, JOB_DELAY)
        pc.add(sets, *P1WQ, JOB_DELAY)
        for j0 in range(0, DA, LANES):
            k_step(pc, xsr, j0)
        for r0 in range(0, DA, GM):
            for c0 in range(0, DA, GN):
                g_step(pc, xsr, r0, c0, i > 0)
        pc.flush()
        return carry

    x_copy(4).wait()
    wq_copy.wait()
    lax.fori_loop(0, NB1, p1, 0)

    wv_copy.wait()
    wo_copy.wait()
    zero_u = zero_v[...]
    zrow = jnp.sum(jnp.concatenate([zacc_v[r:r + 8, :] for r in _n_groups()], axis=0).T, axis=0, keepdims=True)
    wr8 = wr_v[...].astype(F32)
    wr_row = jnp.concatenate([wr8[c:c + 1, :] for c in range(NC)], axis=1)

    row_h = lax.broadcasted_iota(I32, (LANES, LANES), 0) // DH
    col_h = lax.broadcasted_iota(I32, (LANES, LANES), 1) // DH
    diag = row_h == col_h

    def colsum(t):
        acc = t[:, 0:LANES]
        for c in range(1, NC):
            acc = acc + t[:, c * LANES:(c + 1) * LANES]
        return acc

    wrc = wr_row - jnp.sum(wr_row, axis=-1, keepdims=True) * (1.0 / D)
    m_raw = _raw_ops(LO)

    def kv_part(c):
        cs = slice(c * LANES, (c + 1) * LANES)
        kv = None
        for k0 in range(0, D, TX):
            g = g_v[cs, k0:k0 + TX]
            for o, sign in _C_FORM[(c * LANES // HD) * 2 + k0 // HD]:
                t = gs_v[o, c * LANES % HD:c * LANES % HD + LANES, k0 % HD:k0 % HD + TX]
                g = g + t if sign > 0 else g - t
            p = pc.dot(g.astype(BF16), wload(wv_v, k0, TX, cs))
            kv = p if kv is None else kv + p
        return jnp.where(diag, kv, 0.0)

    def m_part(c, kvs):
        e, b = c // 4, c % 4
        for j0 in range(0, DO, LANES):
            ms = [jnp.concatenate(
                [pc.dot(kv, wload(wo_v, (c + k) * LANES, LANES, slice(f * DO + j0, f * DO + j0 + LANES)))
                 for f in range(NO)], axis=1) for k, kv in enumerate(kvs)]
            deps = []
            for a in range(4):
                rows = [jnp.concatenate([m[a * DH + 8 * o:a * DH + 8 * o + 8, :] for m in ms], axis=0)
                        for o in range(4)]
                for o in range(4):
                    r = ((2 * o + e) * LANES + _n_off(a, b)) // 2
                    for f in range(NO):
                        mp_v[r:r + 8, f * DO + j0:f * DO + j0 + LANES] = pltpu.bitcast(
                            rows[o][:, f * LANES:(f + 1) * LANES].astype(BF16), U32)
                for t in range(4 // NO):
                    r = ((2 * t + e) * LANES + _n_off(a, b)) // 2
                    for op, v in enumerate(_b_set(_blocks(rows[t::4 // NO], NO))):
                        if op not in m_raw:
                            ms_v.at[op][r:r + 8, j0:j0 + LANES] = pltpu.bitcast(v.astype(BF16), U32)
                            deps.append(v[0:8, 0:LANES])
            pc.due(_or_all(deps[::4]), POST_DELAY)

    pc = _Pacer(zero_u)
    pc.due(jnp.broadcast_to(zrow, (8, D)), 1000)
    perms, sets = wq_jobs(NB1 * 8 * WQP, DA // 16 - NB1 * WQP)
    pc.add(perms, 60, 700, JOB_DELAY)
    pc.add(sets, 1300, 3500, JOB_DELAY)
    kv_prev = None
    for c in range(0, NC + 2, 2):
        kvs = [kv_part(c).astype(BF16), kv_part(c + 1).astype(BF16)] if c < NC else None
        if c:
            m_part(c - 2, kv_prev)
        kv_prev = kvs
    pc.flush()

    def make_key(score, row):
        b = pltpu.bitcast(score, I32)
        srt = b ^ ((b >> 31) & 0x7FFFFFFF)
        return (srt & jnp.int32(-65536)) | (0xFFFF - row)

    def push_keys(key, top1, top2):
        for gidx in range(key.shape[0] // 8):
            kx = key[gidx * 8:(gidx + 1) * 8, :]
            top2 = jnp.maximum(top2, jnp.minimum(top1, kx))
            top1 = jnp.maximum(top1, kx)
        return top1, top2

    lane = lax.broadcasted_iota(I32, (1, LANES), 1)

    def interleave(parts):
        return jnp.concatenate([p[g * 16:(g + 1) * 16, :] for g in range(parts[0].shape[0] // 16) for p in parts],
                               axis=0)

    def q_part(pc, xsr, l0, r0, n, hint=None):
        m = n // NA
        sums = {}

        def park(v, g, c):
            for t in range(m // 16):
                r = r0 + (t * NA + g) * 16
                pq_v[r:r + 16, c * LANES:(c + 1) * LANES] = v[t * 16:(t + 1) * 16, :]

        def fin(k, q):
            q = [[_phi(v) for v in r] for r in q]
            deps = []
            for a, r in enumerate(q):
                for b, v in enumerate(r):
                    i, c = (k // 2) * (NA // 2) + a, (((k % 2) * (NA // 2) + b) * DA + j0) // LANES
                    park(v, _goff(i, LA), c)
                    for name, row in (("z", zrow),) + ((("u", hint["u"]),) if hint else ()):
                        t = v * row[:, c * LANES:(c + 1) * LANES]
                        key = (name, _goff(i, LA), c % 2)
                        sums[key] = t if key not in sums else sums[key] + t
                deps.append(sums[key])
            if hint:
                pc.due(_or_all(deps), POST_DELAY)
            return q

        for j0 in range(0, DA, LANES):
            _strassen(lambda i: pc.dot(xs_load(xsr, i, (l0 + r0) // NA, m),
                                       pltpu.bitcast(wqs_v[i, :, j0:j0 + LANES], BF16)), LA, fin=fin)
        if hint:
            pc.flush()
        den = jnp.concatenate([sums["z", g, e] for g in range(NA) for e in range(2)], axis=0)
        for s in (1, 2, 4):
            den = den + jnp.where((lane & s) == 0, pltpu.roll(den, LANES - s, 1), pltpu.roll(den, s, 1))
        inv_all = 1.0 / (den + 1e-6)

        def inv_of(g):
            return [inv_all[(g * 2 + e) * m:(g * 2 + e + 1) * m, :] for e in range(2)]

        for g in range(NA):
            for e in range(2):
                park(inv_of(g)[e], g, NC + e)
        if hint:
            for g in range(NA):
                starts = [r0 + (t * NA + g) * 16 for t in range(m // 16)]
                num = jnp.sum(jnp.concatenate([xw_v[t:t + 16, :] for t in starts], axis=0)
                              + sums["u", g, 0] * inv_of(g)[0] + sums["u", g, 1] * inv_of(g)[1],
                              axis=-1, keepdims=True)
                row = jnp.concatenate([(l0 + t) + lax.broadcasted_iota(I32, (16, 1), 0) for t in starts], axis=0)
                hint["p1"], hint["p2"] = push_keys(make_key(num, row), hint["p1"], hint["p2"])
            pc.due(jnp.broadcast_to(hint["p1"], (8, LANES)), 1200)


    def post_jobs(r0, n, plain=False):
        def scaled(t, c0, w, tok):
            inv = pq_v[t:t + 16, D:D + 2 * LANES]
            if tok is not None:
                inv = inv + jnp.concatenate([jnp.concatenate([tok, tok], axis=0)] * 2, axis=1)
            return pq_v[t:t + 16, c0:c0 + w] * jnp.concatenate([inv] * (w // (2 * LANES)), axis=1)

        def post_plain(t):
            def job(tok):
                v = scaled(t, 0, D, tok)
                pqn_v[t // 2:t // 2 + 8, :] = pltpu.bitcast(v.astype(BF16), U32)
                return v[0:8, 0:LANES]
            return job

        def post(t0, outer):
            def job(tok):
                deps = []
                for c0 in range(0, DO, 2 * LANES):
                    blk = {}

                    def get(i, f):
                        if (i, f) not in blk:
                            blk[i, f] = scaled(t0 + _goff(i, LO) * 16, f * DO + c0, 2 * LANES, tok)
                        return blk[i, f]

                    for o in outer:
                        ops = _a_set(_outer(_A_FORM[o], get, NO))
                        for op, v in enumerate(ops):
                            pqs_v.at[o * len(ops) + op][t0 // NO // 2:t0 // NO // 2 + 8, c0:c0 + 2 * LANES] = (
                                pltpu.bitcast(v.astype(BF16), U32))
                        deps.append(ops[0][0:8, 0:LANES])
                return _or_all(deps)
            return job

        if plain:
            return [post_plain(t) for t in range(r0, r0 + n, 16)]
        outers = [range(7)] if LO == 1 else [(o,) for o in range(7)]
        return [post(t0, outer) for t0 in range(r0, r0 + n, 16 * NO) for outer in outers]

    def m_operand(i, c0, c1):
        if i not in m_raw:
            return pltpu.bitcast(ms_v[i, :, c0 * LANES:c1 * LANES], BF16)
        bi, bj = m_raw[i]
        return wload(mp_v, bi * DO, DO, slice(bj * DO + c0 * LANES, bj * DO + c1 * LANES))

    def o_part(dot, xr, x0, r0, n):
        a0, m = r0 // NO, n // NO
        nw = LANES * NO // 2
        cols = [[[] for _ in range(NO)] for _ in range(NO)]
        for c0 in range(0, DO, nw):
            init = [[jnp.concatenate(
                [xr[x0 + r0 + (g * NO + _goff(i, LO)) * 16:x0 + r0 + (g * NO + _goff(i, LO) + 1) * 16,
                    f * DO + c0:f * DO + c0 + nw] for g in range(m // 16)], axis=0).astype(F32)
                for f in range(NO)] for i in range(NO)]
            cb = _strassen(lambda i: dot(pltpu.bitcast(pqs_v[i, a0 // 2:(a0 + m) // 2, :], BF16),
                                         m_operand(i, c0 // LANES, (c0 + nw) // LANES)), LO, init=init)
            for i in range(NO):
                for f in range(NO):
                    cols[i][f].append(cb[i][f])
        parts = [None] * NO
        for i in range(NO):
            parts[_goff(i, LO)] = jnp.concatenate([c for f in range(NO) for c in cols[i][f]], axis=1)
        return interleave(parts)

    def ln2_unit(h, l2r, outr, r0, row0, valid, top1, top2, tok, fast=False):
        n = h.shape[0]
        if fast:
            ln2, r = _layernorm(h, tok, wr_row)
        else:
            ln2 = _layernorm(h, tok)
            r = jnp.sum(ln2 * wr_row, axis=-1, keepdims=True)
        l2r[r0:r0 + n, :] = ln2.astype(BF16)
        res = h + ln2
        outr[r0:r0 + n, :] = res.astype(BF16)
        r = r.astype(BF16).astype(F32) + 0.0
        key = make_key(r, (row0 + r0) + lax.broadcasted_iota(I32, (n, 1), 0))
        if valid is not None:
            key = jnp.where(valid, key, INT_MIN)
        top1, top2 = push_keys(key, top1, top2)
        ntok = pltpu.bitcast(pltpu.bitcast(jnp.broadcast_to(r[n - 8:n, :], (8, LANES)), U32) & zero_u, F32)
        return top1, top2, ntok

    def ln2_jobs(h, l2r, outr, r0, row0, valid, st, fast=False):
        def unit(j):
            def job(tok):
                st["top1"], st["top2"], dep = ln2_unit(h[j * LNU:(j + 1) * LNU, :], l2r, outr, r0 + j * LNU, row0,
                                                       valid, st["top1"], st["top2"], tok, fast)
                return dep
            return job
        return [unit(j) for j in range(h.shape[0] // LNU)]

    QC = 16 * 7 ** LA / 8 ** LA

    def p2(i, carry):
        st = dict(top1=carry[0], top2=carry[1])
        b0 = pl.multiple_of(i * TB2, 16)
        xsr = xs_v.at[:, pl.ds(pl.multiple_of(i * (TB2 // NA // 2), 8), TB2 // NA // 2), :]
        xr = x_v.at[pl.ds(b0, TB2 + DEF), :]
        l2r = ln2_v.at[pl.ds(b0, TB2 + DEF), :]
        outr = out_v.at[pl.ds(b0, TB2 + DEF), :]
        row0 = b0 - DEF
        pc = _Pacer(zero_u)
        toks = []

        def chain(jobs):
            for job in jobs:
                toks.append(job(toks[-LAG] if len(toks) >= LAG else None))

        chain(ln2_jobs(attn_v, l2r, outr, 0, row0, i > 0, st))

        @pl.when(i > 0)
        def _():
            out_copy(pl.multiple_of((i - 1) * TB2, 16), TB2, 0).start()

        pc.due(toks[-1], QA * QC)

        nu, nx = D // NB2, RL // NB2
        mr = mp_v.at[pl.ds(pl.multiple_of(i * (nu // 2), 8), nu // 2), :]
        ur = uacc_v.at[pl.ds(pl.multiple_of(i * nu, 8), nu), :]
        xl = x_v.at[pl.ds(pl.multiple_of(DEF + L0 + i * nx, 16), nx), :]
        xwr = xw_v.at[pl.ds(pl.multiple_of(i * nx, 8), nx), :]

        def hint_job(load, dst, r):
            def job(tok):
                v = colsum(load(r).astype(F32) * wrc) + jnp.concatenate([tok, tok], axis=0)
                dst[r:r + 16, :] = v
                return v
            return job

        pc.add([hint_job(lambda r: wload(mr, r, 16, slice(None)), ur, r) for r in range(0, nu, 16)]
               + [hint_job(lambda r: xl[r:r + 16, :], xwr, r) for r in range(0, nx, 16)], *P2U, JOB_DELAY)
        for r0, n in ((0, QA), (QA, TB2 - QA)):
            q_part(pc, xsr, 0, r0, n)
            for job in post_jobs(r0, n):
                job(None)
        r0 = 0
        for n in OCH[:-1]:
            chain(ln2_jobs(o_part(pc.dot, xr, DEF, r0, n), l2r, outr, DEF + r0, row0, None, st))
            r0 += n
        attn_v[...] = o_part(pc.dot, xr, DEF, r0, DEF)
        return st["top1"], st["top2"]

    init = jnp.full((8, 1), INT_MIN, I32)
    top1, top2 = lax.fori_loop(0, NB2, p2, (init, init))

    wg_copy.wait()
    wu_copy.wait()
    wd_copy.wait()
    sub8 = lax.broadcasted_iota(I32, (8, LANES), 0)
    urow = jnp.sum(uacc_v[...].T, axis=0, keepdims=True)

    def submax(v):
        for sh in (4, 2, 1):
            v = jnp.maximum(v, pltpu.roll(v, sh, 0))
        return v

    def subsum(v):
        for sh in (4, 2, 1):
            v = v + pltpu.roll(v, sh, 0)
        return v

    def best2(t1, t2):
        t1 = jnp.broadcast_to(t1, (8, LANES))
        t2 = jnp.broadcast_to(t2, (8, LANES))
        k1v = submax(t1)
        return k1v, submax(jnp.where(t1 == k1v, t2, t1))

    def key_row(k):
        return 0xFFFF - (k & 0xFFFF)

    def wide(m):
        return jnp.concatenate([m] * NC, axis=1)

    st = dict(top1=top1, top2=top2, pend=[], step=0, sent=0)
    pc = _Pacer(zero_u, EV2)
    hint = dict(u=urow, p1=init, p2=init)

    pc.add(ln2_jobs(attn_v, ln2_v, out_v, L0, -DEF, None, st), 60, QS[0] * QC - 600, LN2_DELAY)
    r0 = 0
    for k, n in enumerate(QS):
        q_part(pc, xs_v, L0, r0, n, hint)
        if k == 0:
            out_copy(L0 - TB2, TB2, 0).start()
            top1, top2 = st["top1"], st["top2"]
            pc.add(post_jobs(0, OCL[0][0], OCL[0][1]), pc.t + 600, pc.t + (RL - n) * QC - 300, QP_DELAY)
        r0 += n
    pc.every = 0
    oldk = best2(top1, top2)
    oldx = []
    for kk in oldk:
        g8 = pl.multiple_of(((jnp.clip(key_row(kk[0, 0]), 0, S - 1) >> 3) << 3) + DEF, 8)
        rows = ln2_v[pl.ds(g8, 8), :].astype(F32)
        oldx.append(subsum(jnp.where(wide((key_row(kk) & 7) == sub8), rows, 0.0)))

    def gated(v):
        tok = None
        while st["pend"] and st["pend"][0][0] <= st["step"]:
            t = st["pend"].pop(0)[1]
            tok = t if tok is None else tok | t
        if tok is None:
            return v
        u = pltpu.bitcast(v, U32)
        return pltpu.bitcast(jnp.concatenate([u[:, 0:LANES] | tok, u[:, LANES:]], axis=1), BF16)

    res = {}

    def c_units():
        pc.flush()
        p1, p2_ = hint["p1"], hint["p2"]
        cand_p, cand_x = [], []
        for pk_ in (p1, p2_):
            cp, cx = None, None
            for s in range(8):
                g8 = pl.multiple_of((jnp.clip(key_row(pk_[s, 0]) - L0, 0, RL - 1) >> 3) << 3, 8)
                vp = pq_v[pl.ds(g8, 8), :]
                vx = x_v[pl.ds(pl.multiple_of(g8 + (L0 + DEF), 8), 8), :].astype(F32)
                cp = vp if cp is None else jnp.where(jnp.concatenate([sub8 == s] * (NC + 2), axis=1), vp, cp)
                cx = vx if cx is None else jnp.where(wide(sub8 == s), vx, cx)
            cand_p.append(cp[:, 0:D] * jnp.concatenate([cp[:, D:]] * (NC // 2), axis=1))
            cand_x.append(cx)
        cand_p = jnp.concatenate(cand_p, axis=0).astype(BF16)
        cand_x = jnp.concatenate(cand_x, axis=0)
        ids_lo = key_row(jnp.broadcast_to(p1, (8, LANES)))
        ids_hi = jnp.where(sub8 < 6, key_row(jnp.broadcast_to(p2_, (8, LANES))),
                           jnp.where(sub8 == 6, key_row(oldk[0]), key_row(oldk[1])))
        res["ids"] = (ids_lo, ids_hi)
        parts = []
        for c in range(NC):
            parts.append(jnp.dot(cand_p, wload(mp_v, 0, D, slice(c * LANES, (c + 1) * LANES)), preferred_element_type=F32))
            yield
        xs = _layernorm(cand_x + jnp.concatenate(parts, axis=1))
        hi = jnp.where(wide(sub8 < 6), xs[8:16, :], jnp.where(wide(sub8 == 6), oldx[0], oldx[1]))
        res["xs"] = jnp.concatenate([xs[0:8, :], hi], axis=0).astype(BF16)

    def f_units():
        xs = res["xs"]
        acts = []
        for j in range(F // LANES):
            cs = slice(j * LANES, (j + 1) * LANES)
            g = jnp.dot(gated(xs), wload(wg_v, 0, D, cs), preferred_element_type=F32)
            yield
            u = jnp.dot(xs, wload(wu_v, 0, D, cs), preferred_element_type=F32)
            acts.append((g * jax.nn.sigmoid(g) * u).astype(BF16))
            yield
        act = jnp.concatenate(acts, axis=1)
        zf = pltpu.bitcast(zero_u, F32)
        ys = []
        KF = (F // D) * D
        for c in range(0, NC, 2):
            acc = jnp.concatenate([jnp.concatenate([zf, zf], axis=0)] * 2, axis=1)
            acc = acc + jnp.dot(gated(act[:, KF:]), wload(wd_v, KF, F - KF, slice(c * LANES, (c + 2) * LANES)),
                                preferred_element_type=F32)
            yield
            for cc in range(2):
                y = acc[:, cc * LANES:(cc + 1) * LANES]
                for k0 in range(0, KF, D):
                    y = y + jnp.dot(gated(act[:, k0:k0 + D]),
                                    wload(wd_v, k0, D, slice((c + cc) * LANES, (c + cc + 1) * LANES)),
                                    preferred_element_type=F32)
                    yield
                ys.append(y)
        res["y"] = jnp.concatenate(ys, axis=1)

    def side_units():
        yield from range(NPRE)
        yield from c_units()
        yield from range(NGAP)
        yield from f_units()

    side = side_units()

    def o_dot(lhs, rhs):
        p = pc.dot(lhs, rhs) if st["step"] < NPRE else jnp.dot(lhs, rhs, preferred_element_type=F32)
        next(side, None)
        st["step"] += 1
        return p

    def o_plain(r0, n):
        lhs = pltpu.bitcast(pqn_v[r0 // 2:(r0 + n) // 2, :], BF16)
        parts = []
        for c0 in range(0, NC, 2):
            acc = x_v[DEF + L0 + r0:DEF + L0 + r0 + n, c0 * LANES:(c0 + 2) * LANES].astype(F32)
            for k0 in range(0, D, 2 * LANES):
                acc = acc + o_dot(lhs[:, k0:k0 + 2 * LANES], wload(mp_v, k0, 2 * LANES, slice(c0 * LANES, (c0 + 2) * LANES)))
            parts.append(acc)
        return jnp.concatenate(parts, axis=1)

    toks = []
    r0 = 0
    pc.add(post_jobs(OCL[0][0], *OCL[1]), pc.t + 200, pc.t + 1000, QP_DELAY)
    for ci, (n, plain) in enumerate(OCL):
        h = o_plain(r0, n) if plain else o_part(o_dot, x_v, DEF + L0, r0, n)
        last = r0 + n == RL
        units = ln2_jobs(h, ln2_v, out_v, DEF + L0 + r0, -DEF, None, st, fast=last)
        posts = post_jobs(r0 + n + OCL[ci + 1][0], *OCL[ci + 2]) if ci + 2 < len(OCL) else []
        for k, job in enumerate(units):
            toks.append(job(toks[-LAG_L] if len(toks) >= LAG_L and not last else None))
            if posts:
                posts.pop(0)(toks[-1])
        if GLAG[ci] is not None:
            st["pend"].append((st["step"] + GLAG[ci],
                               pltpu.bitcast(jnp.broadcast_to(st["top1"], (8, LANES)), U32) & zero_u))
        r0 += n
        if last or r0 in OUT_AT:
            out_copy(L0 + st["sent"], r0 - st["sent"], 2 if last else 1).start()
            if not last:
                st["sent"] = r0
    for _ in side:
        st["step"] += 1

    keyv = best2(st["top1"], st["top2"])
    idx = [jnp.clip(key_row(kk[0, 0]), 0, S - 1) for kk in keyv]
    grp = [pl.multiple_of((ii >> 3) << 3, 8) for ii in idx]
    vgrp = [pl.multiple_of(gg + DEF, 8) for gg in grp]
    y = res["y"]
    ids_lo, ids_hi = res["ids"]
    hits = None
    yrows = []
    for c in range(2):
        m_lo = ids_lo == key_row(keyv[c])
        m_hi = ids_hi == key_row(keyv[c])
        yrows.append(subsum(jnp.where(wide(m_lo), y[0:8, :], 0.0) + jnp.where(wide(m_hi), y[8:16, :], 0.0)))
        hit = submax(jnp.where(m_lo | m_hi, 1, 0))
        hits = hit if hits is None else hits + hit
    hit_all = hits[0, 0] == 2

    tail0 = L0 + st["sent"]
    tail_copy = out_copy(tail0, S - tail0, 2)
    in_tail = jnp.maximum(grp[0], grp[1]) >= tail0
    two_groups = grp[1] != grp[0]

    def fix_copy(c):
        return out_copy(grp[c], 8, 3 + c)

    def finish(ysel):
        for c in range(2):
            hi = keyv[c] & jnp.int32(-65536)
            score = pltpu.bitcast(hi ^ ((hi >> 31) & 0x7FFF0000), F32)
            sel = (key_row(keyv[c]) & 7) == sub8
            upd = jnp.where(wide(sel), ysel[c] * wide(jax.nn.sigmoid(score)), 0.0)
            out_v[pl.ds(vgrp[c], 8), :] = (out_v[pl.ds(vgrp[c], 8), :].astype(F32) + upd).astype(BF16)
        fix_copy(0).start()

        @pl.when(two_groups)
        def _():
            fix_copy(1).start()

    out_copy(0, L0, 0).wait()
    out_copy(L0, tail0 - L0, 1).wait()

    @pl.when(in_tail)
    def _():
        tail_copy.wait()

    @pl.when(hit_all)
    def _():
        finish(yrows)

    @pl.when(jnp.logical_not(hit_all))
    def _():
        xsel = jnp.concatenate([ln2_v[pl.ds(vgrp[c], 8), :] for c in range(2)], axis=0)

        def ffn_tile(j, acc):
            cs = pl.ds(pl.multiple_of(j * LANES, LANES), LANES)
            g = jnp.dot(xsel, wload(wg_v, 0, D, cs), preferred_element_type=F32)
            u = jnp.dot(xsel, wload(wu_v, 0, D, cs), preferred_element_type=F32)
            a = (g * jax.nn.sigmoid(g) * u).astype(BF16)
            return acc + jnp.dot(a, wd_v[cs, 0:D], preferred_element_type=F32)

        yf = lax.fori_loop(0, F // LANES, ffn_tile, jnp.zeros((16, D), F32))
        finish([yf[0:8, :], yf[8:16, :]])

    @pl.when(jnp.logical_not(in_tail))
    def _():
        tail_copy.wait()

    fix_copy(0).wait()

    @pl.when(two_groups)
    def _():
        fix_copy(1).wait()


@jax.jit
def pallas_sequential_preLN__linear_attn_block__moe_arch_mod__prompt_kernel(
    A_x: jax.Array,
    A_wqkv: jax.Array,
    A_wo: jax.Array,
    B_x: jax.Array,
    B_w_r: jax.Array,
    B_w_gate: jax.Array,
    B_w_up: jax.Array,
    B_w_down: jax.Array,
):
    del B_x
    x = A_x.reshape(S, D)
    wr = B_w_r.reshape(NC, LANES)
    any_spec = pl.BlockSpec(memory_space=pl.ANY)
    out = pl.pallas_call(
        _kernel,
        out_shape=jax.ShapeDtypeStruct((S, D), BF16),
        in_specs=[any_spec] * 7,
        out_specs=any_spec,
        scratch_shapes=[
            pltpu.VMEM((S + DEF, D), BF16),
            pltpu.VMEM((D, D + LANES), BF16),
            pltpu.VMEM((D, D), BF16),
            pltpu.VMEM((2, D, D + LANES), BF16),
            pltpu.VMEM((NC, LANES), BF16),
            pltpu.VMEM((2, D, F), BF16),
            pltpu.VMEM((F, D + LANES), BF16),
            pltpu.VMEM((P0 // 2, D), U32),
            pltpu.VMEM((7 ** LA, S // NA // 2, DA), U32),
            pltpu.VMEM((7 ** LA, DA // 2, DA), U32),
            pltpu.VMEM((D // 2, P0), U32),
            pltpu.VMEM((DA // 2, 7 ** LA * MA), U32),
            pltpu.VMEM((D, LANES), F32),
            pltpu.VMEM((D, LANES), F32),
            pltpu.VMEM((RL, LANES), F32),
            pltpu.VMEM((D, D), F32),
            pltpu.VMEM((7, HD, HD), F32),
            pltpu.VMEM((D // 2, D), U32),
            pltpu.VMEM((7 ** LA, DA // 2, DA), U32),
            pltpu.VMEM((D // 2, D), U32),
            pltpu.VMEM((7 ** LO, DO // 2, DO), U32),
            pltpu.VMEM((max(TB2, RL), D + 2 * LANES), F32),
            pltpu.VMEM((RL // 2, D), U32),
            pltpu.VMEM((7 ** LO, max(TB2, RL) // NO // 2, DO), U32),
            pltpu.VMEM((DEF, D), F32),
            pltpu.VMEM((2, S + DEF, D), BF16),
            pltpu.VMEM((TB, D), F32),
            pltpu.VMEM((8, LANES), U32),
            pltpu.SemaphoreType.DMA((NSEM,)),
        ],
        compiler_params=pltpu.CompilerParams(vmem_limit_bytes=110 * 1024 * 1024, disable_bounds_checks=True,
                                             disable_semaphore_checks=True),
    )(x, A_wqkv, A_wo, wr, B_w_gate, B_w_up, B_w_down)
    return out.reshape(1, S, D)
```
